```python
import jax
import jax.numpy as jnp

def _softmax(x, axis=-1):
    return jax.nn.softmax(x, axis=axis)

def _gelu(x):
    return jax.nn.gelu(x, approximate=True)

def _silu(x):
    return jax.nn.silu(x)

def _sigmoid(x):
    return jax.nn.sigmoid(x)

def _layernorm(x, axis=-1, eps=1e-05):
    m = jnp.mean(x, axis=axis, keepdims=True)
    v = jnp.var(x, axis=axis, keepdims=True)
    return (x - m) / jnp.sqrt(v + eps)

def _scatter_add(tgt, idx, src, axis=0):
    return tgt.at[idx].add(src)

def _segment_sum(src, seg, n):
    return jax.ops.segment_sum(src, seg, n)

class _Rng:

    def __init__(self, key):
        self._k = key

    def _next(self):
        self._k, sub = jax.random.split(self._k)
        return sub

    def normal(self, shape):
        return jax.random.normal(self._next(), shape, dtype=jnp.bfloat16)

    def randint(self, lo, hi, shape):
        return jax.random.randint(self._next(), shape, lo, hi, dtype=jnp.int32)

    def uniform(self, shape, lo=0.0, hi=1.0):
        return jax.random.uniform(self._next(), shape, jnp.bfloat16, lo, hi)

    def permutation(self, n):
        return jax.random.permutation(self._next(), n)
kernel_name = 'interleave_layers__memory_aug_recurrent_mem_tr__ssm_conv_h3__prompt'

def setup_inputs():
    _rng = _Rng(jax.random.key(int.from_bytes(__import__("os").urandom(4), "little")))
    _w = lambda a: (lambda t: t.astype(jnp.bfloat16) if jnp.issubdtype(t.dtype, jnp.floating) else t)(jnp.asarray(a))

    def _A_setup():
        B, S, Dm = (1, 2048, 640)
        H, Dh = (32, 128)
        M, seg = (8, 32)
        seg = min(seg, S)
        S = S // seg * seg
        return {'x': _w((lambda *s: _rng.normal(s) * 0.05)(B, S, Dm)), 'mem0': _w((lambda *s: _rng.normal(s) * 0.05)(B, M, Dm)), 'Wq': _w((lambda *s: _rng.normal(s) * 0.05)(Dm, H, Dh) * Dm ** (-0.5)), 'Wk': _w((lambda *s: _rng.normal(s) * 0.05)(Dm, H, Dh) * Dm ** (-0.5)), 'Wv': _w((lambda *s: _rng.normal(s) * 0.05)(Dm, H, Dh) * Dm ** (-0.5)), 'Wo': _w((lambda *s: _rng.normal(s) * 0.05)(H, Dh, Dm) * (H * Dh) ** (-0.5)), 'seg_len': seg}
    _A_in = _A_setup()

    def _B_setup():
        B, S, D = (1, 2048, 640)
        ks = 4
        return {'q': _w((lambda *s: _rng.normal(s) * 0.05)(B, S, D)), 'k': _w((lambda *s: _rng.normal(s) * 0.05)(B, S, D)), 'v': _w((lambda *s: _rng.normal(s) * 0.05)(B, S, D)), 'shift_k': _w((lambda *s: _rng.normal(s) * 0.05)(D, ks) * 0.5), 'ssm_k': _w((lambda *s: _rng.normal(s) * 0.05)(D, S) * (1.0 / S ** 0.5)), 'ssm_D': _w((lambda *s: _rng.normal(s) * 0.05)(D))}
    _B_in = _B_setup()
    return {'A_x': _A_in['x'], 'A_mem0': _A_in['mem0'], 'A_Wq': _A_in['Wq'], 'A_Wk': _A_in['Wk'], 'A_Wv': _A_in['Wv'], 'A_Wo': _A_in['Wo'], 'A_seg_len': _A_in['seg_len'], 'B_q': _B_in['q'], 'B_k': _B_in['k'], 'B_v': _B_in['v'], 'B_shift_k': _B_in['shift_k'], 'B_ssm_k': _B_in['ssm_k'], 'B_ssm_D': _B_in['ssm_D']}

def reference(A_x, A_mem0, A_Wq, A_Wk, A_Wv, A_Wo, A_seg_len, B_q, B_k, B_v, B_shift_k, B_ssm_k, B_ssm_D):

    def _A_ref(x, mem0, Wq, Wk, Wv, Wo, seg_len):
        B, S, Dm = x.shape
        H, Dh = (Wq.shape[1], Wq.shape[2])
        M = mem0.shape[1]
        scale = Dh ** (-0.5)
        n_seg = S // seg_len
        L = M + seg_len
        idx = jnp.arange(L)
        mask = (idx[:, None] < M) | (idx[:, None] >= idx[None, :])
        mem = mem0
        outs = []
        for s in range(n_seg):
            xs = x[:, s * seg_len:(s + 1) * seg_len, :].copy()
            h = jnp.concatenate([mem, xs], axis=1)
            q = jnp.einsum('btd,dhe->bhte', h, Wq)
            k = jnp.einsum('btd,dhe->bhte', h, Wk)
            v = jnp.einsum('btd,dhe->bhte', h, Wv)
            scores = jnp.einsum('bhqe,bhke->bhqk', q, k) * scale
            scores = jnp.where(mask[None, None], scores, -1000000000.0)
            p = _softmax(scores, axis=-1)
            o = jnp.einsum('bhqk,bhke->bhqe', p, v)
            o = jnp.einsum('bhte,hed->btd', o, Wo)
            mem = o[:, :M, :].copy()
            outs.append(o[:, M:, :])
        return jnp.concatenate(outs, axis=1)

    def _B_ref(q, k, v, shift_k, ssm_k, ssm_D):
        B, S, D = q.shape
        ks = shift_k.shape[-1]
        k_pad = jnp.pad(k, ((0, 0), (ks - 1, 0), (0, 0)))
        k_shift = jnp.zeros_like(k)
        for t in range(ks):
            k_shift = k_shift + k_pad[:, t:t + S, :] * shift_k[:, ks - 1 - t][None, None, :]
        kv = k_shift * v
        L = 2 * S
        kv_pad = jnp.pad(kv, ((0, 0), (0, S), (0, 0)))
        kf_pad = jnp.pad(ssm_k, ((0, 0), (0, S)))
        kv_f = (lambda x, axes=(-2, -1): jnp.fft.rfft2(x.astype(jnp.float32), axes=axes))(kv_pad[:, None, :, :], axes=(1, 2))
        kf_f = (lambda x, axes=(-2, -1): jnp.fft.rfft2(x.astype(jnp.float32), axes=axes))(kf_pad[:, None, :], axes=(1, 2))
        kf_f = (lambda x, *d: x.transpose(*d))(kf_f, 1, 2, 0)
        y_f = kv_f * kf_f[None, :, :, :]
        y = (lambda x, s, axes=(-2, -1): jnp.fft.irfft2(x, s=s, axes=axes).astype(jnp.bfloat16))(y_f, (1, L), axes=(1, 2))[:, 0, :S, :]
        y = y + kv * ssm_D[None, None, :]
        return q * y
    x = A_x
    x = x + _A_ref(_layernorm(x, axis=-1), A_mem0, A_Wq, A_Wk, A_Wv, A_Wo, A_seg_len)
    x = x + _B_ref(_layernorm(x, axis=-1), B_k, B_v, B_shift_k, B_ssm_k, B_ssm_D)
    x = x + _A_ref(_layernorm(x, axis=-1), A_mem0, A_Wq, A_Wk, A_Wv, A_Wo, A_seg_len)
    x = x + _B_ref(_layernorm(x, axis=-1), B_k, B_v, B_shift_k, B_ssm_k, B_ssm_D)
    return x
```

```python
import functools

import numpy as np
import jax
import jax.numpy as jnp
import jax.experimental.pallas as pl
import jax.experimental.pallas.tpu as pltpu

F32 = jnp.float32
BF16 = jnp.bfloat16
U32 = jnp.uint32

CB = 128


def _dft_constants():
    f = np.arange(CB, dtype=np.float64)
    n = np.arange(CB, dtype=np.float64)
    w = np.pi * (2.0 * f + 1.0) / (2 * CB)
    ang = w[:, None] * n[None, :]
    fwd = np.concatenate([np.cos(ang), -np.sin(ang)], axis=0)
    inv = np.concatenate([np.cos(ang).T, -np.sin(ang).T], axis=1) / CB
    return fwd.astype(np.float32), inv.astype(np.float32)


def _ln(x, eps=1e-5):
    d = x.shape[-1]
    m = jnp.sum(x, axis=-1, keepdims=True) * (1.0 / d)
    xc = x - m
    v = jnp.sum(xc * xc, axis=-1, keepdims=True) * (1.0 / d)
    return xc * jax.lax.rsqrt(v + eps)


def _kernel(x_ref, mem0_ref, wq_ref, wk_ref, wv_ref, wo_ref, k_ref, v_ref,
            sh_ref, sk_ref, sd_ref, fwd_ref, inv_ref, o_ref,
            w_sc, h_sc, o_sc, op_sc, x2_sc, y_sc, u_sc, uf_sc, kf_sc,
            *, S, DM, H, DH, M, SEG):
    NSEG = S // SEG
    R = 2 * (M + SEG)
    NB = S // CB

    def relayout(b, c):
        d0 = pl.multiple_of(b * 16, 16)
        r0 = pl.multiple_of(b * 8, 8)
        for mi, wr in enumerate((wq_ref, wk_ref, wv_ref)):
            xw = pltpu.bitcast(wr[pl.ds(d0, 16)], U32).reshape(8, 2, H // 2, DH)
            a = xw[:, 0]
            bb = xw[:, 1]
            lo = jnp.swapaxes((a & U32(0xFFFF)) | (bb << 16), 0, 1)
            hi = jnp.swapaxes((a >> 16) | (bb & U32(0xFFFF0000)), 0, 1)
            for j in range(H // 2):
                w_sc[2 * j, pl.ds(r0, 8), mi * DH:(mi + 1) * DH] = lo[j]
                w_sc[2 * j + 1, pl.ds(r0, 8), mi * DH:(mi + 1) * DH] = hi[j]
        return c
    jax.lax.fori_loop(0, DM // 16, relayout, 0)

    sh = sh_ref[...].astype(F32)
    KS = sh.shape[0]
    sd = sd_ref[...].astype(F32)
    fwd = fwd_ref[...]
    inv = inv_ref[...]
    rowi = jax.lax.broadcasted_iota(jnp.int32, (CB + 16, DM), 0)
    sgn = jnp.where(jax.lax.broadcasted_iota(jnp.int32, (CB, DM), 0) % 2 == 0, 1.0, -1.0).astype(F32)

    def conv_fwd(c, carry):
        t0 = pl.multiple_of(c * CB, CB)
        tp = pl.multiple_of(jnp.maximum(t0 - 16, 0), 16)
        prev = k_ref[pl.ds(tp, 16), :].astype(F32)
        prev = jnp.where(c > 0, prev, 0.0)
        kk = jnp.concatenate([prev, k_ref[pl.ds(t0, CB), :].astype(F32)], axis=0)
        ks = kk[16:] * sh[0:1]
        for j in range(1, KS):
            ks = ks + pltpu.roll(kk, j, 0)[16:] * sh[j:j + 1]
        u = (ks * v_ref[pl.ds(t0, CB), :].astype(F32)).astype(BF16)
        u_sc[pl.ds(t0, CB), :] = u
        uf_sc[c] = jnp.dot(fwd, u, preferred_element_type=F32)
        kb = sk_ref[:, pl.ds(t0, CB)]
        kf = jax.lax.dot_general(fwd, kb, (((1,), (1,)), ((), ())), preferred_element_type=F32)
        pr, pi = carry
        kr, ki = kf[:CB], kf[CB:]
        kf_sc[c, :CB] = kr - sgn * pi
        kf_sc[c, CB:] = ki + sgn * pr
        return kr, ki
    z = jnp.zeros((CB, DM), F32)
    jax.lax.fori_loop(0, NB, conv_fwd, (z, z))

    def conv_inv(c, carry):
        t0 = pl.multiple_of(c * CB, CB)
        parts_r = []
        parts_i = []
        for rb in range(CB // 8):
            def mac(j, acc):
                ar, ai = acc
                ur = uf_sc[j, rb * 8:rb * 8 + 8, :]
                ui = uf_sc[j, CB + rb * 8:CB + rb * 8 + 8, :]
                kr = kf_sc[c - j, rb * 8:rb * 8 + 8, :]
                ki = kf_sc[c - j, CB + rb * 8:CB + rb * 8 + 8, :]
                return ar + (ur * kr - ui * ki), ai + (ur * ki + ui * kr)
            z8 = jnp.zeros((8, DM), F32)
            ar, ai = jax.lax.fori_loop(0, c + 1, mac, (z8, z8))
            parts_r.append(ar)
            parts_i.append(ai)
        w = jnp.concatenate(parts_r + parts_i, axis=0).astype(BF16)
        yc = jnp.dot(inv, w, preferred_element_type=F32)
        y_sc[pl.ds(t0, CB), :] = yc + u_sc[pl.ds(t0, CB), :].astype(F32) * sd
        return carry
    jax.lax.fori_loop(0, NB, conv_inv, 0)

    qi = jax.lax.broadcasted_iota(jnp.int32, (R, R), 0)
    ki = jax.lax.broadcasted_iota(jnp.int32, (R, R), 1)

    def layer(i):
        return jnp.where(i < M, 0, jnp.where(i < 2 * M, 1, jnp.where(i < 2 * M + SEG, 0, 1)))
    same = layer(qi) == layer(ki)
    ok = same & ((qi < 2 * M) | (ki < 2 * M) | (qi >= ki))
    scale = DH ** -0.5
    fill = jnp.where(same, -1e9 / scale, -jnp.inf).astype(F32)
    cexp = scale * float(np.log2(np.e))

    mem0 = mem0_ref[...].astype(F32)
    h_sc[0:2 * M, :] = jnp.concatenate([mem0, mem0], axis=0).astype(BF16)
    h_sc[2 * M:2 * M + SEG, :] = _ln(x_ref[0:SEG, :].astype(F32)).astype(BF16)
    h_sc[2 * M + SEG:, :] = jnp.zeros((SEG, DM), BF16)
    op_sc[...] = jnp.zeros(op_sc.shape, F32)
    x2_sc[...] = jnp.zeros(x2_sc.shape, F32)

    def seg(i):
        i = jnp.clip(i, 0, NSEG - 1)
        return pl.ds(pl.multiple_of(i * SEG, SEG), SEG)

    def side(t):
        a1 = op_sc[0:SEG, :]
        a2 = op_sc[SEG:, :]
        x1 = x_ref[seg(t - 1), :].astype(F32) + a1
        x2 = x1 + _ln(x1) * y_sc[seg(t - 1), :]
        x3 = x2_sc[(t - 3) & 3] + a2
        x4 = x3 + _ln(x3) * y_sc[seg(t - 3), :]
        x2_sc[(t - 1) & 3] = x2
        o_ref[seg(t - 3), :] = x4.astype(o_ref.dtype)
        return _ln(x2).astype(BF16)

    D1, D2 = 1, 2

    def step(t, carry):
        h = h_sc[...]
        xn2 = side(t)
        xn1 = _ln(x_ref[seg(t + 1), :].astype(F32)).astype(BF16)
        qkvs = {}
        ps = {}
        for it in range(H + D1 + D2):
            g = it
            if g < H:
                qkvs[g] = jnp.dot(h, pltpu.bitcast(w_sc[g], BF16),
                                  preferred_element_type=F32).astype(BF16)
            g = it - D1
            if 0 <= g < H:
                q = qkvs[g][:, 0:DH]
                k = qkvs[g][:, DH:2 * DH]
                s = jax.lax.dot_general(q, k, (((1,), (1,)), ((), ())), preferred_element_type=F32)
                s = jnp.where(ok, s, fill)
                m = jnp.max(s, axis=-1, keepdims=True)
                p = jnp.exp2((s - m) * cexp)
                l = jnp.sum(p, axis=-1, keepdims=True)
                r = pl.reciprocal(l, approx=True)
                r = r * (2.0 - l * r)
                ps[g] = (p * r).astype(BF16)
            g = it - D1 - D2
            if 0 <= g < H:
                v = qkvs[g][:, 2 * DH:3 * DH]
                o = jnp.dot(ps[g], v, preferred_element_type=F32)
                o_sc[:, g * DH:(g + 1) * DH] = o.astype(BF16)
        out = jnp.dot(o_sc[...], wo_ref[...], preferred_element_type=F32)
        m2 = jnp.where(t < 2, mem0, out[M:2 * M])
        h_sc[0:2 * M, :] = jnp.concatenate([out[0:M], m2], axis=0).astype(BF16)
        h_sc[2 * M:2 * M + SEG, :] = xn1
        h_sc[2 * M + SEG:, :] = xn2
        op_sc[...] = out[2 * M:]
        return carry

    jax.lax.fori_loop(0, NSEG + 2, step, 0)
    side(NSEG + 2)


@functools.partial(jax.jit, static_argnames=("A_seg_len",))
def pallas_interleave_layers__memory_aug_recurrent_mem_tr__ssm_conv_h3__prompt_kernel(
    A_x, A_mem0, A_Wq, A_Wk, A_Wv, A_Wo, A_seg_len,
    B_q, B_k, B_v, B_shift_k, B_ssm_k, B_ssm_D,
):
    del B_q
    B, S, DM = A_x.shape
    assert B == 1
    H, DH = A_Wq.shape[1], A_Wq.shape[2]
    M = A_mem0.shape[1]
    SEG = int(A_seg_len)
    R = 2 * (M + SEG)
    NB = S // CB
    fwd, inv = _dft_constants()

    kern = functools.partial(_kernel, S=S, DM=DM, H=H, DH=DH, M=M, SEG=SEG)
    out = pl.pallas_call(
        kern,
        out_shape=jax.ShapeDtypeStruct((S, DM), A_x.dtype),
        scratch_shapes=[
            pltpu.VMEM((H, DM // 2, 3 * DH), U32),
            pltpu.VMEM((R, DM), BF16),
            pltpu.VMEM((R, H * DH), BF16),
            pltpu.VMEM((2 * SEG, DM), F32),
            pltpu.VMEM((4, SEG, DM), F32),
            pltpu.VMEM((S, DM), F32),
            pltpu.VMEM((S, DM), BF16),
            pltpu.VMEM((NB, 2 * CB, DM), F32),
            pltpu.VMEM((NB, 2 * CB, DM), F32),
        ],
        compiler_params=pltpu.CompilerParams(vmem_limit_bytes=120 * 1024 * 1024),
    )(
        A_x.reshape(S, DM), A_mem0.reshape(M, DM), A_Wq, A_Wk, A_Wv,
        A_Wo.reshape(H * DH, DM), B_k.reshape(S, DM), B_v.reshape(S, DM),
        B_shift_k.T, B_ssm_k, B_ssm_D.reshape(1, DM),
        jnp.asarray(fwd, BF16), jnp.asarray(inv, BF16),
    )
    return out.reshape(B, S, DM)
```

```python
import functools

import numpy as np
import jax
import jax.numpy as jnp
import jax.experimental.pallas as pl
import jax.experimental.pallas.tpu as pltpu

F32 = jnp.float32
BF16 = jnp.bfloat16
U32 = jnp.uint32

CB = 128
NQ = 4
KPAD = 16
PH = 8
NPRE = 4
D1, D2 = 1, 2


def _dft_constants():
    qb = CB // NQ
    n = np.arange(CB, dtype=np.float64)
    fwd = np.zeros((NQ, 2 * qb, CB))
    for q in range(NQ):
        f = q * qb + np.concatenate([np.arange(0, qb, 2), np.arange(1, qb, 2)])
        ang = (np.pi * (2.0 * f + 1.0) / (2 * CB))[:, None] * n[None, :]
        fwd[q, :qb] = np.cos(ang)
        fwd[q, qb:] = -np.sin(ang)
    inv = fwd.reshape(2 * CB, CB).T / CB
    return fwd.astype(np.float32), inv.reshape(NQ, CB // NQ, 2 * CB).astype(np.float32)


def _ln(x, eps=1e-5):
    d = x.shape[-1]
    m = jnp.sum(x, axis=-1, keepdims=True) * (1.0 / d)
    xc = x - m
    v = jnp.sum(xc * xc, axis=-1, keepdims=True) * (1.0 / d)
    return xc * jax.lax.rsqrt(v + eps)


def _dot(a, b):
    return jnp.dot(a, b, preferred_element_type=F32)


def _dot_nt(a, b):
    return jax.lax.dot_general(a, b, (((1,), (1,)), ((), ())), preferred_element_type=F32)


def _in_order(actions):
    def body(i, c):
        for j, act in enumerate(actions):
            pl.when(i == j)(act)
        return c
    jax.lax.fori_loop(0, len(actions), body, 0)


def _kernel(x_hbm, mem0_hbm, wq_hbm, wk_hbm, wv_hbm, wo_hbm, k_hbm, v_hbm,
            sh_hbm, sk_hbm, sd_hbm, fwd_hbm, inv_hbm, o_hbm,
            mem0_ref, sh_ref, sd_ref, fwd_ref, inv_ref,
            x_sc, k_sc, v_sc, sk_sc, st_sc, wo_sc, out_sc,
            w_sc, hp_sc, pre_sc, h_sc, o_sc, op_sc, x2_sc, y_sc, u_sc, sp_sc, kr_sc, wf_sc,
            sem_s, sem_in, sem_w, sem_out,
            *, S, DM, H, DH, M, SEG):
    NSEG = S // SEG
    M2 = 2 * M
    R = M2 + 2 * SEG
    RH = M2 + SEG
    NB = S // CB
    QB = CB // NQ
    HB = QB // 2
    NT = DM // 128
    assert QB == SEG and NSEG % PH == 0 and 2 <= NPRE <= PH
    NPH = NSEG // PH
    HG = H // 2

    small = [pltpu.make_async_copy(s, d, sem_s.at[i]) for i, (s, d) in enumerate([
        (mem0_hbm, mem0_ref), (sh_hbm, sh_ref), (sd_hbm, sd_ref), (fwd_hbm, fwd_ref), (inv_hbm, inv_ref)])]

    xb = (0, NPRE * SEG, 2 * PH * SEG, S)
    kb = (0, (2 * NQ + 2) * SEG, 2 * PH * SEG, S)
    sb = (0, 2 * CB, 2 * PH * SEG, S)

    def in_copies(part):
        def rng(b):
            return pl.ds(b[part], b[part + 1] - b[part])
        return [
            pltpu.make_async_copy(x_hbm.at[rng(xb)], x_sc.at[rng(xb)], sem_in.at[part * 4]),
            pltpu.make_async_copy(k_hbm.at[rng(kb)],
                                  k_sc.at[pl.ds(KPAD + kb[part], kb[part + 1] - kb[part])],
                                  sem_in.at[part * 4 + 1]),
            pltpu.make_async_copy(v_hbm.at[rng(kb)], v_sc.at[rng(kb)], sem_in.at[part * 4 + 2]),
            pltpu.make_async_copy(sk_hbm.at[:, rng(sb)], sk_sc.at[:, rng(sb)], sem_in.at[part * 4 + 3]),
        ]

    def w_copy(ci):
        src = (wq_hbm, wk_hbm, wv_hbm)[ci % 3]
        return pltpu.make_async_copy(src.at[:, pl.ds((ci // 3) * HG, HG), :], st_sc.at[ci], sem_w.at[ci])

    wo_copy = pltpu.make_async_copy(wo_hbm, wo_sc, sem_w.at[6])

    def out_copy(i):
        rows = pl.ds(pl.multiple_of(i * PH * SEG, PH * SEG), PH * SEG)
        return pltpu.make_async_copy(out_sc.at[rows], o_hbm.at[rows], sem_out.at[i])

    def start_all(cps):
        def act():
            for cp in cps:
                cp.start()
        return act

    _in_order([start_all(small + in_copies(0))]
              + [start_all([w_copy(ci)]) for ci in range(6)]
              + [start_all([wo_copy]), start_all(in_copies(1)), start_all(in_copies(2))])

    k_sc[0:KPAD, :] = jnp.zeros((KPAD, DM), BF16)
    sp_sc[NB + 1] = jnp.zeros(sp_sc.shape[1:], F32)
    op_sc[...] = jnp.zeros(op_sc.shape, F32)
    x2_sc[...] = jnp.zeros(x2_sc.shape, F32)
    y_sc[...] = jnp.zeros(y_sc.shape, F32)
    h_sc[...] = jnp.zeros(h_sc.shape, BF16)
    for cp in small + in_copies(0):
        cp.wait()

    sh = sh_ref[...].astype(F32)
    KS = sh.shape[0]
    sd = sd_ref[...].astype(F32)

    def seg(i):
        i = jnp.clip(i, 0, NSEG - 1)
        return pl.ds(pl.multiple_of(i * SEG, SEG), SEG)

    def conv_u(s):
        s = jnp.clip(s, 0, NSEG - 1)
        r0 = pl.multiple_of(s * SEG, SEG)
        kk = k_sc[pl.ds(r0, KPAD + SEG), :].astype(F32)
        ks = kk[KPAD:] * sh[0:1]
        for j in range(1, KS):
            ks = ks + pltpu.roll(kk, j, 0)[KPAD:] * sh[j:j + 1]
        u_sc[pl.ds(r0, SEG), :] = (ks * v_sc[pl.ds(r0, SEG), :].astype(F32)).astype(BF16)

    def conv_fwd(c, q):
        cc = jnp.minimum(c, NB - 1)
        t0 = pl.multiple_of(cc * CB, CB)
        f = fwd_ref[q]
        uf = _dot(f, u_sc[pl.ds(t0, CB), :])
        kf = _dot_nt(f, sk_sc[:, pl.ds(t0, CB)])
        return uf, kf

    def put_spec(cs, q, which, val):
        for rb in range(QB // 8):
            for n in range(NT):
                ln = slice(n * 128, (n + 1) * 128)
                sp_sc[cs, q, rb, n, which] = val[rb * 8:rb * 8 + 8, ln]
                sp_sc[cs, q, rb, n, which + 1] = val[QB + rb * 8:QB + rb * 8 + 8, ln]

    def conv_spec(c, q):
        uf, kf = conv_fwd(c, q)
        cs = jnp.minimum(c, NB)
        put_spec(cs, q, 0, uf)
        pk = kr_sc[q]
        kr_sc[q] = kf
        kp = jnp.concatenate([
            kf[0:HB] - pk[QB:QB + HB],
            kf[HB:QB] + pk[QB + HB:],
            kf[QB:QB + HB] + pk[0:HB],
            kf[QB + HB:] - pk[HB:QB]], axis=0)
        put_spec(cs, q, 2, kp)

    MAC_PIECES = [(rb, n) for rb in range(QB // 16) for n in range(NT)]

    def conv_mac(c, q, piece, nterms):
        rb2, n = piece
        cs = jnp.minimum(c, NB)
        acc = []
        for rb in (2 * rb2, 2 * rb2 + 1):
            ar = None
            ai = None
            for j in range(nterms):
                uj = jnp.minimum(j, cs)
                kj = jnp.where(cs - j >= 0, cs - j, NB + 1)
                ur = sp_sc[uj, q, rb, n, 0]
                um = sp_sc[uj, q, rb, n, 1]
                kr = sp_sc[kj, q, rb, n, 2]
                km = sp_sc[kj, q, rb, n, 3]
                tr = ur * kr - um * km
                ti = ur * km + um * kr
                ar = tr if ar is None else ar + tr
                ai = ti if ai is None else ai + ti
            acc.append((ar, ai))
        ln = slice(n * 128, (n + 1) * 128)
        wf_sc[c & 1, q, rb2 * 16:rb2 * 16 + 16, ln] = jnp.concatenate(
            [acc[0][0], acc[1][0]], axis=0).astype(BF16)
        wf_sc[c & 1, q, QB + rb2 * 16:QB + rb2 * 16 + 16, ln] = jnp.concatenate(
            [acc[0][1], acc[1][1]], axis=0).astype(BF16)

    def conv_inv(s):
        w = wf_sc[(s // NQ) & 1].reshape(2 * CB, DM)
        yc = _dot(inv_ref[s % NQ], w)
        y_sc[s & 3] = yc + u_sc[seg(s), :].astype(F32) * sd

    scale = DH ** -0.5
    cexp = scale * float(np.log2(np.e))

    def make_mask(n, x_layers):
        qi = jax.lax.broadcasted_iota(jnp.int32, (n, n), 0)
        ki = jax.lax.broadcasted_iota(jnp.int32, (n, n), 1)

        def layer(i):
            xl = jnp.where(i < M2 + SEG, x_layers[0], x_layers[-1])
            return jnp.where(i < M, 0, jnp.where(i < M2, 1, xl))
        same = layer(qi) == layer(ki)
        ok = same & ((qi < M2) | (ki < M2) | (qi >= ki))
        fill = jnp.where(same, -1e9 / scale, -jnp.inf).astype(F32)
        return ok, fill

    def probs(qkv, mask):
        ok, fill = mask
        s = _dot_nt(qkv[:, 0:DH], qkv[:, DH:2 * DH])
        s = jnp.where(ok, s, fill)
        m = jnp.max(s, axis=-1, keepdims=True)
        p = jnp.exp2((s - m) * cexp)
        l = jnp.sum(p, axis=-1, keepdims=True)
        r = pl.reciprocal(l, approx=True)
        r = r * (2.0 - l * r)
        return (p * r).astype(BF16)

    def w_head(g):
        return pltpu.bitcast(w_sc[g], BF16)

    def pre_rows(g, w0, n):
        return pltpu.bitcast(pre_sc[g, pl.ds(w0, n // 2), :], BF16)

    def attend(proj, n, mask, hook=None):
        HA = H - D1 - D2 - 1
        qkvs = {}
        ps = {}
        outs = {}
        for it in range(H + D1 + D2):
            if it < H:
                qkvs[it] = proj(it)
            g = it - D1
            if 0 <= g < H:
                ps[g] = probs(qkvs[g], mask)
            g = it - D1 - D2
            if 0 <= g < H:
                o = _dot(ps.pop(g), qkvs.pop(g)[:, 2 * DH:3 * DH])
                o_sc[0:n, g * DH:(g + 1) * DH] = o.astype(BF16)
            if hook is not None:
                hook(it)
            j = it - (H - 1)
            if 0 <= j < D1 + D2:
                outs[j] = _dot(o_sc[0:n, :HA * DH], wo_sc[:HA * DH, j * 128:(j + 1) * 128])
        for j in range(D1 + D2, NT):
            outs[j] = _dot(o_sc[0:n, :], wo_sc[:, j * 128:(j + 1) * 128])
        for j in range(D1 + D2):
            outs[j] = _dot(o_sc[0:n, HA * DH:], wo_sc[HA * DH:, j * 128:(j + 1) * 128]) + outs[j]
        return jnp.concatenate([outs[j] for j in range(NT)], axis=1)

    def side1(t):
        x1 = x_sc[seg(t - 1), :].astype(F32) + op_sc[0:SEG, :]
        x2 = x1 + _ln(x1) * y_sc[(t - 1) & 3]
        x2_sc[(t - 1) & 3] = x2
        return _ln(x2).astype(BF16)

    def side2(t):
        x3 = x2_sc[(t - 3) & 3] + op_sc[SEG:, :]
        x4 = x3 + _ln(x3) * y_sc[(t - 3) & 3]
        out_sc[seg(t - 3), :] = x4.astype(out_sc.dtype)

    def mac_hook(c, q, nterms):
        def hook(it):
            if it % 3 == 2 and it // 3 < len(MAC_PIECES):
                conv_mac(c, q, MAC_PIECES[it // 3], nterms)
        return hook

    def pro_u(s, c):
        conv_u(s)
        return c
    jax.lax.fori_loop(0, 2 * NQ + 1, pro_u, 0)

    def pro_c(q, c):
        uf, kf = conv_fwd(0, q)
        put_spec(0, q, 0, uf)
        put_spec(0, q, 2, kf)
        kr_sc[q] = kf
        ur, um, kr, km = uf[:QB], uf[QB:], kf[:QB], kf[QB:]
        wf_sc[0, q, :QB] = (ur * kr - um * km).astype(BF16)
        wf_sc[0, q, QB:] = (ur * km + um * kr).astype(BF16)
        return c
    jax.lax.fori_loop(0, NQ, pro_c, 0)
    conv_spec(1, 0)
    for piece in MAC_PIECES:
        conv_mac(1, 0, piece, 2)
    conv_inv(0)

    mem0 = mem0_ref[...].astype(F32)
    hp_sc[0:M2, :] = jnp.concatenate([mem0, mem0], axis=0).astype(BF16)

    def pro_h(s, c):
        hp_sc[pl.ds(pl.multiple_of(M2 + s * SEG, 16), SEG), :] = _ln(x_sc[seg(s), :].astype(F32)).astype(BF16)
        return c
    jax.lax.fori_loop(0, NPRE, pro_h, 0)

    mask1 = make_mask(RH, (0,))

    def chunk(ci, carry):
        g0 = (ci // 3) * HG
        cols = pl.ds(pl.multiple_of((ci % 3) * DH, DH), DH)
        with jax.named_scope("wait_w"):
            pltpu.make_async_copy(wq_hbm.at[:, pl.ds(0, HG), :], st_sc.at[ci], sem_w.at[ci]).wait()

        def relayout(b, c):
            d0 = pl.multiple_of(b * 16, 16)
            r0 = pl.multiple_of(b * 8, 8)
            xw = pltpu.bitcast(st_sc[ci, pl.ds(d0, 16)], U32).reshape(8, 2, HG // 2, DH)
            a = xw[:, 0]
            bb = xw[:, 1]
            lo = jnp.swapaxes((a & U32(0xFFFF)) | (bb << 16), 0, 1)
            hi = jnp.swapaxes((a >> 16) | (bb & U32(0xFFFF0000)), 0, 1)
            for j in range(HG // 2):
                w_sc[g0 + 2 * j, pl.ds(r0, 8), cols] = lo[j]
                w_sc[g0 + 2 * j + 1, pl.ds(r0, 8), cols] = hi[j]
            return c
        with jax.named_scope("relayout"):
            jax.lax.fori_loop(0, DM // 16, relayout, 0, unroll=2)

        with jax.named_scope("preproj"):
            hp = hp_sc[...]
            for j in range(HG):
                res = _dot(hp, pltpu.bitcast(w_sc[g0 + j, :, cols], BF16)).astype(BF16)
                pre_sc[g0 + j, :, cols] = pltpu.bitcast(res, U32)

        @pl.when(ci % 3 == 2)
        def _():
            ps = {}
            for it in range(HG + 2):
                if it < HG:
                    ps[it] = probs(pre_rows(g0 + it, 0, RH), mask1)
                j = it - 2
                if j >= 0:
                    o = _dot(ps.pop(j), pre_rows(g0 + j, 0, RH)[:, 2 * DH:])
                    o_sc[0:RH, pl.ds(pl.multiple_of((g0 + j) * DH, DH), DH)] = o.astype(BF16)
        return carry
    jax.lax.fori_loop(0, 6, chunk, 0)

    with jax.named_scope("wait_wo"):
        wo_copy.wait()
    out = _dot(o_sc[0:RH, :], wo_sc[...])
    h_sc[0:M2, :] = jnp.concatenate([out[0:M], mem0], axis=0).astype(BF16)
    op_sc[0:SEG, :] = out[M2:]

    with jax.named_scope("step1"):
        hm = h_sc[0:M2, :]
        conv_spec(1, 1)
        xn2 = side1(1)
        out = attend(lambda g: jnp.concatenate(
            [_dot(hm, w_head(g)).astype(BF16), pre_rows(g, M + SEG // 2, SEG)], axis=0),
            RH, mask1, mac_hook(1, 1, 2))
        conv_inv(1)
        conv_u(1 + 2 * NQ)
        h_sc[0:M2, :] = jnp.concatenate([out[0:M], mem0], axis=0).astype(BF16)
        h_sc[RH:, :] = xn2
        op_sc[0:SEG, :] = out[M2:]

    for cp in in_copies(1):
        cp.wait()

    mask12 = make_mask(R, (0, 1))

    def step(t, pre):
        c = t // NQ + 1
        q = t % NQ
        if pre:
            h = jnp.concatenate([h_sc[0:M2, :], h_sc[RH:, :]], axis=0)

            def proj(g):
                r = _dot(h, w_head(g)).astype(BF16)
                x1 = pre_rows(g, pl.multiple_of(M + t * (SEG // 2), 8), SEG)
                return jnp.concatenate([r[0:M2], x1, r[M2:]], axis=0)
            nterms = (NPRE - 1) // NQ + 2
        else:
            h = h_sc[...]

            def proj(g):
                return _dot(h, w_head(g)).astype(BF16)
            nterms = NB
        conv_spec(c, q)
        xn2 = side1(t)
        side2(t)
        xn1 = _ln(x_sc[seg(t + 1), :].astype(F32)).astype(BF16)
        out = attend(proj, R, mask12, mac_hook(c, q, nterms))
        conv_inv(t)
        conv_u(t + 2 * NQ)
        h_sc[0:M2, :] = out[0:M2].astype(BF16)
        h_sc[M2:RH, :] = xn1
        h_sc[RH:, :] = xn2
        op_sc[...] = out[M2:]

    def step_pre(t, carry):
        step(t, True)
        return carry

    def step_full(t, carry):
        step(t, False)
        return carry

    with jax.named_scope("steps_pre"):
        jax.lax.fori_loop(2, NPRE, step_pre, 0)

    def phase(p, carry):
        @pl.when(p == 1)
        def _():
            for cp in in_copies(2):
                cp.wait()

        @pl.when(p >= 2)
        def _():
            out_copy(p - 2).start()

        with jax.named_scope("steps"):
            jax.lax.fori_loop(jnp.maximum(p * PH, NPRE), p * PH + PH, step_full, 0)
        return carry

    jax.lax.fori_loop(0, NPH, phase, 0)
    out_copy(NPH - 2).start()

    mask2 = make_mask(RH, (1,))

    def step_l2(t, carry):
        h = jnp.concatenate([h_sc[0:M2, :], h_sc[RH:, :]], axis=0)
        xn2 = side1(t)
        side2(t)
        out = attend(lambda g: _dot(h, w_head(g)).astype(BF16), RH, mask2)
        h_sc[0:M2, :] = out[0:M2].astype(BF16)
        h_sc[RH:, :] = xn2
        op_sc[SEG:, :] = out[M2:]
        return carry

    with jax.named_scope("steps_l2"):
        jax.lax.fori_loop(NSEG, NSEG + 2, step_l2, 0)
    side2(NSEG + 2)
    out_copy(NPH - 1).start()
    for i in range(NPH):
        out_copy(i).wait()


@functools.partial(jax.jit, static_argnames=("A_seg_len",))
def pallas_interleave_layers__memory_aug_recurrent_mem_tr__ssm_conv_h3__prompt_kernel(
    A_x, A_mem0, A_Wq, A_Wk, A_Wv, A_Wo, A_seg_len,
    B_q, B_k, B_v, B_shift_k, B_ssm_k, B_ssm_D,
):
    del B_q
    B, S, DM = A_x.shape
    assert B == 1
    H, DH = A_Wq.shape[1], A_Wq.shape[2]
    M = A_mem0.shape[1]
    SEG = int(A_seg_len)
    KS = B_shift_k.shape[1]
    R = 2 * (M + SEG)
    RP = 2 * M + NPRE * SEG
    NB = S // CB
    QB = CB // NQ
    fwd, inv = _dft_constants()

    kern = functools.partial(_kernel, S=S, DM=DM, H=H, DH=DH, M=M, SEG=SEG)
    any_spec = pl.BlockSpec(memory_space=pl.ANY)
    out = pl.pallas_call(
        kern,
        out_shape=jax.ShapeDtypeStruct((S, DM), A_x.dtype),
        in_specs=[any_spec] * 13,
        out_specs=any_spec,
        scratch_shapes=[
            pltpu.VMEM((M, DM), BF16),
            pltpu.VMEM((KS, DM), BF16),
            pltpu.VMEM((1, DM), BF16),
            pltpu.VMEM(fwd.shape, BF16),
            pltpu.VMEM(inv.shape, BF16),
            pltpu.VMEM((S, DM), BF16),
            pltpu.VMEM((S + KPAD, DM), BF16),
            pltpu.VMEM((S, DM), BF16),
            pltpu.VMEM((DM, S), BF16),
            pltpu.VMEM((6, DM, H // 2, DH), BF16),
            pltpu.VMEM((H * DH, DM), BF16),
            pltpu.VMEM((S, DM), A_x.dtype),
            pltpu.VMEM((H, DM // 2, 3 * DH), U32),
            pltpu.VMEM((RP, DM), BF16),
            pltpu.VMEM((H, RP // 2, 3 * DH), U32),
            pltpu.VMEM((R, DM), BF16),
            pltpu.VMEM((R, H * DH), BF16),
            pltpu.VMEM((2 * SEG, DM), F32),
            pltpu.VMEM((4, SEG, DM), F32),
            pltpu.VMEM((4, SEG, DM), F32),
            pltpu.VMEM((S, DM), BF16),
            pltpu.VMEM((NB + 2, NQ, QB // 8, DM // 128, 4, 8, 128), F32),
            pltpu.VMEM((NQ, 2 * QB, DM), F32),
            pltpu.VMEM((2, NQ, 2 * QB, DM), BF16),
            pltpu.SemaphoreType.DMA((5,)),
            pltpu.SemaphoreType.DMA((12,)),
            pltpu.SemaphoreType.DMA((7,)),
            pltpu.SemaphoreType.DMA((S // SEG // PH,)),
        ],
        compiler_params=pltpu.CompilerParams(vmem_limit_bytes=120 * 1024 * 1024),
    )(
        A_x.reshape(S, DM), A_mem0.reshape(M, DM), A_Wq, A_Wk, A_Wv,
        A_Wo.reshape(H * DH, DM), B_k.reshape(S, DM), B_v.reshape(S, DM),
        B_shift_k.T, B_ssm_k, B_ssm_D.reshape(1, DM),
        jnp.asarray(fwd, BF16), jnp.asarray(inv, BF16),
    )
    return out.reshape(B, S, DM)
```

```python
import functools

import numpy as np
import jax
import jax.numpy as jnp
import jax.experimental.pallas as pl
import jax.experimental.pallas.tpu as pltpu

F32 = jnp.float32
BF16 = jnp.bfloat16
U32 = jnp.uint32

CB = 128
NQ = 4
KPAD = 16
PH = 8
NPRE = 4
PINS = (3, 12, 16, 20)
SPEC_AT = 4
D1, D2 = 1, 2


def _dft_constants():
    qb = CB // NQ
    n = np.arange(CB, dtype=np.float64)
    fwd = np.zeros((NQ, 2 * qb, CB))
    for q in range(NQ):
        f = q * qb + np.concatenate([np.arange(0, qb, 2), np.arange(1, qb, 2)])
        ang = (np.pi * (2.0 * f + 1.0) / (2 * CB))[:, None] * n[None, :]
        fwd[q, :qb] = np.cos(ang)
        fwd[q, qb:] = -np.sin(ang)
    inv = fwd.reshape(2 * CB, CB).T / CB
    return fwd.astype(np.float32), inv.reshape(NQ, CB // NQ, 2 * CB).astype(np.float32)


def _ln(x, eps=1e-5):
    d = x.shape[-1]
    m = jnp.sum(x, axis=-1, keepdims=True) * (1.0 / d)
    xc = x - m
    v = jnp.sum(xc * xc, axis=-1, keepdims=True) * (1.0 / d)
    return xc * jax.lax.rsqrt(v + eps)


def _dot(a, b):
    return jnp.dot(a, b, preferred_element_type=F32)


def _dot_nt(a, b):
    return jax.lax.dot_general(a, b, (((1,), (1,)), ((), ())), preferred_element_type=F32)


def _pack(x):
    return pltpu.bitcast(x.astype(BF16), U32)


def _unpack(x):
    return pltpu.bitcast(x, BF16)


def _in_order(actions):
    def body(i, c):
        for j, act in enumerate(actions):
            pl.when(i == j)(act)
        return c
    jax.lax.fori_loop(0, len(actions), body, 0)


def _kernel(x_hbm, mem0_hbm, wq_hbm, wk_hbm, wv_hbm, wo_hbm, k_hbm, v_hbm,
            sh_hbm, sk_hbm, sd_hbm, fwd_hbm, inv_hbm, o_hbm,
            mem0_ref, sh_ref, sd_ref, fwd_ref, inv_ref,
            x_sc, k_sc, v_sc, sk_sc, st_sc, wo_st, wo_sc, out_sc,
            w_sc, hp_sc, pre_sc, h_sc, o_sc, op_sc, x2_sc, y_sc, u_sc, sp_sc, kr_sc, wf_sc,
            never_sm, sem_s, sem_in, sem_w, sem_out,
            *, S, DM, H, DH, M, SEG):
    NSEG = S // SEG
    M2 = 2 * M
    R = M2 + 2 * SEG
    RH = M2 + SEG
    NB = S // CB
    QB = CB // NQ
    HB = QB // 2
    NT = DM // 128
    assert QB == SEG and NSEG % PH == 0 and 2 <= NPRE <= PH
    NPH = NSEG // PH
    HG = H // 2

    small = [pltpu.make_async_copy(s, d, sem_s.at[i]) for i, (s, d) in enumerate([
        (mem0_hbm, mem0_ref), (sh_hbm, sh_ref), (sd_hbm, sd_ref), (fwd_hbm, fwd_ref), (inv_hbm, inv_ref)])]

    xb = (0, NPRE * SEG, 2 * PH * SEG, S)
    kb = (0, (2 * NQ + 2) * SEG, 2 * PH * SEG, S)
    sb = (0, 2 * CB, 2 * PH * SEG, S)

    def in_copies(part):
        def rng(b):
            return pl.ds(b[part], b[part + 1] - b[part])
        return [
            pltpu.make_async_copy(x_hbm.at[rng(xb)], x_sc.at[rng(xb)], sem_in.at[part * 4]),
            pltpu.make_async_copy(k_hbm.at[rng(kb)],
                                  k_sc.at[pl.ds(KPAD + kb[part], kb[part + 1] - kb[part])],
                                  sem_in.at[part * 4 + 1]),
            pltpu.make_async_copy(v_hbm.at[rng(kb)], v_sc.at[rng(kb)], sem_in.at[part * 4 + 2]),
            pltpu.make_async_copy(sk_hbm.at[:, rng(sb)], sk_sc.at[:, rng(sb)], sem_in.at[part * 4 + 3]),
        ]

    def w_copy(ci):
        src = (wq_hbm, wk_hbm, wv_hbm)[ci % 3]
        return pltpu.make_async_copy(src.at[:, pl.ds((ci // 3) * HG, HG), :], st_sc.at[ci], sem_w.at[ci])

    wo_copy = pltpu.make_async_copy(wo_hbm, wo_st, sem_w.at[6])

    def out_copy(i):
        rows = pl.ds(pl.multiple_of(i * PH * SEG, PH * SEG), PH * SEG)
        return pltpu.make_async_copy(out_sc.at[rows], o_hbm.at[rows], sem_out.at[i])

    def start_all(cps):
        def act():
            for cp in cps:
                cp.start()
        return act

    _in_order([start_all(small + in_copies(0))]
              + [start_all([w_copy(ci)]) for ci in range(6)]
              + [start_all([wo_copy]), start_all(in_copies(1)), start_all(in_copies(2))])

    never_sm[0] = 0
    k_sc[0:KPAD, :] = jnp.zeros((KPAD, DM), BF16)
    sp_sc[NB + 1] = jnp.zeros(sp_sc.shape[1:], F32)
    op_sc[...] = jnp.zeros(op_sc.shape, F32)
    x2_sc[...] = jnp.zeros(x2_sc.shape, F32)
    y_sc[...] = jnp.zeros(y_sc.shape, F32)
    h_sc[...] = jnp.zeros(h_sc.shape, BF16)
    for cp in small + in_copies(0):
        cp.wait()

    sh = sh_ref[...].astype(F32)
    KS = sh.shape[0]
    sd = sd_ref[...].astype(F32)

    def seg(i):
        i = jnp.clip(i, 0, NSEG - 1)
        return pl.ds(pl.multiple_of(i * SEG, SEG), SEG)

    def conv_u(s):
        s = jnp.clip(s, 0, NSEG - 1)
        r0 = pl.multiple_of(s * SEG, SEG)
        kk = k_sc[pl.ds(r0, KPAD + SEG), :].astype(F32)
        ks = kk[KPAD:] * sh[0:1]
        for j in range(1, KS):
            ks = ks + pltpu.roll(kk, j, 0)[KPAD:] * sh[j:j + 1]
        u = (ks * v_sc[pl.ds(r0, SEG), :].astype(F32)).astype(BF16)
        u_sc[pl.ds(r0, SEG), :] = u
        return u

    def conv_fwd(c, q):
        cc = jnp.minimum(c, NB - 1)
        t0 = pl.multiple_of(cc * CB, CB)
        f = fwd_ref[q]
        uf = _dot(f, u_sc[pl.ds(t0, CB), :])
        kf = _dot_nt(f, sk_sc[:, pl.ds(t0, CB)])
        return uf, kf

    def put_spec(cs, q, which, val):
        for rb in range(QB // 8):
            for n in range(NT):
                ln = slice(n * 128, (n + 1) * 128)
                sp_sc[cs, q, rb, n, which] = val[rb * 8:rb * 8 + 8, ln]
                sp_sc[cs, q, rb, n, which + 1] = val[QB + rb * 8:QB + rb * 8 + 8, ln]

    def conv_spec(c, q):
        uf, kf = conv_fwd(c, q)
        cs = jnp.minimum(c, NB)
        put_spec(cs, q, 0, uf)
        pk = kr_sc[q]
        kr_sc[q] = kf
        kp = jnp.concatenate([
            kf[0:HB] - pk[QB:QB + HB],
            kf[HB:QB] + pk[QB + HB:],
            kf[QB:QB + HB] + pk[0:HB],
            kf[QB + HB:] - pk[HB:QB]], axis=0)
        put_spec(cs, q, 2, kp)

    MAC_PIECES = [(rb, n) for rb in range(QB // 16) for n in range(NT)]

    def conv_mac(c, q, piece, nterms):
        rb2, n = piece
        cs = jnp.minimum(c, NB)
        acc = []
        for rb in (2 * rb2, 2 * rb2 + 1):
            ar = None
            ai = None
            for j in range(nterms):
                uj = jnp.minimum(j, cs)
                kj = jnp.where(cs - j >= 0, cs - j, NB + 1)
                ur = sp_sc[uj, q, rb, n, 0]
                um = sp_sc[uj, q, rb, n, 1]
                kr = sp_sc[kj, q, rb, n, 2]
                km = sp_sc[kj, q, rb, n, 3]
                tr = ur * kr - um * km
                ti = ur * km + um * kr
                ar = tr if ar is None else ar + tr
                ai = ti if ai is None else ai + ti
            acc.append((ar, ai))
        ln = slice(n * 128, (n + 1) * 128)
        wf_sc[c & 1, q, rb2 * 16:rb2 * 16 + 16, ln] = jnp.concatenate(
            [acc[0][0], acc[1][0]], axis=0).astype(BF16)
        wf_sc[c & 1, q, QB + rb2 * 16:QB + rb2 * 16 + 16, ln] = jnp.concatenate(
            [acc[0][1], acc[1][1]], axis=0).astype(BF16)

    def conv_inv(s):
        w = wf_sc[(s // NQ) & 1].reshape(2 * CB, DM)
        yc = _dot(inv_ref[s % NQ], w)
        y_sc[s & 3] = yc + u_sc[seg(s), :].astype(F32) * sd

    scale = DH ** -0.5
    cexp = scale * float(np.log2(np.e))

    def make_mask(n, x_layers):
        qi = jax.lax.broadcasted_iota(jnp.int32, (n, n), 0)
        ki = jax.lax.broadcasted_iota(jnp.int32, (n, n), 1)

        def layer(i):
            xl = jnp.where(i < M2 + SEG, x_layers[0], x_layers[-1])
            return jnp.where(i < M, 0, jnp.where(i < M2, 1, xl))
        same = layer(qi) == layer(ki)
        ok = same & ((qi < M2) | (ki < M2) | (qi >= ki))
        fill = jnp.where(same, -1e9 / scale, -jnp.inf).astype(F32)
        return ok, fill

    def probs(qkv, mask):
        ok, fill = mask
        s = _dot_nt(qkv[:, 0:DH], qkv[:, DH:2 * DH])
        s = jnp.where(ok, s, fill)
        m = jnp.max(s, axis=-1, keepdims=True)
        p = jnp.exp2((s - m) * cexp)
        l = jnp.sum(p, axis=-1, keepdims=True)
        r = pl.reciprocal(l, approx=True)
        r = r * (2.0 - l * r)
        return (p * r).astype(BF16)

    def w_head(g):
        return pltpu.bitcast(w_sc[g], BF16)

    def pre_rows(g, w0, n):
        return pltpu.bitcast(pre_sc[g, pl.ds(w0, n // 2), :], BF16)

    def out_proj(n, g0, g1, j):
        return _dot(_unpack(o_sc[0:n // 2, g0 * DH:g1 * DH]),
                    _unpack(wo_sc[g0 * DH // 2:g1 * DH // 2, j * 128:(j + 1) * 128]))

    def attend(proj, n, mask, hook=None):
        HA = H - D1 - D2 - 1
        qkvs = {}
        ps = {}
        outs = {}
        for it in range(H + D1 + D2):
            if it < H:
                qkvs[it] = proj(it)
            g = it - D1
            if 0 <= g < H:
                ps[g] = probs(qkvs[g], mask)
            g = it - D1 - D2
            if 0 <= g < H:
                o = _dot(ps.pop(g), qkvs.pop(g)[:, 2 * DH:3 * DH])
                o_sc[0:n // 2, g * DH:(g + 1) * DH] = _pack(o)
            if hook is not None:
                hook(it)
            j = it - (H - 1)
            if 0 <= j < D1 + D2:
                outs[j] = out_proj(n, 0, HA, j)
        for j in range(D1 + D2, NT):
            outs[j] = out_proj(n, 0, H, j)
        for j in range(D1 + D2):
            outs[j] = out_proj(n, HA, H, j) + outs[j]
        return jnp.concatenate([outs[j] for j in range(NT)], axis=1)

    def side1(t):
        x1 = x_sc[seg(t - 1), :].astype(F32) + op_sc[0:SEG, :]
        x2 = x1 + _ln(x1) * y_sc[(t - 1) & 3]
        x2_sc[(t - 1) & 3] = x2
        return _ln(x2).astype(BF16)

    def side2(t):
        x3 = x2_sc[(t - 3) & 3] + op_sc[SEG:, :]
        x4 = x3 + _ln(x3) * y_sc[(t - 3) & 3]
        x4 = x4.astype(out_sc.dtype)
        out_sc[seg(t - 3), :] = x4
        return x4

    def mac_hook(c, q, nterms):
        def hook(it):
            if it % 3 == 2 and it // 3 < len(MAC_PIECES):
                conv_mac(c, q, MAC_PIECES[it // 3], nterms)
        return hook

    def pro_u(s, c):
        conv_u(s)
        return c
    jax.lax.fori_loop(0, 2 * NQ + 1, pro_u, 0)

    def pro_c(q, c):
        uf, kf = conv_fwd(0, q)
        put_spec(0, q, 0, uf)
        put_spec(0, q, 2, kf)
        kr_sc[q] = kf
        ur, um, kr, km = uf[:QB], uf[QB:], kf[:QB], kf[QB:]
        wf_sc[0, q, :QB] = (ur * kr - um * km).astype(BF16)
        wf_sc[0, q, QB:] = (ur * km + um * kr).astype(BF16)
        return c
    jax.lax.fori_loop(0, NQ, pro_c, 0)
    conv_spec(1, 0)
    for piece in MAC_PIECES:
        conv_mac(1, 0, piece, 2)
    conv_inv(0)

    mem0 = mem0_ref[...].astype(F32)
    hp_sc[0:M2, :] = jnp.concatenate([mem0, mem0], axis=0).astype(BF16)

    def pro_h(s, c):
        hp_sc[pl.ds(pl.multiple_of(M2 + s * SEG, 16), SEG), :] = _ln(x_sc[seg(s), :].astype(F32)).astype(BF16)
        return c
    jax.lax.fori_loop(0, NPRE, pro_h, 0)

    mask1 = make_mask(RH, (0,))

    def chunk(ci, carry):
        g0 = (ci // 3) * HG
        cols = pl.ds(pl.multiple_of((ci % 3) * DH, DH), DH)
        with jax.named_scope("wait_w"):
            pltpu.make_async_copy(wq_hbm.at[:, pl.ds(0, HG), :], st_sc.at[ci], sem_w.at[ci]).wait()

        def relayout(b, c):
            d0 = pl.multiple_of(b * 16, 16)
            r0 = pl.multiple_of(b * 8, 8)
            xw = pltpu.bitcast(st_sc[ci, pl.ds(d0, 16)], U32).reshape(8, 2, HG // 2, DH)
            a = xw[:, 0]
            bb = xw[:, 1]
            lo = jnp.swapaxes((a & U32(0xFFFF)) | (bb << 16), 0, 1)
            hi = jnp.swapaxes((a >> 16) | (bb & U32(0xFFFF0000)), 0, 1)
            for j in range(HG // 2):
                w_sc[g0 + 2 * j, pl.ds(r0, 8), cols] = lo[j]
                w_sc[g0 + 2 * j + 1, pl.ds(r0, 8), cols] = hi[j]
            return c
        with jax.named_scope("relayout"):
            jax.lax.fori_loop(0, DM // 16, relayout, 0, unroll=2)

        with jax.named_scope("preproj"):
            hp = hp_sc[...]
            for j in range(HG):
                res = _dot(hp, pltpu.bitcast(w_sc[g0 + j, :, cols], BF16)).astype(BF16)
                pre_sc[g0 + j, :, cols] = pltpu.bitcast(res, U32)

        @pl.when(ci % 3 == 2)
        def _():
            ps = {}
            for it in range(HG + 2):
                if it < HG:
                    ps[it] = probs(pre_rows(g0 + it, 0, RH), mask1)
                j = it - 2
                if j >= 0:
                    o = _dot(ps.pop(j), pre_rows(g0 + j, 0, RH)[:, 2 * DH:])
                    o_sc[0:RH // 2, pl.ds(pl.multiple_of((g0 + j) * DH, DH), DH)] = _pack(o)
        return carry
    jax.lax.fori_loop(0, 6, chunk, 0)

    with jax.named_scope("wait_wo"):
        wo_copy.wait()
    wo = wo_st[...]
    wo_sc[...] = _pack(wo)
    out = _dot(_unpack(o_sc[0:RH // 2, :]), wo)
    h_sc[0:M2, :] = jnp.concatenate([out[0:M], mem0], axis=0).astype(BF16)
    op_sc[0:SEG, :] = out[M2:]

    with jax.named_scope("step1"):
        hm = h_sc[0:M2, :]
        conv_spec(1, 1)
        xn2 = side1(1)
        out = attend(lambda g: jnp.concatenate(
            [_dot(hm, w_head(g)).astype(BF16), pre_rows(g, M + SEG // 2, SEG)], axis=0),
            RH, mask1, mac_hook(1, 1, 2))
        conv_inv(1)
        conv_u(1 + 2 * NQ)
        h_sc[0:M2, :] = jnp.concatenate([out[0:M], mem0], axis=0).astype(BF16)
        h_sc[RH:, :] = xn2
        op_sc[0:SEG, :] = out[M2:]

    for cp in in_copies(1):
        cp.wait()

    mask12 = make_mask(R, (0, 1))

    def pinned(never, h, pins):
        hs = {0: h}
        r = _pack(h[-SEG:])
        for g, d in pins:
            r = jnp.where(never, _pack(d), r)
            hs[g] = jnp.concatenate([h[:-SEG], _unpack(r)], axis=0)
        return lambda g: hs[max(k for k in hs if k <= g)]

    def step(t, pre):
        c = t // NQ + 1
        q = t % NQ
        x4 = side2(t)
        xn2 = side1(t)
        xn1 = _ln(x_sc[seg(t + 1), :].astype(F32)).astype(BF16)
        un = conv_u(t + 2 * NQ)
        pins = list(zip(PINS, (un, xn1, x4, xn2)))
        never = never_sm[0] > 0
        if pre:
            h = pinned(never, jnp.concatenate([h_sc[0:M2, :], h_sc[RH:, :]], axis=0), pins)

            def proj(g):
                r = _dot(h(g), w_head(g)).astype(BF16)
                x1 = pre_rows(g, pl.multiple_of(M + t * (SEG // 2), 8), SEG)
                return jnp.concatenate([r[0:M2], x1, r[M2:]], axis=0)
            nterms = (NPRE - 1) // NQ + 2
        else:
            h = pinned(never, h_sc[...], pins)

            def proj(g):
                return _dot(h(g), w_head(g)).astype(BF16)
            nterms = NB
        h_sc[M2:RH, :] = xn1
        h_sc[RH:, :] = xn2

        def hook(it):
            if it == SPEC_AT:
                conv_spec(c, q)
            if it == SPEC_AT + 1:
                for piece in MAC_PIECES:
                    conv_mac(c, q, piece, nterms)
        out = attend(proj, R, mask12, hook)
        conv_inv(t)
        h_sc[0:M2, :] = out[0:M2].astype(BF16)
        op_sc[...] = out[M2:]

    def step_pre(t, carry):
        step(t, True)
        return carry

    def step_full(t, carry):
        step(t, False)
        return carry

    with jax.named_scope("steps_pre"):
        jax.lax.fori_loop(2, NPRE, step_pre, 0)

    def phase(p, carry):
        @pl.when(p == 1)
        def _():
            for cp in in_copies(2):
                cp.wait()

        @pl.when(p >= 2)
        def _():
            out_copy(p - 2).start()

        with jax.named_scope("steps"):
            jax.lax.fori_loop(jnp.maximum(p * PH, NPRE), p * PH + PH, step_full, 0)
        return carry

    jax.lax.fori_loop(0, NPH, phase, 0)
    out_copy(NPH - 2).start()

    mask2 = make_mask(RH, (1,))

    def step_l2(t, carry):
        h = jnp.concatenate([h_sc[0:M2, :], h_sc[RH:, :]], axis=0)
        side2(t)
        xn2 = side1(t)
        out = attend(lambda g: _dot(h, w_head(g)).astype(BF16), RH, mask2)
        h_sc[0:M2, :] = out[0:M2].astype(BF16)
        h_sc[RH:, :] = xn2
        op_sc[SEG:, :] = out[M2:]
        return carry

    with jax.named_scope("steps_l2"):
        jax.lax.fori_loop(NSEG, NSEG + 2, step_l2, 0)
    side2(NSEG + 2)
    out_copy(NPH - 1).start()
    for i in range(NPH):
        out_copy(i).wait()


@functools.partial(jax.jit, static_argnames=("A_seg_len",))
def pallas_interleave_layers__memory_aug_recurrent_mem_tr__ssm_conv_h3__prompt_kernel(
    A_x, A_mem0, A_Wq, A_Wk, A_Wv, A_Wo, A_seg_len,
    B_q, B_k, B_v, B_shift_k, B_ssm_k, B_ssm_D,
):
    del B_q
    B, S, DM = A_x.shape
    assert B == 1
    H, DH = A_Wq.shape[1], A_Wq.shape[2]
    M = A_mem0.shape[1]
    SEG = int(A_seg_len)
    KS = B_shift_k.shape[1]
    R = 2 * (M + SEG)
    RP = 2 * M + NPRE * SEG
    NB = S // CB
    QB = CB // NQ
    fwd, inv = _dft_constants()

    kern = functools.partial(_kernel, S=S, DM=DM, H=H, DH=DH, M=M, SEG=SEG)
    any_spec = pl.BlockSpec(memory_space=pl.ANY)
    out = pl.pallas_call(
        kern,
        out_shape=jax.ShapeDtypeStruct((S, DM), A_x.dtype),
        in_specs=[any_spec] * 13,
        out_specs=any_spec,
        scratch_shapes=[
            pltpu.VMEM((M, DM), BF16),
            pltpu.VMEM((KS, DM), BF16),
            pltpu.VMEM((1, DM), BF16),
            pltpu.VMEM(fwd.shape, BF16),
            pltpu.VMEM(inv.shape, BF16),
            pltpu.VMEM((S, DM), BF16),
            pltpu.VMEM((S + KPAD, DM), BF16),
            pltpu.VMEM((S, DM), BF16),
            pltpu.VMEM((DM, S), BF16),
            pltpu.VMEM((6, DM, H // 2, DH), BF16),
            pltpu.VMEM((H * DH, DM), BF16),
            pltpu.VMEM((H * DH // 2, DM), U32),
            pltpu.VMEM((S, DM), A_x.dtype),
            pltpu.VMEM((H, DM // 2, 3 * DH), U32),
            pltpu.VMEM((RP, DM), BF16),
            pltpu.VMEM((H, RP // 2, 3 * DH), U32),
            pltpu.VMEM((R, DM), BF16),
            pltpu.VMEM((R // 2, H * DH), U32),
            pltpu.VMEM((2 * SEG, DM), F32),
            pltpu.VMEM((4, SEG, DM), F32),
            pltpu.VMEM((4, SEG, DM), F32),
            pltpu.VMEM((S, DM), BF16),
            pltpu.VMEM((NB + 2, NQ, QB // 8, DM // 128, 4, 8, 128), F32),
            pltpu.VMEM((NQ, 2 * QB, DM), F32),
            pltpu.VMEM((2, NQ, 2 * QB, DM), BF16),
            pltpu.SMEM((1,), jnp.int32),
            pltpu.SemaphoreType.DMA((5,)),
            pltpu.SemaphoreType.DMA((12,)),
            pltpu.SemaphoreType.DMA((7,)),
            pltpu.SemaphoreType.DMA((S // SEG // PH,)),
        ],
        compiler_params=pltpu.CompilerParams(vmem_limit_bytes=120 * 1024 * 1024),
    )(
        A_x.reshape(S, DM), A_mem0.reshape(M, DM), A_Wq, A_Wk, A_Wv,
        A_Wo.reshape(H * DH, DM), B_k.reshape(S, DM), B_v.reshape(S, DM),
        B_shift_k.T, B_ssm_k, B_ssm_D.reshape(1, DM),
        jnp.asarray(fwd, BF16), jnp.asarray(inv, BF16),
    )
    return out.reshape(B, S, DM)
```

```python
import functools

import numpy as np
import jax
import jax.numpy as jnp
import jax.experimental.pallas as pl
import jax.experimental.pallas.tpu as pltpu

F32 = jnp.float32
BF16 = jnp.bfloat16
U32 = jnp.uint32

CB = 128
NQ = 4
KPAD = 16
PH = 8
NPRE = 4
PINS = (3, 12, 16, 20)
SPEC_AT = 4
UNROLL = 2
D1, D2 = 1, 2


def _dft_constants():
    qb = CB // NQ
    n = np.arange(CB, dtype=np.float64)
    fwd = np.zeros((NQ, 2 * qb, CB))
    for q in range(NQ):
        f = q * qb + np.concatenate([np.arange(0, qb, 2), np.arange(1, qb, 2)])
        ang = (np.pi * (2.0 * f + 1.0) / (2 * CB))[:, None] * n[None, :]
        fwd[q, :qb] = np.cos(ang)
        fwd[q, qb:] = -np.sin(ang)
    inv = fwd.reshape(2 * CB, CB).T / CB
    return fwd.astype(np.float32), inv.reshape(NQ, CB // NQ, 2 * CB).astype(np.float32)


def _ln(x, eps=1e-5):
    d = x.shape[-1]
    m = jnp.sum(x, axis=-1, keepdims=True) * (1.0 / d)
    xc = x - m
    v = jnp.sum(xc * xc, axis=-1, keepdims=True) * (1.0 / d)
    return xc * jax.lax.rsqrt(v + eps)


def _dot(a, b):
    return jnp.dot(a, b, preferred_element_type=F32)


def _dot_nt(a, b):
    return jax.lax.dot_general(a, b, (((1,), (1,)), ((), ())), preferred_element_type=F32)


def _pack(x):
    return pltpu.bitcast(x.astype(BF16), U32)


def _unpack(x):
    return pltpu.bitcast(x, BF16)


def _in_order(actions):
    def body(i, c):
        for j, act in enumerate(actions):
            pl.when(i == j)(act)
        return c
    jax.lax.fori_loop(0, len(actions), body, 0)


def _kernel(x_hbm, mem0_hbm, wq_hbm, wk_hbm, wv_hbm, wo_hbm, k_hbm, v_hbm,
            sh_hbm, sk_hbm, sd_hbm, fwd_hbm, inv_hbm, o_hbm,
            mem0_ref, sh_ref, sd_ref, fwd_ref, inv_ref,
            x_sc, k_sc, v_sc, sk_sc, st_sc, wo_st, wo_sc, out_sc,
            w_sc, hp_sc, pre_sc, h_sc, o_sc, op_sc, x2_sc, y_sc, u_sc, sp_sc, kr_sc, wf_sc,
            never_sm, sem_s, sem_in, sem_w, sem_out,
            *, S, DM, H, DH, M, SEG):
    NSEG = S // SEG
    M2 = 2 * M
    R = M2 + 2 * SEG
    RH = M2 + SEG
    NB = S // CB
    QB = CB // NQ
    HB = QB // 2
    NT = DM // 128
    assert QB == SEG and NSEG % PH == 0 and 2 <= NPRE <= PH
    NPH = NSEG // PH
    HG = H // 2

    small = [pltpu.make_async_copy(s, d, sem_s.at[i]) for i, (s, d) in enumerate([
        (mem0_hbm, mem0_ref), (sh_hbm, sh_ref), (sd_hbm, sd_ref), (fwd_hbm, fwd_ref), (inv_hbm, inv_ref)])]

    xb = (0, NPRE * SEG, 2 * PH * SEG, S)
    kb = (0, (2 * NQ + 2) * SEG, 2 * PH * SEG, S)
    sb = (0, 2 * CB, 2 * PH * SEG, S)

    def in_copies(part):
        def rng(b):
            return pl.ds(b[part], b[part + 1] - b[part])
        return [
            pltpu.make_async_copy(x_hbm.at[rng(xb)], x_sc.at[rng(xb)], sem_in.at[part * 4]),
            pltpu.make_async_copy(k_hbm.at[rng(kb)],
                                  k_sc.at[pl.ds(KPAD + kb[part], kb[part + 1] - kb[part])],
                                  sem_in.at[part * 4 + 1]),
            pltpu.make_async_copy(v_hbm.at[rng(kb)], v_sc.at[rng(kb)], sem_in.at[part * 4 + 2]),
            pltpu.make_async_copy(sk_hbm.at[:, rng(sb)], sk_sc.at[:, rng(sb)], sem_in.at[part * 4 + 3]),
        ]

    def w_copy(ci):
        src = (wq_hbm, wk_hbm, wv_hbm)[ci % 3]
        return pltpu.make_async_copy(src.at[:, pl.ds((ci // 3) * HG, HG), :], st_sc.at[ci], sem_w.at[ci])

    wo_copy = pltpu.make_async_copy(wo_hbm, wo_st, sem_w.at[6])

    def out_copy(i):
        rows = pl.ds(pl.multiple_of(i * PH * SEG, PH * SEG), PH * SEG)
        return pltpu.make_async_copy(out_sc.at[rows], o_hbm.at[rows], sem_out.at[i])

    def start_all(cps):
        def act():
            for cp in cps:
                cp.start()
        return act

    _in_order([start_all(small + in_copies(0))]
              + [start_all([w_copy(ci)]) for ci in range(6)]
              + [start_all([wo_copy]), start_all(in_copies(1)), start_all(in_copies(2))])

    never_sm[0] = 0
    k_sc[0:KPAD, :] = jnp.zeros((KPAD, DM), BF16)
    sp_sc[NB + 1] = jnp.zeros(sp_sc.shape[1:], F32)
    op_sc[...] = jnp.zeros(op_sc.shape, F32)
    x2_sc[...] = jnp.zeros(x2_sc.shape, F32)
    y_sc[...] = jnp.zeros(y_sc.shape, F32)
    h_sc[...] = jnp.zeros(h_sc.shape, BF16)
    for cp in small + in_copies(0):
        cp.wait()

    sh = sh_ref[...].astype(F32)
    KS = sh.shape[0]
    sd = sd_ref[...].astype(F32)

    def seg(i):
        i = jnp.clip(i, 0, NSEG - 1)
        return pl.ds(pl.multiple_of(i * SEG, SEG), SEG)

    def conv_u(s):
        s = jnp.clip(s, 0, NSEG - 1)
        r0 = pl.multiple_of(s * SEG, SEG)
        kk = k_sc[pl.ds(r0, KPAD + SEG), :].astype(F32)
        ks = kk[KPAD:] * sh[0:1]
        for j in range(1, KS):
            ks = ks + pltpu.roll(kk, j, 0)[KPAD:] * sh[j:j + 1]
        u = (ks * v_sc[pl.ds(r0, SEG), :].astype(F32)).astype(BF16)
        u_sc[pl.ds(r0, SEG), :] = u
        return u

    def conv_fwd(c, q):
        cc = jnp.minimum(c, NB - 1)
        t0 = pl.multiple_of(cc * CB, CB)
        f = fwd_ref[q]
        uf = _dot(f, u_sc[pl.ds(t0, CB), :])
        kf = _dot_nt(f, sk_sc[:, pl.ds(t0, CB)])
        return uf, kf

    def put_spec(cs, q, which, val):
        for rb in range(QB // 8):
            for n in range(NT):
                ln = slice(n * 128, (n + 1) * 128)
                sp_sc[cs, q, rb, n, which] = val[rb * 8:rb * 8 + 8, ln]
                sp_sc[cs, q, rb, n, which + 1] = val[QB + rb * 8:QB + rb * 8 + 8, ln]

    def conv_spec(c, q):
        uf, kf = conv_fwd(c, q)
        cs = jnp.minimum(c, NB)
        put_spec(cs, q, 0, uf)
        pk = kr_sc[q]
        kr_sc[q] = kf
        kp = jnp.concatenate([
            kf[0:HB] - pk[QB:QB + HB],
            kf[HB:QB] + pk[QB + HB:],
            kf[QB:QB + HB] + pk[0:HB],
            kf[QB + HB:] - pk[HB:QB]], axis=0)
        put_spec(cs, q, 2, kp)

    MAC_PIECES = [(rb, n) for rb in range(QB // 16) for n in range(NT)]

    def conv_mac(c, q, piece, nterms):
        rb2, n = piece
        cs = jnp.minimum(c, NB)
        acc = []
        for rb in (2 * rb2, 2 * rb2 + 1):
            ar = None
            ai = None
            for j in range(nterms):
                uj = jnp.minimum(j, cs)
                kj = jnp.where(cs - j >= 0, cs - j, NB + 1)
                ur = sp_sc[uj, q, rb, n, 0]
                um = sp_sc[uj, q, rb, n, 1]
                kr = sp_sc[kj, q, rb, n, 2]
                km = sp_sc[kj, q, rb, n, 3]
                tr = ur * kr - um * km
                ti = ur * km + um * kr
                ar = tr if ar is None else ar + tr
                ai = ti if ai is None else ai + ti
            acc.append((ar, ai))
        ln = slice(n * 128, (n + 1) * 128)
        wf_sc[c & 1, q, rb2 * 16:rb2 * 16 + 16, ln] = jnp.concatenate(
            [acc[0][0], acc[1][0]], axis=0).astype(BF16)
        wf_sc[c & 1, q, QB + rb2 * 16:QB + rb2 * 16 + 16, ln] = jnp.concatenate(
            [acc[0][1], acc[1][1]], axis=0).astype(BF16)

    def conv_inv(s):
        w = wf_sc[(s // NQ) & 1].reshape(2 * CB, DM)
        yc = _dot(inv_ref[s % NQ], w)
        y_sc[s & 3] = yc + u_sc[seg(s), :].astype(F32) * sd

    scale = DH ** -0.5
    cexp = scale * float(np.log2(np.e))

    def make_mask(n, x_layers):
        qi = jax.lax.broadcasted_iota(jnp.int32, (n, n), 0)
        ki = jax.lax.broadcasted_iota(jnp.int32, (n, n), 1)

        def layer(i):
            xl = jnp.where(i < M2 + SEG, x_layers[0], x_layers[-1])
            return jnp.where(i < M, 0, jnp.where(i < M2, 1, xl))
        same = layer(qi) == layer(ki)
        ok = same & ((qi < M2) | (ki < M2) | (qi >= ki))
        fill = jnp.where(same, -1e9 / scale, -jnp.inf).astype(F32)
        return ok, fill

    def probs(qkv, mask):
        ok, fill = mask
        s = _dot_nt(qkv[:, 0:DH], qkv[:, DH:2 * DH])
        s = jnp.where(ok, s, fill)
        m = jnp.max(s, axis=-1, keepdims=True)
        p = jnp.exp2((s - m) * cexp)
        l = jnp.sum(p, axis=-1, keepdims=True)
        r = pl.reciprocal(l, approx=True)
        r = r * (2.0 - l * r)
        return (p * r).astype(BF16)

    def w_head(g):
        return pltpu.bitcast(w_sc[g], BF16)

    def pre_rows(g, w0, n):
        return pltpu.bitcast(pre_sc[g, pl.ds(w0, n // 2), :], BF16)

    def out_proj(n, g0, g1, j):
        return _dot(_unpack(o_sc[0:n // 2, g0 * DH:g1 * DH]),
                    _unpack(wo_sc[g0 * DH // 2:g1 * DH // 2, j * 128:(j + 1) * 128]))

    def attend(proj, n, mask, hook=None):
        HA = H - D1 - D2 - 1
        qkvs = {}
        ps = {}
        outs = {}
        for it in range(H + D1 + D2):
            if it < H:
                qkvs[it] = proj(it)
            g = it - D1
            if 0 <= g < H:
                ps[g] = probs(qkvs[g], mask)
            g = it - D1 - D2
            if 0 <= g < H:
                o = _dot(ps.pop(g), qkvs.pop(g)[:, 2 * DH:3 * DH])
                o_sc[0:n // 2, g * DH:(g + 1) * DH] = _pack(o)
            if hook is not None:
                hook(it)
            j = it - (H - 1)
            if 0 <= j < D1 + D2:
                outs[j] = out_proj(n, 0, HA, j)
        for j in range(D1 + D2, NT):
            outs[j] = out_proj(n, 0, H, j)
        for j in range(D1 + D2):
            outs[j] = out_proj(n, HA, H, j) + outs[j]
        return jnp.concatenate([outs[j] for j in range(NT)], axis=1)

    def side1(t):
        x1 = x_sc[seg(t - 1), :].astype(F32) + op_sc[0:SEG, :]
        x2 = x1 + _ln(x1) * y_sc[(t - 1) & 3]
        x2_sc[(t - 1) & 3] = x2
        return _ln(x2).astype(BF16)

    def side2(t):
        x3 = x2_sc[(t - 3) & 3] + op_sc[SEG:, :]
        x4 = x3 + _ln(x3) * y_sc[(t - 3) & 3]
        x4 = x4.astype(out_sc.dtype)
        out_sc[seg(t - 3), :] = x4
        return x4

    def mac_hook(c, q, nterms):
        def hook(it):
            if it % 3 == 2 and it // 3 < len(MAC_PIECES):
                conv_mac(c, q, MAC_PIECES[it // 3], nterms)
        return hook

    def pro_u(s, c):
        conv_u(s)
        return c
    jax.lax.fori_loop(0, 2 * NQ + 1, pro_u, 0)

    def pro_c(q, c):
        uf, kf = conv_fwd(0, q)
        put_spec(0, q, 0, uf)
        put_spec(0, q, 2, kf)
        kr_sc[q] = kf
        ur, um, kr, km = uf[:QB], uf[QB:], kf[:QB], kf[QB:]
        wf_sc[0, q, :QB] = (ur * kr - um * km).astype(BF16)
        wf_sc[0, q, QB:] = (ur * km + um * kr).astype(BF16)
        return c
    jax.lax.fori_loop(0, NQ, pro_c, 0)
    conv_spec(1, 0)
    for piece in MAC_PIECES:
        conv_mac(1, 0, piece, 2)
    conv_inv(0)

    mem0 = mem0_ref[...].astype(F32)
    hp_sc[0:M2, :] = jnp.concatenate([mem0, mem0], axis=0).astype(BF16)

    def pro_h(s, c):
        hp_sc[pl.ds(pl.multiple_of(M2 + s * SEG, 16), SEG), :] = _ln(x_sc[seg(s), :].astype(F32)).astype(BF16)
        return c
    jax.lax.fori_loop(0, NPRE, pro_h, 0)

    mask1 = make_mask(RH, (0,))

    def chunk(ci, carry):
        g0 = (ci // 3) * HG
        cols = pl.ds(pl.multiple_of((ci % 3) * DH, DH), DH)
        with jax.named_scope("wait_w"):
            pltpu.make_async_copy(wq_hbm.at[:, pl.ds(0, HG), :], st_sc.at[ci], sem_w.at[ci]).wait()

        def relayout(b, c):
            d0 = pl.multiple_of(b * 16, 16)
            r0 = pl.multiple_of(b * 8, 8)
            xw = pltpu.bitcast(st_sc[ci, pl.ds(d0, 16)], U32).reshape(8, 2, HG // 2, DH)
            a = xw[:, 0]
            bb = xw[:, 1]
            lo = jnp.swapaxes((a & U32(0xFFFF)) | (bb << 16), 0, 1)
            hi = jnp.swapaxes((a >> 16) | (bb & U32(0xFFFF0000)), 0, 1)
            for j in range(HG // 2):
                w_sc[g0 + 2 * j, pl.ds(r0, 8), cols] = lo[j]
                w_sc[g0 + 2 * j + 1, pl.ds(r0, 8), cols] = hi[j]
            return c
        with jax.named_scope("relayout"):
            jax.lax.fori_loop(0, DM // 16, relayout, 0, unroll=2)

        with jax.named_scope("preproj"):
            hp = hp_sc[...]
            for j in range(HG):
                res = _dot(hp, pltpu.bitcast(w_sc[g0 + j, :, cols], BF16)).astype(BF16)
                pre_sc[g0 + j, :, cols] = pltpu.bitcast(res, U32)

        @pl.when(ci % 3 == 2)
        def _():
            ps = {}
            for it in range(HG + 2):
                if it < HG:
                    ps[it] = probs(pre_rows(g0 + it, 0, RH), mask1)
                j = it - 2
                if j >= 0:
                    o = _dot(ps.pop(j), pre_rows(g0 + j, 0, RH)[:, 2 * DH:])
                    o_sc[0:RH // 2, pl.ds(pl.multiple_of((g0 + j) * DH, DH), DH)] = _pack(o)
        return carry
    jax.lax.fori_loop(0, 6, chunk, 0)

    with jax.named_scope("wait_wo"):
        wo_copy.wait()
    wo = wo_st[...]
    wo_sc[...] = _pack(wo)
    out = _dot(_unpack(o_sc[0:RH // 2, :]), wo)
    h_sc[0:M2, :] = jnp.concatenate([out[0:M], mem0], axis=0).astype(BF16)
    op_sc[0:SEG, :] = out[M2:]

    with jax.named_scope("step1"):
        hm = h_sc[0:M2, :]
        conv_spec(1, 1)
        xn2 = side1(1)
        out = attend(lambda g: jnp.concatenate(
            [_dot(hm, w_head(g)).astype(BF16), pre_rows(g, M + SEG // 2, SEG)], axis=0),
            RH, mask1, mac_hook(1, 1, 2))
        conv_inv(1)
        conv_u(1 + 2 * NQ)
        h_sc[0:M2, :] = jnp.concatenate([out[0:M], mem0], axis=0).astype(BF16)
        h_sc[RH:, :] = xn2
        op_sc[0:SEG, :] = out[M2:]

    for cp in in_copies(1):
        cp.wait()

    mask12 = make_mask(R, (0, 1))

    def pinned(never, h, pins):
        hs = {0: h}
        r = _pack(h[-SEG:])
        for g, d in pins:
            r = jnp.where(never, _pack(d), r)
            hs[g] = jnp.concatenate([h[:-SEG], _unpack(r)], axis=0)
        return lambda g: hs[max(k for k in hs if k <= g)]

    def step(t, pre, spec_first=False):
        c = t // NQ + 1
        q = t % NQ
        if spec_first:
            conv_spec(c, q)
        x4 = side2(t)
        xn2 = side1(t)
        xn1 = _ln(x_sc[seg(t + 1), :].astype(F32)).astype(BF16)
        un = conv_u(t + 2 * NQ)
        pins = list(zip(PINS, (un, xn1, x4, xn2)))
        never = never_sm[0] > 0
        if pre:
            h = pinned(never, jnp.concatenate([h_sc[0:M2, :], h_sc[RH:, :]], axis=0), pins)

            def proj(g):
                r = _dot(h(g), w_head(g)).astype(BF16)
                x1 = pre_rows(g, pl.multiple_of(M + t * (SEG // 2), 8), SEG)
                return jnp.concatenate([r[0:M2], x1, r[M2:]], axis=0)
            nterms = (NPRE - 1) // NQ + 2
        else:
            h = pinned(never, h_sc[...], pins)

            def proj(g):
                return _dot(h(g), w_head(g)).astype(BF16)
            nterms = NB
        h_sc[M2:RH, :] = xn1
        h_sc[RH:, :] = xn2

        def hook(it):
            if it == SPEC_AT and not spec_first:
                conv_spec(c, q)
            if it == SPEC_AT + 1:
                for piece in MAC_PIECES:
                    conv_mac(c, q, piece, nterms)
        out = attend(proj, R, mask12, hook)
        conv_inv(t)
        h_sc[0:M2, :] = out[0:M2].astype(BF16)
        op_sc[...] = out[M2:]

    def step_pre(t, carry):
        step(t, True)
        return carry

    def step_full(i, carry):
        for j in range(UNROLL):
            step(i * UNROLL + j, False, j > 0)
        return carry

    with jax.named_scope("steps_pre"):
        jax.lax.fori_loop(2, NPRE, step_pre, 0)

    def phase(p, carry):
        @pl.when(p == 1)
        def _():
            for cp in in_copies(2):
                cp.wait()

        @pl.when(p >= 2)
        def _():
            out_copy(p - 2).start()

        with jax.named_scope("steps"):
            jax.lax.fori_loop(jnp.maximum(p * PH, NPRE) // UNROLL, (p * PH + PH) // UNROLL, step_full, 0)
        return carry

    jax.lax.fori_loop(0, NPH, phase, 0)
    out_copy(NPH - 2).start()

    mask2 = make_mask(RH, (1,))

    def step_l2(t, carry):
        h = jnp.concatenate([h_sc[0:M2, :], h_sc[RH:, :]], axis=0)
        side2(t)
        xn2 = side1(t)
        out = attend(lambda g: _dot(h, w_head(g)).astype(BF16), RH, mask2)
        h_sc[0:M2, :] = out[0:M2].astype(BF16)
        h_sc[RH:, :] = xn2
        op_sc[SEG:, :] = out[M2:]
        return carry

    with jax.named_scope("steps_l2"):
        jax.lax.fori_loop(NSEG, NSEG + 2, step_l2, 0)
    side2(NSEG + 2)
    out_copy(NPH - 1).start()
    for i in range(NPH):
        out_copy(i).wait()


@functools.partial(jax.jit, static_argnames=("A_seg_len",))
def pallas_interleave_layers__memory_aug_recurrent_mem_tr__ssm_conv_h3__prompt_kernel(
    A_x, A_mem0, A_Wq, A_Wk, A_Wv, A_Wo, A_seg_len,
    B_q, B_k, B_v, B_shift_k, B_ssm_k, B_ssm_D,
):
    del B_q
    B, S, DM = A_x.shape
    assert B == 1
    H, DH = A_Wq.shape[1], A_Wq.shape[2]
    M = A_mem0.shape[1]
    SEG = int(A_seg_len)
    KS = B_shift_k.shape[1]
    R = 2 * (M + SEG)
    RP = 2 * M + NPRE * SEG
    NB = S // CB
    QB = CB // NQ
    fwd, inv = _dft_constants()

    kern = functools.partial(_kernel, S=S, DM=DM, H=H, DH=DH, M=M, SEG=SEG)
    any_spec = pl.BlockSpec(memory_space=pl.ANY)
    out = pl.pallas_call(
        kern,
        out_shape=jax.ShapeDtypeStruct((S, DM), A_x.dtype),
        in_specs=[any_spec] * 13,
        out_specs=any_spec,
        scratch_shapes=[
            pltpu.VMEM((M, DM), BF16),
            pltpu.VMEM((KS, DM), BF16),
            pltpu.VMEM((1, DM), BF16),
            pltpu.VMEM(fwd.shape, BF16),
            pltpu.VMEM(inv.shape, BF16),
            pltpu.VMEM((S, DM), BF16),
            pltpu.VMEM((S + KPAD, DM), BF16),
            pltpu.VMEM((S, DM), BF16),
            pltpu.VMEM((DM, S), BF16),
            pltpu.VMEM((6, DM, H // 2, DH), BF16),
            pltpu.VMEM((H * DH, DM), BF16),
            pltpu.VMEM((H * DH // 2, DM), U32),
            pltpu.VMEM((S, DM), A_x.dtype),
            pltpu.VMEM((H, DM // 2, 3 * DH), U32),
            pltpu.VMEM((RP, DM), BF16),
            pltpu.VMEM((H, RP // 2, 3 * DH), U32),
            pltpu.VMEM((R, DM), BF16),
            pltpu.VMEM((R // 2, H * DH), U32),
            pltpu.VMEM((2 * SEG, DM), F32),
            pltpu.VMEM((4, SEG, DM), F32),
            pltpu.VMEM((4, SEG, DM), F32),
            pltpu.VMEM((S, DM), BF16),
            pltpu.VMEM((NB + 2, NQ, QB // 8, DM // 128, 4, 8, 128), F32),
            pltpu.VMEM((NQ, 2 * QB, DM), F32),
            pltpu.VMEM((2, NQ, 2 * QB, DM), BF16),
            pltpu.SMEM((1,), jnp.int32),
            pltpu.SemaphoreType.DMA((5,)),
            pltpu.SemaphoreType.DMA((12,)),
            pltpu.SemaphoreType.DMA((7,)),
            pltpu.SemaphoreType.DMA((S // SEG // PH,)),
        ],
        compiler_params=pltpu.CompilerParams(vmem_limit_bytes=120 * 1024 * 1024),
    )(
        A_x.reshape(S, DM), A_mem0.reshape(M, DM), A_Wq, A_Wk, A_Wv,
        A_Wo.reshape(H * DH, DM), B_k.reshape(S, DM), B_v.reshape(S, DM),
        B_shift_k.T, B_ssm_k, B_ssm_D.reshape(1, DM),
        jnp.asarray(fwd, BF16), jnp.asarray(inv, BF16),
    )
    return out.reshape(B, S, DM)
```

```python
import functools

import numpy as np
import jax
import jax.numpy as jnp
import jax.experimental.pallas as pl
import jax.experimental.pallas.tpu as pltpu

F32 = jnp.float32
BF16 = jnp.bfloat16
U32 = jnp.uint32

CB = 128
NQ = 4
KPAD = 16
PH = 8
NPRE = 8
PINS = (3, 12, 16, 20)
SPEC_AT = 4
UNROLL = 2
D1, D2 = 1, 2


def _dft_constants():
    qb = CB // NQ
    n = np.arange(CB, dtype=np.float64)
    fwd = np.zeros((NQ, 2 * qb, CB))
    for q in range(NQ):
        f = q * qb + np.concatenate([np.arange(0, qb, 2), np.arange(1, qb, 2)])
        ang = (np.pi * (2.0 * f + 1.0) / (2 * CB))[:, None] * n[None, :]
        fwd[q, :qb] = np.cos(ang)
        fwd[q, qb:] = -np.sin(ang)
    inv = fwd.reshape(2 * CB, CB).T / CB
    return fwd.astype(np.float32), inv.reshape(NQ, CB // NQ, 2 * CB).astype(np.float32)


def _ln(x, eps=1e-5):
    d = x.shape[-1]
    m = jnp.sum(x, axis=-1, keepdims=True) * (1.0 / d)
    xc = x - m
    v = jnp.sum(xc * xc, axis=-1, keepdims=True) * (1.0 / d)
    return xc * jax.lax.rsqrt(v + eps)


def _dot(a, b):
    return jnp.dot(a, b, preferred_element_type=F32)


def _dot_nt(a, b):
    return jax.lax.dot_general(a, b, (((1,), (1,)), ((), ())), preferred_element_type=F32)


def _pack(x):
    return pltpu.bitcast(x.astype(BF16), U32)


def _unpack(x):
    return pltpu.bitcast(x, BF16)


def _in_order(actions):
    def body(i, c):
        for j, act in enumerate(actions):
            pl.when(i == j)(act)
        return c
    jax.lax.fori_loop(0, len(actions), body, 0)


def _kernel(x_hbm, mem0_hbm, wq_hbm, wk_hbm, wv_hbm, wo_hbm, k_hbm, v_hbm,
            sh_hbm, sk_hbm, sd_hbm, fwd_hbm, inv_hbm, o_hbm,
            sp_sc, kr_sc, wf_sc, x2_sc, y_sc, u_sc, op_sc, pre_sc, pre0_sc, wa_sc, wb_sc, wo_sc, o_sc,
            x_sc, v_sc, sk_sc, st_sc, wo_st, out_sc, fwd_ref, inv_ref,
            k_sc, hp_sc, h_sc, mem0_ref, sh_ref, sd_ref,
            never_sm, sem_s, sem_in, sem_w, sem_out,
            *, S, DM, H, DH, M, SEG):
    NSEG = S // SEG
    M2 = 2 * M
    R = M2 + 2 * SEG
    RH = M2 + SEG
    NB = S // CB
    QB = CB // NQ
    HB = QB // 2
    NT = DM // 128
    assert QB == SEG and NSEG % PH == 0 and 2 <= NPRE <= PH
    NPH = NSEG // PH
    HG = H // 2

    small = [pltpu.make_async_copy(s, d, sem_s.at[i]) for i, (s, d) in enumerate([
        (mem0_hbm, mem0_ref), (sh_hbm, sh_ref), (sd_hbm, sd_ref), (fwd_hbm, fwd_ref), (inv_hbm, inv_ref)])]

    xb = (0, NPRE * SEG, 2 * PH * SEG, S)
    kb = (0, (2 * NQ + 2) * SEG, 2 * PH * SEG, S)
    sb = (0, 2 * CB, 2 * PH * SEG, S)

    def in_copies(part):
        def rng(b):
            return pl.ds(b[part], b[part + 1] - b[part])
        return [
            pltpu.make_async_copy(x_hbm.at[rng(xb)], x_sc.at[rng(xb)], sem_in.at[part * 4]),
            pltpu.make_async_copy(k_hbm.at[rng(kb)],
                                  k_sc.at[pl.ds(KPAD + kb[part], kb[part + 1] - kb[part])],
                                  sem_in.at[part * 4 + 1]),
            pltpu.make_async_copy(v_hbm.at[rng(kb)], v_sc.at[rng(kb)], sem_in.at[part * 4 + 2]),
            pltpu.make_async_copy(sk_hbm.at[:, rng(sb)], sk_sc.at[:, rng(sb)], sem_in.at[part * 4 + 3]),
        ]

    def w_copy(ci):
        src = (wq_hbm, wk_hbm, wv_hbm)[ci % 3]
        return pltpu.make_async_copy(src.at[:, pl.ds((ci // 3) * HG, HG), :], st_sc.at[ci], sem_w.at[ci])

    wo_copy = pltpu.make_async_copy(wo_hbm, wo_st, sem_w.at[6])

    def out_copy(i):
        rows = pl.ds(pl.multiple_of(i * PH * SEG, PH * SEG), PH * SEG)
        return pltpu.make_async_copy(out_sc.at[rows], o_hbm.at[rows], sem_out.at[i])

    def start_all(cps):
        def act():
            for cp in cps:
                cp.start()
        return act

    _in_order([start_all(small + in_copies(0))]
              + [start_all([w_copy(ci)]) for ci in range(6)]
              + [start_all([wo_copy]), start_all(in_copies(1)), start_all(in_copies(2))])

    never_sm[0] = 0
    k_sc[0:KPAD, :] = jnp.zeros((KPAD, DM), BF16)
    sp_sc[NB + 1] = jnp.zeros(sp_sc.shape[1:], F32)
    op_sc[...] = jnp.zeros(op_sc.shape, F32)
    x2_sc[...] = jnp.zeros(x2_sc.shape, F32)
    y_sc[...] = jnp.zeros(y_sc.shape, F32)
    h_sc[...] = jnp.zeros(h_sc.shape, BF16)
    for cp in small + in_copies(0):
        cp.wait()

    sh = sh_ref[...].astype(F32)
    KS = sh.shape[0]
    sd = sd_ref[...].astype(F32)

    def seg(i):
        i = jnp.clip(i, 0, NSEG - 1)
        return pl.ds(pl.multiple_of(i * SEG, SEG), SEG)

    def conv_u(s):
        s = jnp.clip(s, 0, NSEG - 1)
        r0 = pl.multiple_of(s * SEG, SEG)
        kk = k_sc[pl.ds(r0, KPAD + SEG), :].astype(F32)
        ks = kk[KPAD:] * sh[0:1]
        for j in range(1, KS):
            ks = ks + pltpu.roll(kk, j, 0)[KPAD:] * sh[j:j + 1]
        u = (ks * v_sc[pl.ds(r0, SEG), :].astype(F32)).astype(BF16)
        u_sc[pl.ds(r0, SEG), :] = u
        return u

    def conv_fwd(c, q):
        cc = jnp.minimum(c, NB - 1)
        t0 = pl.multiple_of(cc * CB, CB)
        f = fwd_ref[q]
        uf = _dot(f, u_sc[pl.ds(t0, CB), :])
        kf = _dot_nt(f, sk_sc[:, pl.ds(t0, CB)])
        return uf, kf

    def put_spec(cs, q, which, val):
        for rb in range(QB // 8):
            for n in range(NT):
                ln = slice(n * 128, (n + 1) * 128)
                sp_sc[cs, q, rb, n, which] = val[rb * 8:rb * 8 + 8, ln]
                sp_sc[cs, q, rb, n, which + 1] = val[QB + rb * 8:QB + rb * 8 + 8, ln]

    def conv_spec(c, q):
        uf, kf = conv_fwd(c, q)
        cs = jnp.minimum(c, NB)
        put_spec(cs, q, 0, uf)
        pk = kr_sc[q]
        kr_sc[q] = kf
        kp = jnp.concatenate([
            kf[0:HB] - pk[QB:QB + HB],
            kf[HB:QB] + pk[QB + HB:],
            kf[QB:QB + HB] + pk[0:HB],
            kf[QB + HB:] - pk[HB:QB]], axis=0)
        put_spec(cs, q, 2, kp)

    MAC_PIECES = [(rb, n) for rb in range(QB // 16) for n in range(NT)]

    def conv_mac(c, q, piece, nterms):
        rb2, n = piece
        cs = jnp.minimum(c, NB)
        acc = []
        for rb in (2 * rb2, 2 * rb2 + 1):
            ar = None
            ai = None
            for j in range(nterms):
                uj = jnp.minimum(j, cs)
                kj = jnp.where(cs - j >= 0, cs - j, NB + 1)
                ur = sp_sc[uj, q, rb, n, 0]
                um = sp_sc[uj, q, rb, n, 1]
                kr = sp_sc[kj, q, rb, n, 2]
                km = sp_sc[kj, q, rb, n, 3]
                tr = ur * kr - um * km
                ti = ur * km + um * kr
                ar = tr if ar is None else ar + tr
                ai = ti if ai is None else ai + ti
            acc.append((ar, ai))
        ln = slice(n * 128, (n + 1) * 128)
        wf_sc[c & 1, q, rb2 * 16:rb2 * 16 + 16, ln] = jnp.concatenate(
            [acc[0][0], acc[1][0]], axis=0).astype(BF16)
        wf_sc[c & 1, q, QB + rb2 * 16:QB + rb2 * 16 + 16, ln] = jnp.concatenate(
            [acc[0][1], acc[1][1]], axis=0).astype(BF16)

    def conv_inv(s):
        w = wf_sc[(s // NQ) & 1].reshape(2 * CB, DM)
        yc = _dot(inv_ref[s % NQ], w)
        y_sc[s & 3] = yc + u_sc[seg(s), :].astype(F32) * sd

    scale = DH ** -0.5
    cexp = scale * float(np.log2(np.e))

    def make_mask(n, x_layers):
        qi = jax.lax.broadcasted_iota(jnp.int32, (n, n), 0)
        ki = jax.lax.broadcasted_iota(jnp.int32, (n, n), 1)

        def layer(i):
            xl = jnp.where(i < M2 + SEG, x_layers[0], x_layers[-1])
            return jnp.where(i < M, 0, jnp.where(i < M2, 1, xl))
        same = layer(qi) == layer(ki)
        ok = same & ((qi < M2) | (ki < M2) | (qi >= ki))
        fill = jnp.where(same, -1e9 / scale, -jnp.inf).astype(F32)
        return ok, fill

    def probs(qkv, mask):
        ok, fill = mask
        s = _dot_nt(qkv[:, 0:DH], qkv[:, DH:2 * DH])
        s = jnp.where(ok, s, fill)
        m = jnp.max(s, axis=-1, keepdims=True)
        p = jnp.exp2((s - m) * cexp)
        l = jnp.sum(p, axis=-1, keepdims=True)
        r = pl.reciprocal(l, approx=True)
        r = r * (2.0 - l * r)
        return (p * r).astype(BF16)

    def w_piece(ci, j):
        return (wa_sc, wb_sc)[ci % 2][ci // 2, j]

    def w_head(g):
        return _unpack(jnp.concatenate(
            [w_piece(3 * (g // HG) + mi, g % HG) for mi in range(3)], axis=1))

    def pre_rows(ref, half, j):
        return _unpack(jnp.concatenate([ref[3 * half + mi, j] for mi in range(3)], axis=1))

    def out_proj(n, g0, g1, j):
        return _dot(_unpack(o_sc[0:n // 2, g0 * DH:g1 * DH]),
                    _unpack(wo_sc[g0 * DH // 2:g1 * DH // 2, j * 128:(j + 1) * 128]))

    def attend(proj, n, mask, hook=None):
        HA = H - D1 - D2 - 1
        qkvs = {}
        ps = {}
        outs = {}
        for it in range(H + D1 + D2):
            if it < H:
                qkvs[it] = proj(it)
            g = it - D1
            if 0 <= g < H:
                ps[g] = probs(qkvs[g], mask)
            g = it - D1 - D2
            if 0 <= g < H:
                o = _dot(ps.pop(g), qkvs.pop(g)[:, 2 * DH:3 * DH])
                o_sc[0:n // 2, g * DH:(g + 1) * DH] = _pack(o)
            if hook is not None:
                hook(it)
            j = it - (H - 1)
            if 0 <= j < D1 + D2:
                outs[j] = out_proj(n, 0, HA, j)
        for j in range(D1 + D2, NT):
            outs[j] = out_proj(n, 0, H, j)
        for j in range(D1 + D2):
            outs[j] = out_proj(n, HA, H, j) + outs[j]
        return jnp.concatenate([outs[j] for j in range(NT)], axis=1)

    def side1(t):
        x1 = x_sc[seg(t - 1), :].astype(F32) + op_sc[0:SEG, :]
        x2 = x1 + _ln(x1) * y_sc[(t - 1) & 3]
        x2_sc[(t - 1) & 3] = x2
        return _ln(x2).astype(BF16)

    def side2(t):
        x3 = x2_sc[(t - 3) & 3] + op_sc[SEG:, :]
        x4 = x3 + _ln(x3) * y_sc[(t - 3) & 3]
        x4 = x4.astype(out_sc.dtype)
        out_sc[seg(t - 3), :] = x4
        return x4

    def pro_u(s, c):
        conv_u(s)
        return c
    jax.lax.fori_loop(0, 2 * NQ + 2, pro_u, 0)

    def pro_c(q, c):
        uf, kf = conv_fwd(0, q)
        put_spec(0, q, 0, uf)
        put_spec(0, q, 2, kf)
        kr_sc[q] = kf
        ur, um, kr, km = uf[:QB], uf[QB:], kf[:QB], kf[QB:]
        wf_sc[0, q, :QB] = (ur * kr - um * km).astype(BF16)
        wf_sc[0, q, QB:] = (ur * km + um * kr).astype(BF16)
        return c
    jax.lax.fori_loop(0, NQ, pro_c, 0)

    def pro_s(t, c):
        conv_spec(1, t)
        for piece in MAC_PIECES:
            conv_mac(1, t, piece, 2)
        conv_inv(t)
        return c
    jax.lax.fori_loop(0, 2, pro_s, 0)

    mem0 = mem0_ref[...].astype(F32)
    hp_sc[0:M, :] = _pack(jnp.concatenate([mem0, mem0], axis=0))

    def pro_h(s, c):
        xn = _ln(x_sc[seg(s), :].astype(F32))
        hp_sc[pl.ds(pl.multiple_of(M + jnp.maximum(s - 1, 0) * (SEG // 2), 8), SEG // 2), :] = _pack(xn)
        return c
    jax.lax.fori_loop(2, NPRE, pro_h, 0)
    pro_h(0, 0)
    h_sc[M2:RH, :] = _ln(x_sc[SEG:2 * SEG, :].astype(F32)).astype(BF16)

    mask1 = make_mask(RH, (0,))

    def wait_chunk(ci):
        with jax.named_scope("wait_w"):
            pltpu.make_async_copy(wq_hbm.at[:, pl.ds(0, HG), :], st_sc.at[ci], sem_w.at[ci]).wait()

    def relayout(ci, dst, slot, b):
        d0 = pl.multiple_of(b * 16, 16)
        r0 = pl.multiple_of(b * 8, 8)
        xw = pltpu.bitcast(st_sc[ci, pl.ds(d0, 16)], U32).reshape(8, 2, HG // 2, DH)
        a = xw[:, 0]
        bb = xw[:, 1]
        lo = jnp.swapaxes((a & U32(0xFFFF)) | (bb << 16), 0, 1)
        hi = jnp.swapaxes((a >> 16) | (bb & U32(0xFFFF0000)), 0, 1)
        for j in range(HG // 2):
            dst[slot, 2 * j, pl.ds(r0, 8), :] = lo[j]
            dst[slot, 2 * j + 1, pl.ds(r0, 8), :] = hi[j]

    NSUB = 2
    NBLK = DM // 16

    def fused(cr, dst, cp, src):
        def sub(i, c):
            hp = _unpack(hp_sc[...])
            nh = HG // NSUB
            nb = NBLK // NSUB
            for jj in range(nh):
                j = i * nh + jj
                r = _pack(_dot(hp, _unpack(src[cp // 2, j])))
                pre0_sc[cp, j] = r[0:RH // 2]
                for sg in range(NPRE - 2):
                    pre_sc[sg, cp, j] = r[(RH + sg * SEG) // 2:(RH + (sg + 1) * SEG) // 2]
                for bb in range(jj * nb // nh, (jj + 1) * nb // nh):
                    relayout(cr, dst, cr // 2, i * nb + bb)
            return c
        with jax.named_scope("fused"):
            jax.lax.fori_loop(0, NSUB, sub, 0)

    wait_chunk(0)

    def relayout0(b, c):
        relayout(0, wa_sc, 0, b)
        return c
    with jax.named_scope("relayout"):
        jax.lax.fori_loop(0, NBLK, relayout0, 0, unroll=2)

    def chunk_pair(k, carry):
        wait_chunk(2 * k + 1)
        fused(2 * k + 1, wb_sc, 2 * k, wa_sc)

        @pl.when(k < 2)
        def _():
            wait_chunk(2 * k + 2)
        fused(jnp.minimum(2 * k + 2, 4), wa_sc, 2 * k + 1, wb_sc)

        @pl.when(k >= 1)
        def _():
            g0 = (k - 1) * HG
            ps = {}
            for it in range(HG + 4):
                if it < HG:
                    ps[it] = probs(pre_rows(pre0_sc, k - 1, it), mask1)
                j = it - 4
                if j >= 0:
                    o = _dot(ps.pop(j), _unpack(pre0_sc[3 * (k - 1) + 2, j]))
                    o_sc[0:RH // 2, pl.ds(pl.multiple_of((g0 + j) * DH, DH), DH)] = _pack(o)
        return carry
    jax.lax.fori_loop(0, 3, chunk_pair, 0)

    with jax.named_scope("wait_wo"):
        wo_copy.wait()
    wo = wo_st[...]
    wo_sc[...] = _pack(wo)
    out = _dot(_unpack(o_sc[0:RH // 2, :]), wo)
    h_sc[0:M2, :] = jnp.concatenate([out[0:M], mem0], axis=0).astype(BF16)
    op_sc[0:SEG, :] = out[M2:]

    mask12 = make_mask(R, (0, 1))

    def pinned(never, h, pins):
        hs = {0: h}
        r = _pack(h[-SEG:])
        for g, d in pins:
            r = jnp.where(never, _pack(d), r)
            hs[g] = jnp.concatenate([h[:-SEG], _unpack(r)], axis=0)
        return lambda g: hs[max(k for k in hs if k <= g)]

    def step(t, pre, spec_first=False):
        c = t // NQ + 1
        q = t % NQ
        if spec_first:
            conv_spec(c, q)
        x4 = side2(t)
        xn2 = side1(t)
        xn1 = _ln(x_sc[seg(t + 1), :].astype(F32)).astype(BF16)
        un = conv_u(t + 2 * NQ)
        pins = list(zip(PINS, (un, xn1, x4, xn2)))
        never = never_sm[0] > 0
        if pre:
            h = pinned(never, jnp.concatenate([h_sc[0:M2, :], h_sc[RH:, :]], axis=0), pins)

            def proj(g):
                r = _dot(h(g), w_head(g)).astype(BF16)
                x1 = pre_rows(pre_sc.at[t - 2], g // HG, g % HG)
                return jnp.concatenate([r[0:M2], x1, r[M2:]], axis=0)
            nterms = (NPRE - 1) // NQ + 2
        else:
            h = pinned(never, h_sc[...], pins)

            def proj(g):
                return _dot(h(g), w_head(g)).astype(BF16)
            nterms = NB
        h_sc[M2:RH, :] = xn1
        h_sc[RH:, :] = xn2

        def hook(it):
            if it == SPEC_AT and not spec_first:
                conv_spec(c, q)
            if it == SPEC_AT + 1:
                for piece in MAC_PIECES:
                    conv_mac(c, q, piece, nterms)
        out = attend(proj, R, mask12, hook)
        conv_inv(t)
        h_sc[0:M2, :] = out[0:M2].astype(BF16)
        op_sc[...] = out[M2:]

    def step_pre(t, carry):
        step(t, True)
        return carry

    def step_full(i, carry):
        for j in range(UNROLL):
            step(i * UNROLL + j, False, j > 0)
        return carry

    def phase(p, carry):
        @pl.when(p == 1)
        def _():
            for cp in in_copies(2):
                cp.wait()

        @pl.when(p >= 2)
        def _():
            out_copy(p - 2).start()

        with jax.named_scope("steps"):
            jax.lax.fori_loop(jnp.maximum(p * PH, NPRE) // UNROLL, (p * PH + PH) // UNROLL, step_full, 0)
        return carry

    mask2 = make_mask(RH, (1,))

    def step_half(t, carry):
        first = t < NSEG
        lo = pl.multiple_of(jnp.where(first, 0, SEG), SEG)
        mask = (jnp.where(first, mask1[0].astype(jnp.int32), mask2[0].astype(jnp.int32)) > 0,
                jnp.where(first, mask1[1], mask2[1]))
        h = jnp.concatenate([h_sc[0:M2, :], h_sc[pl.ds(pl.multiple_of(M2 + lo, 16), SEG), :]], axis=0)
        side2(t)
        xn2 = side1(t)
        out = attend(lambda g: _dot(h, w_head(g)).astype(BF16), RH, mask)
        m2 = jnp.where(first, mem0, out[M:M2])
        h_sc[0:M2, :] = jnp.concatenate([out[0:M], m2], axis=0).astype(BF16)
        h_sc[RH:, :] = xn2
        op_sc[pl.ds(lo, SEG), :] = out[M2:]
        return carry

    def stage(i, carry):
        with jax.named_scope("steps_half"):
            jax.lax.fori_loop(jnp.where(i == 0, 1, NSEG), jnp.where(i == 0, 2, NSEG + 2), step_half, 0)

        @pl.when(i == 0)
        def _():
            for cp in in_copies(1):
                cp.wait()
            with jax.named_scope("steps_pre"):
                jax.lax.fori_loop(2, NPRE, step_pre, 0)
            jax.lax.fori_loop(0, NPH, phase, 0)
            out_copy(NPH - 2).start()
        return carry

    jax.lax.fori_loop(0, 2, stage, 0)
    side2(NSEG + 2)
    out_copy(NPH - 1).start()
    for i in range(NPH):
        out_copy(i).wait()


@functools.partial(jax.jit, static_argnames=("A_seg_len",))
def pallas_interleave_layers__memory_aug_recurrent_mem_tr__ssm_conv_h3__prompt_kernel(
    A_x, A_mem0, A_Wq, A_Wk, A_Wv, A_Wo, A_seg_len,
    B_q, B_k, B_v, B_shift_k, B_ssm_k, B_ssm_D,
):
    del B_q
    B, S, DM = A_x.shape
    assert B == 1
    H, DH = A_Wq.shape[1], A_Wq.shape[2]
    M = A_mem0.shape[1]
    SEG = int(A_seg_len)
    KS = B_shift_k.shape[1]
    R = 2 * (M + SEG)
    RP = 2 * M + (NPRE - 1) * SEG
    NB = S // CB
    QB = CB // NQ
    fwd, inv = _dft_constants()

    kern = functools.partial(_kernel, S=S, DM=DM, H=H, DH=DH, M=M, SEG=SEG)
    any_spec = pl.BlockSpec(memory_space=pl.ANY)
    out = pl.pallas_call(
        kern,
        out_shape=jax.ShapeDtypeStruct((S, DM), A_x.dtype),
        in_specs=[any_spec] * 13,
        out_specs=any_spec,
        scratch_shapes=[
            pltpu.VMEM((NB + 2, NQ, QB // 8, DM // 128, 4, 8, 128), F32),
            pltpu.VMEM((NQ, 2 * QB, DM), F32),
            pltpu.VMEM((2, NQ, 2 * QB, DM), BF16),
            pltpu.VMEM((4, SEG, DM), F32),
            pltpu.VMEM((4, SEG, DM), F32),
            pltpu.VMEM((S, DM), BF16),
            pltpu.VMEM((2 * SEG, DM), F32),
            pltpu.VMEM((NPRE - 2, 6, H // 2, SEG // 2, DH), U32),
            pltpu.VMEM((6, H // 2, M + SEG // 2, DH), U32),
            pltpu.VMEM((3, H // 2, DM // 2, DH), U32),
            pltpu.VMEM((3, H // 2, DM // 2, DH), U32),
            pltpu.VMEM((H * DH // 2, DM), U32),
            pltpu.VMEM((R // 2, H * DH), U32),
            pltpu.VMEM((S, DM), BF16),
            pltpu.VMEM((S, DM), BF16),
            pltpu.VMEM((DM, S), BF16),
            pltpu.VMEM((6, DM, H // 2, DH), BF16),
            pltpu.VMEM((H * DH, DM), BF16),
            pltpu.VMEM((S, DM), A_x.dtype),
            pltpu.VMEM(fwd.shape, BF16),
            pltpu.VMEM(inv.shape, BF16),
            pltpu.VMEM((S + KPAD, DM), BF16),
            pltpu.VMEM((RP // 2, DM), U32),
            pltpu.VMEM((R, DM), BF16),
            pltpu.VMEM((M, DM), BF16),
            pltpu.VMEM((KS, DM), BF16),
            pltpu.VMEM((1, DM), BF16),
            pltpu.SMEM((1,), jnp.int32),
            pltpu.SemaphoreType.DMA((5,)),
            pltpu.SemaphoreType.DMA((12,)),
            pltpu.SemaphoreType.DMA((7,)),
            pltpu.SemaphoreType.DMA((S // SEG // PH,)),
        ],
        compiler_params=pltpu.CompilerParams(vmem_limit_bytes=120 * 1024 * 1024),
    )(
        A_x.reshape(S, DM), A_mem0.reshape(M, DM), A_Wq, A_Wk, A_Wv,
        A_Wo.reshape(H * DH, DM), B_k.reshape(S, DM), B_v.reshape(S, DM),
        B_shift_k.T, B_ssm_k, B_ssm_D.reshape(1, DM),
        jnp.asarray(fwd, BF16), jnp.asarray(inv, BF16),
    )
    return out.reshape(B, S, DM)
```

```python
import functools

import numpy as np
import jax
import jax.numpy as jnp
import jax.experimental.pallas as pl
import jax.experimental.pallas.tpu as pltpu

F32 = jnp.float32
BF16 = jnp.bfloat16
U32 = jnp.uint32

CB = 128
NQ = 4
KPAD = 16
PH = 8
NPRE = 8
PINS = (3, 12, 16, 20)
SPEC_AT = 4
UNROLL = 2
NSUB = 1
D1, D2 = 1, 2


def _dft_constants():
    qb = CB // NQ
    n = np.arange(CB, dtype=np.float64)
    fwd = np.zeros((NQ, 2 * qb, CB))
    for q in range(NQ):
        f = q * qb + np.concatenate([np.arange(0, qb, 2), np.arange(1, qb, 2)])
        ang = (np.pi * (2.0 * f + 1.0) / (2 * CB))[:, None] * n[None, :]
        fwd[q, :qb] = np.cos(ang)
        fwd[q, qb:] = -np.sin(ang)
    inv = fwd.reshape(2 * CB, CB).T / CB
    return fwd.astype(np.float32), inv.reshape(NQ, CB // NQ, 2 * CB).astype(np.float32)


def _ln(x, eps=1e-5):
    d = x.shape[-1]
    m = jnp.sum(x, axis=-1, keepdims=True) * (1.0 / d)
    xc = x - m
    v = jnp.sum(xc * xc, axis=-1, keepdims=True) * (1.0 / d)
    return xc * jax.lax.rsqrt(v + eps)


def _dot(a, b):
    return jnp.dot(a, b, preferred_element_type=F32)


def _dot_nt(a, b):
    return jax.lax.dot_general(a, b, (((1,), (1,)), ((), ())), preferred_element_type=F32)


def _pack(x):
    return pltpu.bitcast(x.astype(BF16), U32)


def _unpack(x):
    return pltpu.bitcast(x, BF16)


def _in_order(actions):
    def body(i, c):
        for j, act in enumerate(actions):
            pl.when(i == j)(act)
        return c
    jax.lax.fori_loop(0, len(actions), body, 0)


def _kernel(x_hbm, mem0_hbm, wq_hbm, wk_hbm, wv_hbm, wo_hbm, k_hbm, v_hbm,
            sh_hbm, sk_hbm, sd_hbm, fwd_hbm, inv_hbm, o_hbm,
            sp_sc, kr_sc, wf_sc, x2_sc, y_sc, u_sc, op_sc, pre_sc, pre0_sc, wa_sc, wb_sc, wo_sc, o_sc,
            x_sc, v_sc, sk_sc, st_sc, wo_st, out_sc, fwd_ref, inv_ref,
            k_sc, hp_sc, h_sc, mem0_ref, sh_ref, sd_ref,
            never_sm, sem_s, sem_in, sem_w, sem_out,
            *, S, DM, H, DH, M, SEG):
    NSEG = S // SEG
    M2 = 2 * M
    R = M2 + 2 * SEG
    RH = M2 + SEG
    NB = S // CB
    QB = CB // NQ
    HB = QB // 2
    NT = DM // 128
    assert QB == SEG and NSEG % PH == 0 and 2 <= NPRE <= PH
    NPH = NSEG // PH
    HG = H // 2

    small = [pltpu.make_async_copy(s, d, sem_s.at[i]) for i, (s, d) in enumerate([
        (mem0_hbm, mem0_ref), (sh_hbm, sh_ref), (sd_hbm, sd_ref), (fwd_hbm, fwd_ref), (inv_hbm, inv_ref)])]

    xb = (0, NPRE * SEG, 2 * PH * SEG, S)
    kb = (0, (2 * NQ + 2) * SEG, 2 * PH * SEG, S)
    sb = (0, 2 * CB, 2 * PH * SEG, S)

    def in_copies(part):
        def rng(b):
            return pl.ds(b[part], b[part + 1] - b[part])
        return [
            pltpu.make_async_copy(x_hbm.at[rng(xb)], x_sc.at[rng(xb)], sem_in.at[part * 4]),
            pltpu.make_async_copy(k_hbm.at[rng(kb)],
                                  k_sc.at[pl.ds(KPAD + kb[part], kb[part + 1] - kb[part])],
                                  sem_in.at[part * 4 + 1]),
            pltpu.make_async_copy(v_hbm.at[rng(kb)], v_sc.at[rng(kb)], sem_in.at[part * 4 + 2]),
            pltpu.make_async_copy(sk_hbm.at[:, rng(sb)], sk_sc.at[:, rng(sb)], sem_in.at[part * 4 + 3]),
        ]

    def w_copy(ci):
        src = (wq_hbm, wk_hbm, wv_hbm)[ci % 3]
        return pltpu.make_async_copy(src.at[:, pl.ds((ci // 3) * HG, HG), :], st_sc.at[ci], sem_w.at[ci])

    wo_copy = pltpu.make_async_copy(wo_hbm, wo_st, sem_w.at[6])

    def out_copy(i):
        rows = pl.ds(pl.multiple_of(i * PH * SEG, PH * SEG), PH * SEG)
        return pltpu.make_async_copy(out_sc.at[rows], o_hbm.at[rows], sem_out.at[i])

    def start_all(cps):
        def act():
            for cp in cps:
                cp.start()
        return act

    _in_order([start_all(small + in_copies(0))]
              + [start_all([w_copy(ci)]) for ci in range(6)]
              + [start_all([wo_copy]), start_all(in_copies(1)), start_all(in_copies(2))])

    never_sm[0] = 0
    k_sc[0:KPAD, :] = jnp.zeros((KPAD, DM), BF16)
    sp_sc[NB + 1] = jnp.zeros(sp_sc.shape[1:], F32)
    op_sc[...] = jnp.zeros(op_sc.shape, F32)
    x2_sc[...] = jnp.zeros(x2_sc.shape, F32)
    y_sc[...] = jnp.zeros(y_sc.shape, F32)
    h_sc[...] = jnp.zeros(h_sc.shape, BF16)
    for cp in small + in_copies(0):
        cp.wait()

    sh = sh_ref[...].astype(F32)
    KS = sh.shape[0]
    sd = sd_ref[...].astype(F32)

    def seg(i):
        i = jnp.clip(i, 0, NSEG - 1)
        return pl.ds(pl.multiple_of(i * SEG, SEG), SEG)

    def conv_u(s):
        s = jnp.clip(s, 0, NSEG - 1)
        r0 = pl.multiple_of(s * SEG, SEG)
        kk = k_sc[pl.ds(r0, KPAD + SEG), :].astype(F32)
        ks = kk[KPAD:] * sh[0:1]
        for j in range(1, KS):
            ks = ks + pltpu.roll(kk, j, 0)[KPAD:] * sh[j:j + 1]
        u = (ks * v_sc[pl.ds(r0, SEG), :].astype(F32)).astype(BF16)
        u_sc[pl.ds(r0, SEG), :] = u
        return u

    def conv_fwd(c, q):
        cc = jnp.minimum(c, NB - 1)
        t0 = pl.multiple_of(cc * CB, CB)
        f = fwd_ref[q]
        uf = _dot(f, u_sc[pl.ds(t0, CB), :])
        kf = _dot_nt(f, sk_sc[:, pl.ds(t0, CB)])
        return uf, kf

    def put_spec(cs, q, which, val):
        for rb in range(QB // 8):
            for n in range(NT):
                ln = slice(n * 128, (n + 1) * 128)
                sp_sc[cs, q, rb, n, which] = val[rb * 8:rb * 8 + 8, ln]
                sp_sc[cs, q, rb, n, which + 1] = val[QB + rb * 8:QB + rb * 8 + 8, ln]

    def conv_spec(c, q):
        uf, kf = conv_fwd(c, q)
        cs = jnp.minimum(c, NB)
        put_spec(cs, q, 0, uf)
        pk = kr_sc[q]
        kr_sc[q] = kf
        kp = jnp.concatenate([
            kf[0:HB] - pk[QB:QB + HB],
            kf[HB:QB] + pk[QB + HB:],
            kf[QB:QB + HB] + pk[0:HB],
            kf[QB + HB:] - pk[HB:QB]], axis=0)
        put_spec(cs, q, 2, kp)

    MAC_PIECES = [(rb, n) for rb in range(QB // 16) for n in range(NT)]

    def conv_mac(c, q, piece, nterms):
        rb2, n = piece
        cs = jnp.minimum(c, NB)
        acc = []
        for rb in (2 * rb2, 2 * rb2 + 1):
            ar = None
            ai = None
            for j in range(nterms):
                uj = jnp.minimum(j, cs)
                kj = jnp.where(cs - j >= 0, cs - j, NB + 1)
                ur = sp_sc[uj, q, rb, n, 0]
                um = sp_sc[uj, q, rb, n, 1]
                kr = sp_sc[kj, q, rb, n, 2]
                km = sp_sc[kj, q, rb, n, 3]
                tr = ur * kr - um * km
                ti = ur * km + um * kr
                ar = tr if ar is None else ar + tr
                ai = ti if ai is None else ai + ti
            acc.append((ar, ai))
        ln = slice(n * 128, (n + 1) * 128)
        wf_sc[c & 1, q, rb2 * 16:rb2 * 16 + 16, ln] = jnp.concatenate(
            [acc[0][0], acc[1][0]], axis=0).astype(BF16)
        wf_sc[c & 1, q, QB + rb2 * 16:QB + rb2 * 16 + 16, ln] = jnp.concatenate(
            [acc[0][1], acc[1][1]], axis=0).astype(BF16)

    def conv_inv(s):
        w = wf_sc[(s // NQ) & 1].reshape(2 * CB, DM)
        yc = _dot(inv_ref[s % NQ], w)
        y_sc[s & 3] = yc + u_sc[seg(s), :].astype(F32) * sd

    scale = DH ** -0.5
    cexp = scale * float(np.log2(np.e))

    def make_mask(n, x_layers):
        qi = jax.lax.broadcasted_iota(jnp.int32, (n, n), 0)
        ki = jax.lax.broadcasted_iota(jnp.int32, (n, n), 1)

        def layer(i):
            xl = jnp.where(i < M2 + SEG, x_layers[0], x_layers[-1])
            return jnp.where(i < M, 0, jnp.where(i < M2, 1, xl))
        same = layer(qi) == layer(ki)
        ok = same & ((qi < M2) | (ki < M2) | (qi >= ki))
        fill = jnp.where(same, -1e9 / scale, -jnp.inf).astype(F32)
        return ok, fill

    def probs(qkv, mask):
        ok, fill = mask
        s = _dot_nt(qkv[:, 0:DH], qkv[:, DH:2 * DH])
        s = jnp.where(ok, s, fill)
        m = jnp.max(s, axis=-1, keepdims=True)
        p = jnp.exp2((s - m) * cexp)
        l = jnp.sum(p, axis=-1, keepdims=True)
        r = pl.reciprocal(l, approx=True)
        r = r * (2.0 - l * r)
        return (p * r).astype(BF16)

    def w_piece(ci, j):
        return (wa_sc, wb_sc)[ci % 2][ci // 2, j]

    def w_head(g):
        return _unpack(jnp.concatenate(
            [w_piece(3 * (g // HG) + mi, g % HG) for mi in range(3)], axis=1))

    def pre_rows(ref, half, j):
        return _unpack(jnp.concatenate([ref[3 * half + mi, j] for mi in range(3)], axis=1))

    def out_proj(n, g0, g1, j):
        return _dot(_unpack(o_sc[0:n // 2, g0 * DH:g1 * DH]),
                    _unpack(wo_sc[g0 * DH // 2:g1 * DH // 2, j * 128:(j + 1) * 128]))

    def attend(proj, n, mask, hook=None):
        HA = H - D1 - D2 - 1
        qkvs = {}
        ps = {}
        outs = {}
        for it in range(H + D1 + D2):
            if it < H:
                qkvs[it] = proj(it)
            g = it - D1
            if 0 <= g < H:
                ps[g] = probs(qkvs[g], mask)
            g = it - D1 - D2
            if 0 <= g < H:
                o = _dot(ps.pop(g), qkvs.pop(g)[:, 2 * DH:3 * DH])
                o_sc[0:n // 2, g * DH:(g + 1) * DH] = _pack(o)
            if hook is not None:
                hook(it)
            j = it - (H - 1)
            if 0 <= j < D1 + D2:
                outs[j] = out_proj(n, 0, HA, j)
        for j in range(D1 + D2, NT):
            outs[j] = out_proj(n, 0, H, j)
        for j in range(D1 + D2):
            outs[j] = out_proj(n, HA, H, j) + outs[j]
        return jnp.concatenate([outs[j] for j in range(NT)], axis=1)

    def side1(t):
        x1 = x_sc[seg(t - 1), :].astype(F32) + op_sc[0:SEG, :]
        x2 = x1 + _ln(x1) * y_sc[(t - 1) & 3]
        x2_sc[(t - 1) & 3] = x2
        return _ln(x2).astype(BF16)

    def side2(t):
        x3 = x2_sc[(t - 3) & 3] + op_sc[SEG:, :]
        x4 = x3 + _ln(x3) * y_sc[(t - 3) & 3]
        x4 = x4.astype(out_sc.dtype)
        out_sc[seg(t - 3), :] = x4
        return x4

    def pro_u(s, c):
        conv_u(s)
        return c
    jax.lax.fori_loop(0, 2 * NQ + 2, pro_u, 0)

    def pro_c(q, c):
        uf, kf = conv_fwd(0, q)
        put_spec(0, q, 0, uf)
        put_spec(0, q, 2, kf)
        kr_sc[q] = kf
        ur, um, kr, km = uf[:QB], uf[QB:], kf[:QB], kf[QB:]
        wf_sc[0, q, :QB] = (ur * kr - um * km).astype(BF16)
        wf_sc[0, q, QB:] = (ur * km + um * kr).astype(BF16)
        return c
    jax.lax.fori_loop(0, NQ, pro_c, 0)

    def pro_s(t, c):
        conv_spec(1, t)
        for piece in MAC_PIECES:
            conv_mac(1, t, piece, 2)
        conv_inv(t)
        return c
    jax.lax.fori_loop(0, 2, pro_s, 0)

    mem0 = mem0_ref[...].astype(F32)
    hp_sc[0:M, :] = _pack(jnp.concatenate([mem0, mem0], axis=0))

    def pro_h(s, c):
        xn = _ln(x_sc[seg(s), :].astype(F32))
        hp_sc[pl.ds(pl.multiple_of(M + jnp.maximum(s - 1, 0) * (SEG // 2), 8), SEG // 2), :] = _pack(xn)
        return c
    jax.lax.fori_loop(2, NPRE, pro_h, 0)
    pro_h(0, 0)
    h_sc[M2:RH, :] = _ln(x_sc[SEG:2 * SEG, :].astype(F32)).astype(BF16)

    mask1 = make_mask(RH, (0,))

    def wait_chunk(ci):
        with jax.named_scope("wait_w"):
            pltpu.make_async_copy(wq_hbm.at[:, pl.ds(0, HG), :], st_sc.at[ci], sem_w.at[ci]).wait()

    def relayout(ci, dst, slot, b):
        d0 = b * 16 if isinstance(b, int) else pl.multiple_of(b * 16, 16)
        r0 = b * 8 if isinstance(b, int) else pl.multiple_of(b * 8, 8)
        xw = pltpu.bitcast(st_sc[ci, pl.ds(d0, 16)], U32).reshape(8, 2, HG // 2, DH)
        a = xw[:, 0]
        bb = xw[:, 1]
        lo = jnp.swapaxes((a & U32(0xFFFF)) | (bb << 16), 0, 1)
        hi = jnp.swapaxes((a >> 16) | (bb & U32(0xFFFF0000)), 0, 1)
        for j in range(HG // 2):
            dst[slot, 2 * j, pl.ds(r0, 8), :] = lo[j]
            dst[slot, 2 * j + 1, pl.ds(r0, 8), :] = hi[j]

    NBLK = DM // 16

    def fused(cr, dst, rslot, cp, src, pslot):
        S2 = SEG // 2
        cuts = [0, RH // 2 + S2, RH // 2 + 3 * S2, RH // 2 + (NPRE - 2) * S2]
        npc = len(cuts) - 1

        def sub(i, c):
            nh = HG // NSUB
            nb = NBLK // NSUB
            done = 0
            for jj in range(nh):
                j = i * nh + jj
                w = _unpack(src[pslot, j])
                for pi in range(npc):
                    upto = min(nb, -(-(jj * npc + pi + 1) * nb // (nh * npc - 2)))
                    for bb in range(done, upto):
                        relayout(cr, dst, rslot, i * nb + bb)
                    done = upto
                    lo, hi = cuts[pi], cuts[pi + 1]
                    r = _pack(_dot(_unpack(hp_sc[lo:hi, :]), w))
                    if pi == 0:
                        pre0_sc[cp, j] = r[0:RH // 2]
                    for sg in range(NPRE - 2):
                        a = RH // 2 + sg * S2
                        if lo <= a < hi:
                            pre_sc[sg, cp, j] = r[a - lo:a - lo + S2]
            return c
        with jax.named_scope("fused"):
            if NSUB == 1:
                jax.lax.fori_loop(0, never_sm[0] + 1, lambda i, c: sub(0, c), 0)
            else:
                jax.lax.fori_loop(0, NSUB, sub, 0)

    wait_chunk(0)

    def relayout0(b, c):
        relayout(0, wa_sc, 0, b)
        return c
    with jax.named_scope("relayout"):
        jax.lax.fori_loop(0, NBLK, relayout0, 0, unroll=2)

    def chunk_pair(k, carry):
        wait_chunk(2 * k + 1)
        kc = jnp.minimum(k + never_sm[0], 2)
        fused(2 * kc + 1, wb_sc, kc, 2 * k, wa_sc, k)

        @pl.when(k < 2)
        def _():
            wait_chunk(2 * k + 2)
        kn = jnp.minimum(k + 1, 2)
        fused(2 * kn, wa_sc, kn, 2 * k + 1, wb_sc, k)

        @pl.when(k >= 1)
        def _():
            g0 = (k - 1) * HG
            ps = {}
            for it in range(HG + 4):
                if it < HG:
                    ps[it] = probs(pre_rows(pre0_sc, k - 1, it), mask1)
                j = it - 4
                if j >= 0:
                    o = _dot(ps.pop(j), _unpack(pre0_sc[3 * (k - 1) + 2, j]))
                    o_sc[0:RH // 2, pl.ds(pl.multiple_of((g0 + j) * DH, DH), DH)] = _pack(o)
        return carry
    jax.lax.fori_loop(0, 3, chunk_pair, 0)

    with jax.named_scope("wait_wo"):
        wo_copy.wait()
    wo = wo_st[...]
    wo_sc[...] = _pack(wo)
    out = _dot(_unpack(o_sc[0:RH // 2, :]), wo)
    h_sc[0:M2, :] = jnp.concatenate([out[0:M], mem0], axis=0).astype(BF16)
    op_sc[0:SEG, :] = out[M2:]

    mask12 = make_mask(R, (0, 1))

    def pinned(never, h, pins):
        hs = {0: h}
        r = _pack(h[-SEG:])
        for g, d in pins:
            r = jnp.where(never, _pack(d), r)
            hs[g] = jnp.concatenate([h[:-SEG], _unpack(r)], axis=0)
        return lambda g: hs[max(k for k in hs if k <= g)]

    def step(t, pre, spec_first=False):
        c = t // NQ + 1
        q = t % NQ
        if spec_first:
            conv_spec(c, q)
        x4 = side2(t)
        xn2 = side1(t)
        xn1 = _ln(x_sc[seg(t + 1), :].astype(F32)).astype(BF16)
        un = conv_u(t + 2 * NQ)
        pins = list(zip(PINS, (un, xn1, x4, xn2)))
        never = never_sm[0] > 0
        if pre:
            h = pinned(never, jnp.concatenate([h_sc[0:M2, :], h_sc[RH:, :]], axis=0), pins)

            def proj(g):
                r = _dot(h(g), w_head(g)).astype(BF16)
                x1 = pre_rows(pre_sc.at[t - 2], g // HG, g % HG)
                return jnp.concatenate([r[0:M2], x1, r[M2:]], axis=0)
            nterms = (NPRE - 1) // NQ + 2
        else:
            h = pinned(never, h_sc[...], pins)

            def proj(g):
                return _dot(h(g), w_head(g)).astype(BF16)
            nterms = NB
        h_sc[M2:RH, :] = xn1
        h_sc[RH:, :] = xn2

        def hook(it):
            if it == SPEC_AT and not spec_first:
                conv_spec(c, q)
            if it == SPEC_AT + 1:
                for piece in MAC_PIECES:
                    conv_mac(c, q, piece, nterms)
        out = attend(proj, R, mask12, hook)
        conv_inv(t)
        h_sc[0:M2, :] = out[0:M2].astype(BF16)
        op_sc[...] = out[M2:]

    def step_pre(t, carry):
        step(t, True)
        return carry

    def step_full(i, carry):
        for j in range(UNROLL):
            step(i * UNROLL + j, False, j > 0)
        return carry

    def phase(p, carry):
        @pl.when(p == 1)
        def _():
            for cp in in_copies(2):
                cp.wait()

        @pl.when(p >= 2)
        def _():
            out_copy(p - 2).start()

        with jax.named_scope("steps"):
            jax.lax.fori_loop(jnp.maximum(p * PH, NPRE) // UNROLL, (p * PH + PH) // UNROLL, step_full, 0)
        return carry

    mask2 = make_mask(RH, (1,))

    def step_half(t, carry):
        first = t < NSEG
        lo = pl.multiple_of(jnp.where(first, 0, SEG), SEG)
        mask = (jnp.where(first, mask1[0].astype(jnp.int32), mask2[0].astype(jnp.int32)) > 0,
                jnp.where(first, mask1[1], mask2[1]))
        h = jnp.concatenate([h_sc[0:M2, :], h_sc[pl.ds(pl.multiple_of(M2 + lo, 16), SEG), :]], axis=0)
        side2(t)
        xn2 = side1(t)
        out = attend(lambda g: _dot(h, w_head(g)).astype(BF16), RH, mask)
        m2 = jnp.where(first, mem0, out[M:M2])
        h_sc[0:M2, :] = jnp.concatenate([out[0:M], m2], axis=0).astype(BF16)
        h_sc[RH:, :] = xn2
        op_sc[pl.ds(lo, SEG), :] = out[M2:]
        return carry

    def stage(i, carry):
        with jax.named_scope("steps_half"):
            jax.lax.fori_loop(jnp.where(i == 0, 1, NSEG), jnp.where(i == 0, 2, NSEG + 2), step_half, 0)

        @pl.when(i == 0)
        def _():
            for cp in in_copies(1):
                cp.wait()
            with jax.named_scope("steps_pre"):
                jax.lax.fori_loop(2, NPRE, step_pre, 0)
            jax.lax.fori_loop(0, NPH, phase, 0)
            out_copy(NPH - 2).start()
        return carry

    jax.lax.fori_loop(0, 2, stage, 0)
    side2(NSEG + 2)
    out_copy(NPH - 1).start()
    for i in range(NPH):
        out_copy(i).wait()


@functools.partial(jax.jit, static_argnames=("A_seg_len",))
def pallas_interleave_layers__memory_aug_recurrent_mem_tr__ssm_conv_h3__prompt_kernel(
    A_x, A_mem0, A_Wq, A_Wk, A_Wv, A_Wo, A_seg_len,
    B_q, B_k, B_v, B_shift_k, B_ssm_k, B_ssm_D,
):
    del B_q
    B, S, DM = A_x.shape
    assert B == 1
    H, DH = A_Wq.shape[1], A_Wq.shape[2]
    M = A_mem0.shape[1]
    SEG = int(A_seg_len)
    KS = B_shift_k.shape[1]
    R = 2 * (M + SEG)
    RP = 2 * M + (NPRE - 1) * SEG
    NB = S // CB
    QB = CB // NQ
    fwd, inv = _dft_constants()

    kern = functools.partial(_kernel, S=S, DM=DM, H=H, DH=DH, M=M, SEG=SEG)
    any_spec = pl.BlockSpec(memory_space=pl.ANY)
    out = pl.pallas_call(
        kern,
        out_shape=jax.ShapeDtypeStruct((S, DM), A_x.dtype),
        in_specs=[any_spec] * 13,
        out_specs=any_spec,
        scratch_shapes=[
            pltpu.VMEM((NB + 2, NQ, QB // 8, DM // 128, 4, 8, 128), F32),
            pltpu.VMEM((NQ, 2 * QB, DM), F32),
            pltpu.VMEM((2, NQ, 2 * QB, DM), BF16),
            pltpu.VMEM((4, SEG, DM), F32),
            pltpu.VMEM((4, SEG, DM), F32),
            pltpu.VMEM((S, DM), BF16),
            pltpu.VMEM((2 * SEG, DM), F32),
            pltpu.VMEM((NPRE - 2, 6, H // 2, SEG // 2, DH), U32),
            pltpu.VMEM((6, H // 2, M + SEG // 2, DH), U32),
            pltpu.VMEM((3, H // 2, DM // 2, DH), U32),
            pltpu.VMEM((3, H // 2, DM // 2, DH), U32),
            pltpu.VMEM((H * DH // 2, DM), U32),
            pltpu.VMEM((R // 2, H * DH), U32),
            pltpu.VMEM((S, DM), BF16),
            pltpu.VMEM((S, DM), BF16),
            pltpu.VMEM((DM, S), BF16),
            pltpu.VMEM((6, DM, H // 2, DH), BF16),
            pltpu.VMEM((H * DH, DM), BF16),
            pltpu.VMEM((S, DM), A_x.dtype),
            pltpu.VMEM(fwd.shape, BF16),
            pltpu.VMEM(inv.shape, BF16),
            pltpu.VMEM((S + KPAD, DM), BF16),
            pltpu.VMEM((RP // 2, DM), U32),
            pltpu.VMEM((R, DM), BF16),
            pltpu.VMEM((M, DM), BF16),
            pltpu.VMEM((KS, DM), BF16),
            pltpu.VMEM((1, DM), BF16),
            pltpu.SMEM((1,), jnp.int32),
            pltpu.SemaphoreType.DMA((5,)),
            pltpu.SemaphoreType.DMA((12,)),
            pltpu.SemaphoreType.DMA((7,)),
            pltpu.SemaphoreType.DMA((S // SEG // PH,)),
        ],
        compiler_params=pltpu.CompilerParams(vmem_limit_bytes=120 * 1024 * 1024),
    )(
        A_x.reshape(S, DM), A_mem0.reshape(M, DM), A_Wq, A_Wk, A_Wv,
        A_Wo.reshape(H * DH, DM), B_k.reshape(S, DM), B_v.reshape(S, DM),
        B_shift_k.T, B_ssm_k, B_ssm_D.reshape(1, DM),
        jnp.asarray(fwd, BF16), jnp.asarray(inv, BF16),
    )
    return out.reshape(B, S, DM)
```

```python
import functools

import numpy as np
import jax
import jax.numpy as jnp
import jax.experimental.pallas as pl
import jax.experimental.pallas.tpu as pltpu

F32 = jnp.float32
BF16 = jnp.bfloat16
U32 = jnp.uint32

CB = 128
NQ = 4
KPAD = 16
PH = 8
NPRE = 8
PINS = (3, 12, 16, 20)
SPEC_AT = 4
UNROLL = 2
NSUB = 1
DIST, DIST_PRE, DIST_HALF = (1, 2), (2, 3), (1, 3)


def _dft_constants():
    qb = CB // NQ
    n = np.arange(CB, dtype=np.float64)
    fwd = np.zeros((NQ, 2 * qb, CB))
    for q in range(NQ):
        f = q * qb + np.concatenate([np.arange(0, qb, 2), np.arange(1, qb, 2)])
        ang = (np.pi * (2.0 * f + 1.0) / (2 * CB))[:, None] * n[None, :]
        fwd[q, :qb] = np.cos(ang)
        fwd[q, qb:] = -np.sin(ang)
    inv = fwd.reshape(2 * CB, CB).T / CB
    return fwd.astype(np.float32), inv.reshape(NQ, CB // NQ, 2 * CB).astype(np.float32)


def _ln(x, eps=1e-5):
    d = x.shape[-1]
    m = jnp.sum(x, axis=-1, keepdims=True) * (1.0 / d)
    xc = x - m
    v = jnp.sum(xc * xc, axis=-1, keepdims=True) * (1.0 / d)
    return xc * jax.lax.rsqrt(v + eps)


def _dot(a, b):
    return jnp.dot(a, b, preferred_element_type=F32)


def _dot_nt(a, b):
    return jax.lax.dot_general(a, b, (((1,), (1,)), ((), ())), preferred_element_type=F32)


def _pack(x):
    return pltpu.bitcast(x.astype(BF16), U32)


def _unpack(x):
    return pltpu.bitcast(x, BF16)


def _in_order(actions):
    def body(i, c):
        for j, act in enumerate(actions):
            pl.when(i == j)(act)
        return c
    jax.lax.fori_loop(0, len(actions), body, 0)


def _kernel(x_hbm, mem0_hbm, wq_hbm, wk_hbm, wv_hbm, wo_hbm, k_hbm, v_hbm,
            sh_hbm, sk_hbm, sd_hbm, fwd_hbm, inv_hbm, o_hbm,
            sp_sc, kr_sc, wf_sc, x2_sc, y_sc, u_sc, op_sc, pre_sc, pre0_sc, wa_sc, wb_sc, wo_sc, o_sc,
            x_sc, v_sc, sk_sc, st_sc, wo_st, out_sc, fwd_ref, inv_ref,
            k_sc, hp_sc, h_sc, mem0_ref, sh_ref, sd_ref,
            never_sm, sem_s, sem_in, sem_w, sem_out,
            *, S, DM, H, DH, M, SEG):
    NSEG = S // SEG
    M2 = 2 * M
    R = M2 + 2 * SEG
    RH = M2 + SEG
    NB = S // CB
    QB = CB // NQ
    HB = QB // 2
    NT = DM // 128
    assert QB == SEG and NSEG % PH == 0 and 2 <= NPRE <= PH
    NPH = NSEG // PH
    HG = H // 2

    small = [pltpu.make_async_copy(s, d, sem_s.at[i]) for i, (s, d) in enumerate([
        (mem0_hbm, mem0_ref), (sh_hbm, sh_ref), (sd_hbm, sd_ref), (fwd_hbm, fwd_ref), (inv_hbm, inv_ref)])]

    xb = (0, NPRE * SEG, 2 * PH * SEG, S)
    kb = (0, (2 * NQ + 2) * SEG, 2 * PH * SEG, S)
    sb = (0, 2 * CB, 2 * PH * SEG, S)

    def in_copies(part):
        def rng(b):
            return pl.ds(b[part], b[part + 1] - b[part])
        return [
            pltpu.make_async_copy(x_hbm.at[rng(xb)], x_sc.at[rng(xb)], sem_in.at[part * 4]),
            pltpu.make_async_copy(k_hbm.at[rng(kb)],
                                  k_sc.at[pl.ds(KPAD + kb[part], kb[part + 1] - kb[part])],
                                  sem_in.at[part * 4 + 1]),
            pltpu.make_async_copy(v_hbm.at[rng(kb)], v_sc.at[rng(kb)], sem_in.at[part * 4 + 2]),
            pltpu.make_async_copy(sk_hbm.at[:, rng(sb)], sk_sc.at[:, rng(sb)], sem_in.at[part * 4 + 3]),
        ]

    def w_copy(ci):
        src = (wq_hbm, wk_hbm, wv_hbm)[ci % 3]
        return pltpu.make_async_copy(src.at[:, pl.ds((ci // 3) * HG, HG), :], st_sc.at[ci], sem_w.at[ci])

    wo_copy = pltpu.make_async_copy(wo_hbm, wo_st, sem_w.at[6])

    def out_copy(i):
        rows = pl.ds(pl.multiple_of(i * PH * SEG, PH * SEG), PH * SEG)
        return pltpu.make_async_copy(out_sc.at[rows], o_hbm.at[rows], sem_out.at[i])

    def out_tail(j):
        b = ((NPH - 1) * PH * SEG, (NSEG - 3) * SEG, S)
        rows = pl.ds(b[j], b[j + 1] - b[j])
        return pltpu.make_async_copy(out_sc.at[rows], o_hbm.at[rows], sem_out.at[NPH - 1 + j])

    def start_all(cps):
        def act():
            for cp in cps:
                cp.start()
        return act

    _in_order([start_all(small + in_copies(0))]
              + [start_all([w_copy(ci)]) for ci in range(6)]
              + [start_all([wo_copy]), start_all(in_copies(1)), start_all(in_copies(2))])

    never_sm[0] = 0
    k_sc[0:KPAD, :] = jnp.zeros((KPAD, DM), BF16)
    sp_sc[NB + 1] = jnp.zeros(sp_sc.shape[1:], F32)
    op_sc[...] = jnp.zeros(op_sc.shape, F32)
    x2_sc[...] = jnp.zeros(x2_sc.shape, F32)
    y_sc[...] = jnp.zeros(y_sc.shape, F32)
    h_sc[...] = jnp.zeros(h_sc.shape, BF16)
    for cp in small + in_copies(0):
        cp.wait()

    sh = sh_ref[...].astype(F32)
    KS = sh.shape[0]
    sd = sd_ref[...].astype(F32).reshape(1, DM)

    def seg(i):
        i = jnp.clip(i, 0, NSEG - 1)
        return pl.ds(pl.multiple_of(i * SEG, SEG), SEG)

    def conv_u(s):
        s = jnp.clip(s, 0, NSEG - 1)
        r0 = pl.multiple_of(s * SEG, SEG)
        kk = k_sc[pl.ds(r0, KPAD + SEG), :].astype(F32)
        ks = kk[KPAD:] * sh[0:1]
        for j in range(1, KS):
            ks = ks + pltpu.roll(kk, j, 0)[KPAD:] * sh[j:j + 1]
        u = (ks * v_sc[pl.ds(r0, SEG), :].astype(F32)).astype(BF16)
        u_sc[pl.ds(r0, SEG), :] = u
        return u

    def conv_fwd(c, q):
        cc = jnp.minimum(c, NB - 1)
        t0 = pl.multiple_of(cc * CB, CB)
        f = fwd_ref[q]
        uf = _dot(f, u_sc[pl.ds(t0, CB), :])
        kf = _dot_nt(f, sk_sc[:, pl.ds(t0, CB)])
        return uf, kf

    def put_spec(cs, q, which, val):
        for rb in range(QB // 8):
            for n in range(NT):
                ln = slice(n * 128, (n + 1) * 128)
                sp_sc[cs, q, rb, n, which] = val[rb * 8:rb * 8 + 8, ln]
                sp_sc[cs, q, rb, n, which + 1] = val[QB + rb * 8:QB + rb * 8 + 8, ln]

    def conv_spec(c, q):
        uf, kf = conv_fwd(c, q)
        cs = jnp.minimum(c, NB)
        put_spec(cs, q, 0, uf)
        pk = kr_sc[q]
        kr_sc[q] = kf
        kp = jnp.concatenate([
            kf[0:HB] - pk[QB:QB + HB],
            kf[HB:QB] + pk[QB + HB:],
            kf[QB:QB + HB] + pk[0:HB],
            kf[QB + HB:] - pk[HB:QB]], axis=0)
        put_spec(cs, q, 2, kp)

    MAC_PIECES = [(rb, n) for rb in range(QB // 16) for n in range(NT)]

    def conv_mac(c, q, piece, nterms):
        rb2, n = piece
        cs = jnp.minimum(c, NB)
        acc = []
        for rb in (2 * rb2, 2 * rb2 + 1):
            ar = None
            ai = None
            for j in range(nterms):
                uj = jnp.minimum(j, cs)
                kj = jnp.where(cs - j >= 0, cs - j, NB + 1)
                ur = sp_sc[uj, q, rb, n, 0]
                um = sp_sc[uj, q, rb, n, 1]
                kr = sp_sc[kj, q, rb, n, 2]
                km = sp_sc[kj, q, rb, n, 3]
                tr = ur * kr - um * km
                ti = ur * km + um * kr
                ar = tr if ar is None else ar + tr
                ai = ti if ai is None else ai + ti
            acc.append((ar, ai))
        ln = slice(n * 128, (n + 1) * 128)
        wf_sc[c & 1, q, rb2 * 16:rb2 * 16 + 16, ln] = jnp.concatenate(
            [acc[0][0], acc[1][0]], axis=0).astype(BF16)
        wf_sc[c & 1, q, QB + rb2 * 16:QB + rb2 * 16 + 16, ln] = jnp.concatenate(
            [acc[0][1], acc[1][1]], axis=0).astype(BF16)

    def conv_inv(s):
        w = wf_sc[(s // NQ) & 1].reshape(2 * CB, DM)
        yc = _dot(inv_ref[s % NQ], w)
        y_sc[s & 3] = yc + u_sc[seg(s), :].astype(F32) * sd

    scale = DH ** -0.5
    cexp = scale * float(np.log2(np.e))

    def make_mask(n, x_layers):
        qi = jax.lax.broadcasted_iota(jnp.int32, (n, n), 0)
        ki = jax.lax.broadcasted_iota(jnp.int32, (n, n), 1)

        def layer(i):
            xl = jnp.where(i < M2 + SEG, x_layers[0], x_layers[-1])
            return jnp.where(i < M, 0, jnp.where(i < M2, 1, xl))
        same = layer(qi) == layer(ki)
        ok = same & ((qi < M2) | (ki < M2) | (qi >= ki))
        fill = jnp.where(same, -1e9 / scale, -jnp.inf).astype(F32)
        return ok, fill

    def probs(qkv, mask):
        ok, fill = mask
        s = _dot_nt(qkv[:, 0:DH], qkv[:, DH:2 * DH])
        s = jnp.where(ok, s, fill)
        m = jnp.max(s, axis=-1, keepdims=True)
        p = jnp.exp2((s - m) * cexp)
        l = jnp.sum(p, axis=-1, keepdims=True)
        r = pl.reciprocal(l, approx=True)
        r = r * (2.0 - l * r)
        return (p * r).astype(BF16)

    def w_piece(ci, j):
        return (wa_sc, wb_sc)[ci % 2][ci // 2, j]

    def w_head(g):
        return _unpack(jnp.concatenate(
            [w_piece(3 * (g // HG) + mi, g % HG) for mi in range(3)], axis=1))

    def pre_rows(ref, half, j):
        return _unpack(jnp.concatenate([ref[3 * half + mi, j] for mi in range(3)], axis=1))

    def out_proj(n, g0, g1, j):
        return _dot(_unpack(o_sc[0:n // 2, g0 * DH:g1 * DH]),
                    _unpack(wo_sc[g0 * DH // 2:g1 * DH // 2, j * 128:(j + 1) * 128]))

    def attend(proj, n, mask, dist, hook=None):
        D1, D2 = dist
        HA = H - D1 - D2 - 1
        qkvs = {}
        ps = {}
        outs = {}
        for it in range(H + D1 + D2):
            if it < H:
                qkvs[it] = proj(it)
            g = it - D1
            if 0 <= g < H:
                ps[g] = probs(qkvs[g], mask)
            g = it - D1 - D2
            if 0 <= g < H:
                o = _dot(ps.pop(g), qkvs.pop(g)[:, 2 * DH:3 * DH])
                o_sc[0:n // 2, g * DH:(g + 1) * DH] = _pack(o)
            if hook is not None:
                hook(it)
            j = it - (H - 1)
            if 0 <= j < D1 + D2:
                outs[j] = out_proj(n, 0, HA, j)
        for j in range(D1 + D2, NT):
            outs[j] = out_proj(n, 0, H, j)
        for j in range(D1 + D2):
            outs[j] = out_proj(n, HA, H, j) + outs[j]
        return jnp.concatenate([outs[j] for j in range(NT)], axis=1)

    def side1(t):
        x1 = x_sc[seg(t - 1), :].astype(F32) + op_sc[0:SEG, :]
        x2 = x1 + _ln(x1) * y_sc[(t - 1) & 3]
        x2_sc[(t - 1) & 3] = x2
        return _ln(x2).astype(BF16)

    def side2(t):
        x3 = x2_sc[(t - 3) & 3] + op_sc[SEG:, :]
        x4 = x3 + _ln(x3) * y_sc[(t - 3) & 3]
        x4 = x4.astype(out_sc.dtype)
        out_sc[seg(t - 3), :] = x4
        return x4

    def pro_u(s, c):
        conv_u(s)
        return c
    jax.lax.fori_loop(0, 2 * NQ + 2, pro_u, 0)

    def pro_c(q, c):
        uf, kf = conv_fwd(0, q)
        put_spec(0, q, 0, uf)
        put_spec(0, q, 2, kf)
        kr_sc[q] = kf
        ur, um, kr, km = uf[:QB], uf[QB:], kf[:QB], kf[QB:]
        wf_sc[0, q, :QB] = (ur * kr - um * km).astype(BF16)
        wf_sc[0, q, QB:] = (ur * km + um * kr).astype(BF16)
        return c
    jax.lax.fori_loop(0, NQ, pro_c, 0)

    def pro_s(t, c):
        conv_spec(1, t)
        for piece in MAC_PIECES:
            conv_mac(1, t, piece, 2)
        conv_inv(t)
        return c
    jax.lax.fori_loop(0, 2, pro_s, 0)

    mem0 = mem0_ref[...].astype(F32)
    hp_sc[0:M, :] = _pack(jnp.concatenate([mem0, mem0], axis=0))

    def pro_h(s, c):
        xn = _ln(x_sc[seg(s), :].astype(F32))
        hp_sc[pl.ds(pl.multiple_of(M + jnp.maximum(s - 1, 0) * (SEG // 2), 8), SEG // 2), :] = _pack(xn)
        return c
    jax.lax.fori_loop(2, NPRE, pro_h, 0)
    pro_h(0, 0)
    h_sc[M2:RH, :] = _ln(x_sc[SEG:2 * SEG, :].astype(F32)).astype(BF16)

    mask1 = make_mask(RH, (0,))

    def wait_chunk(ci):
        with jax.named_scope("wait_w"):
            pltpu.make_async_copy(wq_hbm.at[:, pl.ds(0, HG), :], st_sc.at[ci], sem_w.at[ci]).wait()

    def relayout(ci, dst, slot, b):
        d0 = b * 16 if isinstance(b, int) else pl.multiple_of(b * 16, 16)
        r0 = b * 8 if isinstance(b, int) else pl.multiple_of(b * 8, 8)
        xw = pltpu.bitcast(st_sc[ci, pl.ds(d0, 16)], U32).reshape(8, 2, HG // 2, DH)
        a = xw[:, 0]
        bb = xw[:, 1]
        lo = jnp.swapaxes((a & U32(0xFFFF)) | (bb << 16), 0, 1)
        hi = jnp.swapaxes((a >> 16) | (bb & U32(0xFFFF0000)), 0, 1)
        for j in range(HG // 2):
            dst[slot, 2 * j, pl.ds(r0, 8), :] = lo[j]
            dst[slot, 2 * j + 1, pl.ds(r0, 8), :] = hi[j]

    NBLK = DM // 16

    def fused(cr, dst, rslot, cp, src, pslot):
        S2 = SEG // 2
        cuts = [0, RH // 2 + S2, RH // 2 + 3 * S2, RH // 2 + (NPRE - 2) * S2]
        npc = len(cuts) - 1

        def sub(i, c):
            nh = HG // NSUB
            nb = NBLK // NSUB
            done = 0
            for jj in range(nh):
                j = i * nh + jj
                w = _unpack(src[pslot, j])
                for pi in range(npc):
                    upto = min(nb, -(-(jj * npc + pi + 1) * nb // (nh * npc - 2)))
                    for bb in range(done, upto):
                        relayout(cr, dst, rslot, i * nb + bb)
                    done = upto
                    lo, hi = cuts[pi], cuts[pi + 1]
                    r = _pack(_dot(_unpack(hp_sc[lo:hi, :]), w))
                    if pi == 0:
                        pre0_sc[cp, j] = r[0:RH // 2]
                    for sg in range(NPRE - 2):
                        a = RH // 2 + sg * S2
                        if lo <= a < hi:
                            pre_sc[sg, cp, j] = r[a - lo:a - lo + S2]
            return c
        with jax.named_scope("fused"):
            if NSUB == 1:
                jax.lax.fori_loop(0, never_sm[0] + 1, lambda i, c: sub(0, c), 0)
            else:
                jax.lax.fori_loop(0, NSUB, sub, 0)

    wait_chunk(0)

    def relayout0(b, c):
        relayout(0, wa_sc, 0, b)
        return c
    with jax.named_scope("relayout"):
        jax.lax.fori_loop(0, NBLK, relayout0, 0, unroll=2)

    def chunk_pair(k, carry):
        wait_chunk(2 * k + 1)
        kc = jnp.minimum(k + never_sm[0], 2)
        fused(2 * kc + 1, wb_sc, kc, 2 * k, wa_sc, k)

        @pl.when(k < 2)
        def _():
            wait_chunk(2 * k + 2)
        kn = jnp.minimum(k + 1, 2)
        fused(2 * kn, wa_sc, kn, 2 * k + 1, wb_sc, k)

        return carry
    jax.lax.fori_loop(0, 3, chunk_pair, 0)

    with jax.named_scope("wait_wo"):
        wo_copy.wait()
    ps = {}
    os_ = []
    out = None
    GW, E1, E2 = 4, 2, 1
    for it in range(H // GW + E1 + E2):
        for j in range(it * GW, (it + 1) * GW):
            if j < H:
                ps[j] = probs(pre_rows(pre0_sc, j // HG, j % HG), mask1)
        for j in range((it - E1) * GW, (it - E1 + 1) * GW):
            if 0 <= j < H:
                os_.append(_dot(ps.pop(j), _unpack(pre0_sc[3 * (j // HG) + 2, j % HG])).astype(BF16))
        g0 = (it - E1 - E2) * GW
        if g0 >= 0:
            wo = wo_st[g0 * DH:(g0 + GW) * DH, :]
            wo_sc[g0 * DH // 2:(g0 + GW) * DH // 2, :] = _pack(wo)
            part = _dot(jnp.concatenate(os_[g0:g0 + GW], axis=1), wo)
            out = part if out is None else part + out
    h_sc[0:M2, :] = jnp.concatenate([out[0:M], mem0], axis=0).astype(BF16)
    op_sc[0:SEG, :] = out[M2:]

    mask12 = make_mask(R, (0, 1))

    def pinned(never, h, pins):
        hs = {0: h}
        r = _pack(h[-SEG:])
        for g, d in pins:
            r = jnp.where(never, _pack(d), r)
            hs[g] = jnp.concatenate([h[:-SEG], _unpack(r)], axis=0)
        return lambda g: hs[max(k for k in hs if k <= g)]

    def step(t, pre, spec_first=False):
        c = t // NQ + 1
        q = t % NQ
        if spec_first:
            conv_spec(c, q)
        x4 = side2(t)
        xn2 = side1(t)
        xn1 = _ln(x_sc[seg(t + 1), :].astype(F32)).astype(BF16)
        un = conv_u(t + 2 * NQ)
        pins = list(zip(PINS, (un, xn1, x4, xn2)))
        never = never_sm[0] > 0
        if pre:
            h = pinned(never, jnp.concatenate([h_sc[0:M2, :], h_sc[RH:, :]], axis=0), pins)

            def proj(g):
                r = _dot(h(g), w_head(g)).astype(BF16)
                x1 = pre_rows(pre_sc.at[t - 2], g // HG, g % HG)
                return jnp.concatenate([r[0:M2], x1, r[M2:]], axis=0)
            nterms = (NPRE - 1) // NQ + 2
        else:
            h = pinned(never, h_sc[...], pins)

            def proj(g):
                return _dot(h(g), w_head(g)).astype(BF16)
            nterms = NB
        h_sc[M2:RH, :] = xn1
        h_sc[RH:, :] = xn2

        def hook(it):
            if it == SPEC_AT and not spec_first:
                conv_spec(c, q)
            if it == SPEC_AT + 1:
                for piece in MAC_PIECES:
                    conv_mac(c, q, piece, nterms)
        out = attend(proj, R, mask12, DIST_PRE if pre else DIST, hook)
        conv_inv(t)
        h_sc[0:M2, :] = out[0:M2].astype(BF16)
        op_sc[...] = out[M2:]

    def step_pre(t, carry):
        step(t, True)
        return carry

    def step_full(i, carry):
        for j in range(UNROLL):
            step(i * UNROLL + j, False, j > 0)
        return carry

    def phase(p, carry):
        @pl.when(p == 1)
        def _():
            for cp in in_copies(2):
                cp.wait()

        @pl.when(p >= 2)
        def _():
            out_copy(p - 2).start()

        with jax.named_scope("steps"):
            jax.lax.fori_loop(jnp.maximum(p * PH, NPRE) // UNROLL, (p * PH + PH) // UNROLL, step_full, 0)
        return carry

    mask2 = make_mask(RH, (1,))

    def step_half(t, carry):
        first = t < NSEG
        lo = pl.multiple_of(jnp.where(first, 0, SEG), SEG)
        mask = (jnp.where(first, mask1[0].astype(jnp.int32), mask2[0].astype(jnp.int32)) > 0,
                jnp.where(first, mask1[1], mask2[1]))
        h = jnp.concatenate([h_sc[0:M2, :], h_sc[pl.ds(pl.multiple_of(M2 + lo, 16), SEG), :]], axis=0)
        side2(t)
        xn2 = side1(t)
        out = attend(lambda g: _dot(h, w_head(g)).astype(BF16), RH, mask, DIST_HALF)
        m2 = jnp.where(first, mem0, out[M:M2])
        h_sc[0:M2, :] = jnp.concatenate([out[0:M], m2], axis=0).astype(BF16)
        h_sc[RH:, :] = xn2
        op_sc[pl.ds(lo, SEG), :] = out[M2:]
        return carry

    def stage(i, carry):
        with jax.named_scope("steps_half"):
            jax.lax.fori_loop(jnp.where(i == 0, 1, NSEG), jnp.where(i == 0, 2, NSEG + 2), step_half, 0)

        @pl.when(i == 0)
        def _():
            for cp in in_copies(1):
                cp.wait()
            with jax.named_scope("steps_pre"):
                jax.lax.fori_loop(2, NPRE, step_pre, 0)
            jax.lax.fori_loop(0, NPH, phase, 0)
            out_copy(NPH - 2).start()
            out_tail(0).start()
        return carry

    jax.lax.fori_loop(0, 2, stage, 0)
    side2(NSEG + 2)
    out_tail(1).start()
    for i in range(NPH - 1):
        out_copy(i).wait()
    out_tail(0).wait()
    out_tail(1).wait()


@functools.partial(jax.jit, static_argnames=("A_seg_len",))
def pallas_interleave_layers__memory_aug_recurrent_mem_tr__ssm_conv_h3__prompt_kernel(
    A_x, A_mem0, A_Wq, A_Wk, A_Wv, A_Wo, A_seg_len,
    B_q, B_k, B_v, B_shift_k, B_ssm_k, B_ssm_D,
):
    del B_q
    B, S, DM = A_x.shape
    assert B == 1
    H, DH = A_Wq.shape[1], A_Wq.shape[2]
    M = A_mem0.shape[1]
    SEG = int(A_seg_len)
    KS = B_shift_k.shape[1]
    R = 2 * (M + SEG)
    RP = 2 * M + (NPRE - 1) * SEG
    NB = S // CB
    QB = CB // NQ
    fwd, inv = _dft_constants()

    kern = functools.partial(_kernel, S=S, DM=DM, H=H, DH=DH, M=M, SEG=SEG)
    any_spec = pl.BlockSpec(memory_space=pl.ANY)
    out = pl.pallas_call(
        kern,
        out_shape=jax.ShapeDtypeStruct((S, DM), A_x.dtype),
        in_specs=[any_spec] * 13,
        out_specs=any_spec,
        scratch_shapes=[
            pltpu.VMEM((NB + 2, NQ, QB // 8, DM // 128, 4, 8, 128), F32),
            pltpu.VMEM((NQ, 2 * QB, DM), F32),
            pltpu.VMEM((2, NQ, 2 * QB, DM), BF16),
            pltpu.VMEM((4, SEG, DM), F32),
            pltpu.VMEM((4, SEG, DM), F32),
            pltpu.VMEM((S, DM), BF16),
            pltpu.VMEM((2 * SEG, DM), F32),
            pltpu.VMEM((NPRE - 2, 6, H // 2, SEG // 2, DH), U32),
            pltpu.VMEM((6, H // 2, M + SEG // 2, DH), U32),
            pltpu.VMEM((3, H // 2, DM // 2, DH), U32),
            pltpu.VMEM((3, H // 2, DM // 2, DH), U32),
            pltpu.VMEM((H * DH // 2, DM), U32),
            pltpu.VMEM((R // 2, H * DH), U32),
            pltpu.VMEM((S, DM), BF16),
            pltpu.VMEM((S, DM), BF16),
            pltpu.VMEM((DM, S), BF16),
            pltpu.VMEM((6, DM, H // 2, DH), BF16),
            pltpu.VMEM((H * DH, DM), BF16),
            pltpu.VMEM((S, DM), A_x.dtype),
            pltpu.VMEM(fwd.shape, BF16),
            pltpu.VMEM(inv.shape, BF16),
            pltpu.VMEM((S + KPAD, DM), BF16),
            pltpu.VMEM((RP // 2, DM), U32),
            pltpu.VMEM((R, DM), BF16),
            pltpu.VMEM((M, DM), BF16),
            pltpu.VMEM((KS, DM), BF16),
            pltpu.VMEM((DM,), BF16),
            pltpu.SMEM((1,), jnp.int32),
            pltpu.SemaphoreType.DMA((5,)),
            pltpu.SemaphoreType.DMA((12,)),
            pltpu.SemaphoreType.DMA((7,)),
            pltpu.SemaphoreType.DMA((S // SEG // PH + 1,)),
        ],
        compiler_params=pltpu.CompilerParams(vmem_limit_bytes=120 * 1024 * 1024),
    )(
        A_x.reshape(S, DM), A_mem0.reshape(M, DM), A_Wq, A_Wk, A_Wv,
        A_Wo.reshape(H * DH, DM), B_k.reshape(S, DM), B_v.reshape(S, DM),
        B_shift_k.T, B_ssm_k, B_ssm_D,
        jnp.asarray(fwd, BF16), jnp.asarray(inv, BF16),
    )
    return out.reshape(B, S, DM)
```

```python
import functools

import numpy as np
import jax
import jax.numpy as jnp
import jax.experimental.pallas as pl
import jax.experimental.pallas.tpu as pltpu

F32 = jnp.float32
BF16 = jnp.bfloat16
U32 = jnp.uint32

CB = 128
NQ = 4
KPAD = 16
PH = 8
NPRE = 8
PINS = (3, 12, 16, 20)
SPEC_AT = 4
UNROLL = 2
NSUB = 1
DIST, DIST_PRE, DIST_HALF = (1, 2), (2, 3), (1, 3)


def _dft_constants():
    qb = CB // NQ
    n = np.arange(CB, dtype=np.float64)
    fwd = np.zeros((NQ, 2 * qb, CB))
    for q in range(NQ):
        f = q * qb + np.concatenate([np.arange(0, qb, 2), np.arange(1, qb, 2)])
        ang = (np.pi * (2.0 * f + 1.0) / (2 * CB))[:, None] * n[None, :]
        fwd[q, :qb] = np.cos(ang)
        fwd[q, qb:] = -np.sin(ang)
    inv = fwd.reshape(2 * CB, CB).T / CB
    return fwd.astype(np.float32), inv.reshape(NQ, CB // NQ, 2 * CB).astype(np.float32)


def _ln(x, eps=1e-5):
    d = x.shape[-1]
    m = jnp.sum(x, axis=-1, keepdims=True) * (1.0 / d)
    xc = x - m
    v = jnp.sum(xc * xc, axis=-1, keepdims=True) * (1.0 / d)
    return xc * jax.lax.rsqrt(v + eps)


def _dot(a, b):
    return jnp.dot(a, b, preferred_element_type=F32)


def _dot_nt(a, b):
    return jax.lax.dot_general(a, b, (((1,), (1,)), ((), ())), preferred_element_type=F32)


def _pack(x):
    return pltpu.bitcast(x.astype(BF16), U32)


def _unpack(x):
    return pltpu.bitcast(x, BF16)


def _in_order(actions):
    def body(i, c):
        for j, act in enumerate(actions):
            pl.when(i == j)(act)
        return c
    jax.lax.fori_loop(0, len(actions), body, 0)


def _kernel(x_hbm, mem0_hbm, wq_hbm, wk_hbm, wv_hbm, wo_hbm, k_hbm, v_hbm,
            sh_hbm, sk_hbm, sd_hbm, fwd_hbm, inv_hbm, o_hbm,
            sp_sc, kr_sc, wf_sc, x2_sc, y_sc, u_sc, op_sc, pre_sc, pre0_sc, wa_sc, wb_sc, wo_sc, o_sc,
            x_sc, v_sc, sk_sc, st_sc, wo_st, out_sc, fwd_ref, inv_ref,
            k_sc, hp_sc, h_sc, mem0_ref, sh_ref, sd_ref,
            never_sm, sem_s, sem_in, sem_w, sem_out,
            *, S, DM, H, DH, M, SEG):
    NSEG = S // SEG
    M2 = 2 * M
    R = M2 + 2 * SEG
    RH = M2 + SEG
    NB = S // CB
    QB = CB // NQ
    HB = QB // 2
    NT = DM // 128
    assert QB == SEG and NSEG % PH == 0 and 2 <= NPRE <= PH
    NPH = NSEG // PH
    HG = H // 2

    small = [pltpu.make_async_copy(s, d, sem_s.at[i]) for i, (s, d) in enumerate([
        (mem0_hbm, mem0_ref), (sh_hbm, sh_ref), (sd_hbm, sd_ref), (fwd_hbm, fwd_ref), (inv_hbm, inv_ref)])]

    xb = (0, NPRE * SEG, 2 * PH * SEG, S)
    kb = (0, (2 * NQ + 2) * SEG, 2 * PH * SEG, S)
    sb = (0, 2 * CB, 2 * PH * SEG, S)

    def in_copies(part):
        def rng(b):
            return pl.ds(b[part], b[part + 1] - b[part])
        return [
            pltpu.make_async_copy(x_hbm.at[rng(xb)], x_sc.at[rng(xb)], sem_in.at[part * 4]),
            pltpu.make_async_copy(k_hbm.at[rng(kb)],
                                  k_sc.at[pl.ds(KPAD + kb[part], kb[part + 1] - kb[part])],
                                  sem_in.at[part * 4 + 1]),
            pltpu.make_async_copy(v_hbm.at[rng(kb)], v_sc.at[rng(kb)], sem_in.at[part * 4 + 2]),
            pltpu.make_async_copy(sk_hbm.at[:, rng(sb)], sk_sc.at[:, rng(sb)], sem_in.at[part * 4 + 3]),
        ]

    def w_copy(ci):
        src = (wq_hbm, wk_hbm, wv_hbm)[ci % 3]
        return pltpu.make_async_copy(src.at[:, pl.ds((ci // 3) * HG, HG), :], st_sc.at[ci], sem_w.at[ci])

    wo_copy = pltpu.make_async_copy(wo_hbm, wo_st, sem_w.at[6])

    def out_copy(i):
        rows = pl.ds(pl.multiple_of(i * PH * SEG, PH * SEG), PH * SEG)
        return pltpu.make_async_copy(out_sc.at[rows], o_hbm.at[rows], sem_out.at[i])

    def out_tail(j):
        b = ((NPH - 1) * PH * SEG, (NSEG - 3) * SEG, S)
        rows = pl.ds(b[j], b[j + 1] - b[j])
        return pltpu.make_async_copy(out_sc.at[rows], o_hbm.at[rows], sem_out.at[NPH - 1 + j])

    def start_all(cps):
        def act():
            for cp in cps:
                cp.start()
        return act

    _in_order([start_all(small + in_copies(0))]
              + [start_all([w_copy(ci)]) for ci in range(6)]
              + [start_all([wo_copy]), start_all(in_copies(1)), start_all(in_copies(2))])

    never_sm[0] = 0
    k_sc[0:KPAD, :] = jnp.zeros((KPAD, DM), BF16)
    sp_sc[NB + 1] = jnp.zeros(sp_sc.shape[1:], F32)
    op_sc[...] = jnp.zeros(op_sc.shape, F32)
    x2_sc[...] = jnp.zeros(x2_sc.shape, F32)
    y_sc[...] = jnp.zeros(y_sc.shape, F32)
    h_sc[...] = jnp.zeros(h_sc.shape, BF16)
    for cp in small + in_copies(0):
        cp.wait()

    sh = sh_ref[...].astype(F32)
    KS = sh.shape[0]
    sd = sd_ref[...].astype(F32).reshape(1, DM)

    def seg(i):
        i = jnp.clip(i, 0, NSEG - 1)
        return pl.ds(pl.multiple_of(i * SEG, SEG), SEG)

    def conv_u(s):
        s = jnp.clip(s, 0, NSEG - 1)
        r0 = pl.multiple_of(s * SEG, SEG)
        kk = k_sc[pl.ds(r0, KPAD + SEG), :].astype(F32)
        ks = kk[KPAD:] * sh[0:1]
        for j in range(1, KS):
            ks = ks + pltpu.roll(kk, j, 0)[KPAD:] * sh[j:j + 1]
        u = (ks * v_sc[pl.ds(r0, SEG), :].astype(F32)).astype(BF16)
        u_sc[pl.ds(r0, SEG), :] = u
        return u

    def conv_fwd(c, q):
        cc = jnp.minimum(c, NB - 1)
        t0 = pl.multiple_of(cc * CB, CB)
        f = fwd_ref[q]
        uf = _dot(f, u_sc[pl.ds(t0, CB), :])
        kf = _dot_nt(f, sk_sc[:, pl.ds(t0, CB)])
        return uf, kf

    def put_spec(cs, q, which, val):
        for rb in range(QB // 8):
            for n in range(NT):
                ln = slice(n * 128, (n + 1) * 128)
                sp_sc[cs, q, rb, n, which] = val[rb * 8:rb * 8 + 8, ln]
                sp_sc[cs, q, rb, n, which + 1] = val[QB + rb * 8:QB + rb * 8 + 8, ln]

    def conv_spec(c, q):
        uf, kf = conv_fwd(c, q)
        cs = jnp.minimum(c, NB)
        put_spec(cs, q, 0, uf)
        pk = kr_sc[q]
        kr_sc[q] = kf
        kp = jnp.concatenate([
            kf[0:HB] - pk[QB:QB + HB],
            kf[HB:QB] + pk[QB + HB:],
            kf[QB:QB + HB] + pk[0:HB],
            kf[QB + HB:] - pk[HB:QB]], axis=0)
        put_spec(cs, q, 2, kp)

    MAC_PIECES = [(rb, n) for rb in range(QB // 16) for n in range(NT)]

    def conv_mac(c, q, piece, nterms):
        rb2, n = piece
        cs = jnp.minimum(c, NB)
        acc = []
        for rb in (2 * rb2, 2 * rb2 + 1):
            ar = None
            ai = None
            for j in range(nterms):
                uj = jnp.minimum(j, cs)
                kj = jnp.where(cs - j >= 0, cs - j, NB + 1)
                ur = sp_sc[uj, q, rb, n, 0]
                um = sp_sc[uj, q, rb, n, 1]
                kr = sp_sc[kj, q, rb, n, 2]
                km = sp_sc[kj, q, rb, n, 3]
                tr = ur * kr - um * km
                ti = ur * km + um * kr
                ar = tr if ar is None else ar + tr
                ai = ti if ai is None else ai + ti
            acc.append((ar, ai))
        ln = slice(n * 128, (n + 1) * 128)
        wf_sc[c & 1, q, rb2 * 16:rb2 * 16 + 16, ln] = jnp.concatenate(
            [acc[0][0], acc[1][0]], axis=0).astype(BF16)
        wf_sc[c & 1, q, QB + rb2 * 16:QB + rb2 * 16 + 16, ln] = jnp.concatenate(
            [acc[0][1], acc[1][1]], axis=0).astype(BF16)

    def conv_inv(s):
        w = wf_sc[(s // NQ) & 1].reshape(2 * CB, DM)
        yc = _dot(inv_ref[s % NQ], w)
        y_sc[s & 3] = yc + u_sc[seg(s), :].astype(F32) * sd

    scale = DH ** -0.5
    cexp = scale * float(np.log2(np.e))

    def make_mask(n, x_layers):
        qi = jax.lax.broadcasted_iota(jnp.int32, (n, n), 0)
        ki = jax.lax.broadcasted_iota(jnp.int32, (n, n), 1)

        def layer(i):
            xl = jnp.where(i < M2 + SEG, x_layers[0], x_layers[-1])
            return jnp.where(i < M, 0, jnp.where(i < M2, 1, xl))
        same = layer(qi) == layer(ki)
        ok = same & ((qi < M2) | (ki < M2) | (qi >= ki))
        fill = jnp.where(same, -1e9 / scale, -jnp.inf).astype(F32)
        return ok, fill

    def probs(qkv, mask):
        ok, fill = mask
        s = _dot_nt(qkv[:, 0:DH], qkv[:, DH:2 * DH])
        s = jnp.where(ok, s, fill)
        m = jnp.max(s, axis=-1, keepdims=True)
        p = jnp.exp2((s - m) * cexp)
        l = jnp.sum(p, axis=-1, keepdims=True)
        r = pl.reciprocal(l, approx=True)
        r = r * (2.0 - l * r)
        return (p * r).astype(BF16)

    def w_piece(ci, j):
        return (wa_sc, wb_sc)[ci % 2][ci // 2, j]

    def w_head(g):
        return _unpack(jnp.concatenate(
            [w_piece(3 * (g // HG) + mi, g % HG) for mi in range(3)], axis=1))

    def pre_rows(ref, half, j):
        return _unpack(jnp.concatenate([ref[3 * half + mi, j] for mi in range(3)], axis=1))

    def out_proj(n, g0, g1, j):
        return _dot(_unpack(o_sc[0:n // 2, g0 * DH:g1 * DH]),
                    _unpack(wo_sc[g0 * DH // 2:g1 * DH // 2, j * 128:(j + 1) * 128]))

    def attend(proj, n, mask, dist, hook=None):
        D1, D2 = dist
        HA = H - D1 - D2 - 1
        qkvs = {}
        ps = {}
        outs = {}
        for it in range(H + D1 + D2):
            if it < H:
                qkvs[it] = proj(it)
            g = it - D1
            if 0 <= g < H:
                ps[g] = probs(qkvs[g], mask)
            g = it - D1 - D2
            if 0 <= g < H:
                o = _dot(ps.pop(g), qkvs.pop(g)[:, 2 * DH:3 * DH])
                o_sc[0:n // 2, g * DH:(g + 1) * DH] = _pack(o)
            if hook is not None:
                hook(it)
            j = it - (H - 1)
            if 0 <= j < D1 + D2:
                outs[j] = out_proj(n, 0, HA, j)
        for j in range(D1 + D2, NT):
            outs[j] = out_proj(n, 0, H, j)
        for j in range(D1 + D2):
            outs[j] = out_proj(n, HA, H, j) + outs[j]
        return jnp.concatenate([outs[j] for j in range(NT)], axis=1)

    def side1(t):
        x1 = x_sc[seg(t - 1), :].astype(F32) + op_sc[0:SEG, :]
        x2 = x1 + _ln(x1) * y_sc[(t - 1) & 3]
        x2_sc[(t - 1) & 3] = x2
        return _ln(x2).astype(BF16)

    def side2(t):
        x3 = x2_sc[(t - 3) & 3] + op_sc[SEG:, :]
        x4 = x3 + _ln(x3) * y_sc[(t - 3) & 3]
        x4 = x4.astype(out_sc.dtype)
        out_sc[seg(t - 3), :] = x4
        return x4

    def pro_u(s, c):
        conv_u(s)
        return c
    jax.lax.fori_loop(0, 2 * NQ + 2, pro_u, 0)

    def pro_c(q, c):
        uf, kf = conv_fwd(0, q)
        put_spec(0, q, 0, uf)
        put_spec(0, q, 2, kf)
        kr_sc[q] = kf
        ur, um, kr, km = uf[:QB], uf[QB:], kf[:QB], kf[QB:]
        wf_sc[0, q, :QB] = (ur * kr - um * km).astype(BF16)
        wf_sc[0, q, QB:] = (ur * km + um * kr).astype(BF16)
        return c
    jax.lax.fori_loop(0, NQ, pro_c, 0)

    def pro_s(t, c):
        conv_spec(1, t)
        for piece in MAC_PIECES:
            conv_mac(1, t, piece, 2)
        conv_inv(t)
        return c
    jax.lax.fori_loop(0, 2, pro_s, 0)

    mem0 = mem0_ref[...].astype(F32)
    hp_sc[0:M, :] = _pack(jnp.concatenate([mem0, mem0], axis=0))

    def pro_h(s, c):
        xn = _ln(x_sc[seg(s), :].astype(F32))
        hp_sc[pl.ds(pl.multiple_of(M + jnp.maximum(s - 1, 0) * (SEG // 2), 8), SEG // 2), :] = _pack(xn)
        return c
    jax.lax.fori_loop(2, NPRE, pro_h, 0)
    pro_h(0, 0)
    h_sc[M2:RH, :] = _ln(x_sc[SEG:2 * SEG, :].astype(F32)).astype(BF16)

    mask1 = make_mask(RH, (0,))

    def wait_chunk(ci):
        with jax.named_scope("wait_w"):
            pltpu.make_async_copy(wq_hbm.at[:, pl.ds(0, HG), :], st_sc.at[ci], sem_w.at[ci]).wait()

    def relayout(ci, dst, slot, b):
        d0 = b * 16 if isinstance(b, int) else pl.multiple_of(b * 16, 16)
        r0 = b * 8 if isinstance(b, int) else pl.multiple_of(b * 8, 8)
        xw = pltpu.bitcast(st_sc[ci, pl.ds(d0, 16)], U32).reshape(8, 2, HG // 2, DH)
        a = xw[:, 0]
        bb = xw[:, 1]
        lo = jnp.swapaxes((a & U32(0xFFFF)) | (bb << 16), 0, 1)
        hi = jnp.swapaxes((a >> 16) | (bb & U32(0xFFFF0000)), 0, 1)
        for j in range(HG // 2):
            dst[slot, 2 * j, pl.ds(r0, 8), :] = lo[j]
            dst[slot, 2 * j + 1, pl.ds(r0, 8), :] = hi[j]

    NBLK = DM // 16

    def fused(cr, dst, rslot, cp, src, pslot):
        S2 = SEG // 2
        cuts = [0, RH // 2 + S2, RH // 2 + 3 * S2, RH // 2 + (NPRE - 2) * S2]
        npc = len(cuts) - 1

        def sub(i, c):
            nh = HG // NSUB
            nb = NBLK // NSUB
            done = 0
            for jj in range(nh):
                j = i * nh + jj
                w = _unpack(src[pslot, j])
                for pi in range(npc):
                    upto = min(nb, -(-(jj * npc + pi + 1) * nb // (nh * npc - 2)))
                    for bb in range(done, upto):
                        relayout(cr, dst, rslot, i * nb + bb)
                    done = upto
                    lo, hi = cuts[pi], cuts[pi + 1]
                    r = _pack(_dot(_unpack(hp_sc[lo:hi, :]), w))
                    if pi == 0:
                        pre0_sc[cp, j] = r[0:RH // 2]
                    for sg in range(NPRE - 2):
                        a = RH // 2 + sg * S2
                        if lo <= a < hi:
                            pre_sc[sg, cp, j] = r[a - lo:a - lo + S2]
            return c
        with jax.named_scope("fused"):
            if NSUB == 1:
                jax.lax.fori_loop(0, never_sm[0] + 1, lambda i, c: sub(0, c), 0)
            else:
                jax.lax.fori_loop(0, NSUB, sub, 0)

    wait_chunk(0)

    def relayout0(b, c):
        relayout(0, wa_sc, 0, b)
        return c
    with jax.named_scope("relayout"):
        jax.lax.fori_loop(0, NBLK, relayout0, 0, unroll=2)

    def chunk_pair(k, carry):
        wait_chunk(2 * k + 1)
        kc = jnp.minimum(k + never_sm[0], 2)
        fused(2 * kc + 1, wb_sc, kc, 2 * k, wa_sc, k)

        @pl.when(k < 2)
        def _():
            wait_chunk(2 * k + 2)
        kn = jnp.minimum(k + 1, 2)
        fused(2 * kn, wa_sc, kn, 2 * k + 1, wb_sc, k)

        return carry
    jax.lax.fori_loop(0, 3, chunk_pair, 0)

    with jax.named_scope("wait_wo"):
        wo_copy.wait()
    ps = {}
    os_ = []
    out = None
    GW, E1, E2 = 4, 2, 1
    for it in range(H // GW + E1 + E2):
        for j in range(it * GW, (it + 1) * GW):
            if j < H:
                ps[j] = probs(pre_rows(pre0_sc, j // HG, j % HG), mask1)
        for j in range((it - E1) * GW, (it - E1 + 1) * GW):
            if 0 <= j < H:
                os_.append(_dot(ps.pop(j), _unpack(pre0_sc[3 * (j // HG) + 2, j % HG])).astype(BF16))
        g0 = (it - E1 - E2) * GW
        if g0 >= 0:
            wo = wo_st[g0 * DH:(g0 + GW) * DH, :]
            wo_sc[g0 * DH // 2:(g0 + GW) * DH // 2, :] = _pack(wo)
            part = _dot(jnp.concatenate(os_[g0:g0 + GW], axis=1), wo)
            out = part if out is None else part + out
    h_sc[0:M2, :] = jnp.concatenate([out[0:M], mem0], axis=0).astype(BF16)
    op_sc[0:SEG, :] = out[M2:]

    mask12 = make_mask(R, (0, 1))

    def pinned(never, h, pins):
        hs = {0: h}
        r = _pack(h[-SEG:])
        for g, d in pins:
            r = jnp.where(never, _pack(d), r)
            hs[g] = jnp.concatenate([h[:-SEG], _unpack(r)], axis=0)
        return lambda g: hs[max(k for k in hs if k <= g)]

    def step(t, pre, spec_first=False):
        c = t // NQ + 1
        q = t % NQ
        if spec_first:
            conv_spec(c, q)
        x4 = side2(t)
        xn2 = side1(t)
        xn1 = _ln(x_sc[seg(t + 1), :].astype(F32)).astype(BF16)
        un = conv_u(t + 2 * NQ)
        pins = list(zip(PINS, (un, xn1, x4, xn2)))
        never = never_sm[0] > 0
        if pre:
            h = pinned(never, jnp.concatenate([h_sc[0:M2, :], h_sc[RH:, :]], axis=0), pins)

            def proj(g):
                r = _dot(h(g), w_head(g)).astype(BF16)
                x1 = pre_rows(pre_sc.at[t - 2], g // HG, g % HG)
                return jnp.concatenate([r[0:M2], x1, r[M2:]], axis=0)
            nterms = (NPRE - 1) // NQ + 2
        else:
            h = pinned(never, h_sc[...], pins)

            def proj(g):
                return _dot(h(g), w_head(g)).astype(BF16)
            nterms = NB
        h_sc[M2:RH, :] = xn1
        h_sc[RH:, :] = xn2

        def hook(it):
            if it == SPEC_AT and not spec_first:
                conv_spec(c, q)
            if it == SPEC_AT + 1:
                for piece in MAC_PIECES:
                    conv_mac(c, q, piece, nterms)
        out = attend(proj, R, mask12, DIST_PRE if pre else DIST, hook)
        conv_inv(t)
        h_sc[0:M2, :] = out[0:M2].astype(BF16)
        op_sc[...] = out[M2:]

    def step_pre(t, carry):
        step(t, True)
        return carry

    def step_full(i, carry):
        for j in range(UNROLL):
            step(i * UNROLL + j, False, j > 0)
        return carry

    def phase(p, carry):
        @pl.when(p == 1)
        def _():
            for cp in in_copies(2):
                cp.wait()

        @pl.when(p >= 2)
        def _():
            out_copy(p - 2).start()

        with jax.named_scope("steps"):
            jax.lax.fori_loop(jnp.maximum(p * PH, NPRE) // UNROLL, (p * PH + PH) // UNROLL, step_full, 0)
        return carry

    mask2 = make_mask(RH, (1,))

    def step_half(t, carry):
        first = t < NSEG
        lo = pl.multiple_of(jnp.where(first, 0, SEG), SEG)
        mask = (jnp.where(first, mask1[0].astype(jnp.int32), mask2[0].astype(jnp.int32)) > 0,
                jnp.where(first, mask1[1], mask2[1]))
        h = jnp.concatenate([h_sc[0:M2, :], h_sc[pl.ds(pl.multiple_of(M2 + lo, 16), SEG), :]], axis=0)
        side2(t)
        xn2 = side1(t)
        out = attend(lambda g: _dot(h, w_head(g)).astype(BF16), RH, mask, DIST_HALF)
        m2 = jnp.where(first, mem0, out[M:M2])
        h_sc[0:M2, :] = jnp.concatenate([out[0:M], m2], axis=0).astype(BF16)
        h_sc[RH:, :] = xn2
        op_sc[pl.ds(lo, SEG), :] = out[M2:]
        return carry

    def stage(i, carry):
        with jax.named_scope("steps_half"):
            jax.lax.fori_loop(jnp.where(i == 0, 1, NSEG), jnp.where(i == 0, 2, NSEG + 2), step_half, 0)

        @pl.when(i == 0)
        def _():
            for cp in in_copies(1):
                cp.wait()
            with jax.named_scope("steps_pre"):
                jax.lax.fori_loop(2, NPRE, step_pre, 0)
            jax.lax.fori_loop(0, NPH, phase, 0)
            out_copy(NPH - 2).start()
            out_tail(0).start()
        return carry

    jax.lax.fori_loop(0, 2, stage, 0)
    side2(NSEG + 2)
    out_tail(1).start()
    for i in range(NPH - 1):
        out_copy(i).wait()
    out_tail(0).wait()
    out_tail(1).wait()


def pallas_interleave_layers__memory_aug_recurrent_mem_tr__ssm_conv_h3__prompt_kernel(
    A_x, A_mem0, A_Wq, A_Wk, A_Wv, A_Wo, A_seg_len,
    B_q, B_k, B_v, B_shift_k, B_ssm_k, B_ssm_D,
):
    del B_q
    seg = int(A_seg_len) if isinstance(A_seg_len, (int, np.integer)) else CB // NQ
    return _run(A_x, A_mem0, A_Wq, A_Wk, A_Wv, A_Wo, B_k, B_v, B_shift_k, B_ssm_k, B_ssm_D, SEG=seg)


@functools.partial(jax.jit, static_argnames=("SEG",))
def _run(A_x, A_mem0, A_Wq, A_Wk, A_Wv, A_Wo, B_k, B_v, B_shift_k, B_ssm_k, B_ssm_D, *, SEG):
    B, S, DM = A_x.shape
    assert B == 1
    H, DH = A_Wq.shape[1], A_Wq.shape[2]
    M = A_mem0.shape[1]
    KS = B_shift_k.shape[1]
    R = 2 * (M + SEG)
    RP = 2 * M + (NPRE - 1) * SEG
    NB = S // CB
    QB = CB // NQ
    fwd, inv = _dft_constants()

    kern = functools.partial(_kernel, S=S, DM=DM, H=H, DH=DH, M=M, SEG=SEG)
    any_spec = pl.BlockSpec(memory_space=pl.ANY)
    out = pl.pallas_call(
        kern,
        out_shape=jax.ShapeDtypeStruct((S, DM), A_x.dtype),
        in_specs=[any_spec] * 13,
        out_specs=any_spec,
        scratch_shapes=[
            pltpu.VMEM((NB + 2, NQ, QB // 8, DM // 128, 4, 8, 128), F32),
            pltpu.VMEM((NQ, 2 * QB, DM), F32),
            pltpu.VMEM((2, NQ, 2 * QB, DM), BF16),
            pltpu.VMEM((4, SEG, DM), F32),
            pltpu.VMEM((4, SEG, DM), F32),
            pltpu.VMEM((S, DM), BF16),
            pltpu.VMEM((2 * SEG, DM), F32),
            pltpu.VMEM((NPRE - 2, 6, H // 2, SEG // 2, DH), U32),
            pltpu.VMEM((6, H // 2, M + SEG // 2, DH), U32),
            pltpu.VMEM((3, H // 2, DM // 2, DH), U32),
            pltpu.VMEM((3, H // 2, DM // 2, DH), U32),
            pltpu.VMEM((H * DH // 2, DM), U32),
            pltpu.VMEM((R // 2, H * DH), U32),
            pltpu.VMEM((S, DM), BF16),
            pltpu.VMEM((S, DM), BF16),
            pltpu.VMEM((DM, S), BF16),
            pltpu.VMEM((6, DM, H // 2, DH), BF16),
            pltpu.VMEM((H * DH, DM), BF16),
            pltpu.VMEM((S, DM), A_x.dtype),
            pltpu.VMEM(fwd.shape, BF16),
            pltpu.VMEM(inv.shape, BF16),
            pltpu.VMEM((S + KPAD, DM), BF16),
            pltpu.VMEM((RP // 2, DM), U32),
            pltpu.VMEM((R, DM), BF16),
            pltpu.VMEM((M, DM), BF16),
            pltpu.VMEM((KS, DM), BF16),
            pltpu.VMEM((DM,), BF16),
            pltpu.SMEM((1,), jnp.int32),
            pltpu.SemaphoreType.DMA((5,)),
            pltpu.SemaphoreType.DMA((12,)),
            pltpu.SemaphoreType.DMA((7,)),
            pltpu.SemaphoreType.DMA((S // SEG // PH + 1,)),
        ],
        compiler_params=pltpu.CompilerParams(vmem_limit_bytes=120 * 1024 * 1024),
    )(
        A_x.reshape(S, DM), A_mem0.reshape(M, DM), A_Wq, A_Wk, A_Wv,
        A_Wo.reshape(H * DH, DM), B_k.reshape(S, DM), B_v.reshape(S, DM),
        B_shift_k.T, B_ssm_k, B_ssm_D,
        jnp.asarray(fwd, BF16), jnp.asarray(inv, BF16),
    )
    return out.reshape(B, S, DM)
```

```python
import functools

import numpy as np
import jax
import jax.numpy as jnp
import jax.experimental.pallas as pl
import jax.experimental.pallas.tpu as pltpu

F32 = jnp.float32
BF16 = jnp.bfloat16
U32 = jnp.uint32

CB = 128
NQ = 4
KPAD = 16
PH = 8
NPRE = 10
PINS = (3, 12, 16, 20)
SPEC_AT = 4
UNROLL = 2
HG = 8
DIST, DIST_PRE, DIST_HALF = (1, 2), (2, 3), (1, 3)


def _dft_constants():
    qb = CB // NQ
    n = np.arange(CB, dtype=np.float64)
    fwd = np.zeros((NQ, 2 * qb, CB))
    for q in range(NQ):
        f = q * qb + np.concatenate([np.arange(0, qb, 2), np.arange(1, qb, 2)])
        ang = (np.pi * (2.0 * f + 1.0) / (2 * CB))[:, None] * n[None, :]
        fwd[q, :qb] = np.cos(ang)
        fwd[q, qb:] = -np.sin(ang)
    inv = fwd.reshape(2 * CB, CB).T / CB
    return fwd.astype(np.float32), inv.reshape(NQ, CB // NQ, 2 * CB).astype(np.float32)


def _ln(x, eps=1e-5):
    d = x.shape[-1]
    m = jnp.sum(x, axis=-1, keepdims=True) * (1.0 / d)
    xc = x - m
    v = jnp.sum(xc * xc, axis=-1, keepdims=True) * (1.0 / d)
    return xc * jax.lax.rsqrt(v + eps)


def _dot(a, b):
    return jnp.dot(a, b, preferred_element_type=F32)


def _dot_nt(a, b):
    return jax.lax.dot_general(a, b, (((1,), (1,)), ((), ())), preferred_element_type=F32)


def _pack(x):
    return pltpu.bitcast(x.astype(BF16), U32)


def _unpack(x):
    return pltpu.bitcast(x, BF16)


def _in_order(actions):
    def body(i, c):
        for j, act in enumerate(actions):
            pl.when(i == j)(act)
        return c
    jax.lax.fori_loop(0, len(actions), body, 0)


def _kernel(x_hbm, mem0_hbm, wq_hbm, wk_hbm, wv_hbm, wo_hbm, k_hbm, v_hbm,
            sh_hbm, sk_hbm, sd_hbm, fwd_hbm, inv_hbm, o_hbm,
            sp_sc, kr_sc, wf_sc, x2_sc, y_sc, u_sc, op_sc, pre_sc, pre0_sc, wa_sc, wb_sc, wo_sc, o_sc,
            x_sc, v_sc, sk_sc, st_sc, wo_st, out_sc, fwd_ref, inv_ref,
            k_sc, hp_sc, h_sc, mem0_ref, sh_ref, sd_ref,
            never_sm, sem_s, sem_in, sem_w, sem_out,
            *, S, DM, H, DH, M, SEG):
    NSEG = S // SEG
    M2 = 2 * M
    R = M2 + 2 * SEG
    RH = M2 + SEG
    NB = S // CB
    QB = CB // NQ
    HB = QB // 2
    NT = DM // 128
    assert QB == SEG and NSEG % PH == 0 and NPRE % UNROLL == 0 and PH % UNROLL == 0
    NPH = NSEG // PH
    NCH = 3 * H // HG
    DH2 = DM // 2

    small = [pltpu.make_async_copy(s, d, sem_s.at[i]) for i, (s, d) in enumerate([
        (mem0_hbm, mem0_ref), (sh_hbm, sh_ref), (sd_hbm, sd_ref), (fwd_hbm, fwd_ref), (inv_hbm, inv_ref)])]

    xb = (0, NPRE * SEG, (NPRE + 1) * SEG, S)
    kb = (0, (2 * NQ + 2) * SEG, (2 * NQ + NPRE) * SEG, S)
    sb = (0, 2 * CB, ((NPRE - 1) // NQ + 2) * CB, S)

    def in_copies(part):
        def rng(b):
            return pl.ds(b[part], b[part + 1] - b[part])
        return [
            pltpu.make_async_copy(x_hbm.at[rng(xb)], x_sc.at[rng(xb)], sem_in.at[part * 4]),
            pltpu.make_async_copy(k_hbm.at[rng(kb)],
                                  k_sc.at[pl.ds(KPAD + kb[part], kb[part + 1] - kb[part])],
                                  sem_in.at[part * 4 + 1]),
            pltpu.make_async_copy(v_hbm.at[rng(kb)], v_sc.at[rng(kb)], sem_in.at[part * 4 + 2]),
            pltpu.make_async_copy(sk_hbm.at[:, rng(sb)], sk_sc.at[:, rng(sb)], sem_in.at[part * 4 + 3]),
        ]

    def w_copies(src, g, ci):
        return [pltpu.make_async_copy(src.at[pl.ds(hf * DH2, DH2), pl.ds(pl.multiple_of(g * HG, HG), HG), :],
                                      st_sc.at[ci, :, pl.ds(hf * HG, HG), :], sem_w.at[2 * ci + hf])
                for hf in range(2)]

    wo_copy = pltpu.make_async_copy(wo_hbm, wo_st, sem_w.at[2 * NCH])

    def out_copy(i):
        rows = pl.ds(pl.multiple_of(i * PH * SEG, PH * SEG), PH * SEG)
        return pltpu.make_async_copy(out_sc.at[rows], o_hbm.at[rows], sem_out.at[i])

    def out_tail(j):
        b = ((NPH - 1) * PH * SEG, (NSEG - 3) * SEG, S)
        rows = pl.ds(b[j], b[j + 1] - b[j])
        return pltpu.make_async_copy(out_sc.at[rows], o_hbm.at[rows], sem_out.at[NPH - 1 + j])

    def start_all(cps):
        def act():
            for cp in cps:
                cp.start()
        return act

    in0 = in_copies(0)
    _in_order([start_all(small[:1] + in0[:1]), start_all(small[1:] + in0[1:])])

    def start_group(g, c):
        _in_order([start_all(w_copies(src, g, 3 * g + mi))
                   for mi, src in enumerate((wq_hbm, wk_hbm, wv_hbm))])
        return c
    jax.lax.fori_loop(0, H // HG, start_group, 0)
    _in_order([start_all([wo_copy]), start_all(in_copies(1)), start_all(in_copies(2))])

    never_sm[0] = 0
    k_sc[0:KPAD, :] = jnp.zeros((KPAD, DM), BF16)
    sp_sc[NB + 1] = jnp.zeros(sp_sc.shape[1:], F32)
    op_sc[...] = jnp.zeros(op_sc.shape, F32)
    x2_sc[...] = jnp.zeros(x2_sc.shape, F32)
    y_sc[...] = jnp.zeros(y_sc.shape, F32)
    h_sc[...] = jnp.zeros(h_sc.shape, BF16)
    for cp in small[:1] + in0[:1]:
        cp.wait()

    mem0 = mem0_ref[...].astype(F32)
    hp_sc[0:M, :] = _pack(jnp.concatenate([mem0, mem0], axis=0))
    for sg in range(NPRE):
        xn = _ln(x_sc[sg * SEG:(sg + 1) * SEG, :].astype(F32))
        if sg == 1:
            h_sc[M2:RH, :] = xn.astype(BF16)
        else:
            w0 = M + max(sg - 1, 0) * (SEG // 2)
            hp_sc[w0:w0 + SEG // 2, :] = _pack(xn)

    for cp in small[1:] + in0[1:]:
        cp.wait()

    sh = sh_ref[...].astype(F32)
    KS = sh.shape[0]
    sd = sd_ref[...].astype(F32).reshape(1, DM)

    def seg(i):
        i = jnp.clip(i, 0, NSEG - 1)
        return pl.ds(pl.multiple_of(i * SEG, SEG), SEG)

    def conv_u(s):
        s = jnp.clip(s, 0, NSEG - 1)
        r0 = pl.multiple_of(s * SEG, SEG)
        kk = k_sc[pl.ds(r0, KPAD + SEG), :].astype(F32)
        ks = kk[KPAD:] * sh[0:1]
        for j in range(1, KS):
            ks = ks + pltpu.roll(kk, j, 0)[KPAD:] * sh[j:j + 1]
        u = (ks * v_sc[pl.ds(r0, SEG), :].astype(F32)).astype(BF16)
        u_sc[pl.ds(r0, SEG), :] = u
        return u

    def conv_fwd(c, q):
        cc = jnp.minimum(c, NB - 1)
        t0 = pl.multiple_of(cc * CB, CB)
        f = fwd_ref[q]
        uf = _dot(f, u_sc[pl.ds(t0, CB), :])
        kf = _dot_nt(f, sk_sc[:, pl.ds(t0, CB)])
        return uf, kf

    def put_spec(cs, q, which, val):
        for rb in range(QB // 8):
            for n in range(NT):
                ln = slice(n * 128, (n + 1) * 128)
                sp_sc[cs, q, rb, n, which] = val[rb * 8:rb * 8 + 8, ln]
                sp_sc[cs, q, rb, n, which + 1] = val[QB + rb * 8:QB + rb * 8 + 8, ln]

    def conv_spec(c, q):
        uf, kf = conv_fwd(c, q)
        cs = jnp.minimum(c, NB)
        put_spec(cs, q, 0, uf)
        pk = kr_sc[q]
        kr_sc[q] = kf
        kp = jnp.concatenate([
            kf[0:HB] - pk[QB:QB + HB],
            kf[HB:QB] + pk[QB + HB:],
            kf[QB:QB + HB] + pk[0:HB],
            kf[QB + HB:] - pk[HB:QB]], axis=0)
        put_spec(cs, q, 2, kp)

    MAC_PIECES = [(rb, n) for rb in range(QB // 16) for n in range(NT)]

    def conv_mac(c, q, piece, nterms):
        rb2, n = piece
        cs = jnp.minimum(c, NB)
        acc = []
        for rb in (2 * rb2, 2 * rb2 + 1):
            ar = None
            ai = None
            for j in range(nterms):
                uj = jnp.minimum(j, cs)
                kj = jnp.where(cs - j >= 0, cs - j, NB + 1)
                ur = sp_sc[uj, q, rb, n, 0]
                um = sp_sc[uj, q, rb, n, 1]
                kr = sp_sc[kj, q, rb, n, 2]
                km = sp_sc[kj, q, rb, n, 3]
                tr = ur * kr - um * km
                ti = ur * km + um * kr
                ar = tr if ar is None else ar + tr
                ai = ti if ai is None else ai + ti
            acc.append((ar, ai))
        ln = slice(n * 128, (n + 1) * 128)
        wf_sc[c & 1, q, rb2 * 16:rb2 * 16 + 16, ln] = jnp.concatenate(
            [acc[0][0], acc[1][0]], axis=0).astype(BF16)
        wf_sc[c & 1, q, QB + rb2 * 16:QB + rb2 * 16 + 16, ln] = jnp.concatenate(
            [acc[0][1], acc[1][1]], axis=0).astype(BF16)

    def conv_inv(s):
        w = wf_sc[(s // NQ) & 1].reshape(2 * CB, DM)
        yc = _dot(inv_ref[s % NQ], w)
        y_sc[s & 3] = yc + u_sc[seg(s), :].astype(F32) * sd

    scale = DH ** -0.5
    cexp = scale * float(np.log2(np.e))

    def make_mask(n, x_layers):
        qi = jax.lax.broadcasted_iota(jnp.int32, (n, n), 0)
        ki = jax.lax.broadcasted_iota(jnp.int32, (n, n), 1)

        def layer(i):
            xl = jnp.where(i < M2 + SEG, x_layers[0], x_layers[-1])
            return jnp.where(i < M, 0, jnp.where(i < M2, 1, xl))
        same = layer(qi) == layer(ki)
        ok = same & ((qi < M2) | (ki < M2) | (qi >= ki))
        fill = jnp.where(same, -1e9 / scale, -jnp.inf).astype(F32)
        return ok, fill

    def probs(qkv, mask):
        ok, fill = mask
        s = _dot_nt(qkv[:, 0:DH], qkv[:, DH:2 * DH])
        s = jnp.where(ok, s, fill)
        m = jnp.max(s, axis=-1, keepdims=True)
        p = jnp.exp2((s - m) * cexp)
        l = jnp.sum(p, axis=-1, keepdims=True)
        r = pl.reciprocal(l, approx=True)
        r = r * (2.0 - l * r)
        return (p * r).astype(BF16)

    def w_piece(ci, j):
        return (wa_sc, wb_sc)[ci % 2][ci // 2, j]

    def w_head(g):
        return _unpack(jnp.concatenate(
            [w_piece(3 * (g // HG) + mi, g % HG) for mi in range(3)], axis=1))

    def pre_rows(ref, grp, j):
        return _unpack(jnp.concatenate([ref[3 * grp + mi, j] for mi in range(3)], axis=1))

    def out_proj(n, g0, g1, j):
        return _dot(_unpack(o_sc[0:n // 2, g0 * DH:g1 * DH]),
                    _unpack(wo_sc[g0 * DH // 2:g1 * DH // 2, j * 128:(j + 1) * 128]))

    def attend(proj, n, mask, dist, hook=None):
        D1, D2 = dist
        HA = H - D1 - D2 - 1
        qkvs = {}
        ps = {}
        outs = {}
        for it in range(H + D1 + D2):
            if it < H:
                qkvs[it] = proj(it)
            g = it - D1
            if 0 <= g < H:
                ps[g] = probs(qkvs[g], mask)
            g = it - D1 - D2
            if 0 <= g < H:
                o = _dot(ps.pop(g), qkvs.pop(g)[:, 2 * DH:3 * DH])
                o_sc[0:n // 2, g * DH:(g + 1) * DH] = _pack(o)
            if hook is not None:
                hook(it)
            j = it - (H - 1)
            if 0 <= j < D1 + D2:
                outs[j] = out_proj(n, 0, HA, j)
        for j in range(D1 + D2, NT):
            outs[j] = out_proj(n, 0, H, j)
        for j in range(D1 + D2):
            outs[j] = out_proj(n, HA, H, j) + outs[j]
        return jnp.concatenate([outs[j] for j in range(NT)], axis=1)

    def side1(t):
        x1 = x_sc[seg(t - 1), :].astype(F32) + op_sc[0:SEG, :]
        x2 = x1 + _ln(x1) * y_sc[(t - 1) & 3]
        x2_sc[(t - 1) & 3] = x2
        return _ln(x2).astype(BF16)

    def side2(t):
        x3 = x2_sc[(t - 3) & 3] + op_sc[SEG:, :]
        x4 = x3 + _ln(x3) * y_sc[(t - 3) & 3]
        x4 = x4.astype(out_sc.dtype)
        out_sc[seg(t - 3), :] = x4
        return x4

    def pro_u(s, c):
        conv_u(s)
        return c
    jax.lax.fori_loop(0, 2 * NQ + 2, pro_u, 0, unroll=2)

    def pro_c(q, c):
        uf, kf = conv_fwd(0, q)
        put_spec(0, q, 0, uf)
        put_spec(0, q, 2, kf)
        kr_sc[q] = kf
        ur, um, kr, km = uf[:QB], uf[QB:], kf[:QB], kf[QB:]
        wf_sc[0, q, :QB] = (ur * kr - um * km).astype(BF16)
        wf_sc[0, q, QB:] = (ur * km + um * kr).astype(BF16)
        return c
    for q in range(NQ):
        pro_c(q, 0)

    def pro_s(t, c):
        conv_spec(1, t)
        for piece in MAC_PIECES:
            conv_mac(1, t, piece, 2)
        conv_inv(t)
        return c
    for t in range(2):
        pro_s(t, 0)

    mask1 = make_mask(RH, (0,))

    def wait_chunk(ci):
        with jax.named_scope("wait_w"):
            for cp in w_copies(wq_hbm, 0, ci):
                cp.wait()

    def relayout(ci, dst, slot, b):
        d0 = b * 16 if isinstance(b, int) else pl.multiple_of(b * 16, 16)
        r0 = b * 8 if isinstance(b, int) else pl.multiple_of(b * 8, 8)
        xw = pltpu.bitcast(st_sc[ci, pl.ds(d0, 16)], U32).reshape(8, 2, HG, DH)
        a = xw[:, 0]
        bb = xw[:, 1]
        lo = jnp.swapaxes((a & U32(0xFFFF)) | (bb << 16), 0, 1)
        hi = jnp.swapaxes((a >> 16) | (bb & U32(0xFFFF0000)), 0, 1)
        for j in range(HG):
            rows = pl.ds(r0 + (2 * j // HG) * (DH2 // 2), 8)
            dst[slot, 2 * j % HG, rows, :] = lo[j]
            dst[slot, 2 * j % HG + 1, rows, :] = hi[j]

    NBLK = DH2 // 16

    def fused(cr, dst, rslot, cp, src, pslot):
        S2 = SEG // 2
        cuts = [0] + [RH // 2 + n * S2 for n in range(1, NPRE - 3, 2)] + [RH // 2 + (NPRE - 2) * S2]
        npc = len(cuts) - 1

        def body(i, c):
            done = 0
            for j in range(HG):
                w = _unpack(src[pslot, j])
                for pi in range(npc):
                    upto = min(NBLK, -(-(j * npc + pi + 1) * NBLK // (HG * npc - 2)))
                    for bb in range(done, upto):
                        relayout(cr, dst, rslot, bb)
                    done = upto
                    lo, hi = cuts[pi], cuts[pi + 1]
                    r = _pack(_dot(_unpack(hp_sc[lo:hi, :]), w))
                    if pi == 0:
                        pre0_sc[cp, j] = r[0:RH // 2]
                    for sg in range(NPRE - 2):
                        a = RH // 2 + sg * S2
                        if lo <= a < hi:
                            pre_sc[sg, cp, j] = r[a - lo:a - lo + S2]
            return c
        with jax.named_scope("fused"):
            jax.lax.fori_loop(0, never_sm[0] + 1, body, 0)

    wait_chunk(0)

    def relayout0(b, c):
        relayout(0, wa_sc, 0, b)
        return c
    with jax.named_scope("relayout"):
        jax.lax.fori_loop(0, NBLK, relayout0, 0, unroll=2)

    KL = NCH // 2 - 1

    def chunk_pair(k, carry):
        wait_chunk(2 * k + 1)
        kc = jnp.minimum(k + never_sm[0], KL)
        fused(2 * kc + 1, wb_sc, kc, 2 * k, wa_sc, k)

        @pl.when(k < KL)
        def _():
            wait_chunk(2 * k + 2)
        kn = jnp.minimum(k + 1, KL)
        fused(2 * kn, wa_sc, kn, 2 * k + 1, wb_sc, k)
        return carry
    jax.lax.fori_loop(0, KL + 1, chunk_pair, 0)

    with jax.named_scope("wait_wo"):
        wo_copy.wait()
    ps = {}
    os_ = []
    out = None
    GW, E1, E2 = 4, 2, 1
    for it in range(H // GW + E1 + E2):
        for j in range(it * GW, (it + 1) * GW):
            if j < H:
                ps[j] = probs(pre_rows(pre0_sc, j // HG, j % HG), mask1)
        for j in range((it - E1) * GW, (it - E1 + 1) * GW):
            if 0 <= j < H:
                os_.append(_dot(ps.pop(j), _unpack(pre0_sc[3 * (j // HG) + 2, j % HG])).astype(BF16))
        g0 = (it - E1 - E2) * GW
        if g0 >= 0:
            wo = wo_st[g0 * DH:(g0 + GW) * DH, :]
            wo_sc[g0 * DH // 2:(g0 + GW) * DH // 2, :] = _pack(wo)
            part = _dot(jnp.concatenate(os_[g0:g0 + GW], axis=1), wo)
            out = part if out is None else part + out
    h_sc[0:M2, :] = jnp.concatenate([out[0:M], mem0], axis=0).astype(BF16)
    op_sc[0:SEG, :] = out[M2:]

    mask12 = make_mask(R, (0, 1))

    def pinned(never, h, pins):
        hs = {0: h}
        r = _pack(h[-SEG:])
        for g, d in pins:
            r = jnp.where(never, _pack(d), r)
            hs[g] = jnp.concatenate([h[:-SEG], _unpack(r)], axis=0)
        return lambda g: hs[max(k for k in hs if k <= g)]

    def step(t, pre, spec_first=False):
        c = t // NQ + 1
        q = t % NQ
        if spec_first:
            conv_spec(c, q)
        x4 = side2(t)
        xn2 = side1(t)
        xn1 = _ln(x_sc[seg(t + 1), :].astype(F32)).astype(BF16)
        un = conv_u(t + 2 * NQ)
        pins = list(zip(PINS, (un, xn1, x4, xn2)))
        never = never_sm[0] > 0
        if pre:
            h = pinned(never, jnp.concatenate([h_sc[0:M2, :], h_sc[RH:, :]], axis=0), pins)

            def proj(g):
                r = _dot(h(g), w_head(g)).astype(BF16)
                x1 = pre_rows(pre_sc.at[t - 2], g // HG, g % HG)
                return jnp.concatenate([r[0:M2], x1, r[M2:]], axis=0)
            nterms = (NPRE - 1) // NQ + 2
        else:
            h = pinned(never, h_sc[...], pins)

            def proj(g):
                return _dot(h(g), w_head(g)).astype(BF16)
            nterms = NB
        h_sc[M2:RH, :] = xn1
        h_sc[RH:, :] = xn2

        def hook(it):
            if it == SPEC_AT and not spec_first:
                conv_spec(c, q)
            if it == SPEC_AT + 1:
                for piece in MAC_PIECES:
                    conv_mac(c, q, piece, nterms)
        out = attend(proj, R, mask12, DIST_PRE if pre else DIST, hook)
        conv_inv(t)
        h_sc[0:M2, :] = out[0:M2].astype(BF16)
        op_sc[...] = out[M2:]

    def step_pre(t, carry):
        step(t, True)
        return carry

    def step_full(i, carry):
        for j in range(UNROLL):
            step(i * UNROLL + j, False, j > 0)
        return carry

    def phase(p, carry):
        @pl.when(p >= 2)
        def _():
            out_copy(p - 2).start()

        with jax.named_scope("steps"):
            jax.lax.fori_loop(jnp.maximum(p * PH, NPRE) // UNROLL, (p * PH + PH) // UNROLL, step_full, 0)
        return carry

    mask2 = make_mask(RH, (1,))

    def step_half(t, carry):
        first = t < NSEG
        lo = pl.multiple_of(jnp.where(first, 0, SEG), SEG)
        mask = (jnp.where(first, mask1[0].astype(jnp.int32), mask2[0].astype(jnp.int32)) > 0,
                jnp.where(first, mask1[1], mask2[1]))
        h = jnp.concatenate([h_sc[0:M2, :], h_sc[pl.ds(pl.multiple_of(M2 + lo, 16), SEG), :]], axis=0)
        side2(t)
        xn2 = side1(t)
        out = attend(lambda g: _dot(h, w_head(g)).astype(BF16), RH, mask, DIST_HALF)
        m2 = jnp.where(first, mem0, out[M:M2])
        h_sc[0:M2, :] = jnp.concatenate([out[0:M], m2], axis=0).astype(BF16)
        h_sc[RH:, :] = xn2
        op_sc[pl.ds(lo, SEG), :] = out[M2:]
        return carry

    def stage(i, carry):
        with jax.named_scope("steps_half"):
            jax.lax.fori_loop(jnp.where(i == 0, 1, NSEG), jnp.where(i == 0, 2, NSEG + 2), step_half, 0)

        @pl.when(i == 0)
        def _():
            for cp in in_copies(1):
                cp.wait()
            with jax.named_scope("steps_pre"):
                jax.lax.fori_loop(2, NPRE, step_pre, 0)
            for cp in in_copies(2):
                cp.wait()
            jax.lax.fori_loop(NPRE // PH, NPH, phase, 0)
            out_copy(NPH - 2).start()
            out_tail(0).start()
        return carry

    jax.lax.fori_loop(0, 2, stage, 0)
    side2(NSEG + 2)
    out_tail(1).start()
    for i in range(NPH - 1):
        out_copy(i).wait()
    out_tail(0).wait()
    out_tail(1).wait()


def pallas_interleave_layers__memory_aug_recurrent_mem_tr__ssm_conv_h3__prompt_kernel(
    A_x, A_mem0, A_Wq, A_Wk, A_Wv, A_Wo, A_seg_len,
    B_q, B_k, B_v, B_shift_k, B_ssm_k, B_ssm_D,
):
    del B_q
    seg = int(A_seg_len) if isinstance(A_seg_len, (int, np.integer)) else CB // NQ
    return _run(A_x, A_mem0, A_Wq, A_Wk, A_Wv, A_Wo, B_k, B_v, B_shift_k, B_ssm_k, B_ssm_D, SEG=seg)


@functools.partial(jax.jit, static_argnames=("SEG",))
def _run(A_x, A_mem0, A_Wq, A_Wk, A_Wv, A_Wo, B_k, B_v, B_shift_k, B_ssm_k, B_ssm_D, *, SEG):
    B, S, DM = A_x.shape
    assert B == 1
    H, DH = A_Wq.shape[1], A_Wq.shape[2]
    M = A_mem0.shape[1]
    KS = B_shift_k.shape[1]
    R = 2 * (M + SEG)
    RP = 2 * M + (NPRE - 1) * SEG
    NB = S // CB
    QB = CB // NQ
    NCH = 3 * H // HG
    fwd, inv = _dft_constants()

    kern = functools.partial(_kernel, S=S, DM=DM, H=H, DH=DH, M=M, SEG=SEG)
    any_spec = pl.BlockSpec(memory_space=pl.ANY)
    out = pl.pallas_call(
        kern,
        out_shape=jax.ShapeDtypeStruct((S, DM), A_x.dtype),
        in_specs=[any_spec] * 13,
        out_specs=any_spec,
        scratch_shapes=[
            pltpu.VMEM((NB + 2, NQ, QB // 8, DM // 128, 4, 8, 128), F32),
            pltpu.VMEM((NQ, 2 * QB, DM), F32),
            pltpu.VMEM((2, NQ, 2 * QB, DM), BF16),
            pltpu.VMEM((4, SEG, DM), F32),
            pltpu.VMEM((4, SEG, DM), F32),
            pltpu.VMEM((S, DM), BF16),
            pltpu.VMEM((2 * SEG, DM), F32),
            pltpu.VMEM((NPRE - 2, NCH, HG, SEG // 2, DH), U32),
            pltpu.VMEM((NCH, HG, M + SEG // 2, DH), U32),
            pltpu.VMEM((NCH // 2, HG, DM // 2, DH), U32),
            pltpu.VMEM((NCH // 2, HG, DM // 2, DH), U32),
            pltpu.VMEM((H * DH // 2, DM), U32),
            pltpu.VMEM((R // 2, H * DH), U32),
            pltpu.VMEM((S, DM), BF16),
            pltpu.VMEM((S, DM), BF16),
            pltpu.VMEM((DM, S), BF16),
            pltpu.VMEM((NCH, DM // 2, 2 * HG, DH), BF16),
            pltpu.VMEM((H * DH, DM), BF16),
            pltpu.VMEM((S, DM), A_x.dtype),
            pltpu.VMEM(fwd.shape, BF16),
            pltpu.VMEM(inv.shape, BF16),
            pltpu.VMEM((S + KPAD, DM), BF16),
            pltpu.VMEM((RP // 2, DM), U32),
            pltpu.VMEM((R, DM), BF16),
            pltpu.VMEM((M, DM), BF16),
            pltpu.VMEM((KS, DM), BF16),
            pltpu.VMEM((DM,), BF16),
            pltpu.SMEM((1,), jnp.int32),
            pltpu.SemaphoreType.DMA((5,)),
            pltpu.SemaphoreType.DMA((12,)),
            pltpu.SemaphoreType.DMA((2 * NCH + 1,)),
            pltpu.SemaphoreType.DMA((S // SEG // PH + 1,)),
        ],
        compiler_params=pltpu.CompilerParams(vmem_limit_bytes=120 * 1024 * 1024),
    )(
        A_x.reshape(S, DM), A_mem0.reshape(M, DM), A_Wq, A_Wk, A_Wv,
        A_Wo.reshape(H * DH, DM), B_k.reshape(S, DM), B_v.reshape(S, DM),
        B_shift_k.T, B_ssm_k, B_ssm_D,
        jnp.asarray(fwd, BF16), jnp.asarray(inv, BF16),
    )
    return out.reshape(B, S, DM)
```

```python
import functools

import numpy as np
import jax
import jax.numpy as jnp
import jax.experimental.pallas as pl
import jax.experimental.pallas.tpu as pltpu

F32 = jnp.float32
BF16 = jnp.bfloat16
U32 = jnp.uint32

CB = 128
NQ = 4
KPAD = 16
PH = 8
NPRE = 10
PINS = (3, 12, 16, 20)
SPEC_AT = 4
UNROLL = 2
HG = 8
DIST, DIST_PRE, DIST_HALF = (1, 2), (2, 3), (1, 3)


def _dft_constants():
    qb = CB // NQ
    n = np.arange(CB, dtype=np.float64)
    fwd = np.zeros((NQ, 2 * qb, CB))
    for q in range(NQ):
        f = q * qb + np.concatenate([np.arange(0, qb, 2), np.arange(1, qb, 2)])
        ang = (np.pi * (2.0 * f + 1.0) / (2 * CB))[:, None] * n[None, :]
        fwd[q, :qb] = np.cos(ang)
        fwd[q, qb:] = -np.sin(ang)
    inv = fwd.reshape(2 * CB, CB).T / CB
    return fwd.astype(np.float32), inv.reshape(NQ, CB // NQ, 2 * CB).astype(np.float32)


def _ln(x, eps=1e-5):
    d = x.shape[-1]
    m = jnp.sum(x, axis=-1, keepdims=True) * (1.0 / d)
    xc = x - m
    v = jnp.sum(xc * xc, axis=-1, keepdims=True) * (1.0 / d)
    return xc * jax.lax.rsqrt(v + eps)


def _dot(a, b):
    return jnp.dot(a, b, preferred_element_type=F32)


def _dot_nt(a, b):
    return jax.lax.dot_general(a, b, (((1,), (1,)), ((), ())), preferred_element_type=F32)


def _pack(x):
    return pltpu.bitcast(x.astype(BF16), U32)


def _unpack(x):
    return pltpu.bitcast(x, BF16)


def _in_order(actions):
    def body(i, c):
        for j, act in enumerate(actions):
            pl.when(i == j)(act)
        return c
    jax.lax.fori_loop(0, len(actions), body, 0)


def _kernel(x_hbm, mem0_hbm, wq_hbm, wk_hbm, wv_hbm, wo_hbm, k_hbm, v_hbm,
            sh_hbm, sk_hbm, sd_hbm, fwd_hbm, inv_hbm, o_hbm,
            sp_sc, kr_sc, wf_sc, x2_sc, y_sc, u_sc, op_sc, pre_sc, pre0_sc, wa_sc, wb_sc, wo_sc, o_sc,
            x_sc, v_sc, sk_sc, st_sc, wo_st, out_sc, fwd_ref, inv_ref,
            k_sc, hp_sc, h_sc, mem0_ref, sh_ref, sd_ref,
            never_sm, sem_in, sem_w, sem_out,
            *, S, DM, H, DH, M, SEG):
    NSEG = S // SEG
    M2 = 2 * M
    R = M2 + 2 * SEG
    RH = M2 + SEG
    NB = S // CB
    QB = CB // NQ
    HB = QB // 2
    NT = DM // 128
    assert QB == SEG and NSEG % PH == 0 and NPRE % UNROLL == 0 and PH % UNROLL == 0
    NPH = NSEG // PH
    NCH = 3 * H // HG
    DH2 = DM // 2

    small = [pltpu.make_async_copy(s, d, sem_in.at[min(i, 1)]) for i, (s, d) in enumerate([
        (mem0_hbm, mem0_ref), (sh_hbm, sh_ref), (sd_hbm, sd_ref), (fwd_hbm, fwd_ref), (inv_hbm, inv_ref)])]

    xb = (0, NPRE * SEG, (NPRE + 1) * SEG, S)
    kb = (0, (2 * NQ + 2) * SEG, (2 * NQ + NPRE) * SEG, S)
    sb = (0, 2 * CB, ((NPRE - 1) // NQ + 2) * CB, S)

    def in_copies(part):
        def rng(b):
            return pl.ds(b[part], b[part + 1] - b[part])
        sem = sem_in.at[part + 1]
        return [
            pltpu.make_async_copy(x_hbm.at[rng(xb)], x_sc.at[rng(xb)], sem if part else sem_in.at[0]),
            pltpu.make_async_copy(k_hbm.at[rng(kb)],
                                  k_sc.at[pl.ds(KPAD + kb[part], kb[part + 1] - kb[part])], sem),
            pltpu.make_async_copy(v_hbm.at[rng(kb)], v_sc.at[rng(kb)], sem),
            pltpu.make_async_copy(sk_hbm.at[:, rng(sb)], sk_sc.at[:, rng(sb)], sem),
        ]

    def w_copies(src, g, ci):
        return [pltpu.make_async_copy(src.at[pl.ds(hf * DH2, DH2), pl.ds(pl.multiple_of(g * HG, HG), HG), :],
                                      st_sc.at[ci, :, pl.ds(hf * HG, HG), :], sem_w.at[ci])
                for hf in range(2)]

    wo_copy = pltpu.make_async_copy(wo_hbm, wo_st, sem_w.at[NCH])

    def out_copy(i):
        rows = pl.ds(pl.multiple_of(i * PH * SEG, PH * SEG), PH * SEG)
        return pltpu.make_async_copy(out_sc.at[rows], o_hbm.at[rows], sem_out)

    def out_tail(j):
        b = ((NPH - 1) * PH * SEG, (NSEG - 3) * SEG, S)
        rows = pl.ds(b[j], b[j + 1] - b[j])
        return pltpu.make_async_copy(out_sc.at[rows], o_hbm.at[rows], sem_out)

    def start_all(cps):
        def act():
            for cp in cps:
                cp.start()
        return act

    in0 = in_copies(0)
    _in_order([start_all(small[:1] + in0[:1]), start_all(small[1:] + in0[1:])])

    def start_group(g, c):
        _in_order([start_all(w_copies(src, g, 3 * g + mi))
                   for mi, src in enumerate((wq_hbm, wk_hbm, wv_hbm))])
        return c
    jax.lax.fori_loop(0, H // HG, start_group, 0)
    _in_order([start_all([wo_copy]), start_all(in_copies(1)), start_all(in_copies(2))])

    never_sm[0] = 0
    k_sc[0:KPAD, :] = jnp.zeros((KPAD, DM), BF16)
    sp_sc[NB + 1] = jnp.zeros(sp_sc.shape[1:], F32)
    op_sc[...] = jnp.zeros(op_sc.shape, F32)
    x2_sc[...] = jnp.zeros(x2_sc.shape, F32)
    y_sc[...] = jnp.zeros(y_sc.shape, F32)
    h_sc[...] = jnp.zeros(h_sc.shape, BF16)
    for cp in small[:1] + in0[:1]:
        cp.wait()

    mem0 = mem0_ref[...].astype(F32)
    hp_sc[0:M, :] = _pack(jnp.concatenate([mem0, mem0], axis=0))
    for sg in range(NPRE):
        xn = _ln(x_sc[sg * SEG:(sg + 1) * SEG, :].astype(F32))
        if sg == 1:
            h_sc[M2:RH, :] = xn.astype(BF16)
        else:
            w0 = M + max(sg - 1, 0) * (SEG // 2)
            hp_sc[w0:w0 + SEG // 2, :] = _pack(xn)

    for cp in small[1:] + in0[1:]:
        cp.wait()

    sh = sh_ref[...].astype(F32)
    KS = sh.shape[0]
    sd = sd_ref[...].astype(F32).reshape(1, DM)

    def seg(i):
        i = jnp.clip(i, 0, NSEG - 1)
        return pl.ds(pl.multiple_of(i * SEG, SEG), SEG)

    def conv_u(s):
        s = jnp.clip(s, 0, NSEG - 1)
        r0 = pl.multiple_of(s * SEG, SEG)
        kk = k_sc[pl.ds(r0, KPAD + SEG), :].astype(F32)
        ks = kk[KPAD:] * sh[0:1]
        for j in range(1, KS):
            ks = ks + pltpu.roll(kk, j, 0)[KPAD:] * sh[j:j + 1]
        u = (ks * v_sc[pl.ds(r0, SEG), :].astype(F32)).astype(BF16)
        u_sc[pl.ds(r0, SEG), :] = u
        return u

    def conv_fwd(c, q):
        cc = jnp.minimum(c, NB - 1)
        t0 = pl.multiple_of(cc * CB, CB)
        f = fwd_ref[q]
        uf = _dot(f, u_sc[pl.ds(t0, CB), :])
        kf = _dot_nt(f, sk_sc[:, pl.ds(t0, CB)])
        return uf, kf

    def put_spec(cs, q, which, val):
        for rb in range(QB // 8):
            for n in range(NT):
                ln = slice(n * 128, (n + 1) * 128)
                sp_sc[cs, q, rb, n, which] = val[rb * 8:rb * 8 + 8, ln]
                sp_sc[cs, q, rb, n, which + 1] = val[QB + rb * 8:QB + rb * 8 + 8, ln]

    def conv_spec(c, q):
        uf, kf = conv_fwd(c, q)
        cs = jnp.minimum(c, NB)
        put_spec(cs, q, 0, uf)
        pk = kr_sc[q]
        kr_sc[q] = kf
        kp = jnp.concatenate([
            kf[0:HB] - pk[QB:QB + HB],
            kf[HB:QB] + pk[QB + HB:],
            kf[QB:QB + HB] + pk[0:HB],
            kf[QB + HB:] - pk[HB:QB]], axis=0)
        put_spec(cs, q, 2, kp)

    MAC_PIECES = [(rb, n) for rb in range(QB // 16) for n in range(NT)]

    def conv_mac(c, q, piece, nterms):
        rb2, n = piece
        cs = jnp.minimum(c, NB)
        acc = []
        for rb in (2 * rb2, 2 * rb2 + 1):
            ar = None
            ai = None
            for j in range(nterms):
                uj = jnp.minimum(j, cs)
                kj = jnp.where(cs - j >= 0, cs - j, NB + 1)
                ur = sp_sc[uj, q, rb, n, 0]
                um = sp_sc[uj, q, rb, n, 1]
                kr = sp_sc[kj, q, rb, n, 2]
                km = sp_sc[kj, q, rb, n, 3]
                tr = ur * kr - um * km
                ti = ur * km + um * kr
                ar = tr if ar is None else ar + tr
                ai = ti if ai is None else ai + ti
            acc.append((ar, ai))
        ln = slice(n * 128, (n + 1) * 128)
        wf_sc[c & 1, q, rb2 * 16:rb2 * 16 + 16, ln] = jnp.concatenate(
            [acc[0][0], acc[1][0]], axis=0).astype(BF16)
        wf_sc[c & 1, q, QB + rb2 * 16:QB + rb2 * 16 + 16, ln] = jnp.concatenate(
            [acc[0][1], acc[1][1]], axis=0).astype(BF16)

    def conv_inv(s):
        w = wf_sc[(s // NQ) & 1].reshape(2 * CB, DM)
        yc = _dot(inv_ref[s % NQ], w)
        y_sc[s & 3] = yc + u_sc[seg(s), :].astype(F32) * sd

    scale = DH ** -0.5
    cexp = scale * float(np.log2(np.e))

    def make_mask(n, x_layers):
        qi = jax.lax.broadcasted_iota(jnp.int32, (n, n), 0)
        ki = jax.lax.broadcasted_iota(jnp.int32, (n, n), 1)

        def layer(i):
            xl = jnp.where(i < M2 + SEG, x_layers[0], x_layers[-1])
            return jnp.where(i < M, 0, jnp.where(i < M2, 1, xl))
        same = layer(qi) == layer(ki)
        ok = same & ((qi < M2) | (ki < M2) | (qi >= ki))
        fill = jnp.where(same, -1e9 / scale, -jnp.inf).astype(F32)
        return ok, fill

    def probs(qkv, mask):
        ok, fill = mask
        s = _dot_nt(qkv[:, 0:DH], qkv[:, DH:2 * DH])
        s = jnp.where(ok, s, fill)
        m = jnp.max(s, axis=-1, keepdims=True)
        p = jnp.exp2((s - m) * cexp)
        l = jnp.sum(p, axis=-1, keepdims=True)
        r = pl.reciprocal(l, approx=True)
        r = r * (2.0 - l * r)
        return (p * r).astype(BF16)

    def w_piece(ci, j):
        return (wa_sc, wb_sc)[ci % 2][ci // 2, j]

    def w_head(g):
        return _unpack(jnp.concatenate(
            [w_piece(3 * (g // HG) + mi, g % HG) for mi in range(3)], axis=1))

    def pre_rows(ref, grp, j):
        return _unpack(jnp.concatenate([ref[3 * grp + mi, j] for mi in range(3)], axis=1))

    def out_proj(n, g0, g1, j):
        return _dot(_unpack(o_sc[0:n // 2, g0 * DH:g1 * DH]),
                    _unpack(wo_sc[g0 * DH // 2:g1 * DH // 2, j * 128:(j + 1) * 128]))

    def attend(proj, n, mask, dist, hook=None):
        D1, D2 = dist
        HA = H - D1 - D2 - 1
        qkvs = {}
        ps = {}
        outs = {}
        for it in range(H + D1 + D2):
            if it < H:
                qkvs[it] = proj(it)
            g = it - D1
            if 0 <= g < H:
                ps[g] = probs(qkvs[g], mask)
            g = it - D1 - D2
            if 0 <= g < H:
                o = _dot(ps.pop(g), qkvs.pop(g)[:, 2 * DH:3 * DH])
                o_sc[0:n // 2, g * DH:(g + 1) * DH] = _pack(o)
            if hook is not None:
                hook(it)
            j = it - (H - 1)
            if 0 <= j < D1 + D2:
                outs[j] = out_proj(n, 0, HA, j)
        for j in range(D1 + D2, NT):
            outs[j] = out_proj(n, 0, H, j)
        for j in range(D1 + D2):
            outs[j] = out_proj(n, HA, H, j) + outs[j]
        return jnp.concatenate([outs[j] for j in range(NT)], axis=1)

    def side1(t):
        x1 = x_sc[seg(t - 1), :].astype(F32) + op_sc[0:SEG, :]
        x2 = x1 + _ln(x1) * y_sc[(t - 1) & 3]
        x2_sc[(t - 1) & 3] = x2
        return _ln(x2).astype(BF16)

    def side2(t):
        x3 = x2_sc[(t - 3) & 3] + op_sc[SEG:, :]
        x4 = x3 + _ln(x3) * y_sc[(t - 3) & 3]
        x4 = x4.astype(out_sc.dtype)
        out_sc[seg(t - 3), :] = x4
        return x4

    def pro_u(s, c):
        conv_u(s)
        return c
    jax.lax.fori_loop(0, 2 * NQ + 2, pro_u, 0, unroll=2)

    def pro_c(q, c):
        uf, kf = conv_fwd(0, q)
        put_spec(0, q, 0, uf)
        put_spec(0, q, 2, kf)
        kr_sc[q] = kf
        ur, um, kr, km = uf[:QB], uf[QB:], kf[:QB], kf[QB:]
        wf_sc[0, q, :QB] = (ur * kr - um * km).astype(BF16)
        wf_sc[0, q, QB:] = (ur * km + um * kr).astype(BF16)
        return c
    for q in range(NQ):
        pro_c(q, 0)

    def pro_s(t, c):
        conv_spec(1, t)
        for piece in MAC_PIECES:
            conv_mac(1, t, piece, 2)
        conv_inv(t)
        return c
    for t in range(2):
        pro_s(t, 0)

    mask1 = make_mask(RH, (0,))

    def wait_chunk(ci):
        with jax.named_scope("wait_w"):
            for cp in w_copies(wq_hbm, 0, ci):
                cp.wait()

    def relayout(ci, dst, slot, b):
        d0 = b * 16 if isinstance(b, int) else pl.multiple_of(b * 16, 16)
        r0 = b * 8 if isinstance(b, int) else pl.multiple_of(b * 8, 8)
        xw = pltpu.bitcast(st_sc[ci, pl.ds(d0, 16)], U32).reshape(8, 2, HG, DH)
        a = xw[:, 0]
        bb = xw[:, 1]
        lo = jnp.swapaxes((a & U32(0xFFFF)) | (bb << 16), 0, 1)
        hi = jnp.swapaxes((a >> 16) | (bb & U32(0xFFFF0000)), 0, 1)
        for j in range(HG):
            rows = pl.ds(r0 + (2 * j // HG) * (DH2 // 2), 8)
            dst[slot, 2 * j % HG, rows, :] = lo[j]
            dst[slot, 2 * j % HG + 1, rows, :] = hi[j]

    NBLK = DH2 // 16

    def fused(cr, dst, rslot, cp, src, pslot):
        S2 = SEG // 2
        cuts = [0] + [RH // 2 + n * S2 for n in range(0, NPRE - 1, 2)]
        npc = len(cuts) - 1

        def body(i, c):
            done = 0
            for j in range(HG):
                w = _unpack(src[pslot, j])
                for pi in range(npc):
                    upto = min(NBLK, -(-(j * npc + pi) * NBLK // (HG * npc - 1)))
                    for bb in range(done, upto):
                        relayout(cr, dst, rslot, bb)
                    done = upto
                    lo, hi = cuts[pi], cuts[pi + 1]
                    r = _pack(_dot(_unpack(hp_sc[lo:hi, :]), w))
                    if pi == 0:
                        pre0_sc[cp, j] = r[0:RH // 2]
                    for sg in range(NPRE - 2):
                        a = RH // 2 + sg * S2
                        if lo <= a < hi:
                            pre_sc[sg, cp, j] = r[a - lo:a - lo + S2]
            return c
        with jax.named_scope("fused"):
            jax.lax.fori_loop(0, never_sm[0] + 1, body, 0)

    wait_chunk(0)

    def relayout0(b, c):
        relayout(0, wa_sc, 0, b)
        return c
    with jax.named_scope("relayout"):
        jax.lax.fori_loop(0, NBLK, relayout0, 0, unroll=2)

    KL = NCH // 2 - 1

    def chunk_pair(k, carry):
        wait_chunk(2 * k + 1)
        kc = jnp.minimum(k + never_sm[0], KL)
        fused(2 * kc + 1, wb_sc, kc, 2 * k, wa_sc, k)

        @pl.when(k < KL)
        def _():
            wait_chunk(2 * k + 2)
        kn = jnp.minimum(k + 1, KL)
        fused(2 * kn, wa_sc, kn, 2 * k + 1, wb_sc, k)
        return carry
    jax.lax.fori_loop(0, KL + 1, chunk_pair, 0)

    with jax.named_scope("wait_wo"):
        wo_copy.wait()
    ps = {}
    os_ = []
    out = None
    GW, E1, E2 = 4, 2, 1
    for it in range(H // GW + E1 + E2):
        for j in range(it * GW, (it + 1) * GW):
            if j < H:
                ps[j] = probs(pre_rows(pre0_sc, j // HG, j % HG), mask1)
        for j in range((it - E1) * GW, (it - E1 + 1) * GW):
            if 0 <= j < H:
                os_.append(_dot(ps.pop(j), _unpack(pre0_sc[3 * (j // HG) + 2, j % HG])).astype(BF16))
        g0 = (it - E1 - E2) * GW
        if g0 >= 0:
            wo = wo_st[g0 * DH:(g0 + GW) * DH, :]
            wo_sc[g0 * DH // 2:(g0 + GW) * DH // 2, :] = _pack(wo)
            part = _dot(jnp.concatenate(os_[g0:g0 + GW], axis=1), wo)
            out = part if out is None else part + out
    h_sc[0:M2, :] = jnp.concatenate([out[0:M], mem0], axis=0).astype(BF16)
    op_sc[0:SEG, :] = out[M2:]

    mask12 = make_mask(R, (0, 1))

    def pinned(never, h, pins):
        hs = {0: h}
        r = _pack(h[-SEG:])
        for g, d in pins:
            r = jnp.where(never, _pack(d), r)
            hs[g] = jnp.concatenate([h[:-SEG], _unpack(r)], axis=0)
        return lambda g: hs[max(k for k in hs if k <= g)]

    def step(t, pre, spec_first=False):
        c = t // NQ + 1
        q = t % NQ
        if spec_first:
            conv_spec(c, q)
        x4 = side2(t)
        xn2 = side1(t)
        xn1 = _ln(x_sc[seg(t + 1), :].astype(F32)).astype(BF16)
        un = conv_u(t + 2 * NQ)
        pins = list(zip(PINS, (un, xn1, x4, xn2)))
        never = never_sm[0] > 0
        if pre:
            h = pinned(never, jnp.concatenate([h_sc[0:M2, :], h_sc[RH:, :]], axis=0), pins)

            def proj(g):
                r = _dot(h(g), w_head(g)).astype(BF16)
                x1 = pre_rows(pre_sc.at[t - 2], g // HG, g % HG)
                return jnp.concatenate([r[0:M2], x1, r[M2:]], axis=0)
            nterms = (NPRE - 1) // NQ + 2
        else:
            h = pinned(never, h_sc[...], pins)

            def proj(g):
                return _dot(h(g), w_head(g)).astype(BF16)
            nterms = NB
        h_sc[M2:RH, :] = xn1
        h_sc[RH:, :] = xn2

        def hook(it):
            if it == SPEC_AT and not spec_first:
                conv_spec(c, q)
            if it == SPEC_AT + 1:
                for piece in MAC_PIECES:
                    conv_mac(c, q, piece, nterms)
        out = attend(proj, R, mask12, DIST_PRE if pre else DIST, hook)
        conv_inv(t)
        h_sc[0:M2, :] = out[0:M2].astype(BF16)
        op_sc[...] = out[M2:]

    def step_pre(t, carry):
        step(t, True)
        return carry

    def step_full(i, carry):
        for j in range(UNROLL):
            step(i * UNROLL + j, False, j > 0)
        return carry

    def phase(p, carry):
        @pl.when(p >= 2)
        def _():
            out_copy(p - 2).start()

        with jax.named_scope("steps"):
            jax.lax.fori_loop(jnp.maximum(p * PH, NPRE) // UNROLL, (p * PH + PH) // UNROLL, step_full, 0)
        return carry

    mask2 = make_mask(RH, (1,))

    def step_half(t, carry):
        first = t < NSEG
        lo = pl.multiple_of(jnp.where(first, 0, SEG), SEG)
        mask = (jnp.where(first, mask1[0].astype(jnp.int32), mask2[0].astype(jnp.int32)) > 0,
                jnp.where(first, mask1[1], mask2[1]))
        h = jnp.concatenate([h_sc[0:M2, :], h_sc[pl.ds(pl.multiple_of(M2 + lo, 16), SEG), :]], axis=0)
        side2(t)
        xn2 = side1(t)
        out = attend(lambda g: _dot(h, w_head(g)).astype(BF16), RH, mask, DIST_HALF)
        m2 = jnp.where(first, mem0, out[M:M2])
        h_sc[0:M2, :] = jnp.concatenate([out[0:M], m2], axis=0).astype(BF16)
        h_sc[RH:, :] = xn2
        op_sc[pl.ds(lo, SEG), :] = out[M2:]
        return carry

    def stage(i, carry):
        with jax.named_scope("steps_half"):
            jax.lax.fori_loop(jnp.where(i == 0, 1, NSEG), jnp.where(i == 0, 2, NSEG + 2), step_half, 0)

        @pl.when(i == 0)
        def _():
            for cp in in_copies(1):
                cp.wait()
            with jax.named_scope("steps_pre"):
                jax.lax.fori_loop(2, NPRE, step_pre, 0)
            for cp in in_copies(2):
                cp.wait()
            jax.lax.fori_loop(NPRE // PH, NPH, phase, 0)
            out_copy(NPH - 2).start()
            out_tail(0).start()
        return carry

    jax.lax.fori_loop(0, 2, stage, 0)
    side2(NSEG + 2)
    out_tail(1).start()
    pltpu.make_async_copy(out_sc, o_hbm, sem_out).wait()


def pallas_interleave_layers__memory_aug_recurrent_mem_tr__ssm_conv_h3__prompt_kernel(
    A_x, A_mem0, A_Wq, A_Wk, A_Wv, A_Wo, A_seg_len,
    B_q, B_k, B_v, B_shift_k, B_ssm_k, B_ssm_D,
):
    del B_q
    seg = int(A_seg_len) if isinstance(A_seg_len, (int, np.integer)) else CB // NQ
    return _run(A_x, A_mem0, A_Wq, A_Wk, A_Wv, A_Wo, B_k, B_v, B_shift_k, B_ssm_k, B_ssm_D, SEG=seg)


@functools.partial(jax.jit, static_argnames=("SEG",))
def _run(A_x, A_mem0, A_Wq, A_Wk, A_Wv, A_Wo, B_k, B_v, B_shift_k, B_ssm_k, B_ssm_D, *, SEG):
    B, S, DM = A_x.shape
    assert B == 1
    H, DH = A_Wq.shape[1], A_Wq.shape[2]
    M = A_mem0.shape[1]
    KS = B_shift_k.shape[1]
    R = 2 * (M + SEG)
    RP = 2 * M + (NPRE - 1) * SEG
    NB = S // CB
    QB = CB // NQ
    NCH = 3 * H // HG
    fwd, inv = _dft_constants()

    kern = functools.partial(_kernel, S=S, DM=DM, H=H, DH=DH, M=M, SEG=SEG)
    any_spec = pl.BlockSpec(memory_space=pl.ANY)
    out = pl.pallas_call(
        kern,
        out_shape=jax.ShapeDtypeStruct((S, DM), A_x.dtype),
        in_specs=[any_spec] * 13,
        out_specs=any_spec,
        scratch_shapes=[
            pltpu.VMEM((NB + 2, NQ, QB // 8, DM // 128, 4, 8, 128), F32),
            pltpu.VMEM((NQ, 2 * QB, DM), F32),
            pltpu.VMEM((2, NQ, 2 * QB, DM), BF16),
            pltpu.VMEM((4, SEG, DM), F32),
            pltpu.VMEM((4, SEG, DM), F32),
            pltpu.VMEM((S, DM), BF16),
            pltpu.VMEM((2 * SEG, DM), F32),
            pltpu.VMEM((NPRE - 2, NCH, HG, SEG // 2, DH), U32),
            pltpu.VMEM((NCH, HG, M + SEG // 2, DH), U32),
            pltpu.VMEM((NCH // 2, HG, DM // 2, DH), U32),
            pltpu.VMEM((NCH // 2, HG, DM // 2, DH), U32),
            pltpu.VMEM((H * DH // 2, DM), U32),
            pltpu.VMEM((R // 2, H * DH), U32),
            pltpu.VMEM((S, DM), BF16),
            pltpu.VMEM((S, DM), BF16),
            pltpu.VMEM((DM, S), BF16),
            pltpu.VMEM((NCH, DM // 2, 2 * HG, DH), BF16),
            pltpu.VMEM((H * DH, DM), BF16),
            pltpu.VMEM((S, DM), A_x.dtype),
            pltpu.VMEM(fwd.shape, BF16),
            pltpu.VMEM(inv.shape, BF16),
            pltpu.VMEM((S + KPAD, DM), BF16),
            pltpu.VMEM((RP // 2, DM), U32),
            pltpu.VMEM((R, DM), BF16),
            pltpu.VMEM((M, DM), BF16),
            pltpu.VMEM((KS, DM), BF16),
            pltpu.VMEM((DM,), BF16),
            pltpu.SMEM((1,), jnp.int32),
            pltpu.SemaphoreType.DMA((4,)),
            pltpu.SemaphoreType.DMA((NCH + 1,)),
            pltpu.SemaphoreType.DMA(()),
        ],
        compiler_params=pltpu.CompilerParams(vmem_limit_bytes=120 * 1024 * 1024),
    )(
        A_x.reshape(S, DM), A_mem0.reshape(M, DM), A_Wq, A_Wk, A_Wv,
        A_Wo.reshape(H * DH, DM), B_k.reshape(S, DM), B_v.reshape(S, DM),
        B_shift_k.T, B_ssm_k, B_ssm_D,
        jnp.asarray(fwd, BF16), jnp.asarray(inv, BF16),
    )
    return out.reshape(B, S, DM)
```

```python
import functools

import numpy as np
import jax
import jax.numpy as jnp
import jax.experimental.pallas as pl
import jax.experimental.pallas.tpu as pltpu

F32 = jnp.float32
BF16 = jnp.bfloat16
U32 = jnp.uint32

CB = 128
NQ = 4
KPAD = 16
PH = 8
NPRE = 10
PINS = (3, 12, 16, 20)
SPEC_AT = 4
UNROLL = 2
HG = 8
DIST, DIST_PRE, DIST_HALF = (1, 2), (2, 3), (1, 3)


def _dft_constants():
    qb = CB // NQ
    n = np.arange(CB, dtype=np.float64)
    fwd = np.zeros((NQ, 2 * qb, CB))
    for q in range(NQ):
        f = q * qb + np.concatenate([np.arange(0, qb, 2), np.arange(1, qb, 2)])
        ang = (np.pi * (2.0 * f + 1.0) / (2 * CB))[:, None] * n[None, :]
        fwd[q, :qb] = np.cos(ang)
        fwd[q, qb:] = -np.sin(ang)
    inv = fwd.reshape(2 * CB, CB).T / CB
    return fwd.astype(np.float32), inv.reshape(NQ, CB // NQ, 2 * CB).astype(np.float32)


def _ln(x, eps=1e-5):
    d = x.shape[-1]
    m = jnp.sum(x, axis=-1, keepdims=True) * (1.0 / d)
    xc = x - m
    v = jnp.sum(xc * xc, axis=-1, keepdims=True) * (1.0 / d)
    return xc * jax.lax.rsqrt(v + eps)


def _dot(a, b):
    return jnp.dot(a, b, preferred_element_type=F32)


def _dot_nt(a, b):
    return jax.lax.dot_general(a, b, (((1,), (1,)), ((), ())), preferred_element_type=F32)


def _pack(x):
    return pltpu.bitcast(x.astype(BF16), U32)


def _unpack(x):
    return pltpu.bitcast(x, BF16)


def _in_order(actions):
    def body(i, c):
        for j, act in enumerate(actions):
            pl.when(i == j)(act)
        return c
    jax.lax.fori_loop(0, len(actions), body, 0)


def _kernel(x_hbm, mem0_hbm, wq_hbm, wk_hbm, wv_hbm, wo_hbm, k_hbm, v_hbm,
            sh_hbm, sk_hbm, sd_hbm, fwd_hbm, inv_hbm, o_hbm,
            sp_sc, kr_sc, wf_sc, x2_sc, y_sc, u_sc, op_sc, pre_sc, pre0_sc, wa_sc, wb_sc, wo_sc, o_sc,
            x_sc, v_sc, sk_sc, st_sc, wo_st, out_sc, fwd_ref, inv_ref,
            k_sc, hp_sc, h_sc, mem0_ref, sh_ref, sd_ref,
            never_sm, sem_in, sem_w, sem_out,
            *, S, DM, H, DH, M, SEG):
    NSEG = S // SEG
    M2 = 2 * M
    R = M2 + 2 * SEG
    RH = M2 + SEG
    NB = S // CB
    QB = CB // NQ
    HB = QB // 2
    NT = DM // 128
    assert QB == SEG and NSEG % PH == 0 and NPRE % UNROLL == 0 and PH % UNROLL == 0
    NPH = NSEG // PH
    NCH = 3 * H // HG
    DH2 = DM // 2

    small = [pltpu.make_async_copy(s, d, sem_in.at[min(i, 1)]) for i, (s, d) in enumerate([
        (mem0_hbm, mem0_ref), (sh_hbm, sh_ref), (sd_hbm, sd_ref), (fwd_hbm, fwd_ref), (inv_hbm, inv_ref)])]

    xb = (0, NPRE * SEG, (NPRE + 1) * SEG, S)
    kb = (0, (2 * NQ + 2) * SEG, (2 * NQ + NPRE) * SEG, S)
    sb = (0, 2 * CB, ((NPRE - 1) // NQ + 2) * CB, S)

    def in_copies(part):
        def rng(b):
            return pl.ds(b[part], b[part + 1] - b[part])
        sem = sem_in.at[part + 1]
        return [
            pltpu.make_async_copy(x_hbm.at[rng(xb)], x_sc.at[rng(xb)], sem if part else sem_in.at[0]),
            pltpu.make_async_copy(k_hbm.at[rng(kb)],
                                  k_sc.at[pl.ds(KPAD + kb[part], kb[part + 1] - kb[part])], sem),
            pltpu.make_async_copy(v_hbm.at[rng(kb)], v_sc.at[rng(kb)], sem),
            pltpu.make_async_copy(sk_hbm.at[:, rng(sb)], sk_sc.at[:, rng(sb)], sem),
        ]

    def w_copies(src, g, ci):
        return [pltpu.make_async_copy(src.at[pl.ds(hf * DH2, DH2), pl.ds(pl.multiple_of(g * HG, HG), HG), :],
                                      st_sc.at[ci, :, pl.ds(hf * HG, HG), :], sem_w.at[ci])
                for hf in range(2)]

    wo_copy = pltpu.make_async_copy(wo_hbm, wo_st, sem_w.at[NCH])

    def out_copy(i):
        rows = pl.ds(pl.multiple_of(i * PH * SEG, PH * SEG), PH * SEG)
        return pltpu.make_async_copy(out_sc.at[rows], o_hbm.at[rows], sem_out)

    def out_tail(j):
        b = ((NPH - 1) * PH * SEG, (NSEG - 3) * SEG, S)
        rows = pl.ds(b[j], b[j + 1] - b[j])
        return pltpu.make_async_copy(out_sc.at[rows], o_hbm.at[rows], sem_out)

    def start_all(cps):
        def act():
            for cp in cps:
                cp.start()
        return act

    in0 = in_copies(0)
    start_all(small[:1] + in0[:1])()

    def start_group(g, c):
        _in_order([start_all(w_copies(src, g, 3 * g + mi))
                   for mi, src in enumerate((wq_hbm, wk_hbm, wv_hbm))])
        return c
    jax.lax.fori_loop(0, H // HG, start_group, 0)
    _in_order([start_all(small[1:] + in0[1:]), start_all([wo_copy]),
               start_all(in_copies(1)), start_all(in_copies(2))])

    never_sm[0] = 0
    k_sc[0:KPAD, :] = jnp.zeros((KPAD, DM), BF16)
    sp_sc[NB + 1] = jnp.zeros(sp_sc.shape[1:], F32)
    op_sc[...] = jnp.zeros(op_sc.shape, F32)
    x2_sc[...] = jnp.zeros(x2_sc.shape, F32)
    y_sc[...] = jnp.zeros(y_sc.shape, F32)
    h_sc[...] = jnp.zeros(h_sc.shape, BF16)
    for cp in small[:1] + in0[:1]:
        cp.wait()

    mem0 = mem0_ref[...].astype(F32)
    hp_sc[0:M, :] = _pack(jnp.concatenate([mem0, mem0], axis=0))
    for sg in range(NPRE):
        xn = _ln(x_sc[sg * SEG:(sg + 1) * SEG, :].astype(F32))
        if sg == 1:
            h_sc[M2:RH, :] = xn.astype(BF16)
        else:
            w0 = M + max(sg - 1, 0) * (SEG // 2)
            hp_sc[w0:w0 + SEG // 2, :] = _pack(xn)

    KS = sh_ref.shape[0]

    def clip(i, hi):
        return min(max(i, 0), hi) if isinstance(i, int) else jnp.clip(i, 0, hi)

    def scaled(i, m):
        return i * m if isinstance(i, int) else pl.multiple_of(i * m, m)

    def seg(i):
        return pl.ds(scaled(clip(i, NSEG - 1), SEG), SEG)

    def conv_u(s):
        r0 = scaled(clip(s, NSEG - 1), SEG)
        sh = sh_ref[...].astype(F32)
        kk = k_sc[pl.ds(r0, KPAD + SEG), :].astype(F32)
        ks = kk[KPAD:] * sh[0:1]
        for j in range(1, KS):
            ks = ks + pltpu.roll(kk, j, 0)[KPAD:] * sh[j:j + 1]
        u = (ks * v_sc[pl.ds(r0, SEG), :].astype(F32)).astype(BF16)
        u_sc[pl.ds(r0, SEG), :] = u
        return u

    def conv_fwd(c, q):
        t0 = scaled(clip(c, NB - 1), CB)
        f = fwd_ref[q]
        uf = _dot(f, u_sc[pl.ds(t0, CB), :])
        kf = _dot_nt(f, sk_sc[:, pl.ds(t0, CB)])
        return uf, kf

    def put_spec(cs, q, which, val):
        for rb in range(QB // 8):
            for n in range(NT):
                ln = slice(n * 128, (n + 1) * 128)
                sp_sc[cs, q, rb, n, which] = val[rb * 8:rb * 8 + 8, ln]
                sp_sc[cs, q, rb, n, which + 1] = val[QB + rb * 8:QB + rb * 8 + 8, ln]

    def conv_spec(c, q):
        uf, kf = conv_fwd(c, q)
        cs = clip(c, NB)
        put_spec(cs, q, 0, uf)
        pk = kr_sc[q]
        kr_sc[q] = kf
        kp = jnp.concatenate([
            kf[0:HB] - pk[QB:QB + HB],
            kf[HB:QB] + pk[QB + HB:],
            kf[QB:QB + HB] + pk[0:HB],
            kf[QB + HB:] - pk[HB:QB]], axis=0)
        put_spec(cs, q, 2, kp)

    MAC_PIECES = [(rb, n) for rb in range(QB // 16) for n in range(NT)]

    def conv_mac(c, q, piece, nterms):
        rb2, n = piece
        cs = clip(c, NB)
        acc = []
        for rb in (2 * rb2, 2 * rb2 + 1):
            ar = None
            ai = None
            for j in range(nterms):
                if isinstance(cs, int):
                    uj, kj = j, cs - j
                else:
                    uj = jnp.minimum(j, cs)
                    kj = jnp.where(cs - j >= 0, cs - j, NB + 1)
                ur = sp_sc[uj, q, rb, n, 0]
                um = sp_sc[uj, q, rb, n, 1]
                kr = sp_sc[kj, q, rb, n, 2]
                km = sp_sc[kj, q, rb, n, 3]
                tr = ur * kr - um * km
                ti = ur * km + um * kr
                ar = tr if ar is None else ar + tr
                ai = ti if ai is None else ai + ti
            acc.append((ar, ai))
        ln = slice(n * 128, (n + 1) * 128)
        wf_sc[c & 1, q, rb2 * 16:rb2 * 16 + 16, ln] = jnp.concatenate(
            [acc[0][0], acc[1][0]], axis=0).astype(BF16)
        wf_sc[c & 1, q, QB + rb2 * 16:QB + rb2 * 16 + 16, ln] = jnp.concatenate(
            [acc[0][1], acc[1][1]], axis=0).astype(BF16)

    def conv_inv(s):
        w = wf_sc[(s // NQ) & 1].reshape(2 * CB, DM)
        yc = _dot(inv_ref[s % NQ], w)
        sd = sd_ref[...].astype(F32).reshape(1, DM)
        y_sc[s & 3] = yc + u_sc[seg(s), :].astype(F32) * sd

    scale = DH ** -0.5
    cexp = scale * float(np.log2(np.e))

    def make_mask(n, x_layers):
        qi = jax.lax.broadcasted_iota(jnp.int32, (n, n), 0)
        ki = jax.lax.broadcasted_iota(jnp.int32, (n, n), 1)

        def layer(i):
            xl = jnp.where(i < M2 + SEG, x_layers[0], x_layers[-1])
            return jnp.where(i < M, 0, jnp.where(i < M2, 1, xl))
        same = layer(qi) == layer(ki)
        ok = same & ((qi < M2) | (ki < M2) | (qi >= ki))
        fill = jnp.where(same, -1e9 / scale, -jnp.inf).astype(F32)
        return ok, fill

    def probs(qkv, mask):
        ok, fill = mask
        s = _dot_nt(qkv[:, 0:DH], qkv[:, DH:2 * DH])
        s = jnp.where(ok, s, fill)
        m = jnp.max(s, axis=-1, keepdims=True)
        p = jnp.exp2((s - m) * cexp)
        l = jnp.sum(p, axis=-1, keepdims=True)
        r = pl.reciprocal(l, approx=True)
        r = r * (2.0 - l * r)
        return (p * r).astype(BF16)

    def w_piece(ci, j):
        return (wa_sc, wb_sc)[ci % 2][ci // 2, j]

    def w_head(g):
        return _unpack(jnp.concatenate(
            [w_piece(3 * (g // HG) + mi, g % HG) for mi in range(3)], axis=1))

    def pre_rows(ref, grp, j):
        return _unpack(jnp.concatenate([ref[3 * grp + mi, j] for mi in range(3)], axis=1))

    def out_proj(n, g0, g1, j):
        return _dot(_unpack(o_sc[0:n // 2, g0 * DH:g1 * DH]),
                    _unpack(wo_sc[g0 * DH // 2:g1 * DH // 2, j * 128:(j + 1) * 128]))

    def attend(proj, n, mask, dist, hook=None):
        D1, D2 = dist
        HA = H - D1 - D2 - 1
        qkvs = {}
        ps = {}
        outs = {}
        for it in range(H + D1 + D2):
            if it < H:
                qkvs[it] = proj(it)
            g = it - D1
            if 0 <= g < H:
                ps[g] = probs(qkvs[g], mask)
            g = it - D1 - D2
            if 0 <= g < H:
                o = _dot(ps.pop(g), qkvs.pop(g)[:, 2 * DH:3 * DH])
                o_sc[0:n // 2, g * DH:(g + 1) * DH] = _pack(o)
            if hook is not None:
                hook(it)
            j = it - (H - 1)
            if 0 <= j < D1 + D2:
                outs[j] = out_proj(n, 0, HA, j)
        for j in range(D1 + D2, NT):
            outs[j] = out_proj(n, 0, H, j)
        for j in range(D1 + D2):
            outs[j] = out_proj(n, HA, H, j) + outs[j]
        return jnp.concatenate([outs[j] for j in range(NT)], axis=1)

    def side1(t):
        x1 = x_sc[seg(t - 1), :].astype(F32) + op_sc[0:SEG, :]
        x2 = x1 + _ln(x1) * y_sc[(t - 1) & 3]
        x2_sc[(t - 1) & 3] = x2
        return _ln(x2).astype(BF16)

    def side2(t):
        x3 = x2_sc[(t - 3) & 3] + op_sc[SEG:, :]
        x4 = x3 + _ln(x3) * y_sc[(t - 3) & 3]
        x4 = x4.astype(out_sc.dtype)
        out_sc[seg(t - 3), :] = x4
        return x4

    def warm_block0(q):
        uf, kf = conv_fwd(0, q)
        put_spec(0, q, 0, uf)
        put_spec(0, q, 2, kf)
        kr_sc[q] = kf
        ur, um, kr, km = uf[:QB], uf[QB:], kf[:QB], kf[QB:]
        wf_sc[0, q, :QB] = (ur * kr - um * km).astype(BF16)
        wf_sc[0, q, QB:] = (ur * km + um * kr).astype(BF16)

    def warm_spec(t):
        conv_spec(1, t)
        for piece in MAC_PIECES:
            conv_mac(1, t, piece, 2)

    warm = {
        0: [functools.partial(conv_u, s) for s in range(2 * NQ + 2)],
        1: [functools.partial(warm_block0, q) for q in range(NQ)],
        3: [functools.partial(warm_spec, t) for t in range(2)],
        5: [functools.partial(conv_inv, t) for t in range(2)],
    }

    mask1 = make_mask(RH, (0,))

    def wait_chunk(ci):
        with jax.named_scope("wait_w"):
            for cp in w_copies(wq_hbm, 0, ci):
                cp.wait()

    def relayout(ci, dst, slot, b):
        d0 = b * 16 if isinstance(b, int) else pl.multiple_of(b * 16, 16)
        r0 = b * 8 if isinstance(b, int) else pl.multiple_of(b * 8, 8)
        xw = pltpu.bitcast(st_sc[ci, pl.ds(d0, 16)], U32).reshape(8, 2, HG, DH)
        a = xw[:, 0]
        bb = xw[:, 1]
        lo = jnp.swapaxes((a & U32(0xFFFF)) | (bb << 16), 0, 1)
        hi = jnp.swapaxes((a >> 16) | (bb & U32(0xFFFF0000)), 0, 1)
        for j in range(HG):
            rows = pl.ds(r0 + (2 * j // HG) * (DH2 // 2), 8)
            dst[slot, 2 * j % HG, rows, :] = lo[j]
            dst[slot, 2 * j % HG + 1, rows, :] = hi[j]

    NBLK = DH2 // 16

    def fused(cr, dst, rslot, cp, src, pslot):
        S2 = SEG // 2
        cuts = [0] + [RH // 2 + n * S2 for n in range(0, NPRE - 1, 2)]
        npc = len(cuts) - 1

        def body(i, c):
            done = 0
            for j in range(HG):
                w = _unpack(src[pslot, j])
                for pi in range(npc):
                    upto = min(NBLK, -(-(j * npc + pi) * NBLK // (HG * npc - 1)))
                    for bb in range(done, upto):
                        relayout(cr, dst, rslot, bb)
                    done = upto
                    lo, hi = cuts[pi], cuts[pi + 1]
                    r = _pack(_dot(_unpack(hp_sc[lo:hi, :]), w))
                    if pi == 0:
                        pre0_sc[cp, j] = r[0:RH // 2]
                    for sg in range(NPRE - 2):
                        a = RH // 2 + sg * S2
                        if lo <= a < hi:
                            pre_sc[sg, cp, j] = r[a - lo:a - lo + S2]
            return c
        with jax.named_scope("fused"):
            jax.lax.fori_loop(0, never_sm[0] + 1, body, 0)

    wait_chunk(0)

    def relayout0(b, c):
        relayout(0, wa_sc, 0, b)
        return c
    with jax.named_scope("relayout"):
        jax.lax.fori_loop(0, NBLK, relayout0, 0, unroll=2)

    KL = NCH // 2 - 1

    def chunk_pair(k, carry):
        wait_chunk(2 * k + 1)
        kc = jnp.minimum(k + never_sm[0], KL)
        fused(2 * kc + 1, wb_sc, kc, 2 * k, wa_sc, k)

        @pl.when(k < KL)
        def _():
            wait_chunk(2 * k + 2)
        kn = jnp.minimum(k + 1, KL)
        fused(2 * kn, wa_sc, kn, 2 * k + 1, wb_sc, k)
        return carry
    jax.lax.fori_loop(0, KL + 1, chunk_pair, 0)

    with jax.named_scope("wait_wo"):
        for cp in small[1:] + in0[1:] + [wo_copy]:
            cp.wait()
    ps = {}
    os_ = []
    out = None
    GW, E1, E2 = 4, 2, 1
    for it in range(H // GW + E1 + E2):
        for j in range(it * GW, (it + 1) * GW):
            if j < H:
                ps[j] = probs(pre_rows(pre0_sc, j // HG, j % HG), mask1)
        for j in range((it - E1) * GW, (it - E1 + 1) * GW):
            if 0 <= j < H:
                os_.append(_dot(ps.pop(j), _unpack(pre0_sc[3 * (j // HG) + 2, j % HG])).astype(BF16))
        g0 = (it - E1 - E2) * GW
        if g0 >= 0:
            wo = wo_st[g0 * DH:(g0 + GW) * DH, :]
            wo_sc[g0 * DH // 2:(g0 + GW) * DH // 2, :] = _pack(wo)
            part = _dot(jnp.concatenate(os_[g0:g0 + GW], axis=1), wo)
            out = part if out is None else part + out
        for act in warm.get(it, ()):
            act()
    h_sc[0:M2, :] = jnp.concatenate([out[0:M], mem0], axis=0).astype(BF16)
    op_sc[0:SEG, :] = out[M2:]

    mask12 = make_mask(R, (0, 1))

    def pinned(never, h, pins):
        hs = {0: h}
        r = _pack(h[-SEG:])
        for g, d in pins:
            r = jnp.where(never, _pack(d), r)
            hs[g] = jnp.concatenate([h[:-SEG], _unpack(r)], axis=0)
        return lambda g: hs[max(k for k in hs if k <= g)]

    def step(t, pre, spec_first=False):
        c = t // NQ + 1
        q = t % NQ
        if spec_first:
            conv_spec(c, q)
        x4 = side2(t)
        xn2 = side1(t)
        xn1 = _ln(x_sc[seg(t + 1), :].astype(F32)).astype(BF16)
        un = conv_u(t + 2 * NQ)
        pins = list(zip(PINS, (un, xn1, x4, xn2)))
        never = never_sm[0] > 0
        if pre:
            h = pinned(never, jnp.concatenate([h_sc[0:M2, :], h_sc[RH:, :]], axis=0), pins)

            def proj(g):
                r = _dot(h(g), w_head(g)).astype(BF16)
                x1 = pre_rows(pre_sc.at[t - 2], g // HG, g % HG)
                return jnp.concatenate([r[0:M2], x1, r[M2:]], axis=0)
            nterms = (NPRE - 1) // NQ + 2
        else:
            h = pinned(never, h_sc[...], pins)

            def proj(g):
                return _dot(h(g), w_head(g)).astype(BF16)
            nterms = NB
        h_sc[M2:RH, :] = xn1
        h_sc[RH:, :] = xn2

        def hook(it):
            if it == SPEC_AT and not spec_first:
                conv_spec(c, q)
            if it == SPEC_AT + 1:
                for piece in MAC_PIECES:
                    conv_mac(c, q, piece, nterms)
        out = attend(proj, R, mask12, DIST_PRE if pre else DIST, hook)
        conv_inv(t)
        h_sc[0:M2, :] = out[0:M2].astype(BF16)
        op_sc[...] = out[M2:]

    def step_pre(t, carry):
        step(t, True)
        return carry

    def step_full(i, carry):
        for j in range(UNROLL):
            step(i * UNROLL + j, False, j > 0)
        return carry

    def phase(p, carry):
        @pl.when(p >= 2)
        def _():
            out_copy(p - 2).start()

        with jax.named_scope("steps"):
            jax.lax.fori_loop(jnp.maximum(p * PH, NPRE) // UNROLL, (p * PH + PH) // UNROLL, step_full, 0)
        return carry

    mask2 = make_mask(RH, (1,))

    def step_half(t, carry):
        first = t < NSEG
        lo = pl.multiple_of(jnp.where(first, 0, SEG), SEG)
        mask = (jnp.where(first, mask1[0].astype(jnp.int32), mask2[0].astype(jnp.int32)) > 0,
                jnp.where(first, mask1[1], mask2[1]))
        h = jnp.concatenate([h_sc[0:M2, :], h_sc[pl.ds(pl.multiple_of(M2 + lo, 16), SEG), :]], axis=0)
        side2(t)
        xn2 = side1(t)
        out = attend(lambda g: _dot(h, w_head(g)).astype(BF16), RH, mask, DIST_HALF)
        m2 = jnp.where(first, mem0, out[M:M2])
        h_sc[0:M2, :] = jnp.concatenate([out[0:M], m2], axis=0).astype(BF16)
        h_sc[RH:, :] = xn2
        op_sc[pl.ds(lo, SEG), :] = out[M2:]
        return carry

    def stage(i, carry):
        with jax.named_scope("steps_half"):
            jax.lax.fori_loop(jnp.where(i == 0, 1, NSEG), jnp.where(i == 0, 2, NSEG + 2), step_half, 0)

        @pl.when(i == 0)
        def _():
            for cp in in_copies(1):
                cp.wait()
            with jax.named_scope("steps_pre"):
                jax.lax.fori_loop(2, NPRE, step_pre, 0)
            for cp in in_copies(2):
                cp.wait()
            jax.lax.fori_loop(NPRE // PH, NPH, phase, 0)
            out_copy(NPH - 2).start()
            out_tail(0).start()
        return carry

    jax.lax.fori_loop(0, 2, stage, 0)
    side2(NSEG + 2)
    out_tail(1).start()
    pltpu.make_async_copy(out_sc, o_hbm, sem_out).wait()


def pallas_interleave_layers__memory_aug_recurrent_mem_tr__ssm_conv_h3__prompt_kernel(
    A_x, A_mem0, A_Wq, A_Wk, A_Wv, A_Wo, A_seg_len,
    B_q, B_k, B_v, B_shift_k, B_ssm_k, B_ssm_D,
):
    del B_q
    seg = int(A_seg_len) if isinstance(A_seg_len, (int, np.integer)) else CB // NQ
    return _run(A_x, A_mem0, A_Wq, A_Wk, A_Wv, A_Wo, B_k, B_v, B_shift_k, B_ssm_k, B_ssm_D, SEG=seg)


@functools.partial(jax.jit, static_argnames=("SEG",))
def _run(A_x, A_mem0, A_Wq, A_Wk, A_Wv, A_Wo, B_k, B_v, B_shift_k, B_ssm_k, B_ssm_D, *, SEG):
    B, S, DM = A_x.shape
    assert B == 1
    H, DH = A_Wq.shape[1], A_Wq.shape[2]
    M = A_mem0.shape[1]
    KS = B_shift_k.shape[1]
    R = 2 * (M + SEG)
    RP = 2 * M + (NPRE - 1) * SEG
    NB = S // CB
    QB = CB // NQ
    NCH = 3 * H // HG
    fwd, inv = _dft_constants()

    kern = functools.partial(_kernel, S=S, DM=DM, H=H, DH=DH, M=M, SEG=SEG)
    any_spec = pl.BlockSpec(memory_space=pl.ANY)
    out = pl.pallas_call(
        kern,
        out_shape=jax.ShapeDtypeStruct((S, DM), A_x.dtype),
        in_specs=[any_spec] * 13,
        out_specs=any_spec,
        scratch_shapes=[
            pltpu.VMEM((NB + 2, NQ, QB // 8, DM // 128, 4, 8, 128), F32),
            pltpu.VMEM((NQ, 2 * QB, DM), F32),
            pltpu.VMEM((2, NQ, 2 * QB, DM), BF16),
            pltpu.VMEM((4, SEG, DM), F32),
            pltpu.VMEM((4, SEG, DM), F32),
            pltpu.VMEM((S, DM), BF16),
            pltpu.VMEM((2 * SEG, DM), F32),
            pltpu.VMEM((NPRE - 2, NCH, HG, SEG // 2, DH), U32),
            pltpu.VMEM((NCH, HG, M + SEG // 2, DH), U32),
            pltpu.VMEM((NCH // 2, HG, DM // 2, DH), U32),
            pltpu.VMEM((NCH // 2, HG, DM // 2, DH), U32),
            pltpu.VMEM((H * DH // 2, DM), U32),
            pltpu.VMEM((R // 2, H * DH), U32),
            pltpu.VMEM((S, DM), BF16),
            pltpu.VMEM((S, DM), BF16),
            pltpu.VMEM((DM, S), BF16),
            pltpu.VMEM((NCH, DM // 2, 2 * HG, DH), BF16),
            pltpu.VMEM((H * DH, DM), BF16),
            pltpu.VMEM((S, DM), A_x.dtype),
            pltpu.VMEM(fwd.shape, BF16),
            pltpu.VMEM(inv.shape, BF16),
            pltpu.VMEM((S + KPAD, DM), BF16),
            pltpu.VMEM((RP // 2, DM), U32),
            pltpu.VMEM((R, DM), BF16),
            pltpu.VMEM((M, DM), BF16),
            pltpu.VMEM((KS, DM), BF16),
            pltpu.VMEM((DM,), BF16),
            pltpu.SMEM((1,), jnp.int32),
            pltpu.SemaphoreType.DMA((4,)),
            pltpu.SemaphoreType.DMA((NCH + 1,)),
            pltpu.SemaphoreType.DMA(()),
        ],
        compiler_params=pltpu.CompilerParams(vmem_limit_bytes=120 * 1024 * 1024),
    )(
        A_x.reshape(S, DM), A_mem0.reshape(M, DM), A_Wq, A_Wk, A_Wv,
        A_Wo.reshape(H * DH, DM), B_k.reshape(S, DM), B_v.reshape(S, DM),
        B_shift_k.T, B_ssm_k, B_ssm_D,
        jnp.asarray(fwd, BF16), jnp.asarray(inv, BF16),
    )
    return out.reshape(B, S, DM)
```

```python
import functools

import numpy as np
import jax
import jax.numpy as jnp
import jax.experimental.pallas as pl
import jax.experimental.pallas.tpu as pltpu

F32 = jnp.float32
BF16 = jnp.bfloat16
U32 = jnp.uint32

CB = 128
NQ = 4
KPAD = 16
PH = 8
NPRE = 10
PINS = (3, 12, 16, 20)
SPEC_AT = 4
UNROLL = 2
HG = 8
DIST, DIST_PRE, DIST_HALF = (1, 2), (2, 3), (1, 3)


def _dft_constants():
    qb = CB // NQ
    n = np.arange(CB, dtype=np.float64)
    fwd = np.zeros((NQ, 2 * qb, CB))
    for q in range(NQ):
        f = q * qb + np.concatenate([np.arange(0, qb, 2), np.arange(1, qb, 2)])
        ang = (np.pi * (2.0 * f + 1.0) / (2 * CB))[:, None] * n[None, :]
        fwd[q, :qb] = np.cos(ang)
        fwd[q, qb:] = -np.sin(ang)
    inv = fwd.reshape(2 * CB, CB).T / CB
    return fwd.astype(np.float32), inv.reshape(NQ, CB // NQ, 2 * CB).astype(np.float32)


def _ln(x, eps=1e-5):
    d = x.shape[-1]
    m = jnp.sum(x, axis=-1, keepdims=True) * (1.0 / d)
    xc = x - m
    v = jnp.sum(xc * xc, axis=-1, keepdims=True) * (1.0 / d)
    return xc * jax.lax.rsqrt(v + eps)


def _dot(a, b):
    return jnp.dot(a, b, preferred_element_type=F32)


def _dot_nt(a, b):
    return jax.lax.dot_general(a, b, (((1,), (1,)), ((), ())), preferred_element_type=F32)


def _pack(x):
    return pltpu.bitcast(x.astype(BF16), U32)


def _unpack(x):
    return pltpu.bitcast(x, BF16)


def _in_order(actions):
    def body(i, c):
        for j, act in enumerate(actions):
            pl.when(i == j)(act)
        return c
    jax.lax.fori_loop(0, len(actions), body, 0)


def _kernel(x_hbm, mem0_hbm, wq_hbm, wk_hbm, wv_hbm, wo_hbm, k_hbm, v_hbm,
            sh_hbm, sk_hbm, sd_hbm, fwd_hbm, inv_hbm, o_hbm,
            sp_sc, kr_sc, wf_sc, x2_sc, y_sc, u_sc, op_sc, pre_sc, pre0_sc, wa_sc, wb_sc, wo_sc, o_sc,
            x_sc, v_sc, sk_sc, st_sc, wo_st, out_sc, fwd_ref, inv_ref,
            k_sc, hp_sc, h_sc, mem0_ref, sh_ref, sd_ref,
            never_sm, sem_in, sem_w, sem_out,
            *, S, DM, H, DH, M, SEG):
    NSEG = S // SEG
    M2 = 2 * M
    R = M2 + 2 * SEG
    RH = M2 + SEG
    NB = S // CB
    QB = CB // NQ
    HB = QB // 2
    NT = DM // 128
    assert QB == SEG and NSEG % PH == 0 and NPRE % UNROLL == 0 and PH % UNROLL == 0
    NPH = NSEG // PH
    NCH = 3 * H // HG
    DH2 = DM // 2

    small = [pltpu.make_async_copy(s, d, sem_in.at[min(i, 1)]) for i, (s, d) in enumerate([
        (mem0_hbm, mem0_ref), (sh_hbm, sh_ref), (sd_hbm, sd_ref), (fwd_hbm, fwd_ref), (inv_hbm, inv_ref)])]

    xb = (0, NPRE * SEG, (NPRE + 1) * SEG, S)
    kb = (0, (2 * NQ + 2) * SEG, (2 * NQ + NPRE) * SEG, S)
    sb = (0, 2 * CB, ((NPRE - 1) // NQ + 2) * CB, S)

    def in_copies(part):
        def rng(b):
            return pl.ds(b[part], b[part + 1] - b[part])
        sem = sem_in.at[part + 1]
        return [
            pltpu.make_async_copy(x_hbm.at[rng(xb)], x_sc.at[rng(xb)], sem if part else sem_in.at[0]),
            pltpu.make_async_copy(k_hbm.at[rng(kb)],
                                  k_sc.at[pl.ds(KPAD + kb[part], kb[part + 1] - kb[part])], sem),
            pltpu.make_async_copy(v_hbm.at[rng(kb)], v_sc.at[rng(kb)], sem),
            pltpu.make_async_copy(sk_hbm.at[:, rng(sb)], sk_sc.at[:, rng(sb)], sem),
        ]

    def w_copies(src, g, ci):
        return [pltpu.make_async_copy(src.at[pl.ds(hf * DH2, DH2), pl.ds(pl.multiple_of(g * HG, HG), HG), :],
                                      st_sc.at[ci, :, pl.ds(hf * HG, HG), :], sem_w.at[ci])
                for hf in range(2)]

    wo_copy = pltpu.make_async_copy(wo_hbm, wo_st, sem_w.at[NCH])

    def out_copy(i):
        rows = pl.ds(pl.multiple_of(i * PH * SEG, PH * SEG), PH * SEG)
        return pltpu.make_async_copy(out_sc.at[rows], o_hbm.at[rows], sem_out)

    def out_tail(j):
        b = ((NPH - 1) * PH * SEG, (NSEG - 3) * SEG, S)
        rows = pl.ds(b[j], b[j + 1] - b[j])
        return pltpu.make_async_copy(out_sc.at[rows], o_hbm.at[rows], sem_out)

    def start_all(cps):
        def act():
            for cp in cps:
                cp.start()
        return act

    in0 = in_copies(0)
    start_all(small[:1] + in0[:1])()

    def start_group(g, c):
        _in_order([start_all(w_copies(src, g, 3 * g + mi))
                   for mi, src in enumerate((wq_hbm, wk_hbm, wv_hbm))])
        return c
    jax.lax.fori_loop(0, H // HG, start_group, 0)
    _in_order([start_all(small[1:] + in0[1:]), start_all([wo_copy]),
               start_all(in_copies(1)), start_all(in_copies(2))])

    never_sm[0] = 0
    k_sc[0:KPAD, :] = jnp.zeros((KPAD, DM), BF16)
    sp_sc[NB + 1] = jnp.zeros(sp_sc.shape[1:], F32)
    op_sc[...] = jnp.zeros(op_sc.shape, F32)
    x2_sc[...] = jnp.zeros(x2_sc.shape, F32)
    y_sc[...] = jnp.zeros(y_sc.shape, F32)
    h_sc[...] = jnp.zeros(h_sc.shape, BF16)
    for cp in small[:1] + in0[:1]:
        cp.wait()

    mem0 = mem0_ref[...].astype(F32)
    hp_sc[0:M, :] = _pack(jnp.concatenate([mem0, mem0], axis=0))
    for sg in range(NPRE):
        xn = _ln(x_sc[sg * SEG:(sg + 1) * SEG, :].astype(F32))
        if sg == 1:
            h_sc[M2:RH, :] = xn.astype(BF16)
        else:
            w0 = M + max(sg - 1, 0) * (SEG // 2)
            hp_sc[w0:w0 + SEG // 2, :] = _pack(xn)

    KS = sh_ref.shape[0]

    def clip(i, hi):
        return min(max(i, 0), hi) if isinstance(i, int) else jnp.clip(i, 0, hi)

    def scaled(i, m):
        return i * m if isinstance(i, int) else pl.multiple_of(i * m, m)

    def seg(i):
        return pl.ds(scaled(clip(i, NSEG - 1), SEG), SEG)

    def conv_u(s, ln=slice(None)):
        r0 = scaled(clip(s, NSEG - 1), SEG)
        sh = sh_ref[:, ln].astype(F32)
        kk = k_sc[pl.ds(r0, KPAD + SEG), ln].astype(F32)
        ks = kk[KPAD:] * sh[0:1]
        for j in range(1, KS):
            ks = ks + pltpu.roll(kk, j, 0)[KPAD:] * sh[j:j + 1]
        u = (ks * v_sc[pl.ds(r0, SEG), ln].astype(F32)).astype(BF16)
        u_sc[pl.ds(r0, SEG), ln] = u
        return u

    def conv_fwd(c, q):
        t0 = scaled(clip(c, NB - 1), CB)
        f = fwd_ref[q]
        uf = _dot(f, u_sc[pl.ds(t0, CB), :])
        kf = _dot_nt(f, sk_sc[:, pl.ds(t0, CB)])
        return uf, kf

    def put_spec(cs, q, which, val):
        for rb in range(QB // 8):
            for n in range(NT):
                ln = slice(n * 128, (n + 1) * 128)
                sp_sc[cs, q, rb, n, which] = val[rb * 8:rb * 8 + 8, ln]
                sp_sc[cs, q, rb, n, which + 1] = val[QB + rb * 8:QB + rb * 8 + 8, ln]

    def conv_spec(c, q):
        uf, kf = conv_fwd(c, q)
        cs = clip(c, NB)
        put_spec(cs, q, 0, uf)
        pk = kr_sc[q]
        kr_sc[q] = kf
        kp = jnp.concatenate([
            kf[0:HB] - pk[QB:QB + HB],
            kf[HB:QB] + pk[QB + HB:],
            kf[QB:QB + HB] + pk[0:HB],
            kf[QB + HB:] - pk[HB:QB]], axis=0)
        put_spec(cs, q, 2, kp)

    MAC_PIECES = [(rb, n) for rb in range(QB // 16) for n in range(NT)]

    def conv_mac(c, q, piece, nterms):
        rb2, n = piece
        cs = clip(c, NB)
        acc = []
        for rb in (2 * rb2, 2 * rb2 + 1):
            ar = None
            ai = None
            for j in range(nterms):
                if isinstance(cs, int):
                    uj, kj = j, cs - j
                else:
                    uj = jnp.minimum(j, cs)
                    kj = jnp.where(cs - j >= 0, cs - j, NB + 1)
                ur = sp_sc[uj, q, rb, n, 0]
                um = sp_sc[uj, q, rb, n, 1]
                kr = sp_sc[kj, q, rb, n, 2]
                km = sp_sc[kj, q, rb, n, 3]
                tr = ur * kr - um * km
                ti = ur * km + um * kr
                ar = tr if ar is None else ar + tr
                ai = ti if ai is None else ai + ti
            acc.append((ar, ai))
        ln = slice(n * 128, (n + 1) * 128)
        wf_sc[c & 1, q, rb2 * 16:rb2 * 16 + 16, ln] = jnp.concatenate(
            [acc[0][0], acc[1][0]], axis=0).astype(BF16)
        wf_sc[c & 1, q, QB + rb2 * 16:QB + rb2 * 16 + 16, ln] = jnp.concatenate(
            [acc[0][1], acc[1][1]], axis=0).astype(BF16)

    def conv_inv(s):
        w = wf_sc[(s // NQ) & 1].reshape(2 * CB, DM)
        yc = _dot(inv_ref[s % NQ], w)
        sd = sd_ref[...].astype(F32).reshape(1, DM)
        y_sc[s & 3] = yc + u_sc[seg(s), :].astype(F32) * sd

    scale = DH ** -0.5
    cexp = scale * float(np.log2(np.e))

    def make_mask(n, x_layers):
        qi = jax.lax.broadcasted_iota(jnp.int32, (n, n), 0)
        ki = jax.lax.broadcasted_iota(jnp.int32, (n, n), 1)

        def layer(i):
            xl = jnp.where(i < M2 + SEG, x_layers[0], x_layers[-1])
            return jnp.where(i < M, 0, jnp.where(i < M2, 1, xl))
        same = layer(qi) == layer(ki)
        ok = same & ((qi < M2) | (ki < M2) | (qi >= ki))
        fill = jnp.where(same, -1e9 / scale, -jnp.inf).astype(F32)
        return ok, fill

    def probs(qkv, mask):
        ok, fill = mask
        s = _dot_nt(qkv[:, 0:DH], qkv[:, DH:2 * DH])
        s = jnp.where(ok, s, fill)
        m = jnp.max(s, axis=-1, keepdims=True)
        p = jnp.exp2((s - m) * cexp)
        l = jnp.sum(p, axis=-1, keepdims=True)
        r = pl.reciprocal(l, approx=True)
        r = r * (2.0 - l * r)
        return (p * r).astype(BF16)

    def w_piece(ci, j):
        return (wa_sc, wb_sc)[ci % 2][ci // 2, j]

    def w_head(g):
        return _unpack(jnp.concatenate(
            [w_piece(3 * (g // HG) + mi, g % HG) for mi in range(3)], axis=1))

    def pre_rows(ref, grp, j):
        return _unpack(jnp.concatenate([ref[3 * grp + mi, j] for mi in range(3)], axis=1))

    def out_proj(n, g0, g1, j):
        return _dot(_unpack(o_sc[0:n // 2, g0 * DH:g1 * DH]),
                    _unpack(wo_sc[g0 * DH // 2:g1 * DH // 2, j * 128:(j + 1) * 128]))

    def attend(proj, n, mask, dist, hook=None):
        D1, D2 = dist
        HA = H - D1 - D2 - 1
        qkvs = {}
        ps = {}
        outs = {}
        for it in range(H + D1 + D2):
            if it < H:
                qkvs[it] = proj(it)
            g = it - D1
            if 0 <= g < H:
                ps[g] = probs(qkvs[g], mask)
            g = it - D1 - D2
            if 0 <= g < H:
                o = _dot(ps.pop(g), qkvs.pop(g)[:, 2 * DH:3 * DH])
                o_sc[0:n // 2, g * DH:(g + 1) * DH] = _pack(o)
            if hook is not None:
                hook(it)
            j = it - (H - 1)
            if 0 <= j < D1 + D2:
                outs[j] = out_proj(n, 0, HA, j)
        for j in range(D1 + D2, NT):
            outs[j] = out_proj(n, 0, H, j)
        for j in range(D1 + D2):
            outs[j] = out_proj(n, HA, H, j) + outs[j]
        return jnp.concatenate([outs[j] for j in range(NT)], axis=1)

    def side1(t):
        x1 = x_sc[seg(t - 1), :].astype(F32) + op_sc[0:SEG, :]
        x2 = x1 + _ln(x1) * y_sc[(t - 1) & 3]
        x2_sc[(t - 1) & 3] = x2
        return _ln(x2).astype(BF16)

    def side2(t):
        x3 = x2_sc[(t - 3) & 3] + op_sc[SEG:, :]
        x4 = x3 + _ln(x3) * y_sc[(t - 3) & 3]
        x4 = x4.astype(out_sc.dtype)
        out_sc[seg(t - 3), :] = x4
        return x4

    def warm_block0(q):
        uf, kf = conv_fwd(0, q)
        put_spec(0, q, 0, uf)
        put_spec(0, q, 2, kf)
        kr_sc[q] = kf
        ur, um, kr, km = uf[:QB], uf[QB:], kf[:QB], kf[QB:]
        wf_sc[0, q, :QB] = (ur * kr - um * km).astype(BF16)
        wf_sc[0, q, QB:] = (ur * km + um * kr).astype(BF16)

    def warm_spec(t):
        conv_spec(1, t)
        for piece in MAC_PIECES:
            conv_mac(1, t, piece, 2)

    warm = {
        1: [functools.partial(warm_block0, q) for q in range(NQ)],
        3: [functools.partial(warm_spec, t) for t in range(2)],
        5: [functools.partial(conv_inv, t) for t in range(2)],
    }

    mask1 = make_mask(RH, (0,))

    def wait_chunk(ci):
        with jax.named_scope("wait_w"):
            for cp in w_copies(wq_hbm, 0, ci):
                cp.wait()

    def relayout(ci, dst, slot, b):
        d0 = b * 16 if isinstance(b, int) else pl.multiple_of(b * 16, 16)
        r0 = b * 8 if isinstance(b, int) else pl.multiple_of(b * 8, 8)
        xw = pltpu.bitcast(st_sc[ci, pl.ds(d0, 16)], U32).reshape(8, 2, HG, DH)
        a = xw[:, 0]
        bb = xw[:, 1]
        lo = jnp.swapaxes((a & U32(0xFFFF)) | (bb << 16), 0, 1)
        hi = jnp.swapaxes((a >> 16) | (bb & U32(0xFFFF0000)), 0, 1)
        for j in range(HG):
            rows = pl.ds(r0 + (2 * j // HG) * (DH2 // 2), 8)
            dst[slot, 2 * j % HG, rows, :] = lo[j]
            dst[slot, 2 * j % HG + 1, rows, :] = hi[j]

    NBLK = DH2 // 16

    def fused(filler, cp, src, pslot):
        S2 = SEG // 2
        cuts = [0] + [RH // 2 + n * S2 for n in range(0, NPRE - 1, 2)]
        npc = len(cuts) - 1

        def body(i, c):
            done = 0
            for j in range(HG):
                w = _unpack(src[pslot, j])
                for pi in range(npc):
                    upto = min(NBLK, -(-(j * npc + pi) * NBLK // (HG * npc - 1)))
                    for bb in range(done, upto):
                        filler(bb)
                    done = upto
                    lo, hi = cuts[pi], cuts[pi + 1]
                    r = _pack(_dot(_unpack(hp_sc[lo:hi, :]), w))
                    if pi == 0:
                        pre0_sc[cp, j] = r[0:RH // 2]
                    for sg in range(NPRE - 2):
                        a = RH // 2 + sg * S2
                        if lo <= a < hi:
                            pre_sc[sg, cp, j] = r[a - lo:a - lo + S2]
            return c
        with jax.named_scope("fused"):
            jax.lax.fori_loop(0, never_sm[0] + 1, body, 0)

    wait_chunk(0)

    def relayout0(b, c):
        relayout(0, wa_sc, 0, b)
        return c
    with jax.named_scope("relayout"):
        jax.lax.fori_loop(0, NBLK, relayout0, 0, unroll=2)

    KL = NCH // 2 - 1

    def chunk_pair(k, carry):
        wait_chunk(2 * k + 1)
        kc = jnp.minimum(k + never_sm[0], KL)
        fused(functools.partial(relayout, 2 * kc + 1, wb_sc, kc), 2 * k, wa_sc, k)

        @pl.when(k < KL)
        def _():
            wait_chunk(2 * k + 2)
            kn = jnp.minimum(k + 1, KL)
            fused(functools.partial(relayout, 2 * kn, wa_sc, kn), 2 * k + 1, wb_sc, k)
        return carry
    jax.lax.fori_loop(0, KL + 1, chunk_pair, 0)

    for cp in small[1:] + in0[1:]:
        cp.wait()
    assert NBLK == 2 * (2 * NQ + 2)
    fused(lambda b: conv_u(b // 2 + never_sm[0], (slice(0, 256), slice(256, DM))[b % 2]),
          NCH - 1, wb_sc, KL)

    with jax.named_scope("wait_wo"):
        wo_copy.wait()
    ps = {}
    os_ = []
    out = None
    GW, E1, E2 = 4, 2, 1
    for it in range(H // GW + E1 + E2):
        for j in range(it * GW, (it + 1) * GW):
            if j < H:
                ps[j] = probs(pre_rows(pre0_sc, j // HG, j % HG), mask1)
        for j in range((it - E1) * GW, (it - E1 + 1) * GW):
            if 0 <= j < H:
                os_.append(_dot(ps.pop(j), _unpack(pre0_sc[3 * (j // HG) + 2, j % HG])).astype(BF16))
        g0 = (it - E1 - E2) * GW
        if g0 >= 0:
            wo = wo_st[g0 * DH:(g0 + GW) * DH, :]
            wo_sc[g0 * DH // 2:(g0 + GW) * DH // 2, :] = _pack(wo)
            part = _dot(jnp.concatenate(os_[g0:g0 + GW], axis=1), wo)
            out = part if out is None else part + out
        for act in warm.get(it, ()):
            act()
    h_sc[0:M2, :] = jnp.concatenate([out[0:M], mem0], axis=0).astype(BF16)
    op_sc[0:SEG, :] = out[M2:]

    mask12 = make_mask(R, (0, 1))

    def pinned(never, h, pins):
        hs = {0: h}
        r = _pack(h[-SEG:])
        for g, d in pins:
            r = jnp.where(never, _pack(d), r)
            hs[g] = jnp.concatenate([h[:-SEG], _unpack(r)], axis=0)
        return lambda g: hs[max(k for k in hs if k <= g)]

    def step(t, pre, spec_first=False):
        c = t // NQ + 1
        q = t % NQ
        if spec_first:
            conv_spec(c, q)
        x4 = side2(t)
        xn2 = side1(t)
        xn1 = _ln(x_sc[seg(t + 1), :].astype(F32)).astype(BF16)
        un = conv_u(t + 2 * NQ)
        pins = list(zip(PINS, (un, xn1, x4, xn2)))
        never = never_sm[0] > 0
        if pre:
            h = pinned(never, jnp.concatenate([h_sc[0:M2, :], h_sc[RH:, :]], axis=0), pins)

            def proj(g):
                r = _dot(h(g), w_head(g)).astype(BF16)
                x1 = pre_rows(pre_sc.at[t - 2], g // HG, g % HG)
                return jnp.concatenate([r[0:M2], x1, r[M2:]], axis=0)
            nterms = (NPRE - 1) // NQ + 2
        else:
            h = pinned(never, h_sc[...], pins)

            def proj(g):
                return _dot(h(g), w_head(g)).astype(BF16)
            nterms = NB
        h_sc[M2:RH, :] = xn1
        h_sc[RH:, :] = xn2

        def hook(it):
            if it == SPEC_AT and not spec_first:
                conv_spec(c, q)
            if it == SPEC_AT + 1:
                for piece in MAC_PIECES:
                    conv_mac(c, q, piece, nterms)
        out = attend(proj, R, mask12, DIST_PRE if pre else DIST, hook)
        conv_inv(t)
        h_sc[0:M2, :] = out[0:M2].astype(BF16)
        op_sc[...] = out[M2:]

    def step_pre(t, carry):
        step(t, True)
        return carry

    def step_full(i, carry):
        for j in range(UNROLL):
            step(i * UNROLL + j, False, j > 0)
        return carry

    def phase(p, carry):
        @pl.when(p >= 2)
        def _():
            out_copy(p - 2).start()

        with jax.named_scope("steps"):
            jax.lax.fori_loop(jnp.maximum(p * PH, NPRE) // UNROLL, (p * PH + PH) // UNROLL, step_full, 0)
        return carry

    mask2 = make_mask(RH, (1,))

    def step_half(t, carry):
        first = t < NSEG
        lo = pl.multiple_of(jnp.where(first, 0, SEG), SEG)
        mask = (jnp.where(first, mask1[0].astype(jnp.int32), mask2[0].astype(jnp.int32)) > 0,
                jnp.where(first, mask1[1], mask2[1]))
        h = jnp.concatenate([h_sc[0:M2, :], h_sc[pl.ds(pl.multiple_of(M2 + lo, 16), SEG), :]], axis=0)
        side2(t)
        xn2 = side1(t)
        out = attend(lambda g: _dot(h, w_head(g)).astype(BF16), RH, mask, DIST_HALF)
        m2 = jnp.where(first, mem0, out[M:M2])
        h_sc[0:M2, :] = jnp.concatenate([out[0:M], m2], axis=0).astype(BF16)
        h_sc[RH:, :] = xn2
        op_sc[pl.ds(lo, SEG), :] = out[M2:]
        return carry

    def stage(i, carry):
        with jax.named_scope("steps_half"):
            jax.lax.fori_loop(jnp.where(i == 0, 1, NSEG), jnp.where(i == 0, 2, NSEG + 2), step_half, 0)

        @pl.when(i == 0)
        def _():
            for cp in in_copies(1):
                cp.wait()
            with jax.named_scope("steps_pre"):
                jax.lax.fori_loop(2, NPRE, step_pre, 0)
            for cp in in_copies(2):
                cp.wait()
            jax.lax.fori_loop(NPRE // PH, NPH, phase, 0)
            out_copy(NPH - 2).start()
            out_tail(0).start()
        return carry

    jax.lax.fori_loop(0, 2, stage, 0)
    side2(NSEG + 2)
    out_tail(1).start()
    pltpu.make_async_copy(out_sc, o_hbm, sem_out).wait()


def pallas_interleave_layers__memory_aug_recurrent_mem_tr__ssm_conv_h3__prompt_kernel(
    A_x, A_mem0, A_Wq, A_Wk, A_Wv, A_Wo, A_seg_len,
    B_q, B_k, B_v, B_shift_k, B_ssm_k, B_ssm_D,
):
    del B_q
    seg = int(A_seg_len) if isinstance(A_seg_len, (int, np.integer)) else CB // NQ
    return _run(A_x, A_mem0, A_Wq, A_Wk, A_Wv, A_Wo, B_k, B_v, B_shift_k, B_ssm_k, B_ssm_D, SEG=seg)


@functools.partial(jax.jit, static_argnames=("SEG",))
def _run(A_x, A_mem0, A_Wq, A_Wk, A_Wv, A_Wo, B_k, B_v, B_shift_k, B_ssm_k, B_ssm_D, *, SEG):
    B, S, DM = A_x.shape
    assert B == 1
    H, DH = A_Wq.shape[1], A_Wq.shape[2]
    M = A_mem0.shape[1]
    KS = B_shift_k.shape[1]
    R = 2 * (M + SEG)
    RP = 2 * M + (NPRE - 1) * SEG
    NB = S // CB
    QB = CB // NQ
    NCH = 3 * H // HG
    fwd, inv = _dft_constants()

    kern = functools.partial(_kernel, S=S, DM=DM, H=H, DH=DH, M=M, SEG=SEG)
    any_spec = pl.BlockSpec(memory_space=pl.ANY)
    out = pl.pallas_call(
        kern,
        out_shape=jax.ShapeDtypeStruct((S, DM), A_x.dtype),
        in_specs=[any_spec] * 13,
        out_specs=any_spec,
        scratch_shapes=[
            pltpu.VMEM((NB + 2, NQ, QB // 8, DM // 128, 4, 8, 128), F32),
            pltpu.VMEM((NQ, 2 * QB, DM), F32),
            pltpu.VMEM((2, NQ, 2 * QB, DM), BF16),
            pltpu.VMEM((4, SEG, DM), F32),
            pltpu.VMEM((4, SEG, DM), F32),
            pltpu.VMEM((S, DM), BF16),
            pltpu.VMEM((2 * SEG, DM), F32),
            pltpu.VMEM((NPRE - 2, NCH, HG, SEG // 2, DH), U32),
            pltpu.VMEM((NCH, HG, M + SEG // 2, DH), U32),
            pltpu.VMEM((NCH // 2, HG, DM // 2, DH), U32),
            pltpu.VMEM((NCH // 2, HG, DM // 2, DH), U32),
            pltpu.VMEM((H * DH // 2, DM), U32),
            pltpu.VMEM((R // 2, H * DH), U32),
            pltpu.VMEM((S, DM), BF16),
            pltpu.VMEM((S, DM), BF16),
            pltpu.VMEM((DM, S), BF16),
            pltpu.VMEM((NCH, DM // 2, 2 * HG, DH), BF16),
            pltpu.VMEM((H * DH, DM), BF16),
            pltpu.VMEM((S, DM), A_x.dtype),
            pltpu.VMEM(fwd.shape, BF16),
            pltpu.VMEM(inv.shape, BF16),
            pltpu.VMEM((S + KPAD, DM), BF16),
            pltpu.VMEM((RP // 2, DM), U32),
            pltpu.VMEM((R, DM), BF16),
            pltpu.VMEM((M, DM), BF16),
            pltpu.VMEM((KS, DM), BF16),
            pltpu.VMEM((DM,), BF16),
            pltpu.SMEM((1,), jnp.int32),
            pltpu.SemaphoreType.DMA((4,)),
            pltpu.SemaphoreType.DMA((NCH + 1,)),
            pltpu.SemaphoreType.DMA(()),
        ],
        compiler_params=pltpu.CompilerParams(vmem_limit_bytes=120 * 1024 * 1024),
    )(
        A_x.reshape(S, DM), A_mem0.reshape(M, DM), A_Wq, A_Wk, A_Wv,
        A_Wo.reshape(H * DH, DM), B_k.reshape(S, DM), B_v.reshape(S, DM),
        B_shift_k.T, B_ssm_k, B_ssm_D,
        jnp.asarray(fwd, BF16), jnp.asarray(inv, BF16),
    )
    return out.reshape(B, S, DM)
```

```python
import functools

import numpy as np
import jax
import jax.numpy as jnp
import jax.experimental.pallas as pl
import jax.experimental.pallas.tpu as pltpu

F32 = jnp.float32
BF16 = jnp.bfloat16
U32 = jnp.uint32

CB = 128
NQ = 4
KPAD = 16
PH = 8
NPRE = 10
PINS = (3, 10, 14, 19, 24)
SPEC_AT = 4
UNROLL = 2
HG = 8
DIST, DIST_PRE, DIST_HALF = (1, 2), (2, 3), (1, 3)


def _dft_constants():
    qb = CB // NQ
    n = np.arange(CB, dtype=np.float64)
    fwd = np.zeros((NQ, 2 * qb, CB))
    for q in range(NQ):
        f = q * qb + np.concatenate([np.arange(0, qb, 2), np.arange(1, qb, 2)])
        ang = (np.pi * (2.0 * f + 1.0) / (2 * CB))[:, None] * n[None, :]
        fwd[q, :qb] = np.cos(ang)
        fwd[q, qb:] = -np.sin(ang)
    inv = fwd.reshape(2 * CB, CB).T / CB
    return fwd.astype(np.float32), inv.reshape(NQ, CB // NQ, 2 * CB).astype(np.float32)


def _ln(x, eps=1e-5):
    d = x.shape[-1]
    m = jnp.sum(x, axis=-1, keepdims=True) * (1.0 / d)
    xc = x - m
    v = jnp.sum(xc * xc, axis=-1, keepdims=True) * (1.0 / d)
    return xc * jax.lax.rsqrt(v + eps)


def _dot(a, b):
    return jnp.dot(a, b, preferred_element_type=F32)


def _dot_nt(a, b):
    return jax.lax.dot_general(a, b, (((1,), (1,)), ((), ())), preferred_element_type=F32)


def _pack(x):
    return pltpu.bitcast(x.astype(BF16), U32)


def _unpack(x):
    return pltpu.bitcast(x, BF16)


def _in_order(actions):
    def body(i, c):
        for j, act in enumerate(actions):
            pl.when(i == j)(act)
        return c
    jax.lax.fori_loop(0, len(actions), body, 0)


def _kernel(x_hbm, mem0_hbm, wq_hbm, wk_hbm, wv_hbm, wo_hbm, k_hbm, v_hbm,
            sh_hbm, sk_hbm, sd_hbm, fwd_hbm, inv_hbm, o_hbm,
            sp_sc, kr_sc, wf_sc, x2_sc, y_sc, u_sc, op_sc, pre_sc, pre0_sc, wa_sc, wb_sc, wo_sc, o_sc,
            x_sc, v_sc, sk_sc, st_sc, out_sc, fwd_ref, inv_ref,
            k_sc, hp_sc, h_sc, mem0_ref, sh_ref, sd_ref,
            never_sm, sem_in, sem_w, sem_out,
            *, S, DM, H, DH, M, SEG):
    NSEG = S // SEG
    M2 = 2 * M
    R = M2 + 2 * SEG
    RH = M2 + SEG
    NB = S // CB
    QB = CB // NQ
    HB = QB // 2
    NT = DM // 128
    assert QB == SEG and NSEG % PH == 0 and NPRE % UNROLL == 0 and PH % UNROLL == 0
    NPH = NSEG // PH
    NCH = 3 * H // HG
    DH2 = DM // 2

    small = [pltpu.make_async_copy(s, d, sem_in.at[min(i, 1)]) for i, (s, d) in enumerate([
        (mem0_hbm, mem0_ref), (sh_hbm, sh_ref), (sd_hbm, sd_ref), (fwd_hbm, fwd_ref), (inv_hbm, inv_ref)])]

    xb = (0, NPRE * SEG, (NPRE + 1) * SEG, S)
    kb = (0, (2 * NQ + 2) * SEG, (2 * NQ + NPRE) * SEG, S)
    sb = (0, 2 * CB, ((NPRE - 1) // NQ + 2) * CB, S)

    def in_copies(part):
        def rng(b):
            return pl.ds(b[part], b[part + 1] - b[part])
        sem = sem_in.at[part + 1]
        return [
            pltpu.make_async_copy(x_hbm.at[rng(xb)], x_sc.at[rng(xb)], sem if part else sem_in.at[0]),
            pltpu.make_async_copy(k_hbm.at[rng(kb)],
                                  k_sc.at[pl.ds(KPAD + kb[part], kb[part + 1] - kb[part])], sem),
            pltpu.make_async_copy(v_hbm.at[rng(kb)], v_sc.at[rng(kb)], sem),
            pltpu.make_async_copy(sk_hbm.at[:, rng(sb)], sk_sc.at[:, rng(sb)], sem),
        ]

    def w_copies(src, g, ci):
        return [pltpu.make_async_copy(src.at[pl.ds(hf * DH2, DH2), pl.ds(pl.multiple_of(g * HG, HG), HG), :],
                                      st_sc.at[ci, :, pl.ds(hf * HG, HG), :], sem_w.at[ci])
                for hf in range(2)]

    wo_copy = pltpu.make_async_copy(wo_hbm, wo_sc, sem_w.at[NCH])

    def out_copy(i):
        rows = pl.ds(pl.multiple_of(i * PH * SEG, PH * SEG), PH * SEG)
        return pltpu.make_async_copy(out_sc.at[rows], o_hbm.at[rows], sem_out)

    def out_tail(j):
        b = ((NPH - 1) * PH * SEG, (NSEG - 3) * SEG, S)
        rows = pl.ds(b[j], b[j + 1] - b[j])
        return pltpu.make_async_copy(out_sc.at[rows], o_hbm.at[rows], sem_out)

    def start_all(cps):
        def act():
            for cp in cps:
                cp.start()
        return act

    in0 = in_copies(0)
    start_all(small[:1] + in0[:1])()

    def start_group(g, c):
        _in_order([start_all(w_copies(src, g, 3 * g + mi))
                   for mi, src in enumerate((wq_hbm, wk_hbm, wv_hbm))])
        return c
    jax.lax.fori_loop(0, H // HG, start_group, 0)
    _in_order([start_all(small[1:] + in0[1:]), start_all([wo_copy]),
               start_all(in_copies(1)), start_all(in_copies(2))])

    never_sm[0] = 0
    k_sc[0:KPAD, :] = jnp.zeros((KPAD, DM), BF16)
    sp_sc[NB + 1] = jnp.zeros(sp_sc.shape[1:], F32)
    op_sc[...] = jnp.zeros(op_sc.shape, F32)
    x2_sc[...] = jnp.zeros(x2_sc.shape, F32)
    y_sc[...] = jnp.zeros(y_sc.shape, F32)
    h_sc[...] = jnp.zeros(h_sc.shape, BF16)
    for cp in small[:1] + in0[:1]:
        cp.wait()

    mem0 = mem0_ref[...].astype(F32)
    hp_sc[0:M, :] = _pack(jnp.concatenate([mem0, mem0], axis=0))
    for sg in range(NPRE):
        xn = _ln(x_sc[sg * SEG:(sg + 1) * SEG, :].astype(F32))
        if sg == 1:
            h_sc[M2:RH, :] = xn.astype(BF16)
        else:
            w0 = M + max(sg - 1, 0) * (SEG // 2)
            hp_sc[w0:w0 + SEG // 2, :] = _pack(xn)

    KS = sh_ref.shape[0]

    def clip(i, hi):
        return min(max(i, 0), hi) if isinstance(i, int) else jnp.clip(i, 0, hi)

    def scaled(i, m):
        return i * m if isinstance(i, int) else pl.multiple_of(i * m, m)

    def seg(i):
        return pl.ds(scaled(clip(i, NSEG - 1), SEG), SEG)

    def conv_u(s, ln=slice(None)):
        r0 = scaled(clip(s, NSEG - 1), SEG)
        sh = sh_ref[:, ln].astype(F32)
        kk = k_sc[pl.ds(r0, KPAD + SEG), ln].astype(F32)
        ks = kk[KPAD:] * sh[0:1]
        for j in range(1, KS):
            ks = ks + pltpu.roll(kk, j, 0)[KPAD:] * sh[j:j + 1]
        u = (ks * v_sc[pl.ds(r0, SEG), ln].astype(F32)).astype(BF16)
        u_sc[pl.ds(r0, SEG), ln] = u
        return u

    def conv_fwd(c, q):
        t0 = scaled(clip(c, NB - 1), CB)
        f = fwd_ref[q]
        uf = _dot(f, u_sc[pl.ds(t0, CB), :])
        kf = _dot_nt(f, sk_sc[:, pl.ds(t0, CB)])
        return uf, kf

    def put_spec(cs, q, which, val):
        for rb in range(QB // 8):
            for n in range(NT):
                ln = slice(n * 128, (n + 1) * 128)
                sp_sc[cs, q, rb, n, which] = val[rb * 8:rb * 8 + 8, ln]
                sp_sc[cs, q, rb, n, which + 1] = val[QB + rb * 8:QB + rb * 8 + 8, ln]

    def conv_spec(c, q):
        uf, kf = conv_fwd(c, q)
        cs = clip(c, NB)
        put_spec(cs, q, 0, uf)
        pk = kr_sc[q]
        kr_sc[q] = kf
        kp = jnp.concatenate([
            kf[0:HB] - pk[QB:QB + HB],
            kf[HB:QB] + pk[QB + HB:],
            kf[QB:QB + HB] + pk[0:HB],
            kf[QB + HB:] - pk[HB:QB]], axis=0)
        put_spec(cs, q, 2, kp)

    MAC_PIECES = [(rb, n) for rb in range(QB // 16) for n in range(NT)]

    def conv_mac(c, q, piece, nterms):
        rb2, n = piece
        cs = clip(c, NB)
        acc = []
        for rb in (2 * rb2, 2 * rb2 + 1):
            ar = None
            ai = None
            for j in range(nterms):
                if isinstance(cs, int):
                    uj, kj = j, cs - j
                else:
                    uj = jnp.minimum(j, cs)
                    kj = jnp.where(cs - j >= 0, cs - j, NB + 1)
                ur = sp_sc[uj, q, rb, n, 0]
                um = sp_sc[uj, q, rb, n, 1]
                kr = sp_sc[kj, q, rb, n, 2]
                km = sp_sc[kj, q, rb, n, 3]
                tr = ur * kr - um * km
                ti = ur * km + um * kr
                ar = tr if ar is None else ar + tr
                ai = ti if ai is None else ai + ti
            acc.append((ar, ai))
        ln = slice(n * 128, (n + 1) * 128)
        wf_sc[c & 1, q, rb2 * 16:rb2 * 16 + 16, ln] = jnp.concatenate(
            [acc[0][0], acc[1][0]], axis=0).astype(BF16)
        wf_sc[c & 1, q, QB + rb2 * 16:QB + rb2 * 16 + 16, ln] = jnp.concatenate(
            [acc[0][1], acc[1][1]], axis=0).astype(BF16)

    def conv_inv(s):
        w = wf_sc[(s // NQ) & 1].reshape(2 * CB, DM)
        yc = _dot(inv_ref[s % NQ], w)
        sd = sd_ref[...].astype(F32).reshape(1, DM)
        y_sc[s & 3] = yc + u_sc[seg(s), :].astype(F32) * sd

    scale = DH ** -0.5
    cexp = scale * float(np.log2(np.e))

    def make_mask(n, x_layers):
        qi = jax.lax.broadcasted_iota(jnp.int32, (n, n), 0)
        ki = jax.lax.broadcasted_iota(jnp.int32, (n, n), 1)

        def layer(i):
            xl = jnp.where(i < M2 + SEG, x_layers[0], x_layers[-1])
            return jnp.where(i < M, 0, jnp.where(i < M2, 1, xl))
        same = layer(qi) == layer(ki)
        ok = same & ((qi < M2) | (ki < M2) | (qi >= ki))
        fill = jnp.where(same, -1e9 / scale, -jnp.inf).astype(F32)
        return ok, fill

    def probs(qkv, mask):
        ok, fill = mask
        s = _dot_nt(qkv[:, 0:DH], qkv[:, DH:2 * DH])
        s = jnp.where(ok, s, fill)
        m = jnp.max(s, axis=-1, keepdims=True)
        p = jnp.exp2((s - m) * cexp)
        l = jnp.sum(p, axis=-1, keepdims=True)
        r = pl.reciprocal(l, approx=True)
        r = r * (2.0 - l * r)
        return (p * r).astype(BF16)

    def w_piece(ci, j):
        return (wa_sc, wb_sc)[ci % 2][ci // 2, j]

    def w_head(g):
        return _unpack(jnp.concatenate(
            [w_piece(3 * (g // HG) + mi, g % HG) for mi in range(3)], axis=1))

    def pre_rows(ref, grp, j):
        return _unpack(jnp.concatenate([ref[3 * grp + mi, j] for mi in range(3)], axis=1))

    def out_proj(n, g0, g1, j):
        return _dot(_unpack(o_sc[0:n // 2, g0 * DH:g1 * DH]),
                    wo_sc[g0 * DH:g1 * DH, j * 128:(j + 1) * 128])

    def attend(proj, n, mask, dist, hook=None):
        D1, D2 = dist
        HA = H - D1 - D2 - 1
        qkvs = {}
        ps = {}
        outs = {}
        for it in range(H + D1 + D2):
            if it < H:
                qkvs[it] = proj(it)
            g = it - D1
            if 0 <= g < H:
                ps[g] = probs(qkvs[g], mask)
            g = it - D1 - D2
            if 0 <= g < H:
                o = _dot(ps.pop(g), qkvs.pop(g)[:, 2 * DH:3 * DH])
                o_sc[0:n // 2, g * DH:(g + 1) * DH] = _pack(o)
            if hook is not None:
                hook(it)
            j = it - (H - 1)
            if 0 <= j < D1 + D2:
                outs[j] = out_proj(n, 0, HA, j)
        for j in range(D1 + D2, NT):
            outs[j] = out_proj(n, 0, H, j)
        for j in range(D1 + D2):
            outs[j] = out_proj(n, HA, H, j) + outs[j]
        return jnp.concatenate([outs[j] for j in range(NT)], axis=1)

    def side1(t):
        x1 = x_sc[seg(t - 1), :].astype(F32) + op_sc[0:SEG, :]
        x2 = x1 + _ln(x1) * y_sc[(t - 1) & 3]
        x2_sc[(t - 1) & 3] = x2
        return x2, _ln(x2).astype(BF16)

    def side2(t):
        x3 = x2_sc[(t - 3) & 3] + op_sc[SEG:, :]
        x4 = x3 + _ln(x3) * y_sc[(t - 3) & 3]
        x4 = x4.astype(out_sc.dtype)
        out_sc[seg(t - 3), :] = x4
        return x4

    def warm_block0(q):
        uf, kf = conv_fwd(0, q)
        put_spec(0, q, 0, uf)
        put_spec(0, q, 2, kf)
        kr_sc[q] = kf
        ur, um, kr, km = uf[:QB], uf[QB:], kf[:QB], kf[QB:]
        wf_sc[0, q, :QB] = (ur * kr - um * km).astype(BF16)
        wf_sc[0, q, QB:] = (ur * km + um * kr).astype(BF16)

    def warm_spec(t):
        conv_spec(1, t)
        for piece in MAC_PIECES:
            conv_mac(1, t, piece, 2)

    warm = {
        1: [functools.partial(warm_block0, q) for q in range(NQ)],
        3: [functools.partial(warm_spec, t) for t in range(2)],
        5: [functools.partial(conv_inv, t) for t in range(2)],
    }

    mask1 = make_mask(RH, (0,))

    def wait_chunk(ci):
        with jax.named_scope("wait_w"):
            for cp in w_copies(wq_hbm, 0, ci):
                cp.wait()

    def relayout(ci, dst, slot, b):
        d0 = b * 16 if isinstance(b, int) else pl.multiple_of(b * 16, 16)
        r0 = b * 8 if isinstance(b, int) else pl.multiple_of(b * 8, 8)
        xw = pltpu.bitcast(st_sc[ci, pl.ds(d0, 16)], U32).reshape(8, 2, HG, DH)
        a = xw[:, 0]
        bb = xw[:, 1]
        lo = jnp.swapaxes((a & U32(0xFFFF)) | (bb << 16), 0, 1)
        hi = jnp.swapaxes((a >> 16) | (bb & U32(0xFFFF0000)), 0, 1)
        for j in range(HG):
            rows = pl.ds(r0 + (2 * j // HG) * (DH2 // 2), 8)
            dst[slot, 2 * j % HG, rows, :] = lo[j]
            dst[slot, 2 * j % HG + 1, rows, :] = hi[j]

    NBLK = DH2 // 16

    def fused(filler, cp, src, pslot):
        S2 = SEG // 2
        cuts = [0] + [RH // 2 + n * S2 for n in range(0, NPRE - 1, 2)]
        npc = len(cuts) - 1

        def body(i, c):
            done = 0
            for j in range(HG):
                w = _unpack(src[pslot, j])
                for pi in range(npc):
                    upto = min(NBLK, -(-(j * npc + pi) * NBLK // (HG * npc - 1)))
                    for bb in range(done, upto):
                        filler(bb)
                    done = upto
                    lo, hi = cuts[pi], cuts[pi + 1]
                    r = _pack(_dot(_unpack(hp_sc[lo:hi, :]), w))
                    if pi == 0:
                        pre0_sc[cp, j] = r[0:RH // 2]
                    for sg in range(NPRE - 2):
                        a = RH // 2 + sg * S2
                        if lo <= a < hi:
                            pre_sc[sg, cp, j] = r[a - lo:a - lo + S2]
            return c
        with jax.named_scope("fused"):
            jax.lax.fori_loop(0, never_sm[0] + 1, body, 0)

    wait_chunk(0)

    def relayout0(b, c):
        relayout(0, wa_sc, 0, b)
        return c
    with jax.named_scope("relayout"):
        jax.lax.fori_loop(0, NBLK, relayout0, 0, unroll=2)

    KL = NCH // 2 - 1

    def chunk_pair(k, carry):
        wait_chunk(2 * k + 1)
        kc = jnp.minimum(k + never_sm[0], KL)
        fused(functools.partial(relayout, 2 * kc + 1, wb_sc, kc), 2 * k, wa_sc, k)

        @pl.when(k < KL)
        def _():
            wait_chunk(2 * k + 2)
            kn = jnp.minimum(k + 1, KL)
            fused(functools.partial(relayout, 2 * kn, wa_sc, kn), 2 * k + 1, wb_sc, k)
        return carry
    jax.lax.fori_loop(0, KL + 1, chunk_pair, 0)

    for cp in small[1:] + in0[1:]:
        cp.wait()
    assert NBLK == 2 * (2 * NQ + 2)
    fused(lambda b: conv_u(b // 2 + never_sm[0], (slice(0, 256), slice(256, DM))[b % 2]),
          NCH - 1, wb_sc, KL)

    with jax.named_scope("wait_wo"):
        wo_copy.wait()
    ps = {}
    os_ = []
    out = None
    GW, E1, E2 = 4, 2, 1
    for it in range(H // GW + E1 + E2):
        for j in range(it * GW, (it + 1) * GW):
            if j < H:
                ps[j] = probs(pre_rows(pre0_sc, j // HG, j % HG), mask1)
        for j in range((it - E1) * GW, (it - E1 + 1) * GW):
            if 0 <= j < H:
                os_.append(_dot(ps.pop(j), _unpack(pre0_sc[3 * (j // HG) + 2, j % HG])).astype(BF16))
        g0 = (it - E1 - E2) * GW
        if g0 >= 0:
            part = _dot(jnp.concatenate(os_[g0:g0 + GW], axis=1), wo_sc[g0 * DH:(g0 + GW) * DH, :])
            out = part if out is None else part + out
        for act in warm.get(it, ()):
            act()
    h_sc[0:M2, :] = jnp.concatenate([out[0:M], mem0], axis=0).astype(BF16)
    op_sc[0:SEG, :] = out[M2:]

    mask12 = make_mask(R, (0, 1))

    def pinned(never, h, pins):
        hs = {0: h}
        r = _pack(h[-SEG:])
        for g, d in pins:
            r = jnp.where(never, _pack(d), r)
            hs[g] = jnp.concatenate([h[:-SEG], _unpack(r)], axis=0)
        return lambda g: hs[max(k for k in hs if k <= g)]

    def step(t, pre, spec_first=False):
        c = t // NQ + 1
        q = t % NQ
        if spec_first:
            conv_spec(c, q)
        x4 = side2(t)
        x2, xn2 = side1(t)
        xn1 = _ln(x_sc[seg(t + 1), :].astype(F32)).astype(BF16)
        un = conv_u(t + 2 * NQ)
        pins = list(zip(PINS, (un, xn1, x4, x2, xn2)))
        never = never_sm[0] > 0
        if pre:
            h = pinned(never, jnp.concatenate([h_sc[0:M2, :], h_sc[RH:, :]], axis=0), pins)

            def proj(g):
                r = _dot(h(g), w_head(g)).astype(BF16)
                x1 = pre_rows(pre_sc.at[t - 2], g // HG, g % HG)
                return jnp.concatenate([r[0:M2], x1, r[M2:]], axis=0)
            nterms = (NPRE - 1) // NQ + 2
        else:
            h = pinned(never, h_sc[...], pins)

            def proj(g):
                return _dot(h(g), w_head(g)).astype(BF16)
            nterms = NB
        h_sc[M2:RH, :] = xn1
        h_sc[RH:, :] = xn2

        def hook(it):
            if it == SPEC_AT and not spec_first:
                conv_spec(c, q)
            if it == SPEC_AT + 1:
                for piece in MAC_PIECES:
                    conv_mac(c, q, piece, nterms)
        out = attend(proj, R, mask12, DIST_PRE if pre else DIST, hook)
        conv_inv(t)
        h_sc[0:M2, :] = out[0:M2].astype(BF16)
        op_sc[...] = out[M2:]

    def step_pre(t, carry):
        step(t, True)
        return carry

    def step_full(i, carry):
        for j in range(UNROLL):
            step(i * UNROLL + j, False, j > 0)
        return carry

    def phase(p, carry):
        @pl.when(p >= 2)
        def _():
            out_copy(p - 2).start()

        with jax.named_scope("steps"):
            jax.lax.fori_loop(jnp.maximum(p * PH, NPRE) // UNROLL, (p * PH + PH) // UNROLL, step_full, 0)
        return carry

    mask2 = make_mask(RH, (1,))

    def step_half(t, carry):
        first = t < NSEG
        lo = pl.multiple_of(jnp.where(first, 0, SEG), SEG)
        mask = (jnp.where(first, mask1[0].astype(jnp.int32), mask2[0].astype(jnp.int32)) > 0,
                jnp.where(first, mask1[1], mask2[1]))
        h = jnp.concatenate([h_sc[0:M2, :], h_sc[pl.ds(pl.multiple_of(M2 + lo, 16), SEG), :]], axis=0)
        side2(t)
        _, xn2 = side1(t)
        out = attend(lambda g: _dot(h, w_head(g)).astype(BF16), RH, mask, DIST_HALF)
        m2 = jnp.where(first, mem0, out[M:M2])
        h_sc[0:M2, :] = jnp.concatenate([out[0:M], m2], axis=0).astype(BF16)
        h_sc[RH:, :] = xn2
        op_sc[pl.ds(lo, SEG), :] = out[M2:]
        return carry

    def stage(i, carry):
        with jax.named_scope("steps_half"):
            jax.lax.fori_loop(jnp.where(i == 0, 1, NSEG), jnp.where(i == 0, 2, NSEG + 2), step_half, 0)

        @pl.when(i == 0)
        def _():
            for cp in in_copies(1):
                cp.wait()
            with jax.named_scope("steps_pre"):
                jax.lax.fori_loop(2, NPRE, step_pre, 0)
            for cp in in_copies(2):
                cp.wait()
            jax.lax.fori_loop(NPRE // PH, NPH, phase, 0)
            out_copy(NPH - 2).start()
            out_tail(0).start()
        return carry

    jax.lax.fori_loop(0, 2, stage, 0)
    side2(NSEG + 2)
    out_tail(1).start()
    pltpu.make_async_copy(out_sc, o_hbm, sem_out).wait()


def pallas_interleave_layers__memory_aug_recurrent_mem_tr__ssm_conv_h3__prompt_kernel(
    A_x, A_mem0, A_Wq, A_Wk, A_Wv, A_Wo, A_seg_len,
    B_q, B_k, B_v, B_shift_k, B_ssm_k, B_ssm_D,
):
    del B_q
    seg = int(A_seg_len) if isinstance(A_seg_len, (int, np.integer)) else CB // NQ
    return _run(A_x, A_mem0, A_Wq, A_Wk, A_Wv, A_Wo, B_k, B_v, B_shift_k, B_ssm_k, B_ssm_D, SEG=seg)


@functools.partial(jax.jit, static_argnames=("SEG",))
def _run(A_x, A_mem0, A_Wq, A_Wk, A_Wv, A_Wo, B_k, B_v, B_shift_k, B_ssm_k, B_ssm_D, *, SEG):
    B, S, DM = A_x.shape
    assert B == 1
    H, DH = A_Wq.shape[1], A_Wq.shape[2]
    M = A_mem0.shape[1]
    KS = B_shift_k.shape[1]
    R = 2 * (M + SEG)
    RP = 2 * M + (NPRE - 1) * SEG
    NB = S // CB
    QB = CB // NQ
    NCH = 3 * H // HG
    fwd, inv = _dft_constants()

    kern = functools.partial(_kernel, S=S, DM=DM, H=H, DH=DH, M=M, SEG=SEG)
    any_spec = pl.BlockSpec(memory_space=pl.ANY)
    out = pl.pallas_call(
        kern,
        out_shape=jax.ShapeDtypeStruct((S, DM), A_x.dtype),
        in_specs=[any_spec] * 13,
        out_specs=any_spec,
        scratch_shapes=[
            pltpu.VMEM((NB + 2, NQ, QB // 8, DM // 128, 4, 8, 128), F32),
            pltpu.VMEM((NQ, 2 * QB, DM), F32),
            pltpu.VMEM((2, NQ, 2 * QB, DM), BF16),
            pltpu.VMEM((4, SEG, DM), F32),
            pltpu.VMEM((4, SEG, DM), F32),
            pltpu.VMEM((S, DM), BF16),
            pltpu.VMEM((2 * SEG, DM), F32),
            pltpu.VMEM((NPRE - 2, NCH, HG, SEG // 2, DH), U32),
            pltpu.VMEM((NCH, HG, M + SEG // 2, DH), U32),
            pltpu.VMEM((NCH // 2, HG, DM // 2, DH), U32),
            pltpu.VMEM((NCH // 2, HG, DM // 2, DH), U32),
            pltpu.VMEM((H * DH, DM), BF16),
            pltpu.VMEM((R // 2, H * DH), U32),
            pltpu.VMEM((S, DM), BF16),
            pltpu.VMEM((S, DM), BF16),
            pltpu.VMEM((DM, S), BF16),
            pltpu.VMEM((NCH, DM // 2, 2 * HG, DH), BF16),
            pltpu.VMEM((S, DM), A_x.dtype),
            pltpu.VMEM(fwd.shape, BF16),
            pltpu.VMEM(inv.shape, BF16),
            pltpu.VMEM((S + KPAD, DM), BF16),
            pltpu.VMEM((RP // 2, DM), U32),
            pltpu.VMEM((R, DM), BF16),
            pltpu.VMEM((M, DM), BF16),
            pltpu.VMEM((KS, DM), BF16),
            pltpu.VMEM((DM,), BF16),
            pltpu.SMEM((1,), jnp.int32),
            pltpu.SemaphoreType.DMA((4,)),
            pltpu.SemaphoreType.DMA((NCH + 1,)),
            pltpu.SemaphoreType.DMA(()),
        ],
        compiler_params=pltpu.CompilerParams(vmem_limit_bytes=120 * 1024 * 1024),
    )(
        A_x.reshape(S, DM), A_mem0.reshape(M, DM), A_Wq, A_Wk, A_Wv,
        A_Wo.reshape(H * DH, DM), B_k.reshape(S, DM), B_v.reshape(S, DM),
        B_shift_k.T, B_ssm_k, B_ssm_D,
        jnp.asarray(fwd, BF16), jnp.asarray(inv, BF16),
    )
    return out.reshape(B, S, DM)
```

```python
import functools

import numpy as np
import jax
import jax.numpy as jnp
import jax.experimental.pallas as pl
import jax.experimental.pallas.tpu as pltpu

F32 = jnp.float32
BF16 = jnp.bfloat16
U32 = jnp.uint32

CB = 128
NQ = 4
KPAD = 16
HG = 8
NPA = 16
NPB = 12
RB = 9
UNROLL = 3
PHI = 3
PIN_U2, X4S = 1, 0
SPEC_AT, PIN_U, PIN_X4 = 7, 1, 16
DIST, DIST_HALF, DIST_LAST = (1, 2), (1, 3), (2, 3)


def _dft_constants():
    qb = CB // NQ
    n = np.arange(CB, dtype=np.float64)
    fwd = np.zeros((NQ, 2 * qb, CB))
    for q in range(NQ):
        f = q * qb + np.concatenate([np.arange(0, qb, 2), np.arange(1, qb, 2)])
        ang = (np.pi * (2.0 * f + 1.0) / (2 * CB))[:, None] * n[None, :]
        fwd[q, :qb] = np.cos(ang)
        fwd[q, qb:] = -np.sin(ang)
    inv = fwd.reshape(2 * CB, CB).T / CB
    return fwd.astype(np.float32), inv.reshape(NQ, CB // NQ, 2 * CB).astype(np.float32)


def _ln(x, eps=1e-5):
    d = x.shape[-1]
    m = jnp.sum(x, axis=-1, keepdims=True) * (1.0 / d)
    xc = x - m
    v = jnp.sum(xc * xc, axis=-1, keepdims=True) * (1.0 / d)
    return xc * jax.lax.rsqrt(v + eps)


def _dot(a, b):
    return jnp.dot(a, b, preferred_element_type=F32)


def _dot_nt(a, b):
    return jax.lax.dot_general(a, b, (((1,), (1,)), ((), ())), preferred_element_type=F32)


def _pack(x):
    return pltpu.bitcast(x.astype(BF16), U32)


def _unpack(x):
    return pltpu.bitcast(x, BF16)


def _in_order(actions):
    def body(i, c):
        for j, act in enumerate(actions):
            pl.when(i == j)(act)
        return c
    jax.lax.fori_loop(0, len(actions), body, 0)


def _kernel(x_hbm, mem0_hbm, wq_hbm, wk_hbm, wv_hbm, wo_hbm, k_hbm, v_hbm,
            sh_hbm, sk_hbm, sd_hbm, fwd_hbm, inv_hbm, o_hbm,
            sp_sc, kr_sc, wf_sc, x2_sc, y_sc, u_sc, op_sc, pre_sc, fill_sc, xn_sc, w_sc, wp_sc, wo_sc, o_sc,
            x_sc, v_sc, sk_sc, st_sc, out_sc, fwd_ref, inv_ref,
            k_sc, hp_sc, h_sc, mem0_ref, sh_ref, sd_ref,
            never_sm, sem_x, sem_in, sem_w, sem_out,
            *, S, DM, H, DH, M, SEG):
    NSEG = S // SEG
    M2 = 2 * M
    S2 = SEG // 2
    R = M2 + 2 * SEG
    RH = M2 + SEG
    NB = S // CB
    QB = CB // NQ
    HB = QB // 2
    NT = DM // 128
    PH = PHI * UNROLL
    NRB = (NSEG - 1) // RB
    NPH = (NSEG - 1) // PH
    NG = H // HG
    NCH = 3 * NG
    NPASS = NPA // HG
    DH2 = DM // 2
    KS = sh_ref.shape[0]
    assert QB == SEG and NRB * RB == NSEG - 1 and NPH * PH == NSEG - 1 and NPASS * NRB >= NCH + 1

    mem0_copy = pltpu.make_async_copy(mem0_hbm, mem0_ref, sem_x.at[0])
    small = [pltpu.make_async_copy(s, d, sem_in.at[0]) for s, d in [
        (sh_hbm, sh_ref), (sd_hbm, sd_ref), (fwd_hbm, fwd_ref), (inv_hbm, inv_ref)]]

    def x_copy(b):
        if isinstance(b, int) and b == 0:
            rows = pl.ds(0, (RB + 1) * SEG)
        else:
            rows = pl.ds(pl.multiple_of((b * RB + 1) * SEG, SEG), RB * SEG)
        return pltpu.make_async_copy(x_hbm.at[rows], x_sc.at[rows], sem_x.at[b])

    kb = (0, (2 * NQ + 1) * SEG, (2 * NQ + PH + 1) * SEG, S)
    sb = (0, 2 * CB, ((PH + 1) // NQ + 2) * CB, S)

    def in_copies(part):
        def rng(b):
            return pl.ds(b[part], b[part + 1] - b[part])
        sem = sem_in.at[part]
        return [
            pltpu.make_async_copy(k_hbm.at[rng(kb)],
                                  k_sc.at[pl.ds(KPAD + kb[part], kb[part + 1] - kb[part])], sem),
            pltpu.make_async_copy(v_hbm.at[rng(kb)], v_sc.at[rng(kb)], sem),
            pltpu.make_async_copy(sk_hbm.at[:, rng(sb)], sk_sc.at[:, rng(sb)], sem),
        ]

    def w_copies(ci, dst=None):
        src = (wq_hbm, wk_hbm, wv_hbm)[ci // NG]
        dst = ci if dst is None else dst
        return [pltpu.make_async_copy(src.at[pl.ds(hf * DH2, DH2), pl.ds((ci % NG) * HG, HG), :],
                                      st_sc.at[dst, :, pl.ds(hf * HG, HG), :], sem_w.at[dst])
                for hf in range(2)]

    wo_copy = pltpu.make_async_copy(wo_hbm, wo_sc, sem_w.at[NCH])

    def out_copy(lo, n):
        rows = pl.ds(lo * SEG if isinstance(lo, int) else pl.multiple_of(lo * SEG, SEG), n * SEG)
        return pltpu.make_async_copy(out_sc.at[rows], o_hbm.at[rows], sem_out)

    def start_all(cps):
        def act():
            for cp in cps:
                cp.start()
        return act

    order = [[mem0_copy, x_copy(0)], w_copies(0), [x_copy(1)], [x_copy(2)]]
    for ci in range(1, NCH):
        order.append(w_copies(ci) + ([x_copy(ci + 2)] if ci + 2 < NRB else []))
    order += [small + in_copies(0), [wo_copy], in_copies(1), in_copies(2)]
    for i in range(0, len(order), 5):
        _in_order([start_all(cps) for cps in order[i:i + 5]])

    never_sm[0] = 0
    k_sc[0:KPAD, :] = jnp.zeros((KPAD, DM), BF16)
    sp_sc[NB + 1] = jnp.zeros(sp_sc.shape[1:], F32)
    op_sc[...] = jnp.zeros(op_sc.shape, F32)
    x2_sc[...] = jnp.zeros(x2_sc.shape, F32)
    y_sc[...] = jnp.zeros(y_sc.shape, F32)
    mem0_copy.wait()
    x_copy(0).wait()
    for sg in range(RB + 1):
        xn_sc[sg, :, 0:DM] = _pack(_ln(x_sc[sg * SEG:(sg + 1) * SEG, :].astype(F32)))

    def clip(i, hi):
        return min(max(i, 0), hi) if isinstance(i, int) else jnp.clip(i, 0, hi)

    def scaled(i, m):
        return i * m if isinstance(i, int) else pl.multiple_of(i * m, m)

    def seg(i):
        return pl.ds(scaled(clip(i, NSEG - 1), SEG), SEG)

    def conv_u(s, ln=slice(None)):
        r0 = scaled(clip(s, NSEG - 1), SEG)
        sh = sh_ref[:, ln].astype(F32)
        kk = k_sc[pl.ds(r0, KPAD + SEG), ln].astype(F32)
        ks = kk[KPAD:] * sh[0:1]
        for j in range(1, KS):
            ks = ks + pltpu.roll(kk, j, 0)[KPAD:] * sh[j:j + 1]
        u = (ks * v_sc[pl.ds(r0, SEG), ln].astype(F32)).astype(BF16)
        u_sc[pl.ds(r0, SEG), ln] = u
        return u

    def conv_fwd(c, q):
        t0 = scaled(clip(c, NB - 1), CB)
        f = fwd_ref[q]
        uf = _dot(f, u_sc[pl.ds(t0, CB), :])
        kf = _dot_nt(f, sk_sc[:, pl.ds(t0, CB)])
        return uf, kf

    def put_spec(cs, q, which, val):
        for rb in range(QB // 8):
            for n in range(NT):
                ln = slice(n * 128, (n + 1) * 128)
                sp_sc[cs, q, rb, n, which] = val[rb * 8:rb * 8 + 8, ln]
                sp_sc[cs, q, rb, n, which + 1] = val[QB + rb * 8:QB + rb * 8 + 8, ln]

    def conv_spec(c, q):
        uf, kf = conv_fwd(c, q)
        cs = clip(c, NB)
        put_spec(cs, q, 0, uf)
        pk = kr_sc[q]
        kr_sc[q] = kf
        kp = jnp.concatenate([
            kf[0:HB] - pk[QB:QB + HB],
            kf[HB:QB] + pk[QB + HB:],
            kf[QB:QB + HB] + pk[0:HB],
            kf[QB + HB:] - pk[HB:QB]], axis=0)
        put_spec(cs, q, 2, kp)

    MAC_PIECES = [(rb, n) for rb in range(QB // 16) for n in range(NT)]

    def conv_mac(c, q, piece, nterms):
        rb2, n = piece
        cs = clip(c, NB)
        acc = []
        for rb in (2 * rb2, 2 * rb2 + 1):
            ar = None
            ai = None
            for j in range(nterms):
                if isinstance(cs, int):
                    uj, kj = j, cs - j
                else:
                    uj = jnp.minimum(j, cs)
                    kj = jnp.where(cs - j >= 0, cs - j, NB + 1)
                ur = sp_sc[uj, q, rb, n, 0]
                um = sp_sc[uj, q, rb, n, 1]
                kr = sp_sc[kj, q, rb, n, 2]
                km = sp_sc[kj, q, rb, n, 3]
                tr = ur * kr - um * km
                ti = ur * km + um * kr
                ar = tr if ar is None else ar + tr
                ai = ti if ai is None else ai + ti
            acc.append((ar, ai))
        ln = slice(n * 128, (n + 1) * 128)
        w = jnp.concatenate([acc[0][0], acc[1][0], acc[0][1], acc[1][1]], axis=0).astype(BF16)
        wf_sc[c & 1, q, rb2 * 16:rb2 * 16 + 16, ln] = w[0:16]
        wf_sc[c & 1, q, QB + rb2 * 16:QB + rb2 * 16 + 16, ln] = w[16:]

    def conv_inv(s):
        w = wf_sc[(s // NQ) & 1].reshape(2 * CB, DM)
        yc = _dot(inv_ref[s % NQ], w)
        sd = sd_ref[...].astype(F32).reshape(1, DM)
        y_sc[s & 3] = yc + u_sc[seg(s), :].astype(F32) * sd

    scale = DH ** -0.5
    cexp = scale * float(np.log2(np.e))

    def make_mask(n, x_layers, q0=0):
        qi = jax.lax.broadcasted_iota(jnp.int32, (n - q0, n), 0) + q0
        ki = jax.lax.broadcasted_iota(jnp.int32, (n - q0, n), 1)

        def layer(i):
            xl = jnp.where(i < M2 + SEG, x_layers[0], x_layers[-1])
            return jnp.where(i < M, 0, jnp.where(i < M2, 1, xl))
        same = layer(qi) == layer(ki)
        ok = same & ((qi < M2) | (ki < M2) | (qi >= ki))
        fill = jnp.where(same, -1e9 / scale, -jnp.inf).astype(F32)
        return ok, fill

    def probs(q, k, mask):
        ok, fill = mask
        s = _dot_nt(q, k)
        s = jnp.where(ok, s, fill)
        m = jnp.max(s, axis=-1, keepdims=True)
        p = jnp.exp2((s - m) * cexp)
        l = jnp.sum(p, axis=-1, keepdims=True)
        r = pl.reciprocal(l, approx=True)
        r = r * (2.0 - l * r)
        return (p * r).astype(BF16)

    def w_head(g, mats):
        return _unpack(jnp.concatenate([w_sc[mi * NG + g // HG, g % HG] for mi in mats], axis=1))

    def proj_split(hq, hkv, g):
        q = _dot(hq, w_head(g, (0,))).astype(BF16)
        kv = _dot(hkv, w_head(g, (1, 2))).astype(BF16)
        return q, kv[:, :DH], kv[:, DH:]

    def xn(s):
        return _unpack(xn_sc[clip(s, NSEG - 1), :, 0:DM])

    def out_proj(n, g0, g1, j):
        return _dot(_unpack(o_sc[0:n // 2, g0 * DH:g1 * DH]),
                    wo_sc[g0 * DH:g1 * DH, j * 128:(j + 1) * 128])

    def attend(proj, n, mask, dist, hook=None):
        D1, D2 = dist
        HA = H - D1 - D2 - 1
        NE = min(D1 + D2, NT - 1)
        qkvs = {}
        ps = {}
        outs = {}
        for it in range(H + D1 + D2):
            if it < H:
                qkvs[it] = proj(it)
            g = it - D1
            if 0 <= g < H:
                ps[g] = probs(qkvs[g][0], qkvs[g][1], mask)
            g = it - D1 - D2
            if 0 <= g < H:
                o = _dot(ps.pop(g), qkvs.pop(g)[2])
                o_sc[0:n // 2, g * DH:(g + 1) * DH] = _pack(o)
            if hook is not None:
                hook(it)
            j = it - (H - 1)
            if 0 <= j < NE:
                outs[j] = out_proj(n, 0, HA, j)
        for j in range(NE, NT):
            outs[j] = out_proj(n, 0, H, j)
        for j in range(NE):
            outs[j] = out_proj(n, HA, H, j) + outs[j]
        return jnp.concatenate([outs[j] for j in range(NT)], axis=1)

    def side2(t, a2):
        x3 = x2_sc[(t - 2) & 3] + a2
        x4 = x3 + _ln(x3) * y_sc[(t - 2) & 3]
        x4 = x4.astype(out_sc.dtype)
        out_sc[seg(t - 2), :] = x4
        return x4

    def finish(t, xr, yt, mem, a1, spec):
        if spec:
            conv_spec((t + 1) // NQ + 1, (t + 1) % NQ)
        xq = xn(t + 1)
        for g in range(NPA, NPA + NPB):
            fill_sc[g - NPA] = _pack(_dot(xq, w_head(g, (0,))))
        conv_inv(t + 1)
        x1 = xr.astype(F32) + a1
        x2 = x1 + _ln(x1) * yt
        h_sc[0:M, :] = _pack(mem)
        h_sc[M:, :] = _pack(_ln(x2))
        x2_sc[t & 3] = x2

    def pinned(rows, pins):
        never = never_sm[0] > 0
        hs = {0: rows}
        r = _pack(rows)
        tiles = [r[:, n * 128:(n + 1) * 128] for n in range(NT)]
        for g, n, d in sorted(pins, key=lambda p: p[0]):
            tiles[n] = jnp.where(never, d, tiles[n])
            hs[g] = _unpack(jnp.concatenate(tiles, axis=1))
        return lambda g: hs[max(k for k in hs if k <= g)]

    def pin_tiles(g0, stride, val):
        v = _pack(val)
        return [(g0 + n * stride, n, v[:, n * 128:(n + 1) * 128]) for n in range(NT)]

    def wait_chunk(ci):
        for cp in w_copies(0, ci):
            cp.wait()

    def relayout(ci, b):
        d0 = scaled(b, 16)
        r0 = scaled(b, 8)
        xw = pltpu.bitcast(st_sc[ci, pl.ds(d0, 16)], U32).reshape(8, 2, HG, DH)
        a = xw[:, 0]
        bb = xw[:, 1]
        lo = jnp.swapaxes((a & U32(0xFFFF)) | (bb << 16), 0, 1)
        hi = jnp.swapaxes((a >> 16) | (bb & U32(0xFFFF0000)), 0, 1)
        for j in range(HG):
            rows = pl.ds(r0 + (2 * j // HG) * (DH2 // 2), 8)
            w_sc[ci, 2 * j % HG, rows, :] = lo[j]
            w_sc[ci, 2 * j % HG + 1, rows, :] = hi[j]

    NBLK = DH2 // 16
    with jax.named_scope("wait_w"):
        wait_chunk(0)

    def relayout0(b, c):
        relayout(0, b)
        return c
    with jax.named_scope("relayout"):
        jax.lax.fori_loop(0, NBLK, relayout0, 0, unroll=2)

    def pro_stage(ps_, b):
        n = ps_ * NRB + b
        with jax.named_scope("wait_w"):
            @pl.when(n + 1 < NRB)
            def _():
                x_copy(n + 1).wait()

            @pl.when((n >= 2) & (n <= NCH))
            def _():
                wait_chunk(n - 1)
        cr = jnp.clip(n - 1, 0, NCH - 1)
        bl = jnp.minimum(n + 1, NRB - 1)
        cuts = list(range(0, RB - 2, 2)) + [RB]
        npc = len(cuts) - 1
        LAG = 6

        def body(i, c):
            done_r = 0
            s0 = b * RB + 1
            for sg in range(RB):
                hp_sc[sg * S2:(sg + 1) * S2, :] = xn_sc[s0 + sg, :, 0:DM]
            for j in range(HG):
                w = _unpack(wp_sc[j])
                for pi in range(npc):
                    pos = j * npc + pi
                    hx = hp_sc[cuts[pi] * S2:cuts[pi + 1] * S2, :]
                    if pos >= LAG and (pos - LAG) % 3 == 0 and (pos - LAG) // 3 < RB:
                        sn = bl * RB + 1 + (pos - LAG) // 3
                        xv = _pack(_ln(x_sc[seg(sn), :].astype(F32)))
                        xn_sc[sn, :, 0:DM] = xv
                        hx = jnp.concatenate([hx[:-S2], jnp.where(never_sm[0] > 0, xv, hx[-S2:])], axis=0)
                    upto = min(NBLK, -(-pos * NBLK // (HG * npc - 1)))
                    for bb in range(done_r, upto):
                        relayout(cr, bb)
                    done_r = upto
                    r = _pack(_dot(_unpack(hx), w))
                    for sg in range(cuts[pi], cuts[pi + 1]):
                        a = (sg - cuts[pi]) * S2
                        pre_sc[s0 + sg, ps_ * HG + j] = r[a:a + S2]
            return c
        with jax.named_scope("fused"):
            jax.lax.fori_loop(0, never_sm[0] + 1, body, 0)

    def pro_pass(ps_, carry):
        wp_sc[...] = w_sc[ps_]

        def blk(b, c):
            pro_stage(ps_, b)
            return c
        jax.lax.fori_loop(0, NRB, blk, 0)
        return carry
    jax.lax.fori_loop(0, NPASS, pro_pass, 0)

    def warm_block0(q):
        uf, kf = conv_fwd(0, q)
        put_spec(0, q, 0, uf)
        put_spec(0, q, 2, kf)
        kr_sc[q] = kf
        ur, um, kr, km = uf[:QB], uf[QB:], kf[:QB], kf[QB:]
        wf_sc[0, q, :QB] = (ur * kr - um * km).astype(BF16)
        wf_sc[0, q, QB:] = (ur * km + um * kr).astype(BF16)

    with jax.named_scope("wait_in0"):
        for cp in small + in_copies(0):
            cp.wait()
    with jax.named_scope("warm"):
        for sg in range(2 * NQ + 1):
            conv_u(sg)
        for q in range(NQ):
            warm_block0(q)
        conv_spec(1, 0)
        for piece in MAC_PIECES:
            conv_mac(1, 0, piece, 2)
        conv_inv(0)
    with jax.named_scope("wait_wo"):
        wo_copy.wait()
    with jax.named_scope("step0"):
        mem0 = mem0_ref[...].astype(F32)
        h0 = jnp.concatenate([jnp.concatenate([mem0, mem0], axis=0).astype(BF16), xn(0)], axis=0)
        out = attend(lambda g: proj_split(h0, h0, g), RH, make_mask(RH, (0,)), DIST_HALF)
        finish(0, x_sc[0:SEG, :], y_sc[0], jnp.concatenate([out[0:M], mem0], axis=0), out[M2:], False)

    mask12 = make_mask(R, (0, 1))

    def step(t, first, last):
        if first:
            conv_spec_later = functools.partial(conv_spec, t // NQ + 1, t % NQ)
        x4 = side2(t, op_sc[...])
        un = conv_u(t + 2 * NQ)
        hm = _unpack(h_sc[0:M, :])
        hx2 = _unpack(h_sc[M:, :])
        h48 = jnp.concatenate([hm, hx2], axis=0)
        x1n = pinned(xn(t), pin_tiles(PIN_U if first else PIN_U2, 1, un) + pin_tiles(PIN_X4, X4S, x4))

        def proj(g):
            h80 = jnp.concatenate([hm, x1n(g), hx2], axis=0)
            if g >= NPA + NPB:
                return proj_split(h80, h80, g)
            q, k, v = proj_split(h48, h80, g)
            q1 = pre_sc[t, g] if g < NPA else fill_sc[g - NPA]
            return jnp.concatenate([q[0:M2], _unpack(q1), q[M2:]], axis=0), k, v

        held = {}

        def hook(it):
            if it == SPEC_AT:
                if first:
                    conv_spec_later()
                for piece in MAC_PIECES:
                    conv_mac(t // NQ + 1, t % NQ, piece, NB)
            if it == H:
                held["x"] = x_sc[seg(t), :]
                held["y"] = y_sc[t & 3]
        out = attend(proj, R, mask12, DIST, hook)
        op_sc[...] = out[RH:]
        finish(t, held["x"], held["y"], out[0:M2], out[M2:RH], not last)

    def steps(i, carry):
        for j in range(UNROLL):
            step(1 + i * UNROLL + j, j == 0, j == UNROLL - 1)
        return carry

    def phase(p, carry):
        @pl.when(p == 1)
        def _():
            for cp in in_copies(2):
                cp.wait()

        @pl.when(p >= 2)
        def _():
            out_copy((p - 2) * PH, PH).start()

        with jax.named_scope("steps"):
            jax.lax.fori_loop(p * PHI, (p + 1) * PHI, steps, 0)
        return carry

    for cp in in_copies(1):
        cp.wait()
    jax.lax.fori_loop(0, NPH, phase, 0)
    out_copy((NPH - 2) * PH, NSEG - 2 - (NPH - 2) * PH).start()

    with jax.named_scope("step_last"):
        x4 = side2(NSEG, op_sc[...])
        hm = _unpack(h_sc[0:M, :])
        hx = pinned(_unpack(h_sc[M:, :]), pin_tiles(PIN_X4, 0, x4))
        out = attend(lambda g: proj_split(hx(g), jnp.concatenate([hm, hx(g)], axis=0), g),
                     SEG, make_mask(RH, (1,), M2), DIST_LAST)
        side2(NSEG + 1, out)
    out_copy(NSEG - 2, 2).start()
    pltpu.make_async_copy(out_sc, o_hbm, sem_out).wait()


def pallas_interleave_layers__memory_aug_recurrent_mem_tr__ssm_conv_h3__prompt_kernel(
    A_x, A_mem0, A_Wq, A_Wk, A_Wv, A_Wo, A_seg_len,
    B_q, B_k, B_v, B_shift_k, B_ssm_k, B_ssm_D,
):
    del B_q
    seg = int(A_seg_len) if isinstance(A_seg_len, (int, np.integer)) else CB // NQ
    return _run(A_x, A_mem0, A_Wq, A_Wk, A_Wv, A_Wo, B_k, B_v, B_shift_k, B_ssm_k, B_ssm_D, SEG=seg)


@functools.partial(jax.jit, static_argnames=("SEG",))
def _run(A_x, A_mem0, A_Wq, A_Wk, A_Wv, A_Wo, B_k, B_v, B_shift_k, B_ssm_k, B_ssm_D, *, SEG):
    B, S, DM = A_x.shape
    assert B == 1
    H, DH = A_Wq.shape[1], A_Wq.shape[2]
    M = A_mem0.shape[1]
    KS = B_shift_k.shape[1]
    R = 2 * (M + SEG)
    NSEG = S // SEG
    NB = S // CB
    QB = CB // NQ
    NCH = 3 * H // HG
    fwd, inv = _dft_constants()

    kern = functools.partial(_kernel, S=S, DM=DM, H=H, DH=DH, M=M, SEG=SEG)
    any_spec = pl.BlockSpec(memory_space=pl.ANY)
    out = pl.pallas_call(
        kern,
        out_shape=jax.ShapeDtypeStruct((S, DM), A_x.dtype),
        in_specs=[any_spec] * 13,
        out_specs=any_spec,
        scratch_shapes=[
            pltpu.VMEM((NB + 2, NQ, QB // 8, DM // 128, 4, 8, 128), F32),
            pltpu.VMEM((NQ, 2 * QB, DM), F32),
            pltpu.VMEM((2, NQ, 2 * QB, DM), BF16),
            pltpu.VMEM((4, SEG, DM), F32),
            pltpu.VMEM((4, SEG, DM), F32),
            pltpu.VMEM((S, DM), BF16),
            pltpu.VMEM((SEG, DM), F32),
            pltpu.VMEM((NSEG, NPA, SEG // 2, DH), U32),
            pltpu.VMEM((NPB, SEG // 2, DH), U32),
            pltpu.VMEM((NSEG, SEG // 2, -(-DM // 256) * 256), U32),
            pltpu.VMEM((NCH, HG, DM // 2, DH), U32),
            pltpu.VMEM((HG, DM // 2, DH), U32),
            pltpu.VMEM((H * DH, DM), BF16),
            pltpu.VMEM((R // 2, H * DH), U32),
            pltpu.VMEM((S, DM), BF16),
            pltpu.VMEM((S, DM), BF16),
            pltpu.VMEM((DM, S), BF16),
            pltpu.VMEM((NCH, DM // 2, 2 * HG, DH), BF16),
            pltpu.VMEM((S, DM), A_x.dtype),
            pltpu.VMEM(fwd.shape, BF16),
            pltpu.VMEM(inv.shape, BF16),
            pltpu.VMEM((S + KPAD, DM), BF16),
            pltpu.VMEM((RB * SEG // 2, DM), U32),
            pltpu.VMEM((M + SEG // 2, DM), U32),
            pltpu.VMEM((M, DM), BF16),
            pltpu.VMEM((KS, DM), BF16),
            pltpu.VMEM((DM,), BF16),
            pltpu.SMEM((1,), jnp.int32),
            pltpu.SemaphoreType.DMA(((NSEG - 1) // RB,)),
            pltpu.SemaphoreType.DMA((3,)),
            pltpu.SemaphoreType.DMA((NCH + 1,)),
            pltpu.SemaphoreType.DMA(()),
        ],
        compiler_params=pltpu.CompilerParams(vmem_limit_bytes=120 * 1024 * 1024),
    )(
        A_x.reshape(S, DM), A_mem0.reshape(M, DM), A_Wq, A_Wk, A_Wv,
        A_Wo.reshape(H * DH, DM), B_k.reshape(S, DM), B_v.reshape(S, DM),
        B_shift_k.T, B_ssm_k, B_ssm_D,
        jnp.asarray(fwd, BF16), jnp.asarray(inv, BF16),
    )
    return out.reshape(B, S, DM)
```

```python
import functools

import numpy as np
import jax
import jax.numpy as jnp
import jax.experimental.pallas as pl
import jax.experimental.pallas.tpu as pltpu

F32 = jnp.float32
BF16 = jnp.bfloat16
U32 = jnp.uint32

CB = 128
NQ = 4
KPAD = 16
HG = 8
NPA = 16
NPB = 12
RB = 9
UNROLL = 3
PHI = 3
PIN_U2, X4S = 1, 0
SPEC_AT, PIN_U, PIN_X4 = 7, 1, 16
DIST, DIST_HALF, DIST_LAST = (1, 2), (1, 3), (2, 3)


def _dft_constants():
    qb = CB // NQ
    n = np.arange(CB, dtype=np.float64)
    fwd = np.zeros((NQ, 2 * qb, CB))
    for q in range(NQ):
        f = q * qb + np.concatenate([np.arange(0, qb, 2), np.arange(1, qb, 2)])
        ang = (np.pi * (2.0 * f + 1.0) / (2 * CB))[:, None] * n[None, :]
        fwd[q, :qb] = np.cos(ang)
        fwd[q, qb:] = -np.sin(ang)
    inv = fwd.reshape(2 * CB, CB).T / CB
    return fwd.astype(np.float32), inv.reshape(NQ, CB // NQ, 2 * CB).astype(np.float32)


def _ln(x, eps=1e-5):
    d = x.shape[-1]
    m = jnp.sum(x, axis=-1, keepdims=True) * (1.0 / d)
    xc = x - m
    v = jnp.sum(xc * xc, axis=-1, keepdims=True) * (1.0 / d)
    return xc * jax.lax.rsqrt(v + eps)


def _dot(a, b):
    return jnp.dot(a, b, preferred_element_type=F32)


def _dot_nt(a, b):
    return jax.lax.dot_general(a, b, (((1,), (1,)), ((), ())), preferred_element_type=F32)


def _pack(x):
    return pltpu.bitcast(x.astype(BF16), U32)


def _unpack(x):
    return pltpu.bitcast(x, BF16)


def _in_order(actions):
    def body(i, c):
        for j, act in enumerate(actions):
            pl.when(i == j)(act)
        return c
    jax.lax.fori_loop(0, len(actions), body, 0)


def _kernel(x_hbm, mem0_hbm, wq_hbm, wk_hbm, wv_hbm, wo_hbm, k_hbm, v_hbm,
            sh_hbm, sk_hbm, sd_hbm, fwd_hbm, inv_hbm, o_hbm,
            sp_sc, kr_sc, wf_sc, x2_sc, y_sc, u_sc, op_sc, pre_sc, fill_sc, xn_sc, wa_sc, wb_sc, wo_sc, o_sc,
            x_sc, v_sc, sk_sc, st_sc, out_sc, fwd_ref, inv_ref,
            k_sc, hp_sc, h_sc, mem0_ref, sh_ref, sd_ref,
            never_sm, sem_x, sem_in, sem_w, sem_out,
            *, S, DM, H, DH, M, SEG):
    NSEG = S // SEG
    M2 = 2 * M
    S2 = SEG // 2
    R = M2 + 2 * SEG
    RH = M2 + SEG
    NB = S // CB
    QB = CB // NQ
    HB = QB // 2
    NT = DM // 128
    PH = PHI * UNROLL
    NRB = (NSEG - 1) // RB
    NPH = (NSEG - 1) // PH
    NG = H // HG
    NCH = 3 * NG
    NPASS = NPA // HG
    DH2 = DM // 2
    KS = sh_ref.shape[0]
    assert QB == SEG and NRB * RB == NSEG - 1 and NPH * PH == NSEG - 1 and NPASS == 2 and 2 * NRB >= NCH + 1

    mem0_copy = pltpu.make_async_copy(mem0_hbm, mem0_ref, sem_x.at[0])
    small = [pltpu.make_async_copy(s, d, sem_in.at[0]) for s, d in [
        (sh_hbm, sh_ref), (sd_hbm, sd_ref), (fwd_hbm, fwd_ref), (inv_hbm, inv_ref)]]

    def x_copy(b):
        if isinstance(b, int) and b == 0:
            rows = pl.ds(0, (RB + 1) * SEG)
        else:
            rows = pl.ds(pl.multiple_of((b * RB + 1) * SEG, SEG), RB * SEG)
        return pltpu.make_async_copy(x_hbm.at[rows], x_sc.at[rows], sem_x.at[b])

    kb = (0, (2 * NQ + 1) * SEG, (2 * NQ + PH + 1) * SEG, S)
    sb = (0, 2 * CB, ((PH + 1) // NQ + 2) * CB, S)

    def in_copies(part):
        def rng(b):
            return pl.ds(b[part], b[part + 1] - b[part])
        sem = sem_in.at[part]
        return [
            pltpu.make_async_copy(k_hbm.at[rng(kb)],
                                  k_sc.at[pl.ds(KPAD + kb[part], kb[part + 1] - kb[part])], sem),
            pltpu.make_async_copy(v_hbm.at[rng(kb)], v_sc.at[rng(kb)], sem),
            pltpu.make_async_copy(sk_hbm.at[:, rng(sb)], sk_sc.at[:, rng(sb)], sem),
        ]

    def w_copies(ci, dst=None):
        src = (wq_hbm, wk_hbm, wv_hbm)[ci // NG]
        dst = ci if dst is None else dst
        return [pltpu.make_async_copy(src.at[pl.ds(hf * DH2, DH2), pl.ds((ci % NG) * HG, HG), :],
                                      st_sc.at[dst, :, pl.ds(hf * HG, HG), :], sem_w.at[dst])
                for hf in range(2)]

    wo_copy = pltpu.make_async_copy(wo_hbm, wo_sc, sem_w.at[NCH])

    def out_copy(lo, n):
        rows = pl.ds(lo * SEG if isinstance(lo, int) else pl.multiple_of(lo * SEG, SEG), n * SEG)
        return pltpu.make_async_copy(out_sc.at[rows], o_hbm.at[rows], sem_out)

    def start_all(cps):
        def act():
            for cp in cps:
                cp.start()
        return act

    order = [[mem0_copy, x_copy(0)], w_copies(0), [x_copy(1)], [x_copy(2)]]
    for ci in range(1, NCH):
        order.append(w_copies(ci) + ([x_copy(ci + 2)] if ci + 2 < NRB else []))
        if ci == NRB - 2:
            order.append(small + in_copies(0))
    order += [[wo_copy], in_copies(1), in_copies(2)]
    for i in range(0, len(order), 5):
        _in_order([start_all(cps) for cps in order[i:i + 5]])

    never_sm[0] = 0
    k_sc[0:KPAD, :] = jnp.zeros((KPAD, DM), BF16)
    sp_sc[NB + 1] = jnp.zeros(sp_sc.shape[1:], F32)
    op_sc[...] = jnp.zeros(op_sc.shape, F32)
    x2_sc[...] = jnp.zeros(x2_sc.shape, F32)
    y_sc[...] = jnp.zeros(y_sc.shape, F32)
    mem0_copy.wait()
    x_copy(0).wait()
    for sg in range(RB + 1):
        xn_sc[sg, :, 0:DM] = _pack(_ln(x_sc[sg * SEG:(sg + 1) * SEG, :].astype(F32)))

    def clip(i, hi):
        return min(max(i, 0), hi) if isinstance(i, int) else jnp.clip(i, 0, hi)

    def scaled(i, m):
        return i * m if isinstance(i, int) else pl.multiple_of(i * m, m)

    def seg(i):
        return pl.ds(scaled(clip(i, NSEG - 1), SEG), SEG)

    def conv_u(s, ln=slice(None)):
        r0 = scaled(clip(s, NSEG - 1), SEG)
        sh = sh_ref[:, ln].astype(F32)
        kk = k_sc[pl.ds(r0, KPAD + SEG), ln].astype(F32)
        ks = kk[KPAD:] * sh[0:1]
        for j in range(1, KS):
            ks = ks + pltpu.roll(kk, j, 0)[KPAD:] * sh[j:j + 1]
        u = (ks * v_sc[pl.ds(r0, SEG), ln].astype(F32)).astype(BF16)
        u_sc[pl.ds(r0, SEG), ln] = u
        return u

    def conv_fwd(c, q):
        t0 = scaled(clip(c, NB - 1), CB)
        f = fwd_ref[q]
        uf = _dot(f, u_sc[pl.ds(t0, CB), :])
        kf = _dot_nt(f, sk_sc[:, pl.ds(t0, CB)])
        return uf, kf

    def put_spec(cs, q, which, val):
        for rb in range(QB // 8):
            for n in range(NT):
                ln = slice(n * 128, (n + 1) * 128)
                sp_sc[cs, q, rb, n, which] = val[rb * 8:rb * 8 + 8, ln]
                sp_sc[cs, q, rb, n, which + 1] = val[QB + rb * 8:QB + rb * 8 + 8, ln]

    def conv_spec(c, q):
        uf, kf = conv_fwd(c, q)
        cs = clip(c, NB)
        put_spec(cs, q, 0, uf)
        pk = kr_sc[q]
        kr_sc[q] = kf
        kp = jnp.concatenate([
            kf[0:HB] - pk[QB:QB + HB],
            kf[HB:QB] + pk[QB + HB:],
            kf[QB:QB + HB] + pk[0:HB],
            kf[QB + HB:] - pk[HB:QB]], axis=0)
        put_spec(cs, q, 2, kp)

    MAC_PIECES = [(rb, n) for rb in range(QB // 16) for n in range(NT)]

    def conv_mac(c, q, piece, nterms):
        rb2, n = piece
        cs = clip(c, NB)
        acc = []
        for rb in (2 * rb2, 2 * rb2 + 1):
            ar = None
            ai = None
            for j in range(nterms):
                if isinstance(cs, int):
                    uj, kj = j, cs - j
                else:
                    uj = jnp.minimum(j, cs)
                    kj = jnp.where(cs - j >= 0, cs - j, NB + 1)
                ur = sp_sc[uj, q, rb, n, 0]
                um = sp_sc[uj, q, rb, n, 1]
                kr = sp_sc[kj, q, rb, n, 2]
                km = sp_sc[kj, q, rb, n, 3]
                tr = ur * kr - um * km
                ti = ur * km + um * kr
                ar = tr if ar is None else ar + tr
                ai = ti if ai is None else ai + ti
            acc.append((ar, ai))
        ln = slice(n * 128, (n + 1) * 128)
        w = jnp.concatenate([acc[0][0], acc[1][0], acc[0][1], acc[1][1]], axis=0).astype(BF16)
        wf_sc[c & 1, q, rb2 * 16:rb2 * 16 + 16, ln] = w[0:16]
        wf_sc[c & 1, q, QB + rb2 * 16:QB + rb2 * 16 + 16, ln] = w[16:]

    def conv_inv(s):
        w = wf_sc[(s // NQ) & 1].reshape(2 * CB, DM)
        yc = _dot(inv_ref[s % NQ], w)
        sd = sd_ref[...].astype(F32).reshape(1, DM)
        y_sc[s & 3] = yc + u_sc[seg(s), :].astype(F32) * sd

    scale = DH ** -0.5
    cexp = scale * float(np.log2(np.e))

    def make_mask(n, x_layers, q0=0):
        qi = jax.lax.broadcasted_iota(jnp.int32, (n - q0, n), 0) + q0
        ki = jax.lax.broadcasted_iota(jnp.int32, (n - q0, n), 1)

        def layer(i):
            xl = jnp.where(i < M2 + SEG, x_layers[0], x_layers[-1])
            return jnp.where(i < M, 0, jnp.where(i < M2, 1, xl))
        same = layer(qi) == layer(ki)
        ok = same & ((qi < M2) | (ki < M2) | (qi >= ki))
        fill = jnp.where(same, -1e9 / scale, -jnp.inf).astype(F32)
        return ok, fill

    def probs(q, k, mask):
        ok, fill = mask
        s = _dot_nt(q, k)
        s = jnp.where(ok, s, fill)
        m = jnp.max(s, axis=-1, keepdims=True)
        p = jnp.exp2((s - m) * cexp)
        l = jnp.sum(p, axis=-1, keepdims=True)
        r = pl.reciprocal(l, approx=True)
        r = r * (2.0 - l * r)
        return (p * r).astype(BF16)

    def w_slot(ci):
        return (wb_sc, ci) if 1 <= ci < NRB - 1 else (wa_sc, max(ci - (NRB - 2), 0))

    def w_head(g, mats):
        slots = [w_slot(mi * NG + g // HG) for mi in mats]
        return _unpack(jnp.concatenate([ref[i, g % HG] for ref, i in slots], axis=1))

    def proj_split(hq, hkv, g):
        q = _dot(hq, w_head(g, (0,))).astype(BF16)
        kv = _dot(hkv, w_head(g, (1, 2))).astype(BF16)
        return q, kv[:, :DH], kv[:, DH:]

    def xn(s):
        return _unpack(xn_sc[clip(s, NSEG - 1), :, 0:DM])

    def out_proj(n, g0, g1, j):
        return _dot(_unpack(o_sc[0:n // 2, g0 * DH:g1 * DH]),
                    wo_sc[g0 * DH:g1 * DH, j * 128:(j + 1) * 128])

    def attend(proj, n, mask, dist, hook=None):
        D1, D2 = dist
        HA = H - D1 - D2 - 1
        NE = min(D1 + D2, NT - 1)
        qkvs = {}
        ps = {}
        outs = {}
        for it in range(H + D1 + D2):
            if it < H:
                qkvs[it] = proj(it)
            g = it - D1
            if 0 <= g < H:
                ps[g] = probs(qkvs[g][0], qkvs[g][1], mask)
            g = it - D1 - D2
            if 0 <= g < H:
                o = _dot(ps.pop(g), qkvs.pop(g)[2])
                o_sc[0:n // 2, g * DH:(g + 1) * DH] = _pack(o)
            if hook is not None:
                hook(it)
            j = it - (H - 1)
            if 0 <= j < NE:
                outs[j] = out_proj(n, 0, HA, j)
        for j in range(NE, NT):
            outs[j] = out_proj(n, 0, H, j)
        for j in range(NE):
            outs[j] = out_proj(n, HA, H, j) + outs[j]
        return jnp.concatenate([outs[j] for j in range(NT)], axis=1)

    def side2(t, a2):
        x3 = x2_sc[(t - 2) & 3] + a2
        x4 = x3 + _ln(x3) * y_sc[(t - 2) & 3]
        x4 = x4.astype(out_sc.dtype)
        out_sc[seg(t - 2), :] = x4
        return x4

    def finish(t, xr, yt, mem, a1, spec):
        if spec:
            conv_spec((t + 1) // NQ + 1, (t + 1) % NQ)
        xq = xn(t + 1)
        for g in range(NPA, NPA + NPB):
            fill_sc[g - NPA] = _pack(_dot(xq, w_head(g, (0,))))
        conv_inv(t + 1)
        x1 = xr.astype(F32) + a1
        x2 = x1 + _ln(x1) * yt
        h_sc[0:M, :] = _pack(mem)
        h_sc[M:, :] = _pack(_ln(x2))
        x2_sc[t & 3] = x2

    def pinned(rows, pins):
        never = never_sm[0] > 0
        hs = {0: rows}
        r = _pack(rows)
        tiles = [r[:, n * 128:(n + 1) * 128] for n in range(NT)]
        for g, n, d in sorted(pins, key=lambda p: p[0]):
            tiles[n] = jnp.where(never, d, tiles[n])
            hs[g] = _unpack(jnp.concatenate(tiles, axis=1))
        return lambda g: hs[max(k for k in hs if k <= g)]

    def pin_tiles(g0, stride, val):
        v = _pack(val)
        return [(g0 + n * stride, n, v[:, n * 128:(n + 1) * 128]) for n in range(NT)]

    def wait_chunk(ci):
        for cp in w_copies(0, ci):
            cp.wait()

    def relayout(ci, dst, slot, b):
        d0 = scaled(b, 16)
        r0 = scaled(b, 8)
        xw = pltpu.bitcast(st_sc[ci, pl.ds(d0, 16)], U32).reshape(8, 2, HG, DH)
        a = xw[:, 0]
        bb = xw[:, 1]
        lo = jnp.swapaxes((a & U32(0xFFFF)) | (bb << 16), 0, 1)
        hi = jnp.swapaxes((a >> 16) | (bb & U32(0xFFFF0000)), 0, 1)
        for j in range(HG):
            rows = pl.ds(r0 + (2 * j // HG) * (DH2 // 2), 8)
            dst[slot, 2 * j % HG, rows, :] = lo[j]
            dst[slot, 2 * j % HG + 1, rows, :] = hi[j]

    NBLK = DH2 // 16
    with jax.named_scope("wait_w"):
        wait_chunk(0)

    def relayout0(b, c):
        relayout(0, wa_sc, 0, b)
        return c
    with jax.named_scope("relayout"):
        jax.lax.fori_loop(0, NBLK, relayout0, 0, unroll=2)

    def pro_stage(ps_, b):
        n = ps_ * NRB + b
        with jax.named_scope("wait_w"):
            if ps_ == 0:
                @pl.when(b + 1 < NRB)
                def _():
                    x_copy(b + 1).wait()

            @pl.when((n >= 2) & (n <= NCH))
            def _():
                wait_chunk(n - 1)
        cr = jnp.clip(n - 1, 0, NCH - 1)
        dst, slot = (wb_sc, cr) if ps_ == 0 else (wa_sc, cr - (NRB - 2))
        src, si = w_slot(ps_)
        bl = jnp.minimum(b + 1, NRB - 1)
        cuts = list(range(0, RB - 2, 2)) + [RB]
        npc = len(cuts) - 1
        LAG = 6

        def body(i, c):
            done_r = 0
            s0 = b * RB + 1
            for sg in range(RB):
                hp_sc[sg * S2:(sg + 1) * S2, :] = xn_sc[s0 + sg, :, 0:DM]
            for j in range(HG):
                w = _unpack(src[si, j])
                for pi in range(npc):
                    pos = j * npc + pi
                    hx = hp_sc[cuts[pi] * S2:cuts[pi + 1] * S2, :]
                    if ps_ == 0 and pos >= LAG and (pos - LAG) % 3 == 0 and (pos - LAG) // 3 < RB:
                        sn = bl * RB + 1 + (pos - LAG) // 3
                        xv = _pack(_ln(x_sc[seg(sn), :].astype(F32)))
                        xn_sc[sn, :, 0:DM] = xv
                        hx = jnp.concatenate([hx[:-S2], jnp.where(never_sm[0] > 0, xv, hx[-S2:])], axis=0)
                    if ps_ == 1 and pos % 3 == 1 and pos // 3 < 2 * NT:
                        k = pos // 3
                        conv_u(jnp.minimum(2 * b + k // NT, 2 * NQ),
                               slice((k % NT) * 128, (k % NT + 1) * 128))
                    upto = min(NBLK, -(-pos * NBLK // (HG * npc - 1)))
                    for bb in range(done_r, upto):
                        relayout(cr, dst, slot, bb)
                    done_r = upto
                    r = _pack(_dot(_unpack(hx), w))
                    for sg in range(cuts[pi], cuts[pi + 1]):
                        a = (sg - cuts[pi]) * S2
                        pre_sc[s0 + sg, ps_ * HG + j] = r[a:a + S2]
            return c
        with jax.named_scope("fused"):
            jax.lax.fori_loop(0, never_sm[0] + 1, body, 0)

    for ps_ in range(NPASS):
        if ps_ == 1:
            with jax.named_scope("wait_in0"):
                for cp in small + in_copies(0):
                    cp.wait()

        def blk(b, c, ps_=ps_):
            pro_stage(ps_, b)
            return c
        jax.lax.fori_loop(0, NRB, blk, 0)

    def warm_block0(q):
        uf, kf = conv_fwd(0, q)
        put_spec(0, q, 0, uf)
        put_spec(0, q, 2, kf)
        kr_sc[q] = kf
        ur, um, kr, km = uf[:QB], uf[QB:], kf[:QB], kf[QB:]
        wf_sc[0, q, :QB] = (ur * kr - um * km).astype(BF16)
        wf_sc[0, q, QB:] = (ur * km + um * kr).astype(BF16)

    with jax.named_scope("wait_wo"):
        wo_copy.wait()
    with jax.named_scope("step0"):
        mem0 = mem0_ref[...].astype(F32)
        h0 = jnp.concatenate([jnp.concatenate([mem0, mem0], axis=0).astype(BF16), xn(0)], axis=0)

        def hook0(it):
            if it in (2, 6, 10, 14):
                warm_block0((it - 2) // 4)
            if it == 18:
                conv_spec(1, 0)
                for piece in MAC_PIECES:
                    conv_mac(1, 0, piece, 2)
            if it == 22:
                conv_inv(0)
        out = attend(lambda g: proj_split(h0, h0, g), RH, make_mask(RH, (0,)), DIST_HALF, hook0)
        finish(0, x_sc[0:SEG, :], y_sc[0], jnp.concatenate([out[0:M], mem0], axis=0), out[M2:], False)

    mask12 = make_mask(R, (0, 1))

    def step(t, first, last):
        if first:
            conv_spec_later = functools.partial(conv_spec, t // NQ + 1, t % NQ)
        x4 = side2(t, op_sc[...])
        un = conv_u(t + 2 * NQ)
        hm = _unpack(h_sc[0:M, :])
        hx2 = _unpack(h_sc[M:, :])
        h48 = jnp.concatenate([hm, hx2], axis=0)
        x1n = pinned(xn(t), pin_tiles(PIN_U if first else PIN_U2, 1, un) + pin_tiles(PIN_X4, X4S, x4))

        def proj(g):
            h80 = jnp.concatenate([hm, x1n(g), hx2], axis=0)
            if g >= NPA + NPB:
                return proj_split(h80, h80, g)
            q, k, v = proj_split(h48, h80, g)
            q1 = pre_sc[t, g] if g < NPA else fill_sc[g - NPA]
            return jnp.concatenate([q[0:M2], _unpack(q1), q[M2:]], axis=0), k, v

        held = {}

        def hook(it):
            if it == SPEC_AT:
                if first:
                    conv_spec_later()
                for piece in MAC_PIECES:
                    conv_mac(t // NQ + 1, t % NQ, piece, NB)
            if it == H:
                held["x"] = x_sc[seg(t), :]
                held["y"] = y_sc[t & 3]
        out = attend(proj, R, mask12, DIST, hook)
        op_sc[...] = out[RH:]
        finish(t, held["x"], held["y"], out[0:M2], out[M2:RH], not last)

    def steps(i, carry):
        for j in range(UNROLL):
            step(1 + i * UNROLL + j, j == 0, j == UNROLL - 1)
        return carry

    def phase(p, carry):
        @pl.when(p == 1)
        def _():
            for cp in in_copies(2):
                cp.wait()

        @pl.when(p >= 2)
        def _():
            out_copy((p - 2) * PH, PH).start()

        with jax.named_scope("steps"):
            jax.lax.fori_loop(p * PHI, (p + 1) * PHI, steps, 0)
        return carry

    for cp in in_copies(1):
        cp.wait()
    jax.lax.fori_loop(0, NPH, phase, 0)
    out_copy((NPH - 2) * PH, NSEG - 2 - (NPH - 2) * PH).start()

    with jax.named_scope("step_last"):
        x4 = side2(NSEG, op_sc[...])
        hm = _unpack(h_sc[0:M, :])
        hx = pinned(_unpack(h_sc[M:, :]), pin_tiles(PIN_X4, 0, x4))
        out = attend(lambda g: proj_split(hx(g), jnp.concatenate([hm, hx(g)], axis=0), g),
                     SEG, make_mask(RH, (1,), M2), DIST_LAST)
        side2(NSEG + 1, out)
    out_copy(NSEG - 2, 2).start()
    pltpu.make_async_copy(out_sc, o_hbm, sem_out).wait()


def pallas_interleave_layers__memory_aug_recurrent_mem_tr__ssm_conv_h3__prompt_kernel(
    A_x, A_mem0, A_Wq, A_Wk, A_Wv, A_Wo, A_seg_len,
    B_q, B_k, B_v, B_shift_k, B_ssm_k, B_ssm_D,
):
    del B_q
    seg = int(A_seg_len) if isinstance(A_seg_len, (int, np.integer)) else CB // NQ
    return _run(A_x, A_mem0, A_Wq, A_Wk, A_Wv, A_Wo, B_k, B_v, B_shift_k, B_ssm_k, B_ssm_D, SEG=seg)


@functools.partial(jax.jit, static_argnames=("SEG",))
def _run(A_x, A_mem0, A_Wq, A_Wk, A_Wv, A_Wo, B_k, B_v, B_shift_k, B_ssm_k, B_ssm_D, *, SEG):
    B, S, DM = A_x.shape
    assert B == 1
    H, DH = A_Wq.shape[1], A_Wq.shape[2]
    M = A_mem0.shape[1]
    KS = B_shift_k.shape[1]
    R = 2 * (M + SEG)
    NSEG = S // SEG
    NRB = (NSEG - 1) // RB
    NB = S // CB
    QB = CB // NQ
    NCH = 3 * H // HG
    fwd, inv = _dft_constants()

    kern = functools.partial(_kernel, S=S, DM=DM, H=H, DH=DH, M=M, SEG=SEG)
    any_spec = pl.BlockSpec(memory_space=pl.ANY)
    out = pl.pallas_call(
        kern,
        out_shape=jax.ShapeDtypeStruct((S, DM), A_x.dtype),
        in_specs=[any_spec] * 13,
        out_specs=any_spec,
        scratch_shapes=[
            pltpu.VMEM((NB + 2, NQ, QB // 8, DM // 128, 4, 8, 128), F32),
            pltpu.VMEM((NQ, 2 * QB, DM), F32),
            pltpu.VMEM((2, NQ, 2 * QB, DM), BF16),
            pltpu.VMEM((4, SEG, DM), F32),
            pltpu.VMEM((4, SEG, DM), F32),
            pltpu.VMEM((S, DM), BF16),
            pltpu.VMEM((SEG, DM), F32),
            pltpu.VMEM((NSEG, NPA, SEG // 2, DH), U32),
            pltpu.VMEM((NPB, SEG // 2, DH), U32),
            pltpu.VMEM((NSEG, SEG // 2, -(-DM // 256) * 256), U32),
            pltpu.VMEM((NCH - NRB + 2, HG, DM // 2, DH), U32),
            pltpu.VMEM((NRB - 1, HG, DM // 2, DH), U32),
            pltpu.VMEM((H * DH, DM), BF16),
            pltpu.VMEM((R // 2, H * DH), U32),
            pltpu.VMEM((S, DM), BF16),
            pltpu.VMEM((S, DM), BF16),
            pltpu.VMEM((DM, S), BF16),
            pltpu.VMEM((NCH, DM // 2, 2 * HG, DH), BF16),
            pltpu.VMEM((S, DM), A_x.dtype),
            pltpu.VMEM(fwd.shape, BF16),
            pltpu.VMEM(inv.shape, BF16),
            pltpu.VMEM((S + KPAD, DM), BF16),
            pltpu.VMEM((RB * SEG // 2, DM), U32),
            pltpu.VMEM((M + SEG // 2, DM), U32),
            pltpu.VMEM((M, DM), BF16),
            pltpu.VMEM((KS, DM), BF16),
            pltpu.VMEM((DM,), BF16),
            pltpu.SMEM((1,), jnp.int32),
            pltpu.SemaphoreType.DMA(((NSEG - 1) // RB,)),
            pltpu.SemaphoreType.DMA((3,)),
            pltpu.SemaphoreType.DMA((NCH + 1,)),
            pltpu.SemaphoreType.DMA(()),
        ],
        compiler_params=pltpu.CompilerParams(vmem_limit_bytes=120 * 1024 * 1024),
    )(
        A_x.reshape(S, DM), A_mem0.reshape(M, DM), A_Wq, A_Wk, A_Wv,
        A_Wo.reshape(H * DH, DM), B_k.reshape(S, DM), B_v.reshape(S, DM),
        B_shift_k.T, B_ssm_k, B_ssm_D,
        jnp.asarray(fwd, BF16), jnp.asarray(inv, BF16),
    )
    return out.reshape(B, S, DM)
```

```python
import functools

import numpy as np
import jax
import jax.numpy as jnp
import jax.experimental.pallas as pl
import jax.experimental.pallas.tpu as pltpu

F32 = jnp.float32
BF16 = jnp.bfloat16
U32 = jnp.uint32

CB = 128
NQ = 4
KPAD = 16
HG = 8
NPA = 16
NPB = 12
RB = 9
PRO_PW, PRO_X0, PRO_XS, PRO_R0, PRO_RS = 24, 11, 4, 2, 2
UNROLL = 3
PHI = 3
PIN_U2, X4S = 1, 0
SPEC_AT, PIN_U, PIN_X4 = 7, 1, 16
DIST, DIST_HALF, DIST_LAST = (1, 2), (1, 3), (2, 3)


def _dft_constants():
    qb = CB // NQ
    n = np.arange(CB, dtype=np.float64)
    fwd = np.zeros((NQ, 2 * qb, CB))
    for q in range(NQ):
        f = q * qb + np.concatenate([np.arange(0, qb, 2), np.arange(1, qb, 2)])
        ang = (np.pi * (2.0 * f + 1.0) / (2 * CB))[:, None] * n[None, :]
        fwd[q, :qb] = np.cos(ang)
        fwd[q, qb:] = -np.sin(ang)
    inv = fwd.reshape(2 * CB, CB).T / CB
    return fwd.astype(np.float32), inv.reshape(NQ, CB // NQ, 2 * CB).astype(np.float32)


def _ln(x, eps=1e-5):
    d = x.shape[-1]
    m = jnp.sum(x, axis=-1, keepdims=True) * (1.0 / d)
    xc = x - m
    v = jnp.sum(xc * xc, axis=-1, keepdims=True) * (1.0 / d)
    return xc * jax.lax.rsqrt(v + eps)


def _dot(a, b):
    return jnp.dot(a, b, preferred_element_type=F32)


def _dot_nt(a, b):
    return jax.lax.dot_general(a, b, (((1,), (1,)), ((), ())), preferred_element_type=F32)


def _pack(x):
    return pltpu.bitcast(x.astype(BF16), U32)


def _unpack(x):
    return pltpu.bitcast(x, BF16)


def _in_order(actions):
    def body(i, c):
        for j, act in enumerate(actions):
            pl.when(i == j)(act)
        return c
    jax.lax.fori_loop(0, len(actions), body, 0)


def _kernel(x_hbm, mem0_hbm, wq_hbm, wk_hbm, wv_hbm, wo_hbm, k_hbm, v_hbm,
            sh_hbm, sk_hbm, sd_hbm, fwd_hbm, inv_hbm, o_hbm,
            sp_sc, kr_sc, wf_sc, x2_sc, y_sc, u_sc, op_sc, pre_sc, fill_sc, xn_sc, wa_sc, wb_sc, wo_sc, o_sc,
            x_sc, v_sc, sk_sc, st_sc, out_sc, fwd_ref, inv_ref,
            k_sc, hp_sc, h_sc, mem0_ref, sh_ref, sd_ref,
            never_sm, sem_x, sem_in, sem_w, sem_out,
            *, S, DM, H, DH, M, SEG):
    NSEG = S // SEG
    M2 = 2 * M
    S2 = SEG // 2
    R = M2 + 2 * SEG
    RH = M2 + SEG
    NB = S // CB
    QB = CB // NQ
    HB = QB // 2
    NT = DM // 128
    PH = PHI * UNROLL
    NRB = (NSEG - 1) // RB
    NPH = (NSEG - 1) // PH
    NG = H // HG
    NCH = 3 * NG
    NPASS = NPA // HG
    DH2 = DM // 2
    KS = sh_ref.shape[0]
    assert QB == SEG and NRB * RB == NSEG - 1 and NPH * PH == NSEG - 1 and NPASS == 2 and 2 * NRB >= NCH + 1

    mem0_copy = pltpu.make_async_copy(mem0_hbm, mem0_ref, sem_x.at[0])
    small = [pltpu.make_async_copy(s, d, sem_in.at[0]) for s, d in [
        (sh_hbm, sh_ref), (sd_hbm, sd_ref), (fwd_hbm, fwd_ref), (inv_hbm, inv_ref)]]

    def x_copy(b):
        if isinstance(b, int) and b == 0:
            rows = pl.ds(0, (RB + 1) * SEG)
        else:
            rows = pl.ds(pl.multiple_of((b * RB + 1) * SEG, SEG), RB * SEG)
        return pltpu.make_async_copy(x_hbm.at[rows], x_sc.at[rows], sem_x.at[b])

    kb = (0, (2 * NQ + 1) * SEG, (2 * NQ + PH + 1) * SEG, S)
    sb = (0, 2 * CB, ((PH + 1) // NQ + 2) * CB, S)

    def in_copies(part):
        def rng(b):
            return pl.ds(b[part], b[part + 1] - b[part])
        sem = sem_in.at[part]
        return [
            pltpu.make_async_copy(k_hbm.at[rng(kb)],
                                  k_sc.at[pl.ds(KPAD + kb[part], kb[part + 1] - kb[part])], sem),
            pltpu.make_async_copy(v_hbm.at[rng(kb)], v_sc.at[rng(kb)], sem),
            pltpu.make_async_copy(sk_hbm.at[:, rng(sb)], sk_sc.at[:, rng(sb)], sem),
        ]

    def w_copies(ci, dst=None):
        src = (wq_hbm, wk_hbm, wv_hbm)[ci // NG]
        dst = ci if dst is None else dst
        return [pltpu.make_async_copy(src.at[pl.ds(hf * DH2, DH2), pl.ds((ci % NG) * HG, HG), :],
                                      st_sc.at[dst, :, pl.ds(hf * HG, HG), :], sem_w.at[dst])
                for hf in range(2)]

    wo_copy = pltpu.make_async_copy(wo_hbm, wo_sc, sem_w.at[NCH])

    def out_copy(lo, n):
        rows = pl.ds(lo * SEG if isinstance(lo, int) else pl.multiple_of(lo * SEG, SEG), n * SEG)
        return pltpu.make_async_copy(out_sc.at[rows], o_hbm.at[rows], sem_out)

    def start_all(cps):
        def act():
            for cp in cps:
                cp.start()
        return act

    order = [[mem0_copy, x_copy(0)], w_copies(0), [x_copy(1)], [x_copy(2)]]
    for ci in range(1, NCH):
        order.append(w_copies(ci) + ([x_copy(ci + 2)] if ci + 2 < NRB else []))
        if ci == NRB - 2:
            order.append(small + in_copies(0))
    order += [[wo_copy], in_copies(1), in_copies(2)]
    for i in range(0, len(order), 5):
        _in_order([start_all(cps) for cps in order[i:i + 5]])

    never_sm[0] = 0
    k_sc[0:KPAD, :] = jnp.zeros((KPAD, DM), BF16)
    sp_sc[NB + 1] = jnp.zeros(sp_sc.shape[1:], F32)
    op_sc[...] = jnp.zeros(op_sc.shape, F32)
    x2_sc[...] = jnp.zeros(x2_sc.shape, F32)
    y_sc[...] = jnp.zeros(y_sc.shape, F32)
    mem0_copy.wait()
    x_copy(0).wait()
    for sg in range(RB + 1):
        xn_sc[sg, :, 0:DM] = _pack(_ln(x_sc[sg * SEG:(sg + 1) * SEG, :].astype(F32)))

    def clip(i, hi):
        return min(max(i, 0), hi) if isinstance(i, int) else jnp.clip(i, 0, hi)

    def scaled(i, m):
        return i * m if isinstance(i, int) else pl.multiple_of(i * m, m)

    def seg(i):
        return pl.ds(scaled(clip(i, NSEG - 1), SEG), SEG)

    def conv_u(s, ln=slice(None)):
        r0 = scaled(clip(s, NSEG - 1), SEG)
        sh = sh_ref[:, ln].astype(F32)
        kk = k_sc[pl.ds(r0, KPAD + SEG), ln].astype(F32)
        ks = kk[KPAD:] * sh[0:1]
        for j in range(1, KS):
            ks = ks + pltpu.roll(kk, j, 0)[KPAD:] * sh[j:j + 1]
        u = (ks * v_sc[pl.ds(r0, SEG), ln].astype(F32)).astype(BF16)
        u_sc[pl.ds(r0, SEG), ln] = u
        return u

    def conv_fwd(c, q):
        t0 = scaled(clip(c, NB - 1), CB)
        f = fwd_ref[q]
        uf = _dot(f, u_sc[pl.ds(t0, CB), :])
        kf = _dot_nt(f, sk_sc[:, pl.ds(t0, CB)])
        return uf, kf

    def put_spec(cs, q, which, val):
        for rb in range(QB // 8):
            for n in range(NT):
                ln = slice(n * 128, (n + 1) * 128)
                sp_sc[cs, q, rb, n, which] = val[rb * 8:rb * 8 + 8, ln]
                sp_sc[cs, q, rb, n, which + 1] = val[QB + rb * 8:QB + rb * 8 + 8, ln]

    def conv_spec(c, q):
        uf, kf = conv_fwd(c, q)
        cs = clip(c, NB)
        put_spec(cs, q, 0, uf)
        pk = kr_sc[q]
        kr_sc[q] = kf
        kp = jnp.concatenate([
            kf[0:HB] - pk[QB:QB + HB],
            kf[HB:QB] + pk[QB + HB:],
            kf[QB:QB + HB] + pk[0:HB],
            kf[QB + HB:] - pk[HB:QB]], axis=0)
        put_spec(cs, q, 2, kp)

    MAC_PIECES = [(rb, n) for rb in range(QB // 16) for n in range(NT)]

    def conv_mac(c, q, piece, nterms):
        rb2, n = piece
        cs = clip(c, NB)
        acc = []
        for rb in (2 * rb2, 2 * rb2 + 1):
            ar = None
            ai = None
            for j in range(nterms):
                if isinstance(cs, int):
                    uj, kj = j, cs - j
                else:
                    uj = jnp.minimum(j, cs)
                    kj = jnp.where(cs - j >= 0, cs - j, NB + 1)
                ur = sp_sc[uj, q, rb, n, 0]
                um = sp_sc[uj, q, rb, n, 1]
                kr = sp_sc[kj, q, rb, n, 2]
                km = sp_sc[kj, q, rb, n, 3]
                tr = ur * kr - um * km
                ti = ur * km + um * kr
                ar = tr if ar is None else ar + tr
                ai = ti if ai is None else ai + ti
            acc.append((ar, ai))
        ln = slice(n * 128, (n + 1) * 128)
        w = jnp.concatenate([acc[0][0], acc[1][0], acc[0][1], acc[1][1]], axis=0).astype(BF16)
        wf_sc[c & 1, q, rb2 * 16:rb2 * 16 + 16, ln] = w[0:16]
        wf_sc[c & 1, q, QB + rb2 * 16:QB + rb2 * 16 + 16, ln] = w[16:]

    def conv_inv(s):
        w = wf_sc[(s // NQ) & 1].reshape(2 * CB, DM)
        yc = _dot(inv_ref[s % NQ], w)
        sd = sd_ref[...].astype(F32).reshape(1, DM)
        y_sc[s & 3] = yc + u_sc[seg(s), :].astype(F32) * sd

    scale = DH ** -0.5
    cexp = scale * float(np.log2(np.e))

    def make_mask(n, x_layers, q0=0):
        qi = jax.lax.broadcasted_iota(jnp.int32, (n - q0, n), 0) + q0
        ki = jax.lax.broadcasted_iota(jnp.int32, (n - q0, n), 1)

        def layer(i):
            xl = jnp.where(i < M2 + SEG, x_layers[0], x_layers[-1])
            return jnp.where(i < M, 0, jnp.where(i < M2, 1, xl))
        same = layer(qi) == layer(ki)
        ok = same & ((qi < M2) | (ki < M2) | (qi >= ki))
        fill = jnp.where(same, -1e9 / scale, -jnp.inf).astype(F32)
        return ok, fill

    def probs(q, k, mask):
        ok, fill = mask
        s = _dot_nt(q, k)
        s = jnp.where(ok, s, fill)
        m = jnp.max(s, axis=-1, keepdims=True)
        p = jnp.exp2((s - m) * cexp)
        l = jnp.sum(p, axis=-1, keepdims=True)
        r = pl.reciprocal(l, approx=True)
        r = r * (2.0 - l * r)
        return (p * r).astype(BF16)

    def w_slot(ci):
        return (wb_sc, ci) if 1 <= ci < NRB - 1 else (wa_sc, max(ci - (NRB - 2), 0))

    def w_head(g, mats):
        slots = [w_slot(mi * NG + g // HG) for mi in mats]
        return _unpack(jnp.concatenate([ref[i, g % HG] for ref, i in slots], axis=1))

    def proj_split(hq, hkv, g):
        q = _dot(hq, w_head(g, (0,))).astype(BF16)
        kv = _dot(hkv, w_head(g, (1, 2))).astype(BF16)
        return q, kv[:, :DH], kv[:, DH:]

    def xn(s):
        return _unpack(xn_sc[clip(s, NSEG - 1), :, 0:DM])

    def out_proj(n, g0, g1, j):
        return _dot(_unpack(o_sc[0:n // 2, g0 * DH:g1 * DH]),
                    wo_sc[g0 * DH:g1 * DH, j * 128:(j + 1) * 128])

    def attend(proj, n, mask, dist, hook=None):
        D1, D2 = dist
        HA = H - D1 - D2 - 1
        NE = min(D1 + D2, NT - 1)
        qkvs = {}
        ps = {}
        outs = {}
        for it in range(H + D1 + D2):
            if it < H:
                qkvs[it] = proj(it)
            g = it - D1
            if 0 <= g < H:
                ps[g] = probs(qkvs[g][0], qkvs[g][1], mask)
            g = it - D1 - D2
            if 0 <= g < H:
                o = _dot(ps.pop(g), qkvs.pop(g)[2])
                o_sc[0:n // 2, g * DH:(g + 1) * DH] = _pack(o)
            if hook is not None:
                hook(it)
            j = it - (H - 1)
            if 0 <= j < NE:
                outs[j] = out_proj(n, 0, HA, j)
        for j in range(NE, NT):
            outs[j] = out_proj(n, 0, H, j)
        for j in range(NE):
            outs[j] = out_proj(n, HA, H, j) + outs[j]
        return jnp.concatenate([outs[j] for j in range(NT)], axis=1)

    def side2(t, a2):
        x3 = x2_sc[(t - 2) & 3] + a2
        x4 = x3 + _ln(x3) * y_sc[(t - 2) & 3]
        x4 = x4.astype(out_sc.dtype)
        out_sc[seg(t - 2), :] = x4
        return x4

    def finish(t, xr, yt, mem, a1, spec):
        if spec:
            conv_spec((t + 1) // NQ + 1, (t + 1) % NQ)
        xq = xn(t + 1)
        for g in range(NPA, NPA + NPB):
            fill_sc[g - NPA] = _pack(_dot(xq, w_head(g, (0,))))
        conv_inv(t + 1)
        x1 = xr.astype(F32) + a1
        x2 = x1 + _ln(x1) * yt
        h_sc[0:M, :] = _pack(mem)
        h_sc[M:, :] = _pack(_ln(x2))
        x2_sc[t & 3] = x2

    def pinned(rows, pins):
        never = never_sm[0] > 0
        hs = {0: rows}
        r = _pack(rows)
        tiles = [r[:, n * 128:(n + 1) * 128] for n in range(NT)]
        for g, n, d in sorted(pins, key=lambda p: p[0]):
            tiles[n] = jnp.where(never, d, tiles[n])
            hs[g] = _unpack(jnp.concatenate(tiles, axis=1))
        return lambda g: hs[max(k for k in hs if k <= g)]

    def pin_tiles(g0, stride, val):
        v = _pack(val)
        return [(g0 + n * stride, n, v[:, n * 128:(n + 1) * 128]) for n in range(NT)]

    def wait_chunk(ci):
        for cp in w_copies(0, ci):
            cp.wait()

    def relayout(ci, dst, slot, b):
        d0 = scaled(b, 16)
        r0 = scaled(b, 8)
        xw = pltpu.bitcast(st_sc[ci, pl.ds(d0, 16)], U32).reshape(8, 2, HG, DH)
        a = xw[:, 0]
        bb = xw[:, 1]
        lo = jnp.swapaxes((a & U32(0xFFFF)) | (bb << 16), 0, 1)
        hi = jnp.swapaxes((a >> 16) | (bb & U32(0xFFFF0000)), 0, 1)
        for j in range(HG):
            rows = pl.ds(r0 + (2 * j // HG) * (DH2 // 2), 8)
            dst[slot, 2 * j % HG, rows, :] = lo[j]
            dst[slot, 2 * j % HG + 1, rows, :] = hi[j]

    NBLK = DH2 // 16
    with jax.named_scope("wait_w"):
        wait_chunk(0)

    def relayout0(b, c):
        relayout(0, wa_sc, 0, b)
        return c
    with jax.named_scope("relayout"):
        jax.lax.fori_loop(0, NBLK, relayout0, 0, unroll=2)

    def pro_stage(ps_, b):
        n = ps_ * NRB + b
        with jax.named_scope("wait_w"):
            if ps_ == 0:
                @pl.when(b + 1 < NRB)
                def _():
                    x_copy(b + 1).wait()

            @pl.when((n >= 2) & (n <= NCH))
            def _():
                wait_chunk(n - 1)
        cr = jnp.clip(n - 1, 0, NCH - 1)
        dst, slot = (wb_sc, cr) if ps_ == 0 else (wa_sc, cr - (NRB - 2))
        src, si = w_slot(ps_)
        bl = jnp.minimum(b + 1, NRB - 1)
        PW = PRO_PW
        npc = RB * S2 // PW
        assert npc * PW == RB * S2 and PRO_R0 + (NBLK - 1) * PRO_RS < HG * npc
        assert PRO_X0 + (max(RB, 2 * NT) - 1) * PRO_XS < HG * npc and 2 * NRB > 2 * NQ

        def body(i, c):
            s0 = b * RB + 1
            for sg in range(RB):
                hp_sc[sg * S2:(sg + 1) * S2, :] = xn_sc[s0 + sg, :, 0:DM]
            for j in range(HG):
                w = _unpack(src[si, j])
                for pi in range(npc):
                    pos = j * npc + pi
                    hx = hp_sc[pi * PW:(pi + 1) * PW, :]
                    k, rem = divmod(pos - PRO_X0, PRO_XS)
                    if ps_ == 0 and rem == 0 and 0 <= k < RB:
                        sn = bl * RB + 1 + k
                        xv = _pack(_ln(x_sc[seg(sn), :].astype(F32)))
                        xn_sc[sn, :, 0:DM] = xv
                        hx = jnp.concatenate([hx[:-S2], jnp.where(never_sm[0] > 0, xv, hx[-S2:])], axis=0)
                    if ps_ == 1 and rem == 0 and 0 <= k < 2 * NT:
                        conv_u(jnp.minimum(2 * b + k // NT, 2 * NQ),
                               slice((k % NT) * 128, (k % NT + 1) * 128))
                    bb, rem = divmod(pos - PRO_R0, PRO_RS)
                    if rem == 0 and 0 <= bb < NBLK:
                        relayout(cr, dst, slot, bb)
                    r = _pack(_dot(_unpack(hx), w))
                    for a in range(0, PW, 8):
                        sg, off = divmod(pi * PW + a, S2)
                        pre_sc[s0 + sg, ps_ * HG + j, off:off + 8, :] = r[a:a + 8]
            return c
        with jax.named_scope("fused"):
            jax.lax.fori_loop(0, never_sm[0] + 1, body, 0)

    for ps_ in range(NPASS):
        if ps_ == 1:
            with jax.named_scope("wait_in0"):
                for cp in small + in_copies(0):
                    cp.wait()

        def blk(b, c, ps_=ps_):
            pro_stage(ps_, b)
            return c
        jax.lax.fori_loop(0, NRB, blk, 0)

    def warm_block0(q):
        uf, kf = conv_fwd(0, q)
        put_spec(0, q, 0, uf)
        put_spec(0, q, 2, kf)
        kr_sc[q] = kf
        ur, um, kr, km = uf[:QB], uf[QB:], kf[:QB], kf[QB:]
        wf_sc[0, q, :QB] = (ur * kr - um * km).astype(BF16)
        wf_sc[0, q, QB:] = (ur * km + um * kr).astype(BF16)

    with jax.named_scope("wait_wo"):
        wo_copy.wait()
    with jax.named_scope("step0"):
        mem0 = mem0_ref[...].astype(F32)
        h0 = jnp.concatenate([jnp.concatenate([mem0, mem0], axis=0).astype(BF16), xn(0)], axis=0)

        def hook0(it):
            if it in (2, 6, 10, 14):
                warm_block0((it - 2) // 4)
            if it == 18:
                conv_spec(1, 0)
                for piece in MAC_PIECES:
                    conv_mac(1, 0, piece, 2)
            if it == 22:
                conv_inv(0)
        out = attend(lambda g: proj_split(h0, h0, g), RH, make_mask(RH, (0,)), DIST_HALF, hook0)
        finish(0, x_sc[0:SEG, :], y_sc[0], jnp.concatenate([out[0:M], mem0], axis=0), out[M2:], False)

    mask12 = make_mask(R, (0, 1))

    def step(t, first, last):
        if first:
            conv_spec_later = functools.partial(conv_spec, t // NQ + 1, t % NQ)
        x4 = side2(t, op_sc[...])
        un = conv_u(t + 2 * NQ)
        hm = _unpack(h_sc[0:M, :])
        hx2 = _unpack(h_sc[M:, :])
        h48 = jnp.concatenate([hm, hx2], axis=0)
        x1n = pinned(xn(t), pin_tiles(PIN_U if first else PIN_U2, 1, un) + pin_tiles(PIN_X4, X4S, x4))

        def proj(g):
            h80 = jnp.concatenate([hm, x1n(g), hx2], axis=0)
            if g >= NPA + NPB:
                return proj_split(h80, h80, g)
            q, k, v = proj_split(h48, h80, g)
            q1 = pre_sc[t, g] if g < NPA else fill_sc[g - NPA]
            return jnp.concatenate([q[0:M2], _unpack(q1), q[M2:]], axis=0), k, v

        held = {}

        def hook(it):
            if it == SPEC_AT:
                if first:
                    conv_spec_later()
                for piece in MAC_PIECES:
                    conv_mac(t // NQ + 1, t % NQ, piece, NB)
            if it == H:
                held["x"] = x_sc[seg(t), :]
                held["y"] = y_sc[t & 3]
        out = attend(proj, R, mask12, DIST, hook)
        op_sc[...] = out[RH:]
        finish(t, held["x"], held["y"], out[0:M2], out[M2:RH], not last)

    def steps(i, carry):
        for j in range(UNROLL):
            step(1 + i * UNROLL + j, j == 0, j == UNROLL - 1)
        return carry

    def phase(p, carry):
        @pl.when(p == 1)
        def _():
            for cp in in_copies(2):
                cp.wait()

        @pl.when(p >= 2)
        def _():
            out_copy((p - 2) * PH, PH).start()

        with jax.named_scope("steps"):
            jax.lax.fori_loop(p * PHI, (p + 1) * PHI, steps, 0)
        return carry

    for cp in in_copies(1):
        cp.wait()
    jax.lax.fori_loop(0, NPH, phase, 0)
    out_copy((NPH - 2) * PH, NSEG - 2 - (NPH - 2) * PH).start()

    with jax.named_scope("step_last"):
        x4 = side2(NSEG, op_sc[...])
        hm = _unpack(h_sc[0:M, :])
        hx = pinned(_unpack(h_sc[M:, :]), pin_tiles(PIN_X4, 0, x4))
        out = attend(lambda g: proj_split(hx(g), jnp.concatenate([hm, hx(g)], axis=0), g),
                     SEG, make_mask(RH, (1,), M2), DIST_LAST)
        side2(NSEG + 1, out)
    out_copy(NSEG - 2, 2).start()
    pltpu.make_async_copy(out_sc, o_hbm, sem_out).wait()


def pallas_interleave_layers__memory_aug_recurrent_mem_tr__ssm_conv_h3__prompt_kernel(
    A_x, A_mem0, A_Wq, A_Wk, A_Wv, A_Wo, A_seg_len,
    B_q, B_k, B_v, B_shift_k, B_ssm_k, B_ssm_D,
):
    del B_q
    seg = int(A_seg_len) if isinstance(A_seg_len, (int, np.integer)) else CB // NQ
    return _run(A_x, A_mem0, A_Wq, A_Wk, A_Wv, A_Wo, B_k, B_v, B_shift_k, B_ssm_k, B_ssm_D, SEG=seg)


@functools.partial(jax.jit, static_argnames=("SEG",))
def _run(A_x, A_mem0, A_Wq, A_Wk, A_Wv, A_Wo, B_k, B_v, B_shift_k, B_ssm_k, B_ssm_D, *, SEG):
    B, S, DM = A_x.shape
    assert B == 1
    H, DH = A_Wq.shape[1], A_Wq.shape[2]
    M = A_mem0.shape[1]
    KS = B_shift_k.shape[1]
    R = 2 * (M + SEG)
    NSEG = S // SEG
    NRB = (NSEG - 1) // RB
    NB = S // CB
    QB = CB // NQ
    NCH = 3 * H // HG
    fwd, inv = _dft_constants()

    kern = functools.partial(_kernel, S=S, DM=DM, H=H, DH=DH, M=M, SEG=SEG)
    any_spec = pl.BlockSpec(memory_space=pl.ANY)
    out = pl.pallas_call(
        kern,
        out_shape=jax.ShapeDtypeStruct((S, DM), A_x.dtype),
        in_specs=[any_spec] * 13,
        out_specs=any_spec,
        scratch_shapes=[
            pltpu.VMEM((NB + 2, NQ, QB // 8, DM // 128, 4, 8, 128), F32),
            pltpu.VMEM((NQ, 2 * QB, DM), F32),
            pltpu.VMEM((2, NQ, 2 * QB, DM), BF16),
            pltpu.VMEM((4, SEG, DM), F32),
            pltpu.VMEM((4, SEG, DM), F32),
            pltpu.VMEM((S, DM), BF16),
            pltpu.VMEM((SEG, DM), F32),
            pltpu.VMEM((NSEG, NPA, SEG // 2, DH), U32),
            pltpu.VMEM((NPB, SEG // 2, DH), U32),
            pltpu.VMEM((NSEG, SEG // 2, -(-DM // 256) * 256), U32),
            pltpu.VMEM((NCH - NRB + 2, HG, DM // 2, DH), U32),
            pltpu.VMEM((NRB - 1, HG, DM // 2, DH), U32),
            pltpu.VMEM((H * DH, DM), BF16),
            pltpu.VMEM((R // 2, H * DH), U32),
            pltpu.VMEM((S, DM), BF16),
            pltpu.VMEM((S, DM), BF16),
            pltpu.VMEM((DM, S), BF16),
            pltpu.VMEM((NCH, DM // 2, 2 * HG, DH), BF16),
            pltpu.VMEM((S, DM), A_x.dtype),
            pltpu.VMEM(fwd.shape, BF16),
            pltpu.VMEM(inv.shape, BF16),
            pltpu.VMEM((S + KPAD, DM), BF16),
            pltpu.VMEM((RB * SEG // 2, DM), U32),
            pltpu.VMEM((M + SEG // 2, DM), U32),
            pltpu.VMEM((M, DM), BF16),
            pltpu.VMEM((KS, DM), BF16),
            pltpu.VMEM((DM,), BF16),
            pltpu.SMEM((1,), jnp.int32),
            pltpu.SemaphoreType.DMA(((NSEG - 1) // RB,)),
            pltpu.SemaphoreType.DMA((3,)),
            pltpu.SemaphoreType.DMA((NCH + 1,)),
            pltpu.SemaphoreType.DMA(()),
        ],
        compiler_params=pltpu.CompilerParams(vmem_limit_bytes=120 * 1024 * 1024),
    )(
        A_x.reshape(S, DM), A_mem0.reshape(M, DM), A_Wq, A_Wk, A_Wv,
        A_Wo.reshape(H * DH, DM), B_k.reshape(S, DM), B_v.reshape(S, DM),
        B_shift_k.T, B_ssm_k, B_ssm_D,
        jnp.asarray(fwd, BF16), jnp.asarray(inv, BF16),
    )
    return out.reshape(B, S, DM)
```

```python
import functools

import numpy as np
import jax
import jax.numpy as jnp
import jax.experimental.pallas as pl
import jax.experimental.pallas.tpu as pltpu

F32 = jnp.float32
BF16 = jnp.bfloat16
U32 = jnp.uint32

CB = 128
NQ = 4
KPAD = 16
HG = 8
NPA = 16
NPB = 12
RB = 9
PRO_PW, PRO_X0, PRO_XS, PRO_R0, PRO_RS = 24, 11, 4, 2, 2
UNROLL = 3
PHI = 3
PIN_U2, X4S = 1, 0
SPEC_AT, PIN_U, PIN_X4 = 7, 1, 16
DIST, DIST_HALF, DIST_LAST = (1, 2), (1, 3), (2, 3)


def _dft_constants():
    qb = CB // NQ
    n = np.arange(CB, dtype=np.float64)
    fwd = np.zeros((NQ, 2 * qb, CB))
    for q in range(NQ):
        f = q * qb + np.concatenate([np.arange(0, qb, 2), np.arange(1, qb, 2)])
        ang = (np.pi * (2.0 * f + 1.0) / (2 * CB))[:, None] * n[None, :]
        fwd[q, :qb] = np.cos(ang)
        fwd[q, qb:] = -np.sin(ang)
    inv = fwd.reshape(2 * CB, CB).T / CB
    return fwd.astype(np.float32), inv.reshape(NQ, CB // NQ, 2 * CB).astype(np.float32)


def _ln(x, eps=1e-5):
    d = x.shape[-1]
    m = jnp.sum(x, axis=-1, keepdims=True) * (1.0 / d)
    xc = x - m
    v = jnp.sum(xc * xc, axis=-1, keepdims=True) * (1.0 / d)
    return xc * jax.lax.rsqrt(v + eps)


def _dot(a, b):
    return jnp.dot(a, b, preferred_element_type=F32)


def _dot_nt(a, b):
    return jax.lax.dot_general(a, b, (((1,), (1,)), ((), ())), preferred_element_type=F32)


def _pack(x):
    return pltpu.bitcast(x.astype(BF16), U32)


def _unpack(x):
    return pltpu.bitcast(x, BF16)


def _in_order(actions):
    def body(i, c):
        for j, act in enumerate(actions):
            pl.when(i == j)(act)
        return c
    jax.lax.fori_loop(0, len(actions), body, 0)


def _kernel(x_hbm, mem0_hbm, wq_hbm, wk_hbm, wv_hbm, wo_hbm, k_hbm, v_hbm,
            sh_hbm, sk_hbm, sd_hbm, fwd_hbm, inv_hbm, o_hbm,
            sp_sc, kr_sc, wf_sc, x2_sc, y_sc, u_sc, op_sc, pre_sc, fill_sc, xn_sc, wa_sc, wb_sc, wo_sc, o_sc,
            x_sc, v_sc, sk_sc, st_sc, out_sc, fwd_ref, inv_ref,
            k_sc, hp_sc, h_sc, mem0_ref, sh_ref, sd_ref,
            never_sm, sem_x, sem_in, sem_w, sem_out,
            *, S, DM, H, DH, M, SEG):
    NSEG = S // SEG
    M2 = 2 * M
    S2 = SEG // 2
    R = M2 + 2 * SEG
    RH = M2 + SEG
    NB = S // CB
    QB = CB // NQ
    HB = QB // 2
    NT = DM // 128
    PH = PHI * UNROLL
    NRB = (NSEG - 1) // RB
    NPH = (NSEG - 1) // PH
    NG = H // HG
    NCH = 3 * NG
    NPASS = NPA // HG
    DH2 = DM // 2
    KS = sh_ref.shape[0]
    assert QB == SEG and NRB * RB == NSEG - 1 and NPH * PH == NSEG - 1 and NPASS == 2 and 2 * NRB >= NCH + 1

    mem0_copy = pltpu.make_async_copy(mem0_hbm, mem0_ref, sem_x.at[0])
    small = [pltpu.make_async_copy(s, d, sem_in.at[0]) for s, d in [
        (sh_hbm, sh_ref), (sd_hbm, sd_ref), (fwd_hbm, fwd_ref), (inv_hbm, inv_ref)]]

    def x_copy(b):
        if isinstance(b, int) and b == 0:
            rows = pl.ds(0, (RB + 1) * SEG)
        else:
            rows = pl.ds(pl.multiple_of((b * RB + 1) * SEG, SEG), RB * SEG)
        return pltpu.make_async_copy(x_hbm.at[rows], x_sc.at[rows], sem_x.at[b])

    kb = (0, (2 * NQ + 1) * SEG, (2 * NQ + PH + 1) * SEG, S)
    sb = (0, 2 * CB, ((PH + 1) // NQ + 2) * CB, S)

    def in_copies(part):
        def rng(b):
            return pl.ds(b[part], b[part + 1] - b[part])
        sem = sem_in.at[part]
        return [
            pltpu.make_async_copy(k_hbm.at[rng(kb)],
                                  k_sc.at[pl.ds(KPAD + kb[part], kb[part + 1] - kb[part])], sem),
            pltpu.make_async_copy(v_hbm.at[rng(kb)], v_sc.at[rng(kb)], sem),
            pltpu.make_async_copy(sk_hbm.at[:, rng(sb)], sk_sc.at[:, rng(sb)], sem),
        ]

    def w_copies(ci, dst=None):
        src = (wq_hbm, wk_hbm, wv_hbm)[ci // NG]
        dst = ci if dst is None else dst
        return [pltpu.make_async_copy(src.at[pl.ds(hf * DH2, DH2), pl.ds((ci % NG) * HG, HG), :],
                                      st_sc.at[dst, :, pl.ds(hf * HG, HG), :], sem_w.at[dst])
                for hf in range(2)]

    wo_copy = pltpu.make_async_copy(wo_hbm, wo_sc, sem_w.at[NCH])

    def out_copy(lo, n):
        rows = pl.ds(lo * SEG if isinstance(lo, int) else pl.multiple_of(lo * SEG, SEG), n * SEG)
        return pltpu.make_async_copy(out_sc.at[rows], o_hbm.at[rows], sem_out)

    def start_all(cps):
        def act():
            for cp in cps:
                cp.start()
        return act

    order = [[mem0_copy, x_copy(0)], w_copies(0), [x_copy(1)], [x_copy(2)]]
    for ci in range(1, NCH):
        order.append(w_copies(ci) + ([x_copy(ci + 2)] if ci + 2 < NRB else []))
        if ci == NRB - 2:
            order.append(small + in_copies(0))
    order += [[wo_copy], in_copies(1), in_copies(2)]
    for i in range(0, len(order), 5):
        _in_order([start_all(cps) for cps in order[i:i + 5]])

    never_sm[0] = 0
    k_sc[0:KPAD, :] = jnp.zeros((KPAD, DM), BF16)
    sp_sc[NB + 1] = jnp.zeros(sp_sc.shape[1:], F32)
    op_sc[...] = jnp.zeros(op_sc.shape, F32)
    x2_sc[...] = jnp.zeros(x2_sc.shape, F32)
    y_sc[...] = jnp.zeros(y_sc.shape, F32)
    mem0_copy.wait()
    x_copy(0).wait()
    for sg in range(RB + 1):
        xn_sc[sg, :, 0:DM] = _pack(_ln(x_sc[sg * SEG:(sg + 1) * SEG, :].astype(F32)))

    def clip(i, hi):
        return min(max(i, 0), hi) if isinstance(i, int) else jnp.clip(i, 0, hi)

    def scaled(i, m):
        return i * m if isinstance(i, int) else pl.multiple_of(i * m, m)

    def seg(i):
        return pl.ds(scaled(clip(i, NSEG - 1), SEG), SEG)

    def conv_u(s, ln=slice(None)):
        r0 = scaled(clip(s, NSEG - 1), SEG)
        sh = sh_ref[:, ln].astype(F32)
        kk = k_sc[pl.ds(r0, KPAD + SEG), ln].astype(F32)
        ks = kk[KPAD:] * sh[0:1]
        for j in range(1, KS):
            ks = ks + pltpu.roll(kk, j, 0)[KPAD:] * sh[j:j + 1]
        u = (ks * v_sc[pl.ds(r0, SEG), ln].astype(F32)).astype(BF16)
        u_sc[pl.ds(r0, SEG), ln] = u
        return u

    def conv_fwd(c, q):
        t0 = scaled(clip(c, NB - 1), CB)
        f = fwd_ref[q]
        uf = _dot(f, u_sc[pl.ds(t0, CB), :])
        kf = _dot_nt(f, sk_sc[:, pl.ds(t0, CB)])
        return uf, kf

    def put_spec(cs, q, which, val):
        for rb in range(QB // 8):
            for n in range(NT):
                ln = slice(n * 128, (n + 1) * 128)
                sp_sc[cs, q, rb, n, which] = val[rb * 8:rb * 8 + 8, ln]
                sp_sc[cs, q, rb, n, which + 1] = val[QB + rb * 8:QB + rb * 8 + 8, ln]

    def conv_spec(c, q):
        uf, kf = conv_fwd(c, q)
        cs = clip(c, NB)
        put_spec(cs, q, 0, uf)
        pk = kr_sc[q]
        kr_sc[q] = kf
        kp = jnp.concatenate([
            kf[0:HB] - pk[QB:QB + HB],
            kf[HB:QB] + pk[QB + HB:],
            kf[QB:QB + HB] + pk[0:HB],
            kf[QB + HB:] - pk[HB:QB]], axis=0)
        put_spec(cs, q, 2, kp)

    MAC_PIECES = [(rb, n) for rb in range(QB // 16) for n in range(NT)]

    def conv_mac(c, q, piece, nterms):
        rb2, n = piece
        cs = clip(c, NB)
        acc = []
        for rb in (2 * rb2, 2 * rb2 + 1):
            ar = None
            ai = None
            for j in range(nterms):
                if isinstance(cs, int):
                    uj, kj = j, cs - j
                else:
                    uj = jnp.minimum(j, cs)
                    kj = jnp.where(cs - j >= 0, cs - j, NB + 1)
                ur = sp_sc[uj, q, rb, n, 0]
                um = sp_sc[uj, q, rb, n, 1]
                kr = sp_sc[kj, q, rb, n, 2]
                km = sp_sc[kj, q, rb, n, 3]
                tr = ur * kr - um * km
                ti = ur * km + um * kr
                ar = tr if ar is None else ar + tr
                ai = ti if ai is None else ai + ti
            acc.append((ar, ai))
        ln = slice(n * 128, (n + 1) * 128)
        w = jnp.concatenate([acc[0][0], acc[1][0], acc[0][1], acc[1][1]], axis=0).astype(BF16)
        wf_sc[c & 1, q, rb2 * 16:rb2 * 16 + 16, ln] = w[0:16]
        wf_sc[c & 1, q, QB + rb2 * 16:QB + rb2 * 16 + 16, ln] = w[16:]

    def conv_inv(s):
        w = wf_sc[(s // NQ) & 1].reshape(2 * CB, DM)
        yc = _dot(inv_ref[s % NQ], w)
        sd = sd_ref[...].astype(F32).reshape(1, DM)
        y_sc[s & 3] = yc + u_sc[seg(s), :].astype(F32) * sd

    scale = DH ** -0.5
    cexp = scale * float(np.log2(np.e))

    def make_mask(n, x_layers, q0=0):
        qi = jax.lax.broadcasted_iota(jnp.int32, (n - q0, n), 0) + q0
        ki = jax.lax.broadcasted_iota(jnp.int32, (n - q0, n), 1)

        def layer(i):
            xl = jnp.where(i < M2 + SEG, x_layers[0], x_layers[-1])
            return jnp.where(i < M, 0, jnp.where(i < M2, 1, xl))
        same = layer(qi) == layer(ki)
        ok = same & ((qi < M2) | (ki < M2) | (qi >= ki))
        fill = jnp.where(same, -1e9 / scale, -jnp.inf).astype(F32)
        return ok, fill

    def probs(q, k, mask):
        ok, fill = mask
        s = _dot_nt(q, k)
        s = jnp.where(ok, s, fill)
        m = jnp.max(s, axis=-1, keepdims=True)
        p = jnp.exp2((s - m) * cexp)
        l = jnp.sum(p, axis=-1, keepdims=True)
        r = pl.reciprocal(l, approx=True)
        r = r * (2.0 - l * r)
        return (p * r).astype(BF16)

    def w_slot(ci):
        return (wb_sc, ci) if 1 <= ci < NRB - 1 else (wa_sc, max(ci - (NRB - 2), 0))

    def w_head(g, mats):
        slots = [w_slot(mi * NG + g // HG) for mi in mats]
        return _unpack(jnp.concatenate([ref[i, g % HG] for ref, i in slots], axis=1))

    def proj_split(hq, hkv, g):
        q = _dot(hq, w_head(g, (0,))).astype(BF16)
        kv = _dot(hkv, w_head(g, (1, 2))).astype(BF16)
        return q, kv[:, :DH], kv[:, DH:]

    def xn(s):
        return _unpack(xn_sc[clip(s, NSEG - 1), :, 0:DM])

    def out_proj(n, g0, g1, j):
        return _dot(_unpack(o_sc[0:n // 2, g0 * DH:g1 * DH]),
                    wo_sc[g0 * DH:g1 * DH, j * 128:(j + 1) * 128])

    def attend(proj, n, mask, dist, hook=None):
        D1, D2 = dist
        HA = H - D1 - D2 - 1
        NE = min(D1 + D2, NT - 1)
        qkvs = {}
        ps = {}
        outs = {}
        for it in range(H + D1 + D2):
            if it < H:
                qkvs[it] = proj(it)
            g = it - D1
            if 0 <= g < H:
                ps[g] = probs(qkvs[g][0], qkvs[g][1], mask)
            g = it - D1 - D2
            if 0 <= g < H:
                o = _dot(ps.pop(g), qkvs.pop(g)[2])
                o_sc[0:n // 2, g * DH:(g + 1) * DH] = _pack(o)
            if hook is not None:
                hook(it)
            j = it - (H - 1)
            if 0 <= j < NE:
                outs[j] = out_proj(n, 0, HA, j)
        for j in range(NE, NT):
            outs[j] = out_proj(n, 0, H, j)
        for j in range(NE):
            outs[j] = out_proj(n, HA, H, j) + outs[j]
        return jnp.concatenate([outs[j] for j in range(NT)], axis=1)

    def side2(t, a2):
        x3 = x2_sc[(t - 2) & 3] + a2
        x4 = x3 + _ln(x3) * y_sc[(t - 2) & 3]
        x4 = x4.astype(out_sc.dtype)
        out_sc[seg(t - 2), :] = x4
        return x4

    def finish(t, xr, yt, mem, a1, spec):
        if spec:
            conv_spec((t + 1) // NQ + 1, (t + 1) % NQ)
        xq = xn(t + 1)
        for g in range(NPA, NPA + NPB):
            fill_sc[g - NPA] = _pack(_dot(xq, w_head(g, (0,))))
        conv_inv(t + 1)
        x1 = xr.astype(F32) + a1
        x2 = x1 + _ln(x1) * yt
        h_sc[0:M, :] = _pack(mem)
        h_sc[M:, :] = _pack(_ln(x2))
        x2_sc[t & 3] = x2

    def pinned(rows, pins):
        never = never_sm[0] > 0
        hs = {0: rows}
        r = _pack(rows)
        tiles = [r[:, n * 128:(n + 1) * 128] for n in range(NT)]
        for g, n, d in sorted(pins, key=lambda p: p[0]):
            tiles[n] = jnp.where(never, d, tiles[n])
            hs[g] = _unpack(jnp.concatenate(tiles, axis=1))
        return lambda g: hs[max(k for k in hs if k <= g)]

    def pin_tiles(g0, stride, val):
        v = _pack(val)
        return [(g0 + n * stride, n, v[:, n * 128:(n + 1) * 128]) for n in range(NT)]

    def wait_chunk(ci):
        for cp in w_copies(0, ci):
            cp.wait()

    def relayout(ci, dst, slot, b):
        d0 = scaled(b, 16)
        r0 = scaled(b, 8)
        xw = pltpu.bitcast(st_sc[ci, pl.ds(d0, 16)], U32).reshape(8, 2, HG, DH)
        a = xw[:, 0]
        bb = xw[:, 1]
        lo = jnp.swapaxes((a & U32(0xFFFF)) | (bb << 16), 0, 1)
        hi = jnp.swapaxes((a >> 16) | (bb & U32(0xFFFF0000)), 0, 1)
        for j in range(HG):
            rows = pl.ds(r0 + (2 * j // HG) * (DH2 // 2), 8)
            dst[slot, 2 * j % HG, rows, :] = lo[j]
            dst[slot, 2 * j % HG + 1, rows, :] = hi[j]

    NBLK = DH2 // 16
    with jax.named_scope("wait_w"):
        wait_chunk(0)

    def relayout0(b, c):
        relayout(0, wa_sc, 0, b)
        return c
    with jax.named_scope("relayout"):
        jax.lax.fori_loop(0, NBLK, relayout0, 0, unroll=2)

    def pro_stage(ps_, b):
        n = ps_ * NRB + b
        with jax.named_scope("wait_w"):
            if ps_ == 0:
                @pl.when(b + 1 < NRB)
                def _():
                    x_copy(b + 1).wait()

            @pl.when((n >= 2) & (n <= NCH))
            def _():
                wait_chunk(n - 1)
        cr = jnp.clip(n - 1, 0, NCH - 1)
        dst, slot = (wb_sc, cr) if ps_ == 0 else (wa_sc, cr - (NRB - 2))
        src, si = w_slot(ps_)
        bl = jnp.minimum(b + 1, NRB - 1)
        PW = PRO_PW
        npc = RB * S2 // PW
        assert npc * PW == RB * S2 and PRO_R0 + (NBLK - 1) * PRO_RS < HG * npc
        assert PRO_X0 + (max(RB, 2 * NT) - 1) * PRO_XS < HG * npc and 2 * NRB > 2 * NQ

        def body(i, c):
            s0 = b * RB + 1
            for sg in range(RB):
                hp_sc[sg * S2:(sg + 1) * S2, :] = xn_sc[s0 + sg, :, 0:DM]
            for j in range(HG):
                w = _unpack(src[si, j])
                for pi in range(npc):
                    pos = j * npc + pi
                    hx = hp_sc[pi * PW:(pi + 1) * PW, :]
                    k, rem = divmod(pos - PRO_X0, PRO_XS)
                    if ps_ == 0 and rem == 0 and 0 <= k < RB:
                        sn = bl * RB + 1 + k
                        xv = _pack(_ln(x_sc[seg(sn), :].astype(F32)))
                        xn_sc[sn, :, 0:DM] = xv
                        hx = jnp.concatenate([hx[:-S2], jnp.where(never_sm[0] > 0, xv, hx[-S2:])], axis=0)
                    if ps_ == 1 and rem == 0 and 0 <= k < 2 * NT:
                        conv_u(jnp.minimum(2 * b + k // NT, 2 * NQ),
                               slice((k % NT) * 128, (k % NT + 1) * 128))
                    bb, rem = divmod(pos - PRO_R0, PRO_RS)
                    if rem == 0 and 0 <= bb < NBLK:
                        relayout(cr, dst, slot, bb)
                    r = _pack(_dot(_unpack(hx), w))
                    for a in range(0, PW, 8):
                        sg, off = divmod(pi * PW + a, S2)
                        pre_sc[s0 + sg, ps_ * HG + j, off:off + 8, :] = r[a:a + 8]
            return c
        with jax.named_scope("fused"):
            jax.lax.fori_loop(0, never_sm[0] + 1, body, 0)

    for ps_ in range(NPASS):
        if ps_ == 1:
            with jax.named_scope("wait_in0"):
                for cp in small + in_copies(0):
                    cp.wait()

        def blk(b, c, ps_=ps_):
            pro_stage(ps_, b)
            return c
        jax.lax.fori_loop(0, NRB, blk, 0)

    def warm_block0(q):
        uf, kf = conv_fwd(0, q)
        put_spec(0, q, 0, uf)
        put_spec(0, q, 2, kf)
        kr_sc[q] = kf
        ur, um, kr, km = uf[:QB], uf[QB:], kf[:QB], kf[QB:]
        wf_sc[0, q, :QB] = (ur * kr - um * km).astype(BF16)
        wf_sc[0, q, QB:] = (ur * km + um * kr).astype(BF16)

    with jax.named_scope("warm"):
        for q in range(NQ):
            warm_block0(q)
    with jax.named_scope("wait_wo"):
        wo_copy.wait()
    with jax.named_scope("step0"):
        mem0 = mem0_ref[...].astype(F32)
        h0 = jnp.concatenate([jnp.concatenate([mem0, mem0], axis=0).astype(BF16), xn(0)], axis=0)

        def hook0(it):
            if it == 6:
                conv_spec(1, 0)
                for piece in MAC_PIECES:
                    conv_mac(1, 0, piece, 2)
            if it == 14:
                conv_inv(0)
        out = attend(lambda g: proj_split(h0, h0, g), RH, make_mask(RH, (0,)), DIST_HALF, hook0)
        finish(0, x_sc[0:SEG, :], y_sc[0], jnp.concatenate([out[0:M], mem0], axis=0), out[M2:], False)

    mask12 = make_mask(R, (0, 1))

    def step(t, first, last):
        if first:
            conv_spec_later = functools.partial(conv_spec, t // NQ + 1, t % NQ)
        x4 = side2(t, op_sc[...])
        un = conv_u(t + 2 * NQ)
        hm = _unpack(h_sc[0:M, :])
        hx2 = _unpack(h_sc[M:, :])
        h48 = jnp.concatenate([hm, hx2], axis=0)
        x1n = pinned(xn(t), pin_tiles(PIN_U if first else PIN_U2, 1, un) + pin_tiles(PIN_X4, X4S, x4))

        def proj(g):
            h80 = jnp.concatenate([hm, x1n(g), hx2], axis=0)
            if g >= NPA + NPB:
                return proj_split(h80, h80, g)
            q, k, v = proj_split(h48, h80, g)
            q1 = pre_sc[t, g] if g < NPA else fill_sc[g - NPA]
            return jnp.concatenate([q[0:M2], _unpack(q1), q[M2:]], axis=0), k, v

        held = {}

        def hook(it):
            if it == SPEC_AT:
                if first:
                    conv_spec_later()
                for piece in MAC_PIECES:
                    conv_mac(t // NQ + 1, t % NQ, piece, NB)
            if it == H:
                held["x"] = x_sc[seg(t), :]
                held["y"] = y_sc[t & 3]
        out = attend(proj, R, mask12, DIST, hook)
        op_sc[...] = out[RH:]
        finish(t, held["x"], held["y"], out[0:M2], out[M2:RH], not last)

    def steps(i, carry):
        for j in range(UNROLL):
            step(1 + i * UNROLL + j, j == 0, j == UNROLL - 1)
        return carry

    def phase(p, carry):
        @pl.when(p == 1)
        def _():
            for cp in in_copies(2):
                cp.wait()

        @pl.when(p >= 2)
        def _():
            out_copy((p - 2) * PH, PH).start()

        with jax.named_scope("steps"):
            jax.lax.fori_loop(p * PHI, (p + 1) * PHI, steps, 0)
        return carry

    for cp in in_copies(1):
        cp.wait()
    jax.lax.fori_loop(0, NPH, phase, 0)
    out_copy((NPH - 2) * PH, NSEG - 2 - (NPH - 2) * PH).start()

    with jax.named_scope("step_last"):
        x4 = side2(NSEG, op_sc[...])
        hm = _unpack(h_sc[0:M, :])
        hx = pinned(_unpack(h_sc[M:, :]), pin_tiles(PIN_X4, 0, x4))
        out = attend(lambda g: proj_split(hx(g), jnp.concatenate([hm, hx(g)], axis=0), g),
                     SEG, make_mask(RH, (1,), M2), DIST_LAST)
        side2(NSEG + 1, out)
    out_copy(NSEG - 2, 2).start()
    pltpu.make_async_copy(out_sc, o_hbm, sem_out).wait()


def pallas_interleave_layers__memory_aug_recurrent_mem_tr__ssm_conv_h3__prompt_kernel(
    A_x, A_mem0, A_Wq, A_Wk, A_Wv, A_Wo, A_seg_len,
    B_q, B_k, B_v, B_shift_k, B_ssm_k, B_ssm_D,
):
    del B_q
    seg = int(A_seg_len) if isinstance(A_seg_len, (int, np.integer)) else CB // NQ
    return _run(A_x, A_mem0, A_Wq, A_Wk, A_Wv, A_Wo, B_k, B_v, B_shift_k, B_ssm_k, B_ssm_D, SEG=seg)


@functools.partial(jax.jit, static_argnames=("SEG",))
def _run(A_x, A_mem0, A_Wq, A_Wk, A_Wv, A_Wo, B_k, B_v, B_shift_k, B_ssm_k, B_ssm_D, *, SEG):
    B, S, DM = A_x.shape
    assert B == 1
    H, DH = A_Wq.shape[1], A_Wq.shape[2]
    M = A_mem0.shape[1]
    KS = B_shift_k.shape[1]
    R = 2 * (M + SEG)
    NSEG = S // SEG
    NRB = (NSEG - 1) // RB
    NB = S // CB
    QB = CB // NQ
    NCH = 3 * H // HG
    fwd, inv = _dft_constants()

    kern = functools.partial(_kernel, S=S, DM=DM, H=H, DH=DH, M=M, SEG=SEG)
    any_spec = pl.BlockSpec(memory_space=pl.ANY)
    out = pl.pallas_call(
        kern,
        out_shape=jax.ShapeDtypeStruct((S, DM), A_x.dtype),
        in_specs=[any_spec] * 13,
        out_specs=any_spec,
        scratch_shapes=[
            pltpu.VMEM((NB + 2, NQ, QB // 8, DM // 128, 4, 8, 128), F32),
            pltpu.VMEM((NQ, 2 * QB, DM), F32),
            pltpu.VMEM((2, NQ, 2 * QB, DM), BF16),
            pltpu.VMEM((4, SEG, DM), F32),
            pltpu.VMEM((4, SEG, DM), F32),
            pltpu.VMEM((S, DM), BF16),
            pltpu.VMEM((SEG, DM), F32),
            pltpu.VMEM((NSEG, NPA, SEG // 2, DH), U32),
            pltpu.VMEM((NPB, SEG // 2, DH), U32),
            pltpu.VMEM((NSEG, SEG // 2, -(-DM // 256) * 256), U32),
            pltpu.VMEM((NCH - NRB + 2, HG, DM // 2, DH), U32),
            pltpu.VMEM((NRB - 1, HG, DM // 2, DH), U32),
            pltpu.VMEM((H * DH, DM), BF16),
            pltpu.VMEM((R // 2, H * DH), U32),
            pltpu.VMEM((S, DM), BF16),
            pltpu.VMEM((S, DM), BF16),
            pltpu.VMEM((DM, S), BF16),
            pltpu.VMEM((NCH, DM // 2, 2 * HG, DH), BF16),
            pltpu.VMEM((S, DM), A_x.dtype),
            pltpu.VMEM(fwd.shape, BF16),
            pltpu.VMEM(inv.shape, BF16),
            pltpu.VMEM((S + KPAD, DM), BF16),
            pltpu.VMEM((RB * SEG // 2, DM), U32),
            pltpu.VMEM((M + SEG // 2, DM), U32),
            pltpu.VMEM((M, DM), BF16),
            pltpu.VMEM((KS, DM), BF16),
            pltpu.VMEM((DM,), BF16),
            pltpu.SMEM((1,), jnp.int32),
            pltpu.SemaphoreType.DMA(((NSEG - 1) // RB,)),
            pltpu.SemaphoreType.DMA((3,)),
            pltpu.SemaphoreType.DMA((NCH + 1,)),
            pltpu.SemaphoreType.DMA(()),
        ],
        compiler_params=pltpu.CompilerParams(vmem_limit_bytes=120 * 1024 * 1024),
    )(
        A_x.reshape(S, DM), A_mem0.reshape(M, DM), A_Wq, A_Wk, A_Wv,
        A_Wo.reshape(H * DH, DM), B_k.reshape(S, DM), B_v.reshape(S, DM),
        B_shift_k.T, B_ssm_k, B_ssm_D,
        jnp.asarray(fwd, BF16), jnp.asarray(inv, BF16),
    )
    return out.reshape(B, S, DM)
```

```python
import functools

import numpy as np
import jax
import jax.numpy as jnp
import jax.experimental.pallas as pl
import jax.experimental.pallas.tpu as pltpu

F32 = jnp.float32
BF16 = jnp.bfloat16
U32 = jnp.uint32

CB = 128
NQ = 4
KPAD = 16
HG = 8
NPA = 16
NPB = 12
RB = 9
PRO_PW, PRO_X0, PRO_XS, PRO_R0, PRO_RS = 24, 11, 4, 2, 2
UNROLL = 3
PHI = 3
PIN_U2, X4S = 1, 0
SPEC_AT, PIN_U, PIN_X4 = 7, 1, 16
DIST, DIST_HALF, DIST_LAST = (1, 2), (1, 3), (2, 3)


def _dft_constants():
    qb = CB // NQ
    n = np.arange(CB, dtype=np.float64)
    fwd = np.zeros((NQ, 2 * qb, CB))
    for q in range(NQ):
        f = q * qb + np.concatenate([np.arange(0, qb, 2), np.arange(1, qb, 2)])
        ang = (np.pi * (2.0 * f + 1.0) / (2 * CB))[:, None] * n[None, :]
        fwd[q, :qb] = np.cos(ang)
        fwd[q, qb:] = -np.sin(ang)
    inv = fwd.reshape(2 * CB, CB).T / CB
    return fwd.astype(np.float32), inv.reshape(NQ, CB // NQ, 2 * CB).astype(np.float32)


def _ln(x, eps=1e-5):
    d = x.shape[-1]
    m = jnp.sum(x, axis=-1, keepdims=True) * (1.0 / d)
    xc = x - m
    v = jnp.sum(xc * xc, axis=-1, keepdims=True) * (1.0 / d)
    return xc * jax.lax.rsqrt(v + eps)


def _dot(a, b):
    return jnp.dot(a, b, preferred_element_type=F32)


def _dot_nt(a, b):
    return jax.lax.dot_general(a, b, (((1,), (1,)), ((), ())), preferred_element_type=F32)


def _pack(x):
    return pltpu.bitcast(x.astype(BF16), U32)


def _unpack(x):
    return pltpu.bitcast(x, BF16)


def _in_order(actions):
    def body(i, c):
        for j, act in enumerate(actions):
            pl.when(i == j)(act)
        return c
    jax.lax.fori_loop(0, len(actions), body, 0)


def _kernel(x_hbm, mem0_hbm, wq_hbm, wk_hbm, wv_hbm, wo_hbm, k_hbm, v_hbm,
            sh_hbm, sk_hbm, sd_hbm, fwd_hbm, inv_hbm, o_hbm,
            sp_sc, kr_sc, wf_sc, x2_sc, y_sc, u_sc, op_sc, pre_sc, fill_sc, xn_sc, wa_sc, wb_sc, wo_sc, o_sc,
            x_sc, v_sc, sk_sc, st_sc, out_sc, fwd_ref, inv_ref,
            k_sc, hp_sc, h_sc, mem0_ref, sh_ref, sd_ref,
            never_sm, sem_x, sem_in, sem_w, sem_out,
            *, S, DM, H, DH, M, SEG):
    NSEG = S // SEG
    M2 = 2 * M
    S2 = SEG // 2
    R = M2 + 2 * SEG
    RH = M2 + SEG
    NB = S // CB
    QB = CB // NQ
    HB = QB // 2
    NT = DM // 128
    PH = PHI * UNROLL
    NRB = (NSEG - 1) // RB
    NPH = (NSEG - 1) // PH
    NG = H // HG
    NCH = 3 * NG
    NPASS = NPA // HG
    DH2 = DM // 2
    KS = sh_ref.shape[0]
    LN = pl.ds(0, DM)
    assert QB == SEG and NRB * RB == NSEG - 1 and NPH * PH == NSEG - 1 and NPASS == 2 and 2 * NRB >= NCH + 1

    mem0_copy = pltpu.make_async_copy(mem0_hbm, mem0_ref, sem_x.at[0])
    small = [pltpu.make_async_copy(s, d, sem_in.at[0]) for s, d in [
        (sh_hbm, sh_ref), (sd_hbm, sd_ref), (fwd_hbm, fwd_ref), (inv_hbm, inv_ref)]]

    def x_copy(b):
        if isinstance(b, int) and b == 0:
            rows = pl.ds(0, (RB + 1) * SEG)
        else:
            rows = pl.ds(pl.multiple_of((b * RB + 1) * SEG, SEG), RB * SEG)
        return pltpu.make_async_copy(x_hbm.at[rows], x_sc.at[rows, LN], sem_x.at[b])

    kb = (0, (2 * NQ + 1) * SEG, (2 * NQ + PH + 1) * SEG, S)
    sb = (0, 2, (PH + 1) // NQ + 2, NB)

    def in_copies(part):
        def rng(b):
            return pl.ds(b[part], b[part + 1] - b[part])
        sem = sem_in.at[part]
        return [
            pltpu.make_async_copy(k_hbm.at[rng(kb)],
                                  k_sc.at[pl.ds(KPAD + kb[part], kb[part + 1] - kb[part]), LN], sem),
            pltpu.make_async_copy(v_hbm.at[rng(kb)], v_sc.at[rng(kb), LN], sem),
        ] + [pltpu.make_async_copy(sk_hbm.at[:, pl.ds(c * CB, CB)], sk_sc.at[c], sem)
             for c in range(sb[part], sb[part + 1])]

    def w_copies(ci, dst=None):
        src = (wq_hbm, wk_hbm, wv_hbm)[ci // NG]
        dst = ci if dst is None else dst
        return [pltpu.make_async_copy(src.at[pl.ds(hf * DH2, DH2), pl.ds((ci % NG) * HG, HG), :],
                                      st_sc.at[dst, :, pl.ds(hf * HG, HG), :], sem_w.at[dst])
                for hf in range(2)]

    wo_copy = pltpu.make_async_copy(wo_hbm, wo_sc, sem_w.at[NCH])

    def out_copy(lo, n):
        rows = pl.ds(lo * SEG if isinstance(lo, int) else pl.multiple_of(lo * SEG, SEG), n * SEG)
        return pltpu.make_async_copy(out_sc.at[rows, LN], o_hbm.at[rows], sem_out)

    def start_all(cps):
        def act():
            for cp in cps:
                cp.start()
        return act

    order = [[mem0_copy, x_copy(0)], w_copies(0), [x_copy(1)], [x_copy(2)]]
    for ci in range(1, NCH):
        order.append(w_copies(ci) + ([x_copy(ci + 2)] if ci + 2 < NRB else []))
        if ci == NRB - 2:
            order.append(small + in_copies(0))
    order += [[wo_copy], in_copies(1), in_copies(2)]
    for i in range(0, len(order), 5):
        _in_order([start_all(cps) for cps in order[i:i + 5]])

    never_sm[0] = 0
    k_sc[0:KPAD, LN] = jnp.zeros((KPAD, DM), BF16)
    sp_sc[NB + 1] = jnp.zeros(sp_sc.shape[1:], F32)
    op_sc[...] = jnp.zeros(op_sc.shape, F32)
    x2_sc[...] = jnp.zeros(x2_sc.shape, F32)
    y_sc[...] = jnp.zeros(y_sc.shape, F32)
    mem0_copy.wait()
    x_copy(0).wait()
    for sg in range(RB + 1):
        xn_sc[sg, :, 0:DM] = _pack(_ln(x_sc[sg * SEG:(sg + 1) * SEG, LN].astype(F32)))

    def clip(i, hi):
        return min(max(i, 0), hi) if isinstance(i, int) else jnp.clip(i, 0, hi)

    def scaled(i, m):
        return i * m if isinstance(i, int) else pl.multiple_of(i * m, m)

    def seg(i):
        return pl.ds(scaled(clip(i, NSEG - 1), SEG), SEG)

    def conv_u(s, ln=LN):
        r0 = scaled(clip(s, NSEG - 1), SEG)
        sh = sh_ref[:, ln].astype(F32)
        kk = k_sc[pl.ds(r0, KPAD + SEG), ln].astype(F32)
        ks = kk[KPAD:] * sh[0:1]
        for j in range(1, KS):
            ks = ks + pltpu.roll(kk, j, 0)[KPAD:] * sh[j:j + 1]
        u = (ks * v_sc[pl.ds(r0, SEG), ln].astype(F32)).astype(BF16)
        u_sc[pl.ds(r0, SEG), ln] = u
        return u

    def conv_fwd(c, q):
        cc = clip(c, NB - 1)
        f = fwd_ref[q]
        uf = _dot(f, u_sc[pl.ds(scaled(cc, CB), CB), LN])
        kf = _dot_nt(f, sk_sc[cc])
        return uf, kf

    def put_spec(cs, q, which, val):
        for rb in range(QB // 8):
            for n in range(NT):
                ln = slice(n * 128, (n + 1) * 128)
                sp_sc[cs, q, rb, n, which] = val[rb * 8:rb * 8 + 8, ln]
                sp_sc[cs, q, rb, n, which + 1] = val[QB + rb * 8:QB + rb * 8 + 8, ln]

    def conv_spec(c, q):
        uf, kf = conv_fwd(c, q)
        cs = clip(c, NB)
        put_spec(cs, q, 0, uf)
        pk = kr_sc[q]
        kr_sc[q] = kf
        kp = jnp.concatenate([
            kf[0:HB] - pk[QB:QB + HB],
            kf[HB:QB] + pk[QB + HB:],
            kf[QB:QB + HB] + pk[0:HB],
            kf[QB + HB:] - pk[HB:QB]], axis=0)
        put_spec(cs, q, 2, kp)

    MAC_PIECES = [(rb, n) for rb in range(QB // 16) for n in range(NT)]

    def conv_mac(c, q, piece, nterms):
        rb2, n = piece
        cs = clip(c, NB)
        acc = []
        for rb in (2 * rb2, 2 * rb2 + 1):
            ar = None
            ai = None
            for j in range(nterms):
                if isinstance(cs, int):
                    uj, kj = j, cs - j
                else:
                    uj = jnp.minimum(j, cs)
                    kj = jnp.where(cs - j >= 0, cs - j, NB + 1)
                ur = sp_sc[uj, q, rb, n, 0]
                um = sp_sc[uj, q, rb, n, 1]
                kr = sp_sc[kj, q, rb, n, 2]
                km = sp_sc[kj, q, rb, n, 3]
                tr = ur * kr - um * km
                ti = ur * km + um * kr
                ar = tr if ar is None else ar + tr
                ai = ti if ai is None else ai + ti
            acc.append((ar, ai))
        ln = slice(n * 128, (n + 1) * 128)
        w = jnp.concatenate([acc[0][0], acc[1][0], acc[0][1], acc[1][1]], axis=0).astype(BF16)
        wf_sc[c & 1, q, rb2 * 16:rb2 * 16 + 16, ln] = w[0:16]
        wf_sc[c & 1, q, QB + rb2 * 16:QB + rb2 * 16 + 16, ln] = w[16:]

    def conv_inv(s):
        w = wf_sc[(s // NQ) & 1].reshape(2 * CB, DM)
        yc = _dot(inv_ref[s % NQ], w)
        sd = sd_ref[...].astype(F32).reshape(1, DM)
        y_sc[s & 3] = yc + u_sc[seg(s), LN].astype(F32) * sd

    scale = DH ** -0.5
    cexp = scale * float(np.log2(np.e))

    def make_mask(n, x_layers, q0=0):
        qi = jax.lax.broadcasted_iota(jnp.int32, (n - q0, n), 0) + q0
        ki = jax.lax.broadcasted_iota(jnp.int32, (n - q0, n), 1)

        def layer(i):
            xl = jnp.where(i < M2 + SEG, x_layers[0], x_layers[-1])
            return jnp.where(i < M, 0, jnp.where(i < M2, 1, xl))
        same = layer(qi) == layer(ki)
        ok = same & ((qi < M2) | (ki < M2) | (qi >= ki))
        fill = jnp.where(same, -1e9 / scale, -jnp.inf).astype(F32)
        return ok, fill

    def probs(q, k, mask):
        ok, fill = mask
        s = _dot_nt(q, k)
        s = jnp.where(ok, s, fill)
        m = jnp.max(s, axis=-1, keepdims=True)
        p = jnp.exp2((s - m) * cexp)
        l = jnp.sum(p, axis=-1, keepdims=True)
        r = pl.reciprocal(l, approx=True)
        r = r * (2.0 - l * r)
        return (p * r).astype(BF16)

    def w_slot(ci):
        return (wb_sc, ci) if 1 <= ci < NRB - 1 else (wa_sc, max(ci - (NRB - 2), 0))

    def w_head(g, mats):
        slots = [w_slot(mi * NG + g // HG) for mi in mats]
        return _unpack(jnp.concatenate([ref[i, g % HG] for ref, i in slots], axis=1))

    def proj_split(hq, hkv, g):
        q = _dot(hq, w_head(g, (0,))).astype(BF16)
        kv = _dot(hkv, w_head(g, (1, 2))).astype(BF16)
        return q, kv[:, :DH], kv[:, DH:]

    def xn(s):
        return _unpack(xn_sc[clip(s, NSEG - 1), :, 0:DM])

    def out_proj(n, g0, g1, j):
        return _dot(_unpack(o_sc[0:n // 2, g0 * DH:g1 * DH]),
                    wo_sc[g0 * DH:g1 * DH, j * 128:(j + 1) * 128])

    def attend(proj, n, mask, dist, hook=None):
        D1, D2 = dist
        HA = H - D1 - D2 - 1
        NE = min(D1 + D2, NT - 1)
        qkvs = {}
        ps = {}
        outs = {}
        for it in range(H + D1 + D2):
            if it < H:
                qkvs[it] = proj(it)
            g = it - D1
            if 0 <= g < H:
                ps[g] = probs(qkvs[g][0], qkvs[g][1], mask)
            g = it - D1 - D2
            if 0 <= g < H:
                o = _dot(ps.pop(g), qkvs.pop(g)[2])
                o_sc[0:n // 2, g * DH:(g + 1) * DH] = _pack(o)
            if hook is not None:
                hook(it)
            j = it - (H - 1)
            if 0 <= j < NE:
                outs[j] = out_proj(n, 0, HA, j)
        for j in range(NE, NT):
            outs[j] = out_proj(n, 0, H, j)
        for j in range(NE):
            outs[j] = out_proj(n, HA, H, j) + outs[j]
        return jnp.concatenate([outs[j] for j in range(NT)], axis=1)

    def side2(t, a2):
        x3 = x2_sc[(t - 2) & 3] + a2
        x4 = x3 + _ln(x3) * y_sc[(t - 2) & 3]
        x4 = x4.astype(out_sc.dtype)
        out_sc[seg(t - 2), LN] = x4
        return x4

    def finish(t, xr, yt, mem, a1, spec):
        if spec:
            conv_spec((t + 1) // NQ + 1, (t + 1) % NQ)
        xq = xn(t + 1)
        for g in range(NPA, NPA + NPB):
            fill_sc[g - NPA] = _pack(_dot(xq, w_head(g, (0,))))
        conv_inv(t + 1)
        x1 = xr.astype(F32) + a1
        x2 = x1 + _ln(x1) * yt
        h_sc[0:M, :] = _pack(mem)
        h_sc[M:, :] = _pack(_ln(x2))
        x2_sc[t & 3] = x2

    def pinned(rows, pins):
        never = never_sm[0] > 0
        hs = {0: rows}
        r = _pack(rows)
        tiles = [r[:, n * 128:(n + 1) * 128] for n in range(NT)]
        for g, n, d in sorted(pins, key=lambda p: p[0]):
            tiles[n] = jnp.where(never, d, tiles[n])
            hs[g] = _unpack(jnp.concatenate(tiles, axis=1))
        return lambda g: hs[max(k for k in hs if k <= g)]

    def pin_tiles(g0, stride, val):
        v = _pack(val)
        return [(g0 + n * stride, n, v[:, n * 128:(n + 1) * 128]) for n in range(NT)]

    def wait_chunk(ci):
        for cp in w_copies(0, ci):
            cp.wait()

    def relayout(ci, dst, slot, b):
        d0 = scaled(b, 16)
        r0 = scaled(b, 8)
        xw = pltpu.bitcast(st_sc[ci, pl.ds(d0, 16)], U32).reshape(8, 2, HG, DH)
        a = xw[:, 0]
        bb = xw[:, 1]
        lo = jnp.swapaxes((a & U32(0xFFFF)) | (bb << 16), 0, 1)
        hi = jnp.swapaxes((a >> 16) | (bb & U32(0xFFFF0000)), 0, 1)
        for j in range(HG):
            rows = pl.ds(r0 + (2 * j // HG) * (DH2 // 2), 8)
            dst[slot, 2 * j % HG, rows, :] = lo[j]
            dst[slot, 2 * j % HG + 1, rows, :] = hi[j]

    NBLK = DH2 // 16
    with jax.named_scope("wait_w"):
        wait_chunk(0)

    def relayout0(b, c):
        relayout(0, wa_sc, 0, b)
        return c
    with jax.named_scope("relayout"):
        jax.lax.fori_loop(0, NBLK, relayout0, 0, unroll=2)

    def pro_stage(ps_, b):
        n = ps_ * NRB + b
        with jax.named_scope("wait_w"):
            if ps_ == 0:
                @pl.when(b + 1 < NRB)
                def _():
                    x_copy(b + 1).wait()

            @pl.when((n >= 2) & (n <= NCH))
            def _():
                wait_chunk(n - 1)
        cr = jnp.clip(n - 1, 0, NCH - 1)
        dst, slot = (wb_sc, cr) if ps_ == 0 else (wa_sc, cr - (NRB - 2))
        src, si = w_slot(ps_)
        bl = jnp.minimum(b + 1, NRB - 1)
        PW = PRO_PW
        npc = RB * S2 // PW
        assert npc * PW == RB * S2 and PRO_R0 + (NBLK - 1) * PRO_RS < HG * npc
        assert PRO_X0 + (max(RB, 2 * NT) - 1) * PRO_XS < HG * npc and 2 * NRB > 2 * NQ

        def body(i, c):
            s0 = b * RB + 1
            for sg in range(RB):
                hp_sc[sg * S2:(sg + 1) * S2, :] = xn_sc[s0 + sg, :, 0:DM]
            for j in range(HG):
                w = _unpack(src[si, j])
                for pi in range(npc):
                    pos = j * npc + pi
                    hx = hp_sc[pi * PW:(pi + 1) * PW, :]
                    k, rem = divmod(pos - PRO_X0, PRO_XS)
                    if ps_ == 0 and rem == 0 and 0 <= k < RB:
                        sn = bl * RB + 1 + k
                        xv = _pack(_ln(x_sc[seg(sn), LN].astype(F32)))
                        xn_sc[sn, :, 0:DM] = xv
                        hx = jnp.concatenate([hx[:-S2], jnp.where(never_sm[0] > 0, xv, hx[-S2:])], axis=0)
                    if ps_ == 1 and rem == 0 and 0 <= k < 2 * NT:
                        conv_u(jnp.minimum(2 * b + k // NT, 2 * NQ),
                               slice((k % NT) * 128, (k % NT + 1) * 128))
                    bb, rem = divmod(pos - PRO_R0, PRO_RS)
                    if rem == 0 and 0 <= bb < NBLK:
                        relayout(cr, dst, slot, bb)
                    r = _pack(_dot(_unpack(hx), w))
                    for a in range(0, PW, 8):
                        sg, off = divmod(pi * PW + a, S2)
                        pre_sc[s0 + sg, ps_ * HG + j, off:off + 8, :] = r[a:a + 8]
            return c
        with jax.named_scope("fused"):
            jax.lax.fori_loop(0, never_sm[0] + 1, body, 0)

    for ps_ in range(NPASS):
        if ps_ == 1:
            with jax.named_scope("wait_in0"):
                for cp in small + in_copies(0):
                    cp.wait()

        def blk(b, c, ps_=ps_):
            pro_stage(ps_, b)
            return c
        jax.lax.fori_loop(0, NRB, blk, 0)

    def warm_block0(q):
        uf, kf = conv_fwd(0, q)
        put_spec(0, q, 0, uf)
        put_spec(0, q, 2, kf)
        kr_sc[q] = kf
        ur, um, kr, km = uf[:QB], uf[QB:], kf[:QB], kf[QB:]
        wf_sc[0, q, :QB] = (ur * kr - um * km).astype(BF16)
        wf_sc[0, q, QB:] = (ur * km + um * kr).astype(BF16)

    with jax.named_scope("warm"):
        for q in range(NQ):
            warm_block0(q)
    with jax.named_scope("wait_wo"):
        wo_copy.wait()
    with jax.named_scope("step0"):
        mem0 = mem0_ref[...].astype(F32)
        h0 = jnp.concatenate([jnp.concatenate([mem0, mem0], axis=0).astype(BF16), xn(0)], axis=0)

        def hook0(it):
            if it == 6:
                conv_spec(1, 0)
                for piece in MAC_PIECES:
                    conv_mac(1, 0, piece, 2)
            if it == 14:
                conv_inv(0)
        out = attend(lambda g: proj_split(h0, h0, g), RH, make_mask(RH, (0,)), DIST_HALF, hook0)
        finish(0, x_sc[0:SEG, LN], y_sc[0], jnp.concatenate([out[0:M], mem0], axis=0), out[M2:], False)

    mask12 = make_mask(R, (0, 1))

    def step(t, first, last):
        if first:
            conv_spec_later = functools.partial(conv_spec, t // NQ + 1, t % NQ)
        x4 = side2(t, op_sc[...])
        un = conv_u(t + 2 * NQ)
        hm = _unpack(h_sc[0:M, :])
        hx2 = _unpack(h_sc[M:, :])
        h48 = jnp.concatenate([hm, hx2], axis=0)
        x1n = pinned(xn(t), pin_tiles(PIN_U if first else PIN_U2, 1, un) + pin_tiles(PIN_X4, X4S, x4))

        def proj(g):
            h80 = jnp.concatenate([hm, x1n(g), hx2], axis=0)
            if g >= NPA + NPB:
                return proj_split(h80, h80, g)
            q, k, v = proj_split(h48, h80, g)
            q1 = pre_sc[t, g] if g < NPA else fill_sc[g - NPA]
            return jnp.concatenate([q[0:M2], _unpack(q1), q[M2:]], axis=0), k, v

        held = {}

        def hook(it):
            if it == SPEC_AT:
                if first:
                    conv_spec_later()
                for piece in MAC_PIECES:
                    conv_mac(t // NQ + 1, t % NQ, piece, NB)
            if it == H:
                held["x"] = x_sc[seg(t), LN]
                held["y"] = y_sc[t & 3]
        out = attend(proj, R, mask12, DIST, hook)
        op_sc[...] = out[RH:]
        finish(t, held["x"], held["y"], out[0:M2], out[M2:RH], not last)

    def steps(i, carry):
        for j in range(UNROLL):
            step(1 + i * UNROLL + j, j == 0, j == UNROLL - 1)
        return carry

    def phase(p, carry):
        @pl.when(p == 1)
        def _():
            for cp in in_copies(2):
                cp.wait()

        @pl.when(p >= 2)
        def _():
            out_copy((p - 2) * PH, PH).start()

        with jax.named_scope("steps"):
            jax.lax.fori_loop(p * PHI, (p + 1) * PHI, steps, 0)
        return carry

    for cp in in_copies(1):
        cp.wait()
    jax.lax.fori_loop(0, NPH, phase, 0)
    out_copy((NPH - 2) * PH, NSEG - 2 - (NPH - 2) * PH).start()

    with jax.named_scope("step_last"):
        x4 = side2(NSEG, op_sc[...])
        hm = _unpack(h_sc[0:M, :])
        hx = pinned(_unpack(h_sc[M:, :]), pin_tiles(PIN_X4, 0, x4))
        out = attend(lambda g: proj_split(hx(g), jnp.concatenate([hm, hx(g)], axis=0), g),
                     SEG, make_mask(RH, (1,), M2), DIST_LAST)
        side2(NSEG + 1, out)
    out_copy(NSEG - 2, 2).start()
    out_copy(0, NSEG).wait()


def pallas_interleave_layers__memory_aug_recurrent_mem_tr__ssm_conv_h3__prompt_kernel(
    A_x, A_mem0, A_Wq, A_Wk, A_Wv, A_Wo, A_seg_len,
    B_q, B_k, B_v, B_shift_k, B_ssm_k, B_ssm_D,
):
    del B_q
    seg = int(A_seg_len) if isinstance(A_seg_len, (int, np.integer)) else CB // NQ
    return _run(A_x, A_mem0, A_Wq, A_Wk, A_Wv, A_Wo, B_k, B_v, B_shift_k, B_ssm_k, B_ssm_D, SEG=seg)


@functools.partial(jax.jit, static_argnames=("SEG",))
def _run(A_x, A_mem0, A_Wq, A_Wk, A_Wv, A_Wo, B_k, B_v, B_shift_k, B_ssm_k, B_ssm_D, *, SEG):
    B, S, DM = A_x.shape
    assert B == 1
    H, DH = A_Wq.shape[1], A_Wq.shape[2]
    M = A_mem0.shape[1]
    KS = B_shift_k.shape[1]
    R = 2 * (M + SEG)
    NSEG = S // SEG
    NRB = (NSEG - 1) // RB
    NB = S // CB
    QB = CB // NQ
    NCH = 3 * H // HG
    DP = -(-DM // 256) * 256
    fwd, inv = _dft_constants()

    kern = functools.partial(_kernel, S=S, DM=DM, H=H, DH=DH, M=M, SEG=SEG)
    any_spec = pl.BlockSpec(memory_space=pl.ANY)
    out = pl.pallas_call(
        kern,
        out_shape=jax.ShapeDtypeStruct((S, DM), A_x.dtype),
        in_specs=[any_spec] * 13,
        out_specs=any_spec,
        scratch_shapes=[
            pltpu.VMEM((NB + 2, NQ, QB // 8, DM // 128, 4, 8, 128), F32),
            pltpu.VMEM((NQ, 2 * QB, DM), F32),
            pltpu.VMEM((2, NQ, 2 * QB, DM), BF16),
            pltpu.VMEM((4, SEG, DM), F32),
            pltpu.VMEM((4, SEG, DM), F32),
            pltpu.VMEM((S, DP), BF16),
            pltpu.VMEM((SEG, DM), F32),
            pltpu.VMEM((NSEG, NPA, SEG // 2, DH), U32),
            pltpu.VMEM((NPB, SEG // 2, DH), U32),
            pltpu.VMEM((NSEG, SEG // 2, DP), U32),
            pltpu.VMEM((NCH - NRB + 2, HG, DM // 2, DH), U32),
            pltpu.VMEM((NRB - 1, HG, DM // 2, DH), U32),
            pltpu.VMEM((H * DH, DM), BF16),
            pltpu.VMEM((R // 2, H * DH), U32),
            pltpu.VMEM((S, DP), BF16),
            pltpu.VMEM((S, DP), BF16),
            pltpu.VMEM((NB, DM, CB), BF16),
            pltpu.VMEM((NCH, DM // 2, 2 * HG, DH), BF16),
            pltpu.VMEM((S, DP), A_x.dtype),
            pltpu.VMEM(fwd.shape, BF16),
            pltpu.VMEM(inv.shape, BF16),
            pltpu.VMEM((S + KPAD, DP), BF16),
            pltpu.VMEM((RB * SEG // 2, DM), U32),
            pltpu.VMEM((M + SEG // 2, DM), U32),
            pltpu.VMEM((M, DM), BF16),
            pltpu.VMEM((KS, DM), BF16),
            pltpu.VMEM((DM,), BF16),
            pltpu.SMEM((1,), jnp.int32),
            pltpu.SemaphoreType.DMA(((NSEG - 1) // RB,)),
            pltpu.SemaphoreType.DMA((3,)),
            pltpu.SemaphoreType.DMA((NCH + 1,)),
            pltpu.SemaphoreType.DMA(()),
        ],
        compiler_params=pltpu.CompilerParams(vmem_limit_bytes=120 * 1024 * 1024),
    )(
        A_x.reshape(S, DM), A_mem0.reshape(M, DM), A_Wq, A_Wk, A_Wv,
        A_Wo.reshape(H * DH, DM), B_k.reshape(S, DM), B_v.reshape(S, DM),
        B_shift_k.T, B_ssm_k, B_ssm_D,
        jnp.asarray(fwd, BF16), jnp.asarray(inv, BF16),
    )
    return out.reshape(B, S, DM)
```

```python
import functools

import numpy as np
import jax
import jax.numpy as jnp
import jax.experimental.pallas as pl
import jax.experimental.pallas.tpu as pltpu

F32 = jnp.float32
BF16 = jnp.bfloat16
U32 = jnp.uint32

CB = 128
NQ = 4
KPAD = 16
HG = 8
NPA = 16
NPB = 12
RB = 9
PRO_PW, PRO_X0, PRO_XS, PRO_R0, PRO_RS = 24, 11, 4, 2, 2
UNROLL = 3
PHI = 3
PIN_U2, X4S = 1, 0
SPEC_AT, PIN_U, PIN_X4 = 7, 1, 16
DIST, DIST_HALF, DIST_LAST = (1, 2), (1, 3), (2, 3)


def _dft_constants():
    qb = CB // NQ
    n = np.arange(CB, dtype=np.float64)
    fwd = np.zeros((NQ, 2 * qb, CB))
    for q in range(NQ):
        f = q * qb + np.concatenate([np.arange(0, qb, 2), np.arange(1, qb, 2)])
        ang = (np.pi * (2.0 * f + 1.0) / (2 * CB))[:, None] * n[None, :]
        fwd[q, :qb] = np.cos(ang)
        fwd[q, qb:] = -np.sin(ang)
    inv = fwd.reshape(2 * CB, CB).T / CB
    return fwd.astype(np.float32), inv.reshape(NQ, CB // NQ, 2 * CB).astype(np.float32)


def _ln(x, eps=1e-5):
    d = x.shape[-1]
    m = jnp.sum(x, axis=-1, keepdims=True) * (1.0 / d)
    xc = x - m
    v = jnp.sum(xc * xc, axis=-1, keepdims=True) * (1.0 / d)
    return xc * jax.lax.rsqrt(v + eps)


def _dot(a, b):
    return jnp.dot(a, b, preferred_element_type=F32)


def _dot_nt(a, b):
    return jax.lax.dot_general(a, b, (((1,), (1,)), ((), ())), preferred_element_type=F32)


def _pack(x):
    return pltpu.bitcast(x.astype(BF16), U32)


def _unpack(x):
    return pltpu.bitcast(x, BF16)


def _in_order(actions):
    def body(i, c):
        for j, act in enumerate(actions):
            pl.when(i == j)(act)
        return c
    jax.lax.fori_loop(0, len(actions), body, 0)


def _kernel(x_hbm, mem0_hbm, wq_hbm, wk_hbm, wv_hbm, wo_hbm, k_hbm, v_hbm,
            sh_hbm, sk_hbm, sd_hbm, fwd_hbm, inv_hbm, o_hbm,
            sp_sc, kr_sc, wf_sc, x2_sc, y_sc, u_sc, op_sc, pre_sc, fill_sc, xn_sc, wa_sc, wb_sc, wo_sc, o_sc,
            x_sc, v_sc, sk_sc, st_sc, out_sc, fwd_ref, inv_ref,
            k_sc, hp_sc, h_sc, co_sc, mem0_ref, sh_ref, sd_ref,
            never_sm, sem_x, sem_in, sem_w, sem_out,
            *, S, DM, H, DH, M, SEG):
    NSEG = S // SEG
    M2 = 2 * M
    S2 = SEG // 2
    R = M2 + 2 * SEG
    RH = M2 + SEG
    NB = S // CB
    QB = CB // NQ
    HB = QB // 2
    NT = DM // 128
    PH = PHI * UNROLL
    NRB = (NSEG - 1) // RB
    NPH = (NSEG - 1) // PH
    NG = H // HG
    NCH = 3 * NG
    NPASS = NPA // HG
    DH2 = DM // 2
    KS = sh_ref.shape[0]
    LN = pl.ds(0, DM)
    assert 2 <= KS <= 8 and QB == SEG and NRB * RB == NSEG - 1 and NPH * PH == NSEG - 1 and NPASS == 2 and 2 * NRB >= NCH + 1

    mem0_copy = pltpu.make_async_copy(mem0_hbm, mem0_ref, sem_x.at[0])
    small = [pltpu.make_async_copy(s, d, sem_in.at[0]) for s, d in [
        (sh_hbm, sh_ref), (sd_hbm, sd_ref), (fwd_hbm, fwd_ref), (inv_hbm, inv_ref)]]

    def x_copy(b):
        if isinstance(b, int) and b == 0:
            rows = pl.ds(0, (RB + 1) * SEG)
        else:
            rows = pl.ds(pl.multiple_of((b * RB + 1) * SEG, SEG), RB * SEG)
        return pltpu.make_async_copy(x_hbm.at[rows], x_sc.at[rows, LN], sem_x.at[b])

    kb = (0, (2 * NQ + 1) * SEG, (2 * NQ + PH + 1) * SEG, S)
    sb = (0, 2, (PH + 1) // NQ + 2, NB)

    def in_copies(part):
        def rng(b):
            return pl.ds(b[part], b[part + 1] - b[part])
        sem = sem_in.at[part]
        return [
            pltpu.make_async_copy(k_hbm.at[rng(kb)],
                                  k_sc.at[pl.ds(KPAD + kb[part], kb[part + 1] - kb[part]), LN], sem),
            pltpu.make_async_copy(v_hbm.at[rng(kb)], v_sc.at[rng(kb), LN], sem),
        ] + [pltpu.make_async_copy(sk_hbm.at[:, pl.ds(c * CB, CB)], sk_sc.at[c], sem)
             for c in range(sb[part], sb[part + 1])]

    def w_copies(ci, dst=None):
        src = (wq_hbm, wk_hbm, wv_hbm)[ci // NG]
        dst = ci if dst is None else dst
        return [pltpu.make_async_copy(src.at[pl.ds(hf * DH2, DH2), pl.ds((ci % NG) * HG, HG), :],
                                      st_sc.at[dst, :, pl.ds(hf * HG, HG), :], sem_w.at[dst])
                for hf in range(2)]

    wo_copy = pltpu.make_async_copy(wo_hbm, wo_sc, sem_w.at[NCH])

    def out_copy(lo, n):
        rows = pl.ds(lo * SEG if isinstance(lo, int) else pl.multiple_of(lo * SEG, SEG), n * SEG)
        return pltpu.make_async_copy(out_sc.at[rows, LN], o_hbm.at[rows], sem_out)

    def start_all(cps):
        def act():
            for cp in cps:
                cp.start()
        return act

    order = [[mem0_copy, x_copy(0)], w_copies(0), [x_copy(1)], [x_copy(2)]]
    for ci in range(1, NCH):
        order.append(w_copies(ci) + ([x_copy(ci + 2)] if ci + 2 < NRB else []))
        if ci == NRB - 2:
            order.append(small + in_copies(0))
    order += [[wo_copy], in_copies(1), in_copies(2)]
    for i in range(0, len(order), 5):
        _in_order([start_all(cps) for cps in order[i:i + 5]])

    never_sm[0] = 0
    k_sc[0:KPAD, LN] = jnp.zeros((KPAD, DM), BF16)
    sp_sc[NB + 1] = jnp.zeros(sp_sc.shape[1:], F32)
    op_sc[...] = jnp.zeros(op_sc.shape, F32)
    x2_sc[...] = jnp.zeros(x2_sc.shape, F32)
    y_sc[...] = jnp.zeros(y_sc.shape, F32)
    mem0_copy.wait()
    x_copy(0).wait()
    for sg in range(RB + 1):
        xn_sc[sg, :, 0:DM] = _pack(_ln(x_sc[sg * SEG:(sg + 1) * SEG, LN].astype(F32)))

    def clip(i, hi):
        return min(max(i, 0), hi) if isinstance(i, int) else jnp.clip(i, 0, hi)

    def scaled(i, m):
        return i * m if isinstance(i, int) else pl.multiple_of(i * m, m)

    def seg(i):
        return pl.ds(scaled(clip(i, NSEG - 1), SEG), SEG)

    def conv_u(s, ln=LN):
        r0 = scaled(clip(s, NSEG - 1), SEG)
        kk = k_sc[pl.ds(r0, KPAD + SEG), ln].astype(F32)[KPAD - 8:]

        def coef(j, rows):
            return jnp.concatenate([co_sc[j, :, ln]] * (rows // 8), axis=0)
        sft = [kk] + [pltpu.roll(kk, j, 0) for j in range(2, KS, 2)]
        ev = functools.reduce(jnp.add, [sft[j // 2][8:] * coef(j, SEG) for j in range(0, KS, 2)])
        od = functools.reduce(jnp.add, [sft[j // 2] * coef(j, SEG + 8) for j in range(1, KS, 2)])
        ks = ev + pltpu.roll(od, 1, 0)[8:]
        u = (ks * v_sc[pl.ds(r0, SEG), ln].astype(F32)).astype(BF16)
        u_sc[pl.ds(r0, SEG), ln] = u
        return u

    def conv_fwd(c, q):
        cc = clip(c, NB - 1)
        f = fwd_ref[q]
        uf = _dot(f, u_sc[pl.ds(scaled(cc, CB), CB), LN])
        kf = _dot_nt(f, sk_sc[cc])
        return uf, kf

    def put_spec(cs, q, which, val):
        for rb in range(QB // 8):
            for n in range(NT):
                ln = slice(n * 128, (n + 1) * 128)
                sp_sc[cs, q, rb, n, which] = val[rb * 8:rb * 8 + 8, ln]
                sp_sc[cs, q, rb, n, which + 1] = val[QB + rb * 8:QB + rb * 8 + 8, ln]

    def conv_spec(c, q):
        uf, kf = conv_fwd(c, q)
        cs = clip(c, NB)
        put_spec(cs, q, 0, uf)
        pk = kr_sc[q]
        kr_sc[q] = kf
        kp = jnp.concatenate([
            kf[0:HB] - pk[QB:QB + HB],
            kf[HB:QB] + pk[QB + HB:],
            kf[QB:QB + HB] + pk[0:HB],
            kf[QB + HB:] - pk[HB:QB]], axis=0)
        put_spec(cs, q, 2, kp)

    MAC_PIECES = [(rb, n) for rb in range(QB // 16) for n in range(NT)]

    def conv_mac(c, q, piece, nterms):
        rb2, n = piece
        cs = clip(c, NB)
        acc = []
        for rb in (2 * rb2, 2 * rb2 + 1):
            ar = None
            ai = None
            for j in range(nterms):
                if isinstance(cs, int):
                    uj, kj = j, cs - j
                else:
                    uj = jnp.minimum(j, cs)
                    kj = jnp.where(cs - j >= 0, cs - j, NB + 1)
                ur = sp_sc[uj, q, rb, n, 0]
                um = sp_sc[uj, q, rb, n, 1]
                kr = sp_sc[kj, q, rb, n, 2]
                km = sp_sc[kj, q, rb, n, 3]
                tr = ur * kr - um * km
                ti = ur * km + um * kr
                ar = tr if ar is None else ar + tr
                ai = ti if ai is None else ai + ti
            acc.append((ar, ai))
        ln = slice(n * 128, (n + 1) * 128)
        w = jnp.concatenate([acc[0][0], acc[1][0], acc[0][1], acc[1][1]], axis=0).astype(BF16)
        wf_sc[c & 1, q, rb2 * 16:rb2 * 16 + 16, ln] = w[0:16]
        wf_sc[c & 1, q, QB + rb2 * 16:QB + rb2 * 16 + 16, ln] = w[16:]

    def conv_inv(s):
        w = wf_sc[(s // NQ) & 1].reshape(2 * CB, DM)
        yc = _dot(inv_ref[s % NQ], w)
        sd = jnp.concatenate([co_sc[KS]] * (SEG // 8), axis=0)
        y_sc[s & 3] = yc + u_sc[seg(s), LN].astype(F32) * sd

    scale = DH ** -0.5
    cexp = scale * float(np.log2(np.e))

    def make_mask(n, x_layers, q0=0):
        qi = jax.lax.broadcasted_iota(jnp.int32, (n - q0, n), 0) + q0
        ki = jax.lax.broadcasted_iota(jnp.int32, (n - q0, n), 1)

        def layer(i):
            xl = jnp.where(i < M2 + SEG, x_layers[0], x_layers[-1])
            return jnp.where(i < M, 0, jnp.where(i < M2, 1, xl))
        same = layer(qi) == layer(ki)
        ok = same & ((qi < M2) | (ki < M2) | (qi >= ki))
        fill = jnp.where(same, -1e9 / scale, -jnp.inf).astype(F32)
        return ok, fill

    def probs(q, k, mask):
        ok, fill = mask
        s = _dot_nt(q, k)
        s = jnp.where(ok, s, fill)
        m = jnp.max(s, axis=-1, keepdims=True)
        p = jnp.exp2((s - m) * cexp)
        l = jnp.sum(p, axis=-1, keepdims=True)
        r = pl.reciprocal(l, approx=True)
        r = r * (2.0 - l * r)
        return (p * r).astype(BF16)

    def w_slot(ci):
        return (wb_sc, ci) if 1 <= ci < NRB - 1 else (wa_sc, max(ci - (NRB - 2), 0))

    def w_head(g, mats):
        slots = [w_slot(mi * NG + g // HG) for mi in mats]
        return _unpack(jnp.concatenate([ref[i, g % HG] for ref, i in slots], axis=1))

    def proj_split(hq, hkv, g, q1=None):
        q = _dot(hq, w_head(g, (0,)))
        kv = _dot(hkv, w_head(g, (1, 2)))
        if q1 is not None:
            q = jnp.concatenate([q[0:M2], q1, q[M2:]], axis=0)
        return q.astype(BF16), kv[:, :DH].astype(BF16), kv[:, DH:].astype(BF16)

    def xn(s):
        return _unpack(xn_sc[clip(s, NSEG - 1), :, 0:DM])

    def out_proj(n, g0, g1, j):
        return _dot(_unpack(o_sc[0:n // 2, g0 * DH:g1 * DH]),
                    wo_sc[g0 * DH:g1 * DH, j * 128:(j + 1) * 128])

    def attend(proj, n, mask, dist, hook=None):
        D1, D2 = dist
        HA = H - D1 - D2 - 1
        NE = min(D1 + D2, NT - 1)
        qkvs = {}
        ps = {}
        outs = {}
        for it in range(H + D1 + D2):
            if it < H:
                qkvs[it] = proj(it)
            g = it - D1
            if 0 <= g < H:
                ps[g] = probs(qkvs[g][0], qkvs[g][1], mask)
            g = it - D1 - D2
            if 0 <= g < H:
                o = _dot(ps.pop(g), qkvs.pop(g)[2])
                o_sc[0:n // 2, g * DH:(g + 1) * DH] = _pack(o)
            if hook is not None:
                hook(it)
            j = it - (H - 1)
            if 0 <= j < NE:
                outs[j] = out_proj(n, 0, HA, j)
        for j in range(NE, NT):
            outs[j] = out_proj(n, 0, H, j)
        for j in range(NE):
            outs[j] = out_proj(n, HA, H, j) + outs[j]
        return jnp.concatenate([outs[j] for j in range(NT)], axis=1)

    def side2(t, a2):
        x3 = x2_sc[(t - 2) & 3] + a2
        x4 = x3 + _ln(x3) * y_sc[(t - 2) & 3]
        x4 = x4.astype(out_sc.dtype)
        out_sc[seg(t - 2), LN] = x4
        return x4

    def finish(t, xr, yt, mem, a1, spec):
        if spec:
            conv_spec((t + 1) // NQ + 1, (t + 1) % NQ)
        xq = xn(t + 1)
        for g in range(NPA, NPA + NPB):
            fill_sc[g - NPA] = _dot(xq, w_head(g, (0,)))
        conv_inv(t + 1)
        x1 = xr.astype(F32) + a1
        x2 = x1 + _ln(x1) * yt
        h_sc[0:M, :] = _pack(mem)
        h_sc[M:, :] = _pack(_ln(x2))
        x2_sc[t & 3] = x2

    def pinned(rows, pins):
        never = never_sm[0] > 0
        hs = {0: rows}
        r = _pack(rows)
        tiles = [r[:, n * 128:(n + 1) * 128] for n in range(NT)]
        for g, n, d in sorted(pins, key=lambda p: p[0]):
            tiles[n] = jnp.where(never, d, tiles[n])
            hs[g] = _unpack(jnp.concatenate(tiles, axis=1))
        return lambda g: hs[max(k for k in hs if k <= g)]

    def pin_tiles(g0, stride, val):
        v = _pack(val)
        return [(g0 + n * stride, n, v[:, n * 128:(n + 1) * 128]) for n in range(NT)]

    def wait_chunk(ci):
        for cp in w_copies(0, ci):
            cp.wait()

    def relayout(ci, dst, slot, b):
        d0 = scaled(b, 16)
        r0 = scaled(b, 8)
        xw = pltpu.bitcast(st_sc[ci, pl.ds(d0, 16)], U32).reshape(8, 2, HG, DH)
        a = xw[:, 0]
        bb = xw[:, 1]
        lo = jnp.swapaxes((a & U32(0xFFFF)) | (bb << 16), 0, 1)
        hi = jnp.swapaxes((a >> 16) | (bb & U32(0xFFFF0000)), 0, 1)
        for j in range(HG):
            rows = pl.ds(r0 + (2 * j // HG) * (DH2 // 2), 8)
            dst[slot, 2 * j % HG, rows, :] = lo[j]
            dst[slot, 2 * j % HG + 1, rows, :] = hi[j]

    NBLK = DH2 // 16
    with jax.named_scope("wait_w"):
        wait_chunk(0)

    def relayout0(b, c):
        relayout(0, wa_sc, 0, b)
        return c
    with jax.named_scope("relayout"):
        jax.lax.fori_loop(0, NBLK, relayout0, 0, unroll=2)

    def pro_stage(ps_, b):
        n = ps_ * NRB + b
        with jax.named_scope("wait_w"):
            if ps_ == 0:
                @pl.when(b + 1 < NRB)
                def _():
                    x_copy(b + 1).wait()

            @pl.when((n >= 2) & (n <= NCH))
            def _():
                wait_chunk(n - 1)
        cr = jnp.clip(n - 1, 0, NCH - 1)
        dst, slot = (wb_sc, cr) if ps_ == 0 else (wa_sc, cr - (NRB - 2))
        src, si = w_slot(ps_)
        bl = jnp.minimum(b + 1, NRB - 1)
        PW = PRO_PW
        npc = RB * S2 // PW
        assert npc * PW == RB * S2 and PRO_R0 + (NBLK - 1) * PRO_RS < HG * npc
        assert PRO_X0 + (max(RB, 2 * NT) - 1) * PRO_XS < HG * npc and 2 * NRB > 2 * NQ

        def body(i, c):
            s0 = b * RB + 1
            for sg in range(RB):
                hp_sc[sg * S2:(sg + 1) * S2, :] = xn_sc[s0 + sg, :, 0:DM]
            for j in range(HG):
                w = _unpack(src[si, j])
                for pi in range(npc):
                    pos = j * npc + pi
                    hx = hp_sc[pi * PW:(pi + 1) * PW, :]
                    k, rem = divmod(pos - PRO_X0, PRO_XS)
                    if ps_ == 0 and rem == 0 and 0 <= k < RB:
                        sn = bl * RB + 1 + k
                        xv = _pack(_ln(x_sc[seg(sn), LN].astype(F32)))
                        xn_sc[sn, :, 0:DM] = xv
                        hx = jnp.concatenate([hx[:-S2], jnp.where(never_sm[0] > 0, xv, hx[-S2:])], axis=0)
                    if ps_ == 1 and rem == 0 and 0 <= k < 2 * NT:
                        conv_u(jnp.minimum(2 * b + k // NT, 2 * NQ),
                               slice((k % NT) * 128, (k % NT + 1) * 128))
                    bb, rem = divmod(pos - PRO_R0, PRO_RS)
                    if rem == 0 and 0 <= bb < NBLK:
                        relayout(cr, dst, slot, bb)
                    r = _dot(_unpack(hx), w)
                    for a in range(0, 2 * PW, 16):
                        sg, off = divmod(2 * pi * PW + a, SEG)
                        pre_sc[s0 + sg, ps_ * HG + j, off:off + 16, :] = r[a:a + 16]
            return c
        with jax.named_scope("fused"):
            jax.lax.fori_loop(0, never_sm[0] + 1, body, 0)

    for ps_ in range(NPASS):
        if ps_ == 1:
            with jax.named_scope("wait_in0"):
                for cp in small + in_copies(0):
                    cp.wait()
            sh = sh_ref[...].astype(F32)
            for j in range(KS):
                co_sc[j] = jnp.broadcast_to(sh[j:j + 1], (8, DM))
            co_sc[KS] = jnp.broadcast_to(sd_ref[...].astype(F32).reshape(1, DM), (8, DM))

        def blk(b, c, ps_=ps_):
            pro_stage(ps_, b)
            return c
        jax.lax.fori_loop(0, NRB, blk, 0)

    def warm_block0(q):
        uf, kf = conv_fwd(0, q)
        put_spec(0, q, 0, uf)
        put_spec(0, q, 2, kf)
        kr_sc[q] = kf
        ur, um, kr, km = uf[:QB], uf[QB:], kf[:QB], kf[QB:]
        wf_sc[0, q, :QB] = (ur * kr - um * km).astype(BF16)
        wf_sc[0, q, QB:] = (ur * km + um * kr).astype(BF16)

    with jax.named_scope("warm"):
        for q in range(NQ):
            warm_block0(q)
    with jax.named_scope("wait_wo"):
        wo_copy.wait()
    with jax.named_scope("step0"):
        mem0 = mem0_ref[...].astype(F32)
        h0 = jnp.concatenate([jnp.concatenate([mem0, mem0], axis=0).astype(BF16), xn(0)], axis=0)

        def hook0(it):
            if it == 6:
                conv_spec(1, 0)
                for piece in MAC_PIECES:
                    conv_mac(1, 0, piece, 2)
            if it == 14:
                conv_inv(0)
        out = attend(lambda g: proj_split(h0, h0, g), RH, make_mask(RH, (0,)), DIST_HALF, hook0)
        finish(0, x_sc[0:SEG, LN], y_sc[0], jnp.concatenate([out[0:M], mem0], axis=0), out[M2:], False)

    mask12 = make_mask(R, (0, 1))

    def step(t, first, last):
        if first:
            conv_spec_later = functools.partial(conv_spec, t // NQ + 1, t % NQ)
        x4 = side2(t, op_sc[...])
        un = conv_u(t + 2 * NQ)
        hm = _unpack(h_sc[0:M, :])
        hx2 = _unpack(h_sc[M:, :])
        h48 = jnp.concatenate([hm, hx2], axis=0)
        x1n = pinned(xn(t), pin_tiles(PIN_U if first else PIN_U2, 1, un) + pin_tiles(PIN_X4, X4S, x4))

        def proj(g):
            h80 = jnp.concatenate([hm, x1n(g), hx2], axis=0)
            if g >= NPA + NPB:
                return proj_split(h80, h80, g)
            return proj_split(h48, h80, g, pre_sc[t, g] if g < NPA else fill_sc[g - NPA])

        held = {}

        def hook(it):
            if it == SPEC_AT:
                if first:
                    conv_spec_later()
                for piece in MAC_PIECES:
                    conv_mac(t // NQ + 1, t % NQ, piece, NB)
            if it == H:
                held["x"] = x_sc[seg(t), LN]
                held["y"] = y_sc[t & 3]
        out = attend(proj, R, mask12, DIST, hook)
        op_sc[...] = out[RH:]
        finish(t, held["x"], held["y"], out[0:M2], out[M2:RH], not last)

    def steps(i, carry):
        for j in range(UNROLL):
            step(1 + i * UNROLL + j, j == 0, j == UNROLL - 1)
        return carry

    def phase(p, carry):
        @pl.when(p == 1)
        def _():
            for cp in in_copies(2):
                cp.wait()

        @pl.when(p >= 2)
        def _():
            out_copy((p - 2) * PH, PH).start()

        with jax.named_scope("steps"):
            jax.lax.fori_loop(p * PHI, (p + 1) * PHI, steps, 0)
        return carry

    for cp in in_copies(1):
        cp.wait()
    jax.lax.fori_loop(0, NPH, phase, 0)
    out_copy((NPH - 2) * PH, NSEG - 2 - (NPH - 2) * PH).start()

    with jax.named_scope("step_last"):
        x4 = side2(NSEG, op_sc[...])
        hm = _unpack(h_sc[0:M, :])
        hx = pinned(_unpack(h_sc[M:, :]), pin_tiles(PIN_X4, 0, x4))
        out = attend(lambda g: proj_split(hx(g), jnp.concatenate([hm, hx(g)], axis=0), g),
                     SEG, make_mask(RH, (1,), M2), DIST_LAST)
        side2(NSEG + 1, out)
    out_copy(NSEG - 2, 2).start()
    out_copy(0, NSEG).wait()


def pallas_interleave_layers__memory_aug_recurrent_mem_tr__ssm_conv_h3__prompt_kernel(
    A_x, A_mem0, A_Wq, A_Wk, A_Wv, A_Wo, A_seg_len,
    B_q, B_k, B_v, B_shift_k, B_ssm_k, B_ssm_D,
):
    del B_q
    seg = int(A_seg_len) if isinstance(A_seg_len, (int, np.integer)) else CB // NQ
    return _run(A_x, A_mem0, A_Wq, A_Wk, A_Wv, A_Wo, B_k, B_v, B_shift_k, B_ssm_k, B_ssm_D, SEG=seg)


@functools.partial(jax.jit, static_argnames=("SEG",))
def _run(A_x, A_mem0, A_Wq, A_Wk, A_Wv, A_Wo, B_k, B_v, B_shift_k, B_ssm_k, B_ssm_D, *, SEG):
    B, S, DM = A_x.shape
    assert B == 1
    H, DH = A_Wq.shape[1], A_Wq.shape[2]
    M = A_mem0.shape[1]
    KS = B_shift_k.shape[1]
    R = 2 * (M + SEG)
    NSEG = S // SEG
    NRB = (NSEG - 1) // RB
    NB = S // CB
    QB = CB // NQ
    NCH = 3 * H // HG
    DP = -(-DM // 256) * 256
    fwd, inv = _dft_constants()

    kern = functools.partial(_kernel, S=S, DM=DM, H=H, DH=DH, M=M, SEG=SEG)
    any_spec = pl.BlockSpec(memory_space=pl.ANY)
    out = pl.pallas_call(
        kern,
        out_shape=jax.ShapeDtypeStruct((S, DM), A_x.dtype),
        in_specs=[any_spec] * 13,
        out_specs=any_spec,
        scratch_shapes=[
            pltpu.VMEM((NB + 2, NQ, QB // 8, DM // 128, 4, 8, 128), F32),
            pltpu.VMEM((NQ, 2 * QB, DM), F32),
            pltpu.VMEM((2, NQ, 2 * QB, DM), BF16),
            pltpu.VMEM((4, SEG, DM), F32),
            pltpu.VMEM((4, SEG, DM), F32),
            pltpu.VMEM((S, DP), BF16),
            pltpu.VMEM((SEG, DM), F32),
            pltpu.VMEM((NSEG, NPA, SEG, DH), F32),
            pltpu.VMEM((NPB, SEG, DH), F32),
            pltpu.VMEM((NSEG, SEG // 2, DP), U32),
            pltpu.VMEM((NCH - NRB + 2, HG, DM // 2, DH), U32),
            pltpu.VMEM((NRB - 1, HG, DM // 2, DH), U32),
            pltpu.VMEM((H * DH, DM), BF16),
            pltpu.VMEM((R // 2, H * DH), U32),
            pltpu.VMEM((S, DP), BF16),
            pltpu.VMEM((S, DP), BF16),
            pltpu.VMEM((NB, DM, CB), BF16),
            pltpu.VMEM((NCH, DM // 2, 2 * HG, DH), BF16),
            pltpu.VMEM((S, DP), A_x.dtype),
            pltpu.VMEM(fwd.shape, BF16),
            pltpu.VMEM(inv.shape, BF16),
            pltpu.VMEM((S + KPAD, DP), BF16),
            pltpu.VMEM((RB * SEG // 2, DM), U32),
            pltpu.VMEM((M + SEG // 2, DM), U32),
            pltpu.VMEM((KS + 1, 8, DM), F32),
            pltpu.VMEM((M, DM), BF16),
            pltpu.VMEM((KS, DM), BF16),
            pltpu.VMEM((DM,), BF16),
            pltpu.SMEM((1,), jnp.int32),
            pltpu.SemaphoreType.DMA(((NSEG - 1) // RB,)),
            pltpu.SemaphoreType.DMA((3,)),
            pltpu.SemaphoreType.DMA((NCH + 1,)),
            pltpu.SemaphoreType.DMA(()),
        ],
        compiler_params=pltpu.CompilerParams(vmem_limit_bytes=120 * 1024 * 1024),
    )(
        A_x.reshape(S, DM), A_mem0.reshape(M, DM), A_Wq, A_Wk, A_Wv,
        A_Wo.reshape(H * DH, DM), B_k.reshape(S, DM), B_v.reshape(S, DM),
        B_shift_k.T, B_ssm_k, B_ssm_D,
        jnp.asarray(fwd, BF16), jnp.asarray(inv, BF16),
    )
    return out.reshape(B, S, DM)
```

```python
import functools

import numpy as np
import jax
import jax.numpy as jnp
import jax.experimental.pallas as pl
import jax.experimental.pallas.tpu as pltpu

F32 = jnp.float32
BF16 = jnp.bfloat16
U32 = jnp.uint32

CB = 128
NQ = 4
KPAD = 16
HG = 8
NPA = 16
NPB = 12
RB = 9
PRO_PW, PRO_X0, PRO_XS, PRO_R0, PRO_RS = 24, 11, 4, 2, 2
UNROLL = 3
PHI = 3
PIN_U2, X4S = 1, 0
SPEC_AT, PIN_U, PIN_X4 = 7, 1, 16
DIST, DIST_HALF, DIST_LAST = (1, 2), (1, 3), (2, 3)


def _dft_constants():
    qb = CB // NQ
    n = np.arange(CB, dtype=np.float64)
    fwd = np.zeros((NQ, 2 * qb, CB))
    for q in range(NQ):
        f = q * qb + np.concatenate([np.arange(0, qb, 2), np.arange(1, qb, 2)])
        ang = (np.pi * (2.0 * f + 1.0) / (2 * CB))[:, None] * n[None, :]
        fwd[q, :qb] = np.cos(ang)
        fwd[q, qb:] = -np.sin(ang)
    inv = fwd.reshape(2 * CB, CB).T / CB
    return fwd.astype(np.float32), inv.reshape(NQ, CB // NQ, 2 * CB).astype(np.float32)


def _ln(x, eps=1e-5):
    d = x.shape[-1]
    m = jnp.sum(x, axis=-1, keepdims=True) * (1.0 / d)
    xc = x - m
    v = jnp.sum(xc * xc, axis=-1, keepdims=True) * (1.0 / d)
    return xc * jax.lax.rsqrt(v + eps)


def _dot(a, b):
    return jnp.dot(a, b, preferred_element_type=F32)


def _dot_nt(a, b):
    return jax.lax.dot_general(a, b, (((1,), (1,)), ((), ())), preferred_element_type=F32)


def _pack(x):
    return pltpu.bitcast(x.astype(BF16), U32)


def _unpack(x):
    return pltpu.bitcast(x, BF16)


def _in_order(actions):
    def body(i, c):
        for j, act in enumerate(actions):
            pl.when(i == j)(act)
        return c
    jax.lax.fori_loop(0, len(actions), body, 0)


def _kernel(x_hbm, mem0_hbm, wq_hbm, wk_hbm, wv_hbm, wo_hbm, k_hbm, v_hbm,
            sh_hbm, sk_hbm, sd_hbm, fwd_hbm, inv_hbm, o_hbm,
            sp_sc, kr_sc, wf_sc, x2_sc, y_sc, u_sc, op_sc, pre_sc, fill_sc, xn_sc, wa_sc, wb_sc, wo_sc, o_sc,
            x_sc, v_sc, sk_sc, st_sc, out_sc, fwd_ref, inv_ref,
            k_sc, hp_sc, h_sc, co_sc, mem0_ref, sh_ref, sd_ref,
            never_sm, sem_x, sem_in, sem_w, sem_out,
            *, S, DM, H, DH, M, SEG):
    NSEG = S // SEG
    M2 = 2 * M
    S2 = SEG // 2
    R = M2 + 2 * SEG
    RH = M2 + SEG
    NB = S // CB
    QB = CB // NQ
    HB = QB // 2
    NT = DM // 128
    PH = PHI * UNROLL
    NRB = (NSEG - 1) // RB
    NPH = (NSEG - 1) // PH
    NG = H // HG
    NCH = 3 * NG
    NPASS = NPA // HG
    DH2 = DM // 2
    KS = sh_ref.shape[0]
    LN = pl.ds(0, DM)
    assert 2 <= KS <= 8 and QB == SEG and NRB * RB == NSEG - 1 and NPH * PH == NSEG - 1 and NPASS == 2 and 2 * NRB >= NCH + 1

    mem0_copy = pltpu.make_async_copy(mem0_hbm, mem0_ref, sem_x.at[0])
    small = [pltpu.make_async_copy(s, d, sem_in.at[0]) for s, d in [
        (sh_hbm, sh_ref), (sd_hbm, sd_ref), (fwd_hbm, fwd_ref), (inv_hbm, inv_ref)]]

    def x_copy(b):
        if isinstance(b, int) and b == 0:
            rows = pl.ds(0, (RB + 1) * SEG)
        else:
            rows = pl.ds(pl.multiple_of((b * RB + 1) * SEG, SEG), RB * SEG)
        return pltpu.make_async_copy(x_hbm.at[rows], x_sc.at[rows, LN], sem_x.at[b])

    kb = (0, (2 * NQ + 1) * SEG, (2 * NQ + PH + 1) * SEG, S)
    sb = (0, 2, (PH + 1) // NQ + 2, NB)

    def in_copies(part):
        def rng(b):
            return pl.ds(b[part], b[part + 1] - b[part])
        sem = sem_in.at[part]
        return [
            pltpu.make_async_copy(k_hbm.at[rng(kb)],
                                  k_sc.at[pl.ds(KPAD + kb[part], kb[part + 1] - kb[part]), LN], sem),
            pltpu.make_async_copy(v_hbm.at[rng(kb)], v_sc.at[rng(kb), LN], sem),
        ] + [pltpu.make_async_copy(sk_hbm.at[:, pl.ds(c * CB, CB)], sk_sc.at[c], sem)
             for c in range(sb[part], sb[part + 1])]

    def w_copies(ci, dst=None):
        src = (wq_hbm, wk_hbm, wv_hbm)[ci // NG]
        dst = ci if dst is None else dst
        return [pltpu.make_async_copy(src.at[pl.ds(hf * DH2, DH2), pl.ds((ci % NG) * HG, HG), :],
                                      st_sc.at[dst, :, pl.ds(hf * HG, HG), :], sem_w.at[dst])
                for hf in range(2)]

    wo_copy = pltpu.make_async_copy(wo_hbm, wo_sc, sem_w.at[NCH])

    def out_copy(lo, n):
        rows = pl.ds(lo * SEG if isinstance(lo, int) else pl.multiple_of(lo * SEG, SEG), n * SEG)
        return pltpu.make_async_copy(out_sc.at[rows, LN], o_hbm.at[rows], sem_out)

    def start_all(cps):
        def act():
            for cp in cps:
                cp.start()
        return act

    order = [[mem0_copy, x_copy(0)], w_copies(0), [x_copy(1)], [x_copy(2)]]
    for ci in range(1, NCH):
        order.append(w_copies(ci) + ([x_copy(ci + 2)] if ci + 2 < NRB else []))
        if ci == NRB - 2:
            order.append(small + in_copies(0))
    order += [[wo_copy], in_copies(1), in_copies(2)]
    for i in range(0, len(order), 5):
        _in_order([start_all(cps) for cps in order[i:i + 5]])

    never_sm[0] = 0
    k_sc[0:KPAD, LN] = jnp.zeros((KPAD, DM), BF16)
    sp_sc[NB + 1] = jnp.zeros(sp_sc.shape[1:], F32)
    op_sc[...] = jnp.zeros(op_sc.shape, F32)
    x2_sc[...] = jnp.zeros(x2_sc.shape, F32)
    y_sc[...] = jnp.zeros(y_sc.shape, F32)
    mem0_copy.wait()
    x_copy(0).wait()
    for sg in range(RB + 1):
        xn_sc[sg, :, 0:DM] = _pack(_ln(x_sc[sg * SEG:(sg + 1) * SEG, LN].astype(F32)))

    def clip(i, hi):
        return min(max(i, 0), hi) if isinstance(i, int) else jnp.clip(i, 0, hi)

    def scaled(i, m):
        return i * m if isinstance(i, int) else pl.multiple_of(i * m, m)

    def seg(i):
        return pl.ds(scaled(clip(i, NSEG - 1), SEG), SEG)

    def conv_u(s, ln=LN):
        r0 = scaled(clip(s, NSEG - 1), SEG)
        kk = k_sc[pl.ds(r0, KPAD + SEG), ln].astype(F32)[KPAD - 8:]

        def coef(j, rows):
            return jnp.concatenate([co_sc[j, :, ln]] * (rows // 8), axis=0)
        sft = [kk] + [pltpu.roll(kk, j, 0) for j in range(2, KS, 2)]
        ev = functools.reduce(jnp.add, [sft[j // 2][8:] * coef(j, SEG) for j in range(0, KS, 2)])
        od = functools.reduce(jnp.add, [sft[j // 2] * coef(j, SEG + 8) for j in range(1, KS, 2)])
        ks = ev + pltpu.roll(od, 1, 0)[8:]
        u = (ks * v_sc[pl.ds(r0, SEG), ln].astype(F32)).astype(BF16)
        u_sc[pl.ds(r0, SEG), ln] = u
        return u

    def conv_fwd(c, q):
        cc = clip(c, NB - 1)
        f = fwd_ref[q]
        uf = _dot(f, u_sc[pl.ds(scaled(cc, CB), CB), LN])
        kf = _dot_nt(f, sk_sc[cc])
        return uf, kf

    def put_spec(cs, q, which, val):
        for rb in range(QB // 8):
            for n in range(NT):
                ln = slice(n * 128, (n + 1) * 128)
                sp_sc[cs, q, rb, n, which] = val[rb * 8:rb * 8 + 8, ln]
                sp_sc[cs, q, rb, n, which + 1] = val[QB + rb * 8:QB + rb * 8 + 8, ln]

    def conv_spec(c, q):
        uf, kf = conv_fwd(c, q)
        cs = clip(c, NB)
        put_spec(cs, q, 0, uf)
        pk = kr_sc[q]
        kr_sc[q] = kf
        kp = jnp.concatenate([
            kf[0:HB] - pk[QB:QB + HB],
            kf[HB:QB] + pk[QB + HB:],
            kf[QB:QB + HB] + pk[0:HB],
            kf[QB + HB:] - pk[HB:QB]], axis=0)
        put_spec(cs, q, 2, kp)

    MAC_PIECES = [(rb, n) for rb in range(QB // 16) for n in range(NT)]

    def conv_mac(c, q, piece, nterms):
        rb2, n = piece
        cs = clip(c, NB)
        acc = []
        for rb in (2 * rb2, 2 * rb2 + 1):
            ar = None
            ai = None
            for j in range(nterms):
                if isinstance(cs, int):
                    uj, kj = j, cs - j
                else:
                    uj = jnp.minimum(j, cs)
                    kj = jnp.where(cs - j >= 0, cs - j, NB + 1)
                ur = sp_sc[uj, q, rb, n, 0]
                um = sp_sc[uj, q, rb, n, 1]
                kr = sp_sc[kj, q, rb, n, 2]
                km = sp_sc[kj, q, rb, n, 3]
                tr = ur * kr - um * km
                ti = ur * km + um * kr
                ar = tr if ar is None else ar + tr
                ai = ti if ai is None else ai + ti
            acc.append((ar, ai))
        ln = slice(n * 128, (n + 1) * 128)
        w = jnp.concatenate([acc[0][0], acc[1][0], acc[0][1], acc[1][1]], axis=0).astype(BF16)
        wf_sc[c & 1, q, rb2 * 16:rb2 * 16 + 16, ln] = w[0:16]
        wf_sc[c & 1, q, QB + rb2 * 16:QB + rb2 * 16 + 16, ln] = w[16:]

    def conv_inv(s):
        w = wf_sc[(s // NQ) & 1].reshape(2 * CB, DM)
        yc = _dot(inv_ref[s % NQ], w)
        sd = jnp.concatenate([co_sc[KS]] * (SEG // 8), axis=0)
        y_sc[s & 3] = yc + u_sc[seg(s), LN].astype(F32) * sd

    scale = DH ** -0.5
    cexp = scale * float(np.log2(np.e))

    def make_mask(n, x_layers, q0=0):
        qi = jax.lax.broadcasted_iota(jnp.int32, (n - q0, n), 0) + q0
        ki = jax.lax.broadcasted_iota(jnp.int32, (n - q0, n), 1)

        def layer(i):
            xl = jnp.where(i < M2 + SEG, x_layers[0], x_layers[-1])
            return jnp.where(i < M, 0, jnp.where(i < M2, 1, xl))
        same = layer(qi) == layer(ki)
        ok = same & ((qi < M2) | (ki < M2) | (qi >= ki))
        fill = jnp.where(same, -1e9 / scale, -jnp.inf).astype(F32)
        return ok, fill

    def probs(q, k, mask):
        ok, fill = mask
        s = _dot_nt(q, k)
        s = jnp.where(ok, s, fill)
        m = jnp.max(s, axis=-1, keepdims=True)
        p = jnp.exp2((s - m) * cexp)
        l = jnp.sum(p, axis=-1, keepdims=True)
        r = pl.reciprocal(l, approx=True)
        r = r * (2.0 - l * r)
        return (p * r).astype(BF16)

    def w_slot(ci):
        return (wb_sc, ci) if 1 <= ci < NRB - 1 else (wa_sc, max(ci - (NRB - 2), 0))

    def w_head(g, mats):
        slots = [w_slot(mi * NG + g // HG) for mi in mats]
        return _unpack(jnp.concatenate([ref[i, g % HG] for ref, i in slots], axis=1))

    def proj_split(hq, hkv, g, q1=None):
        q = _dot(hq, w_head(g, (0,)))
        kv = _dot(hkv, w_head(g, (1, 2)))
        if q1 is not None:
            q = jnp.concatenate([q[0:M2], q1, q[M2:]], axis=0)
        return q.astype(BF16), kv[:, :DH].astype(BF16), kv[:, DH:].astype(BF16)

    def xn(s):
        return _unpack(xn_sc[clip(s, NSEG - 1), :, 0:DM])

    def out_proj(n, g0, g1, j):
        return _dot(_unpack(o_sc[0:n // 2, g0 * DH:g1 * DH]),
                    wo_sc[g0 * DH:g1 * DH, j * 128:(j + 1) * 128])

    def attend(proj, n, mask, dist, hook=None):
        D1, D2 = dist
        HA = H - D1 - D2 - 1
        NE = min(D1 + D2, NT - 1)
        qkvs = {}
        ps = {}
        outs = {}
        for it in range(H + D1 + D2):
            if it < H:
                qkvs[it] = proj(it)
            g = it - D1
            if 0 <= g < H:
                ps[g] = probs(qkvs[g][0], qkvs[g][1], mask)
            g = it - D1 - D2
            if 0 <= g < H:
                o = _dot(ps.pop(g), qkvs.pop(g)[2])
                o_sc[0:n // 2, g * DH:(g + 1) * DH] = _pack(o)
            if hook is not None:
                hook(it)
            j = it - (H - 1)
            if 0 <= j < NE:
                outs[j] = out_proj(n, 0, HA, j)
        for j in range(NE, NT):
            outs[j] = out_proj(n, 0, H, j)
        for j in range(NE):
            outs[j] = out_proj(n, HA, H, j) + outs[j]
        return jnp.concatenate([outs[j] for j in range(NT)], axis=1)

    def side2(t, a2):
        x3 = x2_sc[(t - 2) & 3] + a2
        x4 = x3 + _ln(x3) * y_sc[(t - 2) & 3]
        x4 = x4.astype(out_sc.dtype)
        out_sc[seg(t - 2), LN] = x4
        return x4

    def finish(t, xr, yt, mem, a1, spec):
        if spec:
            conv_spec((t + 1) // NQ + 1, (t + 1) % NQ)
        xq = xn(t + 1)
        for g in range(NPA, NPA + NPB):
            fill_sc[g - NPA] = _dot(xq, w_head(g, (0,)))
        conv_inv(t + 1)
        x1 = xr.astype(F32) + a1
        x2 = x1 + _ln(x1) * yt
        h_sc[0:M, :] = _pack(mem)
        h_sc[M:, :] = _pack(_ln(x2))
        x2_sc[t & 3] = x2

    def pinned(rows, pins):
        never = never_sm[0] > 0
        hs = {0: rows}
        r = _pack(rows)
        tiles = [r[:, n * 128:(n + 1) * 128] for n in range(NT)]
        for g, n, d in sorted(pins, key=lambda p: p[0]):
            tiles[n] = jnp.where(never, d, tiles[n])
            hs[g] = _unpack(jnp.concatenate(tiles, axis=1))
        return lambda g: hs[max(k for k in hs if k <= g)]

    def pin_tiles(g0, stride, val):
        v = _pack(val)
        return [(g0 + n * stride, n, v[:, n * 128:(n + 1) * 128]) for n in range(NT)]

    def wait_chunk(ci):
        for cp in w_copies(0, ci):
            cp.wait()

    def relayout(ci, dst, slot, b):
        d0 = scaled(b, 16)
        r0 = scaled(b, 8)
        xw = pltpu.bitcast(st_sc[ci, pl.ds(d0, 16)], U32).reshape(8, 2, HG, DH)
        a = xw[:, 0]
        bb = xw[:, 1]
        lo = jnp.swapaxes((a & U32(0xFFFF)) | (bb << 16), 0, 1)
        hi = jnp.swapaxes((a >> 16) | (bb & U32(0xFFFF0000)), 0, 1)
        for j in range(HG):
            rows = pl.ds(r0 + (2 * j // HG) * (DH2 // 2), 8)
            dst[slot, 2 * j % HG, rows, :] = lo[j]
            dst[slot, 2 * j % HG + 1, rows, :] = hi[j]

    def everything(_, carry):
        NBLK = DH2 // 16
        with jax.named_scope("wait_w"):
            wait_chunk(0)

        def relayout0(b, c):
            relayout(0, wa_sc, 0, b)
            return c
        with jax.named_scope("relayout"):
            jax.lax.fori_loop(0, NBLK, relayout0, 0, unroll=2)

        def pro_stage(ps_, b):
            n = ps_ * NRB + b
            with jax.named_scope("wait_w"):
                if ps_ == 0:
                    @pl.when(b + 1 < NRB)
                    def _():
                        x_copy(b + 1).wait()

                @pl.when((n >= 2) & (n <= NCH))
                def _():
                    wait_chunk(n - 1)
            cr = jnp.clip(n - 1, 0, NCH - 1)
            dst, slot = (wb_sc, cr) if ps_ == 0 else (wa_sc, cr - (NRB - 2))
            src, si = w_slot(ps_)
            bl = jnp.minimum(b + 1, NRB - 1)
            PW = PRO_PW
            npc = RB * S2 // PW
            assert npc * PW == RB * S2 and PRO_R0 + (NBLK - 1) * PRO_RS < HG * npc
            assert PRO_X0 + (max(RB, 2 * NT) - 1) * PRO_XS < HG * npc and 2 * NRB > 2 * NQ

            def body(i, c):
                s0 = b * RB + 1
                for sg in range(RB):
                    hp_sc[sg * S2:(sg + 1) * S2, :] = xn_sc[s0 + sg, :, 0:DM]
                for j in range(HG):
                    w = _unpack(src[si, j])
                    for pi in range(npc):
                        pos = j * npc + pi
                        hx = hp_sc[pi * PW:(pi + 1) * PW, :]
                        k, rem = divmod(pos - PRO_X0, PRO_XS)
                        if ps_ == 0 and rem == 0 and 0 <= k < RB:
                            sn = bl * RB + 1 + k
                            xv = _pack(_ln(x_sc[seg(sn), LN].astype(F32)))
                            xn_sc[sn, :, 0:DM] = xv
                            hx = jnp.concatenate([hx[:-S2], jnp.where(never_sm[0] > 0, xv, hx[-S2:])], axis=0)
                        if ps_ == 1 and rem == 0 and 0 <= k < 2 * NT:
                            conv_u(jnp.minimum(2 * b + k // NT, 2 * NQ),
                                   slice((k % NT) * 128, (k % NT + 1) * 128))
                        bb, rem = divmod(pos - PRO_R0, PRO_RS)
                        if rem == 0 and 0 <= bb < NBLK:
                            relayout(cr, dst, slot, bb)
                        r = _dot(_unpack(hx), w)
                        for a in range(0, 2 * PW, 16):
                            sg, off = divmod(2 * pi * PW + a, SEG)
                            pre_sc[s0 + sg, ps_ * HG + j, off:off + 16, :] = r[a:a + 16]
                return c
            with jax.named_scope("fused"):
                jax.lax.fori_loop(0, never_sm[0] + 1, body, 0)

        for ps_ in range(NPASS):
            if ps_ == 1:
                with jax.named_scope("wait_in0"):
                    for cp in small + in_copies(0):
                        cp.wait()
                sh = sh_ref[...].astype(F32)
                for j in range(KS):
                    co_sc[j] = jnp.broadcast_to(sh[j:j + 1], (8, DM))
                co_sc[KS] = jnp.broadcast_to(sd_ref[...].astype(F32).reshape(1, DM), (8, DM))

            def blk(b, c, ps_=ps_):
                pro_stage(ps_, b)
                return c
            jax.lax.fori_loop(0, NRB, blk, 0)

        def warm_block0(q):
            uf, kf = conv_fwd(0, q)
            put_spec(0, q, 0, uf)
            put_spec(0, q, 2, kf)
            kr_sc[q] = kf
            ur, um, kr, km = uf[:QB], uf[QB:], kf[:QB], kf[QB:]
            wf_sc[0, q, :QB] = (ur * kr - um * km).astype(BF16)
            wf_sc[0, q, QB:] = (ur * km + um * kr).astype(BF16)

        with jax.named_scope("warm"):
            for q in range(NQ):
                warm_block0(q)
        with jax.named_scope("wait_wo"):
            wo_copy.wait()
        with jax.named_scope("step0"):
            mem0 = mem0_ref[...].astype(F32)
            h0 = jnp.concatenate([jnp.concatenate([mem0, mem0], axis=0).astype(BF16), xn(0)], axis=0)

            def hook0(it):
                if it == 6:
                    conv_spec(1, 0)
                    for piece in MAC_PIECES:
                        conv_mac(1, 0, piece, 2)
                if it == 14:
                    conv_inv(0)
            out = attend(lambda g: proj_split(h0, h0, g), RH, make_mask(RH, (0,)), DIST_HALF, hook0)
            finish(0, x_sc[0:SEG, LN], y_sc[0], jnp.concatenate([out[0:M], mem0], axis=0), out[M2:], False)

        mask12 = make_mask(R, (0, 1))

        def step(t, first, last):
            if first:
                conv_spec_later = functools.partial(conv_spec, t // NQ + 1, t % NQ)
            x4 = side2(t, op_sc[...])
            un = conv_u(t + 2 * NQ)
            hm = _unpack(h_sc[0:M, :])
            hx2 = _unpack(h_sc[M:, :])
            h48 = jnp.concatenate([hm, hx2], axis=0)
            x1n = pinned(xn(t), pin_tiles(PIN_U if first else PIN_U2, 1, un) + pin_tiles(PIN_X4, X4S, x4))

            def proj(g):
                h80 = jnp.concatenate([hm, x1n(g), hx2], axis=0)
                if g >= NPA + NPB:
                    return proj_split(h80, h80, g)
                return proj_split(h48, h80, g, pre_sc[t, g] if g < NPA else fill_sc[g - NPA])

            held = {}

            def hook(it):
                if it == SPEC_AT:
                    if first:
                        conv_spec_later()
                    for piece in MAC_PIECES:
                        conv_mac(t // NQ + 1, t % NQ, piece, NB)
                if it == H:
                    held["x"] = x_sc[seg(t), LN]
                    held["y"] = y_sc[t & 3]
            out = attend(proj, R, mask12, DIST, hook)
            op_sc[...] = out[RH:]
            finish(t, held["x"], held["y"], out[0:M2], out[M2:RH], not last)

        def steps(i, carry):
            for j in range(UNROLL):
                step(1 + i * UNROLL + j, j == 0, j == UNROLL - 1)
            return carry

        def phase(p, carry):
            @pl.when(p == 1)
            def _():
                for cp in in_copies(2):
                    cp.wait()

            @pl.when(p >= 2)
            def _():
                out_copy((p - 2) * PH, PH).start()

            with jax.named_scope("steps"):
                jax.lax.fori_loop(p * PHI, (p + 1) * PHI, steps, 0)
            return carry

        for cp in in_copies(1):
            cp.wait()
        jax.lax.fori_loop(0, NPH, phase, 0)
        out_copy((NPH - 2) * PH, NSEG - 2 - (NPH - 2) * PH).start()

        with jax.named_scope("step_last"):
            x4 = side2(NSEG, op_sc[...])
            hm = _unpack(h_sc[0:M, :])
            hx = pinned(_unpack(h_sc[M:, :]), pin_tiles(PIN_X4, 0, x4))
            out = attend(lambda g: proj_split(hx(g), jnp.concatenate([hm, hx(g)], axis=0), g),
                         SEG, make_mask(RH, (1,), M2), DIST_LAST)
            side2(NSEG + 1, out)
        out_copy(NSEG - 2, 2).start()
        out_copy(0, NSEG).wait()
        return carry

    jax.lax.fori_loop(0, never_sm[0] + 1, everything, 0)


def pallas_interleave_layers__memory_aug_recurrent_mem_tr__ssm_conv_h3__prompt_kernel(
    A_x, A_mem0, A_Wq, A_Wk, A_Wv, A_Wo, A_seg_len,
    B_q, B_k, B_v, B_shift_k, B_ssm_k, B_ssm_D,
):
    del B_q
    seg = int(A_seg_len) if isinstance(A_seg_len, (int, np.integer)) else CB // NQ
    return _run(A_x, A_mem0, A_Wq, A_Wk, A_Wv, A_Wo, B_k, B_v, B_shift_k, B_ssm_k, B_ssm_D, SEG=seg)


@functools.partial(jax.jit, static_argnames=("SEG",))
def _run(A_x, A_mem0, A_Wq, A_Wk, A_Wv, A_Wo, B_k, B_v, B_shift_k, B_ssm_k, B_ssm_D, *, SEG):
    B, S, DM = A_x.shape
    assert B == 1
    H, DH = A_Wq.shape[1], A_Wq.shape[2]
    M = A_mem0.shape[1]
    KS = B_shift_k.shape[1]
    R = 2 * (M + SEG)
    NSEG = S // SEG
    NRB = (NSEG - 1) // RB
    NB = S // CB
    QB = CB // NQ
    NCH = 3 * H // HG
    DP = -(-DM // 256) * 256
    fwd, inv = _dft_constants()

    kern = functools.partial(_kernel, S=S, DM=DM, H=H, DH=DH, M=M, SEG=SEG)
    any_spec = pl.BlockSpec(memory_space=pl.ANY)
    out = pl.pallas_call(
        kern,
        out_shape=jax.ShapeDtypeStruct((S, DM), A_x.dtype),
        in_specs=[any_spec] * 13,
        out_specs=any_spec,
        scratch_shapes=[
            pltpu.VMEM((NB + 2, NQ, QB // 8, DM // 128, 4, 8, 128), F32),
            pltpu.VMEM((NQ, 2 * QB, DM), F32),
            pltpu.VMEM((2, NQ, 2 * QB, DM), BF16),
            pltpu.VMEM((4, SEG, DM), F32),
            pltpu.VMEM((4, SEG, DM), F32),
            pltpu.VMEM((S, DP), BF16),
            pltpu.VMEM((SEG, DM), F32),
            pltpu.VMEM((NSEG, NPA, SEG, DH), F32),
            pltpu.VMEM((NPB, SEG, DH), F32),
            pltpu.VMEM((NSEG, SEG // 2, DP), U32),
            pltpu.VMEM((NCH - NRB + 2, HG, DM // 2, DH), U32),
            pltpu.VMEM((NRB - 1, HG, DM // 2, DH), U32),
            pltpu.VMEM((H * DH, DM), BF16),
            pltpu.VMEM((R // 2, H * DH), U32),
            pltpu.VMEM((S, DP), BF16),
            pltpu.VMEM((S, DP), BF16),
            pltpu.VMEM((NB, DM, CB), BF16),
            pltpu.VMEM((NCH, DM // 2, 2 * HG, DH), BF16),
            pltpu.VMEM((S, DP), A_x.dtype),
            pltpu.VMEM(fwd.shape, BF16),
            pltpu.VMEM(inv.shape, BF16),
            pltpu.VMEM((S + KPAD, DP), BF16),
            pltpu.VMEM((RB * SEG // 2, DM), U32),
            pltpu.VMEM((M + SEG // 2, DM), U32),
            pltpu.VMEM((KS + 1, 8, DM), F32),
            pltpu.VMEM((M, DM), BF16),
            pltpu.VMEM((KS, DM), BF16),
            pltpu.VMEM((DM,), BF16),
            pltpu.SMEM((1,), jnp.int32),
            pltpu.SemaphoreType.DMA(((NSEG - 1) // RB,)),
            pltpu.SemaphoreType.DMA((3,)),
            pltpu.SemaphoreType.DMA((NCH + 1,)),
            pltpu.SemaphoreType.DMA(()),
        ],
        compiler_params=pltpu.CompilerParams(vmem_limit_bytes=120 * 1024 * 1024),
    )(
        A_x.reshape(S, DM), A_mem0.reshape(M, DM), A_Wq, A_Wk, A_Wv,
        A_Wo.reshape(H * DH, DM), B_k.reshape(S, DM), B_v.reshape(S, DM),
        B_shift_k.T, B_ssm_k, B_ssm_D,
        jnp.asarray(fwd, BF16), jnp.asarray(inv, BF16),
    )
    return out.reshape(B, S, DM)
```

```python
import functools

import numpy as np
import jax
import jax.numpy as jnp
import jax.experimental.pallas as pl
import jax.experimental.pallas.tpu as pltpu

F32 = jnp.float32
BF16 = jnp.bfloat16
U32 = jnp.uint32

CB = 128
NQ = 4
KPAD = 16
HG = 8
NPA = 16
NPB = 12
RB = 9
PRO_PW, PRO_X0, PRO_XS, PRO_R0, PRO_RS = 24, 11, 4, 2, 2
UNROLL = 3
PHI = 3
PIN_U2, X4S = 1, 0
SPEC_AT, PIN_U, PIN_X4 = 7, 1, 16
DIST, DIST_HALF, DIST_LAST = (1, 2), (1, 3), (2, 3)


def _dft_constants():
    qb = CB // NQ
    n = np.arange(CB, dtype=np.float64)
    fwd = np.zeros((NQ, 2 * qb, CB))
    for q in range(NQ):
        f = q * qb + np.concatenate([np.arange(0, qb, 2), np.arange(1, qb, 2)])
        ang = (np.pi * (2.0 * f + 1.0) / (2 * CB))[:, None] * n[None, :]
        fwd[q, :qb] = np.cos(ang)
        fwd[q, qb:] = -np.sin(ang)
    inv = fwd.reshape(2 * CB, CB).T / CB
    return fwd.astype(np.float32), inv.reshape(NQ, CB // NQ, 2 * CB).astype(np.float32)


def _ln(x, eps=1e-5):
    d = x.shape[-1]
    m = jnp.sum(x, axis=-1, keepdims=True) * (1.0 / d)
    xc = x - m
    v = jnp.sum(xc * xc, axis=-1, keepdims=True) * (1.0 / d)
    return xc * jax.lax.rsqrt(v + eps)


def _dot(a, b):
    return jnp.dot(a, b, preferred_element_type=F32)


def _dot_nt(a, b):
    return jax.lax.dot_general(a, b, (((1,), (1,)), ((), ())), preferred_element_type=F32)


def _pack(x):
    return pltpu.bitcast(x.astype(BF16), U32)


def _unpack(x):
    return pltpu.bitcast(x, BF16)


def _in_order(actions):
    def body(i, c):
        for j, act in enumerate(actions):
            pl.when(i == j)(act)
        return c
    jax.lax.fori_loop(0, len(actions), body, 0)


def _kernel(x_hbm, mem0_hbm, wq_hbm, wk_hbm, wv_hbm, wo_hbm, k_hbm, v_hbm,
            sh_hbm, sk_hbm, sd_hbm, fwd_hbm, inv_hbm, o_hbm,
            sp_sc, kr_sc, wf_sc, x2_sc, y_sc, u_sc, op_sc, pre_sc, fill_sc, xn_sc, wa_sc, wb_sc, wo_sc, o_sc,
            x_sc, v_sc, sk_sc, st_sc, out_sc, fwd_ref, inv_ref,
            k_sc, hp_sc, h_sc, co_sc, mem0_ref, sh_ref, sd_ref,
            never_sm, sem_x, sem_in, sem_w, sem_out,
            *, S, DM, H, DH, M, SEG):
    NSEG = S // SEG
    M2 = 2 * M
    S2 = SEG // 2
    R = M2 + 2 * SEG
    RH = M2 + SEG
    NB = S // CB
    QB = CB // NQ
    HB = QB // 2
    NT = DM // 128
    PH = PHI * UNROLL
    NRB = (NSEG - 1) // RB
    NPH = (NSEG - 1) // PH
    NG = H // HG
    NCH = 3 * NG
    NPASS = NPA // HG
    DH2 = DM // 2
    KS = sh_ref.shape[0]
    LN = pl.ds(0, DM)
    assert 2 <= KS <= 8 and QB == SEG and NRB * RB == NSEG - 1 and NPH * PH == NSEG - 1 and NPASS == 2 and 2 * NRB >= NCH + 1

    mem0_copy = pltpu.make_async_copy(mem0_hbm, mem0_ref, sem_x.at[0])
    small = [pltpu.make_async_copy(s, d, sem_in.at[0]) for s, d in [
        (sh_hbm, sh_ref), (sd_hbm, sd_ref), (fwd_hbm, fwd_ref), (inv_hbm, inv_ref)]]

    def x_copy(b):
        if isinstance(b, int) and b == 0:
            rows = pl.ds(0, (RB + 1) * SEG)
        else:
            rows = pl.ds(pl.multiple_of((b * RB + 1) * SEG, SEG), RB * SEG)
        return pltpu.make_async_copy(x_hbm.at[rows], x_sc.at[rows, LN], sem_x.at[b])

    kb = (0, (2 * NQ + 1) * SEG, (2 * NQ + PH + 1) * SEG, S)
    sb = (0, 2, (PH + 1) // NQ + 2, NB)

    def in_copies(part):
        def rng(b):
            return pl.ds(b[part], b[part + 1] - b[part])
        sem = sem_in.at[part]
        return [
            pltpu.make_async_copy(k_hbm.at[rng(kb)],
                                  k_sc.at[pl.ds(KPAD + kb[part], kb[part + 1] - kb[part]), LN], sem),
            pltpu.make_async_copy(v_hbm.at[rng(kb)], v_sc.at[rng(kb), LN], sem),
        ] + [pltpu.make_async_copy(sk_hbm.at[:, pl.ds(c * CB, CB)], sk_sc.at[c], sem)
             for c in range(sb[part], sb[part + 1])]

    def w_copies(ci, dst=None, part=None):
        src = (wq_hbm, wk_hbm, wv_hbm)[ci // NG]
        dst = ci if dst is None else dst
        lo, n = (0, DH2) if part is None else (part * DH2 // 2, DH2 // 2)
        sem = sem_w.at[NCH + 1 if part == 1 else dst]
        return [pltpu.make_async_copy(src.at[pl.ds(hf * DH2 + lo, n), pl.ds((ci % NG) * HG, HG), :],
                                      st_sc.at[dst, pl.ds(lo, n), pl.ds(hf * HG, HG), :], sem)
                for hf in range(2)]

    wo_copy = pltpu.make_async_copy(wo_hbm, wo_sc, sem_w.at[NCH])

    def out_copy(lo, n):
        rows = pl.ds(lo * SEG if isinstance(lo, int) else pl.multiple_of(lo * SEG, SEG), n * SEG)
        return pltpu.make_async_copy(out_sc.at[rows, LN], o_hbm.at[rows], sem_out)

    def start_all(cps):
        def act():
            for cp in cps:
                cp.start()
        return act

    order = [[mem0_copy, x_copy(0)], w_copies(0, part=0), w_copies(0, part=1), [x_copy(1)], [x_copy(2)]]
    for ci in range(1, NCH):
        order.append(w_copies(ci) + ([x_copy(ci + 2)] if ci + 2 < NRB else []))
        if ci == NRB - 2:
            order.append(small + in_copies(0))
    order += [[wo_copy], in_copies(1), in_copies(2)]
    for i in range(0, len(order), 5):
        _in_order([start_all(cps) for cps in order[i:i + 5]])

    never_sm[0] = 0
    k_sc[0:KPAD, LN] = jnp.zeros((KPAD, DM), BF16)
    sp_sc[NB + 1] = jnp.zeros(sp_sc.shape[1:], F32)
    op_sc[...] = jnp.zeros(op_sc.shape, F32)
    x2_sc[...] = jnp.zeros(x2_sc.shape, F32)
    y_sc[...] = jnp.zeros(y_sc.shape, F32)
    mem0_copy.wait()
    x_copy(0).wait()
    for sg in range(RB + 1):
        xn_sc[sg, :, 0:DM] = _pack(_ln(x_sc[sg * SEG:(sg + 1) * SEG, LN].astype(F32)))

    def clip(i, hi):
        return min(max(i, 0), hi) if isinstance(i, int) else jnp.clip(i, 0, hi)

    def scaled(i, m):
        return i * m if isinstance(i, int) else pl.multiple_of(i * m, m)

    def seg(i):
        return pl.ds(scaled(clip(i, NSEG - 1), SEG), SEG)

    def conv_u(s, ln=LN):
        r0 = scaled(clip(s, NSEG - 1), SEG)
        kk = k_sc[pl.ds(r0, KPAD + SEG), ln].astype(F32)[KPAD - 8:]

        def coef(j, rows):
            return jnp.concatenate([co_sc[j, :, ln]] * (rows // 8), axis=0)
        sft = [kk] + [pltpu.roll(kk, j, 0) for j in range(2, KS, 2)]
        ev = functools.reduce(jnp.add, [sft[j // 2][8:] * coef(j, SEG) for j in range(0, KS, 2)])
        od = functools.reduce(jnp.add, [sft[j // 2] * coef(j, SEG + 8) for j in range(1, KS, 2)])
        ks = ev + pltpu.roll(od, 1, 0)[8:]
        u = (ks * v_sc[pl.ds(r0, SEG), ln].astype(F32)).astype(BF16)
        u_sc[pl.ds(r0, SEG), ln] = u
        return u

    def conv_fwd(c, q):
        cc = clip(c, NB - 1)
        f = fwd_ref[q]
        uf = _dot(f, u_sc[pl.ds(scaled(cc, CB), CB), LN])
        kf = _dot_nt(f, sk_sc[cc])
        return uf, kf

    def put_spec(cs, q, which, val):
        for rb in range(QB // 8):
            for n in range(NT):
                ln = slice(n * 128, (n + 1) * 128)
                sp_sc[cs, q, rb, n, which] = val[rb * 8:rb * 8 + 8, ln]
                sp_sc[cs, q, rb, n, which + 1] = val[QB + rb * 8:QB + rb * 8 + 8, ln]

    def conv_spec(c, q):
        uf, kf = conv_fwd(c, q)
        cs = clip(c, NB)
        put_spec(cs, q, 0, uf)
        pk = kr_sc[q]
        kr_sc[q] = kf
        kp = jnp.concatenate([
            kf[0:HB] - pk[QB:QB + HB],
            kf[HB:QB] + pk[QB + HB:],
            kf[QB:QB + HB] + pk[0:HB],
            kf[QB + HB:] - pk[HB:QB]], axis=0)
        put_spec(cs, q, 2, kp)

    MAC_PIECES = [(rb, n) for rb in range(QB // 16) for n in range(NT)]

    def conv_mac(c, q, piece, nterms):
        rb2, n = piece
        cs = clip(c, NB)
        acc = []
        for rb in (2 * rb2, 2 * rb2 + 1):
            ar = None
            ai = None
            for j in range(nterms):
                if isinstance(cs, int):
                    uj, kj = j, cs - j
                else:
                    uj = jnp.minimum(j, cs)
                    kj = jnp.where(cs - j >= 0, cs - j, NB + 1)
                ur = sp_sc[uj, q, rb, n, 0]
                um = sp_sc[uj, q, rb, n, 1]
                kr = sp_sc[kj, q, rb, n, 2]
                km = sp_sc[kj, q, rb, n, 3]
                tr = ur * kr - um * km
                ti = ur * km + um * kr
                ar = tr if ar is None else ar + tr
                ai = ti if ai is None else ai + ti
            acc.append((ar, ai))
        ln = slice(n * 128, (n + 1) * 128)
        w = jnp.concatenate([acc[0][0], acc[1][0], acc[0][1], acc[1][1]], axis=0).astype(BF16)
        wf_sc[c & 1, q, rb2 * 16:rb2 * 16 + 16, ln] = w[0:16]
        wf_sc[c & 1, q, QB + rb2 * 16:QB + rb2 * 16 + 16, ln] = w[16:]

    def conv_inv(s):
        w = wf_sc[(s // NQ) & 1].reshape(2 * CB, DM)
        yc = _dot(inv_ref[s % NQ], w)
        sd = jnp.concatenate([co_sc[KS]] * (SEG // 8), axis=0)
        y_sc[s & 3] = yc + u_sc[seg(s), LN].astype(F32) * sd

    scale = DH ** -0.5
    cexp = scale * float(np.log2(np.e))

    def make_mask(n, x_layers, q0=0):
        qi = jax.lax.broadcasted_iota(jnp.int32, (n - q0, n), 0) + q0
        ki = jax.lax.broadcasted_iota(jnp.int32, (n - q0, n), 1)

        def layer(i):
            xl = jnp.where(i < M2 + SEG, x_layers[0], x_layers[-1])
            return jnp.where(i < M, 0, jnp.where(i < M2, 1, xl))
        same = layer(qi) == layer(ki)
        ok = same & ((qi < M2) | (ki < M2) | (qi >= ki))
        fill = jnp.where(same, -1e9 / scale, -jnp.inf).astype(F32)
        return ok, fill

    def probs(q, k, mask):
        ok, fill = mask
        s = _dot_nt(q, k)
        s = jnp.where(ok, s, fill)
        m = jnp.max(s, axis=-1, keepdims=True)
        p = jnp.exp2((s - m) * cexp)
        l = jnp.sum(p, axis=-1, keepdims=True)
        r = pl.reciprocal(l, approx=True)
        r = r * (2.0 - l * r)
        return (p * r).astype(BF16)

    def w_slot(ci):
        return (wb_sc, ci) if 1 <= ci < NRB - 1 else (wa_sc, max(ci - (NRB - 2), 0))

    def w_head(g, mats):
        slots = [w_slot(mi * NG + g // HG) for mi in mats]
        return _unpack(jnp.concatenate([ref[i, g % HG] for ref, i in slots], axis=1))

    def proj_split(hq, hkv, g, q1=None):
        q = _dot(hq, w_head(g, (0,)))
        kv = _dot(hkv, w_head(g, (1, 2)))
        if q1 is not None:
            q = jnp.concatenate([q[0:M2], q1, q[M2:]], axis=0)
        return q.astype(BF16), kv[:, :DH].astype(BF16), kv[:, DH:].astype(BF16)

    def xn(s):
        return _unpack(xn_sc[clip(s, NSEG - 1), :, 0:DM])

    def out_proj(n, g0, g1, j):
        return _dot(_unpack(o_sc[0:n // 2, g0 * DH:g1 * DH]),
                    wo_sc[g0 * DH:g1 * DH, j * 128:(j + 1) * 128])

    def attend(proj, n, mask, dist, hook=None, early=True):
        D1, D2 = dist
        HA = H - D1 - D2 - 1
        NE = min(D1 + D2, NT - 1) if early else 0
        qkvs = {}
        ps = {}
        outs = {}
        for it in range(H + D1 + D2):
            if it < H:
                qkvs[it] = proj(it)
            g = it - D1
            if 0 <= g < H:
                ps[g] = probs(qkvs[g][0], qkvs[g][1], mask)
            g = it - D1 - D2
            if 0 <= g < H:
                o = _dot(ps.pop(g), qkvs.pop(g)[2])
                o_sc[0:n // 2, g * DH:(g + 1) * DH] = _pack(o)
            if hook is not None:
                hook(it)
            j = it - (H - 1)
            if 0 <= j < NE:
                outs[j] = out_proj(n, 0, HA, j)
        for j in range(NE, NT):
            outs[j] = out_proj(n, 0, H, j)
        for j in range(NE):
            outs[j] = out_proj(n, HA, H, j) + outs[j]
        return jnp.concatenate([outs[j] for j in range(NT)], axis=1)

    def side2(t, a2):
        x3 = x2_sc[(t - 2) & 3] + a2
        x4 = x3 + _ln(x3) * y_sc[(t - 2) & 3]
        x4 = x4.astype(out_sc.dtype)
        out_sc[seg(t - 2), LN] = x4
        return x4

    def finish(t, xr, yt, mem, a1, spec):
        if spec:
            conv_spec((t + 1) // NQ + 1, (t + 1) % NQ)
        xq = xn(t + 1)
        for g in range(NPA, NPA + NPB):
            fill_sc[g - NPA] = _dot(xq, w_head(g, (0,)))
        conv_inv(t + 1)
        x1 = xr.astype(F32) + a1
        x2 = x1 + _ln(x1) * yt
        h_sc[0:M, :] = _pack(mem)
        h_sc[M:, :] = _pack(_ln(x2))
        x2_sc[t & 3] = x2

    def pinned(rows, pins):
        never = never_sm[0] > 0
        hs = {0: rows}
        r = _pack(rows)
        tiles = [r[:, n * 128:(n + 1) * 128] for n in range(NT)]
        for g, n, d in sorted(pins, key=lambda p: p[0]):
            tiles[n] = jnp.where(never, d, tiles[n])
            hs[g] = _unpack(jnp.concatenate(tiles, axis=1))
        return lambda g: hs[max(k for k in hs if k <= g)]

    def pin_tiles(g0, stride, val):
        v = _pack(val)
        return [(g0 + n * stride, n, v[:, n * 128:(n + 1) * 128]) for n in range(NT)]

    def wait_chunk(ci):
        for cp in w_copies(0, ci):
            cp.wait()

    def relayout(ci, dst, slot, b):
        d0 = scaled(b, 16)
        r0 = scaled(b, 8)
        xw = pltpu.bitcast(st_sc[ci, pl.ds(d0, 16)], U32).reshape(8, 2, HG, DH)
        a = xw[:, 0]
        bb = xw[:, 1]
        lo = jnp.swapaxes((a & U32(0xFFFF)) | (bb << 16), 0, 1)
        hi = jnp.swapaxes((a >> 16) | (bb & U32(0xFFFF0000)), 0, 1)
        for j in range(HG):
            rows = pl.ds(r0 + (2 * j // HG) * (DH2 // 2), 8)
            dst[slot, 2 * j % HG, rows, :] = lo[j]
            dst[slot, 2 * j % HG + 1, rows, :] = hi[j]

    def everything(_, carry):
        NBLK = DH2 // 16
        def relayout0(b, c):
            relayout(0, wa_sc, 0, b)
            return c
        for part in range(2):
            with jax.named_scope("wait_w"):
                for cp in w_copies(0, part=part):
                    cp.wait()
            with jax.named_scope("relayout"):
                jax.lax.fori_loop(part * NBLK // 2, (part + 1) * NBLK // 2, relayout0, 0, unroll=2)

        def pro_stage(ps_, b):
            n = ps_ * NRB + b
            with jax.named_scope("wait_w"):
                if ps_ == 0:
                    @pl.when(b + 1 < NRB)
                    def _():
                        x_copy(b + 1).wait()

                @pl.when((n >= 2) & (n <= NCH))
                def _():
                    wait_chunk(n - 1)
            cr = jnp.clip(n - 1, 0, NCH - 1)
            dst, slot = (wb_sc, cr) if ps_ == 0 else (wa_sc, cr - (NRB - 2))
            src, si = w_slot(ps_)
            bl = jnp.minimum(b + 1, NRB - 1)
            PW = PRO_PW
            npc = RB * S2 // PW
            assert npc * PW == RB * S2 and PRO_R0 + (NBLK - 1) * PRO_RS < HG * npc
            assert PRO_X0 + (max(RB, 2 * NT) - 1) * PRO_XS < HG * npc and 2 * NRB > 2 * NQ

            def body(i, c):
                s0 = b * RB + 1
                for sg in range(RB):
                    hp_sc[sg * S2:(sg + 1) * S2, :] = xn_sc[s0 + sg, :, 0:DM]
                for j in range(HG):
                    w = _unpack(src[si, j])
                    for pi in range(npc):
                        pos = j * npc + pi
                        hx = hp_sc[pi * PW:(pi + 1) * PW, :]
                        k, rem = divmod(pos - PRO_X0, PRO_XS)
                        if ps_ == 0 and rem == 0 and 0 <= k < RB:
                            sn = bl * RB + 1 + k
                            xv = _pack(_ln(x_sc[seg(sn), LN].astype(F32)))
                            xn_sc[sn, :, 0:DM] = xv
                            hx = jnp.concatenate([hx[:-S2], jnp.where(never_sm[0] > 0, xv, hx[-S2:])], axis=0)
                        if ps_ == 1 and rem == 0 and 0 <= k < 2 * NT:
                            conv_u(jnp.minimum(2 * b + k // NT, 2 * NQ),
                                   slice((k % NT) * 128, (k % NT + 1) * 128))
                        bb, rem = divmod(pos - PRO_R0, PRO_RS)
                        if rem == 0 and 0 <= bb < NBLK:
                            relayout(cr, dst, slot, bb)
                        r = _dot(_unpack(hx), w)
                        for a in range(0, 2 * PW, 16):
                            sg, off = divmod(2 * pi * PW + a, SEG)
                            pre_sc[s0 + sg, ps_ * HG + j, off:off + 16, :] = r[a:a + 16]
                return c
            with jax.named_scope("fused"):
                jax.lax.fori_loop(0, never_sm[0] + 1, body, 0)

        for ps_ in range(NPASS):
            if ps_ == 1:
                with jax.named_scope("wait_in0"):
                    for cp in small + in_copies(0):
                        cp.wait()
                sh = sh_ref[...].astype(F32)
                for j in range(KS):
                    co_sc[j] = jnp.broadcast_to(sh[j:j + 1], (8, DM))
                co_sc[KS] = jnp.broadcast_to(sd_ref[...].astype(F32).reshape(1, DM), (8, DM))

            def blk(b, c, ps_=ps_):
                pro_stage(ps_, b)
                return c
            jax.lax.fori_loop(0, NRB, blk, 0)

        def warm_block0(q):
            uf, kf = conv_fwd(0, q)
            put_spec(0, q, 0, uf)
            put_spec(0, q, 2, kf)
            kr_sc[q] = kf
            ur, um, kr, km = uf[:QB], uf[QB:], kf[:QB], kf[QB:]
            wf_sc[0, q, :QB] = (ur * kr - um * km).astype(BF16)
            wf_sc[0, q, QB:] = (ur * km + um * kr).astype(BF16)

        with jax.named_scope("step0"):
            mem0 = mem0_ref[...].astype(F32)
            h0 = jnp.concatenate([jnp.concatenate([mem0, mem0], axis=0).astype(BF16), xn(0)], axis=0)

            def hook0(it):
                j = it - (H - 1)
                if 0 <= j < NQ:
                    warm_block0(j)
                if it == H + sum(DIST_HALF) - 1:
                    conv_spec(1, 0)
                    wo_copy.wait()
                    for piece in MAC_PIECES:
                        conv_mac(1, 0, piece, 2)
                    conv_inv(0)
            out = attend(lambda g: proj_split(h0, h0, g), RH, make_mask(RH, (0,)), DIST_HALF, hook0, False)
            finish(0, x_sc[0:SEG, LN], y_sc[0], jnp.concatenate([out[0:M], mem0], axis=0), out[M2:], False)

        mask12 = make_mask(R, (0, 1))

        def step(t, first, last):
            if first:
                conv_spec_later = functools.partial(conv_spec, t // NQ + 1, t % NQ)
            x4 = side2(t, op_sc[...])
            un = conv_u(t + 2 * NQ)
            hm = _unpack(h_sc[0:M, :])
            hx2 = _unpack(h_sc[M:, :])
            h48 = jnp.concatenate([hm, hx2], axis=0)
            x1n = pinned(xn(t), pin_tiles(PIN_U if first else PIN_U2, 1, un) + pin_tiles(PIN_X4, X4S, x4))

            def proj(g):
                h80 = jnp.concatenate([hm, x1n(g), hx2], axis=0)
                if g >= NPA + NPB:
                    return proj_split(h80, h80, g)
                return proj_split(h48, h80, g, pre_sc[t, g] if g < NPA else fill_sc[g - NPA])

            held = {}

            def hook(it):
                if it == SPEC_AT:
                    if first:
                        conv_spec_later()
                    for piece in MAC_PIECES:
                        conv_mac(t // NQ + 1, t % NQ, piece, NB)
                if it == H:
                    held["x"] = x_sc[seg(t), LN]
                    held["y"] = y_sc[t & 3]
            out = attend(proj, R, mask12, DIST, hook)
            op_sc[...] = out[RH:]
            finish(t, held["x"], held["y"], out[0:M2], out[M2:RH], not last)

        def steps(i, carry):
            for j in range(UNROLL):
                step(1 + i * UNROLL + j, j == 0, j == UNROLL - 1)
            return carry

        def phase(p, carry):
            @pl.when(p == 1)
            def _():
                for cp in in_copies(2):
                    cp.wait()

            @pl.when(p >= 2)
            def _():
                out_copy((p - 2) * PH, PH).start()

            with jax.named_scope("steps"):
                jax.lax.fori_loop(p * PHI, (p + 1) * PHI, steps, 0)
            return carry

        for cp in in_copies(1):
            cp.wait()
        jax.lax.fori_loop(0, NPH, phase, 0)
        out_copy((NPH - 2) * PH, NSEG - 2 - (NPH - 2) * PH).start()

        with jax.named_scope("step_last"):
            x4 = side2(NSEG, op_sc[...])
            hm = _unpack(h_sc[0:M, :])
            hx = pinned(_unpack(h_sc[M:, :]), pin_tiles(PIN_X4, 0, x4))
            out = attend(lambda g: proj_split(hx(g), jnp.concatenate([hm, hx(g)], axis=0), g),
                         SEG, make_mask(RH, (1,), M2), DIST_LAST)
            side2(NSEG + 1, out)
        out_copy(NSEG - 2, 2).start()
        out_copy(0, NSEG).wait()
        return carry

    jax.lax.fori_loop(0, never_sm[0] + 1, everything, 0)


def pallas_interleave_layers__memory_aug_recurrent_mem_tr__ssm_conv_h3__prompt_kernel(
    A_x, A_mem0, A_Wq, A_Wk, A_Wv, A_Wo, A_seg_len,
    B_q, B_k, B_v, B_shift_k, B_ssm_k, B_ssm_D,
):
    del B_q
    seg = int(A_seg_len) if isinstance(A_seg_len, (int, np.integer)) else CB // NQ
    return _run(A_x, A_mem0, A_Wq, A_Wk, A_Wv, A_Wo, B_k, B_v, B_shift_k, B_ssm_k, B_ssm_D, SEG=seg)


@functools.partial(jax.jit, static_argnames=("SEG",))
def _run(A_x, A_mem0, A_Wq, A_Wk, A_Wv, A_Wo, B_k, B_v, B_shift_k, B_ssm_k, B_ssm_D, *, SEG):
    B, S, DM = A_x.shape
    assert B == 1
    H, DH = A_Wq.shape[1], A_Wq.shape[2]
    M = A_mem0.shape[1]
    KS = B_shift_k.shape[1]
    R = 2 * (M + SEG)
    NSEG = S // SEG
    NRB = (NSEG - 1) // RB
    NB = S // CB
    QB = CB // NQ
    NCH = 3 * H // HG
    DP = -(-DM // 256) * 256
    fwd, inv = _dft_constants()

    kern = functools.partial(_kernel, S=S, DM=DM, H=H, DH=DH, M=M, SEG=SEG)
    any_spec = pl.BlockSpec(memory_space=pl.ANY)
    out = pl.pallas_call(
        kern,
        out_shape=jax.ShapeDtypeStruct((S, DM), A_x.dtype),
        in_specs=[any_spec] * 13,
        out_specs=any_spec,
        scratch_shapes=[
            pltpu.VMEM((NB + 2, NQ, QB // 8, DM // 128, 4, 8, 128), F32),
            pltpu.VMEM((NQ, 2 * QB, DM), F32),
            pltpu.VMEM((2, NQ, 2 * QB, DM), BF16),
            pltpu.VMEM((4, SEG, DM), F32),
            pltpu.VMEM((4, SEG, DM), F32),
            pltpu.VMEM((S, DP), BF16),
            pltpu.VMEM((SEG, DM), F32),
            pltpu.VMEM((NSEG, NPA, SEG, DH), F32),
            pltpu.VMEM((NPB, SEG, DH), F32),
            pltpu.VMEM((NSEG, SEG // 2, DP), U32),
            pltpu.VMEM((NCH - NRB + 2, HG, DM // 2, DH), U32),
            pltpu.VMEM((NRB - 1, HG, DM // 2, DH), U32),
            pltpu.VMEM((H * DH, DM), BF16),
            pltpu.VMEM((R // 2, H * DH), U32),
            pltpu.VMEM((S, DP), BF16),
            pltpu.VMEM((S, DP), BF16),
            pltpu.VMEM((NB, DM, CB), BF16),
            pltpu.VMEM((NCH, DM // 2, 2 * HG, DH), BF16),
            pltpu.VMEM((S, DP), A_x.dtype),
            pltpu.VMEM(fwd.shape, BF16),
            pltpu.VMEM(inv.shape, BF16),
            pltpu.VMEM((S + KPAD, DP), BF16),
            pltpu.VMEM((RB * SEG // 2, DM), U32),
            pltpu.VMEM((M + SEG // 2, DM), U32),
            pltpu.VMEM((KS + 1, 8, DM), F32),
            pltpu.VMEM((M, DM), BF16),
            pltpu.VMEM((KS, DM), BF16),
            pltpu.VMEM((DM,), BF16),
            pltpu.SMEM((1,), jnp.int32),
            pltpu.SemaphoreType.DMA(((NSEG - 1) // RB,)),
            pltpu.SemaphoreType.DMA((3,)),
            pltpu.SemaphoreType.DMA((NCH + 2,)),
            pltpu.SemaphoreType.DMA(()),
        ],
        compiler_params=pltpu.CompilerParams(vmem_limit_bytes=120 * 1024 * 1024),
    )(
        A_x.reshape(S, DM), A_mem0.reshape(M, DM), A_Wq, A_Wk, A_Wv,
        A_Wo.reshape(H * DH, DM), B_k.reshape(S, DM), B_v.reshape(S, DM),
        B_shift_k.T, B_ssm_k, B_ssm_D,
        jnp.asarray(fwd, BF16), jnp.asarray(inv, BF16),
    )
    return out.reshape(B, S, DM)
```

```python
import functools

import numpy as np
import jax
import jax.numpy as jnp
import jax.experimental.pallas as pl
import jax.experimental.pallas.tpu as pltpu

F32 = jnp.float32
BF16 = jnp.bfloat16
U32 = jnp.uint32

CB = 128
NQ = 4
KPAD = 16
HG = 8
NPA = 16
NPB = 12
RB = 9
PRO_PW, PRO_X0, PRO_XS, PRO_R0, PRO_RS = 24, 11, 4, 2, 2
UNROLL = 3
PHI = 3
PIN_U2, X4S = 1, 0
SPEC_AT, PIN_U, PIN_X4 = 7, 1, 16
DIST, DIST_HALF, DIST_LAST = (1, 2), (1, 3), (2, 3)


def _dft_constants():
    qb = CB // NQ
    n = np.arange(CB, dtype=np.float64)
    fwd = np.zeros((NQ, 2 * qb, CB))
    for q in range(NQ):
        f = q * qb + np.concatenate([np.arange(0, qb, 2), np.arange(1, qb, 2)])
        ang = (np.pi * (2.0 * f + 1.0) / (2 * CB))[:, None] * n[None, :]
        fwd[q, :qb] = np.cos(ang)
        fwd[q, qb:] = -np.sin(ang)
    inv = fwd.reshape(2 * CB, CB).T / CB
    return fwd.astype(np.float32), inv.reshape(NQ, CB // NQ, 2 * CB).astype(np.float32)


def _ln(x, eps=1e-5):
    d = x.shape[-1]
    m = jnp.sum(x, axis=-1, keepdims=True) * (1.0 / d)
    xc = x - m
    v = jnp.sum(xc * xc, axis=-1, keepdims=True) * (1.0 / d)
    return xc * jax.lax.rsqrt(v + eps)


def _dot(a, b):
    return jnp.dot(a, b, preferred_element_type=F32)


def _dot_nt(a, b):
    return jax.lax.dot_general(a, b, (((1,), (1,)), ((), ())), preferred_element_type=F32)


def _pack(x):
    return pltpu.bitcast(x.astype(BF16), U32)


def _unpack(x):
    return pltpu.bitcast(x, BF16)


def _in_order(actions):
    def body(i, c):
        for j, act in enumerate(actions):
            pl.when(i == j)(act)
        return c
    jax.lax.fori_loop(0, len(actions), body, 0)


def _kernel(x_hbm, mem0_hbm, wq_hbm, wk_hbm, wv_hbm, wo_hbm, k_hbm, v_hbm,
            sh_hbm, sk_hbm, sd_hbm, fwd_hbm, inv_hbm, o_hbm,
            sp_sc, kr_sc, wf_sc, x2_sc, y_sc, u_sc, op_sc, pre_sc, fill_sc, xn_sc, wa_sc, wb_sc, wo_sc, o_sc,
            x_sc, v_sc, sk_sc, st_sc, out_sc, fwd_ref, inv_ref,
            k_sc, hp_sc, h_sc, co_sc, mem0_ref, sh_ref, sd_ref,
            never_sm, sem_x, sem_in, sem_w, sem_out,
            *, S, DM, H, DH, M, SEG):
    NSEG = S // SEG
    M2 = 2 * M
    S2 = SEG // 2
    R = M2 + 2 * SEG
    RH = M2 + SEG
    NB = S // CB
    QB = CB // NQ
    HB = QB // 2
    NT = DM // 128
    PH = PHI * UNROLL
    NRB = (NSEG - 1) // RB
    NPH = (NSEG - 1) // PH
    NG = H // HG
    NCH = 3 * NG
    NPASS = NPA // HG
    DH2 = DM // 2
    KS = sh_ref.shape[0]
    LN = pl.ds(0, DM)
    assert 2 <= KS <= 8 and QB == SEG and NRB * RB == NSEG - 1 and NPH * PH == NSEG - 1 and NPASS == 2 and 2 * NRB >= NCH + 1

    mem0_copy = pltpu.make_async_copy(mem0_hbm, mem0_ref, sem_x.at[0])
    small = [pltpu.make_async_copy(s, d, sem_in.at[0]) for s, d in [
        (sh_hbm, sh_ref), (sd_hbm, sd_ref), (fwd_hbm, fwd_ref), (inv_hbm, inv_ref)]]

    def x_copy(b):
        if isinstance(b, int) and b == 0:
            rows = pl.ds(0, (RB + 1) * SEG)
        else:
            rows = pl.ds(pl.multiple_of((b * RB + 1) * SEG, SEG), RB * SEG)
        return pltpu.make_async_copy(x_hbm.at[rows], x_sc.at[rows, LN], sem_x.at[b])

    kb = (0, (2 * NQ + 1) * SEG, (2 * NQ + PH + 1) * SEG, S)
    sb = (0, 2, (PH + 1) // NQ + 2, NB)

    def in_copies(part):
        def rng(b):
            return pl.ds(b[part], b[part + 1] - b[part])
        sem = sem_in.at[part]
        return [
            pltpu.make_async_copy(k_hbm.at[rng(kb)],
                                  k_sc.at[pl.ds(KPAD + kb[part], kb[part + 1] - kb[part]), LN], sem),
            pltpu.make_async_copy(v_hbm.at[rng(kb)], v_sc.at[rng(kb), LN], sem),
        ] + [pltpu.make_async_copy(sk_hbm.at[:, pl.ds(c * CB, CB)], sk_sc.at[c], sem)
             for c in range(sb[part], sb[part + 1])]

    def w_copies(ci, dst=None, part=None):
        src = (wq_hbm, wk_hbm, wv_hbm)[ci // NG]
        dst = ci if dst is None else dst
        lo, n = (0, DH2) if part is None else (part * DH2 // 2, DH2 // 2)
        sem = sem_w.at[NCH + 1 if part == 1 else dst]
        return [pltpu.make_async_copy(src.at[pl.ds(hf * DH2 + lo, n), pl.ds((ci % NG) * HG, HG), :],
                                      st_sc.at[dst, pl.ds(lo, n), pl.ds(hf * HG, HG), :], sem)
                for hf in range(2)]

    wo_copy = pltpu.make_async_copy(wo_hbm, wo_sc, sem_w.at[NCH])

    def out_copy(lo, n):
        rows = pl.ds(lo * SEG if isinstance(lo, int) else pl.multiple_of(lo * SEG, SEG), n * SEG)
        return pltpu.make_async_copy(out_sc.at[rows, LN], o_hbm.at[rows], sem_out)

    def start_all(cps):
        def act():
            for cp in cps:
                cp.start()
        return act

    order = [[mem0_copy, x_copy(0)], w_copies(0, part=0), w_copies(0, part=1), [x_copy(1)], [x_copy(2)]]
    for ci in range(1, NCH):
        order.append(w_copies(ci) + ([x_copy(ci + 2)] if ci + 2 < NRB else []))
        if ci == NRB - 2:
            order.append(small + in_copies(0))
    order += [[wo_copy], in_copies(1), in_copies(2)]
    for i in range(0, len(order), 5):
        _in_order([start_all(cps) for cps in order[i:i + 5]])

    never_sm[0] = 0
    k_sc[0:KPAD, LN] = jnp.zeros((KPAD, DM), BF16)
    sp_sc[NB + 1] = jnp.zeros(sp_sc.shape[1:], F32)
    op_sc[...] = jnp.zeros(op_sc.shape, F32)
    x2_sc[...] = jnp.zeros(x2_sc.shape, F32)
    y_sc[...] = jnp.zeros(y_sc.shape, F32)
    mem0_copy.wait()
    x_copy(0).wait()
    for sg in range(RB + 1):
        xn_sc[sg, :, 0:DM] = _pack(_ln(x_sc[sg * SEG:(sg + 1) * SEG, LN].astype(F32)))

    def clip(i, hi):
        return min(max(i, 0), hi) if isinstance(i, int) else jnp.clip(i, 0, hi)

    def scaled(i, m):
        return i * m if isinstance(i, int) else pl.multiple_of(i * m, m)

    def seg(i):
        return pl.ds(scaled(clip(i, NSEG - 1), SEG), SEG)

    def conv_u(s, ln=LN):
        r0 = scaled(clip(s, NSEG - 1), SEG)
        kk = k_sc[pl.ds(r0, KPAD + SEG), ln].astype(F32)[KPAD - 8:]

        def coef(j, rows):
            return jnp.concatenate([co_sc[j, :, ln]] * (rows // 8), axis=0)
        sft = [kk] + [pltpu.roll(kk, j, 0) for j in range(2, KS, 2)]
        ev = functools.reduce(jnp.add, [sft[j // 2][8:] * coef(j, SEG) for j in range(0, KS, 2)])
        od = functools.reduce(jnp.add, [sft[j // 2] * coef(j, SEG + 8) for j in range(1, KS, 2)])
        ks = ev + pltpu.roll(od, 1, 0)[8:]
        u = (ks * v_sc[pl.ds(r0, SEG), ln].astype(F32)).astype(BF16)
        u_sc[pl.ds(r0, SEG), ln] = u
        return u

    def conv_fwd(c, q):
        cc = clip(c, NB - 1)
        f = fwd_ref[q]
        uf = _dot(f, u_sc[pl.ds(scaled(cc, CB), CB), LN])
        kf = _dot_nt(f, sk_sc[cc])
        return uf, kf

    def put_spec(cs, q, which, val):
        for n in range(NT):
            v = val[:, n * 128:(n + 1) * 128].reshape(2, QB // 8, 8, 128)
            sp_sc[cs, q, :, n, which:which + 2] = jnp.stack([v[0], v[1]], axis=1)

    def conv_spec(c, q):
        uf, kf = conv_fwd(c, q)
        cs = clip(c, NB)
        put_spec(cs, q, 0, uf)
        pk = kr_sc[q]
        kr_sc[q] = kf
        kp = jnp.concatenate([
            kf[0:HB] - pk[QB:QB + HB],
            kf[HB:QB] + pk[QB + HB:],
            kf[QB:QB + HB] + pk[0:HB],
            kf[QB + HB:] - pk[HB:QB]], axis=0)
        put_spec(cs, q, 2, kp)

    MAC_PIECES = [(rb, n) for rb in range(QB // 16) for n in range(NT)]

    def conv_mac(c, q, piece, nterms):
        rb2, n = piece
        cs = clip(c, NB)
        rbs = slice(2 * rb2, 2 * rb2 + 2)
        ar = None
        ai = None
        for j in range(nterms):
            if isinstance(cs, int):
                uj, kj = j, cs - j
            else:
                uj = jnp.minimum(j, cs)
                kj = jnp.where(cs - j >= 0, cs - j, NB + 1)
            u = sp_sc[uj, q, rbs, n, 0:2]
            k = sp_sc[kj, q, rbs, n, 2:4]
            tr = u[:, 0] * k[:, 0] - u[:, 1] * k[:, 1]
            ti = u[:, 0] * k[:, 1] + u[:, 1] * k[:, 0]
            ar = tr if ar is None else ar + tr
            ai = ti if ai is None else ai + ti
        ln = slice(n * 128, (n + 1) * 128)
        w = jnp.concatenate([ar.reshape(16, 128), ai.reshape(16, 128)], axis=0).astype(BF16)
        wf_sc[c & 1, q, rb2 * 16:rb2 * 16 + 16, ln] = w[0:16]
        wf_sc[c & 1, q, QB + rb2 * 16:QB + rb2 * 16 + 16, ln] = w[16:]

    def conv_inv(s):
        w = wf_sc[(s // NQ) & 1].reshape(2 * CB, DM)
        yc = _dot(inv_ref[s % NQ], w)
        sd = jnp.concatenate([co_sc[KS]] * (SEG // 8), axis=0)
        y_sc[s & 3] = yc + u_sc[seg(s), LN].astype(F32) * sd

    scale = DH ** -0.5
    cexp = scale * float(np.log2(np.e))

    def make_mask(n, x_layers, q0=0):
        qi = jax.lax.broadcasted_iota(jnp.int32, (n - q0, n), 0) + q0
        ki = jax.lax.broadcasted_iota(jnp.int32, (n - q0, n), 1)

        def layer(i):
            xl = jnp.where(i < M2 + SEG, x_layers[0], x_layers[-1])
            return jnp.where(i < M, 0, jnp.where(i < M2, 1, xl))
        same = layer(qi) == layer(ki)
        ok = same & ((qi < M2) | (ki < M2) | (qi >= ki))
        fill = jnp.where(same, -1e9 / scale, -jnp.inf).astype(F32)
        return ok, fill

    def probs(q, k, mask):
        ok, fill = mask
        s = _dot_nt(q, k)
        s = jnp.where(ok, s, fill)
        m = jnp.max(s, axis=-1, keepdims=True)
        p = jnp.exp2((s - m) * cexp)
        l = jnp.sum(p, axis=-1, keepdims=True)
        r = pl.reciprocal(l, approx=True)
        r = r * (2.0 - l * r)
        return (p * r).astype(BF16)

    def w_slot(ci):
        return (wb_sc, ci) if 1 <= ci < NRB - 1 else (wa_sc, max(ci - (NRB - 2), 0))

    def w_pos(j):
        return (j % 2) * (HG // 2) + j // 2

    def w_head(g, mats):
        slots = [w_slot(mi * NG + g // HG) for mi in mats]
        return _unpack(jnp.concatenate([ref[i, w_pos(g % HG)] for ref, i in slots], axis=1))

    def proj_split(hq, hkv, g, q1=None):
        q = _dot(hq, w_head(g, (0,)))
        kv = _dot(hkv, w_head(g, (1, 2)))
        if q1 is not None:
            q = jnp.concatenate([q[0:M2], q1, q[M2:]], axis=0)
        return q.astype(BF16), kv[:, :DH].astype(BF16), kv[:, DH:].astype(BF16)

    def xn(s):
        return _unpack(xn_sc[clip(s, NSEG - 1), :, 0:DM])

    def out_proj(n, g0, g1, j):
        return _dot(_unpack(o_sc[0:n // 2, g0 * DH:g1 * DH]),
                    wo_sc[g0 * DH:g1 * DH, j * 128:(j + 1) * 128])

    def attend(proj, n, mask, dist, hook=None, early=True):
        D1, D2 = dist
        HA = H - D1 - D2 - 1
        NE = min(D1 + D2, NT - 1) if early else 0
        qkvs = {}
        ps = {}
        outs = {}
        for it in range(H + D1 + D2):
            if it < H:
                qkvs[it] = proj(it)
            g = it - D1
            if 0 <= g < H:
                ps[g] = probs(qkvs[g][0], qkvs[g][1], mask)
            g = it - D1 - D2
            if 0 <= g < H:
                o = _dot(ps.pop(g), qkvs.pop(g)[2])
                o_sc[0:n // 2, g * DH:(g + 1) * DH] = _pack(o)
            if hook is not None:
                hook(it)
            j = it - (H - 1)
            if 0 <= j < NE:
                outs[j] = out_proj(n, 0, HA, j)
        for j in range(NE, NT):
            outs[j] = out_proj(n, 0, H, j)
        for j in range(NE):
            outs[j] = out_proj(n, HA, H, j) + outs[j]
        return jnp.concatenate([outs[j] for j in range(NT)], axis=1)

    def side2(t, a2):
        x3 = x2_sc[(t - 2) & 3] + a2
        x4 = x3 + _ln(x3) * y_sc[(t - 2) & 3]
        x4 = x4.astype(out_sc.dtype)
        out_sc[seg(t - 2), LN] = x4
        return x4

    def finish(t, xr, yt, mem, a1, spec):
        if spec:
            conv_spec((t + 1) // NQ + 1, (t + 1) % NQ)
        xq = xn(t + 1)
        for g in range(NPA, NPA + NPB):
            fill_sc[g - NPA] = _dot(xq, w_head(g, (0,)))
        conv_inv(t + 1)
        x1 = xr.astype(F32) + a1
        x2 = x1 + _ln(x1) * yt
        h_sc[0:M, :] = _pack(mem)
        h_sc[M:, :] = _pack(_ln(x2))
        x2_sc[t & 3] = x2

    def pinned(rows, pins):
        never = never_sm[0] > 0
        hs = {0: rows}
        r = _pack(rows)
        tiles = [r[:, n * 128:(n + 1) * 128] for n in range(NT)]
        for g, n, d in sorted(pins, key=lambda p: p[0]):
            tiles[n] = jnp.where(never, d, tiles[n])
            hs[g] = _unpack(jnp.concatenate(tiles, axis=1))
        return lambda g: hs[max(k for k in hs if k <= g)]

    def pin_tiles(g0, stride, val):
        v = _pack(val)
        return [(g0 + n * stride, n, v[:, n * 128:(n + 1) * 128]) for n in range(NT)]

    def wait_chunk(ci):
        for cp in w_copies(0, ci):
            cp.wait()

    def relayout(ci, dst, slot, b):
        d0 = scaled(b, 16)
        r0 = scaled(b, 8)
        xw = pltpu.bitcast(st_sc[ci, pl.ds(d0, 16)], U32).reshape(8, 2, HG, DH)
        a = xw[:, 0]
        bb = xw[:, 1]
        lo = jnp.swapaxes((a & U32(0xFFFF)) | (bb << 16), 0, 1)
        hi = jnp.swapaxes((a >> 16) | (bb & U32(0xFFFF0000)), 0, 1)
        for hf in range(2):
            rows = pl.ds(r0 + hf * (DH2 // 2), 8)
            dst[slot, 0:HG // 2, rows, :] = lo[hf * HG // 2:(hf + 1) * HG // 2]
            dst[slot, HG // 2:HG, rows, :] = hi[hf * HG // 2:(hf + 1) * HG // 2]

    def everything(_, carry):
        NBLK = DH2 // 16
        def relayout0(b, c):
            relayout(0, wa_sc, 0, b)
            return c
        for part in range(2):
            with jax.named_scope("wait_w"):
                for cp in w_copies(0, part=part):
                    cp.wait()
            with jax.named_scope("relayout"):
                jax.lax.fori_loop(part * NBLK // 2, (part + 1) * NBLK // 2, relayout0, 0, unroll=2)

        def pro_stage(ps_, b):
            n = ps_ * NRB + b
            with jax.named_scope("wait_w"):
                if ps_ == 0:
                    @pl.when(b + 1 < NRB)
                    def _():
                        x_copy(b + 1).wait()

                @pl.when((n >= 2) & (n <= NCH))
                def _():
                    wait_chunk(n - 1)
            cr = jnp.clip(n - 1, 0, NCH - 1)
            dst, slot = (wb_sc, cr) if ps_ == 0 else (wa_sc, cr - (NRB - 2))
            src, si = w_slot(ps_)
            bl = jnp.minimum(b + 1, NRB - 1)
            PW = PRO_PW
            npc = RB * S2 // PW
            assert npc * PW == RB * S2 and PRO_R0 + (NBLK - 1) * PRO_RS < HG * npc
            assert PRO_X0 + (max(RB, 2 * NT) - 1) * PRO_XS < HG * npc and 2 * NRB > 2 * NQ

            def body(i, c):
                s0 = b * RB + 1
                for sg in range(RB):
                    hp_sc[sg * S2:(sg + 1) * S2, :] = xn_sc[s0 + sg, :, 0:DM]
                for j in range(HG):
                    w = _unpack(src[si, w_pos(j)])
                    for pi in range(npc):
                        pos = j * npc + pi
                        hx = hp_sc[pi * PW:(pi + 1) * PW, :]
                        k, rem = divmod(pos - PRO_X0, PRO_XS)
                        if ps_ == 0 and rem == 0 and 0 <= k < RB:
                            sn = bl * RB + 1 + k
                            xv = _pack(_ln(x_sc[seg(sn), LN].astype(F32)))
                            xn_sc[sn, :, 0:DM] = xv
                            hx = jnp.concatenate([hx[:-S2], jnp.where(never_sm[0] > 0, xv, hx[-S2:])], axis=0)
                        if ps_ == 1 and rem == 0 and 0 <= k < 2 * NT:
                            conv_u(jnp.minimum(2 * b + k // NT, 2 * NQ),
                                   slice((k % NT) * 128, (k % NT + 1) * 128))
                        bb, rem = divmod(pos - PRO_R0, PRO_RS)
                        if rem == 0 and 0 <= bb < NBLK:
                            relayout(cr, dst, slot, bb)
                        r = _dot(_unpack(hx), w)
                        for a in range(0, 2 * PW, 16):
                            sg, off = divmod(2 * pi * PW + a, SEG)
                            pre_sc[s0 + sg, ps_ * HG + j, off:off + 16, :] = r[a:a + 16]
                return c
            with jax.named_scope("fused"):
                jax.lax.fori_loop(0, never_sm[0] + 1, body, 0)

        for ps_ in range(NPASS):
            if ps_ == 1:
                with jax.named_scope("wait_in0"):
                    for cp in small + in_copies(0):
                        cp.wait()
                sh = sh_ref[...].astype(F32)
                for j in range(KS):
                    co_sc[j] = jnp.broadcast_to(sh[j:j + 1], (8, DM))
                co_sc[KS] = jnp.broadcast_to(sd_ref[...].astype(F32).reshape(1, DM), (8, DM))

            def blk(b, c, ps_=ps_):
                pro_stage(ps_, b)
                return c
            jax.lax.fori_loop(0, NRB, blk, 0)

        def warm_block0(q):
            uf, kf = conv_fwd(0, q)
            put_spec(0, q, 0, uf)
            put_spec(0, q, 2, kf)
            kr_sc[q] = kf
            ur, um, kr, km = uf[:QB], uf[QB:], kf[:QB], kf[QB:]
            wf_sc[0, q, :QB] = (ur * kr - um * km).astype(BF16)
            wf_sc[0, q, QB:] = (ur * km + um * kr).astype(BF16)

        with jax.named_scope("step0"):
            mem0 = mem0_ref[...].astype(F32)
            h0 = jnp.concatenate([jnp.concatenate([mem0, mem0], axis=0).astype(BF16), xn(0)], axis=0)

            def hook0(it):
                j = it - (H - 1)
                if 0 <= j < NQ:
                    warm_block0(j)
                if it == H + sum(DIST_HALF) - 1:
                    conv_spec(1, 0)
                    wo_copy.wait()
                    for piece in MAC_PIECES:
                        conv_mac(1, 0, piece, 2)
                    conv_inv(0)
            out = attend(lambda g: proj_split(h0, h0, g), RH, make_mask(RH, (0,)), DIST_HALF, hook0, False)
            finish(0, x_sc[0:SEG, LN], y_sc[0], jnp.concatenate([out[0:M], mem0], axis=0), out[M2:], False)

        mask12 = make_mask(R, (0, 1))

        def step(t, first, last):
            if first:
                conv_spec_later = functools.partial(conv_spec, t // NQ + 1, t % NQ)
            x4 = side2(t, op_sc[...])
            un = conv_u(t + 2 * NQ)
            hm = _unpack(h_sc[0:M, :])
            hx2 = _unpack(h_sc[M:, :])
            h48 = jnp.concatenate([hm, hx2], axis=0)
            x1n = pinned(xn(t), pin_tiles(PIN_U if first else PIN_U2, 1, un) + pin_tiles(PIN_X4, X4S, x4))

            def proj(g):
                h80 = jnp.concatenate([hm, x1n(g), hx2], axis=0)
                if g >= NPA + NPB:
                    return proj_split(h80, h80, g)
                return proj_split(h48, h80, g, pre_sc[t, g] if g < NPA else fill_sc[g - NPA])

            held = {}

            def hook(it):
                if it == SPEC_AT:
                    if first:
                        conv_spec_later()
                    for piece in MAC_PIECES:
                        conv_mac(t // NQ + 1, t % NQ, piece, NB)
                if it == H:
                    held["x"] = x_sc[seg(t), LN]
                    held["y"] = y_sc[t & 3]
            out = attend(proj, R, mask12, DIST, hook)
            op_sc[...] = out[RH:]
            finish(t, held["x"], held["y"], out[0:M2], out[M2:RH], not last)

        def steps(i, carry):
            for j in range(UNROLL):
                step(1 + i * UNROLL + j, j == 0, j == UNROLL - 1)
            return carry

        def phase(p, carry):
            @pl.when(p == 1)
            def _():
                for cp in in_copies(2):
                    cp.wait()

            @pl.when(p >= 2)
            def _():
                out_copy((p - 2) * PH, PH).start()

            with jax.named_scope("steps"):
                jax.lax.fori_loop(p * PHI, (p + 1) * PHI, steps, 0)
            return carry

        for cp in in_copies(1):
            cp.wait()
        jax.lax.fori_loop(0, NPH, phase, 0)
        out_copy((NPH - 2) * PH, NSEG - 2 - (NPH - 2) * PH).start()

        with jax.named_scope("step_last"):
            x4 = side2(NSEG, op_sc[...])
            hm = _unpack(h_sc[0:M, :])
            hx = pinned(_unpack(h_sc[M:, :]), pin_tiles(PIN_X4, 0, x4))
            out = attend(lambda g: proj_split(hx(g), jnp.concatenate([hm, hx(g)], axis=0), g),
                         SEG, make_mask(RH, (1,), M2), DIST_LAST)
            side2(NSEG + 1, out)
        out_copy(NSEG - 2, 2).start()
        out_copy(0, NSEG).wait()
        return carry

    jax.lax.fori_loop(0, never_sm[0] + 1, everything, 0)


def pallas_interleave_layers__memory_aug_recurrent_mem_tr__ssm_conv_h3__prompt_kernel(
    A_x, A_mem0, A_Wq, A_Wk, A_Wv, A_Wo, A_seg_len,
    B_q, B_k, B_v, B_shift_k, B_ssm_k, B_ssm_D,
):
    del B_q
    seg = int(A_seg_len) if isinstance(A_seg_len, (int, np.integer)) else CB // NQ
    return _run(A_x, A_mem0, A_Wq, A_Wk, A_Wv, A_Wo, B_k, B_v, B_shift_k, B_ssm_k, B_ssm_D, SEG=seg)


@functools.partial(jax.jit, static_argnames=("SEG",))
def _run(A_x, A_mem0, A_Wq, A_Wk, A_Wv, A_Wo, B_k, B_v, B_shift_k, B_ssm_k, B_ssm_D, *, SEG):
    B, S, DM = A_x.shape
    assert B == 1
    H, DH = A_Wq.shape[1], A_Wq.shape[2]
    M = A_mem0.shape[1]
    KS = B_shift_k.shape[1]
    R = 2 * (M + SEG)
    NSEG = S // SEG
    NRB = (NSEG - 1) // RB
    NB = S // CB
    QB = CB // NQ
    NCH = 3 * H // HG
    DP = -(-DM // 256) * 256
    fwd, inv = _dft_constants()

    kern = functools.partial(_kernel, S=S, DM=DM, H=H, DH=DH, M=M, SEG=SEG)
    any_spec = pl.BlockSpec(memory_space=pl.ANY)
    out = pl.pallas_call(
        kern,
        out_shape=jax.ShapeDtypeStruct((S, DM), A_x.dtype),
        in_specs=[any_spec] * 13,
        out_specs=any_spec,
        scratch_shapes=[
            pltpu.VMEM((NB + 2, NQ, QB // 8, DM // 128, 4, 8, 128), F32),
            pltpu.VMEM((NQ, 2 * QB, DM), F32),
            pltpu.VMEM((2, NQ, 2 * QB, DM), BF16),
            pltpu.VMEM((4, SEG, DM), F32),
            pltpu.VMEM((4, SEG, DM), F32),
            pltpu.VMEM((S, DP), BF16),
            pltpu.VMEM((SEG, DM), F32),
            pltpu.VMEM((NSEG, NPA, SEG, DH), F32),
            pltpu.VMEM((NPB, SEG, DH), F32),
            pltpu.VMEM((NSEG, SEG // 2, DP), U32),
            pltpu.VMEM((NCH - NRB + 2, HG, DM // 2, DH), U32),
            pltpu.VMEM((NRB - 1, HG, DM // 2, DH), U32),
            pltpu.VMEM((H * DH, DM), BF16),
            pltpu.VMEM((R // 2, H * DH), U32),
            pltpu.VMEM((S, DP), BF16),
            pltpu.VMEM((S, DP), BF16),
            pltpu.VMEM((NB, DM, CB), BF16),
            pltpu.VMEM((NCH, DM // 2, 2 * HG, DH), BF16),
            pltpu.VMEM((S, DP), A_x.dtype),
            pltpu.VMEM(fwd.shape, BF16),
            pltpu.VMEM(inv.shape, BF16),
            pltpu.VMEM((S + KPAD, DP), BF16),
            pltpu.VMEM((RB * SEG // 2, DM), U32),
            pltpu.VMEM((M + SEG // 2, DM), U32),
            pltpu.VMEM((KS + 1, 8, DM), F32),
            pltpu.VMEM((M, DM), BF16),
            pltpu.VMEM((KS, DM), BF16),
            pltpu.VMEM((DM,), BF16),
            pltpu.SMEM((1,), jnp.int32),
            pltpu.SemaphoreType.DMA(((NSEG - 1) // RB,)),
            pltpu.SemaphoreType.DMA((3,)),
            pltpu.SemaphoreType.DMA((NCH + 2,)),
            pltpu.SemaphoreType.DMA(()),
        ],
        compiler_params=pltpu.CompilerParams(vmem_limit_bytes=120 * 1024 * 1024),
    )(
        A_x.reshape(S, DM), A_mem0.reshape(M, DM), A_Wq, A_Wk, A_Wv,
        A_Wo.reshape(H * DH, DM), B_k.reshape(S, DM), B_v.reshape(S, DM),
        B_shift_k.T, B_ssm_k, B_ssm_D,
        jnp.asarray(fwd, BF16), jnp.asarray(inv, BF16),
    )
    return out.reshape(B, S, DM)
```

```python
import functools

import numpy as np
import jax
import jax.numpy as jnp
import jax.experimental.pallas as pl
import jax.experimental.pallas.tpu as pltpu

F32 = jnp.float32
BF16 = jnp.bfloat16
U32 = jnp.uint32

CB = 128
NQ = 4
KPAD = 16
HG = 8
NPA = 16
NPB = 14
RB = 9
PRO_PW, PRO_X0, PRO_XS, PRO_R0, PRO_RS = 24, 11, 4, 2, 2
UNROLL = 3
PHI = 3
PIN_U2, X4S = 1, 0
INV_AT = 22
SPEC_AT, PIN_U, PIN_X4 = 7, 1, 16
DIST, DIST_HALF, DIST_LAST = (1, 2), (1, 3), (2, 3)


def _dft_constants():
    qb = CB // NQ
    hb = qb // 2
    n = np.arange(CB, dtype=np.float64)
    f = np.concatenate([q * qb + np.concatenate([np.arange(0, qb, 2), np.arange(1, qb, 2)])
                        for q in range(NQ)])
    w = np.pi * (2.0 * f + 1.0) / (2 * CB)
    ang = (w[:, None] * (n[None, :] - (CB - 1) / 4.0)).reshape(NQ, qb, CB)
    fwd = np.concatenate([np.cos(ang), -np.sin(ang)], axis=1)
    inv = np.zeros((NQ, 2, hb, CB))
    for p in range(NQ):
        m = (NQ - 1 - p) * hb + np.arange(hb)
        ang = (m[:, None] + 0.5) * w[None, :]
        inv[p, 0] = np.cos(ang) / CB
        inv[p, 1] = -np.sin(ang) / CB
    return fwd.astype(np.float32), inv.astype(np.float32)


def _flip_rows(x):
    i = jax.lax.broadcasted_iota(jnp.int32, (8, x.shape[1]), 0)
    out = []
    for r in range(x.shape[0] - 8, -8, -8):
        v = pltpu.roll(x[r:r + 8], 4, 0)
        for b in (2, 1):
            v = jnp.where((i & b) == 0, pltpu.roll(v, 8 - b, 0), pltpu.roll(v, b, 0))
        out.append(v)
    return jnp.concatenate(out, axis=0)


def _ln(x, eps=1e-5):
    d = x.shape[-1]
    m = jnp.sum(x, axis=-1, keepdims=True) * (1.0 / d)
    xc = x - m
    v = jnp.sum(xc * xc, axis=-1, keepdims=True) * (1.0 / d)
    return xc * jax.lax.rsqrt(v + eps)


def _dot(a, b):
    return jnp.dot(a, b, preferred_element_type=F32)


def _dot_nt(a, b):
    return jax.lax.dot_general(a, b, (((1,), (1,)), ((), ())), preferred_element_type=F32)


def _pack(x):
    return pltpu.bitcast(x.astype(BF16), U32)


def _unpack(x):
    return pltpu.bitcast(x, BF16)


def _in_order(actions):
    def body(i, c):
        for j, act in enumerate(actions):
            pl.when(i == j)(act)
        return c
    jax.lax.fori_loop(0, len(actions), body, 0)


def _kernel(x_hbm, mem0_hbm, wq_hbm, wk_hbm, wv_hbm, wo_hbm, k_hbm, v_hbm,
            sh_hbm, sk_hbm, sd_hbm, fwd_hbm, inv_hbm, o_hbm,
            sp_sc, kr_sc, wf_sc, x2_sc, y_sc, u_sc, op_sc, pre_sc, fill_sc, xn_sc, wa_sc, wb_sc, wo_sc, o_sc,
            x_sc, v_sc, sk_sc, st_sc, out_sc, fwd_ref, inv_ref,
            k_sc, hp_sc, h_sc, co_sc, mem0_ref, sh_ref, sd_ref,
            never_sm, sem_x, sem_in, sem_w, sem_out,
            *, S, DM, H, DH, M, SEG):
    NSEG = S // SEG
    M2 = 2 * M
    S2 = SEG // 2
    R = M2 + 2 * SEG
    RH = M2 + SEG
    NB = S // CB
    QB = CB // NQ
    HB = QB // 2
    NT = DM // 128
    PH = PHI * UNROLL
    NRB = (NSEG - 1) // RB
    NPH = (NSEG - 1) // PH
    NG = H // HG
    NCH = 3 * NG
    NPASS = NPA // HG
    DH2 = DM // 2
    KS = sh_ref.shape[0]
    UL = 2 * NQ + 1
    LN = pl.ds(0, DM)
    assert 2 <= KS <= 8 and QB == SEG and NRB * RB == NSEG - 1 and NPH * PH == NSEG - 1 and NPASS == 2 and 2 * NRB >= NCH + 1

    mem0_copy = pltpu.make_async_copy(mem0_hbm, mem0_ref, sem_x.at[0])
    small = [pltpu.make_async_copy(s, d, sem_in.at[0]) for s, d in [
        (sh_hbm, sh_ref), (sd_hbm, sd_ref), (fwd_hbm, fwd_ref), (inv_hbm, inv_ref)]]

    def x_copy(b):
        if isinstance(b, int) and b == 0:
            rows = pl.ds(0, (RB + 1) * SEG)
        else:
            rows = pl.ds(pl.multiple_of((b * RB + 1) * SEG, SEG), RB * SEG)
        return pltpu.make_async_copy(x_hbm.at[rows], x_sc.at[rows, LN], sem_x.at[b])

    kb = (0, (UL + 1) * SEG, (UL + PH + 1) * SEG, S)
    sb = (0, 2, (PH + 2) // NQ + 2, NB)

    def in_copies(part):
        def rng(b):
            return pl.ds(b[part], b[part + 1] - b[part])
        sem = sem_in.at[part]
        return [
            pltpu.make_async_copy(k_hbm.at[rng(kb)],
                                  k_sc.at[pl.ds(KPAD + kb[part], kb[part + 1] - kb[part]), LN], sem),
            pltpu.make_async_copy(v_hbm.at[rng(kb)], v_sc.at[rng(kb), LN], sem),
        ] + [pltpu.make_async_copy(sk_hbm.at[:, pl.ds(c * CB, CB)], sk_sc.at[c], sem)
             for c in range(sb[part], sb[part + 1])]

    def w_copies(ci, dst=None, part=None):
        src = (wq_hbm, wk_hbm, wv_hbm)[ci // NG]
        dst = ci if dst is None else dst
        lo, n = (0, DH2) if part is None else (part * DH2 // 2, DH2 // 2)
        sem = sem_w.at[NCH + 1 if part == 1 else dst]
        return [pltpu.make_async_copy(src.at[pl.ds(hf * DH2 + lo, n), pl.ds((ci % NG) * HG, HG), :],
                                      st_sc.at[dst, pl.ds(lo, n), pl.ds(hf * HG, HG), :], sem)
                for hf in range(2)]

    wo_copy = pltpu.make_async_copy(wo_hbm, wo_sc, sem_w.at[NCH])

    def out_copy(lo, n):
        rows = pl.ds(lo * SEG if isinstance(lo, int) else pl.multiple_of(lo * SEG, SEG), n * SEG)
        return pltpu.make_async_copy(out_sc.at[rows, LN], o_hbm.at[rows], sem_out)

    def start_all(cps):
        def act():
            for cp in cps:
                cp.start()
        return act

    order = [[mem0_copy, x_copy(0)], w_copies(0, part=0), w_copies(0, part=1), [x_copy(1)], [x_copy(2)]]
    for ci in range(1, NCH):
        order.append(w_copies(ci) + ([x_copy(ci + 2)] if ci + 2 < NRB else []))
        if ci == NRB - 2:
            order.append(small + in_copies(0))
    order += [[wo_copy], in_copies(1), in_copies(2)]
    for i in range(0, len(order), 5):
        _in_order([start_all(cps) for cps in order[i:i + 5]])

    never_sm[0] = 0
    k_sc[0:KPAD, LN] = jnp.zeros((KPAD, DM), BF16)
    sp_sc[NB + 1] = jnp.zeros(sp_sc.shape[1:], F32)
    op_sc[...] = jnp.zeros(op_sc.shape, F32)
    x2_sc[...] = jnp.zeros(x2_sc.shape, F32)
    y_sc[2 * CB - SEG:, LN] = jnp.zeros((SEG, DM), F32)
    mem0_copy.wait()
    x_copy(0).wait()
    for sg in range(RB + 1):
        xn_sc[sg, :, 0:DM] = _pack(_ln(x_sc[sg * SEG:(sg + 1) * SEG, LN].astype(F32)))

    def clip(i, hi):
        return min(max(i, 0), hi) if isinstance(i, int) else jnp.clip(i, 0, hi)

    def scaled(i, m):
        return i * m if isinstance(i, int) else pl.multiple_of(i * m, m)

    def seg(i):
        return pl.ds(scaled(clip(i, NSEG - 1), SEG), SEG)

    def conv_u(s, ln=LN):
        r0 = scaled(clip(s, NSEG - 1), SEG)
        kk = k_sc[pl.ds(r0, KPAD + SEG), ln].astype(F32)[KPAD - 8:]

        def coef(j, rows):
            return jnp.concatenate([co_sc[j, :, ln]] * (rows // 8), axis=0)
        sft = [kk] + [pltpu.roll(kk, j, 0) for j in range(2, KS, 2)]
        ev = functools.reduce(jnp.add, [sft[j // 2][8:] * coef(j, SEG) for j in range(0, KS, 2)])
        od = functools.reduce(jnp.add, [sft[j // 2] * coef(j, SEG + 8) for j in range(1, KS, 2)])
        ks = ev + pltpu.roll(od, 1, 0)[8:]
        u = (ks * v_sc[pl.ds(r0, SEG), ln].astype(F32)).astype(BF16)
        u_sc[pl.ds(r0, SEG), ln] = u
        return u

    def conv_fwd(c, q):
        cc = clip(c, NB - 1)
        f = fwd_ref[q]
        uf = _dot(f, u_sc[pl.ds(scaled(cc, CB), CB), LN])
        kf = _dot_nt(f, sk_sc[cc])
        return uf, kf

    def put_spec(cs, q, which, val):
        for n in range(NT):
            v = val[:, n * 128:(n + 1) * 128].reshape(2, QB // 8, 8, 128)
            sp_sc[cs, q, :, n, which:which + 2] = jnp.stack([v[0], v[1]], axis=1)

    def conv_spec(c, q):
        uf, kf = conv_fwd(c, q)
        cs = clip(c, NB)
        put_spec(cs, q, 0, uf)
        pk = kr_sc[q]
        kr_sc[q] = kf
        kp = jnp.concatenate([
            kf[0:HB] - pk[QB:QB + HB],
            kf[HB:QB] + pk[QB + HB:],
            kf[QB:QB + HB] + pk[0:HB],
            kf[QB + HB:] - pk[HB:QB]], axis=0)
        put_spec(cs, q, 2, kp)

    MAC_PIECES = [(rb, n) for rb in range(QB // 16) for n in range(NT)]

    def conv_mac(c, q, piece, nterms):
        rb2, n = piece
        cs = clip(c, NB)
        rbs = slice(2 * rb2, 2 * rb2 + 2)
        ar = None
        ai = None
        for j in range(nterms):
            if isinstance(cs, int):
                uj, kj = j, cs - j
            else:
                uj = jnp.minimum(j, cs)
                kj = jnp.where(cs - j >= 0, cs - j, NB + 1)
            u = sp_sc[uj, q, rbs, n, 0:2]
            k = sp_sc[kj, q, rbs, n, 2:4]
            tr = u[:, 0] * k[:, 0] - u[:, 1] * k[:, 1]
            ti = u[:, 0] * k[:, 1] + u[:, 1] * k[:, 0]
            ar = tr if ar is None else ar + tr
            ai = ti if ai is None else ai + ti
        ln = slice(n * 128, (n + 1) * 128)
        w = jnp.concatenate([ar.reshape(16, 128), ai.reshape(16, 128)], axis=0).astype(BF16)
        wf_sc[c & 1, 0, q, rb2 * 16:rb2 * 16 + 16, ln] = w[0:16]
        wf_sc[c & 1, 1, q, rb2 * 16:rb2 * 16 + 16, ln] = w[16:]

    def conv_inv(tt, n):
        cb = tt // NQ
        p = tt % NQ
        ln = slice(n * 128, (n + 1) * 128)
        ev = _dot(inv_ref[p, 0], wf_sc[cb & 1, 0, :, :, ln].reshape(CB, 128))
        od = _dot(inv_ref[p, 1], wf_sc[cb & 1, 1, :, :, ln].reshape(CB, 128))
        sd = jnp.concatenate([co_sc[KS, :, ln]] * (HB // 8), axis=0)
        for r, val in ((p, _flip_rows(ev - od)), (2 * NQ - 1 - p, ev + od)):
            ur = scaled(clip(cb, NB - 1) * (2 * NQ) + r, HB)
            yr = scaled((cb & 1) * (2 * NQ) + r, HB)
            y_sc[pl.ds(yr, HB), ln] = val + u_sc[pl.ds(ur, HB), ln].astype(F32) * sd

    def y_seg(s):
        return y_sc[pl.ds(scaled(s & (2 * NQ - 1), SEG), SEG), LN]

    scale = DH ** -0.5
    cexp = scale * float(np.log2(np.e))

    def make_mask(n, x_layers, q0=0):
        qi = jax.lax.broadcasted_iota(jnp.int32, (n - q0, n), 0) + q0
        ki = jax.lax.broadcasted_iota(jnp.int32, (n - q0, n), 1)

        def layer(i):
            xl = jnp.where(i < M2 + SEG, x_layers[0], x_layers[-1])
            return jnp.where(i < M, 0, jnp.where(i < M2, 1, xl))
        same = layer(qi) == layer(ki)
        ok = same & ((qi < M2) | (ki < M2) | (qi >= ki))
        fill = jnp.where(same, -1e9 / scale, -jnp.inf).astype(F32)
        return ok, fill

    def probs(q, k, mask):
        ok, fill = mask
        s = _dot_nt(q, k)
        s = jnp.where(ok, s, fill)
        m = jnp.max(s, axis=-1, keepdims=True)
        p = jnp.exp2((s - m) * cexp)
        l = jnp.sum(p, axis=-1, keepdims=True)
        r = pl.reciprocal(l, approx=True)
        r = r * (2.0 - l * r)
        return (p * r).astype(BF16)

    def w_slot(ci):
        return (wb_sc, ci) if 1 <= ci < NRB - 1 else (wa_sc, max(ci - (NRB - 2), 0))

    def w_pos(j):
        return (j % 2) * (HG // 2) + j // 2

    def w_head(g, mats):
        slots = [w_slot(mi * NG + g // HG) for mi in mats]
        return _unpack(jnp.concatenate([ref[i, w_pos(g % HG)] for ref, i in slots], axis=1))

    def proj_split(hq, hkv, g, q1=None):
        q = _dot(hq, w_head(g, (0,)))
        kv = _dot(hkv, w_head(g, (1, 2)))
        if q1 is not None:
            q = jnp.concatenate([q[0:M2], q1, q[M2:]], axis=0)
        return q.astype(BF16), kv[:, :DH].astype(BF16), kv[:, DH:].astype(BF16)

    def xn(s):
        return _unpack(xn_sc[clip(s, NSEG - 1), :, 0:DM])

    def out_proj(n, g0, g1, j):
        return _dot(_unpack(o_sc[0:n // 2, g0 * DH:g1 * DH]),
                    wo_sc[g0 * DH:g1 * DH, j * 128:(j + 1) * 128])

    def attend(proj, n, mask, dist, hook=None, early=True):
        D1, D2 = dist
        HA = H - D1 - D2 - 1
        NE = min(D1 + D2, NT - 1) if early else 0
        qkvs = {}
        ps = {}
        outs = {}
        for it in range(H + D1 + D2):
            if it < H:
                qkvs[it] = proj(it)
            g = it - D1
            if 0 <= g < H:
                ps[g] = probs(qkvs[g][0], qkvs[g][1], mask)
            g = it - D1 - D2
            if 0 <= g < H:
                o = _dot(ps.pop(g), qkvs.pop(g)[2])
                o_sc[0:n // 2, g * DH:(g + 1) * DH] = _pack(o)
            if hook is not None:
                hook(it)
            j = it - (H - 1)
            if 0 <= j < NE:
                outs[j] = out_proj(n, 0, HA, j)
        for j in range(NE, NT):
            outs[j] = out_proj(n, 0, H, j)
            if hook is not None:
                hook(H + D1 + D2 + j)
        for j in range(NE):
            outs[j] = out_proj(n, HA, H, j) + outs[j]
        return jnp.concatenate([outs[j] for j in range(NT)], axis=1)

    def side2(t, a2):
        x3 = x2_sc[(t - 2) & 3] + a2
        x4 = x3 + _ln(x3) * y_seg(t - 2)
        x4 = x4.astype(out_sc.dtype)
        out_sc[seg(t - 2), LN] = x4
        return x4

    def fill(s, heads):
        xq = xn(s)
        for g in heads:
            fill_sc[g - NPA] = _dot(xq, w_head(g, (0,)))

    def finish(t, xr, yt, mem, a1, spec):
        if spec:
            conv_spec((t + 2) // NQ + 1, (t + 2) % NQ)
        fill(t + 1, range(NPA, NPA + NPB))
        x1 = xr.astype(F32) + a1
        x2 = x1 + _ln(x1) * yt
        h_sc[0:M, :] = _pack(mem)
        h_sc[M:, :] = _pack(_ln(x2))
        x2_sc[t & 3] = x2

    def pinned(rows, pins):
        never = never_sm[0] > 0
        hs = {0: rows}
        r = _pack(rows)
        tiles = [r[:, n * 128:(n + 1) * 128] for n in range(NT)]
        for g, n, d in sorted(pins, key=lambda p: p[0]):
            tiles[n] = jnp.where(never, d, tiles[n])
            hs[g] = _unpack(jnp.concatenate(tiles, axis=1))
        return lambda g: hs[max(k for k in hs if k <= g)]

    def pin_tiles(g0, stride, val):
        v = _pack(val)
        return [(g0 + n * stride, n, v[:, n * 128:(n + 1) * 128]) for n in range(NT)]

    def wait_chunk(ci):
        for cp in w_copies(0, ci):
            cp.wait()

    def relayout(ci, dst, slot, b):
        d0 = scaled(b, 16)
        r0 = scaled(b, 8)
        xw = pltpu.bitcast(st_sc[ci, pl.ds(d0, 16)], U32).reshape(8, 2, HG, DH)
        a = xw[:, 0]
        bb = xw[:, 1]
        lo = jnp.swapaxes((a & U32(0xFFFF)) | (bb << 16), 0, 1)
        hi = jnp.swapaxes((a >> 16) | (bb & U32(0xFFFF0000)), 0, 1)
        for hf in range(2):
            rows = pl.ds(r0 + hf * (DH2 // 2), 8)
            dst[slot, 0:HG // 2, rows, :] = lo[hf * HG // 2:(hf + 1) * HG // 2]
            dst[slot, HG // 2:HG, rows, :] = hi[hf * HG // 2:(hf + 1) * HG // 2]

    def everything(_, carry):
        NBLK = DH2 // 16
        def relayout0(b, c):
            relayout(0, wa_sc, 0, b)
            return c
        for part in range(2):
            with jax.named_scope("wait_w"):
                for cp in w_copies(0, part=part):
                    cp.wait()
            with jax.named_scope("relayout"):
                jax.lax.fori_loop(part * NBLK // 2, (part + 1) * NBLK // 2, relayout0, 0, unroll=2)

        def pro_stage(ps_, b):
            n = ps_ * NRB + b
            with jax.named_scope("wait_w"):
                if ps_ == 0:
                    @pl.when(b + 1 < NRB)
                    def _():
                        x_copy(b + 1).wait()

                @pl.when((n >= 2) & (n <= NCH))
                def _():
                    wait_chunk(n - 1)
            cr = jnp.clip(n - 1, 0, NCH - 1)
            dst, slot = (wb_sc, cr) if ps_ == 0 else (wa_sc, cr - (NRB - 2))
            src, si = w_slot(ps_)
            bl = jnp.minimum(b + 1, NRB - 1)
            PW = PRO_PW
            npc = RB * S2 // PW
            assert npc * PW == RB * S2 and PRO_R0 + (NBLK - 1) * PRO_RS < HG * npc
            assert PRO_X0 + (max(RB, 2 * NT) - 1) * PRO_XS < HG * npc and 2 * NRB > UL

            def body(i, c):
                s0 = b * RB + 1
                for sg in range(RB):
                    hp_sc[sg * S2:(sg + 1) * S2, :] = xn_sc[s0 + sg, :, 0:DM]
                for j in range(HG):
                    w = _unpack(src[si, w_pos(j)])
                    for pi in range(npc):
                        pos = j * npc + pi
                        hx = hp_sc[pi * PW:(pi + 1) * PW, :]
                        k, rem = divmod(pos - PRO_X0, PRO_XS)
                        if ps_ == 0 and rem == 0 and 0 <= k < RB:
                            sn = bl * RB + 1 + k
                            xv = _pack(_ln(x_sc[seg(sn), LN].astype(F32)))
                            xn_sc[sn, :, 0:DM] = xv
                            hx = jnp.concatenate([hx[:-S2], jnp.where(never_sm[0] > 0, xv, hx[-S2:])], axis=0)
                        if ps_ == 1 and rem == 0 and 0 <= k < 2 * NT:
                            conv_u(jnp.minimum(2 * b + k // NT, UL),
                                   slice((k % NT) * 128, (k % NT + 1) * 128))
                        bb, rem = divmod(pos - PRO_R0, PRO_RS)
                        if rem == 0 and 0 <= bb < NBLK:
                            relayout(cr, dst, slot, bb)
                        r = _dot(_unpack(hx), w)
                        for a in range(0, 2 * PW, 16):
                            sg, off = divmod(2 * pi * PW + a, SEG)
                            pre_sc[s0 + sg, ps_ * HG + j, off:off + 16, :] = r[a:a + 16]
                return c
            with jax.named_scope("fused"):
                jax.lax.fori_loop(0, never_sm[0] + 1, body, 0)

        for ps_ in range(NPASS):
            if ps_ == 1:
                with jax.named_scope("wait_in0"):
                    for cp in small + in_copies(0):
                        cp.wait()
                sh = sh_ref[...].astype(F32)
                for j in range(KS):
                    co_sc[j] = jnp.broadcast_to(sh[j:j + 1], (8, DM))
                co_sc[KS] = jnp.broadcast_to(sd_ref[...].astype(F32).reshape(1, DM), (8, DM))

            def blk(b, c, ps_=ps_):
                pro_stage(ps_, b)
                return c
            jax.lax.fori_loop(0, NRB, blk, 0)

        def warm_block0(q):
            uf, kf = conv_fwd(0, q)
            put_spec(0, q, 0, uf)
            put_spec(0, q, 2, kf)
            kr_sc[q] = kf
            ur, um, kr, km = uf[:QB], uf[QB:], kf[:QB], kf[QB:]
            wf_sc[0, 0, q] = (ur * kr - um * km).astype(BF16)
            wf_sc[0, 1, q] = (ur * km + um * kr).astype(BF16)

        with jax.named_scope("step0"):
            mem0 = mem0_ref[...].astype(F32)
            h0 = jnp.concatenate([jnp.concatenate([mem0, mem0], axis=0).astype(BF16), xn(0)], axis=0)

            def hook0(it):
                j = it - (H - 1)
                if 0 <= j < NQ:
                    warm_block0(j)
                j = it - (H + sum(DIST_HALF))
                if j == -1:
                    conv_spec(1, 0)
                    wo_copy.wait()
                    conv_spec(1, 1)
                    for q in range(2):
                        for piece in MAC_PIECES:
                            conv_mac(1, q, piece, 2)
                if 0 <= j < 3:
                    for n in range(NT):
                        conv_inv(j, n)
            out = attend(lambda g: proj_split(h0, h0, g), RH, make_mask(RH, (0,)), DIST_HALF, hook0, False)
            finish(0, x_sc[0:SEG, LN], y_seg(0), jnp.concatenate([out[0:M], mem0], axis=0), out[M2:], False)

        mask12 = make_mask(R, (0, 1))

        def step(t, first, last):
            if first:
                conv_spec_later = functools.partial(conv_spec, (t + 1) // NQ + 1, (t + 1) % NQ)
            x4 = side2(t, op_sc[...])
            un = conv_u(t + UL)
            hm = _unpack(h_sc[0:M, :])
            hx2 = _unpack(h_sc[M:, :])
            h48 = jnp.concatenate([hm, hx2], axis=0)
            x1n = pinned(xn(t), pin_tiles(PIN_U if first else PIN_U2, 1, un) + pin_tiles(PIN_X4, X4S, x4))

            def proj(g):
                h80 = jnp.concatenate([hm, x1n(g), hx2], axis=0)
                if g >= NPA + NPB:
                    return proj_split(h80, h80, g)
                return proj_split(h48, h80, g, pre_sc[t, g] if g < NPA else fill_sc[g - NPA])

            held = {}

            def hook(it):
                if it == SPEC_AT:
                    if first:
                        conv_spec_later()
                    for piece in MAC_PIECES:
                        conv_mac((t + 1) // NQ + 1, (t + 1) % NQ, piece, NB)
                if INV_AT <= it < INV_AT + NT:
                    conv_inv(t + 2, it - INV_AT)
                if it == H:
                    held["x"] = x_sc[seg(t), LN]
                    held["y"] = y_seg(t)
            out = attend(proj, R, mask12, DIST, hook)
            op_sc[...] = out[RH:]
            finish(t, held["x"], held["y"], out[0:M2], out[M2:RH], not last)

        def steps(i, carry):
            for j in range(UNROLL):
                step(1 + i * UNROLL + j, j == 0, j == UNROLL - 1)
            return carry

        def phase(p, carry):
            @pl.when(p == 1)
            def _():
                for cp in in_copies(2):
                    cp.wait()

            @pl.when(p >= 2)
            def _():
                out_copy((p - 2) * PH, PH).start()

            with jax.named_scope("steps"):
                jax.lax.fori_loop(p * PHI, (p + 1) * PHI, steps, 0)
            return carry

        for cp in in_copies(1):
            cp.wait()
        jax.lax.fori_loop(0, NPH, phase, 0)
        out_copy((NPH - 2) * PH, NSEG - 2 - (NPH - 2) * PH).start()

        with jax.named_scope("step_last"):
            x4 = side2(NSEG, op_sc[...])
            hm = _unpack(h_sc[0:M, :])
            hx = pinned(_unpack(h_sc[M:, :]), pin_tiles(PIN_X4, 0, x4))
            out = attend(lambda g: proj_split(hx(g), jnp.concatenate([hm, hx(g)], axis=0), g),
                         SEG, make_mask(RH, (1,), M2), DIST_LAST)
            side2(NSEG + 1, out)
        out_copy(NSEG - 2, 2).start()
        out_copy(0, NSEG).wait()
        return carry

    jax.lax.fori_loop(0, never_sm[0] + 1, everything, 0)


def pallas_interleave_layers__memory_aug_recurrent_mem_tr__ssm_conv_h3__prompt_kernel(
    A_x, A_mem0, A_Wq, A_Wk, A_Wv, A_Wo, A_seg_len,
    B_q, B_k, B_v, B_shift_k, B_ssm_k, B_ssm_D,
):
    del B_q
    seg = int(A_seg_len) if isinstance(A_seg_len, (int, np.integer)) else CB // NQ
    return _run(A_x, A_mem0, A_Wq, A_Wk, A_Wv, A_Wo, B_k, B_v, B_shift_k, B_ssm_k, B_ssm_D, SEG=seg)


@functools.partial(jax.jit, static_argnames=("SEG",))
def _run(A_x, A_mem0, A_Wq, A_Wk, A_Wv, A_Wo, B_k, B_v, B_shift_k, B_ssm_k, B_ssm_D, *, SEG):
    B, S, DM = A_x.shape
    assert B == 1
    H, DH = A_Wq.shape[1], A_Wq.shape[2]
    M = A_mem0.shape[1]
    KS = B_shift_k.shape[1]
    R = 2 * (M + SEG)
    NSEG = S // SEG
    NRB = (NSEG - 1) // RB
    NB = S // CB
    QB = CB // NQ
    NCH = 3 * H // HG
    DP = -(-DM // 256) * 256
    fwd, inv = _dft_constants()

    kern = functools.partial(_kernel, S=S, DM=DM, H=H, DH=DH, M=M, SEG=SEG)
    any_spec = pl.BlockSpec(memory_space=pl.ANY)
    out = pl.pallas_call(
        kern,
        out_shape=jax.ShapeDtypeStruct((S, DM), A_x.dtype),
        in_specs=[any_spec] * 13,
        out_specs=any_spec,
        scratch_shapes=[
            pltpu.VMEM((NB + 2, NQ, QB // 8, DM // 128, 4, 8, 128), F32),
            pltpu.VMEM((NQ, 2 * QB, DM), F32),
            pltpu.VMEM((2, 2, NQ, QB, DM), BF16),
            pltpu.VMEM((4, SEG, DM), F32),
            pltpu.VMEM((2 * CB, DP), F32),
            pltpu.VMEM((S, DP), BF16),
            pltpu.VMEM((SEG, DM), F32),
            pltpu.VMEM((NSEG, NPA, SEG, DH), F32),
            pltpu.VMEM((NPB, SEG, DH), F32),
            pltpu.VMEM((NSEG, SEG // 2, DP), U32),
            pltpu.VMEM((NCH - NRB + 2, HG, DM // 2, DH), U32),
            pltpu.VMEM((NRB - 1, HG, DM // 2, DH), U32),
            pltpu.VMEM((H * DH, DM), BF16),
            pltpu.VMEM((R // 2, H * DH), U32),
            pltpu.VMEM((S, DP), BF16),
            pltpu.VMEM((S, DP), BF16),
            pltpu.VMEM((NB, DM, CB), BF16),
            pltpu.VMEM((NCH, DM // 2, 2 * HG, DH), BF16),
            pltpu.VMEM((S, DP), A_x.dtype),
            pltpu.VMEM(fwd.shape, BF16),
            pltpu.VMEM(inv.shape, BF16),
            pltpu.VMEM((S + KPAD, DP), BF16),
            pltpu.VMEM((RB * SEG // 2, DM), U32),
            pltpu.VMEM((M + SEG // 2, DM), U32),
            pltpu.VMEM((KS + 1, 8, DM), F32),
            pltpu.VMEM((M, DM), BF16),
            pltpu.VMEM((KS, DM), BF16),
            pltpu.VMEM((DM,), BF16),
            pltpu.SMEM((1,), jnp.int32),
            pltpu.SemaphoreType.DMA(((NSEG - 1) // RB,)),
            pltpu.SemaphoreType.DMA((3,)),
            pltpu.SemaphoreType.DMA((NCH + 2,)),
            pltpu.SemaphoreType.DMA(()),
        ],
        compiler_params=pltpu.CompilerParams(vmem_limit_bytes=120 * 1024 * 1024),
    )(
        A_x.reshape(S, DM), A_mem0.reshape(M, DM), A_Wq, A_Wk, A_Wv,
        A_Wo.reshape(H * DH, DM), B_k.reshape(S, DM), B_v.reshape(S, DM),
        B_shift_k.T, B_ssm_k, B_ssm_D,
        jnp.asarray(fwd, BF16), jnp.asarray(inv, BF16),
    )
    return out.reshape(B, S, DM)
```

```python
import functools

import numpy as np
import jax
import jax.numpy as jnp
import jax.experimental.pallas as pl
import jax.experimental.pallas.tpu as pltpu

F32 = jnp.float32
BF16 = jnp.bfloat16
U32 = jnp.uint32

CB = 128
NQ = 4
KPAD = 16
HG = 8
NPA = 16
NPB = 14
RB = 9
PRO_PW, PRO_X0, PRO_XS, PRO_R0, PRO_RS = 24, 11, 4, 2, 2
UNROLL = 3
PHI = 3
SPEC_AT, INV_AT, PIN_U, PIN_X4 = 7, 22, 1, 16
DIST, DIST_HALF, DIST_LAST = (1, 2), (1, 3), (2, 3)


def _dft_constants():
    qb = CB // NQ
    hb = qb // 2
    n = np.arange(CB, dtype=np.float64)
    f = np.concatenate([q * qb + np.concatenate([np.arange(0, qb, 2), np.arange(1, qb, 2)])
                        for q in range(NQ)])
    w = np.pi * (2.0 * f + 1.0) / (2 * CB)
    ang = (w[:, None] * (n[None, :] - (CB - 1) / 4.0)).reshape(NQ, qb, CB)
    fwd = np.concatenate([np.cos(ang), -np.sin(ang)], axis=1)
    inv = np.zeros((NQ, 2, hb, CB))
    for p in range(NQ):
        m = (NQ - 1 - p) * hb + np.arange(hb)
        ang = (m[:, None] + 0.5) * w[None, :]
        inv[p, 0] = np.cos(ang) / CB
        inv[p, 1] = -np.sin(ang) / CB
    return fwd.astype(np.float32), inv.astype(np.float32)


def _flip_rows(x):
    i = jax.lax.broadcasted_iota(jnp.int32, (8, x.shape[1]), 0)
    out = []
    for r in range(x.shape[0] - 8, -8, -8):
        v = pltpu.roll(x[r:r + 8], 4, 0)
        for b in (2, 1):
            v = jnp.where((i & b) == 0, pltpu.roll(v, 8 - b, 0), pltpu.roll(v, b, 0))
        out.append(v)
    return jnp.concatenate(out, axis=0)


def _ln(x, eps=1e-5):
    d = x.shape[-1]
    m = jnp.sum(x, axis=-1, keepdims=True) * (1.0 / d)
    xc = x - m
    v = jnp.sum(xc * xc, axis=-1, keepdims=True) * (1.0 / d)
    return xc * jax.lax.rsqrt(v + eps)


def _dot(a, b):
    return jnp.dot(a, b, preferred_element_type=F32)


def _dot_nt(a, b):
    return jax.lax.dot_general(a, b, (((1,), (1,)), ((), ())), preferred_element_type=F32)


def _pack(x):
    return pltpu.bitcast(x.astype(BF16), U32)


def _unpack(x):
    return pltpu.bitcast(x, BF16)


def _in_order(actions):
    def body(i, c):
        for j, act in enumerate(actions):
            pl.when(i == j)(act)
        return c
    jax.lax.fori_loop(0, len(actions), body, 0)


def _kernel(x_hbm, mem0_hbm, wq_hbm, wk_hbm, wv_hbm, wo_hbm, k_hbm, v_hbm,
            sh_hbm, sk_hbm, sd_hbm, fwd_hbm, inv_hbm, o_hbm,
            sp_sc, kr_sc, wf_sc, x2_sc, y_sc, u_sc, op_sc, pre_sc, fill_sc, xn_sc, wa_sc, wb_sc, wo_sc, o_sc,
            x_sc, v_sc, sk_sc, st_sc, out_sc, fwd_ref, inv_ref,
            k_sc, hp_sc, h_sc, co_sc, mem0_ref, sh_ref, sd_ref,
            never_sm, sem_x, sem_in, sem_w, sem_out,
            *, S, DM, H, DH, M, SEG):
    NSEG = S // SEG
    M2 = 2 * M
    S2 = SEG // 2
    R = M2 + 2 * SEG
    RH = M2 + SEG
    NB = S // CB
    QB = CB // NQ
    HB = QB // 2
    NT = DM // 128
    PH = PHI * UNROLL
    NRB = (NSEG - 1) // RB
    NPH = (NSEG - 1) // PH
    NG = H // HG
    NCH = 3 * NG
    NPASS = NPA // HG
    DH2 = DM // 2
    KS = sh_ref.shape[0]
    UL = 2 * NQ + 1
    LN = pl.ds(0, DM)
    assert 2 <= KS <= 8 and QB == SEG and NRB * RB == NSEG - 1 and NPH * PH == NSEG - 1 and NPASS == 2 and 2 * NRB >= NCH + 1

    mem0_copy = pltpu.make_async_copy(mem0_hbm, mem0_ref, sem_x.at[0])
    small = [pltpu.make_async_copy(s, d, sem_in.at[0]) for s, d in [
        (sh_hbm, sh_ref), (sd_hbm, sd_ref), (fwd_hbm, fwd_ref), (inv_hbm, inv_ref)]]

    def x_copy(b):
        if isinstance(b, int) and b == 0:
            rows = pl.ds(0, (RB + 1) * SEG)
        else:
            rows = pl.ds(pl.multiple_of((b * RB + 1) * SEG, SEG), RB * SEG)
        return pltpu.make_async_copy(x_hbm.at[rows], x_sc.at[rows, LN], sem_x.at[b])

    kb = (0, (UL + 1) * SEG, (UL + PH + 1) * SEG, S)
    sb = (0, 2, (PH + 2) // NQ + 2, NB)

    def in_copies(part):
        def rng(b):
            return pl.ds(b[part], b[part + 1] - b[part])
        sem = sem_in.at[part]
        return [
            pltpu.make_async_copy(k_hbm.at[rng(kb)],
                                  k_sc.at[pl.ds(KPAD + kb[part], kb[part + 1] - kb[part]), LN], sem),
            pltpu.make_async_copy(v_hbm.at[rng(kb)], v_sc.at[rng(kb), LN], sem),
        ] + [pltpu.make_async_copy(sk_hbm.at[:, pl.ds(c * CB, CB)], sk_sc.at[c], sem)
             for c in range(sb[part], sb[part + 1])]

    def w_copies(ci, dst=None, part=None):
        src = (wq_hbm, wk_hbm, wv_hbm)[ci // NG]
        dst = ci if dst is None else dst
        lo, n = (0, DH2) if part is None else (part * DH2 // 2, DH2 // 2)
        sem = sem_w.at[NCH + 1 if part == 1 else dst]
        return [pltpu.make_async_copy(src.at[pl.ds(hf * DH2 + lo, n), pl.ds((ci % NG) * HG, HG), :],
                                      st_sc.at[dst, pl.ds(lo, n), pl.ds(hf * HG, HG), :], sem)
                for hf in range(2)]

    wo_copy = pltpu.make_async_copy(wo_hbm, wo_sc, sem_w.at[NCH])

    def out_copy(lo, n):
        rows = pl.ds(lo * SEG if isinstance(lo, int) else pl.multiple_of(lo * SEG, SEG), n * SEG)
        return pltpu.make_async_copy(out_sc.at[rows, LN], o_hbm.at[rows], sem_out)

    def start_all(cps):
        def act():
            for cp in cps:
                cp.start()
        return act

    order = [[mem0_copy, x_copy(0)], w_copies(0, part=0), w_copies(0, part=1), [x_copy(1)], [x_copy(2)]]
    for ci in range(1, NCH):
        order.append(w_copies(ci) + ([x_copy(ci + 2)] if ci + 2 < NRB else []))
        if ci == NRB - 2:
            order.append(small + in_copies(0))
    order += [[wo_copy], in_copies(1), in_copies(2)]
    for i in range(0, len(order), 5):
        _in_order([start_all(cps) for cps in order[i:i + 5]])

    never_sm[0] = 0
    k_sc[0:KPAD, LN] = jnp.zeros((KPAD, DM), BF16)
    sp_sc[NB + 1] = jnp.zeros(sp_sc.shape[1:], F32)
    op_sc[...] = jnp.zeros(op_sc.shape, F32)
    x2_sc[...] = jnp.zeros(x2_sc.shape, F32)
    y_sc[2 * CB - SEG:, LN] = jnp.zeros((SEG, DM), F32)
    mem0_copy.wait()
    x_copy(0).wait()
    for sg in range(RB + 1):
        xn_sc[sg, :, 0:DM] = _pack(_ln(x_sc[sg * SEG:(sg + 1) * SEG, LN].astype(F32)))

    def clip(i, hi):
        return min(max(i, 0), hi) if isinstance(i, int) else jnp.clip(i, 0, hi)

    def scaled(i, m):
        return i * m if isinstance(i, int) else pl.multiple_of(i * m, m)

    def seg(i):
        return pl.ds(scaled(clip(i, NSEG - 1), SEG), SEG)

    def conv_u(s, ln=LN):
        r0 = scaled(clip(s, NSEG - 1), SEG)
        kk = k_sc[pl.ds(r0, KPAD + SEG), ln].astype(F32)[KPAD - 8:]

        def coef(j, rows):
            return jnp.concatenate([co_sc[j, :, ln]] * (rows // 8), axis=0)
        sft = [kk] + [pltpu.roll(kk, j, 0) for j in range(2, KS, 2)]
        ev = functools.reduce(jnp.add, [sft[j // 2][8:] * coef(j, SEG) for j in range(0, KS, 2)])
        od = functools.reduce(jnp.add, [sft[j // 2] * coef(j, SEG + 8) for j in range(1, KS, 2)])
        ks = ev + pltpu.roll(od, 1, 0)[8:]
        u = (ks * v_sc[pl.ds(r0, SEG), ln].astype(F32)).astype(BF16)
        u_sc[pl.ds(r0, SEG), ln] = u
        return u

    def conv_fwd(c, q):
        cc = clip(c, NB - 1)
        f = fwd_ref[q]
        uf = _dot(f, u_sc[pl.ds(scaled(cc, CB), CB), LN])
        kf = _dot_nt(f, sk_sc[cc])
        return uf, kf

    def put_spec(cs, q, which, val):
        for n in range(NT):
            v = val[:, n * 128:(n + 1) * 128].reshape(2, QB // 8, 8, 128)
            sp_sc[cs, q, :, n, which:which + 2] = jnp.stack([v[0], v[1]], axis=1)

    def conv_spec(c, q):
        uf, kf = conv_fwd(c, q)
        cs = clip(c, NB)
        put_spec(cs, q, 0, uf)
        pk = kr_sc[q]
        kr_sc[q] = kf
        kp = jnp.concatenate([
            kf[0:HB] - pk[QB:QB + HB],
            kf[HB:QB] + pk[QB + HB:],
            kf[QB:QB + HB] + pk[0:HB],
            kf[QB + HB:] - pk[HB:QB]], axis=0)
        put_spec(cs, q, 2, kp)

    MAC_PIECES = [(rb, n) for rb in range(QB // 16) for n in range(NT)]

    def conv_mac(c, q, piece, nterms):
        rb2, n = piece
        cs = clip(c, NB)
        rbs = slice(2 * rb2, 2 * rb2 + 2)
        ar = None
        ai = None
        for j in range(nterms):
            if isinstance(cs, int):
                uj, kj = j, cs - j
            else:
                uj = jnp.minimum(j, cs)
                kj = jnp.where(cs - j >= 0, cs - j, NB + 1)
            u = sp_sc[uj, q, rbs, n, 0:2]
            k = sp_sc[kj, q, rbs, n, 2:4]
            tr = u[:, 0] * k[:, 0] - u[:, 1] * k[:, 1]
            ti = u[:, 0] * k[:, 1] + u[:, 1] * k[:, 0]
            ar = tr if ar is None else ar + tr
            ai = ti if ai is None else ai + ti
        ln = slice(n * 128, (n + 1) * 128)
        w = jnp.concatenate([ar.reshape(16, 128), ai.reshape(16, 128)], axis=0).astype(BF16)
        wf_sc[c & 1, 0, q, rb2 * 16:rb2 * 16 + 16, ln] = w[0:16]
        wf_sc[c & 1, 1, q, rb2 * 16:rb2 * 16 + 16, ln] = w[16:]

    def conv_inv(tt, n):
        cb = tt // NQ
        p = tt % NQ
        ln = slice(n * 128, (n + 1) * 128)
        ev = _dot(inv_ref[p, 0], wf_sc[cb & 1, 0, :, :, ln].reshape(CB, 128))
        od = _dot(inv_ref[p, 1], wf_sc[cb & 1, 1, :, :, ln].reshape(CB, 128))
        sd = jnp.concatenate([co_sc[KS, :, ln]] * (HB // 8), axis=0)
        for r, val in ((p, _flip_rows(ev - od)), (2 * NQ - 1 - p, ev + od)):
            ur = scaled(clip(cb, NB - 1) * (2 * NQ) + r, HB)
            yr = scaled((cb & 1) * (2 * NQ) + r, HB)
            y_sc[pl.ds(yr, HB), ln] = val + u_sc[pl.ds(ur, HB), ln].astype(F32) * sd

    def y_seg(s):
        return y_sc[pl.ds(scaled(s & (2 * NQ - 1), SEG), SEG), LN]

    scale = DH ** -0.5
    cexp = scale * float(np.log2(np.e))

    def make_mask(n, x_layers, q0=0):
        qi = jax.lax.broadcasted_iota(jnp.int32, (n - q0, n), 0) + q0
        ki = jax.lax.broadcasted_iota(jnp.int32, (n - q0, n), 1)

        def layer(i):
            xl = jnp.where(i < M2 + SEG, x_layers[0], x_layers[-1])
            return jnp.where(i < M, 0, jnp.where(i < M2, 1, xl))
        same = layer(qi) == layer(ki)
        ok = same & ((qi < M2) | (ki < M2) | (qi >= ki))
        fill = jnp.where(same, -1e9 / scale, -jnp.inf).astype(F32)
        return ok, fill

    def probs(q, k, mask):
        ok, fill = mask
        s = _dot_nt(q, k)
        s = jnp.where(ok, s, fill)
        m = jnp.max(s, axis=-1, keepdims=True)
        p = jnp.exp2((s - m) * cexp)
        l = jnp.sum(p, axis=-1, keepdims=True)
        r = pl.reciprocal(l, approx=True)
        r = r * (2.0 - l * r)
        return (p * r).astype(BF16)

    def w_slot(ci):
        return (wb_sc, ci) if 1 <= ci < NRB - 1 else (wa_sc, max(ci - (NRB - 2), 0))

    def w_pos(j):
        return (j % 2) * (HG // 2) + j // 2

    def w_head(g, mats):
        slots = [w_slot(mi * NG + g // HG) for mi in mats]
        return _unpack(jnp.concatenate([ref[i, w_pos(g % HG)] for ref, i in slots], axis=1))

    def proj_split(hq, hkv, g, q1=None):
        q = _dot(hq, w_head(g, (0,)))
        kv = _dot(hkv, w_head(g, (1, 2)))
        if q1 is not None:
            q = jnp.concatenate([q[0:M2], q1, q[M2:]], axis=0)
        return q.astype(BF16), kv[:, :DH].astype(BF16), kv[:, DH:].astype(BF16)

    def xn(s):
        return _unpack(xn_sc[clip(s, NSEG - 1), :, 0:DM])

    def out_proj(n, g0, g1, j):
        return _dot(_unpack(o_sc[0:n // 2, g0 * DH:g1 * DH]),
                    wo_sc[g0 * DH:g1 * DH, j * 128:(j + 1) * 128])

    def attend(proj, n, mask, dist, hook=None, early=True):
        D1, D2 = dist
        HA = H - D1 - D2 - 1
        NE = min(D1 + D2, NT - 1) if early else 0
        qkvs = {}
        ps = {}
        outs = {}
        for it in range(H + D1 + D2):
            if it < H:
                qkvs[it] = proj(it)
            g = it - D1
            if 0 <= g < H:
                ps[g] = probs(qkvs[g][0], qkvs[g][1], mask)
            g = it - D1 - D2
            if 0 <= g < H:
                o = _dot(ps.pop(g), qkvs.pop(g)[2])
                o_sc[0:n // 2, g * DH:(g + 1) * DH] = _pack(o)
            if hook is not None:
                hook(it)
            j = it - (H - 1)
            if 0 <= j < NE:
                outs[j] = out_proj(n, 0, HA, j)
        for j in range(NE, NT):
            outs[j] = out_proj(n, 0, H, j)
            if hook is not None:
                hook(H + D1 + D2 + j)
        for j in range(NE):
            outs[j] = out_proj(n, HA, H, j) + outs[j]
        return jnp.concatenate([outs[j] for j in range(NT)], axis=1)

    def side2(t, a2):
        x3 = x2_sc[(t - 2) & 3] + a2
        x4 = x3 + _ln(x3) * y_seg(t - 2)
        x4 = x4.astype(out_sc.dtype)
        out_sc[seg(t - 2), LN] = x4
        return x4

    def fill(s, heads):
        xq = xn(s)
        for g in heads:
            fill_sc[g - NPA] = _dot(xq, w_head(g, (0,)))

    def finish(t, xr, yt, mem, a1, spec):
        if spec:
            conv_spec((t + 2) // NQ + 1, (t + 2) % NQ)
        fill(t + 1, range(NPA, NPA + NPB))
        x1 = xr.astype(F32) + a1
        x2 = x1 + _ln(x1) * yt
        h_sc[0:M, :] = _pack(mem)
        h_sc[M:, :] = _pack(_ln(x2))
        x2_sc[t & 3] = x2

    def pinned(rows, pins):
        never = never_sm[0] > 0
        hs = {0: rows}
        r = _pack(rows)
        tiles = [r[:, n * 128:(n + 1) * 128] for n in range(NT)]
        for g, n, d in sorted(pins, key=lambda p: p[0]):
            tiles[n] = jnp.where(never, d, tiles[n])
            hs[g] = _unpack(jnp.concatenate(tiles, axis=1))
        return lambda g: hs[max(k for k in hs if k <= g)]

    def pin_tiles(g0, stride, val):
        v = _pack(val)
        return [(g0 + n * stride, n, v[:, n * 128:(n + 1) * 128]) for n in range(NT)]

    def wait_chunk(ci):
        for cp in w_copies(0, ci):
            cp.wait()

    def relayout(ci, dst, slot, b):
        d0 = scaled(b, 16)
        r0 = scaled(b, 8)
        xw = pltpu.bitcast(st_sc[ci, pl.ds(d0, 16)], U32).reshape(8, 2, HG, DH)
        a = xw[:, 0]
        bb = xw[:, 1]
        lo = jnp.swapaxes((a & U32(0xFFFF)) | (bb << 16), 0, 1)
        hi = jnp.swapaxes((a >> 16) | (bb & U32(0xFFFF0000)), 0, 1)
        for hf in range(2):
            rows = pl.ds(r0 + hf * (DH2 // 2), 8)
            dst[slot, 0:HG // 2, rows, :] = lo[hf * HG // 2:(hf + 1) * HG // 2]
            dst[slot, HG // 2:HG, rows, :] = hi[hf * HG // 2:(hf + 1) * HG // 2]

    NBLK = DH2 // 16

    def main(_, carry):
        def relayout0(b, c):
            relayout(0, wa_sc, 0, b)
            return c
        for part in range(2):
            with jax.named_scope("wait_w"):
                for cp in w_copies(0, part=part):
                    cp.wait()
            with jax.named_scope("relayout"):
                jax.lax.fori_loop(part * NBLK // 2, (part + 1) * NBLK // 2, relayout0, 0, unroll=2)

        def pro_stage(ps_, b):
            n = ps_ * NRB + b
            with jax.named_scope("wait_w"):
                if ps_ == 0:
                    @pl.when(b + 1 < NRB)
                    def _():
                        x_copy(b + 1).wait()

                @pl.when((n >= 2) & (n <= NCH))
                def _():
                    wait_chunk(n - 1)
            cr = jnp.clip(n - 1, 0, NCH - 1)
            dst, slot = (wb_sc, cr) if ps_ == 0 else (wa_sc, cr - (NRB - 2))
            src, si = w_slot(ps_)
            bl = jnp.minimum(b + 1, NRB - 1)
            PW = PRO_PW
            npc = RB * S2 // PW
            assert npc * PW == RB * S2 and PRO_R0 + (NBLK - 1) * PRO_RS < HG * npc
            assert PRO_X0 + (max(RB, 2 * NT) - 1) * PRO_XS < HG * npc and 2 * NRB > UL

            def body(i, c):
                s0 = b * RB + 1
                for sg in range(RB):
                    hp_sc[sg * S2:(sg + 1) * S2, :] = xn_sc[s0 + sg, :, 0:DM]
                for j in range(HG):
                    w = _unpack(src[si, w_pos(j)])
                    for pi in range(npc):
                        pos = j * npc + pi
                        hx = hp_sc[pi * PW:(pi + 1) * PW, :]
                        k, rem = divmod(pos - PRO_X0, PRO_XS)
                        if ps_ == 0 and rem == 0 and 0 <= k < RB:
                            sn = bl * RB + 1 + k
                            xv = _pack(_ln(x_sc[seg(sn), LN].astype(F32)))
                            xn_sc[sn, :, 0:DM] = xv
                            hx = jnp.concatenate([hx[:-S2], jnp.where(never_sm[0] > 0, xv, hx[-S2:])], axis=0)
                        if ps_ == 1 and rem == 0 and 0 <= k < 2 * NT:
                            conv_u(jnp.minimum(2 * b + k // NT, UL),
                                   slice((k % NT) * 128, (k % NT + 1) * 128))
                        bb, rem = divmod(pos - PRO_R0, PRO_RS)
                        if rem == 0 and 0 <= bb < NBLK:
                            relayout(cr, dst, slot, bb)
                        r = _dot(_unpack(hx), w)
                        for a in range(0, 2 * PW, 16):
                            sg, off = divmod(2 * pi * PW + a, SEG)
                            pre_sc[s0 + sg, ps_ * HG + j, off:off + 16, :] = r[a:a + 16]
                return c
            with jax.named_scope("fused"):
                jax.lax.fori_loop(0, never_sm[0] + 1, body, 0)

        for ps_ in range(NPASS):
            if ps_ == 1:
                with jax.named_scope("wait_in0"):
                    for cp in small + in_copies(0):
                        cp.wait()
                sh = sh_ref[...].astype(F32)
                for j in range(KS):
                    co_sc[j] = jnp.broadcast_to(sh[j:j + 1], (8, DM))
                co_sc[KS] = jnp.broadcast_to(sd_ref[...].astype(F32).reshape(1, DM), (8, DM))

            def blk(b, c, ps_=ps_):
                pro_stage(ps_, b)
                return c
            jax.lax.fori_loop(0, NRB, blk, 0)

        def warm_block0(q):
            uf, kf = conv_fwd(0, q)
            put_spec(0, q, 0, uf)
            put_spec(0, q, 2, kf)
            kr_sc[q] = kf
            ur, um, kr, km = uf[:QB], uf[QB:], kf[:QB], kf[QB:]
            wf_sc[0, 0, q] = (ur * kr - um * km).astype(BF16)
            wf_sc[0, 1, q] = (ur * km + um * kr).astype(BF16)

        with jax.named_scope("step0"):
            mem0 = mem0_ref[...].astype(F32)
            h0 = jnp.concatenate([jnp.concatenate([mem0, mem0], axis=0).astype(BF16), xn(0)], axis=0)

            def hook0(it):
                j = it - (H - 1)
                if 0 <= j < NQ:
                    warm_block0(j)
                j = it - (H + sum(DIST_HALF))
                if j == -1:
                    conv_spec(1, 0)
                    wo_copy.wait()
                    conv_spec(1, 1)
                    for q in range(2):
                        for piece in MAC_PIECES:
                            conv_mac(1, q, piece, 2)
                if 0 <= j < 3:
                    for n in range(NT):
                        conv_inv(j, n)
            out = attend(lambda g: proj_split(h0, h0, g), RH, make_mask(RH, (0,)), DIST_HALF, hook0, False)
            finish(0, x_sc[0:SEG, LN], y_seg(0), jnp.concatenate([out[0:M], mem0], axis=0), out[M2:], False)

        mask12 = make_mask(R, (0, 1))

        def step(t, first, last):
            c, q = (t + 1) // NQ + 1, (t + 1) % NQ
            x4 = side2(t, op_sc[...])
            un = conv_u(t + UL)
            hm = _unpack(h_sc[0:M, :])
            hx2 = _unpack(h_sc[M:, :])
            h48 = jnp.concatenate([hm, hx2], axis=0)
            x1n = pinned(xn(t), pin_tiles(PIN_U, 1, un) + pin_tiles(PIN_X4, 0, x4))

            def proj(g):
                h80 = jnp.concatenate([hm, x1n(g), hx2], axis=0)
                if g >= NPA + NPB:
                    return proj_split(h80, h80, g)
                return proj_split(h48, h80, g, pre_sc[t, g] if g < NPA else fill_sc[g - NPA])

            held = {}

            def hook(it):
                if it == SPEC_AT:
                    if first:
                        conv_spec(c, q)
                    for piece in MAC_PIECES:
                        conv_mac(c, q, piece, NB)
                if INV_AT <= it < INV_AT + NT:
                    conv_inv(t + 2, it - INV_AT)
                if it == H:
                    held["x"] = x_sc[seg(t), LN]
                    held["y"] = y_seg(t)
            out = attend(proj, R, mask12, DIST, hook)
            op_sc[...] = out[RH:]
            finish(t, held["x"], held["y"], out[0:M2], out[M2:RH], not last)

        def steps(i, carry):
            for j in range(UNROLL):
                step(1 + i * UNROLL + j, j == 0, j == UNROLL - 1)
            return carry

        def phase(p, carry):
            @pl.when(p == 1)
            def _():
                for cp in in_copies(2):
                    cp.wait()

            @pl.when(p >= 2)
            def _():
                out_copy((p - 2) * PH, PH).start()

            with jax.named_scope("steps"):
                jax.lax.fori_loop(p * PHI, (p + 1) * PHI, steps, 0)
            return carry

        for cp in in_copies(1):
            cp.wait()
        jax.lax.fori_loop(0, NPH, phase, 0)
        out_copy((NPH - 2) * PH, NSEG - 2 - (NPH - 2) * PH).start()

        with jax.named_scope("step_last"):
            x4 = side2(NSEG, op_sc[...])
            hm = _unpack(h_sc[0:M, :])
            hx = pinned(_unpack(h_sc[M:, :]), pin_tiles(PIN_X4, 0, x4))
            out = attend(lambda g: proj_split(hx(g), jnp.concatenate([hm, hx(g)], axis=0), g),
                         SEG, make_mask(RH, (1,), M2), DIST_LAST)
            side2(NSEG + 1, out)
        out_copy(NSEG - 2, 2).start()
        out_copy(0, NSEG).wait()
        return carry

    jax.lax.fori_loop(0, never_sm[0] + 1, main, 0)


def pallas_interleave_layers__memory_aug_recurrent_mem_tr__ssm_conv_h3__prompt_kernel(
    A_x, A_mem0, A_Wq, A_Wk, A_Wv, A_Wo, A_seg_len,
    B_q, B_k, B_v, B_shift_k, B_ssm_k, B_ssm_D,
):
    del B_q
    seg = int(A_seg_len) if isinstance(A_seg_len, (int, np.integer)) else CB // NQ
    return _run(A_x, A_mem0, A_Wq, A_Wk, A_Wv, A_Wo, B_k, B_v, B_shift_k, B_ssm_k, B_ssm_D, SEG=seg)


@functools.partial(jax.jit, static_argnames=("SEG",))
def _run(A_x, A_mem0, A_Wq, A_Wk, A_Wv, A_Wo, B_k, B_v, B_shift_k, B_ssm_k, B_ssm_D, *, SEG):
    B, S, DM = A_x.shape
    assert B == 1
    H, DH = A_Wq.shape[1], A_Wq.shape[2]
    M = A_mem0.shape[1]
    KS = B_shift_k.shape[1]
    R = 2 * (M + SEG)
    NSEG = S // SEG
    NRB = (NSEG - 1) // RB
    NB = S // CB
    QB = CB // NQ
    NCH = 3 * H // HG
    DP = -(-DM // 256) * 256
    fwd, inv = _dft_constants()

    kern = functools.partial(_kernel, S=S, DM=DM, H=H, DH=DH, M=M, SEG=SEG)
    any_spec = pl.BlockSpec(memory_space=pl.ANY)
    out = pl.pallas_call(
        kern,
        out_shape=jax.ShapeDtypeStruct((S, DM), A_x.dtype),
        in_specs=[any_spec] * 13,
        out_specs=any_spec,
        scratch_shapes=[
            pltpu.VMEM((NB + 2, NQ, QB // 8, DM // 128, 4, 8, 128), F32),
            pltpu.VMEM((NQ, 2 * QB, DM), F32),
            pltpu.VMEM((2, 2, NQ, QB, DM), BF16),
            pltpu.VMEM((4, SEG, DM), F32),
            pltpu.VMEM((2 * CB, DP), F32),
            pltpu.VMEM((S, DP), BF16),
            pltpu.VMEM((SEG, DM), F32),
            pltpu.VMEM((NSEG, NPA, SEG, DH), F32),
            pltpu.VMEM((NPB, SEG, DH), F32),
            pltpu.VMEM((NSEG, SEG // 2, DP), U32),
            pltpu.VMEM((NCH - NRB + 2, HG, DM // 2, DH), U32),
            pltpu.VMEM((NRB - 1, HG, DM // 2, DH), U32),
            pltpu.VMEM((H * DH, DM), BF16),
            pltpu.VMEM((R // 2, H * DH), U32),
            pltpu.VMEM((S, DP), BF16),
            pltpu.VMEM((S, DP), BF16),
            pltpu.VMEM((NB, DM, CB), BF16),
            pltpu.VMEM((NCH, DM // 2, 2 * HG, DH), BF16),
            pltpu.VMEM((S, DP), A_x.dtype),
            pltpu.VMEM(fwd.shape, BF16),
            pltpu.VMEM(inv.shape, BF16),
            pltpu.VMEM((S + KPAD, DP), BF16),
            pltpu.VMEM((RB * SEG // 2, DM), U32),
            pltpu.VMEM((M + SEG // 2, DM), U32),
            pltpu.VMEM((KS + 1, 8, DM), F32),
            pltpu.VMEM((M, DM), BF16),
            pltpu.VMEM((KS, DM), BF16),
            pltpu.VMEM((DM,), BF16),
            pltpu.SMEM((1,), jnp.int32),
            pltpu.SemaphoreType.DMA(((NSEG - 1) // RB,)),
            pltpu.SemaphoreType.DMA((3,)),
            pltpu.SemaphoreType.DMA((NCH + 2,)),
            pltpu.SemaphoreType.DMA(()),
        ],
        compiler_params=pltpu.CompilerParams(vmem_limit_bytes=120 * 1024 * 1024),
    )(
        A_x.reshape(S, DM), A_mem0.reshape(M, DM), A_Wq, A_Wk, A_Wv,
        A_Wo.reshape(H * DH, DM), B_k.reshape(S, DM), B_v.reshape(S, DM),
        B_shift_k.T, B_ssm_k, B_ssm_D,
        jnp.asarray(fwd, BF16), jnp.asarray(inv, BF16),
    )
    return out.reshape(B, S, DM)
```

```python
import functools

import numpy as np
import jax
import jax.numpy as jnp
import jax.experimental.pallas as pl
import jax.experimental.pallas.tpu as pltpu

F32 = jnp.float32
BF16 = jnp.bfloat16
U32 = jnp.uint32

CB = 128
NQ = 4
KPAD = 16
HG = 8
NPA = 16
KH = 256
RB = 9
PRO_PW, PRO_X0, PRO_XS, PRO_R0, PRO_RS = 24, 11, 4, 2, 2
WO_LAG = 2
UNROLL = 3
PHI = 3
SPEC_AT, INV_AT, PIN_U, PIN_X4 = 4, 10, 1, 8
DIST, DIST_HALF = (1, 1), (1, 2)
PLAN = ((1, 2), (3, 4), (7,))
PLAN_HALF = ((1,), (2,), (3,), (4,))


def _dft_constants():
    qb = CB // NQ
    hb = qb // 2
    n = np.arange(CB, dtype=np.float64)
    f = np.concatenate([q * qb + np.concatenate([np.arange(0, qb, 2), np.arange(1, qb, 2)])
                        for q in range(NQ)])
    w = np.pi * (2.0 * f + 1.0) / (2 * CB)
    ang = (w[:, None] * (n[None, :] - (CB - 1) / 4.0)).reshape(NQ, qb, CB)
    fwd = np.concatenate([np.cos(ang), -np.sin(ang)], axis=1)
    inv = np.zeros((NQ, 2, hb, CB))
    for p in range(NQ):
        m = (NQ - 1 - p) * hb + np.arange(hb)
        ang = (m[:, None] + 0.5) * w[None, :]
        inv[p, 0] = np.cos(ang) / CB
        inv[p, 1] = -np.sin(ang) / CB
    return fwd.astype(np.float32), inv.astype(np.float32)


def _flip_rows(x):
    i = jax.lax.broadcasted_iota(jnp.int32, (8, x.shape[1]), 0)
    out = []
    for r in range(x.shape[0] - 8, -8, -8):
        v = pltpu.roll(x[r:r + 8], 4, 0)
        for b in (2, 1):
            v = jnp.where((i & b) == 0, pltpu.roll(v, 8 - b, 0), pltpu.roll(v, b, 0))
        out.append(v)
    return jnp.concatenate(out, axis=0)


def _ln(x, eps=1e-5):
    d = x.shape[-1]
    m = jnp.sum(x, axis=-1, keepdims=True) * (1.0 / d)
    xc = x - m
    v = jnp.sum(xc * xc, axis=-1, keepdims=True) * (1.0 / d)
    return xc * jax.lax.rsqrt(v + eps)


def _dot(a, b):
    return jnp.dot(a, b, preferred_element_type=F32)


def _dot_nt(a, b):
    return jax.lax.dot_general(a, b, (((1,), (1,)), ((), ())), preferred_element_type=F32)


def _pack(x):
    return pltpu.bitcast(x.astype(BF16), U32)


def _unpack(x):
    return pltpu.bitcast(x, BF16)


def _ext(r):
    return _pack(jnp.concatenate([r, r[:, :KH] + r[:, KH:2 * KH]], axis=1))


def _combos(b11, b12, b21, b22):
    f11, f12, f21, f22 = [_unpack(b).astype(F32) for b in (b11, b12, b21, b22)]
    return [_pack(f11 + f22), b11, _pack(f12 - f22), _pack(f21 - f11), b22,
            _pack(f11 + f12), _pack(f21 + f22)]


def _in_order(actions):
    def body(i, c):
        for j, act in enumerate(actions):
            pl.when(i == j)(act)
        return c
    jax.lax.fori_loop(0, len(actions), body, 0)


def _kernel(x_hbm, mem0_hbm, wq_hbm, wk_hbm, wv_hbm, wo_hbm, k_hbm, v_hbm,
            sh_hbm, sk_hbm, sd_hbm, fwd_hbm, inv_hbm, o_hbm,
            sp_sc, kr_sc, wf_sc, x2_sc, y_sc, u_sc, op_sc, pre_sc, fill_sc, xn_sc, wa_sc, wb_sc, wo_sc, wc_sc,
            oe_sc, oo_sc, os_sc, ox_sc, xc_sc,
            x_sc, v_sc, sk_sc, st_sc, out_sc, fwd_ref, inv_ref,
            k_sc, hp_sc, h_sc, co_sc, mem0_ref, sh_ref, sd_ref,
            never_sm, sem_x, sem_in, sem_w, sem_out,
            *, S, DM, H, DH, M, SEG):
    NSEG = S // SEG
    M2 = 2 * M
    S2 = SEG // 2
    R = M2 + 2 * SEG
    RH = M2 + SEG
    NB = S // CB
    QB = CB // NQ
    HB = QB // 2
    NT = DM // 128
    PH = PHI * UNROLL
    NRB = (NSEG - 1) // RB
    NPH = (NSEG - 1) // PH
    NG = H // HG
    NCH = 3 * NG
    NPASS = NPA // HG
    DH2 = DM // 2
    HP = H // 2
    DE = DM + KH
    KT = DM - 2 * KH
    EA, EB, EC, ES = slice(0, KH), slice(KH, 2 * KH), slice(2 * KH, DM), slice(DM, DE)
    KS = sh_ref.shape[0]
    UL = 2 * NQ + 1
    LN = pl.ds(0, DM)
    assert 2 * KT == KH and 2 <= KS <= 8 and QB == SEG and NRB * RB == NSEG - 1 and NPH * PH == NSEG - 1 and NPASS == 2 and 2 * NRB >= NCH + 1

    mem0_copy = pltpu.make_async_copy(mem0_hbm, mem0_ref, sem_x.at[0])
    small = [pltpu.make_async_copy(s, d, sem_in.at[0]) for s, d in [
        (sh_hbm, sh_ref), (sd_hbm, sd_ref), (fwd_hbm, fwd_ref), (inv_hbm, inv_ref)]]

    def x_copy(b):
        if isinstance(b, int) and b == 0:
            rows = pl.ds(0, (RB + 1) * SEG)
        else:
            rows = pl.ds(pl.multiple_of((b * RB + 1) * SEG, SEG), RB * SEG)
        return pltpu.make_async_copy(x_hbm.at[rows], x_sc.at[rows, LN], sem_x.at[b])

    kb = (0, (UL + 1) * SEG, (UL + PH + 1) * SEG, S)
    sb = (0, 2, (PH + 2) // NQ + 2, NB)

    def in_copies(part):
        def rng(b):
            return pl.ds(b[part], b[part + 1] - b[part])
        sem = sem_in.at[part]
        return [
            pltpu.make_async_copy(k_hbm.at[rng(kb)],
                                  k_sc.at[pl.ds(KPAD + kb[part], kb[part + 1] - kb[part]), LN], sem),
            pltpu.make_async_copy(v_hbm.at[rng(kb)], v_sc.at[rng(kb), LN], sem),
        ] + [pltpu.make_async_copy(sk_hbm.at[:, pl.ds(c * CB, CB)], sk_sc.at[c], sem)
             for c in range(sb[part], sb[part + 1])]

    def w_copies(ci, dst=None, part=None):
        src = (wq_hbm, wk_hbm, wv_hbm)[ci // NG]
        dst = ci if dst is None else dst
        spans = {None: [(0, KH), (KH, DH2)], 0: [(0, DH2 // 2)], 1: [(DH2 // 2, KH), (KH, DH2)]}[part]
        sem = sem_w.at[NCH + 1 if part == 1 else dst]
        return [pltpu.make_async_copy(
            src.at[pl.ds(lo + hf * KH if lo < KH else KH + lo + hf * (KT // 2), hi - lo),
                   pl.ds((ci % NG) * HG, HG), :],
            st_sc.at[dst, pl.ds(lo, hi - lo), pl.ds(hf * HG, HG), :], sem)
            for lo, hi in spans for hf in range(2)]

    wo_copy = pltpu.make_async_copy(wo_hbm, wo_sc, sem_w.at[NCH])

    def out_copy(lo, n):
        rows = pl.ds(lo * SEG if isinstance(lo, int) else pl.multiple_of(lo * SEG, SEG), n * SEG)
        return pltpu.make_async_copy(out_sc.at[rows, LN], o_hbm.at[rows], sem_out)

    def start_all(cps):
        def act():
            for cp in cps:
                cp.start()
        return act

    order = [[mem0_copy, x_copy(0)], w_copies(0, part=0), w_copies(0, part=1), [x_copy(1)], [x_copy(2)]]
    for ci in range(1, NCH):
        order.append(w_copies(ci) + ([x_copy(ci + 2)] if ci + 2 < NRB else []))
        if ci == NRB - 2:
            order.append(small + in_copies(0))
    order += [[wo_copy], in_copies(1), in_copies(2)]
    for i in range(0, len(order), 5):
        _in_order([start_all(cps) for cps in order[i:i + 5]])

    never_sm[0] = 0
    k_sc[0:KPAD, LN] = jnp.zeros((KPAD, DM), BF16)
    sp_sc[NB + 1] = jnp.zeros(sp_sc.shape[1:], F32)
    op_sc[...] = jnp.zeros(op_sc.shape, F32)
    x2_sc[...] = jnp.zeros(x2_sc.shape, F32)
    y_sc[2 * CB - SEG:, LN] = jnp.zeros((SEG, DM), F32)
    mem0_copy.wait()
    x_copy(0).wait()
    for sg in range(RB + 1):
        xn_sc[sg, :, 0:DE] = _ext(_ln(x_sc[sg * SEG:(sg + 1) * SEG, LN].astype(F32)))

    def clip(i, hi):
        return min(max(i, 0), hi) if isinstance(i, int) else jnp.clip(i, 0, hi)

    def scaled(i, m):
        return i * m if isinstance(i, int) else pl.multiple_of(i * m, m)

    def seg(i):
        return pl.ds(scaled(clip(i, NSEG - 1), SEG), SEG)

    def conv_u(s, ln=LN):
        r0 = scaled(clip(s, NSEG - 1), SEG)
        kk = k_sc[pl.ds(r0, KPAD + SEG), ln].astype(F32)[KPAD - 8:]

        def coef(j, rows):
            return jnp.concatenate([co_sc[j, :, ln]] * (rows // 8), axis=0)
        sft = [kk] + [pltpu.roll(kk, j, 0) for j in range(2, KS, 2)]
        ev = functools.reduce(jnp.add, [sft[j // 2][8:] * coef(j, SEG) for j in range(0, KS, 2)])
        od = functools.reduce(jnp.add, [sft[j // 2] * coef(j, SEG + 8) for j in range(1, KS, 2)])
        ks = ev + pltpu.roll(od, 1, 0)[8:]
        u = (ks * v_sc[pl.ds(r0, SEG), ln].astype(F32)).astype(BF16)
        u_sc[pl.ds(r0, SEG), ln] = u
        return u

    def conv_fwd(c, q):
        cc = clip(c, NB - 1)
        f = fwd_ref[q]
        uf = _dot(f, u_sc[pl.ds(scaled(cc, CB), CB), LN])
        kf = _dot_nt(f, sk_sc[cc])
        return uf, kf

    def put_spec(cs, q, which, val):
        for n in range(NT):
            v = val[:, n * 128:(n + 1) * 128].reshape(2, QB // 8, 8, 128)
            sp_sc[cs, q, :, n, which:which + 2] = jnp.stack([v[0], v[1]], axis=1)

    def conv_spec(c, q):
        uf, kf = conv_fwd(c, q)
        cs = clip(c, NB)
        put_spec(cs, q, 0, uf)
        pk = kr_sc[q]
        kr_sc[q] = kf
        kp = jnp.concatenate([
            kf[0:HB] - pk[QB:QB + HB],
            kf[HB:QB] + pk[QB + HB:],
            kf[QB:QB + HB] + pk[0:HB],
            kf[QB + HB:] - pk[HB:QB]], axis=0)
        put_spec(cs, q, 2, kp)

    MAC_PIECES = [(rb, n) for rb in range(QB // 16) for n in range(NT)]

    def conv_mac(c, q, piece, nterms):
        rb2, n = piece
        cs = clip(c, NB)
        rbs = slice(2 * rb2, 2 * rb2 + 2)
        ar = None
        ai = None
        for j in range(nterms):
            if isinstance(cs, int):
                uj, kj = j, cs - j
            else:
                uj = jnp.minimum(j, cs)
                kj = jnp.where(cs - j >= 0, cs - j, NB + 1)
            u = sp_sc[uj, q, rbs, n, 0:2]
            k = sp_sc[kj, q, rbs, n, 2:4]
            tr = u[:, 0] * k[:, 0] - u[:, 1] * k[:, 1]
            ti = u[:, 0] * k[:, 1] + u[:, 1] * k[:, 0]
            ar = tr if ar is None else ar + tr
            ai = ti if ai is None else ai + ti
        ln = slice(n * 128, (n + 1) * 128)
        w = jnp.concatenate([ar.reshape(16, 128), ai.reshape(16, 128)], axis=0).astype(BF16)
        wf_sc[c & 1, 0, q, rb2 * 16:rb2 * 16 + 16, ln] = w[0:16]
        wf_sc[c & 1, 1, q, rb2 * 16:rb2 * 16 + 16, ln] = w[16:]

    def conv_inv(tt, n):
        cb = tt // NQ
        p = tt % NQ
        ln = slice(n * 128, (n + 1) * 128)
        ev = _dot(inv_ref[p, 0], wf_sc[cb & 1, 0, :, :, ln].reshape(CB, 128))
        od = _dot(inv_ref[p, 1], wf_sc[cb & 1, 1, :, :, ln].reshape(CB, 128))
        sd = jnp.concatenate([co_sc[KS, :, ln]] * (HB // 8), axis=0)
        for r, val in ((p, _flip_rows(ev - od)), (2 * NQ - 1 - p, ev + od)):
            ur = scaled(clip(cb, NB - 1) * (2 * NQ) + r, HB)
            yr = scaled((cb & 1) * (2 * NQ) + r, HB)
            y_sc[pl.ds(yr, HB), ln] = val + u_sc[pl.ds(ur, HB), ln].astype(F32) * sd

    def y_seg(s):
        return y_sc[pl.ds(scaled(s & (2 * NQ - 1), SEG), SEG), LN]

    scale = DH ** -0.5
    cexp = scale * float(np.log2(np.e))

    def make_mask(n, x_layers, q0=0):
        qi = jax.lax.broadcasted_iota(jnp.int32, (n - q0, n), 0) + q0
        ki = jax.lax.broadcasted_iota(jnp.int32, (n - q0, n), 1)

        def layer(i):
            xl = jnp.where(i < M2 + SEG, x_layers[0], x_layers[-1])
            return jnp.where(i < M, 0, jnp.where(i < M2, 1, xl))
        same = layer(qi) == layer(ki)
        ok = same & ((qi < M2) | (ki < M2) | (qi >= ki))
        fill = jnp.where(same, -1e9 / scale, -jnp.inf).astype(F32)
        return ok, fill

    def probs(q, k, mask):
        ok, fill = mask
        s = _dot_nt(q, k)
        s = jnp.where(ok, s, fill)
        m = jnp.max(s, axis=-1, keepdims=True)
        p = jnp.exp2((s - m) * cexp)
        l = jnp.sum(p, axis=-1, keepdims=True)
        r = pl.reciprocal(l, approx=True)
        r = r * (2.0 - l * r)
        return (p * r).astype(BF16)

    def w_slot(ci):
        return (wb_sc, ci) if 1 <= ci < NRB - 1 else (wa_sc, max(ci - (NRB - 2), 0))

    def rows(*parts):
        return jnp.concatenate(parts, axis=0)

    def cols(*parts):
        return jnp.concatenate(parts, axis=1)

    def w_op(ref, slot, j, i, odd=None):
        return ref[slot, j, i] if odd is None else ref[slot, j, 7, odd * KT // 2:(odd + 1) * KT // 2]

    def w_mats(jp, mats, i, odd=None):
        return cols(*[w_op(*w_slot(mi * NG + 2 * jp // HG), jp % (HG // 2), i, odd) for mi in mats])

    def plain_lhs(e, odd):
        return _unpack(cols(e[:, EA], e[:, ES], e[:, EC]) if odd else cols(e[:, ES], e[:, EB], e[:, EC]))

    def plain_proj(e, jp, mats, odd):
        w = rows(w_mats(jp, mats, 1 + odd), w_mats(jp, mats, 3 + odd), w_mats(jp, mats, 7, odd))
        return _dot(plain_lhs(e, odd), _unpack(w))

    def strassen(lhs, rhs):
        m = [_dot(a, b) for a, b in zip(lhs, rhs)]
        return strassen_out(m)

    def strassen_out(m):
        c21 = m[1] + m[3]
        c12 = m[2] + m[4]
        c11 = m[0] + m[3][M2:] - m[4][M2:] + m[6]
        c22 = m[0] - m[1][M2:] + m[2][M2:] + m[5]
        return rows(c21[:M2], c11, c21[M2:]), rows(c12, c22)

    def bf(*xs):
        return tuple(x.astype(BF16) for x in xs)

    def xn(s):
        return xn_sc[clip(s, NSEG - 1), :, 0:DE]

    def attend(proj, n, mask, dist, plan, hook=None):
        D1, D2 = dist
        PA = HP - D1 - D2 - 1
        full = n == R
        n2 = n // 2

        def prod(i, p0, p1):
            cs = slice(p0 * DH, p1 * DH)
            ws = slice(p0 * DH // 2, p1 * DH // 2)
            if i == 7:
                return _dot(_unpack(cols(oe_sc[0:n2, cs], oo_sc[0:n2, cs])),
                            _unpack(rows(wc_sc[7, ws, 0:KT], wc_sc[7, ws, KT:2 * KT])))
            if i in (0, 5, 6):
                a = ox_sc[max(i - 4, 0), :, cs]
            else:
                ref = {1: os_sc, 2: oe_sc, 3: oo_sc, 4: os_sc}[i]
                if not full:
                    a = ref[0:n2, cs]
                elif i in (2, 4):
                    a = ref[0:RH // 2, cs]
                else:
                    a = rows(ref[0:M, cs], ref[RH // 2:, cs])
            return _dot(_unpack(a), _unpack(wc_sc[i, ws, :]))

        qkvs = {}
        ps = {}
        m = {}
        for it in range(HP + D1 + D2):
            if it < HP:
                qkvs[it] = proj(it)
            g = it - D1
            if 0 <= g < HP:
                ps[g] = [probs(q, k, mask) for q, k, _ in qkvs[g]]
            g = it - D1 - D2
            if 0 <= g < HP:
                oe, oo = [_dot(p, qkv[2]) for p, qkv in zip(ps.pop(g), qkvs.pop(g))]
                cs = slice(g * DH, (g + 1) * DH)
                oe_sc[0:n2, cs] = _pack(oe)
                oo_sc[0:n2, cs] = _pack(oo)
                os_sc[0:n2, cs] = _pack(oe + oo)
                if full:
                    ox_sc[0, :, cs] = _pack(oe[M2:RH] + oo[RH:])
                    ox_sc[1, :, cs] = _pack(oe[RH:] - oe[M2:RH])
                    ox_sc[2, :, cs] = _pack(oo[M2:RH] - oo[RH:])
            if hook is not None:
                hook(it)
            j = it - (HP - 1)
            if j >= 0:
                for i in plan[j]:
                    m[i] = prod(i, 0, PA)
        early = list(m)
        for i in (range(8) if full else (1, 2, 3, 4, 7)):
            if i not in early:
                m[i] = prod(i, 0, HP)
        for i in early:
            m[i] = prod(i, PA, HP) + m[i]
        c1, c2 = strassen_out(m) if full else (m[1] + m[3], m[2] + m[4])
        return cols(c1, c2, m[7])

    def side2(t, a2):
        x3 = x2_sc[(t - 2) & 3] + a2
        x4 = x3 + _ln(x3) * y_seg(t - 2)
        x4 = x4.astype(out_sc.dtype)
        out_sc[seg(t - 2), LN] = x4
        return x4

    def finish(t, xr, yt, mem, a1, spec):
        if spec:
            conv_spec((t + 2) // NQ + 1, (t + 2) % NQ)
        e1 = xn(t + 1)
        for g in range(NPA, H):
            fill_sc[g - NPA] = plain_proj(e1, g // 2, (0,), g % 2)
        x1 = xr.astype(F32) + a1
        x2 = x1 + _ln(x1) * yt
        n1 = _unpack(e1[:, 0:2 * KH]).astype(F32)
        n2 = _ln(x2)
        h_sc[0:M, :] = _ext(mem)
        h_sc[M:, :] = _ext(n2)
        xc_sc[...] = _pack(cols(n1[:, EA] + n2[:, EB], n2[:, EA] - n1[:, EA], n1[:, EB] - n2[:, EB]))
        x2_sc[t & 3] = x2

    def pinned(r, pins):
        never = never_sm[0] > 0
        hs = {0: r}
        tiles = [r[:, n:n + 128] for n in range(0, r.shape[1], 128)]
        for g, n, d in sorted(pins, key=lambda p: p[0]):
            tiles[n] = jnp.where(never, d, tiles[n])
            hs[g] = cols(*tiles)
        return lambda g: hs[max(k for k in hs if k <= g)]

    def pin_tiles(g0, per, val):
        v = _pack(val)
        return [(g0 + n // per, n, v[:, n * 128:(n + 1) * 128]) for n in range(NT)]

    def wait_chunk(ci):
        for cp in w_copies(0, ci):
            cp.wait()

    def relayout(ci, dst, slot, b, tail):
        d0 = scaled(b, 16)
        r0 = scaled(b, 8)
        xw = pltpu.bitcast(st_sc[ci, pl.ds(d0, 16)], U32).reshape(8, 2, HG, DH)
        a = xw[:, 0]
        bb = xw[:, 1]
        lo = jnp.swapaxes((a & U32(0xFFFF)) | (bb << 16), 0, 1)
        hi = jnp.swapaxes((a >> 16) | (bb & U32(0xFFFF0000)), 0, 1)
        P = HG // 2
        if tail:
            for hf in range(2):
                for odd, v in enumerate((lo, hi)):
                    rr = pl.ds(r0 - KH // 2 + odd * (KT // 2) + hf * (KT // 4), 8)
                    dst[slot, :, 7, rr, :] = v[hf * P:(hf + 1) * P]
        else:
            for i, v in enumerate(_combos(lo[:P], hi[:P], lo[P:], hi[P:])):
                dst.at[slot, :, :, pl.ds(r0, 8)][:, i] = v

    NBLK = DH2 // 16

    def main(_, carry):
        def relayout0(b, c):
            relayout(0, wa_sc, 0, b, False)
            return c
        for part in range(2):
            with jax.named_scope("wait_w"):
                for cp in w_copies(0, part=part):
                    cp.wait()
            with jax.named_scope("relayout"):
                jax.lax.fori_loop(part * NBLK // 2, (NBLK // 2, KH // 16)[part], relayout0, 0, unroll=2)
        for b in range(KH // 16, NBLK):
            relayout(0, wa_sc, 0, b, True)

        def pro_stage(ps_, b):
            n = ps_ * NRB + b
            with jax.named_scope("wait_w"):
                if ps_ == 0:
                    @pl.when(b + 1 < NRB)
                    def _():
                        x_copy(b + 1).wait()

                @pl.when((n >= 2) & (n <= NCH))
                def _():
                    wait_chunk(n - 1)
            cr = jnp.clip(n - 1, 0, NCH - 1)
            dst, slot = (wb_sc, cr) if ps_ == 0 else (wa_sc, cr - (NRB - 2))
            src, si = w_slot(ps_)
            bl = jnp.minimum(b + 1, NRB - 1)
            PW = PRO_PW
            npc = RB * S2 // PW
            assert npc * PW == RB * S2 and PRO_R0 + (NBLK - 1) * PRO_RS < HG * npc
            assert PRO_X0 + (max(RB, 2 * NT) - 1) * PRO_XS < HG * npc and 2 * NRB > UL

            def body(i, c):
                s0 = b * RB + 1
                for sg in range(RB):
                    hp_sc[sg * S2:(sg + 1) * S2, :] = xn_sc[s0 + sg, :, 0:DE]
                for j in range(HG):
                    w = _unpack(rows(w_op(src, si, j // 2, 1 + j % 2), w_op(src, si, j // 2, 3 + j % 2),
                                     w_op(src, si, j // 2, 7, j % 2)))
                    for pi in range(npc):
                        pos = j * npc + pi
                        hx = hp_sc[pi * PW:(pi + 1) * PW, :]
                        k, rem = divmod(pos - PRO_X0, PRO_XS)
                        if ps_ == 0 and rem == 0 and 0 <= k < RB:
                            sn = bl * RB + 1 + k
                            xv = _ext(_ln(x_sc[seg(sn), LN].astype(F32)))
                            xn_sc[sn, :, 0:DE] = xv
                            hx = jnp.concatenate([hx[:-S2], jnp.where(never_sm[0] > 0, xv, hx[-S2:])], axis=0)
                        if ps_ == 1 and rem == 0 and 0 <= k < 2 * NT:
                            conv_u(jnp.minimum(2 * b + k // NT, UL),
                                   slice((k % NT) * 128, (k % NT + 1) * 128))
                        bb, rem = divmod(pos - PRO_R0, PRO_RS)
                        if rem == 0 and 0 <= bb < NBLK:
                            relayout(cr, dst, slot, bb, bb >= KH // 16)
                        r = _dot(plain_lhs(hx, j % 2), w)
                        for a in range(0, PW, 8):
                            sg, off = divmod(pi * PW + a, S2)
                            pre_sc.at[s0 + sg][ps_ * HG + j, off:off + 8, :] = _pack(r[2 * a:2 * a + 16])
                return c
            with jax.named_scope("fused"):
                jax.lax.fori_loop(0, never_sm[0] + 1, body, 0)

        for ps_ in range(NPASS):
            if ps_ == 1:
                with jax.named_scope("wait_in0"):
                    for cp in small + in_copies(0):
                        cp.wait()
                sh = sh_ref[...].astype(F32)
                for j in range(KS):
                    co_sc[j] = jnp.broadcast_to(sh[j:j + 1], (8, DM))
                co_sc[KS] = jnp.broadcast_to(sd_ref[...].astype(F32).reshape(1, DM), (8, DM))

            def blk(b, c, ps_=ps_):
                pro_stage(ps_, b)
                return c
            jax.lax.fori_loop(0, NRB, blk, 0)

        def warm_block0(q):
            uf, kf = conv_fwd(0, q)
            put_spec(0, q, 0, uf)
            put_spec(0, q, 2, kf)
            kr_sc[q] = kf
            ur, um, kr, km = uf[:QB], uf[QB:], kf[:QB], kf[QB:]
            wf_sc[0, 0, q] = (ur * kr - um * km).astype(BF16)
            wf_sc[0, 1, q] = (ur * km + um * kr).astype(BF16)

        def wo_combos(d):
            jp, r = d // 4, (d % 4) * 32
            z = pl.multiple_of(jnp.minimum(never_sm[0], 0) * 16, 16)
            we = _pack(wo_sc[2 * jp * DH + r:2 * jp * DH + r + 32, :])
            wd = _pack(wo_sc[(2 * jp + 1) * DH + r:(2 * jp + 1) * DH + r + 32, :])
            ops = _combos(we[:, EA], we[:, EB], wd[:, EA], wd[:, EB]) + [cols(we[:, EC], wd[:, EC])]
            for i, v in enumerate(ops):
                wc_sc[i, pl.ds(d * 16, 16), :] = v
            return wc_sc[jnp.minimum(never_sm[0], 0), pl.ds(z, 8), 0:128]

        def plain_qkv(eq, ekv, jp):
            res = []
            for odd in range(2):
                kv = plain_proj(ekv(4 * jp + 2 * odd), jp, (1, 2), odd)
                res.append(bf(plain_proj(eq(4 * jp + 2 * odd + 1), jp, (0,), odd), kv[:, :DH], kv[:, DH:]))
            return res

        with jax.named_scope("warm"):
            for q in range(NQ):
                warm_block0(q)
        with jax.named_scope("wait_wo"):
            wo_copy.wait()
        with jax.named_scope("step0"):
            mem0 = mem0_ref[...].astype(F32)
            em0 = _ext(rows(mem0, mem0))
            ex0 = xn(0)
            probes = {}

            def e0(d):
                probes[d + WO_LAG] = wo_combos(d)
                if d not in probes:
                    return rows(em0, ex0)
                tl = jnp.where(never_sm[0] > 0, probes.pop(d), em0[:, EC])
                return rows(cols(em0[:, :2 * KH], tl, em0[:, ES]), ex0)

            def hook0(it):
                if it in (1, 3):
                    conv_spec(1, it // 2)
                    for piece in MAC_PIECES:
                        conv_mac(1, it // 2, piece, 2)
                if 5 <= it < 13:
                    for k in range(2 * (it - 5), min(2 * (it - 4), 3 * NT)):
                        conv_inv(*divmod(k, NT))
            out = attend(lambda jp: plain_qkv(e0, e0, jp), RH, make_mask(RH, (0,)), DIST_HALF,
                         PLAN_HALF, hook0)
            finish(0, x_sc[0:SEG, LN], y_seg(0), rows(out[0:M], mem0), out[M2:], False)

        mask12 = make_mask(R, (0, 1))

        def step(t, first, last):
            c, q = (t + 1) // NQ + 1, (t + 1) % NQ
            x4 = side2(t, op_sc[...])
            un = conv_u(t + UL)
            e2 = h_sc[...]
            em = e2[0:M]
            e1 = xn(t)
            xc = pinned(xc_sc[...], pin_tiles(PIN_U, 2, un) + pin_tiles(PIN_X4, NT, x4))

            def proj(jp):
                x = xc(jp)
                lhs = [x[:, 0:KH], e2[:, ES], rows(em[:, EA], e1[:, EA]), e2[:, EB],
                       rows(em[:, ES], e1[:, ES]), x[:, KH:2 * KH], x[:, 2 * KH:]]
                qs = [plain_proj(e2, jp, (0,), odd) for odd in range(2)]
                kvs = strassen([_unpack(a) for a in lhs], [_unpack(w_mats(jp, (1, 2), i)) for i in range(7)])
                tl = _dot(_unpack(rows(em[:, EC], e1[:, EC], e2[M:, EC])),
                          _unpack(cols(w_mats(jp, (1, 2), 7, 0), w_mats(jp, (1, 2), 7, 1))))
                res = []
                for odd in range(2):
                    g = 2 * jp + odd
                    q1 = _unpack(pre_sc[t, g]).astype(F32) if g < NPA else fill_sc[g - NPA]
                    kv = kvs[odd] + tl[:, odd * 2 * DH:(odd + 1) * 2 * DH]
                    res.append(bf(rows(qs[odd][:M2], q1, qs[odd][M2:]), kv[:, :DH], kv[:, DH:]))
                return res

            held = {}

            def hook(it):
                if it == SPEC_AT:
                    if first:
                        conv_spec(c, q)
                    for piece in MAC_PIECES:
                        conv_mac(c, q, piece, NB)
                if INV_AT <= it < INV_AT + NT:
                    conv_inv(t + 2, it - INV_AT)
                if it == HP:
                    held["x"] = x_sc[seg(t), LN]
                    held["y"] = y_seg(t)
            out = attend(proj, R, mask12, DIST, PLAN, hook)
            op_sc[...] = out[RH:]
            finish(t, held["x"], held["y"], out[0:M2], out[M2:RH], not last)

        def steps(i, carry):
            for j in range(UNROLL):
                step(1 + i * UNROLL + j, j == 0, j == UNROLL - 1)
            return carry

        def phase(p, carry):
            @pl.when(p == 1)
            def _():
                for cp in in_copies(2):
                    cp.wait()

            @pl.when(p >= 2)
            def _():
                out_copy((p - 2) * PH, PH).start()

            with jax.named_scope("steps"):
                jax.lax.fori_loop(p * PHI, (p + 1) * PHI, steps, 0)
            return carry

        for cp in in_copies(1):
            cp.wait()
        jax.lax.fori_loop(0, NPH, phase, 0)
        out_copy((NPH - 2) * PH, NSEG - 2 - (NPH - 2) * PH).start()

        with jax.named_scope("step_last"):
            x4 = side2(NSEG, op_sc[...])
            em = h_sc[0:M, :]
            ex = pinned(h_sc[M:, :], pin_tiles(PIN_X4, NT, x4))
            out = attend(lambda jp: plain_qkv(lambda d: ex(jp), lambda d: rows(em, ex(jp)), jp),
                         SEG, make_mask(RH, (1,), M2), DIST_HALF, PLAN_HALF)
            side2(NSEG + 1, out)
        out_copy(NSEG - 2, 2).start()
        out_copy(0, NSEG).wait()
        return carry

    jax.lax.fori_loop(0, never_sm[0] + 1, main, 0)


def pallas_interleave_layers__memory_aug_recurrent_mem_tr__ssm_conv_h3__prompt_kernel(
    A_x, A_mem0, A_Wq, A_Wk, A_Wv, A_Wo, A_seg_len,
    B_q, B_k, B_v, B_shift_k, B_ssm_k, B_ssm_D,
):
    del B_q
    seg = int(A_seg_len) if isinstance(A_seg_len, (int, np.integer)) else CB // NQ
    return _run(A_x, A_mem0, A_Wq, A_Wk, A_Wv, A_Wo, B_k, B_v, B_shift_k, B_ssm_k, B_ssm_D, SEG=seg)


@functools.partial(jax.jit, static_argnames=("SEG",))
def _run(A_x, A_mem0, A_Wq, A_Wk, A_Wv, A_Wo, B_k, B_v, B_shift_k, B_ssm_k, B_ssm_D, *, SEG):
    B, S, DM = A_x.shape
    assert B == 1
    H, DH = A_Wq.shape[1], A_Wq.shape[2]
    M = A_mem0.shape[1]
    KS = B_shift_k.shape[1]
    R = 2 * (M + SEG)
    NSEG = S // SEG
    NRB = (NSEG - 1) // RB
    NB = S // CB
    QB = CB // NQ
    NCH = 3 * H // HG
    DP = -(-DM // 256) * 256
    fwd, inv = _dft_constants()

    kern = functools.partial(_kernel, S=S, DM=DM, H=H, DH=DH, M=M, SEG=SEG)
    any_spec = pl.BlockSpec(memory_space=pl.ANY)
    out = pl.pallas_call(
        kern,
        out_shape=jax.ShapeDtypeStruct((S, DM), A_x.dtype),
        in_specs=[any_spec] * 13,
        out_specs=any_spec,
        scratch_shapes=[
            pltpu.VMEM((NB + 2, NQ, QB // 8, DM // 128, 4, 8, 128), F32),
            pltpu.VMEM((NQ, 2 * QB, DM), F32),
            pltpu.VMEM((2, 2, NQ, QB, DM), BF16),
            pltpu.VMEM((4, SEG, DM), F32),
            pltpu.VMEM((2 * CB, DP), F32),
            pltpu.VMEM((S, DP), BF16),
            pltpu.VMEM((SEG, DM), F32),
            pltpu.VMEM((NSEG, NPA, SEG // 2, DH), U32),
            pltpu.VMEM((H - NPA, SEG, DH), F32),
            pltpu.VMEM((NSEG, SEG // 2, DP + KH), U32),
            pltpu.VMEM((NCH - NRB + 2, HG // 2, 8, KH // 2, DH), U32),
            pltpu.VMEM((NRB - 1, HG // 2, 8, KH // 2, DH), U32),
            pltpu.VMEM((H * DH, DM), BF16),
            pltpu.VMEM((8, H * DH // 4, KH), U32),
            pltpu.VMEM((R // 2, H * DH // 2), U32),
            pltpu.VMEM((R // 2, H * DH // 2), U32),
            pltpu.VMEM((R // 2, H * DH // 2), U32),
            pltpu.VMEM((3, SEG // 2, H * DH // 2), U32),
            pltpu.VMEM((SEG // 2, 3 * KH), U32),
            pltpu.VMEM((S, DP), BF16),
            pltpu.VMEM((S, DP), BF16),
            pltpu.VMEM((NB, DM, CB), BF16),
            pltpu.VMEM((NCH, DM // 2, 2 * HG, DH), BF16),
            pltpu.VMEM((S, DP), A_x.dtype),
            pltpu.VMEM(fwd.shape, BF16),
            pltpu.VMEM(inv.shape, BF16),
            pltpu.VMEM((S + KPAD, DP), BF16),
            pltpu.VMEM((RB * SEG // 2, DM + KH), U32),
            pltpu.VMEM((M + SEG // 2, DM + KH), U32),
            pltpu.VMEM((KS + 1, 8, DM), F32),
            pltpu.VMEM((M, DM), BF16),
            pltpu.VMEM((KS, DM), BF16),
            pltpu.VMEM((DM,), BF16),
            pltpu.SMEM((1,), jnp.int32),
            pltpu.SemaphoreType.DMA(((NSEG - 1) // RB,)),
            pltpu.SemaphoreType.DMA((3,)),
            pltpu.SemaphoreType.DMA((NCH + 2,)),
            pltpu.SemaphoreType.DMA(()),
        ],
        compiler_params=pltpu.CompilerParams(vmem_limit_bytes=120 * 1024 * 1024),
    )(
        A_x.reshape(S, DM), A_mem0.reshape(M, DM), A_Wq, A_Wk, A_Wv,
        A_Wo.reshape(H * DH, DM), B_k.reshape(S, DM), B_v.reshape(S, DM),
        B_shift_k.T, B_ssm_k, B_ssm_D,
        jnp.asarray(fwd, BF16), jnp.asarray(inv, BF16),
    )
    return out.reshape(B, S, DM)
```

```python
import functools

import numpy as np
import jax
import jax.numpy as jnp
import jax.experimental.pallas as pl
import jax.experimental.pallas.tpu as pltpu

F32 = jnp.float32
BF16 = jnp.bfloat16
U32 = jnp.uint32

CB = 128
NQ = 4
KPAD = 16
HG = 8
NPA = 16
KH = 256
RB = 9
PRO_PW, PRO_X0, PRO_XS, PRO_R0, PRO_RS = 24, 11, 4, 2, 2
WO_LAG = 2
UNROLL = 3
PHI = 3
SPEC_AT, INV_AT, PIN_U, PIN_X4 = 4, 10, 1, 8
DIST, DIST_HALF = (1, 1), (1, 2)
PLAN = ((1, 2), (3, 4), (7,))
PLAN_HALF = ((1,), (2,), (3,), (4,))


def _dft_constants():
    qb = CB // NQ
    hb = qb // 2
    n = np.arange(CB, dtype=np.float64)
    f = np.concatenate([q * qb + np.concatenate([np.arange(0, qb, 2), np.arange(1, qb, 2)])
                        for q in range(NQ)])
    w = np.pi * (2.0 * f + 1.0) / (2 * CB)
    ang = (w[:, None] * (n[None, :] - (CB - 1) / 4.0)).reshape(NQ, qb, CB)
    fwd = np.concatenate([np.cos(ang), -np.sin(ang)], axis=1)
    inv = np.zeros((NQ, 2, hb, CB))
    for p in range(NQ):
        m = (NQ - 1 - p) * hb + np.arange(hb)
        ang = (m[:, None] + 0.5) * w[None, :]
        inv[p, 0] = np.cos(ang) / CB
        inv[p, 1] = -np.sin(ang) / CB
    return fwd.astype(np.float32), inv.astype(np.float32)


def _flip_rows(x):
    i = jax.lax.broadcasted_iota(jnp.int32, (8, x.shape[1]), 0)
    out = []
    for r in range(x.shape[0] - 8, -8, -8):
        v = pltpu.roll(x[r:r + 8], 4, 0)
        for b in (2, 1):
            v = jnp.where((i & b) == 0, pltpu.roll(v, 8 - b, 0), pltpu.roll(v, b, 0))
        out.append(v)
    return jnp.concatenate(out, axis=0)


def _ln(x, eps=1e-5):
    d = x.shape[-1]
    m = jnp.sum(x, axis=-1, keepdims=True) * (1.0 / d)
    xc = x - m
    v = jnp.sum(xc * xc, axis=-1, keepdims=True) * (1.0 / d)
    return xc * jax.lax.rsqrt(v + eps)


def _dot(a, b):
    return jnp.dot(a, b, preferred_element_type=F32)


def _dot_nt(a, b):
    return jax.lax.dot_general(a, b, (((1,), (1,)), ((), ())), preferred_element_type=F32)


def _pack(x):
    return pltpu.bitcast(x.astype(BF16), U32)


def _unpack(x):
    return pltpu.bitcast(x, BF16)


def _ext(r):
    return _pack(jnp.concatenate([r, r[:, :KH] + r[:, KH:2 * KH]], axis=1))


def _in_order(actions):
    def body(i, c):
        for j, act in enumerate(actions):
            pl.when(i == j)(act)
        return c
    jax.lax.fori_loop(0, len(actions), body, 0)


def _kernel(x_hbm, mem0_hbm, wq_hbm, wk_hbm, wv_hbm, wo_hbm, k_hbm, v_hbm,
            sh_hbm, sk_hbm, sd_hbm, fwd_hbm, inv_hbm, o_hbm,
            sp_sc, kr_sc, wf_sc, x2_sc, y_sc, u_sc, op_sc, pre_sc, fill_sc, xn_sc, wa_sc, wb_sc, wo_sc, wc_sc,
            oe_sc, oo_sc, os_sc, ox_sc, xc_sc,
            x_sc, v_sc, sk_sc, st_sc, out_sc, fwd_ref, inv_ref,
            k_sc, hp_sc, h_sc, co_sc, mem0_ref, sh_ref, sd_ref,
            never_sm, sem_x, sem_in, sem_w, sem_out,
            *, S, DM, H, DH, M, SEG):
    NSEG = S // SEG
    M2 = 2 * M
    S2 = SEG // 2
    R = M2 + 2 * SEG
    RH = M2 + SEG
    NB = S // CB
    QB = CB // NQ
    HB = QB // 2
    NT = DM // 128
    PH = PHI * UNROLL
    NRB = (NSEG - 1) // RB
    NPH = (NSEG - 1) // PH
    NG = H // HG
    NCH = 3 * NG
    NPASS = NPA // HG
    DH2 = DM // 2
    HP = H // 2
    DE = DM + KH
    KT = DM - 2 * KH
    NKB = KH // 16
    EA, EB, EC, ES = slice(0, KH), slice(KH, 2 * KH), slice(2 * KH, DM), slice(DM, DE)
    KS = sh_ref.shape[0]
    UL = 2 * NQ + 1
    LN = pl.ds(0, DM)
    assert 2 * KT == KH and 2 <= KS <= 8 and QB == SEG and NRB * RB == NSEG - 1 and NPH * PH == NSEG - 1 and NPASS == 2 and 2 * NRB >= NCH + 1

    mem0_copy = pltpu.make_async_copy(mem0_hbm, mem0_ref, sem_x.at[0])
    small = [pltpu.make_async_copy(s, d, sem_in.at[0]) for s, d in [
        (sh_hbm, sh_ref), (sd_hbm, sd_ref), (fwd_hbm, fwd_ref), (inv_hbm, inv_ref)]]

    def x_copy(b):
        if isinstance(b, int) and b == 0:
            rows = pl.ds(0, (RB + 1) * SEG)
        else:
            rows = pl.ds(pl.multiple_of((b * RB + 1) * SEG, SEG), RB * SEG)
        return pltpu.make_async_copy(x_hbm.at[rows], x_sc.at[rows, LN], sem_x.at[b])

    kb = (0, (UL + 1) * SEG, (UL + PH + 1) * SEG, S)
    sb = (0, 2, (PH + 2) // NQ + 2, NB)

    def in_copies(part):
        def rng(b):
            return pl.ds(b[part], b[part + 1] - b[part])
        sem = sem_in.at[part]
        return [
            pltpu.make_async_copy(k_hbm.at[rng(kb)],
                                  k_sc.at[pl.ds(KPAD + kb[part], kb[part + 1] - kb[part]), LN], sem),
            pltpu.make_async_copy(v_hbm.at[rng(kb)], v_sc.at[rng(kb), LN], sem),
        ] + [pltpu.make_async_copy(sk_hbm.at[:, pl.ds(c * CB, CB)], sk_sc.at[c], sem)
             for c in range(sb[part], sb[part + 1])]

    def w_copies(ci, dst=None, part=None):
        src = (wq_hbm, wk_hbm, wv_hbm)[ci // NG]
        dst = ci if dst is None else dst
        h = NKB // 2
        spans = {None: [(0, DM // 16)], 0: [(0, h), (NKB, NKB + h)],
                 1: [(h, NKB), (NKB + h, DM // 16)]}[part]
        sem = sem_w.at[NCH + 1 if part == 1 else dst]
        return [pltpu.make_async_copy(
            src.at[pl.ds(lo, hi - lo), hf, :, pl.ds((ci % NG) * HG, HG), :],
            st_sc.at[dst, pl.ds(lo, hi - lo), :, pl.ds(hf * HG, HG), :], sem)
            for lo, hi in spans for hf in range(2)]

    wo_copy = pltpu.make_async_copy(wo_hbm, wo_sc, sem_w.at[NCH])

    def out_copy(lo, n):
        rows = pl.ds(lo * SEG if isinstance(lo, int) else pl.multiple_of(lo * SEG, SEG), n * SEG)
        return pltpu.make_async_copy(out_sc.at[rows, LN], o_hbm.at[rows], sem_out)

    def start_all(cps):
        def act():
            for cp in cps:
                cp.start()
        return act

    order = [[mem0_copy, x_copy(0)], w_copies(0, part=0), w_copies(0, part=1), [x_copy(1)], [x_copy(2)]]
    for ci in range(1, NCH):
        order.append(w_copies(ci) + ([x_copy(ci + 2)] if ci + 2 < NRB else []))
        if ci == NRB - 2:
            order.append(small + in_copies(0))
    order += [[wo_copy], in_copies(1), in_copies(2)]
    for i in range(0, len(order), 5):
        _in_order([start_all(cps) for cps in order[i:i + 5]])

    never_sm[0] = 0
    k_sc[0:KPAD, LN] = jnp.zeros((KPAD, DM), BF16)
    sp_sc[NB + 1] = jnp.zeros(sp_sc.shape[1:], F32)
    op_sc[...] = jnp.zeros(op_sc.shape, F32)
    x2_sc[...] = jnp.zeros(x2_sc.shape, F32)
    y_sc[2 * CB - SEG:, LN] = jnp.zeros((SEG, DM), F32)
    mem0_copy.wait()
    x_copy(0).wait()
    for sg in range(RB + 1):
        xn_sc[sg, :, 0:DE] = _ext(_ln(x_sc[sg * SEG:(sg + 1) * SEG, LN].astype(F32)))

    def clip(i, hi):
        return min(max(i, 0), hi) if isinstance(i, int) else jnp.clip(i, 0, hi)

    def scaled(i, m):
        return i * m if isinstance(i, int) else pl.multiple_of(i * m, m)

    def seg(i):
        return pl.ds(scaled(clip(i, NSEG - 1), SEG), SEG)

    def conv_u(s, ln=LN):
        r0 = scaled(clip(s, NSEG - 1), SEG)
        kk = k_sc[pl.ds(r0, KPAD + SEG), ln].astype(F32)[KPAD - 8:]

        def coef(j, rows):
            return jnp.concatenate([co_sc[j, :, ln]] * (rows // 8), axis=0)
        sft = [kk] + [pltpu.roll(kk, j, 0) for j in range(2, KS, 2)]
        ev = functools.reduce(jnp.add, [sft[j // 2][8:] * coef(j, SEG) for j in range(0, KS, 2)])
        od = functools.reduce(jnp.add, [sft[j // 2] * coef(j, SEG + 8) for j in range(1, KS, 2)])
        ks = ev + pltpu.roll(od, 1, 0)[8:]
        u = (ks * v_sc[pl.ds(r0, SEG), ln].astype(F32)).astype(BF16)
        u_sc[pl.ds(r0, SEG), ln] = u
        return u

    def conv_fwd(c, q):
        cc = clip(c, NB - 1)
        f = fwd_ref[q]
        uf = _dot(f, u_sc[pl.ds(scaled(cc, CB), CB), LN])
        kf = _dot_nt(f, sk_sc[cc])
        return uf, kf

    def put_spec(cs, q, which, val):
        for n in range(NT):
            v = val[:, n * 128:(n + 1) * 128].reshape(2, QB // 8, 8, 128)
            sp_sc[cs, q, :, n, which:which + 2] = jnp.stack([v[0], v[1]], axis=1)

    def conv_spec(c, q):
        uf, kf = conv_fwd(c, q)
        cs = clip(c, NB)
        put_spec(cs, q, 0, uf)
        pk = kr_sc[q]
        kr_sc[q] = kf
        kp = jnp.concatenate([
            kf[0:HB] - pk[QB:QB + HB],
            kf[HB:QB] + pk[QB + HB:],
            kf[QB:QB + HB] + pk[0:HB],
            kf[QB + HB:] - pk[HB:QB]], axis=0)
        put_spec(cs, q, 2, kp)

    MAC_PIECES = [(rb, n) for rb in range(QB // 16) for n in range(NT)]

    def conv_mac(c, q, piece, nterms):
        rb2, n = piece
        cs = clip(c, NB)
        rbs = slice(2 * rb2, 2 * rb2 + 2)
        ar = None
        ai = None
        for j in range(nterms):
            if isinstance(cs, int):
                uj, kj = j, cs - j
            else:
                uj = jnp.minimum(j, cs)
                kj = jnp.where(cs - j >= 0, cs - j, NB + 1)
            u = sp_sc[uj, q, rbs, n, 0:2]
            k = sp_sc[kj, q, rbs, n, 2:4]
            tr = u[:, 0] * k[:, 0] - u[:, 1] * k[:, 1]
            ti = u[:, 0] * k[:, 1] + u[:, 1] * k[:, 0]
            ar = tr if ar is None else ar + tr
            ai = ti if ai is None else ai + ti
        ln = slice(n * 128, (n + 1) * 128)
        w = jnp.concatenate([ar.reshape(16, 128), ai.reshape(16, 128)], axis=0).astype(BF16)
        wf_sc[c & 1, 0, q, rb2 * 16:rb2 * 16 + 16, ln] = w[0:16]
        wf_sc[c & 1, 1, q, rb2 * 16:rb2 * 16 + 16, ln] = w[16:]

    def conv_inv(tt, n):
        cb = tt // NQ
        p = tt % NQ
        ln = slice(n * 128, (n + 1) * 128)
        ev = _dot(inv_ref[p, 0], wf_sc[cb & 1, 0, :, :, ln].reshape(CB, 128))
        od = _dot(inv_ref[p, 1], wf_sc[cb & 1, 1, :, :, ln].reshape(CB, 128))
        sd = jnp.concatenate([co_sc[KS, :, ln]] * (HB // 8), axis=0)
        for r, val in ((p, _flip_rows(ev - od)), (2 * NQ - 1 - p, ev + od)):
            ur = scaled(clip(cb, NB - 1) * (2 * NQ) + r, HB)
            yr = scaled((cb & 1) * (2 * NQ) + r, HB)
            y_sc[pl.ds(yr, HB), ln] = val + u_sc[pl.ds(ur, HB), ln].astype(F32) * sd

    def y_seg(s):
        return y_sc[pl.ds(scaled(s & (2 * NQ - 1), SEG), SEG), LN]

    scale = DH ** -0.5
    cexp = scale * float(np.log2(np.e))

    def make_mask(n, x_layers, q0=0):
        qi = jax.lax.broadcasted_iota(jnp.int32, (n - q0, n), 0) + q0
        ki = jax.lax.broadcasted_iota(jnp.int32, (n - q0, n), 1)

        def layer(i):
            xl = jnp.where(i < M2 + SEG, x_layers[0], x_layers[-1])
            return jnp.where(i < M, 0, jnp.where(i < M2, 1, xl))
        same = layer(qi) == layer(ki)
        ok = same & ((qi < M2) | (ki < M2) | (qi >= ki))
        fill = jnp.where(same, -1e9 / scale, -jnp.inf).astype(F32)
        return ok, fill

    def probs(q, k, mask):
        ok, fill = mask
        s = _dot_nt(q, k)
        s = jnp.where(ok, s, fill)
        m = jnp.max(s, axis=-1, keepdims=True)
        p = jnp.exp2((s - m) * cexp)
        l = jnp.sum(p, axis=-1, keepdims=True)
        r = pl.reciprocal(l, approx=True)
        r = r * (2.0 - l * r)
        return (p * r).astype(BF16)

    def w_slot(ci):
        return (wb_sc, ci) if 1 <= ci < NRB - 1 else (wa_sc, max(ci - (NRB - 2), 0))

    def rows(*parts):
        return jnp.concatenate(parts, axis=0)

    def cols(*parts):
        return jnp.concatenate(parts, axis=1)

    def w_op(ref, slot, j, i, odd=None):
        return ref[slot, j, i] if odd is None else ref[slot, j, 7, odd * KT // 2:(odd + 1) * KT // 2]

    def w_mats(jp, mats, i, odd=None):
        return cols(*[w_op(*w_slot(mi * NG + 2 * jp // HG), jp % (HG // 2), i, odd) for mi in mats])

    def plain_lhs(e, odd):
        return _unpack(cols(e[:, EA], e[:, ES], e[:, EC]) if odd else cols(e[:, ES], e[:, EB], e[:, EC]))

    def plain_proj(e, jp, mats, odd):
        w = rows(w_mats(jp, mats, 1 + odd), w_mats(jp, mats, 3 + odd), w_mats(jp, mats, 7, odd))
        return _dot(plain_lhs(e, odd), _unpack(w))

    def strassen(lhs, rhs):
        m = [_dot(a, b) for a, b in zip(lhs, rhs)]
        return strassen_out(m)

    def strassen_out(m):
        c21 = m[1] + m[3]
        c12 = m[2] + m[4]
        c11 = m[0] + m[3][M2:] - m[4][M2:] + m[6]
        c22 = m[0] - m[1][M2:] + m[2][M2:] + m[5]
        return rows(c21[:M2], c11, c21[M2:]), rows(c12, c22)

    def bf(*xs):
        return tuple(x.astype(BF16) for x in xs)

    def xn(s):
        return xn_sc[clip(s, NSEG - 1), :, 0:DE]

    def attend(proj, n, mask, dist, plan, hook=None):
        D1, D2 = dist
        PA = HP - D1 - D2 - 1
        full = n == R
        n2 = n // 2

        def prod(i, p0, p1):
            cs = slice(p0 * DH, p1 * DH)
            ws = slice(p0 * DH // 2, p1 * DH // 2)
            if i == 7:
                return _dot(_unpack(cols(oe_sc[0:n2, cs], oo_sc[0:n2, cs])),
                            _unpack(rows(wc_sc[7, ws, 0:KT], wc_sc[7, ws, KT:2 * KT])))
            if i in (0, 5, 6):
                a = ox_sc[max(i - 4, 0), :, cs]
            else:
                ref = {1: os_sc, 2: oe_sc, 3: oo_sc, 4: os_sc}[i]
                if not full:
                    a = ref[0:n2, cs]
                elif i in (2, 4):
                    a = ref[0:RH // 2, cs]
                else:
                    a = rows(ref[0:M, cs], ref[RH // 2:, cs])
            return _dot(_unpack(a), _unpack(wc_sc[i, ws, :]))

        qkvs = {}
        ps = {}
        m = {}
        for it in range(HP + D1 + D2):
            if it < HP:
                qkvs[it] = proj(it)
            g = it - D1
            if 0 <= g < HP:
                ps[g] = [probs(q, k, mask) for q, k, _ in qkvs[g]]
            g = it - D1 - D2
            if 0 <= g < HP:
                oe, oo = [_dot(p, qkv[2]) for p, qkv in zip(ps.pop(g), qkvs.pop(g))]
                cs = slice(g * DH, (g + 1) * DH)
                oe_sc[0:n2, cs] = _pack(oe)
                oo_sc[0:n2, cs] = _pack(oo)
                os_sc[0:n2, cs] = _pack(oe + oo)
                if full:
                    ox_sc[0, :, cs] = _pack(oe[M2:RH] + oo[RH:])
                    ox_sc[1, :, cs] = _pack(oe[RH:] - oe[M2:RH])
                    ox_sc[2, :, cs] = _pack(oo[M2:RH] - oo[RH:])
            if hook is not None:
                hook(it)
            j = it - (HP - 1)
            if j >= 0:
                for i in plan[j]:
                    m[i] = prod(i, 0, PA)
        early = list(m)
        for i in (range(8) if full else (1, 2, 3, 4, 7)):
            if i not in early:
                m[i] = prod(i, 0, HP)
        for i in early:
            m[i] = prod(i, PA, HP) + m[i]
        c1, c2 = strassen_out(m) if full else (m[1] + m[3], m[2] + m[4])
        return cols(c1, c2, m[7])

    def side2(t, a2):
        x3 = x2_sc[(t - 2) & 3] + a2
        x4 = x3 + _ln(x3) * y_seg(t - 2)
        x4 = x4.astype(out_sc.dtype)
        out_sc[seg(t - 2), LN] = x4
        return x4

    def finish(t, xr, yt, mem, a1, spec):
        if spec:
            conv_spec((t + 2) // NQ + 1, (t + 2) % NQ)
        e1 = xn(t + 1)
        for g in range(NPA, H):
            fill_sc[g - NPA] = plain_proj(e1, g // 2, (0,), g % 2)
        x1 = xr.astype(F32) + a1
        x2 = x1 + _ln(x1) * yt
        n1 = _unpack(e1[:, 0:2 * KH]).astype(F32)
        n2 = _ln(x2)
        h_sc[0:M, :] = _ext(mem)
        h_sc[M:, :] = _ext(n2)
        xc_sc[...] = _pack(cols(n1[:, EA] + n2[:, EB], n2[:, EA] - n1[:, EA], n1[:, EB] - n2[:, EB]))
        x2_sc[t & 3] = x2

    def pinned(r, pins):
        never = never_sm[0] > 0
        hs = {0: r}
        tiles = [r[:, n:n + 128] for n in range(0, r.shape[1], 128)]
        for g, n, d in sorted(pins, key=lambda p: p[0]):
            tiles[n] = jnp.where(never, d, tiles[n])
            hs[g] = cols(*tiles)
        return lambda g: hs[max(k for k in hs if k <= g)]

    def pin_tiles(g0, per, val):
        v = _pack(val)
        return [(g0 + n // per, n, v[:, n * 128:(n + 1) * 128]) for n in range(NT)]

    def wait_chunk(ci):
        for cp in w_copies(0, ci):
            cp.wait()

    def w_block(ci, b):
        x = pltpu.bitcast(st_sc[ci, b], U32)
        sub = jax.lax.broadcasted_iota(jnp.int32, (8, DH), 0)
        res = []
        for par in range(2):
            v = [x[2 * i + par] for i in range(4)]
            for bit in (2, 1):
                keep = (sub & bit) == 0
                for i in range(4):
                    if not i & bit:
                        a, c = v[i], v[i + bit]
                        v[i] = jnp.where(keep, a, pltpu.roll(c, bit, 0))
                        v[i + bit] = jnp.where(keep, pltpu.roll(a, 8 - bit, 0), c)
            res.append(jnp.stack(v))
        return res

    def relayout(ci, dst, slot, b, tail):
        hi_m = U32(0xFFFF0000)

        def even(t):
            return (t[0] & U32(0xFFFF)) | (t[1] << 16)

        def odd(t):
            return (t[0] >> 16) | (t[1] & hi_m)

        if tail:
            for k in range(2):
                tb = 2 * (b - NKB) + k
                t = w_block(ci, 2 * NKB + tb)
                dst[slot, :, 7, pl.ds(tb * 8, 8), :] = even(t)
                dst[slot, :, 7, pl.ds(KT // 2 + tb * 8, 8), :] = odd(t)
            return
        t1 = w_block(ci, b)
        t2 = w_block(ci, b + NKB)

        def plane(t, f):
            return pltpu.bitcast(jnp.concatenate([f(t[0]), f(t[1])], axis=2), F32)

        def pack(v):
            r = pltpu.bitcast(v.astype(BF16).astype(F32), U32)
            return (r[:, :, :DH] >> 16) | r[:, :, DH:]
        f11, f21 = [plane(t, lambda w: w << 16) for t in (t1, t2)]
        f12, f22 = [plane(t, lambda w: w & hi_m) for t in (t1, t2)]
        ops = [pack(f11 + f22), even(t1), pack(f12 - f22), pack(f21 - f11), odd(t2),
               pack(f11 + f12), pack(f21 + f22)]
        for i, v in enumerate(ops):
            dst[slot, :, i, pl.ds(scaled(b, 8), 8), :] = v

    NBLK = DH2 // 16

    def main(_, carry):
        def relayout0(b, c):
            relayout(0, wa_sc, 0, b, False)
            return c
        for part in range(2):
            with jax.named_scope("wait_w"):
                for cp in w_copies(0, part=part):
                    cp.wait()
            with jax.named_scope("relayout"):
                jax.lax.fori_loop(part * NKB // 2, (part + 1) * NKB // 2, relayout0, 0)
        for b in range(NKB, NBLK):
            relayout(0, wa_sc, 0, b, True)

        def pro_stage(ps_, b):
            n = ps_ * NRB + b
            with jax.named_scope("wait_w"):
                if ps_ == 0:
                    @pl.when(b + 1 < NRB)
                    def _():
                        x_copy(b + 1).wait()

                @pl.when((n >= 2) & (n <= NCH))
                def _():
                    wait_chunk(n - 1)
            cr = jnp.clip(n - 1, 0, NCH - 1)
            dst, slot = (wb_sc, cr) if ps_ == 0 else (wa_sc, cr - (NRB - 2))
            src, si = w_slot(ps_)
            bl = jnp.minimum(b + 1, NRB - 1)
            PW = PRO_PW
            npc = RB * S2 // PW
            assert npc * PW == RB * S2 and PRO_R0 + (NBLK - 1) * PRO_RS < HG * npc
            assert PRO_X0 + (max(RB, 2 * NT) - 1) * PRO_XS < HG * npc and 2 * NRB > UL

            def body(i, c):
                s0 = b * RB + 1
                for sg in range(RB):
                    hp_sc[sg * S2:(sg + 1) * S2, :] = xn_sc[s0 + sg, :, 0:DE]
                for j in range(HG):
                    w = _unpack(rows(w_op(src, si, j // 2, 1 + j % 2), w_op(src, si, j // 2, 3 + j % 2),
                                     w_op(src, si, j // 2, 7, j % 2)))
                    for pi in range(npc):
                        pos = j * npc + pi
                        hx = hp_sc[pi * PW:(pi + 1) * PW, :]
                        k, rem = divmod(pos - PRO_X0, PRO_XS)
                        if ps_ == 0 and rem == 0 and 0 <= k < RB:
                            sn = bl * RB + 1 + k
                            xv = _ext(_ln(x_sc[seg(sn), LN].astype(F32)))
                            xn_sc[sn, :, 0:DE] = xv
                            hx = jnp.concatenate([hx[:-S2], jnp.where(never_sm[0] > 0, xv, hx[-S2:])], axis=0)
                        if ps_ == 1 and rem == 0 and 0 <= k < 2 * NT:
                            conv_u(jnp.minimum(2 * b + k // NT, UL),
                                   slice((k % NT) * 128, (k % NT + 1) * 128))
                        bb, rem = divmod(pos - PRO_R0, PRO_RS)
                        if rem == 0 and 0 <= bb < NBLK:
                            relayout(cr, dst, slot, bb, bb >= NKB)
                        r = _dot(plain_lhs(hx, j % 2), w)
                        for a in range(0, 2 * PW, 16):
                            sg, off = divmod(2 * pi * PW + a, SEG)
                            pre_sc[s0 + sg, ps_ * HG + j, off:off + 16, :] = r[a:a + 16].astype(BF16)
                return c
            with jax.named_scope("fused"):
                jax.lax.fori_loop(0, never_sm[0] + 1, body, 0)

        for ps_ in range(NPASS):
            if ps_ == 1:
                with jax.named_scope("wait_in0"):
                    for cp in small + in_copies(0):
                        cp.wait()
                sh = sh_ref[...].astype(F32)
                for j in range(KS):
                    co_sc[j] = jnp.broadcast_to(sh[j:j + 1], (8, DM))
                co_sc[KS] = jnp.broadcast_to(sd_ref[...].astype(F32).reshape(1, DM), (8, DM))

            def blk(b, c, ps_=ps_):
                pro_stage(ps_, b)
                return c
            jax.lax.fori_loop(0, NRB, blk, 0)

        def warm_block0(q):
            uf, kf = conv_fwd(0, q)
            put_spec(0, q, 0, uf)
            put_spec(0, q, 2, kf)
            kr_sc[q] = kf
            ur, um, kr, km = uf[:QB], uf[QB:], kf[:QB], kf[QB:]
            wf_sc[0, 0, q] = (ur * kr - um * km).astype(BF16)
            wf_sc[0, 1, q] = (ur * km + um * kr).astype(BF16)

        def wo_combos(d):
            jp, r = d // 4, (d % 4) * 32
            z = pl.multiple_of(jnp.minimum(never_sm[0], 0) * 16, 16)
            we = wo_sc[2 * jp * DH + r:2 * jp * DH + r + 32, :]
            wd = wo_sc[(2 * jp + 1) * DH + r:(2 * jp + 1) * DH + r + 32, :]
            f11, f12, f21, f22 = [w[:, c].astype(F32) for w in (we, wd) for c in (EA, EB)]
            ops = [_pack(v) for v in (f11 + f22, we[:, EA], f12 - f22, f21 - f11, wd[:, EB],
                                      f11 + f12, f21 + f22, cols(we[:, EC], wd[:, EC]))]
            for i, v in enumerate(ops):
                wc_sc[i, pl.ds(d * 16, 16), :] = v
            return wc_sc[jnp.minimum(never_sm[0], 0), pl.ds(z, 8), 0:128]

        def plain_qkv(eq, ekv, jp):
            res = []
            for odd in range(2):
                kv = plain_proj(ekv(4 * jp + 2 * odd), jp, (1, 2), odd)
                res.append(bf(plain_proj(eq(4 * jp + 2 * odd + 1), jp, (0,), odd), kv[:, :DH], kv[:, DH:]))
            return res

        with jax.named_scope("warm"):
            for q in range(NQ):
                warm_block0(q)
        with jax.named_scope("wait_wo"):
            wo_copy.wait()
        with jax.named_scope("step0"):
            mem0 = mem0_ref[...].astype(F32)
            em0 = _ext(rows(mem0, mem0))
            ex0 = xn(0)
            probes = {}

            def e0(d):
                probes[d + WO_LAG] = wo_combos(d)
                if d not in probes:
                    return rows(em0, ex0)
                tl = jnp.where(never_sm[0] > 0, probes.pop(d), em0[:, EC])
                return rows(cols(em0[:, :2 * KH], tl, em0[:, ES]), ex0)

            def hook0(it):
                if it in (1, 3):
                    conv_spec(1, it // 2)
                    for piece in MAC_PIECES:
                        conv_mac(1, it // 2, piece, 2)
                if 5 <= it < 13:
                    for k in range(2 * (it - 5), min(2 * (it - 4), 3 * NT)):
                        conv_inv(*divmod(k, NT))
            out = attend(lambda jp: plain_qkv(e0, e0, jp), RH, make_mask(RH, (0,)), DIST_HALF,
                         PLAN_HALF, hook0)
            finish(0, x_sc[0:SEG, LN], y_seg(0), rows(out[0:M], mem0), out[M2:], False)

        mask12 = make_mask(R, (0, 1))

        def step(t, first, last):
            c, q = (t + 1) // NQ + 1, (t + 1) % NQ
            x4 = side2(t, op_sc[...])
            un = conv_u(t + UL)
            e2 = h_sc[...]
            em = e2[0:M]
            e1 = xn(t)
            xc = pinned(xc_sc[...], pin_tiles(PIN_U, 2, un) + pin_tiles(PIN_X4, NT, x4))

            def proj(jp):
                x = xc(jp)
                lhs = [x[:, 0:KH], e2[:, ES], rows(em[:, EA], e1[:, EA]), e2[:, EB],
                       rows(em[:, ES], e1[:, ES]), x[:, KH:2 * KH], x[:, 2 * KH:]]
                qs = [plain_proj(e2, jp, (0,), odd) for odd in range(2)]
                kvs = strassen([_unpack(a) for a in lhs], [_unpack(w_mats(jp, (1, 2), i)) for i in range(7)])
                tl = _dot(_unpack(rows(em[:, EC], e1[:, EC], e2[M:, EC])),
                          _unpack(cols(w_mats(jp, (1, 2), 7, 0), w_mats(jp, (1, 2), 7, 1))))
                res = []
                for odd in range(2):
                    g = 2 * jp + odd
                    q1 = pre_sc[t, g].astype(F32) if g < NPA else fill_sc[g - NPA]
                    kv = kvs[odd] + tl[:, odd * 2 * DH:(odd + 1) * 2 * DH]
                    res.append(bf(rows(qs[odd][:M2], q1, qs[odd][M2:]), kv[:, :DH], kv[:, DH:]))
                return res

            held = {}

            def hook(it):
                if it == SPEC_AT:
                    if first:
                        conv_spec(c, q)
                    for piece in MAC_PIECES:
                        conv_mac(c, q, piece, NB)
                if INV_AT <= it < INV_AT + NT:
                    conv_inv(t + 2, it - INV_AT)
                if it == HP:
                    held["x"] = x_sc[seg(t), LN]
                    held["y"] = y_seg(t)
            out = attend(proj, R, mask12, DIST, PLAN, hook)
            op_sc[...] = out[RH:]
            finish(t, held["x"], held["y"], out[0:M2], out[M2:RH], not last)

        def steps(i, carry):
            for j in range(UNROLL):
                step(1 + i * UNROLL + j, j == 0, j == UNROLL - 1)
            return carry

        def phase(p, carry):
            @pl.when(p == 1)
            def _():
                for cp in in_copies(2):
                    cp.wait()

            @pl.when(p >= 2)
            def _():
                out_copy((p - 2) * PH, PH).start()

            with jax.named_scope("steps"):
                jax.lax.fori_loop(p * PHI, (p + 1) * PHI, steps, 0)
            return carry

        for cp in in_copies(1):
            cp.wait()
        jax.lax.fori_loop(0, NPH, phase, 0)
        out_copy((NPH - 2) * PH, NSEG - 2 - (NPH - 2) * PH).start()

        with jax.named_scope("step_last"):
            x4 = side2(NSEG, op_sc[...])
            em = h_sc[0:M, :]
            ex = pinned(h_sc[M:, :], pin_tiles(PIN_X4, NT, x4))
            out = attend(lambda jp: plain_qkv(lambda d: ex(jp), lambda d: rows(em, ex(jp)), jp),
                         SEG, make_mask(RH, (1,), M2), DIST_HALF, PLAN_HALF)
            side2(NSEG + 1, out)
        out_copy(NSEG - 2, 2).start()
        out_copy(0, NSEG).wait()
        return carry

    jax.lax.fori_loop(0, never_sm[0] + 1, main, 0)


def pallas_interleave_layers__memory_aug_recurrent_mem_tr__ssm_conv_h3__prompt_kernel(
    A_x, A_mem0, A_Wq, A_Wk, A_Wv, A_Wo, A_seg_len,
    B_q, B_k, B_v, B_shift_k, B_ssm_k, B_ssm_D,
):
    del B_q
    seg = int(A_seg_len) if isinstance(A_seg_len, (int, np.integer)) else CB // NQ
    return _run(A_x, A_mem0, A_Wq, A_Wk, A_Wv, A_Wo, B_k, B_v, B_shift_k, B_ssm_k, B_ssm_D, SEG=seg)


@functools.partial(jax.jit, static_argnames=("SEG",))
def _run(A_x, A_mem0, A_Wq, A_Wk, A_Wv, A_Wo, B_k, B_v, B_shift_k, B_ssm_k, B_ssm_D, *, SEG):
    B, S, DM = A_x.shape
    assert B == 1
    H, DH = A_Wq.shape[1], A_Wq.shape[2]
    M = A_mem0.shape[1]
    KS = B_shift_k.shape[1]
    R = 2 * (M + SEG)
    NSEG = S // SEG
    NRB = (NSEG - 1) // RB
    NB = S // CB
    QB = CB // NQ
    NCH = 3 * H // HG
    DP = -(-DM // 256) * 256
    fwd, inv = _dft_constants()

    kern = functools.partial(_kernel, S=S, DM=DM, H=H, DH=DH, M=M, SEG=SEG)
    any_spec = pl.BlockSpec(memory_space=pl.ANY)
    out = pl.pallas_call(
        kern,
        out_shape=jax.ShapeDtypeStruct((S, DM), A_x.dtype),
        in_specs=[any_spec] * 13,
        out_specs=any_spec,
        scratch_shapes=[
            pltpu.VMEM((NB + 2, NQ, QB // 8, DM // 128, 4, 8, 128), F32),
            pltpu.VMEM((NQ, 2 * QB, DM), F32),
            pltpu.VMEM((2, 2, NQ, QB, DM), BF16),
            pltpu.VMEM((4, SEG, DM), F32),
            pltpu.VMEM((2 * CB, DP), F32),
            pltpu.VMEM((S, DP), BF16),
            pltpu.VMEM((SEG, DM), F32),
            pltpu.VMEM((NSEG, NPA, SEG, DH), BF16),
            pltpu.VMEM((H - NPA, SEG, DH), F32),
            pltpu.VMEM((NSEG, SEG // 2, DP + KH), U32),
            pltpu.VMEM((NCH - NRB + 2, HG // 2, 8, KH // 2, DH), U32),
            pltpu.VMEM((NRB - 1, HG // 2, 8, KH // 2, DH), U32),
            pltpu.VMEM((H * DH, DM), BF16),
            pltpu.VMEM((8, H * DH // 4, KH), U32),
            pltpu.VMEM((R // 2, H * DH // 2), U32),
            pltpu.VMEM((R // 2, H * DH // 2), U32),
            pltpu.VMEM((R // 2, H * DH // 2), U32),
            pltpu.VMEM((3, SEG // 2, H * DH // 2), U32),
            pltpu.VMEM((SEG // 2, 3 * KH), U32),
            pltpu.VMEM((S, DP), BF16),
            pltpu.VMEM((S, DP), BF16),
            pltpu.VMEM((NB, DM, CB), BF16),
            pltpu.VMEM((NCH, DM // 16, 8, 2 * HG, DH), BF16),
            pltpu.VMEM((S, DP), A_x.dtype),
            pltpu.VMEM(fwd.shape, BF16),
            pltpu.VMEM(inv.shape, BF16),
            pltpu.VMEM((S + KPAD, DP), BF16),
            pltpu.VMEM((RB * SEG // 2, DM + KH), U32),
            pltpu.VMEM((M + SEG // 2, DM + KH), U32),
            pltpu.VMEM((KS + 1, 8, DM), F32),
            pltpu.VMEM((M, DM), BF16),
            pltpu.VMEM((KS, DM), BF16),
            pltpu.VMEM((DM,), BF16),
            pltpu.SMEM((1,), jnp.int32),
            pltpu.SemaphoreType.DMA(((NSEG - 1) // RB,)),
            pltpu.SemaphoreType.DMA((3,)),
            pltpu.SemaphoreType.DMA((NCH + 2,)),
            pltpu.SemaphoreType.DMA(()),
        ],
        compiler_params=pltpu.CompilerParams(vmem_limit_bytes=120 * 1024 * 1024),
    )(
        A_x.reshape(S, DM), A_mem0.reshape(M, DM),
        *[w.reshape(DM // 16, 2, 8, H, DH) for w in (A_Wq, A_Wk, A_Wv)],
        A_Wo.reshape(H * DH, DM), B_k.reshape(S, DM), B_v.reshape(S, DM),
        B_shift_k.T, B_ssm_k, B_ssm_D,
        jnp.asarray(fwd, BF16), jnp.asarray(inv, BF16),
    )
    return out.reshape(B, S, DM)
```

```python
import functools

import numpy as np
import jax
import jax.numpy as jnp
import jax.experimental.pallas as pl
import jax.experimental.pallas.tpu as pltpu

F32 = jnp.float32
BF16 = jnp.bfloat16
U32 = jnp.uint32

CB = 128
NQ = 4
KPAD = 16
HG = 8
NPA = 16
KH = 256
RB = 9
PRO_PW, PRO_X0, PRO_XS, PRO_R0, PRO_RS = 24, 11, 4, 2, 2
UNROLL = 3
PHI = 3
SPEC_AT, INV_AT, PIN_U, PIN_X4 = 4, 10, 1, 8
DIST, DIST_HALF = (1, 1), (1, 2)
ORDER = (0, 1, 5, 2, 6, 3, 4)
PLAN = ((1, 2), (3, 4), (7,))
PLAN_HALF = ((1,), (2,), (3,), (4,))


def _dft_constants():
    qb = CB // NQ
    hb = qb // 2
    n = np.arange(CB, dtype=np.float64)
    f = np.concatenate([q * qb + np.concatenate([np.arange(0, qb, 2), np.arange(1, qb, 2)])
                        for q in range(NQ)])
    w = np.pi * (2.0 * f + 1.0) / (2 * CB)
    ang = (w[:, None] * (n[None, :] - (CB - 1) / 4.0)).reshape(NQ, qb, CB)
    fwd = np.concatenate([np.cos(ang), -np.sin(ang)], axis=1)
    inv = np.zeros((NQ, 2, hb, CB))
    for p in range(NQ):
        m = (NQ - 1 - p) * hb + np.arange(hb)
        ang = (m[:, None] + 0.5) * w[None, :]
        inv[p, 0] = np.cos(ang) / CB
        inv[p, 1] = -np.sin(ang) / CB
    return fwd.astype(np.float32), inv.astype(np.float32)


def _flip_rows(x):
    i = jax.lax.broadcasted_iota(jnp.int32, (8, x.shape[1]), 0)
    out = []
    for r in range(x.shape[0] - 8, -8, -8):
        v = pltpu.roll(x[r:r + 8], 4, 0)
        for b in (2, 1):
            v = jnp.where((i & b) == 0, pltpu.roll(v, 8 - b, 0), pltpu.roll(v, b, 0))
        out.append(v)
    return jnp.concatenate(out, axis=0)


def _ln(x, eps=1e-5):
    d = x.shape[-1]
    m = jnp.sum(x, axis=-1, keepdims=True) * (1.0 / d)
    xc = x - m
    v = jnp.sum(xc * xc, axis=-1, keepdims=True) * (1.0 / d)
    return xc * jax.lax.rsqrt(v + eps)


def _dot(a, b):
    return jnp.dot(a, b, preferred_element_type=F32)


def _dot_nt(a, b):
    return jax.lax.dot_general(a, b, (((1,), (1,)), ((), ())), preferred_element_type=F32)


def _pack(x):
    return pltpu.bitcast(x.astype(BF16), U32)


def _unpack(x):
    return pltpu.bitcast(x, BF16)


def _ext(r):
    return _pack(jnp.concatenate([r, r[:, :KH] + r[:, KH:2 * KH]], axis=1))


def _in_order(actions):
    def body(i, c):
        for j, act in enumerate(actions):
            pl.when(i == j)(act)
        return c
    jax.lax.fori_loop(0, len(actions), body, 0)


def _kernel(x_hbm, mem0_hbm, wq_hbm, wk_hbm, wv_hbm, wo_hbm, k_hbm, v_hbm,
            sh_hbm, sk_hbm, sd_hbm, fwd_hbm, inv_hbm, o_hbm,
            sp_sc, kr_sc, wf_sc, x2_sc, y_sc, u_sc, op_sc, pre_sc, fill_sc, xn_sc, wa_sc, wb_sc, wo_sc, wc_sc,
            oe_sc, oo_sc, os_sc, ox_sc, xc_sc,
            x_sc, v_sc, sk_sc, st_sc, out_sc, fwd_ref, inv_ref,
            k_sc, hp_sc, h_sc, co_sc, mem0_ref, sh_ref, sd_ref,
            never_sm, sem_x, sem_in, sem_w, sem_out,
            *, S, DM, H, DH, M, SEG):
    NSEG = S // SEG
    M2 = 2 * M
    S2 = SEG // 2
    R = M2 + 2 * SEG
    RH = M2 + SEG
    NB = S // CB
    QB = CB // NQ
    HB = QB // 2
    NT = DM // 128
    PH = PHI * UNROLL
    NRB = (NSEG - 1) // RB
    NPH = (NSEG - 1) // PH
    NG = H // HG
    NCH = 3 * NG
    NPASS = NPA // HG
    DH2 = DM // 2
    HP = H // 2
    DE = DM + KH
    KT = DM - 2 * KH
    NKB = KH // 16
    EA, EB, EC, ES = slice(0, KH), slice(KH, 2 * KH), slice(2 * KH, DM), slice(DM, DE)
    KS = sh_ref.shape[0]
    UL = 2 * NQ + 1
    LN = pl.ds(0, DM)
    assert 2 * KT == KH and 2 <= KS <= 8 and QB == SEG and NRB * RB == NSEG - 1 and NPH * PH == NSEG - 1 and NPASS == 2 and 2 * NRB >= NCH + 1

    mem0_copy = pltpu.make_async_copy(mem0_hbm, mem0_ref, sem_x.at[0])
    small = [pltpu.make_async_copy(s, d, sem_in.at[0]) for s, d in [
        (sh_hbm, sh_ref), (sd_hbm, sd_ref), (fwd_hbm, fwd_ref), (inv_hbm, inv_ref)]]

    def x_copy(b):
        if isinstance(b, int) and b == 0:
            rows = pl.ds(0, (RB + 1) * SEG)
        else:
            rows = pl.ds(pl.multiple_of((b * RB + 1) * SEG, SEG), RB * SEG)
        return pltpu.make_async_copy(x_hbm.at[rows], x_sc.at[rows, LN], sem_x.at[b])

    kb = (0, (UL + 1) * SEG, (UL + PH + 1) * SEG, S)
    sb = (0, 2, (PH + 2) // NQ + 2, NB)

    def in_copies(part):
        def rng(b):
            return pl.ds(b[part], b[part + 1] - b[part])
        sem = sem_in.at[part]
        return [
            pltpu.make_async_copy(k_hbm.at[rng(kb)],
                                  k_sc.at[pl.ds(KPAD + kb[part], kb[part + 1] - kb[part]), LN], sem),
            pltpu.make_async_copy(v_hbm.at[rng(kb)], v_sc.at[rng(kb), LN], sem),
        ] + [pltpu.make_async_copy(sk_hbm.at[:, pl.ds(c * CB, CB)], sk_sc.at[c], sem)
             for c in range(sb[part], sb[part + 1])]

    def w_copies(ci, dst=None, part=None):
        src = (wq_hbm, wk_hbm, wv_hbm)[ci // NG]
        dst = ci if dst is None else dst
        h = NKB // 2
        spans = {None: [(0, DM // 16)], 0: [(0, h), (NKB, NKB + h)],
                 1: [(h, NKB), (NKB + h, DM // 16)]}[part]
        sem = sem_w.at[NCH + 1 if part == 1 else dst]
        return [pltpu.make_async_copy(
            src.at[pl.ds(lo, hi - lo), hf, :, pl.ds((ci % NG) * HG, HG), :],
            st_sc.at[dst, pl.ds(lo, hi - lo), :, pl.ds(hf * HG, HG), :], sem)
            for lo, hi in spans for hf in range(2)]

    wo_copy = pltpu.make_async_copy(wo_hbm, wo_sc, sem_w.at[NCH])

    def out_copy(lo, n):
        rows = pl.ds(lo * SEG if isinstance(lo, int) else pl.multiple_of(lo * SEG, SEG), n * SEG)
        return pltpu.make_async_copy(out_sc.at[rows, LN], o_hbm.at[rows], sem_out)

    def start_all(cps):
        def act():
            for cp in cps:
                cp.start()
        return act

    order = [[mem0_copy, x_copy(0)], w_copies(0, part=0), w_copies(0, part=1), [x_copy(1)], [x_copy(2)]]
    for ci in range(1, NCH):
        order.append(w_copies(ci) + ([x_copy(ci + 2)] if ci + 2 < NRB else []))
        if ci == NRB - 2:
            order.append(small + in_copies(0))
    order += [[wo_copy], in_copies(1), in_copies(2)]
    for i in range(0, len(order), 5):
        _in_order([start_all(cps) for cps in order[i:i + 5]])

    never_sm[0] = 0
    k_sc[0:KPAD, LN] = jnp.zeros((KPAD, DM), BF16)
    sp_sc[NB + 1] = jnp.zeros(sp_sc.shape[1:], F32)
    op_sc[...] = jnp.zeros(op_sc.shape, F32)
    x2_sc[...] = jnp.zeros(x2_sc.shape, F32)
    y_sc[2 * CB - SEG:, LN] = jnp.zeros((SEG, DM), F32)
    mem0_copy.wait()
    x_copy(0).wait()
    for sg in range(RB + 1):
        xn_sc[sg, :, 0:DE] = _ext(_ln(x_sc[sg * SEG:(sg + 1) * SEG, LN].astype(F32)))

    def clip(i, hi):
        return min(max(i, 0), hi) if isinstance(i, int) else jnp.clip(i, 0, hi)

    def scaled(i, m):
        return i * m if isinstance(i, int) else pl.multiple_of(i * m, m)

    def seg(i):
        return pl.ds(scaled(clip(i, NSEG - 1), SEG), SEG)

    def conv_u(s, ln=LN):
        r0 = scaled(clip(s, NSEG - 1), SEG)
        kk = k_sc[pl.ds(r0, KPAD + SEG), ln].astype(F32)[KPAD - 8:]

        def coef(j, rows):
            return jnp.concatenate([co_sc[j, :, ln]] * (rows // 8), axis=0)
        sft = [kk] + [pltpu.roll(kk, j, 0) for j in range(2, KS, 2)]
        ev = functools.reduce(jnp.add, [sft[j // 2][8:] * coef(j, SEG) for j in range(0, KS, 2)])
        od = functools.reduce(jnp.add, [sft[j // 2] * coef(j, SEG + 8) for j in range(1, KS, 2)])
        ks = ev + pltpu.roll(od, 1, 0)[8:]
        u = (ks * v_sc[pl.ds(r0, SEG), ln].astype(F32)).astype(BF16)
        u_sc[pl.ds(r0, SEG), ln] = u
        return u

    def conv_fwd(c, q):
        cc = clip(c, NB - 1)
        f = fwd_ref[q]
        uf = _dot(f, u_sc[pl.ds(scaled(cc, CB), CB), LN])
        kf = _dot_nt(f, sk_sc[cc])
        return uf, kf

    def put_spec(cs, q, which, val):
        for n in range(NT):
            v = val[:, n * 128:(n + 1) * 128].reshape(2, QB // 8, 8, 128)
            sp_sc[cs, q, :, n, which:which + 2] = jnp.stack([v[0], v[1]], axis=1)

    def conv_spec(c, q):
        uf, kf = conv_fwd(c, q)
        cs = clip(c, NB)
        put_spec(cs, q, 0, uf)
        pk = kr_sc[q]
        kr_sc[q] = kf
        kp = jnp.concatenate([
            kf[0:HB] - pk[QB:QB + HB],
            kf[HB:QB] + pk[QB + HB:],
            kf[QB:QB + HB] + pk[0:HB],
            kf[QB + HB:] - pk[HB:QB]], axis=0)
        put_spec(cs, q, 2, kp)

    MAC_PIECES = [(rb, n) for rb in range(QB // 16) for n in range(NT)]

    def conv_mac(c, q, piece, nterms):
        rb2, n = piece
        cs = clip(c, NB)
        rbs = slice(2 * rb2, 2 * rb2 + 2)
        ar = None
        ai = None
        for j in range(nterms):
            if isinstance(cs, int):
                uj, kj = j, cs - j
            else:
                uj = jnp.minimum(j, cs)
                kj = jnp.where(cs - j >= 0, cs - j, NB + 1)
            u = sp_sc[uj, q, rbs, n, 0:2]
            k = sp_sc[kj, q, rbs, n, 2:4]
            tr = u[:, 0] * k[:, 0] - u[:, 1] * k[:, 1]
            ti = u[:, 0] * k[:, 1] + u[:, 1] * k[:, 0]
            ar = tr if ar is None else ar + tr
            ai = ti if ai is None else ai + ti
        ln = slice(n * 128, (n + 1) * 128)
        w = jnp.concatenate([ar.reshape(16, 128), ai.reshape(16, 128)], axis=0).astype(BF16)
        wf_sc[c & 1, 0, q, rb2 * 16:rb2 * 16 + 16, ln] = w[0:16]
        wf_sc[c & 1, 1, q, rb2 * 16:rb2 * 16 + 16, ln] = w[16:]

    def conv_inv(tt, n):
        cb = tt // NQ
        p = tt % NQ
        ln = slice(n * 128, (n + 1) * 128)
        ev = _dot(inv_ref[p, 0], wf_sc[cb & 1, 0, :, :, ln].reshape(CB, 128))
        od = _dot(inv_ref[p, 1], wf_sc[cb & 1, 1, :, :, ln].reshape(CB, 128))
        sd = jnp.concatenate([co_sc[KS, :, ln]] * (HB // 8), axis=0)
        for r, val in ((p, _flip_rows(ev - od)), (2 * NQ - 1 - p, ev + od)):
            ur = scaled(clip(cb, NB - 1) * (2 * NQ) + r, HB)
            yr = scaled((cb & 1) * (2 * NQ) + r, HB)
            y_sc[pl.ds(yr, HB), ln] = val + u_sc[pl.ds(ur, HB), ln].astype(F32) * sd

    def y_seg(s):
        return y_sc[pl.ds(scaled(s & (2 * NQ - 1), SEG), SEG), LN]

    scale = DH ** -0.5
    cexp = scale * float(np.log2(np.e))

    def make_mask(n, x_layers, q0=0):
        qi = jax.lax.broadcasted_iota(jnp.int32, (n - q0, n), 0) + q0
        ki = jax.lax.broadcasted_iota(jnp.int32, (n - q0, n), 1)

        def layer(i):
            xl = jnp.where(i < M2 + SEG, x_layers[0], x_layers[-1])
            return jnp.where(i < M, 0, jnp.where(i < M2, 1, xl))
        same = layer(qi) == layer(ki)
        ok = same & ((qi < M2) | (ki < M2) | (qi >= ki))
        fill = jnp.where(same, -1e9 / scale, -jnp.inf).astype(F32)
        return ok, fill

    def probs(q, k, mask):
        ok, fill = mask
        s = _dot_nt(q, k)
        s = jnp.where(ok, s, fill)
        m = jnp.max(s, axis=-1, keepdims=True)
        p = jnp.exp2((s - m) * cexp)
        l = jnp.sum(p, axis=-1, keepdims=True)
        r = pl.reciprocal(l, approx=True)
        r = r * (2.0 - l * r)
        return (p * r).astype(BF16)

    def w_slot(ci):
        return (wb_sc, ci) if 1 <= ci < NRB - 1 else (wa_sc, max(ci - (NRB - 2), 0))

    def rows(*parts):
        return jnp.concatenate(parts, axis=0)

    def cols(*parts):
        return jnp.concatenate(parts, axis=1)

    def w_op(ref, slot, j, i, odd=None):
        return ref[slot, j, i] if odd is None else ref[slot, j, 7, odd * KT // 2:(odd + 1) * KT // 2]

    def w_mats(jp, mats, i, odd=None):
        return cols(*[w_op(*w_slot(mi * NG + 2 * jp // HG), jp % (HG // 2), i, odd) for mi in mats])

    def plain_lhs(e, odd):
        return _unpack(cols(e[:, EA], e[:, ES], e[:, EC]) if odd else cols(e[:, ES], e[:, EB], e[:, EC]))

    def plain_proj(e, jp, mats, odd):
        w = rows(w_mats(jp, mats, 1 + odd), w_mats(jp, mats, 3 + odd), w_mats(jp, mats, 7, odd))
        return _dot(plain_lhs(e, odd), _unpack(w))

    def strassen(lhs, rhs):
        m = {i: _dot(lhs[i], rhs[i]) for i in ORDER}
        return strassen_out(m)

    def strassen_out(m):
        c21 = m[1] + m[3]
        c12 = m[2] + m[4]
        c11 = m[0] + m[3][M2:] - m[4][M2:] + m[6]
        c22 = m[0] - m[1][M2:] + m[2][M2:] + m[5]
        return rows(c21[:M2], c11, c21[M2:]), rows(c12, c22)

    def bf(*xs):
        return tuple(x.astype(BF16) for x in xs)

    def xn(s):
        return xn_sc[clip(s, NSEG - 1), :, 0:DE]

    def attend(proj, n, mask, dist, plan, hook=None, raw=False):
        D1, D2 = dist
        PA = HP - D1 - D2 - 1
        full = n == R
        n2 = n // 2

        def prod(i, p0, p1):
            cs = slice(p0 * DH, p1 * DH)
            ws = slice(p0 * DH // 2, p1 * DH // 2)
            if raw:
                a = cols(*[ref[0:n2, p * DH:(p + 1) * DH] for p in range(p0, p1) for ref in (oe_sc, oo_sc)])
                return _dot(_unpack(a), wo_sc[2 * p0 * DH:2 * p1 * DH, i * 128:(i + 1) * 128])
            if i == 7:
                return _dot(_unpack(cols(oe_sc[0:n2, cs], oo_sc[0:n2, cs])),
                            _unpack(rows(wc_sc[7, ws, 0:KT], wc_sc[7, ws, KT:2 * KT])))
            if i in (0, 5, 6):
                a = ox_sc[max(i - 4, 0), :, cs]
            else:
                ref = {1: os_sc, 2: oe_sc, 3: oo_sc, 4: os_sc}[i]
                if not full:
                    a = ref[0:n2, cs]
                elif i in (2, 4):
                    a = ref[0:RH // 2, cs]
                else:
                    a = rows(ref[0:M, cs], ref[RH // 2:, cs])
            return _dot(_unpack(a), _unpack(wc_sc[i, ws, :]))

        qkvs = {}
        ps = {}
        m = {}
        for it in range(HP + D1 + D2):
            if it < HP:
                qkvs[it] = proj(it)
            g = it - D1
            if 0 <= g < HP:
                ps[g] = [probs(q, k, mask) for q, k, _ in qkvs[g]]
            g = it - D1 - D2
            if 0 <= g < HP:
                oe, oo = [_dot(p, qkv[2]) for p, qkv in zip(ps.pop(g), qkvs.pop(g))]
                cs = slice(g * DH, (g + 1) * DH)
                oe_sc[0:n2, cs] = _pack(oe)
                oo_sc[0:n2, cs] = _pack(oo)
                if not raw:
                    os_sc[0:n2, cs] = _pack(oe + oo)
                if full:
                    ox_sc[0, :, cs] = _pack(oe[M2:RH] + oo[RH:])
                    ox_sc[1, :, cs] = _pack(oe[RH:] - oe[M2:RH])
                    ox_sc[2, :, cs] = _pack(oo[M2:RH] - oo[RH:])
            if hook is not None:
                hook(it)
            j = it - (HP - 1)
            if j >= 0:
                for i in plan[j]:
                    m[i] = prod(i, 0, PA)
        early = list(m)
        for i in (range(NT) if raw else range(8) if full else (1, 2, 3, 4, 7)):
            if i not in early:
                m[i] = prod(i, 0, HP)
        for i in early:
            m[i] = prod(i, PA, HP) + m[i]
        if raw:
            return cols(*[m[i] for i in range(NT)])
        c1, c2 = strassen_out(m) if full else (m[1] + m[3], m[2] + m[4])
        return cols(c1, c2, m[7])

    def side2(t, a2):
        x3 = x2_sc[(t - 2) & 3] + a2
        x4 = x3 + _ln(x3) * y_seg(t - 2)
        x4 = x4.astype(out_sc.dtype)
        out_sc[seg(t - 2), LN] = x4
        return x4

    def finish(t, xr, yt, mem, a1, spec):
        if spec:
            conv_spec((t + 2) // NQ + 1, (t + 2) % NQ)
        e1 = xn(t + 1)
        for g in range(NPA, H):
            fill_sc[g - NPA] = plain_proj(e1, g // 2, (0,), g % 2)
        x1 = xr.astype(F32) + a1
        x2 = x1 + _ln(x1) * yt
        n1 = _unpack(e1[:, 0:2 * KH]).astype(F32)
        n2 = _ln(x2)
        h_sc[0:M, :] = _ext(mem)
        h_sc[M:, :] = _ext(n2)
        xc_sc[...] = _pack(cols(n1[:, EA] + n2[:, EB], n2[:, EA] - n1[:, EA], n1[:, EB] - n2[:, EB]))
        x2_sc[t & 3] = x2

    def pinned(r, pins):
        never = never_sm[0] > 0
        hs = {0: r}
        tiles = [r[:, n:n + 128] for n in range(0, r.shape[1], 128)]
        for g, n, d in sorted(pins, key=lambda p: p[0]):
            tiles[n] = jnp.where(never, d, tiles[n])
            hs[g] = cols(*tiles)
        return lambda g: hs[max(k for k in hs if k <= g)]

    def pin_tiles(g0, per, val):
        v = _pack(val)
        return [(g0 + n // per, n, v[:, n * 128:(n + 1) * 128]) for n in range(NT)]

    def wait_chunk(ci):
        for cp in w_copies(0, ci):
            cp.wait()

    def w_block(ci, b):
        x = pltpu.bitcast(st_sc[ci, b], U32)
        sub = jax.lax.broadcasted_iota(jnp.int32, (8, DH), 0)
        res = []
        for par in range(2):
            v = [x[2 * i + par] for i in range(4)]
            for bit in (2, 1):
                keep = (sub & bit) == 0
                for i in range(4):
                    if not i & bit:
                        a, c = v[i], v[i + bit]
                        v[i] = jnp.where(keep, a, pltpu.roll(c, bit, 0))
                        v[i + bit] = jnp.where(keep, pltpu.roll(a, 8 - bit, 0), c)
            res.append(jnp.stack(v))
        return res

    def relayout(ci, dst, slot, b, tail):
        hi_m = U32(0xFFFF0000)

        def even(t):
            return (t[0] & U32(0xFFFF)) | (t[1] << 16)

        def odd(t):
            return (t[0] >> 16) | (t[1] & hi_m)

        if tail:
            for k in range(2):
                tb = 2 * (b - NKB) + k
                t = w_block(ci, 2 * NKB + tb)
                dst[slot, :, 7, pl.ds(tb * 8, 8), :] = even(t)
                dst[slot, :, 7, pl.ds(KT // 2 + tb * 8, 8), :] = odd(t)
            return
        t1 = w_block(ci, b)
        t2 = w_block(ci, b + NKB)

        def plane(t, f):
            return pltpu.bitcast(jnp.concatenate([f(t[0]), f(t[1])], axis=2), F32)

        def pack(v):
            r = pltpu.bitcast(v.astype(BF16).astype(F32), U32)
            return (r[:, :, :DH] >> 16) | r[:, :, DH:]
        f11, f21 = [plane(t, lambda w: w << 16) for t in (t1, t2)]
        f12, f22 = [plane(t, lambda w: w & hi_m) for t in (t1, t2)]
        ops = [pack(f11 + f22), even(t1), pack(f12 - f22), pack(f21 - f11), odd(t2),
               pack(f11 + f12), pack(f21 + f22)]
        for i, v in enumerate(ops):
            dst[slot, :, i, pl.ds(scaled(b, 8), 8), :] = v

    NBLK = DH2 // 16

    def main(_, carry):
        def relayout0(b, c):
            relayout(0, wa_sc, 0, b, False)
            return c
        for part in range(2):
            with jax.named_scope("wait_w"):
                for cp in w_copies(0, part=part):
                    cp.wait()
            with jax.named_scope("relayout"):
                jax.lax.fori_loop(part * NKB // 2, (part + 1) * NKB // 2, relayout0, 0)
        for b in range(NKB, NBLK):
            relayout(0, wa_sc, 0, b, True)

        def pro_stage(ps_, b):
            n = ps_ * NRB + b
            with jax.named_scope("wait_w"):
                if ps_ == 0:
                    @pl.when(b + 1 < NRB)
                    def _():
                        x_copy(b + 1).wait()

                @pl.when((n >= 2) & (n <= NCH))
                def _():
                    wait_chunk(n - 1)
            cr = jnp.clip(n - 1, 0, NCH - 1)
            dst, slot = (wb_sc, cr) if ps_ == 0 else (wa_sc, cr - (NRB - 2))
            src, si = w_slot(ps_)
            bl = jnp.minimum(b + 1, NRB - 1)
            PW = PRO_PW
            npc = RB * S2 // PW
            assert npc * PW == RB * S2 and PRO_R0 + (NBLK - 1) * PRO_RS < HG * npc
            assert PRO_X0 + (max(RB, 2 * NT) - 1) * PRO_XS < HG * npc and 2 * NRB > UL

            def body(i, c):
                s0 = b * RB + 1
                for sg in range(RB):
                    hp_sc[sg * S2:(sg + 1) * S2, :] = xn_sc[s0 + sg, :, 0:DE]
                for j in range(HG):
                    w = _unpack(rows(w_op(src, si, j // 2, 1 + j % 2), w_op(src, si, j // 2, 3 + j % 2),
                                     w_op(src, si, j // 2, 7, j % 2)))
                    for pi in range(npc):
                        pos = j * npc + pi
                        hx = hp_sc[pi * PW:(pi + 1) * PW, :]
                        k, rem = divmod(pos - PRO_X0, PRO_XS)
                        if ps_ == 0 and rem == 0 and 0 <= k < RB:
                            sn = bl * RB + 1 + k
                            xv = _ext(_ln(x_sc[seg(sn), LN].astype(F32)))
                            xn_sc[sn, :, 0:DE] = xv
                            hx = jnp.concatenate([hx[:-S2], jnp.where(never_sm[0] > 0, xv, hx[-S2:])], axis=0)
                        if ps_ == 1 and rem == 0 and 0 <= k < 2 * NT:
                            conv_u(jnp.minimum(2 * b + k // NT, UL),
                                   slice((k % NT) * 128, (k % NT + 1) * 128))
                        bb, rem = divmod(pos - PRO_R0, PRO_RS)
                        if rem == 0 and 0 <= bb < NBLK:
                            relayout(cr, dst, slot, bb, bb >= NKB)
                        r = _dot(plain_lhs(hx, j % 2), w)
                        for a in range(0, 2 * PW, 16):
                            sg, off = divmod(2 * pi * PW + a, SEG)
                            pre_sc[s0 + sg, ps_ * HG + j, off:off + 16, :] = r[a:a + 16].astype(BF16)
                return c
            with jax.named_scope("fused"):
                jax.lax.fori_loop(0, never_sm[0] + 1, body, 0)

        for ps_ in range(NPASS):
            if ps_ == 1:
                with jax.named_scope("wait_in0"):
                    for cp in small + in_copies(0):
                        cp.wait()
                sh = sh_ref[...].astype(F32)
                for j in range(KS):
                    co_sc[j] = jnp.broadcast_to(sh[j:j + 1], (8, DM))
                co_sc[KS] = jnp.broadcast_to(sd_ref[...].astype(F32).reshape(1, DM), (8, DM))

            def blk(b, c, ps_=ps_):
                pro_stage(ps_, b)
                return c
            jax.lax.fori_loop(0, NRB, blk, 0)

        def warm_block0(q):
            uf, kf = conv_fwd(0, q)
            put_spec(0, q, 0, uf)
            put_spec(0, q, 2, kf)
            kr_sc[q] = kf
            ur, um, kr, km = uf[:QB], uf[QB:], kf[:QB], kf[QB:]
            wf_sc[0, 0, q] = (ur * kr - um * km).astype(BF16)
            wf_sc[0, 1, q] = (ur * km + um * kr).astype(BF16)

        def wo_combos(d):
            z = jnp.minimum(never_sm[0], 0)
            r = pl.multiple_of(z * 32 + (d // 4) * 2 * DH + (d % 4) * 32, 32)
            we = wo_sc[pl.ds(r, 32), :]
            wd = wo_sc[pl.ds(r + DH, 32), :]
            f11, f12, f21, f22 = [w[:, c].astype(F32) for w in (we, wd) for c in (EA, EB)]
            ops = [_pack(v) for v in (f11 + f22, we[:, EA], f12 - f22, f21 - f11, wd[:, EB],
                                      f11 + f12, f21 + f22, cols(we[:, EC], wd[:, EC]))]
            for i, v in enumerate(ops):
                wc_sc[i, pl.ds(pl.multiple_of((z + d) * 16, 16), 16), :] = v

        def plain_qkv(eq, ekv, jp, after=None):
            res = []
            for odd in range(2):
                kv = plain_proj(ekv, jp, (1, 2), odd)
                if after is not None:
                    after(4 * jp + 2 * odd, kv)
                q = plain_proj(eq, jp, (0,), odd)
                if after is not None:
                    after(4 * jp + 2 * odd + 1, q)
                res.append(bf(q, kv[:, :DH], kv[:, DH:]))
            return res

        with jax.named_scope("warm"):
            for q in range(NQ):
                warm_block0(q)
        with jax.named_scope("wait_wo"):
            wo_copy.wait()
        with jax.named_scope("step0"):
            mem0 = mem0_ref[...].astype(F32)
            e0 = rows(_ext(rows(mem0, mem0)), xn(0))

            def after0(d, r):
                z = jnp.minimum(never_sm[0], 0)
                wc_sc[z, pl.ds(pl.multiple_of(z * 8 + H * DH // 4, 8), 8), 0:DH] = pltpu.bitcast(r[0:8, 0:DH], U32)
                wo_combos(d)

            def hook0(it):
                if it in (1, 3):
                    conv_spec(1, it // 2)
                    for piece in MAC_PIECES:
                        conv_mac(1, it // 2, piece, 2)
                if 5 <= it < 13:
                    for k in range(2 * (it - 5), min(2 * (it - 4), 3 * NT)):
                        conv_inv(*divmod(k, NT))
            out = attend(lambda jp: plain_qkv(e0, e0, jp, after0), RH, make_mask(RH, (0,)), DIST_HALF,
                         PLAN_HALF, hook0, True)
            finish(0, x_sc[0:SEG, LN], y_seg(0), rows(out[0:M], mem0), out[M2:], False)

        mask12 = make_mask(R, (0, 1))

        def step(t, first, last):
            c, q = (t + 1) // NQ + 1, (t + 1) % NQ
            x4 = side2(t, op_sc[...])
            un = conv_u(t + UL)
            e2 = h_sc[...]
            em = e2[0:M]
            e1 = xn(t)
            xc = pinned(xc_sc[...], pin_tiles(PIN_U, 2, un) + pin_tiles(PIN_X4, NT, x4))

            def proj(jp):
                x = xc(jp)
                lhs = [x[:, 0:KH], e2[:, ES], rows(em[:, EA], e1[:, EA]), e2[:, EB],
                       rows(em[:, ES], e1[:, ES]), x[:, KH:2 * KH], x[:, 2 * KH:]]
                qs = [plain_proj(e2, jp, (0,), odd) for odd in range(2)]
                kvs = strassen([_unpack(a) for a in lhs], [_unpack(w_mats(jp, (1, 2), i)) for i in range(7)])
                tl = _dot(_unpack(rows(em[:, EC], e1[:, EC], e2[M:, EC])),
                          _unpack(cols(w_mats(jp, (1, 2), 7, 0), w_mats(jp, (1, 2), 7, 1))))
                res = []
                for odd in range(2):
                    g = 2 * jp + odd
                    q1 = pre_sc[t, g].astype(F32) if g < NPA else fill_sc[g - NPA]
                    kv = kvs[odd] + tl[:, odd * 2 * DH:(odd + 1) * 2 * DH]
                    res.append(bf(rows(qs[odd][:M2], q1, qs[odd][M2:]), kv[:, :DH], kv[:, DH:]))
                return res

            held = {}

            def hook(it):
                if it == SPEC_AT:
                    if first:
                        conv_spec(c, q)
                    for piece in MAC_PIECES:
                        conv_mac(c, q, piece, NB)
                if INV_AT <= it < INV_AT + NT:
                    conv_inv(t + 2, it - INV_AT)
                if it == HP:
                    held["x"] = x_sc[seg(t), LN]
                    held["y"] = y_seg(t)
            out = attend(proj, R, mask12, DIST, PLAN, hook)
            op_sc[...] = out[RH:]
            finish(t, held["x"], held["y"], out[0:M2], out[M2:RH], not last)

        def steps(i, carry):
            for j in range(UNROLL):
                step(1 + i * UNROLL + j, j == 0, j == UNROLL - 1)
            return carry

        def phase(p, carry):
            @pl.when(p == 1)
            def _():
                for cp in in_copies(2):
                    cp.wait()

            @pl.when(p >= 2)
            def _():
                out_copy((p - 2) * PH, PH).start()

            with jax.named_scope("steps"):
                jax.lax.fori_loop(p * PHI, (p + 1) * PHI, steps, 0)
            return carry

        for cp in in_copies(1):
            cp.wait()
        jax.lax.fori_loop(0, NPH, phase, 0)
        out_copy((NPH - 2) * PH, NSEG - 2 - (NPH - 2) * PH).start()

        with jax.named_scope("step_last"):
            x4 = side2(NSEG, op_sc[...])
            em = h_sc[0:M, :]
            ex = pinned(h_sc[M:, :], pin_tiles(PIN_X4, NT, x4))
            out = attend(lambda jp: plain_qkv(ex(jp), rows(em, ex(jp)), jp),
                         SEG, make_mask(RH, (1,), M2), DIST_HALF, PLAN_HALF)
            side2(NSEG + 1, out)
        out_copy(NSEG - 2, 2).start()
        out_copy(0, NSEG).wait()
        return carry

    jax.lax.fori_loop(0, never_sm[0] + 1, main, 0)


def pallas_interleave_layers__memory_aug_recurrent_mem_tr__ssm_conv_h3__prompt_kernel(
    A_x, A_mem0, A_Wq, A_Wk, A_Wv, A_Wo, A_seg_len,
    B_q, B_k, B_v, B_shift_k, B_ssm_k, B_ssm_D,
):
    del B_q
    seg = int(A_seg_len) if isinstance(A_seg_len, (int, np.integer)) else CB // NQ
    return _run(A_x, A_mem0, A_Wq, A_Wk, A_Wv, A_Wo, B_k, B_v, B_shift_k, B_ssm_k, B_ssm_D, SEG=seg)


@functools.partial(jax.jit, static_argnames=("SEG",))
def _run(A_x, A_mem0, A_Wq, A_Wk, A_Wv, A_Wo, B_k, B_v, B_shift_k, B_ssm_k, B_ssm_D, *, SEG):
    B, S, DM = A_x.shape
    assert B == 1
    H, DH = A_Wq.shape[1], A_Wq.shape[2]
    M = A_mem0.shape[1]
    KS = B_shift_k.shape[1]
    R = 2 * (M + SEG)
    NSEG = S // SEG
    NRB = (NSEG - 1) // RB
    NB = S // CB
    QB = CB // NQ
    NCH = 3 * H // HG
    DP = -(-DM // 256) * 256
    fwd, inv = _dft_constants()

    kern = functools.partial(_kernel, S=S, DM=DM, H=H, DH=DH, M=M, SEG=SEG)
    any_spec = pl.BlockSpec(memory_space=pl.ANY)
    out = pl.pallas_call(
        kern,
        out_shape=jax.ShapeDtypeStruct((S, DM), A_x.dtype),
        in_specs=[any_spec] * 13,
        out_specs=any_spec,
        scratch_shapes=[
            pltpu.VMEM((NB + 2, NQ, QB // 8, DM // 128, 4, 8, 128), F32),
            pltpu.VMEM((NQ, 2 * QB, DM), F32),
            pltpu.VMEM((2, 2, NQ, QB, DM), BF16),
            pltpu.VMEM((4, SEG, DM), F32),
            pltpu.VMEM((2 * CB, DP), F32),
            pltpu.VMEM((S, DP), BF16),
            pltpu.VMEM((SEG, DM), F32),
            pltpu.VMEM((NSEG, NPA, SEG, DH), BF16),
            pltpu.VMEM((H - NPA, SEG, DH), F32),
            pltpu.VMEM((NSEG, SEG // 2, DP + KH), U32),
            pltpu.VMEM((NCH - NRB + 2, HG // 2, 8, KH // 2, DH), U32),
            pltpu.VMEM((NRB - 1, HG // 2, 8, KH // 2, DH), U32),
            pltpu.VMEM((H * DH, DM), BF16),
            pltpu.VMEM((8, H * DH // 4 + 16, KH), U32),
            pltpu.VMEM((R // 2, H * DH // 2), U32),
            pltpu.VMEM((R // 2, H * DH // 2), U32),
            pltpu.VMEM((R // 2, H * DH // 2), U32),
            pltpu.VMEM((3, SEG // 2, H * DH // 2), U32),
            pltpu.VMEM((SEG // 2, 3 * KH), U32),
            pltpu.VMEM((S, DP), BF16),
            pltpu.VMEM((S, DP), BF16),
            pltpu.VMEM((NB, DM, CB), BF16),
            pltpu.VMEM((NCH, DM // 16, 8, 2 * HG, DH), BF16),
            pltpu.VMEM((S, DP), A_x.dtype),
            pltpu.VMEM(fwd.shape, BF16),
            pltpu.VMEM(inv.shape, BF16),
            pltpu.VMEM((S + KPAD, DP), BF16),
            pltpu.VMEM((RB * SEG // 2, DM + KH), U32),
            pltpu.VMEM((M + SEG // 2, DM + KH), U32),
            pltpu.VMEM((KS + 1, 8, DM), F32),
            pltpu.VMEM((M, DM), BF16),
            pltpu.VMEM((KS, DM), BF16),
            pltpu.VMEM((DM,), BF16),
            pltpu.SMEM((1,), jnp.int32),
            pltpu.SemaphoreType.DMA(((NSEG - 1) // RB,)),
            pltpu.SemaphoreType.DMA((3,)),
            pltpu.SemaphoreType.DMA((NCH + 2,)),
            pltpu.SemaphoreType.DMA(()),
        ],
        compiler_params=pltpu.CompilerParams(vmem_limit_bytes=120 * 1024 * 1024),
    )(
        A_x.reshape(S, DM), A_mem0.reshape(M, DM),
        *[w.reshape(DM // 16, 2, 8, H, DH) for w in (A_Wq, A_Wk, A_Wv)],
        A_Wo.reshape(H * DH, DM), B_k.reshape(S, DM), B_v.reshape(S, DM),
        B_shift_k.T, B_ssm_k, B_ssm_D,
        jnp.asarray(fwd, BF16), jnp.asarray(inv, BF16),
    )
    return out.reshape(B, S, DM)
```

```python
import functools

import numpy as np
import jax
import jax.numpy as jnp
import jax.experimental.pallas as pl
import jax.experimental.pallas.tpu as pltpu

F32 = jnp.float32
BF16 = jnp.bfloat16
U32 = jnp.uint32

CB = 128
NQ = 4
KPAD = 16
HG = 8
NPA = 16
KH = 256
RB = 9
PRO_PW, PRO_X0, PRO_XS, PRO_R0, PRO_RS = 24, 11, 4, 2, 2
UNROLL = 3
PHI = 3
SPEC_AT, INV_AT, PIN_U, PIN_X4 = 4, 10, 1, 8
DIST, DIST_HALF = (1, 1), (1, 2)
ORDER = (0, 1, 5, 2, 6, 3, 4)
PLAN = ((1, 2), (3, 4), (7,))
PLAN_HALF = ((1,), (2,), (3,), (4,))


def _dft_constants():
    qb = CB // NQ
    hb = qb // 2
    n = np.arange(CB, dtype=np.float64)
    f = np.concatenate([q * qb + np.concatenate([np.arange(0, qb, 2), np.arange(1, qb, 2)])
                        for q in range(NQ)])
    w = np.pi * (2.0 * f + 1.0) / (2 * CB)
    ang = (w[:, None] * (n[None, :] - (CB - 1) / 4.0)).reshape(NQ, qb, CB)
    fwd = np.concatenate([np.cos(ang), -np.sin(ang)], axis=1)
    inv = np.zeros((NQ, 2, hb, CB))
    for p in range(NQ):
        m = (NQ - 1 - p) * hb + np.arange(hb)
        ang = (m[:, None] + 0.5) * w[None, :]
        inv[p, 0] = np.cos(ang) / CB
        inv[p, 1] = -np.sin(ang) / CB
    return fwd.astype(np.float32), inv.astype(np.float32)


def _flip_rows(x):
    i = jax.lax.broadcasted_iota(jnp.int32, (8, x.shape[1]), 0)
    out = []
    for r in range(x.shape[0] - 8, -8, -8):
        v = pltpu.roll(x[r:r + 8], 4, 0)
        for b in (2, 1):
            v = jnp.where((i & b) == 0, pltpu.roll(v, 8 - b, 0), pltpu.roll(v, b, 0))
        out.append(v)
    return jnp.concatenate(out, axis=0)


def _ln(x, eps=1e-5):
    d = x.shape[-1]
    m = jnp.sum(x, axis=-1, keepdims=True) * (1.0 / d)
    xc = x - m
    v = jnp.sum(xc * xc, axis=-1, keepdims=True) * (1.0 / d)
    return xc * jax.lax.rsqrt(v + eps)


def _dot(a, b):
    return jnp.dot(a, b, preferred_element_type=F32)


def _dot_nt(a, b):
    return jax.lax.dot_general(a, b, (((1,), (1,)), ((), ())), preferred_element_type=F32)


def _pack(x):
    return pltpu.bitcast(x.astype(BF16), U32)


def _unpack(x):
    return pltpu.bitcast(x, BF16)


def _ext(r):
    return _pack(jnp.concatenate([r, r[:, :KH] + r[:, KH:2 * KH]], axis=1))


def _in_order(actions):
    def body(i, c):
        for j, act in enumerate(actions):
            pl.when(i == j)(act)
        return c
    jax.lax.fori_loop(0, len(actions), body, 0)


def _kernel(x_hbm, mem0_hbm, wq_hbm, wk_hbm, wv_hbm, wo_hbm, k_hbm, v_hbm,
            sh_hbm, sk_hbm, sd_hbm, fwd_hbm, inv_hbm, o_hbm,
            sp_sc, kr_sc, wf_sc, x2_sc, y_sc, u_sc, op_sc, pre_sc, xn_sc, wa_sc, wb_sc, wo_sc, wc_sc,
            oe_sc, oo_sc, os_sc, ox_sc, xc_sc,
            x_sc, v_sc, sk_sc, st_sc, out_sc, fwd_ref, inv_ref,
            k_sc, hp_sc, h_sc, co_sc, mem0_ref, sh_ref, sd_ref,
            never_sm, sem_x, sem_in, sem_w, sem_out,
            *, S, DM, H, DH, M, SEG):
    NSEG = S // SEG
    M2 = 2 * M
    S2 = SEG // 2
    R = M2 + 2 * SEG
    RH = M2 + SEG
    NB = S // CB
    QB = CB // NQ
    HB = QB // 2
    NT = DM // 128
    PH = PHI * UNROLL
    NRB = (NSEG - 1) // RB
    NPH = (NSEG - 1) // PH
    NG = H // HG
    NCH = 3 * NG
    NPASS = NPA // HG
    DH2 = DM // 2
    HP = H // 2
    DE = DM + KH
    KT = DM - 2 * KH
    NKB = KH // 16
    EA, EB, EC, ES = slice(0, KH), slice(KH, 2 * KH), slice(2 * KH, DM), slice(DM, DE)
    KS = sh_ref.shape[0]
    UL = 2 * NQ + 1
    LN = pl.ds(0, DM)
    assert 2 * KT == KH and 2 <= KS <= 8 and QB == SEG and NRB * RB == NSEG - 1 and NPH * PH == NSEG - 1 and NPASS == 2 and 2 * NRB >= NCH + 1

    mem0_copy = pltpu.make_async_copy(mem0_hbm, mem0_ref, sem_x.at[0])
    small = [pltpu.make_async_copy(s, d, sem_in.at[0]) for s, d in [
        (sh_hbm, sh_ref), (sd_hbm, sd_ref), (fwd_hbm, fwd_ref), (inv_hbm, inv_ref)]]

    def x_copy(b):
        if isinstance(b, int) and b == 0:
            rows = pl.ds(0, (RB + 1) * SEG)
        else:
            rows = pl.ds(pl.multiple_of((b * RB + 1) * SEG, SEG), RB * SEG)
        return pltpu.make_async_copy(x_hbm.at[rows], x_sc.at[rows, LN], sem_x.at[b])

    kb = (0, (UL + 1) * SEG, (UL + PH + 1) * SEG, S)
    sb = (0, 2, (PH + 2) // NQ + 2, NB)

    def in_copies(part):
        def rng(b):
            return pl.ds(b[part], b[part + 1] - b[part])
        sem = sem_in.at[part]
        return [
            pltpu.make_async_copy(k_hbm.at[rng(kb)],
                                  k_sc.at[pl.ds(KPAD + kb[part], kb[part + 1] - kb[part]), LN], sem),
            pltpu.make_async_copy(v_hbm.at[rng(kb)], v_sc.at[rng(kb), LN], sem),
        ] + [pltpu.make_async_copy(sk_hbm.at[:, pl.ds(c * CB, CB)], sk_sc.at[c], sem)
             for c in range(sb[part], sb[part + 1])]

    def w_copies(ci, dst=None, part=None):
        src = (wq_hbm, wk_hbm, wv_hbm)[ci // NG]
        dst = ci if dst is None else dst
        h = NKB // 2
        spans = {None: [(0, DM // 16)], 0: [(0, h), (NKB, NKB + h)],
                 1: [(h, NKB), (NKB + h, DM // 16)]}[part]
        sem = sem_w.at[NCH + 1 if part == 1 else dst]
        return [pltpu.make_async_copy(
            src.at[pl.ds(lo, hi - lo), hf, :, pl.ds((ci % NG) * HG, HG), :],
            st_sc.at[dst, pl.ds(lo, hi - lo), :, pl.ds(hf * HG, HG), :], sem)
            for lo, hi in spans for hf in range(2)]

    wo_copy = pltpu.make_async_copy(wo_hbm, wo_sc, sem_w.at[NCH])

    def out_copy(lo, n):
        rows = pl.ds(lo * SEG if isinstance(lo, int) else pl.multiple_of(lo * SEG, SEG), n * SEG)
        return pltpu.make_async_copy(out_sc.at[rows, LN], o_hbm.at[rows], sem_out)

    def start_all(cps):
        def act():
            for cp in cps:
                cp.start()
        return act

    order = [[mem0_copy, x_copy(0)], w_copies(0, part=0), w_copies(0, part=1), [x_copy(1)], [x_copy(2)]]
    for ci in range(1, NCH):
        order.append(w_copies(ci) + ([x_copy(ci + 2)] if ci + 2 < NRB else []))
        if ci == NRB - 2:
            order.append(small + in_copies(0))
    order += [[wo_copy], in_copies(1), in_copies(2)]
    for i in range(0, len(order), 5):
        _in_order([start_all(cps) for cps in order[i:i + 5]])

    never_sm[0] = 0
    k_sc[0:KPAD, LN] = jnp.zeros((KPAD, DM), BF16)
    sp_sc[NB + 1] = jnp.zeros(sp_sc.shape[1:], F32)
    op_sc[...] = jnp.zeros(op_sc.shape, F32)
    x2_sc[...] = jnp.zeros(x2_sc.shape, F32)
    y_sc[2 * CB - SEG:, LN] = jnp.zeros((SEG, DM), F32)
    mem0_copy.wait()
    x_copy(0).wait()
    for sg in range(RB + 1):
        xn_sc[sg, :, 0:DE] = _ext(_ln(x_sc[sg * SEG:(sg + 1) * SEG, LN].astype(F32)))

    def clip(i, hi):
        return min(max(i, 0), hi) if isinstance(i, int) else jnp.clip(i, 0, hi)

    def scaled(i, m):
        return i * m if isinstance(i, int) else pl.multiple_of(i * m, m)

    def seg(i):
        return pl.ds(scaled(clip(i, NSEG - 1), SEG), SEG)

    def conv_u(s, ln=LN):
        r0 = scaled(clip(s, NSEG - 1), SEG)
        kk = k_sc[pl.ds(r0, KPAD + SEG), ln].astype(F32)[KPAD - 8:]

        def coef(j, rows):
            return jnp.concatenate([co_sc[j, :, ln]] * (rows // 8), axis=0)
        sft = [kk] + [pltpu.roll(kk, j, 0) for j in range(2, KS, 2)]
        ev = functools.reduce(jnp.add, [sft[j // 2][8:] * coef(j, SEG) for j in range(0, KS, 2)])
        od = functools.reduce(jnp.add, [sft[j // 2] * coef(j, SEG + 8) for j in range(1, KS, 2)])
        ks = ev + pltpu.roll(od, 1, 0)[8:]
        u = (ks * v_sc[pl.ds(r0, SEG), ln].astype(F32)).astype(BF16)
        u_sc[pl.ds(r0, SEG), ln] = u
        return u

    def conv_fwd(c, q):
        cc = clip(c, NB - 1)
        f = fwd_ref[q]
        uf = _dot(f, u_sc[pl.ds(scaled(cc, CB), CB), LN])
        kf = _dot_nt(f, sk_sc[cc])
        return uf, kf

    def put_spec(cs, q, which, val):
        for n in range(NT):
            v = val[:, n * 128:(n + 1) * 128].reshape(2, QB // 8, 8, 128)
            sp_sc[cs, q, :, n, which:which + 2] = jnp.stack([v[0], v[1]], axis=1)

    def conv_spec(c, q):
        uf, kf = conv_fwd(c, q)
        cs = clip(c, NB)
        put_spec(cs, q, 0, uf)
        pk = kr_sc[q]
        kr_sc[q] = kf
        kp = jnp.concatenate([
            kf[0:HB] - pk[QB:QB + HB],
            kf[HB:QB] + pk[QB + HB:],
            kf[QB:QB + HB] + pk[0:HB],
            kf[QB + HB:] - pk[HB:QB]], axis=0)
        put_spec(cs, q, 2, kp)

    MAC_PIECES = [(rb, n) for rb in range(QB // 16) for n in range(NT)]

    def conv_mac(c, q, piece, nterms):
        rb2, n = piece
        cs = clip(c, NB)
        rbs = slice(2 * rb2, 2 * rb2 + 2)
        ar = None
        ai = None
        for j in range(nterms):
            if isinstance(cs, int):
                uj, kj = j, cs - j
            else:
                uj = jnp.minimum(j, cs)
                kj = jnp.where(cs - j >= 0, cs - j, NB + 1)
            u = sp_sc[uj, q, rbs, n, 0:2]
            k = sp_sc[kj, q, rbs, n, 2:4]
            tr = u[:, 0] * k[:, 0] - u[:, 1] * k[:, 1]
            ti = u[:, 0] * k[:, 1] + u[:, 1] * k[:, 0]
            ar = tr if ar is None else ar + tr
            ai = ti if ai is None else ai + ti
        ln = slice(n * 128, (n + 1) * 128)
        w = jnp.concatenate([ar.reshape(16, 128), ai.reshape(16, 128)], axis=0).astype(BF16)
        wf_sc[c & 1, 0, q, rb2 * 16:rb2 * 16 + 16, ln] = w[0:16]
        wf_sc[c & 1, 1, q, rb2 * 16:rb2 * 16 + 16, ln] = w[16:]

    def conv_inv(tt, n):
        cb = tt // NQ
        p = tt % NQ
        ln = slice(n * 128, (n + 1) * 128)
        ev = _dot(inv_ref[p, 0], wf_sc[cb & 1, 0, :, :, ln].reshape(CB, 128))
        od = _dot(inv_ref[p, 1], wf_sc[cb & 1, 1, :, :, ln].reshape(CB, 128))
        sd = jnp.concatenate([co_sc[KS, :, ln]] * (HB // 8), axis=0)
        for r, val in ((p, _flip_rows(ev - od)), (2 * NQ - 1 - p, ev + od)):
            ur = scaled(clip(cb, NB - 1) * (2 * NQ) + r, HB)
            yr = scaled((cb & 1) * (2 * NQ) + r, HB)
            y_sc[pl.ds(yr, HB), ln] = val + u_sc[pl.ds(ur, HB), ln].astype(F32) * sd

    def y_seg(s):
        return y_sc[pl.ds(scaled(s & (2 * NQ - 1), SEG), SEG), LN]

    scale = DH ** -0.5
    cexp = scale * float(np.log2(np.e))

    def make_mask(n, x_layers, q0=0):
        qi = jax.lax.broadcasted_iota(jnp.int32, (n - q0, n), 0) + q0
        ki = jax.lax.broadcasted_iota(jnp.int32, (n - q0, n), 1)

        def layer(i):
            xl = jnp.where(i < M2 + SEG, x_layers[0], x_layers[-1])
            return jnp.where(i < M, 0, jnp.where(i < M2, 1, xl))
        same = layer(qi) == layer(ki)
        ok = same & ((qi < M2) | (ki < M2) | (qi >= ki))
        fill = jnp.where(same, -1e9 / scale, -jnp.inf).astype(F32)
        return ok, fill

    def probs(q, k, mask):
        ok, fill = mask
        s = _dot_nt(q, k)
        s = jnp.where(ok, s, fill)
        m = jnp.max(s, axis=-1, keepdims=True)
        p = jnp.exp2((s - m) * cexp)
        l = jnp.sum(p, axis=-1, keepdims=True)
        r = pl.reciprocal(l, approx=True)
        r = r * (2.0 - l * r)
        return (p * r).astype(BF16)

    def w_slot(ci):
        return (wb_sc, ci) if 1 <= ci < NRB - 1 else (wa_sc, max(ci - (NRB - 2), 0))

    def rows(*parts):
        return jnp.concatenate(parts, axis=0)

    def cols(*parts):
        return jnp.concatenate(parts, axis=1)

    def w_op(ref, slot, j, i, odd=None):
        return ref[slot, j, i] if odd is None else ref[slot, j, 7, odd * KT // 2:(odd + 1) * KT // 2]

    def w_mats(jp, mats, i, odd=None):
        return cols(*[w_op(*w_slot(mi * NG + 2 * jp // HG), jp % (HG // 2), i, odd) for mi in mats])

    def plain_lhs(e, odd):
        return _unpack(cols(e[:, EA], e[:, ES], e[:, EC]) if odd else cols(e[:, ES], e[:, EB], e[:, EC]))

    def plain_proj(e, jp, mats, odd):
        w = rows(w_mats(jp, mats, 1 + odd), w_mats(jp, mats, 3 + odd), w_mats(jp, mats, 7, odd))
        return _dot(plain_lhs(e, odd), _unpack(w))

    def strassen(lhs, rhs):
        m = {i: _dot(lhs[i], rhs[i]) for i in ORDER}
        return strassen_out(m, lambda: m[5])

    def strassen_out(m, last):
        c21 = m[1] + m[3]
        c12 = m[2] + m[4]
        c11 = m[0] + m[3][M2:] - m[4][M2:] + m[6]
        c22 = m[0] - m[1][M2:] + m[2][M2:] + last()
        return rows(c21[:M2], c11, c21[M2:]), rows(c12, c22)

    def bf(*xs):
        return tuple(x.astype(BF16) for x in xs)

    def xn(s):
        return xn_sc[clip(s, NSEG - 1), :, 0:DE]

    def attend(proj, n, mask, dist, plan, hook=None, raw=False):
        D1, D2 = dist
        PA = HP - D1 - D2 - 1
        full = n == R
        n2 = n // 2

        def prod(i, p0, p1):
            cs = slice(p0 * DH, p1 * DH)
            ws = slice(p0 * DH // 2, p1 * DH // 2)
            if raw:
                a = cols(*[ref[0:n2, p * DH:(p + 1) * DH] for p in range(p0, p1) for ref in (oe_sc, oo_sc)])
                return _dot(_unpack(a), wo_sc[2 * p0 * DH:2 * p1 * DH, i * 128:(i + 1) * 128])
            if i >= 7:
                rs = slice(RH // 2, n2) if i == 8 else slice(0, min(n2, RH // 2))
                return _dot(_unpack(cols(oe_sc[rs, cs], oo_sc[rs, cs])),
                            _unpack(rows(wc_sc[7, ws, 0:KT], wc_sc[7, ws, KT:2 * KT])))
            if i in (0, 5, 6):
                a = ox_sc[max(i - 4, 0), :, cs]
            else:
                ref = {1: os_sc, 2: oe_sc, 3: oo_sc, 4: os_sc}[i]
                if not full:
                    a = ref[0:n2, cs]
                elif i in (2, 4):
                    a = ref[0:RH // 2, cs]
                else:
                    a = rows(ref[0:M, cs], ref[RH // 2:, cs])
            return _dot(_unpack(a), _unpack(wc_sc[i, ws, :]))

        qkvs = {}
        ps = {}
        m = {}
        for it in range(HP + D1 + D2):
            if it < HP:
                qkvs[it] = proj(it)
            g = it - D1
            if 0 <= g < HP:
                ps[g] = [probs(q, k, mask) for q, k, _ in qkvs[g]]
            g = it - D1 - D2
            if 0 <= g < HP:
                oe, oo = [_dot(p, qkv[2]) for p, qkv in zip(ps.pop(g), qkvs.pop(g))]
                cs = slice(g * DH, (g + 1) * DH)
                oe_sc[0:n2, cs] = _pack(oe)
                oo_sc[0:n2, cs] = _pack(oo)
                if not raw:
                    os_sc[0:n2, cs] = _pack(oe + oo)
                if full:
                    ox_sc[0, :, cs] = _pack(oe[M2:RH] + oo[RH:])
                    ox_sc[1, :, cs] = _pack(oe[RH:] - oe[M2:RH])
                    ox_sc[2, :, cs] = _pack(oo[M2:RH] - oo[RH:])
            if hook is not None:
                hook(it)
            j = it - (HP - 1)
            if j >= 0:
                for i in plan[j]:
                    m[i] = prod(i, 0, PA)
        early = list(m)
        for i in (range(NT) if raw else (0, 1, 2, 3, 4, 6, 7) if full else (1, 2, 3, 4, 7)):
            if i not in early:
                m[i] = prod(i, 0, HP)
        for i in early:
            m[i] = prod(i, PA, HP) + m[i]
        if raw:
            return cols(*[m[i] for i in range(NT)])
        if not full:
            return cols(m[1] + m[3], m[2] + m[4], m[7])
        c1, c2 = strassen_out(m, lambda: prod(5, 0, HP))
        return cols(c1, c2, rows(m[7], prod(8, 0, HP)))

    def side2(t, a2):
        x3 = x2_sc[(t - 2) & 3] + a2
        x4 = x3 + _ln(x3) * y_seg(t - 2)
        x4 = x4.astype(out_sc.dtype)
        out_sc[seg(t - 2), LN] = x4
        return x4

    def finish(t, xr, yt, mem, a1):
        e1 = xn(t + 1)
        x1 = xr.astype(F32) + a1
        x2 = x1 + _ln(x1) * yt
        n1 = _unpack(e1[:, 0:2 * KH]).astype(F32)
        n2 = _ln(x2)
        h_sc[0:M, :] = _ext(mem)
        h_sc[M:, :] = _ext(n2)
        xc_sc[...] = _pack(cols(n1[:, EA] + n2[:, EB], n2[:, EA] - n1[:, EA], n1[:, EB] - n2[:, EB]))
        x2_sc[t & 3] = x2

    def pinned(r, pins):
        never = never_sm[0] > 0
        hs = {0: r}
        tiles = [r[:, n:n + 128] for n in range(0, r.shape[1], 128)]
        for g, n, d in sorted(pins, key=lambda p: p[0]):
            tiles[n] = jnp.where(never, d, tiles[n])
            hs[g] = cols(*tiles)
        return lambda g: hs[max(k for k in hs if k <= g)]

    def pin_tiles(g0, per, val):
        v = _pack(val)
        return [(g0 + n // per, n, v[:, n * 128:(n + 1) * 128]) for n in range(NT)]

    def wait_chunk(ci):
        for cp in w_copies(0, ci):
            cp.wait()

    def w_block(ci, b):
        x = pltpu.bitcast(st_sc[ci, b], U32)
        sub = jax.lax.broadcasted_iota(jnp.int32, (8, DH), 0)
        res = []
        for par in range(2):
            v = [x[2 * i + par] for i in range(4)]
            for bit in (2, 1):
                keep = (sub & bit) == 0
                for i in range(4):
                    if not i & bit:
                        a, c = v[i], v[i + bit]
                        v[i] = jnp.where(keep, a, pltpu.roll(c, bit, 0))
                        v[i + bit] = jnp.where(keep, pltpu.roll(a, 8 - bit, 0), c)
            res.append(jnp.stack(v))
        return res

    def relayout(ci, dst, slot, b, tail):
        hi_m = U32(0xFFFF0000)

        def even(t):
            return (t[0] & U32(0xFFFF)) | (t[1] << 16)

        def odd(t):
            return (t[0] >> 16) | (t[1] & hi_m)

        if tail:
            for k in range(2):
                tb = 2 * (b - NKB) + k
                t = w_block(ci, 2 * NKB + tb)
                dst[slot, :, 7, pl.ds(tb * 8, 8), :] = even(t)
                dst[slot, :, 7, pl.ds(KT // 2 + tb * 8, 8), :] = odd(t)
            return
        t1 = w_block(ci, b)
        t2 = w_block(ci, b + NKB)

        def plane(t, f):
            return pltpu.bitcast(jnp.concatenate([f(t[0]), f(t[1])], axis=2), F32)

        def pack(v):
            r = pltpu.bitcast(v.astype(BF16).astype(F32), U32)
            return (r[:, :, :DH] >> 16) | r[:, :, DH:]
        f11, f21 = [plane(t, lambda w: w << 16) for t in (t1, t2)]
        f12, f22 = [plane(t, lambda w: w & hi_m) for t in (t1, t2)]
        ops = [pack(f11 + f22), even(t1), pack(f12 - f22), pack(f21 - f11), odd(t2),
               pack(f11 + f12), pack(f21 + f22)]
        for i, v in enumerate(ops):
            dst[slot, :, i, pl.ds(scaled(b, 8), 8), :] = v

    NBLK = DH2 // 16

    def main(_, carry):
        def relayout0(b, c):
            relayout(0, wa_sc, 0, b, False)
            return c
        for part in range(2):
            with jax.named_scope("wait_w"):
                for cp in w_copies(0, part=part):
                    cp.wait()
            with jax.named_scope("relayout"):
                jax.lax.fori_loop(part * NKB // 2, (part + 1) * NKB // 2, relayout0, 0)
        for b in range(NKB, NBLK):
            relayout(0, wa_sc, 0, b, True)

        def pro_stage(ps_, b):
            n = ps_ * NRB + b
            with jax.named_scope("wait_w"):
                if ps_ == 0:
                    @pl.when(b + 1 < NRB)
                    def _():
                        x_copy(b + 1).wait()

                @pl.when((n >= 2) & (n <= NCH))
                def _():
                    wait_chunk(n - 1)
            cr = jnp.clip(n - 1, 0, NCH - 1)
            dst, slot = (wb_sc, cr) if ps_ == 0 else (wa_sc, cr - (NRB - 2))
            src, si = w_slot(ps_)
            bl = jnp.minimum(b + 1, NRB - 1)
            PW = PRO_PW
            npc = RB * S2 // PW
            assert npc * PW == RB * S2 and PRO_R0 + (NBLK - 1) * PRO_RS < HG * npc
            assert PRO_X0 + (max(RB, 2 * NT) - 1) * PRO_XS < HG * npc and 2 * NRB > UL

            def body(i, c):
                s0 = b * RB + 1
                for sg in range(RB):
                    hp_sc[sg * S2:(sg + 1) * S2, :] = xn_sc[s0 + sg, :, 0:DE]
                for j in range(HG):
                    w = _unpack(rows(w_op(src, si, j // 2, 1 + j % 2), w_op(src, si, j // 2, 3 + j % 2),
                                     w_op(src, si, j // 2, 7, j % 2)))
                    for pi in range(npc):
                        pos = j * npc + pi
                        hx = hp_sc[pi * PW:(pi + 1) * PW, :]
                        k, rem = divmod(pos - PRO_X0, PRO_XS)
                        if ps_ == 0 and rem == 0 and 0 <= k < RB:
                            sn = bl * RB + 1 + k
                            xv = _ext(_ln(x_sc[seg(sn), LN].astype(F32)))
                            xn_sc[sn, :, 0:DE] = xv
                            hx = jnp.concatenate([hx[:-S2], jnp.where(never_sm[0] > 0, xv, hx[-S2:])], axis=0)
                        if ps_ == 1 and rem == 0 and 0 <= k < 2 * NT:
                            conv_u(jnp.minimum(2 * b + k // NT, UL),
                                   slice((k % NT) * 128, (k % NT + 1) * 128))
                        bb, rem = divmod(pos - PRO_R0, PRO_RS)
                        if rem == 0 and 0 <= bb < NBLK:
                            relayout(cr, dst, slot, bb, bb >= NKB)
                        r = _dot(plain_lhs(hx, j % 2), w)
                        for a in range(0, 2 * PW, 16):
                            sg, off = divmod(2 * pi * PW + a, SEG)
                            pre_sc[s0 + sg, ps_ * HG + j, off:off + 16, :] = r[a:a + 16].astype(BF16)
                return c
            with jax.named_scope("fused"):
                jax.lax.fori_loop(0, never_sm[0] + 1, body, 0)

        for ps_ in range(NPASS):
            if ps_ == 1:
                with jax.named_scope("wait_in0"):
                    for cp in small + in_copies(0):
                        cp.wait()
                sh = sh_ref[...].astype(F32)
                for j in range(KS):
                    co_sc[j] = jnp.broadcast_to(sh[j:j + 1], (8, DM))
                co_sc[KS] = jnp.broadcast_to(sd_ref[...].astype(F32).reshape(1, DM), (8, DM))

            def blk(b, c, ps_=ps_):
                pro_stage(ps_, b)
                return c
            jax.lax.fori_loop(0, NRB, blk, 0)

        def warm_block0(q):
            uf, kf = conv_fwd(0, q)
            put_spec(0, q, 0, uf)
            put_spec(0, q, 2, kf)
            kr_sc[q] = kf
            ur, um, kr, km = uf[:QB], uf[QB:], kf[:QB], kf[QB:]
            wf_sc[0, 0, q] = (ur * kr - um * km).astype(BF16)
            wf_sc[0, 1, q] = (ur * km + um * kr).astype(BF16)

        def wo_combos(d):
            z = jnp.minimum(never_sm[0], 0)
            r = pl.multiple_of(z * 32 + (d // 4) * 2 * DH + (d % 4) * 32, 32)
            we = wo_sc[pl.ds(r, 32), :]
            wd = wo_sc[pl.ds(r + DH, 32), :]
            f11, f12, f21, f22 = [w[:, c].astype(F32) for w in (we, wd) for c in (EA, EB)]
            ops = [_pack(v) for v in (f11 + f22, we[:, EA], f12 - f22, f21 - f11, wd[:, EB],
                                      f11 + f12, f21 + f22, cols(we[:, EC], wd[:, EC]))]
            for i, v in enumerate(ops):
                wc_sc[i, pl.ds(pl.multiple_of((z + d) * 16, 16), 16), :] = v

        def plain_qkv(eq, ekv, jp, after=None):
            res = []
            for odd in range(2):
                kv = plain_proj(ekv, jp, (1, 2), odd)
                if after is not None:
                    after(4 * jp + 2 * odd, kv)
                q = plain_proj(eq, jp, (0,), odd)
                if after is not None:
                    after(4 * jp + 2 * odd + 1, q)
                res.append(bf(q, kv[:, :DH], kv[:, DH:]))
            return res

        with jax.named_scope("warm"):
            for q in range(NQ):
                warm_block0(q)
        with jax.named_scope("wait_wo"):
            wo_copy.wait()
        with jax.named_scope("step0"):
            mem0 = mem0_ref[...].astype(F32)
            e0 = rows(_ext(rows(mem0, mem0)), xn(0))

            def after0(d, r):
                z = jnp.minimum(never_sm[0], 0)
                wc_sc[z, pl.ds(pl.multiple_of(z * 8 + H * DH // 4, 8), 8), 0:DH] = pltpu.bitcast(r[0:8, 0:DH], U32)
                wo_combos(d)

            def hook0(it):
                if 1 <= it <= 2 * NT:
                    conv_inv(*divmod(it - 1, NT))
            out = attend(lambda jp: plain_qkv(e0, e0, jp, after0), RH, make_mask(RH, (0,)), DIST_HALF,
                         PLAN_HALF, hook0, True)
            y0 = y_seg(0)
            for q in range(2):
                conv_spec(1, q)
            for n in range(NT):
                conv_inv(2, n)
            finish(0, x_sc[0:SEG, LN], y0, rows(out[0:M], mem0), out[M2:])
            for q in range(2):
                for piece in MAC_PIECES:
                    conv_mac(1, q, piece, 2)

        mask12 = make_mask(R, (0, 1))

        def step(t, first, last):
            c, q = (t + 1) // NQ + 1, (t + 1) % NQ
            x4 = side2(t, op_sc[...])
            un = conv_u(t + UL)
            e2 = h_sc[...]
            em = e2[0:M]
            e1 = xn(t)
            xc = pinned(xc_sc[...], pin_tiles(PIN_U, 2, un) + pin_tiles(PIN_X4, NT, x4))

            def proj(jp):
                x = xc(jp)
                lhs = [x[:, 0:KH], e2[:, ES], rows(em[:, EA], e1[:, EA]), e2[:, EB],
                       rows(em[:, ES], e1[:, ES]), x[:, KH:2 * KH], x[:, 2 * KH:]]
                pre = 2 * jp < NPA
                mats = (1, 2) if pre else (1, 2, 0)
                w = len(mats) * DH
                if pre:
                    qs = [plain_proj(e2, jp, (0,), odd) for odd in range(2)]
                cs = strassen([_unpack(a) for a in lhs], [_unpack(w_mats(jp, mats, i)) for i in range(7)])
                tl = _dot(_unpack(rows(em[:, EC], e1[:, EC], e2[M:, EC])),
                          _unpack(cols(w_mats(jp, mats, 7, 0), w_mats(jp, mats, 7, 1))))
                res = []
                for odd in range(2):
                    r = cs[odd] + tl[:, odd * w:(odd + 1) * w]
                    if pre:
                        q1 = pre_sc[t, 2 * jp + odd].astype(F32)
                        qq = rows(qs[odd][:M2], q1, qs[odd][M2:])
                    else:
                        qq = r[:, 2 * DH:]
                    res.append(bf(qq, r[:, :DH], r[:, DH:2 * DH]))
                return res

            held = {}

            def hook(it):
                if it == SPEC_AT:
                    if first:
                        conv_spec(c, q)
                    for piece in MAC_PIECES:
                        conv_mac(c, q, piece, NB)
                if INV_AT <= it < INV_AT + NT:
                    conv_inv(t + 2, it - INV_AT)
                if it == HP:
                    held["x"] = x_sc[seg(t), LN]
                    held["y"] = y_seg(t)
            out = attend(proj, R, mask12, DIST, PLAN, hook)
            if not last:
                conv_spec((t + 2) // NQ + 1, (t + 2) % NQ)
            op_sc[...] = out[RH:]
            finish(t, held["x"], held["y"], out[0:M2], out[M2:RH])

        def steps(i, carry):
            for j in range(UNROLL):
                step(1 + i * UNROLL + j, j == 0, j == UNROLL - 1)
            return carry

        def phase(p, carry):
            @pl.when(p == 1)
            def _():
                for cp in in_copies(2):
                    cp.wait()

            @pl.when(p >= 2)
            def _():
                out_copy((p - 2) * PH, PH).start()

            with jax.named_scope("steps"):
                jax.lax.fori_loop(p * PHI, (p + 1) * PHI, steps, 0)
            return carry

        for cp in in_copies(1):
            cp.wait()
        jax.lax.fori_loop(0, NPH, phase, 0)
        out_copy((NPH - 2) * PH, NSEG - 2 - (NPH - 2) * PH).start()

        with jax.named_scope("step_last"):
            x4 = side2(NSEG, op_sc[...])
            em = h_sc[0:M, :]
            ex = pinned(h_sc[M:, :], pin_tiles(PIN_X4, NT, x4))
            out = attend(lambda jp: plain_qkv(ex(jp), rows(em, ex(jp)), jp),
                         SEG, make_mask(RH, (1,), M2), DIST_HALF, PLAN_HALF)
            side2(NSEG + 1, out)
        out_copy(NSEG - 2, 2).start()
        out_copy(0, NSEG).wait()
        return carry

    jax.lax.fori_loop(0, never_sm[0] + 1, main, 0)


def pallas_interleave_layers__memory_aug_recurrent_mem_tr__ssm_conv_h3__prompt_kernel(
    A_x, A_mem0, A_Wq, A_Wk, A_Wv, A_Wo, A_seg_len,
    B_q, B_k, B_v, B_shift_k, B_ssm_k, B_ssm_D,
):
    del B_q
    seg = int(A_seg_len) if isinstance(A_seg_len, (int, np.integer)) else CB // NQ
    return _run(A_x, A_mem0, A_Wq, A_Wk, A_Wv, A_Wo, B_k, B_v, B_shift_k, B_ssm_k, B_ssm_D, SEG=seg)


@functools.partial(jax.jit, static_argnames=("SEG",))
def _run(A_x, A_mem0, A_Wq, A_Wk, A_Wv, A_Wo, B_k, B_v, B_shift_k, B_ssm_k, B_ssm_D, *, SEG):
    B, S, DM = A_x.shape
    assert B == 1
    H, DH = A_Wq.shape[1], A_Wq.shape[2]
    M = A_mem0.shape[1]
    KS = B_shift_k.shape[1]
    R = 2 * (M + SEG)
    NSEG = S // SEG
    NRB = (NSEG - 1) // RB
    NB = S // CB
    QB = CB // NQ
    NCH = 3 * H // HG
    DP = -(-DM // 256) * 256
    fwd, inv = _dft_constants()

    kern = functools.partial(_kernel, S=S, DM=DM, H=H, DH=DH, M=M, SEG=SEG)
    any_spec = pl.BlockSpec(memory_space=pl.ANY)
    out = pl.pallas_call(
        kern,
        out_shape=jax.ShapeDtypeStruct((S, DM), A_x.dtype),
        in_specs=[any_spec] * 13,
        out_specs=any_spec,
        scratch_shapes=[
            pltpu.VMEM((NB + 2, NQ, QB // 8, DM // 128, 4, 8, 128), F32),
            pltpu.VMEM((NQ, 2 * QB, DM), F32),
            pltpu.VMEM((2, 2, NQ, QB, DM), BF16),
            pltpu.VMEM((4, SEG, DM), F32),
            pltpu.VMEM((2 * CB, DP), F32),
            pltpu.VMEM((S, DP), BF16),
            pltpu.VMEM((SEG, DM), F32),
            pltpu.VMEM((NSEG, NPA, SEG, DH), BF16),
            pltpu.VMEM((NSEG, SEG // 2, DP + KH), U32),
            pltpu.VMEM((NCH - NRB + 2, HG // 2, 8, KH // 2, DH), U32),
            pltpu.VMEM((NRB - 1, HG // 2, 8, KH // 2, DH), U32),
            pltpu.VMEM((H * DH, DM), BF16),
            pltpu.VMEM((8, H * DH // 4 + 16, KH), U32),
            pltpu.VMEM((R // 2, H * DH // 2), U32),
            pltpu.VMEM((R // 2, H * DH // 2), U32),
            pltpu.VMEM((R // 2, H * DH // 2), U32),
            pltpu.VMEM((3, SEG // 2, H * DH // 2), U32),
            pltpu.VMEM((SEG // 2, 3 * KH), U32),
            pltpu.VMEM((S, DP), BF16),
            pltpu.VMEM((S, DP), BF16),
            pltpu.VMEM((NB, DM, CB), BF16),
            pltpu.VMEM((NCH, DM // 16, 8, 2 * HG, DH), BF16),
            pltpu.VMEM((S, DP), A_x.dtype),
            pltpu.VMEM(fwd.shape, BF16),
            pltpu.VMEM(inv.shape, BF16),
            pltpu.VMEM((S + KPAD, DP), BF16),
            pltpu.VMEM((RB * SEG // 2, DM + KH), U32),
            pltpu.VMEM((M + SEG // 2, DM + KH), U32),
            pltpu.VMEM((KS + 1, 8, DM), F32),
            pltpu.VMEM((M, DM), BF16),
            pltpu.VMEM((KS, DM), BF16),
            pltpu.VMEM((DM,), BF16),
            pltpu.SMEM((1,), jnp.int32),
            pltpu.SemaphoreType.DMA(((NSEG - 1) // RB,)),
            pltpu.SemaphoreType.DMA((3,)),
            pltpu.SemaphoreType.DMA((NCH + 2,)),
            pltpu.SemaphoreType.DMA(()),
        ],
        compiler_params=pltpu.CompilerParams(vmem_limit_bytes=120 * 1024 * 1024),
    )(
        A_x.reshape(S, DM), A_mem0.reshape(M, DM),
        *[w.reshape(DM // 16, 2, 8, H, DH) for w in (A_Wq, A_Wk, A_Wv)],
        A_Wo.reshape(H * DH, DM), B_k.reshape(S, DM), B_v.reshape(S, DM),
        B_shift_k.T, B_ssm_k, B_ssm_D,
        jnp.asarray(fwd, BF16), jnp.asarray(inv, BF16),
    )
    return out.reshape(B, S, DM)
```

```python
import functools

import numpy as np
import jax
import jax.numpy as jnp
import jax.experimental.pallas as pl
import jax.experimental.pallas.tpu as pltpu

F32 = jnp.float32
BF16 = jnp.bfloat16
U32 = jnp.uint32

CB = 128
NQ = 4
KPAD = 16
HG = 8
NPA = 16
KH = 256
RB = 9
PRO_PW, PRO_X0, PRO_XS, PRO_R0, PRO_RS = 24, 11, 4, 2, 2
UNROLL = 3
PHI = 3
SPEC_AT, INV_AT, PIN_U, PIN_X4 = 0, 10, 3, 8
DIST, DIST_HALF = (1, 1), (1, 2)
AHEAD = (1, 2)
MAC_TOP = True
ORDER = (0, 1, 5, 2, 6, 3, 4)
PLAN = ((1, 2), (3, 4), (7,))
PLAN_HALF = ((1,), (2,), (3,), (4,))


def _dft_constants():
    qb = CB // NQ
    hb = qb // 2
    n = np.arange(CB, dtype=np.float64)
    f = np.concatenate([q * qb + np.concatenate([np.arange(0, qb, 2), np.arange(1, qb, 2)])
                        for q in range(NQ)])
    w = np.pi * (2.0 * f + 1.0) / (2 * CB)
    ang = (w[:, None] * (n[None, :] - (CB - 1) / 4.0)).reshape(NQ, qb, CB)
    fwd = np.concatenate([np.cos(ang), -np.sin(ang)], axis=1)
    inv = np.zeros((NQ, 2, hb, CB))
    for p in range(NQ):
        m = (NQ - 1 - p) * hb + np.arange(hb)
        ang = (m[:, None] + 0.5) * w[None, :]
        inv[p, 0] = np.cos(ang) / CB
        inv[p, 1] = -np.sin(ang) / CB
    return fwd.astype(np.float32), inv.astype(np.float32)


def _flip_rows(x):
    i = jax.lax.broadcasted_iota(jnp.int32, (8, x.shape[1]), 0)
    out = []
    for r in range(x.shape[0] - 8, -8, -8):
        v = pltpu.roll(x[r:r + 8], 4, 0)
        for b in (2, 1):
            v = jnp.where((i & b) == 0, pltpu.roll(v, 8 - b, 0), pltpu.roll(v, b, 0))
        out.append(v)
    return jnp.concatenate(out, axis=0)


def _ln(x, eps=1e-5):
    d = x.shape[-1]
    m = jnp.sum(x, axis=-1, keepdims=True) * (1.0 / d)
    xc = x - m
    v = jnp.sum(xc * xc, axis=-1, keepdims=True) * (1.0 / d)
    return xc * jax.lax.rsqrt(v + eps)


def _dot(a, b):
    return jnp.dot(a, b, preferred_element_type=F32)


def _dot_nt(a, b):
    return jax.lax.dot_general(a, b, (((1,), (1,)), ((), ())), preferred_element_type=F32)


def _pack(x):
    return pltpu.bitcast(x.astype(BF16), U32)


def _unpack(x):
    return pltpu.bitcast(x, BF16)


def _ext(r):
    return _pack(jnp.concatenate([r, r[:, :KH] + r[:, KH:2 * KH]], axis=1))


def _in_order(actions):
    def body(i, c):
        for j, act in enumerate(actions):
            pl.when(i == j)(act)
        return c
    jax.lax.fori_loop(0, len(actions), body, 0)


def _kernel(x_hbm, mem0_hbm, wq_hbm, wk_hbm, wv_hbm, wo_hbm, k_hbm, v_hbm,
            sh_hbm, sk_hbm, sd_hbm, fwd_hbm, inv_hbm, o_hbm,
            sp_sc, kr_sc, wf_sc, x2_sc, y_sc, u_sc, op_sc, pre_sc, xn_sc, wa_sc, wb_sc, wo_sc, wc_sc,
            oe_sc, oo_sc, os_sc, ox_sc,
            x_sc, v_sc, sk_sc, st_sc, out_sc, fwd_ref, inv_ref,
            k_sc, hp_sc, h_sc, co_sc, mem0_ref, sh_ref, sd_ref,
            never_sm, sem_x, sem_in, sem_w, sem_out,
            *, S, DM, H, DH, M, SEG):
    NSEG = S // SEG
    M2 = 2 * M
    S2 = SEG // 2
    R = M2 + 2 * SEG
    RH = M2 + SEG
    NB = S // CB
    QB = CB // NQ
    HB = QB // 2
    NT = DM // 128
    PH = PHI * UNROLL
    NRB = (NSEG - 1) // RB
    NPH = (NSEG - 1) // PH
    NG = H // HG
    NCH = 3 * NG
    NPASS = NPA // HG
    DH2 = DM // 2
    HP = H // 2
    DE = DM + KH
    KT = DM - 2 * KH
    NKB = KH // 16
    EA, EB, EC, ES = slice(0, KH), slice(KH, 2 * KH), slice(2 * KH, DM), slice(DM, DE)
    KS = sh_ref.shape[0]
    UL = 2 * NQ + 1
    LN = pl.ds(0, DM)
    assert 2 * KT == KH and 2 <= KS <= 8 and QB == SEG and NRB * RB == NSEG - 1 and NPH * PH == NSEG - 1 and NPASS == 2 and 2 * NRB >= NCH + 1

    mem0_copy = pltpu.make_async_copy(mem0_hbm, mem0_ref, sem_x.at[0])
    small = [pltpu.make_async_copy(s, d, sem_in.at[0]) for s, d in [
        (sh_hbm, sh_ref), (sd_hbm, sd_ref), (fwd_hbm, fwd_ref), (inv_hbm, inv_ref)]]

    def x_copy(b):
        if isinstance(b, int) and b == 0:
            rows = pl.ds(0, (RB + 1) * SEG)
        else:
            rows = pl.ds(pl.multiple_of((b * RB + 1) * SEG, SEG), RB * SEG)
        return pltpu.make_async_copy(x_hbm.at[rows], x_sc.at[rows, LN], sem_x.at[b])

    kb = (0, (UL + 1) * SEG, (UL + PH + 1) * SEG, S)
    sb = (0, 2, (PH + 2) // NQ + 2, NB)

    def in_copies(part):
        def rng(b):
            return pl.ds(b[part], b[part + 1] - b[part])
        sem = sem_in.at[part]
        return [
            pltpu.make_async_copy(k_hbm.at[rng(kb)],
                                  k_sc.at[pl.ds(KPAD + kb[part], kb[part + 1] - kb[part]), LN], sem),
            pltpu.make_async_copy(v_hbm.at[rng(kb)], v_sc.at[rng(kb), LN], sem),
        ] + [pltpu.make_async_copy(sk_hbm.at[:, pl.ds(c * CB, CB)], sk_sc.at[c], sem)
             for c in range(sb[part], sb[part + 1])]

    def w_copies(ci, dst=None, part=None):
        src = (wq_hbm, wk_hbm, wv_hbm)[ci // NG]
        dst = ci if dst is None else dst
        h = NKB // 2
        spans = {None: [(0, DM // 16)], 0: [(0, h), (NKB, NKB + h)],
                 1: [(h, NKB), (NKB + h, DM // 16)]}[part]
        sem = sem_w.at[NCH + 1 if part == 1 else dst]
        return [pltpu.make_async_copy(
            src.at[pl.ds(lo, hi - lo), hf, :, pl.ds((ci % NG) * HG, HG), :],
            st_sc.at[dst, pl.ds(lo, hi - lo), :, pl.ds(hf * HG, HG), :], sem)
            for lo, hi in spans for hf in range(2)]

    wo_copy = pltpu.make_async_copy(wo_hbm, wo_sc, sem_w.at[NCH])

    def out_copy(lo, n):
        rows = pl.ds(lo * SEG if isinstance(lo, int) else pl.multiple_of(lo * SEG, SEG), n * SEG)
        return pltpu.make_async_copy(out_sc.at[rows, LN], o_hbm.at[rows], sem_out)

    def start_all(cps):
        def act():
            for cp in cps:
                cp.start()
        return act

    order = [[mem0_copy, x_copy(0)], w_copies(0, part=0), w_copies(0, part=1), [x_copy(1)], [x_copy(2)]]
    for ci in range(1, NCH):
        order.append(w_copies(ci) + ([x_copy(ci + 2)] if ci + 2 < NRB else []))
        if ci == NRB - 2:
            order.append(small + in_copies(0))
    order += [[wo_copy], in_copies(1), in_copies(2)]
    for i in range(0, len(order), 5):
        _in_order([start_all(cps) for cps in order[i:i + 5]])

    never_sm[0] = 0
    k_sc[0:KPAD, LN] = jnp.zeros((KPAD, DM), BF16)
    sp_sc[NB + 1] = jnp.zeros(sp_sc.shape[1:], F32)
    op_sc[...] = jnp.zeros(op_sc.shape, F32)
    x2_sc[...] = jnp.zeros(x2_sc.shape, F32)
    y_sc[2 * CB - SEG:, LN] = jnp.zeros((SEG, DM), F32)
    mem0_copy.wait()
    x_copy(0).wait()
    for sg in range(RB + 1):
        xn_sc[sg, :, 0:DE] = _ext(_ln(x_sc[sg * SEG:(sg + 1) * SEG, LN].astype(F32)))

    def clip(i, hi):
        return min(max(i, 0), hi) if isinstance(i, int) else jnp.clip(i, 0, hi)

    def scaled(i, m):
        return i * m if isinstance(i, int) else pl.multiple_of(i * m, m)

    def seg(i):
        return pl.ds(scaled(clip(i, NSEG - 1), SEG), SEG)

    def conv_u(s, ln=LN):
        r0 = scaled(clip(s, NSEG - 1), SEG)
        kk = k_sc[pl.ds(r0, KPAD + SEG), ln].astype(F32)[KPAD - 8:]

        def coef(j, rows):
            return jnp.concatenate([co_sc[j, :, ln]] * (rows // 8), axis=0)
        sft = [kk] + [pltpu.roll(kk, j, 0) for j in range(2, KS, 2)]
        ev = functools.reduce(jnp.add, [sft[j // 2][8:] * coef(j, SEG) for j in range(0, KS, 2)])
        od = functools.reduce(jnp.add, [sft[j // 2] * coef(j, SEG + 8) for j in range(1, KS, 2)])
        ks = ev + pltpu.roll(od, 1, 0)[8:]
        u = (ks * v_sc[pl.ds(r0, SEG), ln].astype(F32)).astype(BF16)
        u_sc[pl.ds(r0, SEG), ln] = u
        return u

    def conv_fwd(c, q):
        cc = clip(c, NB - 1)
        f = fwd_ref[q]
        uf = _dot(f, u_sc[pl.ds(scaled(cc, CB), CB), LN])
        kf = _dot_nt(f, sk_sc[cc])
        return uf, kf

    def put_spec(cs, q, which, val):
        for n in range(NT):
            v = val[:, n * 128:(n + 1) * 128].reshape(2, QB // 8, 8, 128)
            sp_sc[cs, q, :, n, which:which + 2] = jnp.stack([v[0], v[1]], axis=1)

    def conv_spec(c, q):
        uf, kf = conv_fwd(c, q)
        cs = clip(c, NB)
        put_spec(cs, q, 0, uf)
        pk = kr_sc[q]
        kr_sc[q] = kf
        kp = jnp.concatenate([
            kf[0:HB] - pk[QB:QB + HB],
            kf[HB:QB] + pk[QB + HB:],
            kf[QB:QB + HB] + pk[0:HB],
            kf[QB + HB:] - pk[HB:QB]], axis=0)
        put_spec(cs, q, 2, kp)

    MAC_PIECES = [(rb, n) for rb in range(QB // 16) for n in range(NT)]

    def conv_mac(c, q, piece, nterms):
        rb2, n = piece
        cs = clip(c, NB)
        rbs = slice(2 * rb2, 2 * rb2 + 2)
        ar = None
        ai = None
        for j in range(nterms):
            if isinstance(cs, int):
                uj, kj = j, cs - j
            else:
                uj = jnp.minimum(j, cs)
                kj = jnp.where(cs - j >= 0, cs - j, NB + 1)
            u = sp_sc[uj, q, rbs, n, 0:2]
            k = sp_sc[kj, q, rbs, n, 2:4]
            tr = u[:, 0] * k[:, 0] - u[:, 1] * k[:, 1]
            ti = u[:, 0] * k[:, 1] + u[:, 1] * k[:, 0]
            ar = tr if ar is None else ar + tr
            ai = ti if ai is None else ai + ti
        ln = slice(n * 128, (n + 1) * 128)
        w = jnp.concatenate([ar.reshape(16, 128), ai.reshape(16, 128)], axis=0).astype(BF16)
        wf_sc[c & 1, 0, q, rb2 * 16:rb2 * 16 + 16, ln] = w[0:16]
        wf_sc[c & 1, 1, q, rb2 * 16:rb2 * 16 + 16, ln] = w[16:]

    def conv_inv(tt, n):
        cb = tt // NQ
        p = tt % NQ
        ln = slice(n * 128, (n + 1) * 128)
        ev = _dot(inv_ref[p, 0], wf_sc[cb & 1, 0, :, :, ln].reshape(CB, 128))
        od = _dot(inv_ref[p, 1], wf_sc[cb & 1, 1, :, :, ln].reshape(CB, 128))
        sd = jnp.concatenate([co_sc[KS, :, ln]] * (HB // 8), axis=0)
        for r, val in ((p, _flip_rows(ev - od)), (2 * NQ - 1 - p, ev + od)):
            ur = scaled(clip(cb, NB - 1) * (2 * NQ) + r, HB)
            yr = scaled((cb & 1) * (2 * NQ) + r, HB)
            y_sc[pl.ds(yr, HB), ln] = val + u_sc[pl.ds(ur, HB), ln].astype(F32) * sd

    def y_seg(s):
        return y_sc[pl.ds(scaled(s & (2 * NQ - 1), SEG), SEG), LN]

    scale = DH ** -0.5
    cexp = scale * float(np.log2(np.e))

    def make_mask(n, x_layers, q0=0):
        qi = jax.lax.broadcasted_iota(jnp.int32, (n - q0, n), 0) + q0
        ki = jax.lax.broadcasted_iota(jnp.int32, (n - q0, n), 1)

        def layer(i):
            xl = jnp.where(i < M2 + SEG, x_layers[0], x_layers[-1])
            return jnp.where(i < M, 0, jnp.where(i < M2, 1, xl))
        same = layer(qi) == layer(ki)
        ok = same & ((qi < M2) | (ki < M2) | (qi >= ki))
        fill = jnp.where(same, -1e9 / scale, -jnp.inf).astype(F32)
        return ok, fill

    def probs(q, k, mask):
        ok, fill = mask
        s = _dot_nt(q, k)
        s = jnp.where(ok, s, fill)
        m = jnp.max(s, axis=-1, keepdims=True)
        p = jnp.exp2((s - m) * cexp)
        l = jnp.sum(p, axis=-1, keepdims=True)
        r = pl.reciprocal(l, approx=True)
        r = r * (2.0 - l * r)
        return (p * r).astype(BF16)

    def w_slot(ci):
        return (wb_sc, ci) if 1 <= ci < NRB - 1 else (wa_sc, max(ci - (NRB - 2), 0))

    def rows(*parts):
        return jnp.concatenate(parts, axis=0)

    def cols(*parts):
        return jnp.concatenate(parts, axis=1)

    def w_op(ref, slot, j, i, odd=None):
        return ref[slot, j, i] if odd is None else ref[slot, j, 7, odd * KT // 2:(odd + 1) * KT // 2]

    def w_mats(jp, mats, i, odd=None):
        return cols(*[w_op(*w_slot(mi * NG + 2 * jp // HG), jp % (HG // 2), i, odd) for mi in mats])

    def plain_lhs(e, odd):
        return _unpack(cols(e[:, EA], e[:, ES], e[:, EC]) if odd else cols(e[:, ES], e[:, EB], e[:, EC]))

    def plain_proj(e, jp, mats, odd):
        w = rows(w_mats(jp, mats, 1 + odd), w_mats(jp, mats, 3 + odd), w_mats(jp, mats, 7, odd))
        return _dot(plain_lhs(e, odd), _unpack(w))

    def strassen(lhs, rhs, m):
        m = dict(m)
        m.update({i: _dot(lhs[i], rhs[i]) for i in ORDER if i not in m})
        return strassen_out(m, lambda: m[5])

    def strassen_out(m, last):
        c21 = m[1] + m[3]
        c12 = m[2] + m[4]
        c11 = m[0] + m[3][M2:] - m[4][M2:] + m[6]
        c22 = m[0] - m[1][M2:] + m[2][M2:] + last()
        return rows(c21[:M2], c11, c21[M2:]), rows(c12, c22)

    def bf(*xs):
        return tuple(x.astype(BF16) for x in xs)

    def xn(s):
        return xn_sc[clip(s, NSEG - 1), :, 0:DE]

    def attend(proj, n, mask, dist, plan, hook=None, raw=False):
        D1, D2 = dist
        PA = HP - D1 - D2 - 1
        full = n == R
        n2 = n // 2

        def prod(i, p0, p1):
            cs = slice(p0 * DH, p1 * DH)
            ws = slice(p0 * DH // 2, p1 * DH // 2)
            if raw:
                a = cols(*[ref[0:n2, p * DH:(p + 1) * DH] for p in range(p0, p1) for ref in (oe_sc, oo_sc)])
                return _dot(_unpack(a), wo_sc[2 * p0 * DH:2 * p1 * DH, i * 128:(i + 1) * 128])
            if i >= 7:
                rs = slice(RH // 2, n2) if i == 8 else slice(0, min(n2, RH // 2))
                return _dot(_unpack(cols(oe_sc[rs, cs], oo_sc[rs, cs])),
                            _unpack(rows(wc_sc[7, ws, 0:KT], wc_sc[7, ws, KT:2 * KT])))
            if i in (0, 5, 6):
                a = ox_sc[max(i - 4, 0), :, cs]
            else:
                ref = {1: os_sc, 2: oe_sc, 3: oo_sc, 4: os_sc}[i]
                if not full:
                    a = ref[0:n2, cs]
                elif i in (2, 4):
                    a = ref[0:RH // 2, cs]
                else:
                    a = rows(ref[0:M, cs], ref[RH // 2:, cs])
            return _dot(_unpack(a), _unpack(wc_sc[i, ws, :]))

        qkvs = {}
        ps = {}
        m = {}
        for it in range(HP + D1 + D2):
            if it < HP:
                qkvs[it] = proj(it)
            g = it - D1
            if 0 <= g < HP:
                ps[g] = [probs(q, k, mask) for q, k, _ in qkvs[g]]
            g = it - D1 - D2
            if 0 <= g < HP:
                oe, oo = [_dot(p, qkv[2]) for p, qkv in zip(ps.pop(g), qkvs.pop(g))]
                cs = slice(g * DH, (g + 1) * DH)
                oe_sc[0:n2, cs] = _pack(oe)
                oo_sc[0:n2, cs] = _pack(oo)
                if not raw:
                    os_sc[0:n2, cs] = _pack(oe + oo)
                if full:
                    ox_sc[0, :, cs] = _pack(oe[M2:RH] + oo[RH:])
                    ox_sc[1, :, cs] = _pack(oe[RH:] - oe[M2:RH])
                    ox_sc[2, :, cs] = _pack(oo[M2:RH] - oo[RH:])
            if hook is not None:
                hook(it)
            j = it - (HP - 1)
            if j >= 0:
                for i in plan[j]:
                    m[i] = prod(i, 0, PA)
        early = list(m)
        for i in (range(NT) if raw else (0, 1, 2, 3, 4, 6, 7) if full else (1, 2, 3, 4, 7)):
            if i not in early:
                m[i] = prod(i, 0, HP)
        for i in early:
            m[i] = prod(i, PA, HP) + m[i]
        if raw:
            return cols(*[m[i] for i in range(NT)])
        if not full:
            return cols(m[1] + m[3], m[2] + m[4], m[7])
        c1, c2 = strassen_out(m, lambda: prod(5, 0, HP))
        return cols(c1, c2, rows(m[7], prod(8, 0, HP)))

    def side2(t, a2):
        x3 = x2_sc[(t - 2) & 3] + a2
        x4 = x3 + _ln(x3) * y_seg(t - 2)
        x4 = x4.astype(out_sc.dtype)
        out_sc[seg(t - 2), LN] = x4
        return x4

    def finish(t, xr, yt, mem, a1):
        x1 = xr.astype(F32) + a1
        x2 = x1 + _ln(x1) * yt
        h_sc[0:M, :] = _ext(mem)
        x2_sc[t & 3] = x2
        return x2

    def prepare(t, x2):
        n1 = _unpack(xn(t)[:, 0:2 * KH]).astype(F32)
        n2 = _ln(x2)
        return _ext(n2), _pack(cols(n1[:, EA] + n2[:, EB], n2[:, EA] - n1[:, EA], n1[:, EB] - n2[:, EB]))

    def pinned(r, pins):
        never = never_sm[0] > 0
        hs = {0: r}
        tiles = [r[:, n:n + 128] for n in range(0, r.shape[1], 128)]
        for g, n, d in sorted(pins, key=lambda p: p[0]):
            tiles[n] = jnp.where(never, d, tiles[n])
            hs[g] = cols(*tiles)
        return lambda g: hs[max(k for k in hs if k <= g)]

    def pin_tiles(g0, per, val):
        v = _pack(val)
        return [(g0 + n // per, n, v[:, n * 128:(n + 1) * 128]) for n in range(NT)]

    def wait_chunk(ci):
        for cp in w_copies(0, ci):
            cp.wait()

    def w_block(ci, b):
        x = pltpu.bitcast(st_sc[ci, b], U32)
        sub = jax.lax.broadcasted_iota(jnp.int32, (8, DH), 0)
        res = []
        for par in range(2):
            v = [x[2 * i + par] for i in range(4)]
            for bit in (2, 1):
                keep = (sub & bit) == 0
                for i in range(4):
                    if not i & bit:
                        a, c = v[i], v[i + bit]
                        v[i] = jnp.where(keep, a, pltpu.roll(c, bit, 0))
                        v[i + bit] = jnp.where(keep, pltpu.roll(a, 8 - bit, 0), c)
            res.append(jnp.stack(v))
        return res

    def relayout(ci, dst, slot, b, tail):
        hi_m = U32(0xFFFF0000)

        def even(t):
            return (t[0] & U32(0xFFFF)) | (t[1] << 16)

        def odd(t):
            return (t[0] >> 16) | (t[1] & hi_m)

        if tail:
            for k in range(2):
                tb = 2 * (b - NKB) + k
                t = w_block(ci, 2 * NKB + tb)
                dst[slot, :, 7, pl.ds(tb * 8, 8), :] = even(t)
                dst[slot, :, 7, pl.ds(KT // 2 + tb * 8, 8), :] = odd(t)
            return
        t1 = w_block(ci, b)
        t2 = w_block(ci, b + NKB)

        def plane(t, f):
            return pltpu.bitcast(jnp.concatenate([f(t[0]), f(t[1])], axis=2), F32)

        def pack(v):
            r = pltpu.bitcast(v.astype(BF16).astype(F32), U32)
            return (r[:, :, :DH] >> 16) | r[:, :, DH:]
        f11, f21 = [plane(t, lambda w: w << 16) for t in (t1, t2)]
        f12, f22 = [plane(t, lambda w: w & hi_m) for t in (t1, t2)]
        ops = [pack(f11 + f22), even(t1), pack(f12 - f22), pack(f21 - f11), odd(t2),
               pack(f11 + f12), pack(f21 + f22)]
        for i, v in enumerate(ops):
            dst[slot, :, i, pl.ds(scaled(b, 8), 8), :] = v

    NBLK = DH2 // 16

    def main(_, carry):
        def relayout0(b, c):
            relayout(0, wa_sc, 0, b, False)
            return c
        for part in range(2):
            with jax.named_scope("wait_w"):
                for cp in w_copies(0, part=part):
                    cp.wait()
            with jax.named_scope("relayout"):
                jax.lax.fori_loop(part * NKB // 2, (part + 1) * NKB // 2, relayout0, 0)
        for b in range(NKB, NBLK):
            relayout(0, wa_sc, 0, b, True)

        def pro_stage(ps_, b):
            n = ps_ * NRB + b
            with jax.named_scope("wait_w"):
                if ps_ == 0:
                    @pl.when(b + 1 < NRB)
                    def _():
                        x_copy(b + 1).wait()

                @pl.when((n >= 2) & (n <= NCH))
                def _():
                    wait_chunk(n - 1)
            cr = jnp.clip(n - 1, 0, NCH - 1)
            dst, slot = (wb_sc, cr) if ps_ == 0 else (wa_sc, cr - (NRB - 2))
            src, si = w_slot(ps_)
            bl = jnp.minimum(b + 1, NRB - 1)
            PW = PRO_PW
            npc = RB * S2 // PW
            assert npc * PW == RB * S2 and PRO_R0 + (NBLK - 1) * PRO_RS < HG * npc
            assert PRO_X0 + (max(RB, 2 * NT) - 1) * PRO_XS < HG * npc and 2 * NRB > UL

            def body(i, c):
                s0 = b * RB + 1
                for sg in range(RB):
                    hp_sc[sg * S2:(sg + 1) * S2, :] = xn_sc[s0 + sg, :, 0:DE]
                for j in range(HG):
                    w = _unpack(rows(w_op(src, si, j // 2, 1 + j % 2), w_op(src, si, j // 2, 3 + j % 2),
                                     w_op(src, si, j // 2, 7, j % 2)))
                    for pi in range(npc):
                        pos = j * npc + pi
                        hx = hp_sc[pi * PW:(pi + 1) * PW, :]
                        k, rem = divmod(pos - PRO_X0, PRO_XS)
                        if ps_ == 0 and rem == 0 and 0 <= k < RB:
                            sn = bl * RB + 1 + k
                            xv = _ext(_ln(x_sc[seg(sn), LN].astype(F32)))
                            xn_sc[sn, :, 0:DE] = xv
                            hx = jnp.concatenate([hx[:-S2], jnp.where(never_sm[0] > 0, xv, hx[-S2:])], axis=0)
                        if ps_ == 1 and rem == 0 and 0 <= k < 2 * NT:
                            conv_u(jnp.minimum(2 * b + k // NT, UL),
                                   slice((k % NT) * 128, (k % NT + 1) * 128))
                        bb, rem = divmod(pos - PRO_R0, PRO_RS)
                        if rem == 0 and 0 <= bb < NBLK:
                            relayout(cr, dst, slot, bb, bb >= NKB)
                        r = _dot(plain_lhs(hx, j % 2), w)
                        for a in range(0, 2 * PW, 16):
                            sg, off = divmod(2 * pi * PW + a, SEG)
                            pre_sc[s0 + sg, ps_ * HG + j, off:off + 16, :] = r[a:a + 16].astype(BF16)
                return c
            with jax.named_scope("fused"):
                jax.lax.fori_loop(0, never_sm[0] + 1, body, 0)

        for ps_ in range(NPASS):
            if ps_ == 1:
                with jax.named_scope("wait_in0"):
                    for cp in small + in_copies(0):
                        cp.wait()
                sh = sh_ref[...].astype(F32)
                for j in range(KS):
                    co_sc[j] = jnp.broadcast_to(sh[j:j + 1], (8, DM))
                co_sc[KS] = jnp.broadcast_to(sd_ref[...].astype(F32).reshape(1, DM), (8, DM))

            def blk(b, c, ps_=ps_):
                pro_stage(ps_, b)
                return c
            jax.lax.fori_loop(0, NRB, blk, 0)

        def warm_block0(q):
            uf, kf = conv_fwd(0, q)
            put_spec(0, q, 0, uf)
            put_spec(0, q, 2, kf)
            kr_sc[q] = kf
            ur, um, kr, km = uf[:QB], uf[QB:], kf[:QB], kf[QB:]
            wf_sc[0, 0, q] = (ur * kr - um * km).astype(BF16)
            wf_sc[0, 1, q] = (ur * km + um * kr).astype(BF16)

        def wo_combos(d):
            z = jnp.minimum(never_sm[0], 0)
            r = pl.multiple_of(z * 32 + (d // 4) * 2 * DH + (d % 4) * 32, 32)
            we = wo_sc[pl.ds(r, 32), :]
            wd = wo_sc[pl.ds(r + DH, 32), :]
            f11, f12, f21, f22 = [w[:, c].astype(F32) for w in (we, wd) for c in (EA, EB)]
            ops = [_pack(v) for v in (f11 + f22, we[:, EA], f12 - f22, f21 - f11, wd[:, EB],
                                      f11 + f12, f21 + f22, cols(we[:, EC], wd[:, EC]))]
            for i, v in enumerate(ops):
                wc_sc[i, pl.ds(pl.multiple_of((z + d) * 16, 16), 16), :] = v

        def plain_qkv(eq, ekv, jp, after=None):
            res = []
            for odd in range(2):
                kv = plain_proj(ekv, jp, (1, 2), odd)
                if after is not None:
                    after(4 * jp + 2 * odd, kv)
                q = plain_proj(eq, jp, (0,), odd)
                if after is not None:
                    after(4 * jp + 2 * odd + 1, q)
                res.append(bf(q, kv[:, :DH], kv[:, DH:]))
            return res

        with jax.named_scope("warm"):
            for q in range(NQ):
                warm_block0(q)
        with jax.named_scope("wait_wo"):
            wo_copy.wait()
        with jax.named_scope("step0"):
            mem0 = mem0_ref[...].astype(F32)
            e0 = rows(_ext(rows(mem0, mem0)), xn(0))

            def after0(d, r):
                z = jnp.minimum(never_sm[0], 0)
                wc_sc[z, pl.ds(pl.multiple_of(z * 8 + H * DH // 4, 8), 8), 0:DH] = pltpu.bitcast(r[0:8, 0:DH], U32)
                wo_combos(d)

            def hook0(it):
                if 1 <= it <= 2 * NT:
                    conv_inv(*divmod(it - 1, NT))
            out = attend(lambda jp: plain_qkv(e0, e0, jp, after0), RH, make_mask(RH, (0,)), DIST_HALF,
                         PLAN_HALF, hook0, True)
            y0 = y_seg(0)
            for q in range(2):
                conv_spec(1, q)
            for n in range(NT):
                conv_inv(2, n)
            finish(0, x_sc[0:SEG, LN], y0, rows(out[0:M], mem0), out[M2:])
            for q in range(2):
                for piece in MAC_PIECES:
                    conv_mac(1, q, piece, 2)

        mask12 = make_mask(R, (0, 1))

        def step(t, x2, last):
            first = x2 is None
            c, q = (t + 1) // NQ + 1, (t + 1) % NQ
            em = h_sc[0:M, :]
            e1 = xn(t)
            l2, l4 = rows(em[:, EA], e1[:, EA]), rows(em[:, ES], e1[:, ES])
            ahead = {jp: {i: _dot(_unpack(a), _unpack(w_mats(jp, (1, 2), i))) for i, a in ((2, l2), (4, l4))}
                     for jp in range(AHEAD[first])}
            if first:
                x2 = x2_sc[(t - 1) & 3]
                conv_spec(c, q)
            if MAC_TOP:
                for piece in MAC_PIECES:
                    conv_mac(c, q, piece, NB)
            ex2, xc0 = prepare(t, x2)
            x4 = side2(t, op_sc[...])
            un = conv_u(t + UL)
            e2 = rows(em, ex2)
            xc = pinned(xc0, pin_tiles(PIN_U, 2, un) + pin_tiles(PIN_X4, NT, x4))

            def proj(jp):
                x = xc(jp)
                lhs = [x[:, 0:KH], e2[:, ES], l2, e2[:, EB], l4, x[:, KH:2 * KH], x[:, 2 * KH:]]
                pre = 2 * jp < NPA
                mats = (1, 2) if pre else (1, 2, 0)
                w = len(mats) * DH
                if pre:
                    qs = [plain_proj(e2, jp, (0,), odd) for odd in range(2)]
                cs = strassen([_unpack(a) for a in lhs], [_unpack(w_mats(jp, mats, i)) for i in range(7)],
                              ahead.get(jp, {}))
                tl = _dot(_unpack(rows(em[:, EC], e1[:, EC], e2[M:, EC])),
                          _unpack(cols(w_mats(jp, mats, 7, 0), w_mats(jp, mats, 7, 1))))
                res = []
                for odd in range(2):
                    r = cs[odd] + tl[:, odd * w:(odd + 1) * w]
                    if pre:
                        q1 = pre_sc[t, 2 * jp + odd].astype(F32)
                        qq = rows(qs[odd][:M2], q1, qs[odd][M2:])
                    else:
                        qq = r[:, 2 * DH:]
                    res.append(bf(qq, r[:, :DH], r[:, DH:2 * DH]))
                return res

            held = {}

            def hook(it):
                if it == SPEC_AT and not MAC_TOP:
                    for piece in MAC_PIECES:
                        conv_mac(c, q, piece, NB)
                if INV_AT <= it < INV_AT + NT:
                    conv_inv(t + 2, it - INV_AT)
                if it == HP:
                    held["x"] = x_sc[seg(t), LN]
                    held["y"] = y_seg(t)
            out = attend(proj, R, mask12, DIST, PLAN, hook)
            if not last:
                conv_spec((t + 2) // NQ + 1, (t + 2) % NQ)
            op_sc[...] = out[RH:]
            return finish(t, held["x"], held["y"], out[0:M2], out[M2:RH])

        def steps(i, carry):
            x2 = None
            for j in range(UNROLL):
                x2 = step(1 + i * UNROLL + j, x2, j == UNROLL - 1)
            return carry

        def phase(p, carry):
            @pl.when(p == 1)
            def _():
                for cp in in_copies(2):
                    cp.wait()

            @pl.when(p >= 2)
            def _():
                out_copy((p - 2) * PH, PH).start()

            with jax.named_scope("steps"):
                jax.lax.fori_loop(p * PHI, (p + 1) * PHI, steps, 0)
            return carry

        for cp in in_copies(1):
            cp.wait()
        jax.lax.fori_loop(0, NPH, phase, 0)
        out_copy((NPH - 2) * PH, NSEG - 2 - (NPH - 2) * PH).start()

        with jax.named_scope("step_last"):
            x4 = side2(NSEG, op_sc[...])
            em = h_sc[0:M, :]
            ex = pinned(_ext(_ln(x2_sc[(NSEG - 1) & 3])), pin_tiles(PIN_X4, NT, x4))
            out = attend(lambda jp: plain_qkv(ex(jp), rows(em, ex(jp)), jp),
                         SEG, make_mask(RH, (1,), M2), DIST_HALF, PLAN_HALF)
            side2(NSEG + 1, out)
        out_copy(NSEG - 2, 2).start()
        out_copy(0, NSEG).wait()
        return carry

    jax.lax.fori_loop(0, never_sm[0] + 1, main, 0)


def pallas_interleave_layers__memory_aug_recurrent_mem_tr__ssm_conv_h3__prompt_kernel(
    A_x, A_mem0, A_Wq, A_Wk, A_Wv, A_Wo, A_seg_len,
    B_q, B_k, B_v, B_shift_k, B_ssm_k, B_ssm_D,
):
    del B_q
    seg = int(A_seg_len) if isinstance(A_seg_len, (int, np.integer)) else CB // NQ
    return _run(A_x, A_mem0, A_Wq, A_Wk, A_Wv, A_Wo, B_k, B_v, B_shift_k, B_ssm_k, B_ssm_D, SEG=seg)


@functools.partial(jax.jit, static_argnames=("SEG",))
def _run(A_x, A_mem0, A_Wq, A_Wk, A_Wv, A_Wo, B_k, B_v, B_shift_k, B_ssm_k, B_ssm_D, *, SEG):
    B, S, DM = A_x.shape
    assert B == 1
    H, DH = A_Wq.shape[1], A_Wq.shape[2]
    M = A_mem0.shape[1]
    KS = B_shift_k.shape[1]
    R = 2 * (M + SEG)
    NSEG = S // SEG
    NRB = (NSEG - 1) // RB
    NB = S // CB
    QB = CB // NQ
    NCH = 3 * H // HG
    DP = -(-DM // 256) * 256
    fwd, inv = _dft_constants()

    kern = functools.partial(_kernel, S=S, DM=DM, H=H, DH=DH, M=M, SEG=SEG)
    any_spec = pl.BlockSpec(memory_space=pl.ANY)
    out = pl.pallas_call(
        kern,
        out_shape=jax.ShapeDtypeStruct((S, DM), A_x.dtype),
        in_specs=[any_spec] * 13,
        out_specs=any_spec,
        scratch_shapes=[
            pltpu.VMEM((NB + 2, NQ, QB // 8, DM // 128, 4, 8, 128), F32),
            pltpu.VMEM((NQ, 2 * QB, DM), F32),
            pltpu.VMEM((2, 2, NQ, QB, DM), BF16),
            pltpu.VMEM((4, SEG, DM), F32),
            pltpu.VMEM((2 * CB, DP), F32),
            pltpu.VMEM((S, DP), BF16),
            pltpu.VMEM((SEG, DM), F32),
            pltpu.VMEM((NSEG, NPA, SEG, DH), BF16),
            pltpu.VMEM((NSEG, SEG // 2, DP + KH), U32),
            pltpu.VMEM((NCH - NRB + 2, HG // 2, 8, KH // 2, DH), U32),
            pltpu.VMEM((NRB - 1, HG // 2, 8, KH // 2, DH), U32),
            pltpu.VMEM((H * DH, DM), BF16),
            pltpu.VMEM((8, H * DH // 4 + 16, KH), U32),
            pltpu.VMEM((R // 2, H * DH // 2), U32),
            pltpu.VMEM((R // 2, H * DH // 2), U32),
            pltpu.VMEM((R // 2, H * DH // 2), U32),
            pltpu.VMEM((3, SEG // 2, H * DH // 2), U32),
            pltpu.VMEM((S, DP), BF16),
            pltpu.VMEM((S, DP), BF16),
            pltpu.VMEM((NB, DM, CB), BF16),
            pltpu.VMEM((NCH, DM // 16, 8, 2 * HG, DH), BF16),
            pltpu.VMEM((S, DP), A_x.dtype),
            pltpu.VMEM(fwd.shape, BF16),
            pltpu.VMEM(inv.shape, BF16),
            pltpu.VMEM((S + KPAD, DP), BF16),
            pltpu.VMEM((RB * SEG // 2, DM + KH), U32),
            pltpu.VMEM((M, DM + KH), U32),
            pltpu.VMEM((KS + 1, 8, DM), F32),
            pltpu.VMEM((M, DM), BF16),
            pltpu.VMEM((KS, DM), BF16),
            pltpu.VMEM((DM,), BF16),
            pltpu.SMEM((1,), jnp.int32),
            pltpu.SemaphoreType.DMA(((NSEG - 1) // RB,)),
            pltpu.SemaphoreType.DMA((3,)),
            pltpu.SemaphoreType.DMA((NCH + 2,)),
            pltpu.SemaphoreType.DMA(()),
        ],
        compiler_params=pltpu.CompilerParams(vmem_limit_bytes=120 * 1024 * 1024),
    )(
        A_x.reshape(S, DM), A_mem0.reshape(M, DM),
        *[w.reshape(DM // 16, 2, 8, H, DH) for w in (A_Wq, A_Wk, A_Wv)],
        A_Wo.reshape(H * DH, DM), B_k.reshape(S, DM), B_v.reshape(S, DM),
        B_shift_k.T, B_ssm_k, B_ssm_D,
        jnp.asarray(fwd, BF16), jnp.asarray(inv, BF16),
    )
    return out.reshape(B, S, DM)
```

```python
import functools
import itertools

import numpy as np
import jax
import jax.numpy as jnp
import jax.experimental.pallas as pl
import jax.experimental.pallas.tpu as pltpu

F32 = jnp.float32
BF16 = jnp.bfloat16
U32 = jnp.uint32

CB = 128
NQ = 4
KPAD = 16
HG = 8
NPA = 16
KH = 256
RB = 9
PRO_PW, PRO_X0, PRO_XS, PRO_R0, PRO_R1, PRO_PARTS = 24, 11, 4, 2, 37, 2
UNROLL = 3
PHI = 3
INV_AT, PIN_U, PIN_X4 = 10, 3, 8
DIST, DIST_HALF = (1, 1), (1, 2)
AHEAD = (1, 2)
ORDER = (0, 1, 5, 2, 6, 3, 4)
PLAN = ((1, 2), (3, 4), (7,))
PLAN_HALF = ((1,), (2,), (3,), (4,))


def _dft_constants():
    qb = CB // NQ
    hb = qb // 2
    n = np.arange(CB, dtype=np.float64)
    f = np.concatenate([q * qb + np.concatenate([np.arange(0, qb, 2), np.arange(1, qb, 2)])
                        for q in range(NQ)])
    w = np.pi * (2.0 * f + 1.0) / (2 * CB)
    ang = (w[:, None] * (n[None, :] - (CB - 1) / 4.0)).reshape(NQ, qb, CB)
    fwd = np.concatenate([np.cos(ang), -np.sin(ang)], axis=1)
    inv = np.zeros((NQ, 2, hb, CB))
    for p in range(NQ):
        m = (NQ - 1 - p) * hb + np.arange(hb)
        ang = (m[:, None] + 0.5) * w[None, :]
        inv[p, 0] = np.cos(ang) / CB
        inv[p, 1] = -np.sin(ang) / CB
    return fwd.astype(np.float32), inv.astype(np.float32)


def _flip_rows(x):
    i = jax.lax.broadcasted_iota(jnp.int32, (8, x.shape[1]), 0)
    out = []
    for r in range(x.shape[0] - 8, -8, -8):
        v = pltpu.roll(x[r:r + 8], 4, 0)
        for b in (2, 1):
            v = jnp.where((i & b) == 0, pltpu.roll(v, 8 - b, 0), pltpu.roll(v, b, 0))
        out.append(v)
    return jnp.concatenate(out, axis=0)


def _ln(x, eps=1e-5):
    d = x.shape[-1]
    m = jnp.sum(x, axis=-1, keepdims=True) * (1.0 / d)
    xc = x - m
    v = jnp.sum(xc * xc, axis=-1, keepdims=True) * (1.0 / d)
    return xc * jax.lax.rsqrt(v + eps)


def _dot(a, b):
    return jnp.dot(a, b, preferred_element_type=F32)


def _dot_nt(a, b):
    return jax.lax.dot_general(a, b, (((1,), (1,)), ((), ())), preferred_element_type=F32)


def _pack(x):
    return pltpu.bitcast(x.astype(BF16), U32)


def _unpack(x):
    return pltpu.bitcast(x, BF16)


def _ext(r):
    return _pack(jnp.concatenate([r, r[:, :KH] + r[:, KH:2 * KH]], axis=1))


def _in_order(actions):
    def body(i, c):
        for j, act in enumerate(actions):
            pl.when(i == j)(act)
        return c
    jax.lax.fori_loop(0, len(actions), body, 0)


def _kernel(x_hbm, mem0_hbm, wq_hbm, wk_hbm, wv_hbm, wo_hbm, k_hbm, v_hbm,
            sh_hbm, sk_hbm, sd_hbm, fwd_hbm, inv_hbm, o_hbm,
            sp_sc, kr_sc, wf_sc, x2_sc, y_sc, u_sc, op_sc, pre_sc, xn_sc, wa_sc, wb_sc, wo_sc, wc_sc,
            oe_sc, oo_sc, os_sc, ox_sc,
            x_sc, v_sc, sk_sc, st_sc, out_sc, fwd_ref, inv_ref,
            k_sc, hp_sc, h_sc, co_sc, mem0_ref, sh_ref, sd_ref,
            never_sm, sem_x, sem_in, sem_w, sem_out,
            *, S, DM, H, DH, M, SEG):
    NSEG = S // SEG
    M2 = 2 * M
    S2 = SEG // 2
    R = M2 + 2 * SEG
    RH = M2 + SEG
    NB = S // CB
    QB = CB // NQ
    HB = QB // 2
    NT = DM // 128
    PH = PHI * UNROLL
    NRB = (NSEG - 1) // RB
    NPH = (NSEG - 1) // PH
    NG = H // HG
    NCH = 3 * NG
    NPASS = NPA // HG
    DH2 = DM // 2
    HP = H // 2
    DE = DM + KH
    KT = DM - 2 * KH
    NKB = KH // 16
    EA, EB, EC, ES = slice(0, KH), slice(KH, 2 * KH), slice(2 * KH, DM), slice(DM, DE)
    KS = sh_ref.shape[0]
    UL = 2 * NQ + 1
    LN = pl.ds(0, DM)
    assert 2 * KT == KH and 2 <= KS <= 8 and QB == SEG and NRB * RB == NSEG - 1 and NPH * PH == NSEG - 1 and NPASS == 2 and 2 * NRB >= NCH + 1

    mem0_copy = pltpu.make_async_copy(mem0_hbm, mem0_ref, sem_x.at[0])
    small = [pltpu.make_async_copy(s, d, sem_in.at[0]) for s, d in [
        (sh_hbm, sh_ref), (sd_hbm, sd_ref), (fwd_hbm, fwd_ref), (inv_hbm, inv_ref)]]

    def x_copy(b):
        if isinstance(b, int) and b == 0:
            rows = pl.ds(0, (RB + 1) * SEG)
        else:
            rows = pl.ds(pl.multiple_of((b * RB + 1) * SEG, SEG), RB * SEG)
        return pltpu.make_async_copy(x_hbm.at[rows], x_sc.at[rows, LN], sem_x.at[b])

    kb = (0, (UL + 1) * SEG, (UL + PH + 1) * SEG, S)
    sb = (0, 2, (PH + 2) // NQ + 2, NB)

    def in_copies(part):
        def rng(b):
            return pl.ds(b[part], b[part + 1] - b[part])
        sem = sem_in.at[part]
        return [
            pltpu.make_async_copy(k_hbm.at[rng(kb)],
                                  k_sc.at[pl.ds(KPAD + kb[part], kb[part + 1] - kb[part]), LN], sem),
            pltpu.make_async_copy(v_hbm.at[rng(kb)], v_sc.at[rng(kb), LN], sem),
        ] + [pltpu.make_async_copy(sk_hbm.at[:, pl.ds(c * CB, CB)], sk_sc.at[c], sem)
             for c in range(sb[part], sb[part + 1])]

    def w_copies(ci, dst=None, part=None):
        src = (wq_hbm, wk_hbm, wv_hbm)[ci // NG]
        dst = ci if dst is None else dst
        h = NKB // 2
        spans = {None: [(0, DM // 16)], 0: [(0, h), (NKB, NKB + h)],
                 1: [(h, NKB), (NKB + h, DM // 16)]}[part]
        sem = sem_w.at[NCH + 1 if part == 1 else dst]
        return [pltpu.make_async_copy(
            src.at[pl.ds(lo, hi - lo), hf, :, pl.ds((ci % NG) * HG, HG), :],
            st_sc.at[dst, pl.ds(lo, hi - lo), :, pl.ds(hf * HG, HG), :], sem)
            for lo, hi in spans for hf in range(2)]

    wo_copy = pltpu.make_async_copy(wo_hbm, wo_sc, sem_w.at[NCH])

    def out_copy(lo, n):
        rows = pl.ds(lo * SEG if isinstance(lo, int) else pl.multiple_of(lo * SEG, SEG), n * SEG)
        return pltpu.make_async_copy(out_sc.at[rows, LN], o_hbm.at[rows], sem_out)

    def start_all(cps):
        def act():
            for cp in cps:
                cp.start()
        return act

    order = [[mem0_copy, x_copy(0)], w_copies(0, part=0), w_copies(0, part=1), [x_copy(1)], [x_copy(2)]]
    for ci in range(1, NCH):
        order.append(w_copies(ci) + ([x_copy(ci + 2)] if ci + 2 < NRB else []))
        if ci == NRB - 2:
            order.append(small + in_copies(0))
    order += [[wo_copy], in_copies(1), in_copies(2)]
    for i in range(0, len(order), 5):
        _in_order([start_all(cps) for cps in order[i:i + 5]])

    never_sm[0] = 0
    k_sc[0:KPAD, LN] = jnp.zeros((KPAD, DM), BF16)
    sp_sc[NB + 1] = jnp.zeros(sp_sc.shape[1:], F32)
    op_sc[...] = jnp.zeros(op_sc.shape, F32)
    x2_sc[...] = jnp.zeros(x2_sc.shape, F32)
    y_sc[2 * CB - SEG:, LN] = jnp.zeros((SEG, DM), F32)
    mem0_copy.wait()
    x_copy(0).wait()
    for sg in range(RB + 1):
        xn_sc[sg, :, 0:DE] = _ext(_ln(x_sc[sg * SEG:(sg + 1) * SEG, LN].astype(F32)))

    def clip(i, hi):
        return min(max(i, 0), hi) if isinstance(i, int) else jnp.clip(i, 0, hi)

    def scaled(i, m):
        return i * m if isinstance(i, int) else pl.multiple_of(i * m, m)

    def seg(i):
        return pl.ds(scaled(clip(i, NSEG - 1), SEG), SEG)

    def conv_u(s, ln=LN):
        r0 = scaled(clip(s, NSEG - 1), SEG)
        kk = k_sc[pl.ds(r0, KPAD + SEG), ln].astype(F32)[KPAD - 8:]

        def coef(j, rows):
            return jnp.concatenate([co_sc[j, :, ln]] * (rows // 8), axis=0)
        sft = [kk] + [pltpu.roll(kk, j, 0) for j in range(2, KS, 2)]
        ev = functools.reduce(jnp.add, [sft[j // 2][8:] * coef(j, SEG) for j in range(0, KS, 2)])
        od = functools.reduce(jnp.add, [sft[j // 2] * coef(j, SEG + 8) for j in range(1, KS, 2)])
        ks = ev + pltpu.roll(od, 1, 0)[8:]
        u = (ks * v_sc[pl.ds(r0, SEG), ln].astype(F32)).astype(BF16)
        u_sc[pl.ds(r0, SEG), ln] = u
        return u

    def conv_fwd(c, q):
        cc = clip(c, NB - 1)
        f = fwd_ref[q]
        uf = _dot(f, u_sc[pl.ds(scaled(cc, CB), CB), LN])
        kf = _dot_nt(f, sk_sc[cc])
        return uf, kf

    def put_spec(cs, q, which, val):
        for n in range(NT):
            v = val[:, n * 128:(n + 1) * 128].reshape(2, QB // 8, 8, 128)
            sp_sc[cs, q, :, n, which:which + 2] = jnp.stack([v[0], v[1]], axis=1)

    def conv_spec(c, q):
        uf, kf = conv_fwd(c, q)
        cs = clip(c, NB)
        put_spec(cs, q, 0, uf)
        pk = kr_sc[q]
        kr_sc[q] = kf
        kp = jnp.concatenate([
            kf[0:HB] - pk[QB:QB + HB],
            kf[HB:QB] + pk[QB + HB:],
            kf[QB:QB + HB] + pk[0:HB],
            kf[QB + HB:] - pk[HB:QB]], axis=0)
        put_spec(cs, q, 2, kp)

    MAC_PIECES = [(rb, n) for rb in range(QB // 16) for n in range(NT)]

    def conv_mac(c, q, piece, nterms):
        rb2, n = piece
        cs = clip(c, NB)
        rbs = slice(2 * rb2, 2 * rb2 + 2)
        ar = None
        ai = None
        for j in range(nterms):
            if isinstance(cs, int):
                uj, kj = j, cs - j
            else:
                uj = jnp.minimum(j, cs)
                kj = jnp.where(cs - j >= 0, cs - j, NB + 1)
            u = sp_sc[uj, q, rbs, n, 0:2]
            k = sp_sc[kj, q, rbs, n, 2:4]
            tr = u[:, 0] * k[:, 0] - u[:, 1] * k[:, 1]
            ti = u[:, 0] * k[:, 1] + u[:, 1] * k[:, 0]
            ar = tr if ar is None else ar + tr
            ai = ti if ai is None else ai + ti
        ln = slice(n * 128, (n + 1) * 128)
        w = jnp.concatenate([ar.reshape(16, 128), ai.reshape(16, 128)], axis=0).astype(BF16)
        wf_sc[c & 1, 0, q, rb2 * 16:rb2 * 16 + 16, ln] = w[0:16]
        wf_sc[c & 1, 1, q, rb2 * 16:rb2 * 16 + 16, ln] = w[16:]

    def conv_inv(tt, n):
        cb = tt // NQ
        p = tt % NQ
        ln = slice(n * 128, (n + 1) * 128)
        ev = _dot(inv_ref[p, 0], wf_sc[cb & 1, 0, :, :, ln].reshape(CB, 128))
        od = _dot(inv_ref[p, 1], wf_sc[cb & 1, 1, :, :, ln].reshape(CB, 128))
        sd = jnp.concatenate([co_sc[KS, :, ln]] * (HB // 8), axis=0)
        for r, val in ((p, _flip_rows(ev - od)), (2 * NQ - 1 - p, ev + od)):
            ur = scaled(clip(cb, NB - 1) * (2 * NQ) + r, HB)
            yr = scaled((cb & 1) * (2 * NQ) + r, HB)
            y_sc[pl.ds(yr, HB), ln] = val + u_sc[pl.ds(ur, HB), ln].astype(F32) * sd

    def y_seg(s):
        return y_sc[pl.ds(scaled(s & (2 * NQ - 1), SEG), SEG), LN]

    scale = DH ** -0.5
    cexp = scale * float(np.log2(np.e))

    def make_mask(n, x_layers, q0=0):
        qi = jax.lax.broadcasted_iota(jnp.int32, (n - q0, n), 0) + q0
        ki = jax.lax.broadcasted_iota(jnp.int32, (n - q0, n), 1)

        def layer(i):
            xl = jnp.where(i < M2 + SEG, x_layers[0], x_layers[-1])
            return jnp.where(i < M, 0, jnp.where(i < M2, 1, xl))
        same = layer(qi) == layer(ki)
        ok = same & ((qi < M2) | (ki < M2) | (qi >= ki))
        fill = jnp.where(same, -1e9 / scale, -jnp.inf).astype(F32)
        return ok, fill

    def probs(q, k, mask):
        ok, fill = mask
        s = _dot_nt(q, k)
        s = jnp.where(ok, s, fill)
        m = jnp.max(s, axis=-1, keepdims=True)
        p = jnp.exp2((s - m) * cexp)
        l = jnp.sum(p, axis=-1, keepdims=True)
        r = pl.reciprocal(l, approx=True)
        r = r * (2.0 - l * r)
        return (p * r).astype(BF16)

    def w_slot(ci):
        return (wb_sc, ci) if 1 <= ci < NRB - 1 else (wa_sc, max(ci - (NRB - 2), 0))

    def rows(*parts):
        return jnp.concatenate(parts, axis=0)

    def cols(*parts):
        return jnp.concatenate(parts, axis=1)

    def w_op(ref, slot, j, i, odd=None):
        return ref[slot, j, i] if odd is None else ref[slot, j, 7, odd * KT // 2:(odd + 1) * KT // 2]

    def w_mats(jp, mats, i, odd=None):
        return cols(*[w_op(*w_slot(mi * NG + 2 * jp // HG), jp % (HG // 2), i, odd) for mi in mats])

    def plain_lhs(e, odd):
        return _unpack(cols(e[:, EA], e[:, ES], e[:, EC]) if odd else cols(e[:, ES], e[:, EB], e[:, EC]))

    def plain_proj(e, jp, mats, odd):
        w = rows(w_mats(jp, mats, 1 + odd), w_mats(jp, mats, 3 + odd), w_mats(jp, mats, 7, odd))
        return _dot(plain_lhs(e, odd), _unpack(w))

    def strassen(lhs, rhs, m):
        m = dict(m)
        m.update({i: _dot(lhs[i], rhs[i]) for i in ORDER if i not in m})
        return strassen_out(m, lambda: m[5])

    def strassen_out(m, last):
        c21 = m[1] + m[3]
        c12 = m[2] + m[4]
        c11 = m[0] + m[3][M2:] - m[4][M2:] + m[6]
        c22 = m[0] - m[1][M2:] + m[2][M2:] + last()
        return rows(c21[:M2], c11, c21[M2:]), rows(c12, c22)

    def bf(*xs):
        return tuple(x.astype(BF16) for x in xs)

    def xn(s):
        return xn_sc[clip(s, NSEG - 1), :, 0:DE]

    def attend(proj, n, mask, dist, plan, hook=None, raw=False):
        D1, D2 = dist
        PA = HP - D1 - D2 - 1
        full = n == R
        n2 = n // 2

        def prod(i, p0, p1):
            cs = slice(p0 * DH, p1 * DH)
            ws = slice(p0 * DH // 2, p1 * DH // 2)
            if raw:
                a = cols(*[ref[0:n2, p * DH:(p + 1) * DH] for p in range(p0, p1) for ref in (oe_sc, oo_sc)])
                return _dot(_unpack(a), wo_sc[2 * p0 * DH:2 * p1 * DH, i * 128:(i + 1) * 128])
            if i >= 7:
                rs = slice(RH // 2, n2) if i == 8 else slice(0, min(n2, RH // 2))
                return _dot(_unpack(cols(oe_sc[rs, cs], oo_sc[rs, cs])),
                            _unpack(rows(wc_sc[7, ws, 0:KT], wc_sc[7, ws, KT:2 * KT])))
            if i in (0, 5, 6):
                a = ox_sc[max(i - 4, 0), :, cs]
            else:
                ref = {1: os_sc, 2: oe_sc, 3: oo_sc, 4: os_sc}[i]
                if not full:
                    a = ref[0:n2, cs]
                elif i in (2, 4):
                    a = ref[0:RH // 2, cs]
                else:
                    a = rows(ref[0:M, cs], ref[RH // 2:, cs])
            return _dot(_unpack(a), _unpack(wc_sc[i, ws, :]))

        qkvs = {}
        ps = {}
        m = {}
        for it in range(HP + D1 + D2):
            if it < HP:
                qkvs[it] = proj(it)
            g = it - D1
            if 0 <= g < HP:
                ps[g] = [probs(q, k, mask) for q, k, _ in qkvs[g]]
            g = it - D1 - D2
            if 0 <= g < HP:
                oe, oo = [_dot(p, qkv[2]) for p, qkv in zip(ps.pop(g), qkvs.pop(g))]
                cs = slice(g * DH, (g + 1) * DH)
                oe_sc[0:n2, cs] = _pack(oe)
                oo_sc[0:n2, cs] = _pack(oo)
                if not raw:
                    os_sc[0:n2, cs] = _pack(oe + oo)
                if full:
                    ox_sc[0, :, cs] = _pack(oe[M2:RH] + oo[RH:])
                    ox_sc[1, :, cs] = _pack(oe[RH:] - oe[M2:RH])
                    ox_sc[2, :, cs] = _pack(oo[M2:RH] - oo[RH:])
            if hook is not None:
                hook(it)
            j = it - (HP - 1)
            if j >= 0:
                for i in plan[j]:
                    m[i] = prod(i, 0, PA)
        early = list(m)
        for i in (range(NT) if raw else (0, 1, 2, 3, 4, 6, 7) if full else (1, 2, 3, 4, 7)):
            if i not in early:
                m[i] = prod(i, 0, HP)
        for i in early:
            m[i] = prod(i, PA, HP) + m[i]
        if raw:
            return cols(*[m[i] for i in range(NT)])
        if not full:
            return cols(m[1] + m[3], m[2] + m[4], m[7])
        c1, c2 = strassen_out(m, lambda: prod(5, 0, HP))
        return cols(c1, c2, rows(m[7], prod(8, 0, HP)))

    def side2(t, a2):
        x3 = x2_sc[(t - 2) & 3] + a2
        x4 = x3 + _ln(x3) * y_seg(t - 2)
        x4 = x4.astype(out_sc.dtype)
        out_sc[seg(t - 2), LN] = x4
        return x4

    def finish(t, xr, yt, mem, a1):
        x1 = xr.astype(F32) + a1
        x2 = x1 + _ln(x1) * yt
        h_sc[0:M, :] = _ext(mem)
        x2_sc[t & 3] = x2
        return x2

    def prepare(t, x2):
        n1 = _unpack(xn(t)[:, 0:2 * KH]).astype(F32)
        n2 = _ln(x2)
        return _ext(n2), _pack(cols(n1[:, EA] + n2[:, EB], n2[:, EA] - n1[:, EA], n1[:, EB] - n2[:, EB]))

    def pinned(r, pins):
        never = never_sm[0] > 0
        hs = {0: r}
        tiles = [r[:, n:n + 128] for n in range(0, r.shape[1], 128)]
        for g, n, d in sorted(pins, key=lambda p: p[0]):
            tiles[n] = jnp.where(never, d, tiles[n])
            hs[g] = cols(*tiles)
        return lambda g: hs[max(k for k in hs if k <= g)]

    def pin_tiles(g0, per, val):
        v = _pack(val)
        return [(g0 + n // per, n, v[:, n * 128:(n + 1) * 128]) for n in range(NT)]

    def wait_chunk(ci):
        for cp in w_copies(0, ci):
            cp.wait()

    def w_block(ci, b):
        x = pltpu.bitcast(st_sc[ci, b], U32)
        sub = jax.lax.broadcasted_iota(jnp.int32, (8, DH), 0)
        res = []
        for par in range(2):
            v = [x[2 * i + par] for i in range(4)]
            for bit in (2, 1):
                keep = (sub & bit) == 0
                for i in range(4):
                    if not i & bit:
                        a, c = v[i], v[i + bit]
                        v[i] = jnp.where(keep, a, pltpu.roll(c, bit, 0))
                        v[i + bit] = jnp.where(keep, pltpu.roll(a, 8 - bit, 0), c)
            res.append(jnp.stack(v))
        return res

    def relayout(ci, dst, slot, b, tail, parts=1):
        hi_m = U32(0xFFFF0000)

        def even(t):
            return (t[0] & U32(0xFFFF)) | (t[1] << 16)

        def odd(t):
            return (t[0] >> 16) | (t[1] & hi_m)

        if tail:
            for k in range(2):
                tb = 2 * (b - NKB) + k
                t = w_block(ci, 2 * NKB + tb)
                dst[slot, :, 7, pl.ds(tb * 8, 8), :] = even(t)
                dst[slot, :, 7, pl.ds(KT // 2 + tb * 8, 8), :] = odd(t)
            yield
            return
        t1 = w_block(ci, b)
        t2 = w_block(ci, b + NKB)

        def plane(t, f):
            return pltpu.bitcast(jnp.concatenate([f(t[0]), f(t[1])], axis=2), F32)

        def pack(v):
            r = pltpu.bitcast(v.astype(BF16).astype(F32), U32)
            return (r[:, :, :DH] >> 16) | r[:, :, DH:]
        f11, f21 = [plane(t, lambda w: w << 16) for t in (t1, t2)]
        f12, f22 = [plane(t, lambda w: w & hi_m) for t in (t1, t2)]
        ops = [pack(f11 + f22), even(t1), pack(f12 - f22), pack(f21 - f11), odd(t2),
               pack(f11 + f12), pack(f21 + f22)]
        n = HG // 2 // parts
        for p in range(0, HG // 2, n):
            for i, v in enumerate(ops):
                dst[slot, p:p + n, i, pl.ds(scaled(b, 8), 8), :] = v[p:p + n]
            yield

    NBLK = DH2 // 16

    def main(_, carry):
        def relayout0(b, c):
            list(relayout(0, wa_sc, 0, b, False))
            return c
        for part in range(2):
            with jax.named_scope("wait_w"):
                for cp in w_copies(0, part=part):
                    cp.wait()
            with jax.named_scope("relayout"):
                jax.lax.fori_loop(part * NKB // 2, (part + 1) * NKB // 2, relayout0, 0)
        for b in range(NKB, NBLK):
            list(relayout(0, wa_sc, 0, b, True))

        def pro_stage(ps_, b):
            n = ps_ * NRB + b
            with jax.named_scope("wait_w"):
                if ps_ == 0:
                    @pl.when(b + 1 < NRB)
                    def _():
                        x_copy(b + 1).wait()

                @pl.when((n >= 2) & (n <= NCH))
                def _():
                    wait_chunk(n - 1)
            cr = jnp.clip(n - 1, 0, NCH - 1)
            dst, slot = (wb_sc, cr) if ps_ == 0 else (wa_sc, cr - (NRB - 2))
            src, si = w_slot(ps_)
            bl = jnp.minimum(b + 1, NRB - 1)
            PW = PRO_PW
            npc = RB * S2 // PW
            nit = NKB * PRO_PARTS + NBLK - NKB
            assert npc * PW == RB * S2
            assert PRO_X0 + (max(RB, 2 * NT) - 1) * PRO_XS < HG * npc and 2 * NRB > UL

            def body(i, c):
                s0 = b * RB + 1
                work = itertools.chain(*[relayout(cr, dst, slot, k, k >= NKB, PRO_PARTS) for k in range(NBLK)])
                done = 0
                for sg in range(RB):
                    hp_sc[sg * S2:(sg + 1) * S2, :] = xn_sc[s0 + sg, :, 0:DE]
                for j in range(HG):
                    w = _unpack(rows(w_op(src, si, j // 2, 1 + j % 2), w_op(src, si, j // 2, 3 + j % 2),
                                     w_op(src, si, j // 2, 7, j % 2)))
                    for pi in range(npc):
                        pos = j * npc + pi
                        hx = hp_sc[pi * PW:(pi + 1) * PW, :]
                        k, rem = divmod(pos - PRO_X0, PRO_XS)
                        if ps_ == 0 and rem == 0 and 0 <= k < RB:
                            sn = bl * RB + 1 + k
                            xv = _ext(_ln(x_sc[seg(sn), LN].astype(F32)))
                            xn_sc[sn, :, 0:DE] = xv
                            hx = jnp.concatenate([hx[:-S2], jnp.where(never_sm[0] > 0, xv, hx[-S2:])], axis=0)
                        if ps_ == 1 and rem == 0 and 0 <= k < 2 * NT:
                            conv_u(jnp.minimum(2 * b + k // NT, UL),
                                   slice((k % NT) * 128, (k % NT + 1) * 128))
                        upto = min(nit, max(0, -(-(pos - PRO_R0 + 1) * nit // (PRO_R1 - PRO_R0 + 1))))
                        for _ in range(done, upto):
                            next(work)
                        done = upto
                        r = _dot(plain_lhs(hx, j % 2), w)
                        for a in range(0, 2 * PW, 16):
                            sg, off = divmod(2 * pi * PW + a, SEG)
                            pre_sc[s0 + sg, ps_ * HG + j, off:off + 16, :] = r[a:a + 16].astype(BF16)
                assert done == nit
                return c
            with jax.named_scope("fused"):
                jax.lax.fori_loop(0, never_sm[0] + 1, body, 0)

        for ps_ in range(NPASS):
            if ps_ == 1:
                with jax.named_scope("wait_in0"):
                    for cp in small + in_copies(0):
                        cp.wait()
                sh = sh_ref[...].astype(F32)
                for j in range(KS):
                    co_sc[j] = jnp.broadcast_to(sh[j:j + 1], (8, DM))
                co_sc[KS] = jnp.broadcast_to(sd_ref[...].astype(F32).reshape(1, DM), (8, DM))

            def blk(b, c, ps_=ps_):
                pro_stage(ps_, b)
                return c
            jax.lax.fori_loop(0, NRB, blk, 0)

        def warm_block0(q):
            uf, kf = conv_fwd(0, q)
            put_spec(0, q, 0, uf)
            put_spec(0, q, 2, kf)
            kr_sc[q] = kf
            ur, um, kr, km = uf[:QB], uf[QB:], kf[:QB], kf[QB:]
            wf_sc[0, 0, q] = (ur * kr - um * km).astype(BF16)
            wf_sc[0, 1, q] = (ur * km + um * kr).astype(BF16)

        def wo_combos(d):
            z = jnp.minimum(never_sm[0], 0)
            r = (d // 4) * 2 * DH + (d % 4) * 32
            we = wo_sc[r:r + 32, :]
            wd = wo_sc[r + DH:r + DH + 32, :]
            f11, f12, f21, f22 = [w[:, c].astype(F32) for w in (we, wd) for c in (EA, EB)]
            ops = [_pack(v) for v in (f11 + f22, we[:, EA], f12 - f22, f21 - f11, wd[:, EB],
                                      f11 + f12, f21 + f22, cols(we[:, EC], wd[:, EC]))]
            for i, v in enumerate(ops):
                wc_sc[i, pl.ds(pl.multiple_of((z + d) * 16, 16), 16), :] = v

        def plain_qkv(eq, ekv, jp, after=None):
            res = []
            for odd in range(2):
                kv = plain_proj(ekv, jp, (1, 2), odd)
                if after is not None:
                    after(4 * jp + 2 * odd, kv)
                q = plain_proj(eq, jp, (0,), odd)
                if after is not None:
                    after(4 * jp + 2 * odd + 1, q)
                res.append(bf(q, kv[:, :DH], kv[:, DH:]))
            return res

        with jax.named_scope("wait_wo"):
            wo_copy.wait()
        with jax.named_scope("step0"):
            mem0 = mem0_ref[...].astype(F32)
            e0 = rows(_ext(rows(mem0, mem0)), xn(0))

            def after0(d, r):
                z = jnp.minimum(never_sm[0], 0)
                wc_sc[z, pl.ds(pl.multiple_of(z * 8 + H * DH // 4, 8), 8), 0:DH] = pltpu.bitcast(r[0:8, 0:DH], U32)
                wo_combos(d)

            def hook0(it):
                if it < NQ:
                    warm_block0(it)
                if 5 <= it < 5 + 2 * NT:
                    conv_inv(*divmod(it - 5, NT))
            out = attend(lambda jp: plain_qkv(e0, e0, jp, after0), RH, make_mask(RH, (0,)), DIST_HALF,
                         PLAN_HALF, hook0, True)
            y0 = y_seg(0)
            for q in range(2):
                conv_spec(1, q)
            for n in range(NT):
                conv_inv(2, n)
            finish(0, x_sc[0:SEG, LN], y0, rows(out[0:M], mem0), out[M2:])
            for q in range(2):
                for piece in MAC_PIECES:
                    conv_mac(1, q, piece, 2)

        mask12 = make_mask(R, (0, 1))

        def step(t, x2):
            first = x2 is None
            c, q = (t + 1) // NQ + 1, (t + 1) % NQ
            em = h_sc[0:M, :]
            e1 = xn(t)
            l2, l4 = rows(em[:, EA], e1[:, EA]), rows(em[:, ES], e1[:, ES])
            ahead = {jp: {i: _dot(_unpack(a), _unpack(w_mats(jp, (1, 2), i))) for i, a in ((2, l2), (4, l4))}
                     for jp in range(AHEAD[first])}
            if first:
                x2 = x2_sc[(t - 1) & 3]
            conv_spec(c, q)
            for piece in MAC_PIECES:
                conv_mac(c, q, piece, NB)
            ex2, xc0 = prepare(t, x2)
            x4 = side2(t, op_sc[...])
            un = conv_u(t + UL)
            e2 = rows(em, ex2)
            xc = pinned(xc0, pin_tiles(PIN_U, 2, un) + pin_tiles(PIN_X4, NT, x4))

            def proj(jp):
                x = xc(jp)
                lhs = [x[:, 0:KH], e2[:, ES], l2, e2[:, EB], l4, x[:, KH:2 * KH], x[:, 2 * KH:]]
                pre = 2 * jp < NPA
                mats = (1, 2) if pre else (1, 2, 0)
                w = len(mats) * DH
                if pre:
                    qs = [plain_proj(e2, jp, (0,), odd) for odd in range(2)]
                cs = strassen([_unpack(a) for a in lhs], [_unpack(w_mats(jp, mats, i)) for i in range(7)],
                              ahead.get(jp, {}))
                tl = _dot(_unpack(rows(em[:, EC], e1[:, EC], e2[M:, EC])),
                          _unpack(cols(w_mats(jp, mats, 7, 0), w_mats(jp, mats, 7, 1))))
                res = []
                for odd in range(2):
                    r = cs[odd] + tl[:, odd * w:(odd + 1) * w]
                    if pre:
                        q1 = pre_sc[t, 2 * jp + odd].astype(F32)
                        qq = rows(qs[odd][:M2], q1, qs[odd][M2:])
                    else:
                        qq = r[:, 2 * DH:]
                    res.append(bf(qq, r[:, :DH], r[:, DH:2 * DH]))
                return res

            held = {}

            def hook(it):
                if INV_AT <= it < INV_AT + NT:
                    conv_inv(t + 2, it - INV_AT)
                if it == HP:
                    held["x"] = x_sc[seg(t), LN]
                    held["y"] = y_seg(t)
            out = attend(proj, R, mask12, DIST, PLAN, hook)
            op_sc[...] = out[RH:]
            return finish(t, held["x"], held["y"], out[0:M2], out[M2:RH])

        def steps(i, carry):
            x2 = None
            for j in range(UNROLL):
                x2 = step(1 + i * UNROLL + j, x2)
            return carry

        def phase(p, carry):
            @pl.when(p == 1)
            def _():
                for cp in in_copies(2):
                    cp.wait()

            @pl.when(p >= 2)
            def _():
                out_copy((p - 2) * PH, PH).start()

            with jax.named_scope("steps"):
                jax.lax.fori_loop(p * PHI, (p + 1) * PHI, steps, 0)
            return carry

        for cp in in_copies(1):
            cp.wait()
        jax.lax.fori_loop(0, NPH, phase, 0)
        out_copy((NPH - 2) * PH, NSEG - 2 - (NPH - 2) * PH).start()

        with jax.named_scope("step_last"):
            x4 = side2(NSEG, op_sc[...])
            em = h_sc[0:M, :]
            ex = pinned(_ext(_ln(x2_sc[(NSEG - 1) & 3])), pin_tiles(PIN_X4, NT, x4))
            out = attend(lambda jp: plain_qkv(ex(jp), rows(em, ex(jp)), jp),
                         SEG, make_mask(RH, (1,), M2), DIST_HALF, PLAN_HALF)
            side2(NSEG + 1, out)
        out_copy(NSEG - 2, 2).start()
        out_copy(0, NSEG).wait()
        return carry

    jax.lax.fori_loop(0, never_sm[0] + 1, main, 0)


def pallas_interleave_layers__memory_aug_recurrent_mem_tr__ssm_conv_h3__prompt_kernel(
    A_x, A_mem0, A_Wq, A_Wk, A_Wv, A_Wo, A_seg_len,
    B_q, B_k, B_v, B_shift_k, B_ssm_k, B_ssm_D,
):
    del B_q
    seg = int(A_seg_len) if isinstance(A_seg_len, (int, np.integer)) else CB // NQ
    return _run(A_x, A_mem0, A_Wq, A_Wk, A_Wv, A_Wo, B_k, B_v, B_shift_k, B_ssm_k, B_ssm_D, SEG=seg)


@functools.partial(jax.jit, static_argnames=("SEG",))
def _run(A_x, A_mem0, A_Wq, A_Wk, A_Wv, A_Wo, B_k, B_v, B_shift_k, B_ssm_k, B_ssm_D, *, SEG):
    B, S, DM = A_x.shape
    assert B == 1
    H, DH = A_Wq.shape[1], A_Wq.shape[2]
    M = A_mem0.shape[1]
    KS = B_shift_k.shape[1]
    R = 2 * (M + SEG)
    NSEG = S // SEG
    NRB = (NSEG - 1) // RB
    NB = S // CB
    QB = CB // NQ
    NCH = 3 * H // HG
    DP = -(-DM // 256) * 256
    fwd, inv = _dft_constants()

    kern = functools.partial(_kernel, S=S, DM=DM, H=H, DH=DH, M=M, SEG=SEG)
    any_spec = pl.BlockSpec(memory_space=pl.ANY)
    out = pl.pallas_call(
        kern,
        out_shape=jax.ShapeDtypeStruct((S, DM), A_x.dtype),
        in_specs=[any_spec] * 13,
        out_specs=any_spec,
        scratch_shapes=[
            pltpu.VMEM((NB + 2, NQ, QB // 8, DM // 128, 4, 8, 128), F32),
            pltpu.VMEM((NQ, 2 * QB, DM), F32),
            pltpu.VMEM((2, 2, NQ, QB, DM), BF16),
            pltpu.VMEM((4, SEG, DM), F32),
            pltpu.VMEM((2 * CB, DP), F32),
            pltpu.VMEM((S, DP), BF16),
            pltpu.VMEM((SEG, DM), F32),
            pltpu.VMEM((NSEG, NPA, SEG, DH), BF16),
            pltpu.VMEM((NSEG, SEG // 2, DP + KH), U32),
            pltpu.VMEM((NCH - NRB + 2, HG // 2, 8, KH // 2, DH), U32),
            pltpu.VMEM((NRB - 1, HG // 2, 8, KH // 2, DH), U32),
            pltpu.VMEM((H * DH, DM), BF16),
            pltpu.VMEM((8, H * DH // 4 + 16, KH), U32),
            pltpu.VMEM((R // 2, H * DH // 2), U32),
            pltpu.VMEM((R // 2, H * DH // 2), U32),
            pltpu.VMEM((R // 2, H * DH // 2), U32),
            pltpu.VMEM((3, SEG // 2, H * DH // 2), U32),
            pltpu.VMEM((S, DP), BF16),
            pltpu.VMEM((S, DP), BF16),
            pltpu.VMEM((NB, DM, CB), BF16),
            pltpu.VMEM((NCH, DM // 16, 8, 2 * HG, DH), BF16),
            pltpu.VMEM((S, DP), A_x.dtype),
            pltpu.VMEM(fwd.shape, BF16),
            pltpu.VMEM(inv.shape, BF16),
            pltpu.VMEM((S + KPAD, DP), BF16),
            pltpu.VMEM((RB * SEG // 2, DM + KH), U32),
            pltpu.VMEM((M, DM + KH), U32),
            pltpu.VMEM((KS + 1, 8, DM), F32),
            pltpu.VMEM((M, DM), BF16),
            pltpu.VMEM((KS, DM), BF16),
            pltpu.VMEM((DM,), BF16),
            pltpu.SMEM((1,), jnp.int32),
            pltpu.SemaphoreType.DMA(((NSEG - 1) // RB,)),
            pltpu.SemaphoreType.DMA((3,)),
            pltpu.SemaphoreType.DMA((NCH + 2,)),
            pltpu.SemaphoreType.DMA(()),
        ],
        compiler_params=pltpu.CompilerParams(vmem_limit_bytes=120 * 1024 * 1024),
    )(
        A_x.reshape(S, DM), A_mem0.reshape(M, DM),
        *[w.reshape(DM // 16, 2, 8, H, DH) for w in (A_Wq, A_Wk, A_Wv)],
        A_Wo.reshape(H * DH, DM), B_k.reshape(S, DM), B_v.reshape(S, DM),
        B_shift_k.T, B_ssm_k, B_ssm_D,
        jnp.asarray(fwd, BF16), jnp.asarray(inv, BF16),
    )
    return out.reshape(B, S, DM)
```

```python
import functools

import numpy as np
import jax
import jax.numpy as jnp
import jax.experimental.pallas as pl
import jax.experimental.pallas.tpu as pltpu

F32 = jnp.float32
BF16 = jnp.bfloat16
U32 = jnp.uint32

CB = 128
NQ = 4
KPAD = 16
HG = 8
NPA = 16
RB = 9
PRO_PW, PRO_X0, PRO_XN, PRO_XD, PRO_R0 = 24, 4, 3, 2, 1
UNROLL = 3
PHI = 3
INV_AT, PIN_U, PIN_X4 = 7, 2, 6
DIST = (1, 1)

LHS = ({(0, 0): 1}, {(0, 0): 1, (1, 0): 1}, {(0, 1): 1, (1, 1): 1}, {(1, 1): 1}, {(0, 0): 1, (1, 1): 1},
       {(0, 1): 1, (0, 0): -1}, {(1, 1): 1, (1, 0): -1}, {(0, 2): 1}, {(1, 2): 1},
       {(0, 0): 1, (1, 0): 1, (1, 2): -1}, {(0, 2): 1, (1, 2): 1, (0, 0): -1, (1, 0): -1},
       {(1, 2): 1, (1, 0): -1}, {(0, 1): 1, (1, 1): 1, (0, 2): -1},
       {(0, 2): 1, (1, 2): 1, (0, 1): -1, (1, 1): -1}, {(0, 1): 1, (0, 2): -1})
RHS = ({(0, 0): 1, (1, 0): 1, (0, 2): -1}, {(0, 0): 1, (2, 0): 1, (0, 1): -1},
       {(1, 1): 1, (2, 1): 1, (1, 0): -1}, {(1, 1): 1, (0, 1): 1, (1, 2): -1}, {(0, 1): 1, (1, 0): 1},
       {(1, 0): 1}, {(0, 1): 1}, {(2, 2): 1, (1, 2): 1, (2, 0): -1}, {(2, 2): 1, (0, 2): 1, (2, 1): -1},
       {(0, 2): 1, (2, 0): 1}, {(2, 0): 1}, {(0, 2): 1}, {(1, 2): 1, (2, 1): 1}, {(2, 1): 1}, {(1, 2): 1})
RIDE = {0: {0: 1}, 3: {1: 1}, 5: {1: 1, 0: -1}, 6: {1: 1, 0: -1}, 7: {2: 1}, 10: {2: 1}, 11: {0: 1},
        12: {2: 1}, 14: {1: 1, 2: -1}}
RIDE_TILE = ({0: 0, 3: 1, 5: 5, 6: 5}, {0: 2, 3: 3, 5: 6, 6: 6, 7: 4, 10: 4, 11: 2, 12: 4, 14: 7})
AHEAD = 2
PLAN = (((0, 0), (0, 2), (0, 3), (0, 4), (0, 5)), ((1, 0), (1, 2), (1, 3), (1, 4), (1, 5), (1, 7)),
        ((1, 9), (1, 10), (1, 11), (1, 12)))
PLAN_LAST = (((0, 0), (0, 3), (0, 5), (0, 6)), ((1, 0), (1, 3), (1, 5), (1, 6), (1, 7)), ((1, 10), (1, 11), (1, 12)))
ORDER = (0, 1, 5, 2, 3, 4, 6, 8, 7, 9, 10, 13, 11, 12, 14)
TRIPLES = ((0, 1, 2), (4, 5, 3))
T_TRI, T_LAST, T_TAIL, N_TILES = (28, 43), 58, 65, 68


def _lin(terms, get):
    acc = None
    for key, sign in terms.items():
        v = get(key)
        acc = v if acc is None else (acc + v if sign > 0 else acc - v)
    return acc


def _combine(m, n, nr, late=None):
    r = {i: v[:nr] for i, v in m.items() if i in RIDE}
    if n == 2:
        rid = [r[0] + r[5], r[3] - r[6]]
    else:
        v = r[10] + r[11]
        rid = [r[0] + r[5] + v, r[3] - r[6] + r[12] + r[14], r[7] + v + r[14]]
    if 2 not in m:
        return rid
    x = {i: v[nr:] if i in RIDE else v for i, v in m.items()}
    top = [x[0] + x[5], x[2] - x[3] + x[4] + x[5]]
    if n == 3:
        t = x[9] + x[11]
        u = x[12] - x[14]
        t0 = t + x[10]
        top = [top[0] + t0, top[1] - u, x[7] + t0 + x[14]]
    get = late if late is not None else x.get
    bot = [x[4] - x[0] - x[6], x[3] - x[6]]
    if n == 3:
        t1 = u + get(13)
        bot = [bot[0] - t, bot[1] + t1, t1 - x[11] + get(8)]
    bot[0] = bot[0] + get(1)
    return [jnp.concatenate(p, axis=0) for p in zip(rid, top, bot)]


def _dft_constants():
    qb = CB // NQ
    hb = qb // 2
    n = np.arange(CB, dtype=np.float64)
    f = np.concatenate([q * qb + np.concatenate([np.arange(0, qb, 2), np.arange(1, qb, 2)])
                        for q in range(NQ)])
    w = np.pi * (2.0 * f + 1.0) / (2 * CB)
    ang = (w[:, None] * (n[None, :] - (CB - 1) / 4.0)).reshape(NQ, qb, CB)
    fwd = np.concatenate([np.cos(ang), -np.sin(ang)], axis=1)
    inv = np.zeros((NQ, 2, hb, CB))
    for p in range(NQ):
        m = (NQ - 1 - p) * hb + np.arange(hb)
        ang = (m[:, None] + 0.5) * w[None, :]
        inv[p, 0] = np.cos(ang) / CB
        inv[p, 1] = -np.sin(ang) / CB
    return fwd.astype(np.float32), inv.astype(np.float32)


def _flip_rows(x):
    i = jax.lax.broadcasted_iota(jnp.int32, (8, x.shape[1]), 0)
    out = []
    for r in range(x.shape[0] - 8, -8, -8):
        v = pltpu.roll(x[r:r + 8], 4, 0)
        for b in (2, 1):
            v = jnp.where((i & b) == 0, pltpu.roll(v, 8 - b, 0), pltpu.roll(v, b, 0))
        out.append(v)
    return jnp.concatenate(out, axis=0)


def _ln(x, eps=1e-5):
    d = x.shape[-1]
    m = jnp.sum(x, axis=-1, keepdims=True) * (1.0 / d)
    xc = x - m
    v = jnp.sum(xc * xc, axis=-1, keepdims=True) * (1.0 / d)
    return xc * jax.lax.rsqrt(v + eps)


def _dot(a, b):
    return jnp.dot(a, b, preferred_element_type=F32)


def _dot_nt(a, b):
    return jax.lax.dot_general(a, b, (((1,), (1,)), ((), ())), preferred_element_type=F32)


def _pack(x):
    return pltpu.bitcast(x.astype(BF16), U32)


def _unpack(x):
    return pltpu.bitcast(x, BF16)


def _tile(x, n):
    return x[:, n * 128:(n + 1) * 128]


def _ext(r):
    return _pack(jnp.concatenate(
        [r, _tile(r, 1) - _tile(r, 0), _tile(r, 3) - _tile(r, 2), _tile(r, 3) - _tile(r, 4)], axis=1))


def _in_order(actions):
    def body(i, c):
        for j, act in enumerate(actions):
            pl.when(i == j)(act)
        return c
    jax.lax.fori_loop(0, len(actions), body, 0)


def _kernel(x_hbm, mem0_hbm, wq_hbm, wk_hbm, wv_hbm, wo_hbm, k_hbm, v_hbm,
            sh_hbm, sk_hbm, sd_hbm, fwd_hbm, inv_hbm, o_hbm,
            sp_sc, kr_sc, wf_sc, x2_sc, y_sc, u_sc, op_sc, pre_sc, xn_sc, wa_sc, wb_sc, wo_sc, wc_sc,
            x_sc, v_sc, sk_sc, st_sc, out_sc, fwd_ref, inv_ref,
            k_sc, hp_sc, h_sc, co_sc, mem0_ref, sh_ref, sd_ref,
            never_sm, sem_x, sem_in, sem_w, sem_out,
            *, S, DM, H, DH, M, SEG):
    NSEG = S // SEG
    M2 = 2 * M
    S2 = SEG // 2
    R = M2 + 2 * SEG
    RH = M2 + SEG
    NB = S // CB
    QB = CB // NQ
    HB = QB // 2
    NT = DM // 128
    PH = PHI * UNROLL
    NRB = (NSEG - 1) // RB
    NPH = (NSEG - 1) // PH
    NG = H // HG
    NCH = 3 * NG
    NPASS = NPA // HG
    DH2 = DM // 2
    NU = 3 * NG
    DE = DM + 3 * 128
    KS = sh_ref.shape[0]
    UL = 2 * NQ + 1
    LN = pl.ds(0, DM)
    assert NT == 5 and HG == 8 and DH == 128 and 2 <= KS <= 8 and QB == SEG and NRB * RB == NSEG - 1 and NPH * PH == NSEG - 1 and NPASS == 2 and 2 * NRB >= NCH + 1

    mem0_copy = pltpu.make_async_copy(mem0_hbm, mem0_ref, sem_x.at[0])
    small = [pltpu.make_async_copy(s, d, sem_in.at[0]) for s, d in [
        (sh_hbm, sh_ref), (sd_hbm, sd_ref), (fwd_hbm, fwd_ref), (inv_hbm, inv_ref)]]

    def x_copy(b):
        if isinstance(b, int) and b == 0:
            rows = pl.ds(0, (RB + 1) * SEG)
        else:
            rows = pl.ds(pl.multiple_of((b * RB + 1) * SEG, SEG), RB * SEG)
        return pltpu.make_async_copy(x_hbm.at[rows], x_sc.at[rows, LN], sem_x.at[b])

    kb = (0, (UL + 1) * SEG, (UL + PH + 1) * SEG, S)
    sb = (0, 2, (PH + 2) // NQ + 2, NB)

    def in_copies(part):
        def rng(b):
            return pl.ds(b[part], b[part + 1] - b[part])
        sem = sem_in.at[part]
        return [
            pltpu.make_async_copy(k_hbm.at[rng(kb)],
                                  k_sc.at[pl.ds(KPAD + kb[part], kb[part + 1] - kb[part]), LN], sem),
            pltpu.make_async_copy(v_hbm.at[rng(kb)], v_sc.at[rng(kb), LN], sem),
        ] + [pltpu.make_async_copy(sk_hbm.at[:, pl.ds(c * CB, CB)], sk_sc.at[c], sem)
             for c in range(sb[part], sb[part + 1])]

    def w_copies(ci, dst=None, part=None):
        src = (wq_hbm, wk_hbm, wv_hbm)[ci // NG]
        dst = ci if dst is None else dst
        spans = {None: [(0, DM // 16)], 0: [(0, 16)], 1: [(16, DM // 16)]}[part]
        sem = sem_w.at[NCH + 1 if part == 1 else dst]
        return [pltpu.make_async_copy(
            src.at[pl.ds(lo, hi - lo), hf, :, pl.ds((ci % NG) * HG, HG), :],
            st_sc.at[dst, pl.ds(lo, hi - lo), :, pl.ds(hf * HG, HG), :], sem)
            for lo, hi in spans for hf in range(2)]

    wo_copy = pltpu.make_async_copy(wo_hbm, wo_sc, sem_w.at[NCH])

    def out_copy(lo, n):
        rows = pl.ds(lo * SEG if isinstance(lo, int) else pl.multiple_of(lo * SEG, SEG), n * SEG)
        return pltpu.make_async_copy(out_sc.at[rows, LN], o_hbm.at[rows], sem_out)

    def start_all(cps):
        def act():
            for cp in cps:
                cp.start()
        return act

    order = [[mem0_copy, x_copy(0)], w_copies(0, part=0), w_copies(0, part=1), [x_copy(1)], [x_copy(2)]]
    for ci in range(1, NCH):
        order.append(w_copies(ci) + ([x_copy(ci + 2)] if ci + 2 < NRB else []))
        if ci == NRB - 2:
            order.append(small + in_copies(0))
    order += [[wo_copy], in_copies(1), in_copies(2)]
    for i in range(0, len(order), 5):
        _in_order([start_all(cps) for cps in order[i:i + 5]])

    never_sm[0] = 0
    k_sc[0:KPAD, LN] = jnp.zeros((KPAD, DM), BF16)
    sp_sc[NB + 1] = jnp.zeros(sp_sc.shape[1:], F32)
    op_sc[...] = jnp.zeros(op_sc.shape, F32)
    x2_sc[...] = jnp.zeros(x2_sc.shape, F32)
    y_sc[2 * CB - SEG:, LN] = jnp.zeros((SEG, DM), F32)
    mem0_copy.wait()
    x_copy(0).wait()
    for sg in range(RB + 1):
        xn_sc[sg] = _ext(_ln(x_sc[sg * SEG:(sg + 1) * SEG, LN].astype(F32)))

    def clip(i, hi):
        return min(max(i, 0), hi) if isinstance(i, int) else jnp.clip(i, 0, hi)

    def scaled(i, m):
        return i * m if isinstance(i, int) else pl.multiple_of(i * m, m)

    def seg(i):
        return pl.ds(scaled(clip(i, NSEG - 1), SEG), SEG)

    def conv_u(s, ln=LN):
        r0 = scaled(clip(s, NSEG - 1), SEG)
        kk = k_sc[pl.ds(r0, KPAD + SEG), ln].astype(F32)[KPAD - 8:]

        def coef(j, rows):
            return jnp.concatenate([co_sc[j, :, ln]] * (rows // 8), axis=0)
        sft = [kk] + [pltpu.roll(kk, j, 0) for j in range(2, KS, 2)]
        ev = functools.reduce(jnp.add, [sft[j // 2][8:] * coef(j, SEG) for j in range(0, KS, 2)])
        od = functools.reduce(jnp.add, [sft[j // 2] * coef(j, SEG + 8) for j in range(1, KS, 2)])
        ks = ev + pltpu.roll(od, 1, 0)[8:]
        u = (ks * v_sc[pl.ds(r0, SEG), ln].astype(F32)).astype(BF16)
        u_sc[pl.ds(r0, SEG), ln] = u
        return u

    def conv_fwd(c, q):
        cc = clip(c, NB - 1)
        f = fwd_ref[q]
        uf = _dot(f, u_sc[pl.ds(scaled(cc, CB), CB), LN])
        kf = _dot_nt(f, sk_sc[cc])
        return uf, kf

    def put_spec(cs, q, which, val):
        for n in range(NT):
            v = val[:, n * 128:(n + 1) * 128].reshape(2, QB // 8, 8, 128)
            sp_sc[cs, q, :, n, which:which + 2] = jnp.stack([v[0], v[1]], axis=1)

    def conv_spec(c, q):
        uf, kf = conv_fwd(c, q)
        cs = clip(c, NB)
        put_spec(cs, q, 0, uf)
        pk = kr_sc[q]
        kr_sc[q] = kf
        kp = jnp.concatenate([
            kf[0:HB] - pk[QB:QB + HB],
            kf[HB:QB] + pk[QB + HB:],
            kf[QB:QB + HB] + pk[0:HB],
            kf[QB + HB:] - pk[HB:QB]], axis=0)
        put_spec(cs, q, 2, kp)

    MAC_PIECES = [(rb, n) for rb in range(QB // 16) for n in range(NT)]

    def conv_mac(c, q, piece, nterms):
        rb2, n = piece
        cs = clip(c, NB)
        rbs = slice(2 * rb2, 2 * rb2 + 2)
        ar = None
        ai = None
        for j in range(nterms):
            if isinstance(cs, int):
                uj, kj = j, cs - j
            else:
                uj = jnp.minimum(j, cs)
                kj = jnp.where(cs - j >= 0, cs - j, NB + 1)
            u = sp_sc[uj, q, rbs, n, 0:2]
            k = sp_sc[kj, q, rbs, n, 2:4]
            tr = u[:, 0] * k[:, 0] - u[:, 1] * k[:, 1]
            ti = u[:, 0] * k[:, 1] + u[:, 1] * k[:, 0]
            ar = tr if ar is None else ar + tr
            ai = ti if ai is None else ai + ti
        ln = slice(n * 128, (n + 1) * 128)
        w = jnp.concatenate([ar.reshape(16, 128), ai.reshape(16, 128)], axis=0).astype(BF16)
        wf_sc[c & 1, 0, q, rb2 * 16:rb2 * 16 + 16, ln] = w[0:16]
        wf_sc[c & 1, 1, q, rb2 * 16:rb2 * 16 + 16, ln] = w[16:]

    def conv_inv(tt, n):
        cb = tt // NQ
        p = tt % NQ
        ln = slice(n * 128, (n + 1) * 128)
        ev = _dot(inv_ref[p, 0], wf_sc[cb & 1, 0, :, :, ln].reshape(CB, 128))
        od = _dot(inv_ref[p, 1], wf_sc[cb & 1, 1, :, :, ln].reshape(CB, 128))
        sd = jnp.concatenate([co_sc[KS, :, ln]] * (HB // 8), axis=0)
        for r, val in ((p, _flip_rows(ev - od)), (2 * NQ - 1 - p, ev + od)):
            ur = scaled(clip(cb, NB - 1) * (2 * NQ) + r, HB)
            yr = scaled((cb & 1) * (2 * NQ) + r, HB)
            y_sc[pl.ds(yr, HB), ln] = val + u_sc[pl.ds(ur, HB), ln].astype(F32) * sd

    def y_seg(s):
        return y_sc[pl.ds(scaled(s & (2 * NQ - 1), SEG), SEG), LN]

    scale = DH ** -0.5
    cexp = scale * float(np.log2(np.e))

    def make_mask(n, x_layers, q0=0):
        qi = jax.lax.broadcasted_iota(jnp.int32, (n - q0, n), 0) + q0
        ki = jax.lax.broadcasted_iota(jnp.int32, (n - q0, n), 1)

        def layer(i):
            xl = jnp.where(i < M2 + SEG, x_layers[0], x_layers[-1])
            return jnp.where(i < M, 0, jnp.where(i < M2, 1, xl))
        same = layer(qi) == layer(ki)
        ok = same & ((qi < M2) | (ki < M2) | (qi >= ki))
        fill = jnp.where(same, -1e9 / scale, -jnp.inf).astype(F32)
        return ok, fill

    def probs(q, k, mask):
        ok, fill = mask
        s = _dot_nt(q, k)
        s = jnp.where(ok, s, fill)
        m = jnp.max(s, axis=-1, keepdims=True)
        p = jnp.exp2((s - m) * cexp)
        l = jnp.sum(p, axis=-1, keepdims=True)
        r = pl.reciprocal(l, approx=True)
        r = r * (2.0 - l * r)
        return (p * r).astype(BF16)

    def w_slot(ci):
        return (wb_sc, ci) if 1 <= ci < NRB - 1 else (wa_sc, max(ci - (NRB - 2), 0))

    def rows(*parts):
        return jnp.concatenate(parts, axis=0)

    def cols(*parts):
        return jnp.concatenate(parts, axis=1)

    def bf(*xs):
        return tuple(x.astype(BF16) for x in xs)

    def xn(s):
        return xn_sc[clip(s, NSEG - 1)]

    def unit_products(tile, u, xf, rid, only=None):
        def lhs(part, i):
            ps = [_unpack(_tile(rid, RIDE_TILE[part][i]))] if i in RIDE else []
            return rows(*(ps + ([xf(part, i)] if xf is not None else [])))
        base = T_TRI[u] if u < 2 else T_LAST
        m = {}
        for i in ORDER:
            if (xf is None and i not in RIDE) or (only is not None and i not in only):
                continue
            if i < 7:
                m[i] = _dot(cols(lhs(0, i), lhs(1, i)), rows(tile(4 * i + (0, 2, 3)[u]), tile(base + i)))
                if u == 0:
                    m["mid", i] = _dot(lhs(0, i), tile(4 * i + 1))
            elif u < 2:
                m[i] = _dot(lhs(1, i), tile(base + i))
        return m

    def unit(tile, u, xf, rid, carry, ahead=None):
        nr = 2 * rid.shape[0]
        m = dict(ahead or {})
        m.update(unit_products(tile, u, xf, rid, [i for i in range(15) if i not in m]))
        main = {i: v for i, v in m.items() if isinstance(i, int)}
        if u == 2:
            a = rows(*([_unpack(_tile(rid, 4))] + ([xf(1, 7), xf(1, 8)] if xf is not None else [])))
            c = _combine(main, 2, nr)
            return {6 + j: _dot(a, tile(T_TAIL + j)) + c[j] for j in range(2)}
        if u == 0:
            carry[2], carry[3] = _combine({i[1]: v for i, v in m.items() if not isinstance(i, int)}, 2, nr)
        c = _combine(main, 3, nr)
        hs = TRIPLES[u]
        return {hs[0]: c[0], hs[1]: c[1], hs[2]: c[2] + carry.pop(hs[2])}

    def w_tiles(g, mats):
        slots = [w_slot(mi * NG + g) for mi in mats]
        return lambda i: _unpack(cols(*[ref[k, i] for ref, k in slots]))

    def attend(proj, n, mask, plan, hook=None, raw=False):
        D1, D2 = DIST
        full = n == R
        nr = M2 if full else n
        parts = {}
        os_ = {}

        def add_forms(g, hs, ids):
            for i in range(7 if len(hs) == 2 else 15):
                ps = []
                if i in RIDE:
                    ps.append(_lin(RIDE[i], lambda k: os_[hs[k]][:nr]))
                if full:
                    ps.append(_lin(LHS[i], lambda rk: os_[hs[rk[1]]][M2 + rk[0] * SEG:RH + rk[0] * SEG]))
                if ps:
                    a = rows(*ps).astype(BF16)
                    for part, tid in ids(i):
                        parts.setdefault((part, i), []).append((g, a, tid))

        def prod(key, g0, g1):
            if raw:
                a = cols(*[parts[h] for h in range(g0 * HG, g1 * HG)])
                return _dot(a, wo_sc[g0 * HG * DH:g1 * HG * DH, key * 128:(key + 1) * 128])
            sel = [p for p in parts[key] if g0 <= p[0] < g1]
            return _dot(cols(*[p[1] for p in sel]), _unpack(rows(*[wc_sc[p[0], p[2]] for p in sel])))

        qkvs = {}
        ps = {}
        m = {}
        for it in range(NU + D1 + D2):
            if it < NU:
                qkvs[it] = proj(it)
            k = it - D1
            if 0 <= k < NU:
                ps[k] = {h: probs(q, kk, mask) for h, (q, kk, _) in qkvs[k].items()}
            k = it - D1 - D2
            if 0 <= k < NU:
                g, u = divmod(k, 3)
                pk, qk = ps.pop(k), qkvs.pop(k)
                os_.update({h: _dot(pk[h], qk[h][2]) for h in pk})
                if raw:
                    parts.update({g * HG + h: os_[h].astype(BF16) for h in pk})
                elif u < 2:
                    add_forms(g, TRIPLES[u], lambda i: [(1, T_TRI[u] + i)] + ([(0, 4 * i + 2 * u)] if i < 7 else []))
                    if u == 1:
                        add_forms(g, (2, 3), lambda i: [(0, 4 * i + 1)])
                else:
                    add_forms(g, (6, 7), lambda i: [(0, 4 * i + 3), (1, T_LAST + i)])
                    for j in range(2):
                        parts[1, 7].append((g, os_[6 + j][:min(n, RH)].astype(BF16), T_TAIL + j))
                        if full:
                            parts[1, 8].append((g, os_[6 + j][RH:].astype(BF16), T_TAIL + j))
            if hook is not None:
                hook(it)
            j = it - (NU - 1)
            if j >= 0:
                for key in plan[j]:
                    m[key] = prod(key, 0, NG - 1)
        early = list(m)
        last = [(0, 1), (1, 1), (1, 8), (1, 13)]
        keys = range(NT) if raw else sorted(parts, key=lambda k: (k[1] == 6, ORDER.index(k[1]), k[0]))
        for key in keys:
            if key not in early and key not in last and (raw or key[1] != 6):
                m[key] = prod(key, 0, NG)
        for key in early:
            m[key] = prod(key, NG - 1, NG) + m[key]
        if raw:
            return cols(*[m[i] for i in range(NT)])
        for key in ((0, 6), (1, 6)):
            if key not in early:
                m[key] = prod(key, 0, NG)
        res = []
        for part in range(2):
            res += _combine({k[1]: v for k, v in m.items() if k[0] == part}, 2 + part, nr,
                            lambda i: prod((part, i), 0, NG))
        return cols(*res)

    def side2(t, a2):
        x3 = x2_sc[(t - 2) & 3] + a2
        x4 = x3 + _ln(x3) * y_seg(t - 2)
        x4 = x4.astype(out_sc.dtype)
        out_sc[seg(t - 2), LN] = x4
        return x4

    def finish(t, xr, yt, mem, a1):
        x1 = xr.astype(F32) + a1
        x2 = x1 + _ln(x1) * yt
        h_sc[0:M, :] = _ext(mem)
        x2_sc[t & 3] = x2
        return x2

    X1_ONLY = (0, 5, 7, 14)
    X2_TILE = ({3: 1, 6: 5}, {3: 3, 6: 6, 8: 4})

    def prepare(e1, x2):
        n = (_unpack(e1[:, 0:DM]).astype(F32), _ln(x2))
        mixed = {(part, i): _lin(LHS[i], lambda rk: _tile(n[rk[0]], 2 * part + rk[1]))
                 for part in range(2) for i in range((7, 15)[part])
                 if i not in X1_ONLY and i not in X2_TILE[part]}
        return _ext(n[1]), mixed

    def pinned(r, pins):
        never = never_sm[0] > 0
        hs = {0: r}
        tiles = [r[:, n:n + 128] for n in range(0, r.shape[1], 128)]
        for g, n, d in sorted(pins, key=lambda p: p[0]):
            tiles[n] = jnp.where(never, d, tiles[n])
            hs[g] = cols(*tiles)
        return lambda g: hs[max(k for k in hs if k <= g)]

    def pin_tiles(g0, per, val):
        v = _pack(val)
        return [(g0 + n // per, (1, 3, 4, 5, 6)[n], _tile(v, n)) for n in range(NT)]

    def wait_chunk(ci):
        for cp in w_copies(0, ci):
            cp.wait()

    def w_block(ci, b):
        x = pltpu.bitcast(st_sc[ci, b], U32)
        sub = jax.lax.broadcasted_iota(jnp.int32, (8, DH), 0)
        res = []
        for par in range(2):
            v = [x[2 * i + par] for i in range(4)]
            for bit in (2, 1):
                keep = (sub & bit) == 0
                for i in range(4):
                    if not i & bit:
                        a, c = v[i], v[i + bit]
                        v[i] = jnp.where(keep, a, pltpu.roll(c, bit, 0))
                        v[i + bit] = jnp.where(keep, pltpu.roll(a, 8 - bit, 0), c)
            res.append(v)
        return res

    def rhs_tiles(part, plain, value, pack, swap):
        def one(i, base, hs):
            terms = {kj: sg for kj, sg in RHS[i].items() if max(kj) < len(hs)}

            def at(kj):
                k, j = kj[::-1] if swap else kj
                return base + k, hs[j]
            if len(terms) == 1:
                return plain(*at(next(iter(terms))))
            return pack(_lin(terms, lambda kj: value(*at(kj))))
        if part == 0:
            for p in range(4):
                for i in range(7):
                    yield 4 * i + p, one(i, 0, (2 * p, 2 * p + 1))
        else:
            for u in range(2):
                for i in range(15):
                    yield T_TRI[u] + i, one(i, 2, TRIPLES[u])
            for i in range(7):
                yield T_LAST + i, one(i, 2, (6, 7))
            for j in range(2):
                yield T_TAIL + j, plain(4, 6 + j)

    def relayout(ci, dst, slot, part, b):
        hi_m = U32(0xFFFF0000)
        t = {k: w_block(ci, 8 * k + b) for k in ((0, 1), (2, 3, 4))[part]}

        def plain(k, h):
            a, c = t[k][0][h // 2], t[k][1][h // 2]
            return (a >> 16) | (c & hi_m) if h % 2 else (a & U32(0xFFFF)) | (c << 16)

        @functools.lru_cache(None)
        def value(k, h):
            w = cols(t[k][0][h // 2], t[k][1][h // 2])
            return pltpu.bitcast(w & hi_m if h % 2 else w << 16, F32)

        def pack(v):
            r = pltpu.bitcast(v.astype(BF16).astype(F32), U32)
            return (r[:, :DH] >> 16) | r[:, DH:]
        out = dict(rhs_tiles(part, plain, value, pack, False))
        lo = min(out)
        dst[slot, lo:lo + len(out), pl.ds(scaled(b, 8), 8), :] = jnp.stack([out[i] for i in sorted(out)])

    def main(_, carry):
        for part in range(2):
            def relayout0(b, c, part=part):
                relayout(0, wa_sc, 0, part, b)
                return c
            with jax.named_scope("wait_w"):
                for cp in w_copies(0, part=part):
                    cp.wait()
            with jax.named_scope("relayout"):
                jax.lax.fori_loop(0, 8, relayout0, 0)

        def pro_stage(ps_, b):
            n = ps_ * NRB + b
            with jax.named_scope("wait_w"):
                if ps_ == 0:
                    @pl.when(b + 1 < NRB)
                    def _():
                        x_copy(b + 1).wait()

                @pl.when((n >= 2) & (n <= NCH))
                def _():
                    wait_chunk(n - 1)
            cr = jnp.clip(n - 1, 0, NCH - 1)
            dst, slot = (wb_sc, cr) if ps_ == 0 else (wa_sc, cr - (NRB - 2))
            bl = jnp.minimum(b + 1, NRB - 1)
            PW = PRO_PW
            npc = RB * S2 // PW
            assert npc * PW == RB * S2 and 3 * npc >= 16 + PRO_R0 and 2 * NRB > UL

            def body(i, c):
                s0 = b * RB + 1
                for sg in range(RB):
                    hp_sc[sg * S2:(sg + 1) * S2, :] = xn_sc[s0 + sg]
                for pi in range(npc):
                    carry = {}
                    for u in range(3):
                        pos = 3 * pi + u
                        hx = hp_sc[pi * PW:(pi + 1) * PW, :]
                        for k in range(max(RB, 2 * NT)):
                            if PRO_X0 + k * PRO_XN // PRO_XD != pos:
                                continue
                            if ps_ == 0 and k < RB:
                                sn = bl * RB + 1 + k
                                xv = _ext(_ln(x_sc[seg(sn), LN].astype(F32)))
                                xn_sc[sn] = xv
                                hx = rows(hx[:-S2], jnp.where(never_sm[0] > 0, xv, hx[-S2:]))
                            if ps_ == 1 and k < 2 * NT:
                                conv_u(jnp.minimum(2 * b + k // NT, UL),
                                       slice((k % NT) * 128, (k % NT + 1) * 128))
                        if 0 <= pos - PRO_R0 < 16:
                            relayout(cr, dst, slot, (pos - PRO_R0) % 2, (pos - PRO_R0) // 2)
                        for h, r in unit(w_tiles(ps_, (0,)), u, None, hx, carry).items():
                            for a in range(0, 2 * PW, 16):
                                sg, off = divmod(2 * pi * PW + a, SEG)
                                pre_sc[s0 + sg, ps_ * HG + h, off:off + 16, :] = r[a:a + 16].astype(BF16)
                return c
            assert PRO_X0 + (max(RB, 2 * NT) - 1) * PRO_XN // PRO_XD < 3 * npc
            with jax.named_scope("fused"):
                jax.lax.fori_loop(0, never_sm[0] + 1, body, 0)

        for ps_ in range(NPASS):
            if ps_ == 1:
                with jax.named_scope("wait_in0"):
                    for cp in small + in_copies(0):
                        cp.wait()
                sh = sh_ref[...].astype(F32)
                for j in range(KS):
                    co_sc[j] = jnp.broadcast_to(sh[j:j + 1], (8, DM))
                co_sc[KS] = jnp.broadcast_to(sd_ref[...].astype(F32).reshape(1, DM), (8, DM))

            def blk(b, c, ps_=ps_):
                pro_stage(ps_, b)
                return c
            jax.lax.fori_loop(0, NRB, blk, 0)

        def warm_block0(q):
            uf, kf = conv_fwd(0, q)
            put_spec(0, q, 0, uf)
            put_spec(0, q, 2, kf)
            kr_sc[q] = kf
            ur, um, kr, km = uf[:QB], uf[QB:], kf[:QB], kf[QB:]
            wf_sc[0, 0, q] = (ur * kr - um * km).astype(BF16)
            wf_sc[0, 1, q] = (ur * km + um * kr).astype(BF16)

        def wo_operands(d):
            g, b, part = d // 16, (d % 16) // 2, d % 2
            z = jnp.minimum(never_sm[0], 0)

            def src(k, h):
                r = (g * HG + h) * DH + 16 * b
                return wo_sc[r:r + 16, k * 128:(k + 1) * 128]
            out = dict(rhs_tiles(part, lambda k, h: _pack(src(k, h)),
                                 functools.lru_cache(None)(lambda k, h: src(k, h).astype(F32)), _pack, True))
            lo = min(out)
            wc_sc[z + g, lo:lo + len(out), 8 * b:8 * b + 8, :] = jnp.stack([out[i] for i in sorted(out)])

        def plain_qkv(eq, ekv, k, carry, after=None):
            g, u = divmod(k, 3)
            res = []
            for mats, e in (((1,), ekv), ((2,), ekv), ((0,), eq)):
                res.append(unit(w_tiles(g, mats), u, None, e, carry.setdefault(mats, {})))
                if after is not None:
                    after(res[-1])
            return {h: bf(res[2][h], res[0][h], res[1][h]) for h in res[0]}

        with jax.named_scope("wait_wo"):
            wo_copy.wait()
        with jax.named_scope("step0"):
            mem0 = mem0_ref[...].astype(F32)
            e0 = rows(_ext(rows(mem0, mem0)), xn(0))

            todo = list(range(16 * NG))
            carry0 = {}

            def after0(res):
                z = jnp.minimum(never_sm[0], 0)
                for r in list(res.values())[:2]:
                    wc_sc[z, N_TILES - 1, 0:8, :] = pltpu.bitcast(r[0:8], U32)
                    if todo:
                        wo_operands(todo.pop(0))

            def hook0(it):
                if it < NQ:
                    warm_block0(it)
                if 5 <= it < 5 + NT:
                    for p in range(2):
                        conv_inv(p, it - 5)
            out = attend(lambda k: plain_qkv(e0, e0, k, carry0, after0), RH, make_mask(RH, (0,)),
                         ((0, 1), (2,), (3,)), hook0, True)
            assert not todo
            y0 = y_seg(0)
            for q in range(2):
                conv_spec(1, q)
            for n in range(NT):
                conv_inv(2, n)
            finish(0, x_sc[0:SEG, LN], y0, rows(out[0:M], mem0), out[M2:])
            for q in range(2):
                for piece in MAC_PIECES:
                    conv_mac(1, q, piece, 2)

        mask12 = make_mask(R, (0, 1))

        def step(t, x2):
            first = x2 is None
            c, q = (t + 1) // NQ + 1, (t + 1) % NQ
            em = h_sc[0:M, :]
            e1 = xn(t)

            def x1_form(part, i):
                return _unpack(_tile(e1, RIDE_TILE[part][i]))
            ahead = unit_products(w_tiles(0, (1, 2)), 0, x1_form, em, X1_ONLY if first else X1_ONLY[:AHEAD])
            if first:
                x2 = x2_sc[(t - 1) & 3]
            conv_spec(c, q)
            for piece in MAC_PIECES:
                conv_mac(c, q, piece, NB)
            ex2, mixed = prepare(e1, x2)
            mixed = {k: v.astype(BF16) for k, v in mixed.items()}
            x4 = side2(t, op_sc[...])
            un = conv_u(t + UL)
            e2 = pinned(ex2, pin_tiles(PIN_U, 2, un) + pin_tiles(PIN_X4, NT, x4))
            carry = {}

            def proj(k):
                g, u = divmod(k, 3)

                def xf(part, i):
                    if i in X1_ONLY:
                        return x1_form(part, i)
                    if i in X2_TILE[part]:
                        return _unpack(_tile(e2(k), X2_TILE[part][i]))
                    return mixed[part, i]
                pre = g * HG < NPA
                if pre:
                    qs = unit(w_tiles(g, (0,)), u, None, rows(em, e2(k)), carry.setdefault("q", {}))
                rs = unit(w_tiles(g, (1, 2) if pre else (1, 2, 0)), u, xf, em, carry.setdefault("kv", {}),
                          ahead if k == 0 else None)
                res = {}
                for h, r in rs.items():
                    if pre:
                        qq = rows(qs[h][:M2], pre_sc[t, g * HG + h].astype(F32), qs[h][M2:])
                    else:
                        qq = r[:, 2 * DH:]
                    res[h] = bf(qq, r[:, :DH], r[:, DH:2 * DH])
                return res

            held = {}

            def hook(it):
                if INV_AT <= it < INV_AT + NT:
                    conv_inv(t + 2, it - INV_AT)
                if it == NU:
                    held["x"] = x_sc[seg(t), LN]
                    held["y"] = y_seg(t)
            out = attend(proj, R, mask12, PLAN, hook)
            op_sc[...] = out[RH:]
            return finish(t, held["x"], held["y"], out[0:M2], out[M2:RH])

        def steps(i, carry):
            x2 = None
            for j in range(UNROLL):
                x2 = step(1 + i * UNROLL + j, x2)
            return carry

        def phase(p, carry):
            @pl.when(p == 1)
            def _():
                for cp in in_copies(2):
                    cp.wait()

            @pl.when(p >= 2)
            def _():
                out_copy((p - 2) * PH, PH).start()

            with jax.named_scope("steps"):
                jax.lax.fori_loop(p * PHI, (p + 1) * PHI, steps, 0)
            return carry

        for cp in in_copies(1):
            cp.wait()
        jax.lax.fori_loop(0, NPH, phase, 0)
        out_copy((NPH - 2) * PH, NSEG - 2 - (NPH - 2) * PH).start()

        with jax.named_scope("step_last"):
            x4 = side2(NSEG, op_sc[...])
            em = h_sc[0:M, :]
            ex = pinned(_ext(_ln(x2_sc[(NSEG - 1) & 3])), pin_tiles(PIN_X4, NT, x4))
            carry1 = {}
            out = attend(lambda k: plain_qkv(ex(k), rows(em, ex(k)), k, carry1),
                         SEG, make_mask(RH, (1,), M2), PLAN_LAST)
            side2(NSEG + 1, out)
        out_copy(NSEG - 2, 2).start()
        out_copy(0, NSEG).wait()
        return carry

    jax.lax.fori_loop(0, never_sm[0] + 1, main, 0)


def pallas_interleave_layers__memory_aug_recurrent_mem_tr__ssm_conv_h3__prompt_kernel(
    A_x, A_mem0, A_Wq, A_Wk, A_Wv, A_Wo, A_seg_len,
    B_q, B_k, B_v, B_shift_k, B_ssm_k, B_ssm_D,
):
    del B_q
    seg = int(A_seg_len) if isinstance(A_seg_len, (int, np.integer)) else CB // NQ
    return _run(A_x, A_mem0, A_Wq, A_Wk, A_Wv, A_Wo, B_k, B_v, B_shift_k, B_ssm_k, B_ssm_D, SEG=seg)


@functools.partial(jax.jit, static_argnames=("SEG",))
def _run(A_x, A_mem0, A_Wq, A_Wk, A_Wv, A_Wo, B_k, B_v, B_shift_k, B_ssm_k, B_ssm_D, *, SEG):
    B, S, DM = A_x.shape
    assert B == 1
    H, DH = A_Wq.shape[1], A_Wq.shape[2]
    M = A_mem0.shape[1]
    KS = B_shift_k.shape[1]
    R = 2 * (M + SEG)
    NSEG = S // SEG
    NRB = (NSEG - 1) // RB
    NB = S // CB
    QB = CB // NQ
    NCH = 3 * H // HG
    DP = -(-DM // 256) * 256
    fwd, inv = _dft_constants()

    kern = functools.partial(_kernel, S=S, DM=DM, H=H, DH=DH, M=M, SEG=SEG)
    any_spec = pl.BlockSpec(memory_space=pl.ANY)
    out = pl.pallas_call(
        kern,
        out_shape=jax.ShapeDtypeStruct((S, DM), A_x.dtype),
        in_specs=[any_spec] * 13,
        out_specs=any_spec,
        scratch_shapes=[
            pltpu.VMEM((NB + 2, NQ, QB // 8, DM // 128, 4, 8, 128), F32),
            pltpu.VMEM((NQ, 2 * QB, DM), F32),
            pltpu.VMEM((2, 2, NQ, QB, DM), BF16),
            pltpu.VMEM((4, SEG, DM), F32),
            pltpu.VMEM((2 * CB, DP), F32),
            pltpu.VMEM((S, DP), BF16),
            pltpu.VMEM((SEG, DM), F32),
            pltpu.VMEM((NSEG, NPA, SEG, DH), BF16),
            pltpu.VMEM((NSEG, SEG // 2, DM + 384), U32),
            pltpu.VMEM((NCH - NRB + 2, N_TILES, 64, DH), U32),
            pltpu.VMEM((NRB - 1, N_TILES, 64, DH), U32),
            pltpu.VMEM((H * DH, DM), BF16),
            pltpu.VMEM((H // HG, N_TILES, 64, DH), U32),
            pltpu.VMEM((S, DP), BF16),
            pltpu.VMEM((S, DP), BF16),
            pltpu.VMEM((NB, DM, CB), BF16),
            pltpu.VMEM((NCH, DM // 16, 8, 2 * HG, DH), BF16),
            pltpu.VMEM((S, DP), A_x.dtype),
            pltpu.VMEM(fwd.shape, BF16),
            pltpu.VMEM(inv.shape, BF16),
            pltpu.VMEM((S + KPAD, DP), BF16),
            pltpu.VMEM((RB * SEG // 2, DM + 384), U32),
            pltpu.VMEM((M, DM + 384), U32),
            pltpu.VMEM((KS + 1, 8, DM), F32),
            pltpu.VMEM((M, DM), BF16),
            pltpu.VMEM((KS, DM), BF16),
            pltpu.VMEM((DM,), BF16),
            pltpu.SMEM((1,), jnp.int32),
            pltpu.SemaphoreType.DMA(((NSEG - 1) // RB,)),
            pltpu.SemaphoreType.DMA((3,)),
            pltpu.SemaphoreType.DMA((NCH + 2,)),
            pltpu.SemaphoreType.DMA(()),
        ],
        compiler_params=pltpu.CompilerParams(vmem_limit_bytes=120 * 1024 * 1024),
    )(
        A_x.reshape(S, DM), A_mem0.reshape(M, DM),
        *[w.reshape(DM // 16, 2, 8, H, DH) for w in (A_Wq, A_Wk, A_Wv)],
        A_Wo.reshape(H * DH, DM), B_k.reshape(S, DM), B_v.reshape(S, DM),
        B_shift_k.T, B_ssm_k, B_ssm_D,
        jnp.asarray(fwd, BF16), jnp.asarray(inv, BF16),
    )
    return out.reshape(B, S, DM)
```

```python
import functools

import numpy as np
import jax
import jax.numpy as jnp
import jax.experimental.pallas as pl
import jax.experimental.pallas.tpu as pltpu

F32 = jnp.float32
BF16 = jnp.bfloat16
U32 = jnp.uint32

CB = 128
NQ = 4
KPAD = 16
HG = 8
NPA = 16
RB = 9
PRO_PW, PRO_X0, PRO_XN, PRO_XD, PRO_R0 = 24, 4, 3, 2, 1
UNROLL = 3
PHI = 3
INV_AT, PIN_U, PIN_X4 = 7, 2, 6
DIST = (1, 1)

LHS = ({(0, 0): 1}, {(0, 0): 1, (1, 0): 1}, {(0, 1): 1, (1, 1): 1}, {(1, 1): 1}, {(0, 0): 1, (1, 1): 1},
       {(0, 1): 1, (0, 0): -1}, {(1, 1): 1, (1, 0): -1}, {(0, 2): 1}, {(1, 2): 1},
       {(0, 0): 1, (1, 0): 1, (1, 2): -1}, {(0, 2): 1, (1, 2): 1, (0, 0): -1, (1, 0): -1},
       {(1, 2): 1, (1, 0): -1}, {(0, 1): 1, (1, 1): 1, (0, 2): -1},
       {(0, 2): 1, (1, 2): 1, (0, 1): -1, (1, 1): -1}, {(0, 1): 1, (0, 2): -1})
RHS = ({(0, 0): 1, (1, 0): 1, (0, 2): -1}, {(0, 0): 1, (2, 0): 1, (0, 1): -1},
       {(1, 1): 1, (2, 1): 1, (1, 0): -1}, {(1, 1): 1, (0, 1): 1, (1, 2): -1}, {(0, 1): 1, (1, 0): 1},
       {(1, 0): 1}, {(0, 1): 1}, {(2, 2): 1, (1, 2): 1, (2, 0): -1}, {(2, 2): 1, (0, 2): 1, (2, 1): -1},
       {(0, 2): 1, (2, 0): 1}, {(2, 0): 1}, {(0, 2): 1}, {(1, 2): 1, (2, 1): 1}, {(2, 1): 1}, {(1, 2): 1})
RIDE = {0: {0: 1}, 3: {1: 1}, 5: {1: 1, 0: -1}, 6: {1: 1, 0: -1}, 7: {2: 1}, 10: {2: 1}, 11: {0: 1},
        12: {2: 1}, 14: {1: 1, 2: -1}}
RIDE_TILE = ({0: 0, 3: 1, 5: 5, 6: 5}, {0: 2, 3: 3, 5: 6, 6: 6, 7: 4, 10: 4, 11: 2, 12: 4, 14: 7})
AHEAD = ((3, 0), (3, 5), (0, 0), (0, 5), (0, 14), (0, 7), (1, 0), (1, 5))
S_AFTER = 320
AHEAD_N = (8, 8)
PLAN = (((0, 0), (0, 2), (0, 3), (0, 4), (0, 5)), ((1, 0), (1, 2), (1, 3), (1, 4), (1, 5), (1, 7)),
        ((1, 9), (1, 10), (1, 11), (1, 12)))
PLAN_LAST = (((0, 0), (0, 3), (0, 5), (0, 6)), ((1, 0), (1, 3), (1, 5), (1, 6), (1, 7)), ((1, 10), (1, 11), (1, 12)))
ORDER = (0, 4, 5, 2, 3, 1, 6, 9, 11, 10, 13, 12, 8, 14, 7)
TRIPLES = ((0, 1, 2), (4, 5, 3))
T_TRI, T_LAST, T_TAIL, N_TILES = (28, 43), 58, 65, 68


def _lin(terms, get):
    acc = None
    for key, sign in terms.items():
        v = get(key)
        acc = v if acc is None else (acc + v if sign > 0 else acc - v)
    return acc


def _combine(product, n, nr, paired, x2_last=False):
    m = functools.lru_cache(None)(product)

    def r(i):
        return m(i)[:nr]

    def x(i):
        return m(i)[nr:] if i in RIDE else m(i)
    if not paired:
        rid = [m(0) + m(5), m(3) - m(6)]
        if n == 3:
            v = m(10) + m(11)
            rid = [rid[0] + v, rid[1] + m(12) + m(14), m(7) + v + m(14)]
        return rid
    if not x2_last:
        x(0)
        p = x(4) - x(0)
        a = m(0) + m(5)
        w = x(4) + x(5) + x(2) - x(3)
        p = p + x(1)
        b = m(3) - m(6)
        rid, top, bot = [a[:nr], b[:nr]], [a[nr:], w], [p - x(6), b[nr:]]
        if n == 3:
            t = x(9) + x(11)
            t0 = t + x(10)
            v = r(10) + r(11)
            rid[0], top[0], bot[0] = rid[0] + v, top[0] + t0, bot[0] - t
            x(13), x(12)
            z = x(8) - x(11)
            u = x(12) - x(14)
            t1 = u + x(13)
            rid[1], top[1], bot[1] = rid[1] + r(12) + r(14), top[1] - u, bot[1] + t1
            c = m(7) + m(14)
            rid.append(c[:nr] + v)
            top.append(c[nr:] + t0)
            bot.append(z + t1)
        return [jnp.concatenate(p, axis=0) for p in zip(rid, top, bot)]
    a = m(0) + m(5)
    w = x(4) + x(5) - x(3)
    top = [a[nr:], w + x(2)]
    if n == 3:
        t = x(11) + x(9)
        t0 = t + x(10)
        v = r(10) + r(11)
        u = x(12) - x(14)
        top = [top[0] + t0, top[1] - u, x(7) + t0 + x(14)]
    b = m(3) - m(6)
    rid = [a[:nr], b[:nr]]
    bot = [x(4) - x(0) - x(6), b[nr:]]
    if n == 3:
        rid = [rid[0] + v, rid[1] + r(12) + r(14), r(7) + v + r(14)]
        t1 = u + x(13)
        bot = [bot[0] - t, bot[1] + t1, t1 - x(11) + x(8)]
    bot[0] = bot[0] + x(1)
    return [jnp.concatenate(p, axis=0) for p in zip(rid, top, bot)]


def _dft_constants():
    qb = CB // NQ
    hb = qb // 2
    n = np.arange(CB, dtype=np.float64)
    f = np.concatenate([q * qb + np.concatenate([np.arange(0, qb, 2), np.arange(1, qb, 2)])
                        for q in range(NQ)])
    w = np.pi * (2.0 * f + 1.0) / (2 * CB)
    ang = (w[:, None] * (n[None, :] - (CB - 1) / 4.0)).reshape(NQ, qb, CB)
    fwd = np.concatenate([np.cos(ang), -np.sin(ang)], axis=1)
    inv = np.zeros((NQ, 2, hb, CB))
    for p in range(NQ):
        m = (NQ - 1 - p) * hb + np.arange(hb)
        ang = (m[:, None] + 0.5) * w[None, :]
        inv[p, 0] = np.cos(ang) / CB
        inv[p, 1] = -np.sin(ang) / CB
    return fwd.astype(np.float32), inv.astype(np.float32)


def _flip_rows(x):
    i = jax.lax.broadcasted_iota(jnp.int32, (8, x.shape[1]), 0)
    out = []
    for r in range(x.shape[0] - 8, -8, -8):
        v = pltpu.roll(x[r:r + 8], 4, 0)
        for b in (2, 1):
            v = jnp.where((i & b) == 0, pltpu.roll(v, 8 - b, 0), pltpu.roll(v, b, 0))
        out.append(v)
    return jnp.concatenate(out, axis=0)


def _ln(x, eps=1e-5):
    d = x.shape[-1]
    m = jnp.sum(x, axis=-1, keepdims=True) * (1.0 / d)
    xc = x - m
    v = jnp.sum(xc * xc, axis=-1, keepdims=True) * (1.0 / d)
    return xc * jax.lax.rsqrt(v + eps)


def _dot(a, b):
    return jnp.dot(a, b, preferred_element_type=F32)


def _dot_nt(a, b):
    return jax.lax.dot_general(a, b, (((1,), (1,)), ((), ())), preferred_element_type=F32)


def _pack(x):
    return pltpu.bitcast(x.astype(BF16), U32)


def _unpack(x):
    return pltpu.bitcast(x, BF16)


def _tile(x, n):
    return x[:, n * 128:(n + 1) * 128]


def _ext(r):
    return _pack(jnp.concatenate(
        [r, _tile(r, 1) - _tile(r, 0), _tile(r, 3) - _tile(r, 2), _tile(r, 3) - _tile(r, 4)], axis=1))


def _in_order(actions):
    def body(i, c):
        for j, act in enumerate(actions):
            pl.when(i == j)(act)
        return c
    jax.lax.fori_loop(0, len(actions), body, 0)


def _kernel(x_hbm, mem0_hbm, wq_hbm, wk_hbm, wv_hbm, wo_hbm, k_hbm, v_hbm,
            sh_hbm, sk_hbm, sd_hbm, fwd_hbm, inv_hbm, o_hbm,
            sp_sc, kr_sc, wf_sc, x2_sc, y_sc, u_sc, op_sc, pre_sc, xn_sc, wa_sc, wb_sc, wo_sc, wc_sc,
            x_sc, v_sc, sk_sc, st_sc, out_sc, fwd_ref, inv_ref,
            k_sc, hp_sc, h_sc, co_sc, mem0_ref, sh_ref, sd_ref,
            never_sm, sem_x, sem_in, sem_w, sem_out,
            *, S, DM, H, DH, M, SEG):
    NSEG = S // SEG
    M2 = 2 * M
    S2 = SEG // 2
    R = M2 + 2 * SEG
    RH = M2 + SEG
    NB = S // CB
    QB = CB // NQ
    HB = QB // 2
    NT = DM // 128
    PH = PHI * UNROLL
    NRB = (NSEG - 1) // RB
    NPH = (NSEG - 1) // PH
    NG = H // HG
    NCH = 3 * NG
    NPASS = NPA // HG
    DH2 = DM // 2
    NU = 3 * NG
    DE = DM + 3 * 128
    KS = sh_ref.shape[0]
    UL = 2 * NQ + 1
    LN = pl.ds(0, DM)
    assert NT == 5 and HG == 8 and DH == 128 and 2 <= KS <= 8 and QB == SEG and NRB * RB == NSEG - 1 and NPH * PH == NSEG - 1 and NPASS == 2 and 2 * NRB >= NCH + 1

    mem0_copy = pltpu.make_async_copy(mem0_hbm, mem0_ref, sem_x.at[0])
    small = [pltpu.make_async_copy(s, d, sem_in.at[0]) for s, d in [
        (sh_hbm, sh_ref), (sd_hbm, sd_ref), (fwd_hbm, fwd_ref), (inv_hbm, inv_ref)]]

    def x_copy(b):
        if isinstance(b, int) and b == 0:
            rows = pl.ds(0, (RB + 1) * SEG)
        else:
            rows = pl.ds(pl.multiple_of((b * RB + 1) * SEG, SEG), RB * SEG)
        return pltpu.make_async_copy(x_hbm.at[rows], x_sc.at[rows, LN], sem_x.at[b])

    kb = (0, (UL + 1) * SEG, (UL + PH + 1) * SEG, S)
    sb = (0, 2, (PH + 2) // NQ + 2, NB)

    def in_copies(part):
        def rng(b):
            return pl.ds(b[part], b[part + 1] - b[part])
        sem = sem_in.at[part]
        return [
            pltpu.make_async_copy(k_hbm.at[rng(kb)],
                                  k_sc.at[pl.ds(KPAD + kb[part], kb[part + 1] - kb[part]), LN], sem),
            pltpu.make_async_copy(v_hbm.at[rng(kb)], v_sc.at[rng(kb), LN], sem),
        ] + [pltpu.make_async_copy(sk_hbm.at[:, pl.ds(c * CB, CB)], sk_sc.at[c], sem)
             for c in range(sb[part], sb[part + 1])]

    def w_copies(ci, dst=None, part=None):
        src = (wq_hbm, wk_hbm, wv_hbm)[ci // NG]
        dst = ci if dst is None else dst
        spans = {None: [(0, DM // 16)], 0: [(0, 16)], 1: [(16, DM // 16)]}[part]
        sem = sem_w.at[NCH + 1 if part == 1 else dst]
        return [pltpu.make_async_copy(
            src.at[pl.ds(lo, hi - lo), hf, :, pl.ds((ci % NG) * HG, HG), :],
            st_sc.at[dst, pl.ds(lo, hi - lo), :, pl.ds(hf * HG, HG), :], sem)
            for lo, hi in spans for hf in range(2)]

    wo_copy = pltpu.make_async_copy(wo_hbm, wo_sc, sem_w.at[NCH])

    def out_copy(lo, n):
        rows = pl.ds(lo * SEG if isinstance(lo, int) else pl.multiple_of(lo * SEG, SEG), n * SEG)
        return pltpu.make_async_copy(out_sc.at[rows, LN], o_hbm.at[rows], sem_out)

    def start_all(cps):
        def act():
            for cp in cps:
                cp.start()
        return act

    order = [[mem0_copy, x_copy(0)], w_copies(0, part=0), w_copies(0, part=1), [x_copy(1)], [x_copy(2)]]
    for ci in range(1, NCH):
        order.append(w_copies(ci) + ([x_copy(ci + 2)] if ci + 2 < NRB else []))
        if ci == NRB - 2:
            order.append(small + in_copies(0))
    order += [[wo_copy], in_copies(1), in_copies(2)]
    for i in range(0, len(order), 5):
        _in_order([start_all(cps) for cps in order[i:i + 5]])

    never_sm[0] = 0
    k_sc[0:KPAD, LN] = jnp.zeros((KPAD, DM), BF16)
    sp_sc[NB + 1] = jnp.zeros(sp_sc.shape[1:], F32)
    op_sc[...] = jnp.zeros(op_sc.shape, F32)
    x2_sc[...] = jnp.zeros(x2_sc.shape, F32)
    y_sc[2 * CB - SEG:, LN] = jnp.zeros((SEG, DM), F32)
    mem0_copy.wait()
    x_copy(0).wait()
    for sg in range(RB + 1):
        xn_sc[sg] = _ext(_ln(x_sc[sg * SEG:(sg + 1) * SEG, LN].astype(F32)))

    def clip(i, hi):
        return min(max(i, 0), hi) if isinstance(i, int) else jnp.clip(i, 0, hi)

    def scaled(i, m):
        return i * m if isinstance(i, int) else pl.multiple_of(i * m, m)

    def seg(i):
        return pl.ds(scaled(clip(i, NSEG - 1), SEG), SEG)

    def conv_u(s, ln=LN):
        r0 = scaled(clip(s, NSEG - 1), SEG)
        kk = k_sc[pl.ds(r0, KPAD + SEG), ln].astype(F32)[KPAD - 8:]

        def coef(j, rows):
            return jnp.concatenate([co_sc[j, :, ln]] * (rows // 8), axis=0)
        sft = [kk] + [pltpu.roll(kk, j, 0) for j in range(2, KS, 2)]
        ev = functools.reduce(jnp.add, [sft[j // 2][8:] * coef(j, SEG) for j in range(0, KS, 2)])
        od = functools.reduce(jnp.add, [sft[j // 2] * coef(j, SEG + 8) for j in range(1, KS, 2)])
        ks = ev + pltpu.roll(od, 1, 0)[8:]
        u = ks * v_sc[pl.ds(r0, SEG), ln].astype(F32)
        u_sc[pl.ds(r0, SEG), ln] = u.astype(BF16)
        return u

    def conv_fwd(c, q):
        cc = clip(c, NB - 1)
        f = fwd_ref[q]
        uf = _dot(f, u_sc[pl.ds(scaled(cc, CB), CB), LN])
        kf = _dot_nt(f, sk_sc[cc])
        return uf, kf

    def put_spec(cs, q, which, val):
        for n in range(NT):
            v = val[:, n * 128:(n + 1) * 128].reshape(2, QB // 8, 8, 128)
            sp_sc[cs, q, :, n, which:which + 2] = jnp.stack([v[0], v[1]], axis=1)

    def conv_spec(c, q):
        uf, kf = conv_fwd(c, q)
        cs = clip(c, NB)
        put_spec(cs, q, 0, uf)
        pk = kr_sc[q]
        kr_sc[q] = kf
        kp = jnp.concatenate([
            kf[0:HB] - pk[QB:QB + HB],
            kf[HB:QB] + pk[QB + HB:],
            kf[QB:QB + HB] + pk[0:HB],
            kf[QB + HB:] - pk[HB:QB]], axis=0)
        put_spec(cs, q, 2, kp)

    MAC_PIECES = [(rb, n) for rb in range(QB // 16) for n in range(NT)]

    def conv_mac(c, q, piece, nterms, link=None):
        rb2, n = piece
        cs = clip(c, NB)
        rbs = slice(2 * rb2, 2 * rb2 + 2)
        us, ks = [], []
        for j in range(nterms):
            if isinstance(cs, int):
                uj, kj = j, cs - j
            else:
                uj = jnp.minimum(j, cs)
                kj = jnp.where(cs - j >= 0, cs - j, NB + 1)
            us.append(sp_sc[uj, q, rbs, n, 0:2])
            ks.append(sp_sc[kj, q, rbs, n, 2:4])
        acc = []
        for rb in range(2):
            z = jnp.zeros((8, 128), F32) if not link else jnp.where(never_sm[0] > 0, link[0], 0.0)
            ar = ai = z
            for u, k in zip(us, ks):
                ar = ar + u[rb, 0] * k[rb, 0]
                ai = ai + u[rb, 0] * k[rb, 1]
                ar = ar - u[rb, 1] * k[rb, 1]
                ai = ai + u[rb, 1] * k[rb, 0]
            acc.append((ar, ai))
            if link is not None:
                link[:] = [ar]
        ln = slice(n * 128, (n + 1) * 128)
        w = jnp.concatenate([acc[0][0], acc[1][0], acc[0][1], acc[1][1]], axis=0).astype(BF16)
        wf_sc[c & 1, 0, q, rb2 * 16:rb2 * 16 + 16, ln] = w[0:16]
        wf_sc[c & 1, 1, q, rb2 * 16:rb2 * 16 + 16, ln] = w[16:]

    def conv_inv(tt, n):
        cb = tt // NQ
        p = tt % NQ
        ln = slice(n * 128, (n + 1) * 128)
        ev = _dot(inv_ref[p, 0], wf_sc[cb & 1, 0, :, :, ln].reshape(CB, 128))
        od = _dot(inv_ref[p, 1], wf_sc[cb & 1, 1, :, :, ln].reshape(CB, 128))
        sd = jnp.concatenate([co_sc[KS, :, ln]] * (HB // 8), axis=0)
        for r, val in ((p, _flip_rows(ev - od)), (2 * NQ - 1 - p, ev + od)):
            ur = scaled(clip(cb, NB - 1) * (2 * NQ) + r, HB)
            yr = scaled((cb & 1) * (2 * NQ) + r, HB)
            y_sc[pl.ds(yr, HB), ln] = val + u_sc[pl.ds(ur, HB), ln].astype(F32) * sd

    def y_seg(s):
        return y_sc[pl.ds(scaled(s & (2 * NQ - 1), SEG), SEG), LN]

    scale = DH ** -0.5
    cexp = scale * float(np.log2(np.e))

    def make_mask(n, x_layers, q0=0):
        qi = jax.lax.broadcasted_iota(jnp.int32, (n - q0, n), 0) + q0
        ki = jax.lax.broadcasted_iota(jnp.int32, (n - q0, n), 1)

        def layer(i):
            xl = jnp.where(i < M2 + SEG, x_layers[0], x_layers[-1])
            return jnp.where(i < M, 0, jnp.where(i < M2, 1, xl))
        same = layer(qi) == layer(ki)
        ok = same & ((qi < M2) | (ki < M2) | (qi >= ki))
        fill = jnp.where(same, -1e9 / scale, -jnp.inf).astype(F32)
        return ok, fill

    def probs(q, k, mask):
        ok, fill = mask
        s = _dot_nt(q, k)
        s = jnp.where(ok, s, fill)
        m = jnp.max(s, axis=-1, keepdims=True)
        p = jnp.exp2((s - m) * cexp)
        l = jnp.sum(p, axis=-1, keepdims=True)
        r = pl.reciprocal(l, approx=True)
        r = r * (2.0 - l * r)
        return (p * r).astype(BF16)

    def w_slot(ci):
        return (wb_sc, ci) if 1 <= ci < NRB - 1 else (wa_sc, max(ci - (NRB - 2), 0))

    def rows(*parts):
        return jnp.concatenate(parts, axis=0)

    def cols(*parts):
        return jnp.concatenate(parts, axis=1)

    def bf(*xs):
        return tuple(x.astype(BF16) for x in xs)

    def xn(s):
        return xn_sc[clip(s, NSEG - 1)]

    pending = []

    def packed_lhs(rid):
        def lhs(parts, i):
            return _unpack(cols(*[_tile(rid, 4 if i is None else RIDE_TILE[p][i]) for p in parts]))
        return lhs, 2 * rid.shape[0], False

    def value_lhs(rid, pair=None, pins=None):
        @functools.lru_cache(None)
        def lhs(parts, i):
            def one(p):
                if i is None:
                    return rows(*[_tile(r, 4) for r in (rid,) + (pair or ())])
                ps = [_lin(RIDE[i], lambda k: _tile(rid, 2 * p + k))] if i in RIDE else []
                if pair:
                    ps.append(_lin(LHS[i], lambda rk: _tile(pair[rk[0]], 2 * p + rk[1])))
                for v in (pins or {}).get((p, i), ()):
                    ps[-1] = rows(*([ps[-1][:-SEG]] if ps[-1].shape[0] > SEG else []),
                                  jnp.where(never_sm[0] > 0, v, ps[-1][-SEG:]))
                return rows(*ps)
            return cols(*[one(p) for p in parts]).astype(BF16)
        return lhs, rid.shape[0], pair is not None

    def product(tile, u, lhs, i):
        if pending and pending[0] <= 0:
            pending.pop()()
            pending.clear()
        base = T_TRI[u] if u < 2 else T_LAST
        if u == 3:
            a, w = lhs((0,), i), tile(4 * i + 1)
        elif i < 7:
            a, w = lhs((0, 1), i), rows(tile(4 * i + (0, 2, 3)[u]), tile(base + i))
        else:
            a, w = lhs((1,), i), tile(base + i)
        if pending:
            pending[0] -= a.shape[0] * w.size // (4 * 128 * 128)
        return _dot(a, w)

    def unit(tile, u, left, carry, ahead=()):
        lhs, nr, paired = left

        def comb(uu, n):
            return _combine(lambda i: ahead[uu, i] if (uu, i) in ahead else product(tile, uu, lhs, i),
                            n, nr, paired)
        if u == 2:
            c = comb(2, 2)
            return {6 + j: _dot(lhs((1,), None), tile(T_TAIL + j)) + c[j] for j in range(2)}
        if u == 0:
            carry[2], carry[3] = comb(3, 2)
        c = comb(u, 3)
        hs = TRIPLES[u]
        return {hs[0]: c[0], hs[1]: c[1], hs[2]: c[2] + carry.pop(hs[2])}

    def w_tiles(g, mats):
        slots = [w_slot(mi * NG + g) for mi in mats]
        return lambda i: _unpack(cols(*[ref[k, i] for ref, k in slots]))

    def attend(proj, n, mask, plan, hook=None, raw=False):
        D1, D2 = DIST
        full = n == R
        nr = M2 if full else n
        parts = {}
        os_ = {}

        def add_forms(g, hs, ids):
            for i in range(7 if len(hs) == 2 else 15):
                ps = []
                if i in RIDE:
                    ps.append(_lin(RIDE[i], lambda k: os_[hs[k]][:nr]))
                if full:
                    ps.append(_lin(LHS[i], lambda rk: os_[hs[rk[1]]][M2 + rk[0] * SEG:RH + rk[0] * SEG]))
                if ps:
                    a = rows(*ps).astype(BF16)
                    for part, tid in ids(i):
                        parts.setdefault((part, i), []).append((g, a, tid))

        def prod(key, g0, g1):
            if raw:
                a = cols(*[parts[h] for h in range(g0 * HG, g1 * HG)])
                return _dot(a, wo_sc[g0 * HG * DH:g1 * HG * DH, key * 128:(key + 1) * 128])
            sel = [p for p in parts[key] if g0 <= p[0] < g1]
            return _dot(cols(*[p[1] for p in sel]), _unpack(rows(*[wc_sc[p[0], p[2]] for p in sel])))

        qkvs = {}
        ps = {}
        m = {}
        for it in range(NU + D1 + D2):
            def scores(k=it - D1):
                if 0 <= k < NU:
                    ps[k] = {h: probs(q, kk, mask) for h, (q, kk, _) in qkvs[k].items()}
            if it < NU:
                pending[:] = [S_AFTER, scores]
                qkvs[it] = proj(it)
            if pending or it >= NU:
                pending.clear()
                scores()
            k = it - D1 - D2
            if 0 <= k < NU:
                g, u = divmod(k, 3)
                pk, qk = ps.pop(k), qkvs.pop(k)
                os_.update({h: _dot(pk[h], qk[h][2]) for h in pk})
                if raw:
                    parts.update({g * HG + h: os_[h].astype(BF16) for h in pk})
                elif u < 2:
                    add_forms(g, TRIPLES[u], lambda i: [(1, T_TRI[u] + i)] + ([(0, 4 * i + 2 * u)] if i < 7 else []))
                    if u == 1:
                        add_forms(g, (2, 3), lambda i: [(0, 4 * i + 1)])
                else:
                    add_forms(g, (6, 7), lambda i: [(0, 4 * i + 3), (1, T_LAST + i)])
                    for j in range(2):
                        parts[1, 7].append((g, os_[6 + j][:min(n, RH)].astype(BF16), T_TAIL + j))
                        if full:
                            parts[1, 8].append((g, os_[6 + j][RH:].astype(BF16), T_TAIL + j))
            if hook is not None:
                hook(it)
            j = it - (NU - 1)
            if j >= 0:
                for key in plan[j]:
                    m[key] = prod(key, 0, NG - 1)
        early = list(m)
        last = [(0, 1), (1, 1), (1, 8), (1, 13)]
        keys = range(NT) if raw else sorted(parts, key=lambda k: (k[1] == 6, ORDER.index(k[1]), k[0]))
        for key in keys:
            if key not in early and key not in last and (raw or key[1] != 6):
                m[key] = prod(key, 0, NG)
        for key in early:
            m[key] = prod(key, NG - 1, NG) + m[key]
        if raw:
            return cols(*[m[i] for i in range(NT)])
        for key in ((0, 6), (1, 6)):
            if key not in early:
                m[key] = prod(key, 0, NG)
        res = []
        for part in range(2):
            res += _combine(lambda i: m[part, i] if (part, i) in m else prod((part, i), 0, NG),
                            2 + part, nr, full, True)
        return cols(*res)

    def side2(t, a2):
        x3 = x2_sc[(t - 2) & 3] + a2
        x4 = x3 + _ln(x3) * y_seg(t - 2)
        out_sc[seg(t - 2), LN] = x4.astype(out_sc.dtype)
        return x4

    def finish(t, xr, yt, mem, a1):
        x1 = xr.astype(F32) + a1
        x2 = x1 + _ln(x1) * yt
        h_sc[...] = mem
        x2_sc[t & 3] = x2
        return x2

    def staged(make, pins):
        keys = ((0, 0), (1, 0), (0, 3), (1, 3), (0, 5))
        events = sorted({0} | {g0 + n // per for g0, _, per in pins for n in range(NT)})
        made = {}
        for e in events:
            act = {}
            for g0, v, per in pins:
                for n in range(NT):
                    if g0 + n // per <= e:
                        act.setdefault(keys[n], []).append(_tile(v, n))
            made[e] = make(act)
        return lambda k: made[max(e for e in events if e <= k)]

    def wait_chunk(ci):
        for cp in w_copies(0, ci):
            cp.wait()

    def w_block(ci, b):
        x = pltpu.bitcast(st_sc[ci, b], U32)
        sub = jax.lax.broadcasted_iota(jnp.int32, (8, DH), 0)
        res = []
        for par in range(2):
            v = [x[2 * i + par] for i in range(4)]
            for bit in (2, 1):
                keep = (sub & bit) == 0
                for i in range(4):
                    if not i & bit:
                        a, c = v[i], v[i + bit]
                        v[i] = jnp.where(keep, a, pltpu.roll(c, bit, 0))
                        v[i + bit] = jnp.where(keep, pltpu.roll(a, 8 - bit, 0), c)
            res.append(v)
        return res

    def rhs_tiles(part, plain, value, pack, swap):
        def one(i, base, hs):
            terms = {kj: sg for kj, sg in RHS[i].items() if max(kj) < len(hs)}

            def at(kj):
                k, j = kj[::-1] if swap else kj
                return base + k, hs[j]
            if len(terms) == 1:
                return plain(*at(next(iter(terms))))
            return pack(_lin(terms, lambda kj: value(*at(kj))))
        if part == 0:
            for p in range(4):
                for i in range(7):
                    yield 4 * i + p, one(i, 0, (2 * p, 2 * p + 1))
        else:
            for u in range(2):
                for i in range(15):
                    yield T_TRI[u] + i, one(i, 2, TRIPLES[u])
            for i in range(7):
                yield T_LAST + i, one(i, 2, (6, 7))
            for j in range(2):
                yield T_TAIL + j, plain(4, 6 + j)

    def relayout(ci, dst, slot, part, b):
        hi_m = U32(0xFFFF0000)
        t = {k: w_block(ci, 8 * k + b) for k in ((0, 1), (2, 3, 4))[part]}

        def plain(k, h):
            a, c = t[k][0][h // 2], t[k][1][h // 2]
            return (a >> 16) | (c & hi_m) if h % 2 else (a & U32(0xFFFF)) | (c << 16)

        @functools.lru_cache(None)
        def value(k, h):
            w = cols(t[k][0][h // 2], t[k][1][h // 2])
            return pltpu.bitcast(w & hi_m if h % 2 else w << 16, F32)

        def pack(v):
            r = pltpu.bitcast(v.astype(BF16).astype(F32), U32)
            return (r[:, :DH] >> 16) | r[:, DH:]
        out = dict(rhs_tiles(part, plain, value, pack, False))
        lo = min(out)
        dst[slot, lo:lo + len(out), pl.ds(scaled(b, 8), 8), :] = jnp.stack([out[i] for i in sorted(out)])

    def main(_, carry):
        for part in range(2):
            def relayout0(b, c, part=part):
                relayout(0, wa_sc, 0, part, b)
                return c
            with jax.named_scope("wait_w"):
                for cp in w_copies(0, part=part):
                    cp.wait()
            with jax.named_scope("relayout"):
                jax.lax.fori_loop(0, 8, relayout0, 0)

        def pro_stage(ps_, b):
            n = ps_ * NRB + b
            with jax.named_scope("wait_w"):
                if ps_ == 0:
                    @pl.when(b + 1 < NRB)
                    def _():
                        x_copy(b + 1).wait()

                @pl.when((n >= 2) & (n <= NCH))
                def _():
                    wait_chunk(n - 1)
            cr = jnp.clip(n - 1, 0, NCH - 1)
            dst, slot = (wb_sc, cr) if ps_ == 0 else (wa_sc, cr - (NRB - 2))
            bl = jnp.minimum(b + 1, NRB - 1)
            PW = PRO_PW
            npc = RB * S2 // PW
            assert npc * PW == RB * S2 and 3 * npc >= 16 + PRO_R0 and 2 * NRB > UL

            def body(i, c):
                s0 = b * RB + 1
                for sg in range(RB):
                    hp_sc[sg * S2:(sg + 1) * S2, :] = xn_sc[s0 + sg]
                for pi in range(npc):
                    carry = {}
                    for u in range(3):
                        pos = 3 * pi + u
                        hx = hp_sc[pi * PW:(pi + 1) * PW, :]
                        for k in range(max(RB, 2 * NT)):
                            if PRO_X0 + k * PRO_XN // PRO_XD != pos:
                                continue
                            if ps_ == 0 and k < RB:
                                sn = bl * RB + 1 + k
                                xv = _ext(_ln(x_sc[seg(sn), LN].astype(F32)))
                                xn_sc[sn] = xv
                                hx = rows(hx[:-S2], jnp.where(never_sm[0] > 0, xv, hx[-S2:]))
                            if ps_ == 1 and k < 2 * NT:
                                conv_u(jnp.minimum(2 * b + k // NT, UL),
                                       slice((k % NT) * 128, (k % NT + 1) * 128))
                        if 0 <= pos - PRO_R0 < 16:
                            relayout(cr, dst, slot, (pos - PRO_R0) % 2, (pos - PRO_R0) // 2)
                        for h, r in unit(w_tiles(ps_, (0,)), u, packed_lhs(hx), carry).items():
                            for a in range(0, 2 * PW, 16):
                                sg, off = divmod(2 * pi * PW + a, SEG)
                                pre_sc[s0 + sg, ps_ * HG + h, off:off + 16, :] = r[a:a + 16].astype(BF16)
                return c
            assert PRO_X0 + (max(RB, 2 * NT) - 1) * PRO_XN // PRO_XD < 3 * npc
            with jax.named_scope("fused"):
                jax.lax.fori_loop(0, never_sm[0] + 1, body, 0)

        for ps_ in range(NPASS):
            if ps_ == 1:
                with jax.named_scope("wait_in0"):
                    for cp in small + in_copies(0):
                        cp.wait()
                sh = sh_ref[...].astype(F32)
                for j in range(KS):
                    co_sc[j] = jnp.broadcast_to(sh[j:j + 1], (8, DM))
                co_sc[KS] = jnp.broadcast_to(sd_ref[...].astype(F32).reshape(1, DM), (8, DM))

            def blk(b, c, ps_=ps_):
                pro_stage(ps_, b)
                return c
            jax.lax.fori_loop(0, NRB, blk, 0)

        def warm_block0(q):
            uf, kf = conv_fwd(0, q)
            put_spec(0, q, 0, uf)
            put_spec(0, q, 2, kf)
            kr_sc[q] = kf
            ur, um, kr, km = uf[:QB], uf[QB:], kf[:QB], kf[QB:]
            wf_sc[0, 0, q] = (ur * kr - um * km).astype(BF16)
            wf_sc[0, 1, q] = (ur * km + um * kr).astype(BF16)

        def wo_operands(d):
            g, b, part = d // 16, (d % 16) // 2, d % 2
            z = jnp.minimum(never_sm[0], 0)

            def src(k, h):
                r = (g * HG + h) * DH + 16 * b
                return wo_sc[r:r + 16, k * 128:(k + 1) * 128]
            out = dict(rhs_tiles(part, lambda k, h: _pack(src(k, h)),
                                 functools.lru_cache(None)(lambda k, h: src(k, h).astype(F32)), _pack, True))
            lo = min(out)
            wc_sc[z + g, lo:lo + len(out), 8 * b:8 * b + 8, :] = jnp.stack([out[i] for i in sorted(out)])

        def plain_qkv(eq, ekv, k, carry, after=None):
            g, u = divmod(k, 3)
            res = []
            for mats, e in (((1,), ekv), ((2,), ekv), ((0,), eq)):
                res.append(unit(w_tiles(g, mats), u, e, carry.setdefault(mats, {})))
                if after is not None:
                    after(res[-1])
            return {h: bf(res[2][h], res[0][h], res[1][h]) for h in res[0]}

        with jax.named_scope("wait_wo"):
            wo_copy.wait()
        with jax.named_scope("step0"):
            mem0 = mem0_ref[...].astype(F32)
            e0 = packed_lhs(rows(_ext(rows(mem0, mem0)), xn(0)))

            todo = list(range(16 * NG))
            carry0 = {}

            def after0(res):
                z = jnp.minimum(never_sm[0], 0)
                for r in list(res.values())[:2]:
                    wc_sc[z, N_TILES - 1, 0:8, :] = pltpu.bitcast(r[0:8], U32)
                    if todo:
                        wo_operands(todo.pop(0))

            def hook0(it):
                if it < NQ:
                    warm_block0(it)
                if 5 <= it < 5 + NT:
                    for p in range(2):
                        conv_inv(p, it - 5)
            out = attend(lambda k: plain_qkv(e0, e0, k, carry0, after0), RH, make_mask(RH, (0,)),
                         ((0, 1), (2,), (3,)), hook0, True)
            assert not todo
            y0 = y_seg(0)
            for q in range(2):
                conv_spec(1, q)
            for n in range(NT):
                conv_inv(2, n)
            finish(0, x_sc[0:SEG, LN], y0, rows(out[0:M], mem0), out[M2:])
            for q in range(2):
                for piece in MAC_PIECES:
                    conv_mac(1, q, piece, 2)

        mask12 = make_mask(R, (0, 1))

        def step(t, x2):
            first = x2 is None
            c, q = (t + 1) // NQ + 1, (t + 1) % NQ
            mem = h_sc[...]
            n1 = _unpack(xn(t)[:, 0:DM]).astype(F32)
            lead = value_lhs(mem, (n1, None))[0]
            ahead = {ui: product(w_tiles(0, (1, 2)), ui[0], lead, ui[1]) for ui in AHEAD[:AHEAD_N[first]]}
            if first:
                x2 = x2_sc[(t - 1) & 3]
            conv_spec(c, q)
            link = []
            for piece in MAC_PIECES:
                conv_mac(c, q, piece, NB, link)
            n2 = _ln(x2)
            x4 = side2(t, op_sc[...])
            un = conv_u(t + UL)
            left = staged(lambda p: value_lhs(mem, (n1, n2), p), [(PIN_U, un, 2), (PIN_X4, x4, NT)])
            left_q = value_lhs(rows(mem, n2))
            carry = {}

            def proj(k):
                g, u = divmod(k, 3)
                pre = g * HG < NPA
                if pre:
                    qs = unit(w_tiles(g, (0,)), u, left_q, carry.setdefault("q", {}))
                rs = unit(w_tiles(g, (1, 2) if pre else (1, 2, 0)), u, left(k), carry.setdefault("kv", {}),
                          ahead if g == 0 else ())
                res = {}
                for h, r in rs.items():
                    if pre:
                        qq = rows(qs[h][:M2], pre_sc[t, g * HG + h].astype(F32), qs[h][M2:])
                    else:
                        qq = r[:, 2 * DH:]
                    res[h] = bf(qq, r[:, :DH], r[:, DH:2 * DH])
                return res

            held = {}

            def hook(it):
                if INV_AT <= it < INV_AT + NT:
                    conv_inv(t + 2, it - INV_AT)
                if it == NU:
                    held["x"] = x_sc[seg(t), LN]
                    held["y"] = y_seg(t)
            out = attend(proj, R, mask12, PLAN, hook)
            op_sc[...] = out[RH:]
            return finish(t, held["x"], held["y"], out[0:M2], out[M2:RH])

        def steps(i, carry):
            x2 = None
            for j in range(UNROLL):
                x2 = step(1 + i * UNROLL + j, x2)
            return carry

        def phase(p, carry):
            @pl.when(p == 1)
            def _():
                for cp in in_copies(2):
                    cp.wait()

            @pl.when(p >= 2)
            def _():
                out_copy((p - 2) * PH, PH).start()

            with jax.named_scope("steps"):
                jax.lax.fori_loop(p * PHI, (p + 1) * PHI, steps, 0)
            return carry

        for cp in in_copies(1):
            cp.wait()
        jax.lax.fori_loop(0, NPH, phase, 0)
        out_copy((NPH - 2) * PH, NSEG - 2 - (NPH - 2) * PH).start()

        with jax.named_scope("step_last"):
            x4 = side2(NSEG, op_sc[...])
            n2 = _ln(x2_sc[(NSEG - 1) & 3])
            left_q = value_lhs(n2)
            left = staged(lambda p: value_lhs(rows(h_sc[...], n2), None, p), [(PIN_X4, x4, NT)])
            carry1 = {}
            out = attend(lambda k: plain_qkv(left_q, left(k), k, carry1),
                         SEG, make_mask(RH, (1,), M2), PLAN_LAST)
            side2(NSEG + 1, out)
        out_copy(NSEG - 2, 2).start()
        out_copy(0, NSEG).wait()
        return carry

    jax.lax.fori_loop(0, never_sm[0] + 1, main, 0)


def pallas_interleave_layers__memory_aug_recurrent_mem_tr__ssm_conv_h3__prompt_kernel(
    A_x, A_mem0, A_Wq, A_Wk, A_Wv, A_Wo, A_seg_len,
    B_q, B_k, B_v, B_shift_k, B_ssm_k, B_ssm_D,
):
    del B_q
    seg = int(A_seg_len) if isinstance(A_seg_len, (int, np.integer)) else CB // NQ
    return _run(A_x, A_mem0, A_Wq, A_Wk, A_Wv, A_Wo, B_k, B_v, B_shift_k, B_ssm_k, B_ssm_D, SEG=seg)


@functools.partial(jax.jit, static_argnames=("SEG",))
def _run(A_x, A_mem0, A_Wq, A_Wk, A_Wv, A_Wo, B_k, B_v, B_shift_k, B_ssm_k, B_ssm_D, *, SEG):
    B, S, DM = A_x.shape
    assert B == 1
    H, DH = A_Wq.shape[1], A_Wq.shape[2]
    M = A_mem0.shape[1]
    KS = B_shift_k.shape[1]
    R = 2 * (M + SEG)
    NSEG = S // SEG
    NRB = (NSEG - 1) // RB
    NB = S // CB
    QB = CB // NQ
    NCH = 3 * H // HG
    DP = -(-DM // 256) * 256
    fwd, inv = _dft_constants()

    kern = functools.partial(_kernel, S=S, DM=DM, H=H, DH=DH, M=M, SEG=SEG)
    any_spec = pl.BlockSpec(memory_space=pl.ANY)
    out = pl.pallas_call(
        kern,
        out_shape=jax.ShapeDtypeStruct((S, DM), A_x.dtype),
        in_specs=[any_spec] * 13,
        out_specs=any_spec,
        scratch_shapes=[
            pltpu.VMEM((NB + 2, NQ, QB // 8, DM // 128, 4, 8, 128), F32),
            pltpu.VMEM((NQ, 2 * QB, DM), F32),
            pltpu.VMEM((2, 2, NQ, QB, DM), BF16),
            pltpu.VMEM((4, SEG, DM), F32),
            pltpu.VMEM((2 * CB, DP), F32),
            pltpu.VMEM((S, DP), BF16),
            pltpu.VMEM((SEG, DM), F32),
            pltpu.VMEM((NSEG, NPA, SEG, DH), BF16),
            pltpu.VMEM((NSEG, SEG // 2, DM + 384), U32),
            pltpu.VMEM((NCH - NRB + 2, N_TILES, 64, DH), U32),
            pltpu.VMEM((NRB - 1, N_TILES, 64, DH), U32),
            pltpu.VMEM((H * DH, DM), BF16),
            pltpu.VMEM((H // HG, N_TILES, 64, DH), U32),
            pltpu.VMEM((S, DP), BF16),
            pltpu.VMEM((S, DP), BF16),
            pltpu.VMEM((NB, DM, CB), BF16),
            pltpu.VMEM((NCH, DM // 16, 8, 2 * HG, DH), BF16),
            pltpu.VMEM((S, DP), A_x.dtype),
            pltpu.VMEM(fwd.shape, BF16),
            pltpu.VMEM(inv.shape, BF16),
            pltpu.VMEM((S + KPAD, DP), BF16),
            pltpu.VMEM((RB * SEG // 2, DM + 384), U32),
            pltpu.VMEM((2 * M, DM), F32),
            pltpu.VMEM((KS + 1, 8, DM), F32),
            pltpu.VMEM((M, DM), BF16),
            pltpu.VMEM((KS, DM), BF16),
            pltpu.VMEM((DM,), BF16),
            pltpu.SMEM((1,), jnp.int32),
            pltpu.SemaphoreType.DMA(((NSEG - 1) // RB,)),
            pltpu.SemaphoreType.DMA((3,)),
            pltpu.SemaphoreType.DMA((NCH + 2,)),
            pltpu.SemaphoreType.DMA(()),
        ],
        compiler_params=pltpu.CompilerParams(vmem_limit_bytes=120 * 1024 * 1024),
    )(
        A_x.reshape(S, DM), A_mem0.reshape(M, DM),
        *[w.reshape(DM // 16, 2, 8, H, DH) for w in (A_Wq, A_Wk, A_Wv)],
        A_Wo.reshape(H * DH, DM), B_k.reshape(S, DM), B_v.reshape(S, DM),
        B_shift_k.T, B_ssm_k, B_ssm_D,
        jnp.asarray(fwd, BF16), jnp.asarray(inv, BF16),
    )
    return out.reshape(B, S, DM)
```

```python
import functools

import numpy as np
import jax
import jax.numpy as jnp
import jax.experimental.pallas as pl
import jax.experimental.pallas.tpu as pltpu

F32 = jnp.float32
BF16 = jnp.bfloat16
U32 = jnp.uint32

CB = 128
NQ = 4
KPAD = 16
HG = 8
NPA = 16
RB = 9
PRO_PW, PRO_X0, PRO_XN, PRO_XD = 24, 3, 3, 2
PRO_T, WO_T = (20, 2820), (20, 6200)
UNROLL = 3
PHI = 3
INV_AT, PIN_U, PIN_X4 = 7, 2, 6

LHS = ({(0, 0): 1}, {(0, 0): 1, (1, 0): 1}, {(0, 1): 1, (1, 1): 1}, {(1, 1): 1}, {(0, 0): 1, (1, 1): 1},
       {(0, 1): 1, (0, 0): -1}, {(1, 1): 1, (1, 0): -1}, {(0, 2): 1}, {(1, 2): 1},
       {(0, 0): 1, (1, 0): 1, (1, 2): -1}, {(0, 2): 1, (1, 2): 1, (0, 0): -1, (1, 0): -1},
       {(1, 2): 1, (1, 0): -1}, {(0, 1): 1, (1, 1): 1, (0, 2): -1},
       {(0, 2): 1, (1, 2): 1, (0, 1): -1, (1, 1): -1}, {(0, 1): 1, (0, 2): -1})
RHS = ({(0, 0): 1, (1, 0): 1, (0, 2): -1}, {(0, 0): 1, (2, 0): 1, (0, 1): -1},
       {(1, 1): 1, (2, 1): 1, (1, 0): -1}, {(1, 1): 1, (0, 1): 1, (1, 2): -1}, {(0, 1): 1, (1, 0): 1},
       {(1, 0): 1}, {(0, 1): 1}, {(2, 2): 1, (1, 2): 1, (2, 0): -1}, {(2, 2): 1, (0, 2): 1, (2, 1): -1},
       {(0, 2): 1, (2, 0): 1}, {(2, 0): 1}, {(0, 2): 1}, {(1, 2): 1, (2, 1): 1}, {(2, 1): 1}, {(1, 2): 1})
RIDE = {0: {0: 1}, 3: {1: 1}, 5: {1: 1, 0: -1}, 6: {1: 1, 0: -1}, 7: {2: 1}, 10: {2: 1}, 11: {0: 1},
        12: {2: 1}, 14: {1: 1, 2: -1}}
RIDE_TILE = ({0: 0, 3: 1, 5: 5, 6: 5}, {0: 2, 3: 3, 5: 6, 6: 6, 7: 4, 10: 4, 11: 2, 12: 4, 14: 7})
AHEAD = ((3, 0), (3, 5), (0, 0), (0, 5), (0, 14), (0, 7), (1, 0), (1, 5))
SPLIT_PRE, SPLIT = ((1, 2),), ((1, 2, 0),)
LAT_S, GAP_S, LAT_P, LAT_O = 300, 200, 620, 250
AHEAD_N = (8, 8)
ORDER = (0, 4, 5, 2, 3, 1, 6, 9, 11, 10, 13, 12, 8, 14, 7)
TRIPLES = ((0, 1, 2), (4, 5, 3))
T_TRI, T_LAST, T_TAIL, N_TILES = (28, 43), 58, 65, 68


def _lin(terms, get):
    acc = None
    for key, sign in terms.items():
        v = get(key)
        acc = v if acc is None else (acc + v if sign > 0 else acc - v)
    return acc


def _combine(product, n, nr, paired, x2_last=False):
    m = functools.lru_cache(None)(product)

    def r(i):
        return m(i)[:nr]

    def x(i):
        return m(i)[nr:] if i in RIDE else m(i)
    if not paired:
        rid = [m(0) + m(5), m(3) - m(6)]
        if n == 3:
            v = m(10) + m(11)
            rid = [rid[0] + v, rid[1] + m(12) + m(14), m(7) + v + m(14)]
        return rid
    if not x2_last:
        x(0)
        p = x(4) - x(0)
        a = m(0) + m(5)
        w = x(4) + x(5) + x(2) - x(3)
        p = p + x(1)
        b = m(3) - m(6)
        rid, top, bot = [a[:nr], b[:nr]], [a[nr:], w], [p - x(6), b[nr:]]
        if n == 3:
            t = x(9) + x(11)
            t0 = t + x(10)
            v = r(10) + r(11)
            rid[0], top[0], bot[0] = rid[0] + v, top[0] + t0, bot[0] - t
            x(13), x(12)
            z = x(8) - x(11)
            u = x(12) - x(14)
            t1 = u + x(13)
            rid[1], top[1], bot[1] = rid[1] + r(12) + r(14), top[1] - u, bot[1] + t1
            c = m(7) + m(14)
            rid.append(c[:nr] + v)
            top.append(c[nr:] + t0)
            bot.append(z + t1)
        return [jnp.concatenate(p, axis=0) for p in zip(rid, top, bot)]
    a = m(0) + m(5)
    w = x(4) + x(5) - x(3)
    top = [a[nr:], w + x(2)]
    if n == 3:
        t = x(11) + x(9)
        t0 = t + x(10)
        v = r(10) + r(11)
        u = x(12) - x(14)
        top = [top[0] + t0, top[1] - u, x(7) + t0 + x(14)]
    b = m(3) - m(6)
    rid = [a[:nr], b[:nr]]
    bot = [x(4) - x(0) - x(6), b[nr:]]
    if n == 3:
        rid = [rid[0] + v, rid[1] + r(12) + r(14), r(7) + v + r(14)]
        t1 = u + x(13)
        bot = [bot[0] - t, bot[1] + t1, t1 - x(11) + x(8)]
    bot[0] = bot[0] + x(1)
    return [jnp.concatenate(p, axis=0) for p in zip(rid, top, bot)]


def _dft_constants():
    qb = CB // NQ
    hb = qb // 2
    n = np.arange(CB, dtype=np.float64)
    f = np.concatenate([q * qb + np.concatenate([np.arange(0, qb, 2), np.arange(1, qb, 2)])
                        for q in range(NQ)])
    w = np.pi * (2.0 * f + 1.0) / (2 * CB)
    ang = (w[:, None] * (n[None, :] - (CB - 1) / 4.0)).reshape(NQ, qb, CB)
    fwd = np.concatenate([np.cos(ang), -np.sin(ang)], axis=1)
    inv = np.zeros((NQ, 2, hb, CB))
    for p in range(NQ):
        m = (NQ - 1 - p) * hb + np.arange(hb)
        ang = (m[:, None] + 0.5) * w[None, :]
        inv[p, 0] = np.cos(ang) / CB
        inv[p, 1] = -np.sin(ang) / CB
    return fwd.astype(np.float32), inv.astype(np.float32)


def _flip_rows(x):
    i = jax.lax.broadcasted_iota(jnp.int32, (8, x.shape[1]), 0)
    out = []
    for r in range(x.shape[0] - 8, -8, -8):
        v = pltpu.roll(x[r:r + 8], 4, 0)
        for b in (2, 1):
            v = jnp.where((i & b) == 0, pltpu.roll(v, 8 - b, 0), pltpu.roll(v, b, 0))
        out.append(v)
    return jnp.concatenate(out, axis=0)


def _ln(x, eps=1e-5):
    d = x.shape[-1]
    m = jnp.sum(x, axis=-1, keepdims=True) * (1.0 / d)
    xc = x - m
    v = jnp.sum(xc * xc, axis=-1, keepdims=True) * (1.0 / d)
    return xc * jax.lax.rsqrt(v + eps)


def _dot(a, b):
    return jnp.dot(a, b, preferred_element_type=F32)


def _dot_nt(a, b):
    return jax.lax.dot_general(a, b, (((1,), (1,)), ((), ())), preferred_element_type=F32)


def _pack(x):
    return pltpu.bitcast(x.astype(BF16), U32)


def _unpack(x):
    return pltpu.bitcast(x, BF16)


def _tile(x, n):
    return x[:, n * 128:(n + 1) * 128]


def _ext(r):
    return _pack(jnp.concatenate(
        [r, _tile(r, 1) - _tile(r, 0), _tile(r, 3) - _tile(r, 2), _tile(r, 3) - _tile(r, 4)], axis=1))


def _in_order(actions):
    def body(i, c):
        for j, act in enumerate(actions):
            pl.when(i == j)(act)
        return c
    jax.lax.fori_loop(0, len(actions), body, 0)


def _kernel(x_hbm, mem0_hbm, wq_hbm, wk_hbm, wv_hbm, wo_hbm, k_hbm, v_hbm,
            sh_hbm, sk_hbm, sd_hbm, fwd_hbm, inv_hbm, o_hbm,
            sp_sc, kr_sc, wf_sc, x2_sc, y_sc, u_sc, op_sc, pre_sc, xn_sc, wa_sc, wb_sc, wo_sc, wc_sc,
            x_sc, v_sc, sk_sc, st_sc, out_sc, fwd_ref, inv_ref,
            k_sc, hp_sc, h_sc, co_sc, mem0_ref, sh_ref, sd_ref,
            never_sm, sem_x, sem_in, sem_w, sem_out,
            *, S, DM, H, DH, M, SEG):
    NSEG = S // SEG
    M2 = 2 * M
    S2 = SEG // 2
    R = M2 + 2 * SEG
    RH = M2 + SEG
    NB = S // CB
    QB = CB // NQ
    HB = QB // 2
    NT = DM // 128
    PH = PHI * UNROLL
    NRB = (NSEG - 1) // RB
    NPH = (NSEG - 1) // PH
    NG = H // HG
    NCH = 3 * NG
    NPASS = NPA // HG
    DH2 = DM // 2
    NU = 3 * NG
    DE = DM + 3 * 128
    KS = sh_ref.shape[0]
    UL = 2 * NQ + 1
    LN = pl.ds(0, DM)
    assert NT == 5 and HG == 8 and DH == 128 and 2 <= KS <= 8 and QB == SEG and NRB * RB == NSEG - 1 and NPH * PH == NSEG - 1 and NPASS == 2 and 2 * NRB >= NCH + 1

    mem0_copy = pltpu.make_async_copy(mem0_hbm, mem0_ref, sem_x.at[0])
    small = [pltpu.make_async_copy(s, d, sem_in.at[0]) for s, d in [
        (sh_hbm, sh_ref), (sd_hbm, sd_ref), (fwd_hbm, fwd_ref), (inv_hbm, inv_ref)]]

    def x_copy(b):
        if isinstance(b, int) and b == 0:
            rows = pl.ds(0, (RB + 1) * SEG)
        else:
            rows = pl.ds(pl.multiple_of((b * RB + 1) * SEG, SEG), RB * SEG)
        return pltpu.make_async_copy(x_hbm.at[rows], x_sc.at[rows, LN], sem_x.at[b])

    kb = (0, (UL + 1) * SEG, (UL + PH + 1) * SEG, S)
    sb = (0, 2, (PH + 2) // NQ + 2, NB)

    def in_copies(part):
        def rng(b):
            return pl.ds(b[part], b[part + 1] - b[part])
        sem = sem_in.at[part]
        return [
            pltpu.make_async_copy(k_hbm.at[rng(kb)],
                                  k_sc.at[pl.ds(KPAD + kb[part], kb[part + 1] - kb[part]), LN], sem),
            pltpu.make_async_copy(v_hbm.at[rng(kb)], v_sc.at[rng(kb), LN], sem),
        ] + [pltpu.make_async_copy(sk_hbm.at[:, pl.ds(c * CB, CB)], sk_sc.at[c], sem)
             for c in range(sb[part], sb[part + 1])]

    def w_copies(ci, dst=None, part=None):
        src = (wq_hbm, wk_hbm, wv_hbm)[ci // NG]
        dst = ci if dst is None else dst
        spans = {None: [(0, DM // 16)], 0: [(0, 16)], 1: [(16, DM // 16)]}[part]
        sem = sem_w.at[NCH + 1 if part == 1 else dst]
        return [pltpu.make_async_copy(
            src.at[pl.ds(lo, hi - lo), hf, :, pl.ds((ci % NG) * HG, HG), :],
            st_sc.at[dst, pl.ds(lo, hi - lo), :, pl.ds(hf * HG, HG), :], sem)
            for lo, hi in spans for hf in range(2)]

    wo_copy = pltpu.make_async_copy(wo_hbm, wo_sc, sem_w.at[NCH])

    def out_copy(lo, n):
        rows = pl.ds(lo * SEG if isinstance(lo, int) else pl.multiple_of(lo * SEG, SEG), n * SEG)
        return pltpu.make_async_copy(out_sc.at[rows, LN], o_hbm.at[rows], sem_out)

    def start_all(cps):
        def act():
            for cp in cps:
                cp.start()
        return act

    order = [[mem0_copy, x_copy(0)], w_copies(0, part=0), w_copies(0, part=1), [x_copy(1)], [x_copy(2)]]
    for ci in range(1, NCH):
        order.append(w_copies(ci) + ([x_copy(ci + 2)] if ci + 2 < NRB else []))
        if ci == NRB - 2:
            order.append(small + in_copies(0))
    order += [[wo_copy], in_copies(1), in_copies(2)]
    for i in range(0, len(order), 5):
        _in_order([start_all(cps) for cps in order[i:i + 5]])

    never_sm[0] = 0
    k_sc[0:KPAD, LN] = jnp.zeros((KPAD, DM), BF16)
    sp_sc[NB + 1] = jnp.zeros(sp_sc.shape[1:], F32)
    op_sc[...] = jnp.zeros(op_sc.shape, F32)
    x2_sc[...] = jnp.zeros(x2_sc.shape, F32)
    y_sc[2 * CB - SEG:, LN] = jnp.zeros((SEG, DM), F32)
    mem0_copy.wait()
    x_copy(0).wait()
    for sg in range(RB + 1):
        xn_sc[sg] = _ext(_ln(x_sc[sg * SEG:(sg + 1) * SEG, LN].astype(F32)))

    def clip(i, hi):
        return min(max(i, 0), hi) if isinstance(i, int) else jnp.clip(i, 0, hi)

    def scaled(i, m):
        return i * m if isinstance(i, int) else pl.multiple_of(i * m, m)

    def seg(i):
        return pl.ds(scaled(clip(i, NSEG - 1), SEG), SEG)

    def conv_u(s, ln=LN):
        r0 = scaled(clip(s, NSEG - 1), SEG)
        kk = k_sc[pl.ds(r0, KPAD + SEG), ln].astype(F32)[KPAD - 8:]

        def coef(j, rows):
            return jnp.concatenate([co_sc[j, :, ln]] * (rows // 8), axis=0)
        sft = [kk] + [pltpu.roll(kk, j, 0) for j in range(2, KS, 2)]
        ev = functools.reduce(jnp.add, [sft[j // 2][8:] * coef(j, SEG) for j in range(0, KS, 2)])
        od = functools.reduce(jnp.add, [sft[j // 2] * coef(j, SEG + 8) for j in range(1, KS, 2)])
        ks = ev + pltpu.roll(od, 1, 0)[8:]
        u = ks * v_sc[pl.ds(r0, SEG), ln].astype(F32)
        u_sc[pl.ds(r0, SEG), ln] = u.astype(BF16)
        return u

    def conv_fwd(c, q):
        cc = clip(c, NB - 1)
        f = fwd_ref[q]
        uf = _dot(f, u_sc[pl.ds(scaled(cc, CB), CB), LN])
        kf = _dot_nt(f, sk_sc[cc])
        return uf, kf

    def put_spec(cs, q, which, val):
        for n in range(NT):
            v = val[:, n * 128:(n + 1) * 128].reshape(2, QB // 8, 8, 128)
            sp_sc[cs, q, :, n, which:which + 2] = jnp.stack([v[0], v[1]], axis=1)

    def conv_spec(c, q):
        uf, kf = conv_fwd(c, q)
        cs = clip(c, NB)
        put_spec(cs, q, 0, uf)
        pk = kr_sc[q]
        kr_sc[q] = kf
        kp = jnp.concatenate([
            kf[0:HB] - pk[QB:QB + HB],
            kf[HB:QB] + pk[QB + HB:],
            kf[QB:QB + HB] + pk[0:HB],
            kf[QB + HB:] - pk[HB:QB]], axis=0)
        put_spec(cs, q, 2, kp)

    MAC_PIECES = [(rb, n) for rb in range(QB // 16) for n in range(NT)]

    def conv_mac(c, q, piece, nterms, link=None):
        rb2, n = piece
        cs = clip(c, NB)
        rbs = slice(2 * rb2, 2 * rb2 + 2)
        us, ks = [], []
        for j in range(nterms):
            if isinstance(cs, int):
                uj, kj = j, cs - j
            else:
                uj = jnp.minimum(j, cs)
                kj = jnp.where(cs - j >= 0, cs - j, NB + 1)
            us.append(sp_sc[uj, q, rbs, n, 0:2])
            ks.append(sp_sc[kj, q, rbs, n, 2:4])
        acc = []
        for rb in range(2):
            z = jnp.zeros((8, 128), F32) if not link else jnp.where(never_sm[0] > 0, link[0], 0.0)
            ar = ai = z
            for u, k in zip(us, ks):
                ar = ar + u[rb, 0] * k[rb, 0]
                ai = ai + u[rb, 0] * k[rb, 1]
                ar = ar - u[rb, 1] * k[rb, 1]
                ai = ai + u[rb, 1] * k[rb, 0]
            acc.append((ar, ai))
            if link is not None:
                link[:] = [ar]
        ln = slice(n * 128, (n + 1) * 128)
        w = jnp.concatenate([acc[0][0], acc[1][0], acc[0][1], acc[1][1]], axis=0).astype(BF16)
        wf_sc[c & 1, 0, q, rb2 * 16:rb2 * 16 + 16, ln] = w[0:16]
        wf_sc[c & 1, 1, q, rb2 * 16:rb2 * 16 + 16, ln] = w[16:]

    def conv_inv(tt, n):
        cb = tt // NQ
        p = tt % NQ
        ln = slice(n * 128, (n + 1) * 128)
        ev = _dot(inv_ref[p, 0], wf_sc[cb & 1, 0, :, :, ln].reshape(CB, 128))
        od = _dot(inv_ref[p, 1], wf_sc[cb & 1, 1, :, :, ln].reshape(CB, 128))
        sd = jnp.concatenate([co_sc[KS, :, ln]] * (HB // 8), axis=0)
        for r, val in ((p, _flip_rows(ev - od)), (2 * NQ - 1 - p, ev + od)):
            ur = scaled(clip(cb, NB - 1) * (2 * NQ) + r, HB)
            yr = scaled((cb & 1) * (2 * NQ) + r, HB)
            y_sc[pl.ds(yr, HB), ln] = val + u_sc[pl.ds(ur, HB), ln].astype(F32) * sd

    def y_seg(s):
        return y_sc[pl.ds(scaled(s & (2 * NQ - 1), SEG), SEG), LN]

    scale = DH ** -0.5
    cexp = scale * float(np.log2(np.e))

    def make_mask(n, x_layers, q0=0):
        qi = jax.lax.broadcasted_iota(jnp.int32, (n - q0, n), 0) + q0
        ki = jax.lax.broadcasted_iota(jnp.int32, (n - q0, n), 1)

        def layer(i):
            xl = jnp.where(i < M2 + SEG, x_layers[0], x_layers[-1])
            return jnp.where(i < M, 0, jnp.where(i < M2, 1, xl))
        same = layer(qi) == layer(ki)
        ok = same & ((qi < M2) | (ki < M2) | (qi >= ki))
        fill = jnp.where(same, -1e9 / scale, -jnp.inf).astype(F32)
        return ok, fill

    def probs(q, k, mask):
        ok, fill = mask
        s = _dot_nt(q, k)
        s = jnp.where(ok, s, fill)
        m = jnp.max(s, axis=-1, keepdims=True)
        p = jnp.exp2((s - m) * cexp)
        l = jnp.sum(p, axis=-1, keepdims=True)
        r = pl.reciprocal(l, approx=True)
        r = r * (2.0 - l * r)
        return (p * r).astype(BF16)

    def w_slot(ci):
        return (wb_sc, ci) if 1 <= ci < NRB - 1 else (wa_sc, max(ci - (NRB - 2), 0))

    def rows(*parts):
        return jnp.concatenate(parts, axis=0)

    def cols(*parts):
        return jnp.concatenate(parts, axis=1)

    def bf(*xs):
        return tuple(x.astype(BF16) for x in xs)

    def xn(s):
        return xn_sc[clip(s, NSEG - 1)]

    clock = [0]
    queue = []
    recent = [None]

    def later(delay, act):
        queue.append((clock[0] + delay, act))

    def run_due(force=False):
        while queue:
            item = min(queue, key=lambda it: it[0])
            if item[0] > clock[0] and not force:
                break
            queue.remove(item)
            clock[0] = max(clock[0], item[0])
            item[1]()

    def mm(a, w):
        run_due()
        clock[0] += a.shape[0] * w.size // (4 * 128 * 128)
        recent[0] = _dot(a, w)
        return recent[0]

    def spread(work, ref, slot, count, t0, t1):
        def act():
            ref[slot, N_TILES - 1, 0:8, :] = pltpu.bitcast(recent[0][0:8, 0:DH], U32)
            next(work)
        for i in range(count):
            later(t0 + i * (t1 - t0) // count, act)

    def packed_lhs(rid):
        def lhs(parts, i):
            return _unpack(cols(*[_tile(rid, 4 if i is None else RIDE_TILE[p][i]) for p in parts]))
        return lhs, 2 * rid.shape[0], False

    def value_lhs(rid, pair=None, pins=None):
        @functools.lru_cache(None)
        def lhs(parts, i):
            def one(p):
                if i is None:
                    return rows(*[_tile(r, 4) for r in (rid,) + (pair or ())])
                ps = [_lin(RIDE[i], lambda k: _tile(rid, 2 * p + k))] if i in RIDE else []
                if pair:
                    ps.append(_lin(LHS[i], lambda rk: _tile(pair[rk[0]], 2 * p + rk[1])))
                for v in (pins or {}).get((p, i), ()):
                    ps[-1] = rows(*([ps[-1][:-SEG]] if ps[-1].shape[0] > SEG else []),
                                  jnp.where(never_sm[0] > 0, v, ps[-1][-SEG:]))
                return rows(*ps)
            return cols(*[one(p) for p in parts]).astype(BF16)
        return lhs, rid.shape[0], pair is not None

    def product(tile, u, lhs, i):
        base = T_TRI[u] if u < 2 else T_LAST
        if u == 3:
            a, w = lhs((0,), i), tile(4 * i + 1)
        elif i < 7:
            a, w = lhs((0, 1), i), rows(tile(4 * i + (0, 2, 3)[u]), tile(base + i))
        else:
            a, w = lhs((1,), i), tile(base + i)
        return mm(a, w)

    def unit(tile, u, left, carry, ahead=()):
        lhs, nr, paired = left

        def comb(uu, n):
            return _combine(lambda i: ahead[uu, i] if (uu, i) in ahead else product(tile, uu, lhs, i),
                            n, nr, paired)
        if u == 2:
            c = comb(2, 2)
            return {6 + j: mm(lhs((1,), None), tile(T_TAIL + j)) + c[j] for j in range(2)}
        if u == 0:
            carry[2], carry[3] = comb(3, 2)
        c = comb(u, 3)
        hs = TRIPLES[u]
        return {hs[0]: c[0], hs[1]: c[1], hs[2]: c[2] + carry.pop(hs[2])}

    def w_tiles(g, mats):
        slots = [w_slot(mi * NG + g) for mi in mats]
        return lambda i: _unpack(cols(*[ref[k, i] for ref, k in slots]))

    def attend(proj, n, mask, hook=None, raw=False):
        full = n == R
        nr = M2 if full else n
        parts = {}
        os_ = {}

        def add_forms(g, hs, ids):
            for i in range(7 if len(hs) == 2 else 15):
                ps = []
                if i in RIDE:
                    ps.append(_lin(RIDE[i], lambda k: os_[hs[k]][:nr]))
                if full:
                    ps.append(_lin(LHS[i], lambda rk: os_[hs[rk[1]]][M2 + rk[0] * SEG:RH + rk[0] * SEG]))
                if ps:
                    a = rows(*ps).astype(BF16)
                    for part, tid in ids(i):
                        parts.setdefault((part, i), []).append((g, a, tid))

        def prod(key, g0, g1):
            if raw:
                a = cols(*[parts[h] for h in range(g0 * HG, g1 * HG)])
                return mm(a, wo_sc[g0 * HG * DH:g1 * HG * DH, key * 128:(key + 1) * 128])
            sel = [p for p in parts[key] if g0 <= p[0] < g1]
            return mm(cols(*[p[1] for p in sel]), _unpack(rows(*[wc_sc[p[0], p[2]] for p in sel])))

        def forms(g, u, hs):
            if raw:
                parts.update({g * HG + h: os_[h].astype(BF16) for h in hs})
            elif u < 2:
                add_forms(g, TRIPLES[u], lambda i: [(1, T_TRI[u] + i)] + ([(0, 4 * i + 2 * u)] if i < 7 else []))
                if u == 1:
                    add_forms(g, (2, 3), lambda i: [(0, 4 * i + 1)])
            else:
                add_forms(g, (6, 7), lambda i: [(0, 4 * i + 3), (1, T_LAST + i)])
                for j in range(2):
                    parts[1, 7].append((g, os_[6 + j][:min(n, RH)].astype(BF16), T_TAIL + j))
                    if full:
                        parts[1, 8].append((g, os_[6 + j][RH:].astype(BF16), T_TAIL + j))

        def head(g, u, h, qkv, done):
            def values(p):
                os_[h] = _dot(p, qkv[h][2])
                clock[0] += n // 4
                done.append(h)
                if len(done) == len(qkv):
                    forms(g, u, done)

            def scores():
                p = probs(qkv[h][0], qkv[h][1], mask)
                clock[0] += n // 4
                later(LAT_P, lambda: values(p))
            return scores

        for it in range(NU):
            qkv = proj(it)
            done = []
            for i, h in enumerate(qkv):
                later(LAT_S + i * GAP_S * n // R, head(*divmod(it, 3), h, qkv, done))
            if hook is not None:
                hook(it)
        last = [(0, 1), (1, 1), (1, 8), (1, 13)]
        keys = range(NT) if raw else sorted(parts, key=lambda k: (k[1] == 6, k[0], ORDER.index(k[1])))
        m = {}
        end = None
        for key in keys:
            if end is None and not queue:
                end = clock[0] + LAT_O
            if key not in last and (end is None or clock[0] < end):
                m[key] = prod(key, 0, NG - 1)
        run_due(True)
        if hook is not None:
            hook(NU)
        early = list(m)
        for key in keys:
            if key not in early and key not in last and (raw or key[1] != 6):
                m[key] = prod(key, 0, NG)
        for key in early:
            m[key] = prod(key, NG - 1, NG) + m[key]
        if raw:
            return cols(*[m[i] for i in range(NT)])
        for key in ((0, 6), (1, 6)):
            if key not in early:
                m[key] = prod(key, 0, NG)
        res = []
        for part in range(2):
            res += _combine(lambda i: m[part, i] if (part, i) in m else prod((part, i), 0, NG),
                            2 + part, nr, full, True)
        return cols(*res)

    def side2(t, a2):
        x3 = x2_sc[(t - 2) & 3] + a2
        x4 = x3 + _ln(x3) * y_seg(t - 2)
        out_sc[seg(t - 2), LN] = x4.astype(out_sc.dtype)
        return x4

    def finish(t, xr, yt, mem, a1):
        x1 = xr.astype(F32) + a1
        x2 = x1 + _ln(x1) * yt
        h_sc[...] = mem
        x2_sc[t & 3] = x2
        return x2

    def staged(make, pins):
        keys = ((0, 0), (1, 0), (0, 3), (1, 3), (0, 5))
        events = sorted({0} | {g0 + n // per for g0, _, per in pins for n in range(NT)})
        made = {}
        for e in events:
            act = {}
            for g0, v, per in pins:
                for n in range(NT):
                    if g0 + n // per <= e:
                        act.setdefault(keys[n], []).append(_tile(v, n))
            made[e] = make(act)
        return lambda k: made[max(e for e in events if e <= k)]

    def wait_chunk(ci):
        for cp in w_copies(0, ci):
            cp.wait()

    def w_block(ci, b):
        x = pltpu.bitcast(st_sc[ci, b], U32)
        sub = jax.lax.broadcasted_iota(jnp.int32, (8, DH), 0)
        res = []
        for par in range(2):
            v = [x[2 * i + par] for i in range(4)]
            for bit in (2, 1):
                keep = (sub & bit) == 0
                for i in range(4):
                    if not i & bit:
                        a, c = v[i], v[i + bit]
                        v[i] = jnp.where(keep, a, pltpu.roll(c, bit, 0))
                        v[i + bit] = jnp.where(keep, pltpu.roll(a, 8 - bit, 0), c)
            res.append(v)
        return res

    def rhs_tiles(part, plain, value, pack, swap):
        def one(i, base, hs):
            terms = {kj: sg for kj, sg in RHS[i].items() if max(kj) < len(hs)}

            def at(kj):
                k, j = kj[::-1] if swap else kj
                return base + k, hs[j]
            if len(terms) == 1:
                return plain(*at(next(iter(terms))))
            return pack(_lin(terms, lambda kj: value(*at(kj))))
        if part == 0:
            for p in range(4):
                for i in range(7):
                    yield 4 * i + p, one(i, 0, (2 * p, 2 * p + 1))
        else:
            for u in range(2):
                for i in range(15):
                    yield T_TRI[u] + i, one(i, 2, TRIPLES[u])
            for i in range(7):
                yield T_LAST + i, one(i, 2, (6, 7))
            for j in range(2):
                yield T_TAIL + j, plain(4, 6 + j)

    GROUPS = ((0, 12, T_TRI[0]), (T_TRI[0], T_TRI[1], T_LAST, T_TAIL + 2))
    NGRP = 8 * (len(GROUPS[0]) + len(GROUPS[1]) - 2)

    def put_tiles(dst, slot, r0, part, tiles):
        out = dict(tiles)
        for lo, hi in zip(GROUPS[part], GROUPS[part][1:]):
            dst[slot, lo:hi, pl.ds(r0, 8), :] = jnp.stack([out[i] for i in range(lo, hi)])
            yield

    def chunk_work(item):
        for b in range(8):
            for part in range(2):
                yield from item(part, b)

    def relayout(ci, dst, slot, part, b):
        hi_m = U32(0xFFFF0000)
        t = {k: w_block(ci, 8 * k + b) for k in ((0, 1), (2, 3, 4))[part]}

        def plain(k, h):
            a, c = t[k][0][h // 2], t[k][1][h // 2]
            return (a >> 16) | (c & hi_m) if h % 2 else (a & U32(0xFFFF)) | (c << 16)

        @functools.lru_cache(None)
        def value(k, h):
            w = cols(t[k][0][h // 2], t[k][1][h // 2])
            return pltpu.bitcast(w & hi_m if h % 2 else w << 16, F32)

        def pack(v):
            r = pltpu.bitcast(v.astype(BF16).astype(F32), U32)
            return (r[:, :DH] >> 16) | r[:, DH:]
        yield from put_tiles(dst, slot, scaled(b, 8), part, rhs_tiles(part, plain, value, pack, False))

    def main(_, carry):
        for part in range(2):
            def relayout0(b, c, part=part):
                list(relayout(0, wa_sc, 0, part, b))
                return c
            with jax.named_scope("wait_w"):
                for cp in w_copies(0, part=part):
                    cp.wait()
            with jax.named_scope("relayout"):
                jax.lax.fori_loop(0, 8, relayout0, 0)

        def pro_stage(ps_, b):
            n = ps_ * NRB + b
            with jax.named_scope("wait_w"):
                if ps_ == 0:
                    @pl.when(b + 1 < NRB)
                    def _():
                        x_copy(b + 1).wait()

                @pl.when((n >= 2) & (n <= NCH))
                def _():
                    wait_chunk(n - 1)
            cr = jnp.clip(n - 1, 0, NCH - 1)
            dst, slot = (wb_sc, cr) if ps_ == 0 else (wa_sc, cr - (NRB - 2))
            bl = jnp.minimum(b + 1, NRB - 1)
            PW = PRO_PW
            npc = RB * S2 // PW
            assert npc * PW == RB * S2 and 2 * NRB > UL

            def body(i, c):
                s0 = b * RB + 1
                for sg in range(RB):
                    hp_sc[sg * S2:(sg + 1) * S2, :] = xn_sc[s0 + sg]
                spread(chunk_work(functools.partial(relayout, cr, dst, slot)), dst, jnp.minimum(never_sm[0], 0), NGRP, *PRO_T)
                for pi in range(npc):
                    carry = {}
                    for u in range(3):
                        pos = 3 * pi + u
                        hx = hp_sc[pi * PW:(pi + 1) * PW, :]
                        for k in range(max(RB, 2 * NT)):
                            if PRO_X0 + k * PRO_XN // PRO_XD != pos:
                                continue
                            if ps_ == 0 and k < RB:
                                sn = bl * RB + 1 + k
                                xv = _ext(_ln(x_sc[seg(sn), LN].astype(F32)))
                                xn_sc[sn] = xv
                                hx = rows(hx[:-S2], jnp.where(never_sm[0] > 0, xv, hx[-S2:]))
                            if ps_ == 1 and k < 2 * NT:
                                conv_u(jnp.minimum(2 * b + k // NT, UL),
                                       slice((k % NT) * 128, (k % NT + 1) * 128))
                        for h, r in unit(w_tiles(ps_, (0,)), u, packed_lhs(hx), carry).items():
                            for a in range(0, 2 * PW, 16):
                                sg, off = divmod(2 * pi * PW + a, SEG)
                                pre_sc[s0 + sg, ps_ * HG + h, off:off + 16, :] = r[a:a + 16].astype(BF16)
                assert not queue
                return c
            assert PRO_X0 + (max(RB, 2 * NT) - 1) * PRO_XN // PRO_XD < 3 * npc
            with jax.named_scope("fused"):
                jax.lax.fori_loop(0, never_sm[0] + 1, body, 0)

        for ps_ in range(NPASS):
            if ps_ == 1:
                with jax.named_scope("wait_in0"):
                    for cp in small + in_copies(0):
                        cp.wait()
                sh = sh_ref[...].astype(F32)
                for j in range(KS):
                    co_sc[j] = jnp.broadcast_to(sh[j:j + 1], (8, DM))
                co_sc[KS] = jnp.broadcast_to(sd_ref[...].astype(F32).reshape(1, DM), (8, DM))

            def blk(b, c, ps_=ps_):
                pro_stage(ps_, b)
                return c
            jax.lax.fori_loop(0, NRB, blk, 0)

        def warm_block0(q):
            uf, kf = conv_fwd(0, q)
            put_spec(0, q, 0, uf)
            put_spec(0, q, 2, kf)
            kr_sc[q] = kf
            ur, um, kr, km = uf[:QB], uf[QB:], kf[:QB], kf[QB:]
            wf_sc[0, 0, q] = (ur * kr - um * km).astype(BF16)
            wf_sc[0, 1, q] = (ur * km + um * kr).astype(BF16)

        def wo_operands(g, part, b):
            def src(k, h):
                r = (g * HG + h) * DH + 16 * b
                return wo_sc[r:r + 16, k * 128:(k + 1) * 128]
            tiles = rhs_tiles(part, lambda k, h: _pack(src(k, h)),
                              functools.lru_cache(None)(lambda k, h: src(k, h).astype(F32)), _pack, True)
            yield from put_tiles(wc_sc, jnp.minimum(never_sm[0], 0) + g, 8 * b, part, tiles)

        def wo_work():
            for g in range(NG):
                yield from chunk_work(functools.partial(wo_operands, g))

        def plain_qkv(eq, ekv, k, carry):
            g, u = divmod(k, 3)
            res = []
            for mats, e in (((1,), ekv), ((2,), ekv), ((0,), eq)):
                res.append(unit(w_tiles(g, mats), u, e, carry.setdefault(mats, {})))
            return {h: bf(res[2][h], res[0][h], res[1][h]) for h in res[0]}

        with jax.named_scope("wait_wo"):
            wo_copy.wait()
        with jax.named_scope("step0"):
            mem0 = mem0_ref[...].astype(F32)
            e0 = packed_lhs(rows(_ext(rows(mem0, mem0)), xn(0)))

            carry0 = {}
            spread(wo_work(), wc_sc, jnp.minimum(never_sm[0], 0), NG * NGRP, *WO_T)

            def hook0(it):
                if it < NQ:
                    warm_block0(it)
                if 5 <= it < 5 + NT:
                    for p in range(2):
                        conv_inv(p, it - 5)
            out = attend(lambda k: plain_qkv(e0, e0, k, carry0), RH, make_mask(RH, (0,)), hook0, True)
            y0 = y_seg(0)
            for q in range(2):
                conv_spec(1, q)
            for n in range(NT):
                conv_inv(2, n)
            finish(0, x_sc[0:SEG, LN], y0, rows(out[0:M], mem0), out[M2:])
            for q in range(2):
                for piece in MAC_PIECES:
                    conv_mac(1, q, piece, 2)

        mask12 = make_mask(R, (0, 1))

        def step(t, x2):
            first = x2 is None
            c, q = (t + 1) // NQ + 1, (t + 1) % NQ
            mem = h_sc[...]
            n1 = _unpack(xn(t)[:, 0:DM]).astype(F32)
            lead = value_lhs(mem, (n1, None))[0]
            ahead = {ui: product(w_tiles(0, SPLIT_PRE[0]), ui[0], lead, ui[1]) for ui in AHEAD[:AHEAD_N[first]]}
            if first:
                x2 = x2_sc[(t - 1) & 3]
            conv_spec(c, q)
            link = []
            for piece in MAC_PIECES:
                conv_mac(c, q, piece, NB, link)
            n2 = _ln(x2)
            x4 = side2(t, op_sc[...])
            un = conv_u(t + UL)
            left = staged(lambda p: value_lhs(mem, (n1, n2), p), [(PIN_U, un, 2), (PIN_X4, x4, NT)])
            left_q = value_lhs(rows(mem, n2))
            carry = {}

            def proj(k):
                g, u = divmod(k, 3)
                pre = g * HG < NPA
                if pre:
                    qs = unit(w_tiles(g, (0,)), u, left_q, carry.setdefault("q", {}))
                got = {}
                for mats in (SPLIT_PRE if pre else SPLIT):
                    rs = unit(w_tiles(g, mats), u, left(k), carry.setdefault(mats, {}),
                              ahead if g == 0 and mats == SPLIT_PRE[0] else ())
                    for h, r in rs.items():
                        got.update({(h, mi): _tile(r, j) for j, mi in enumerate(mats)})
                res = {}
                for h in rs:
                    if pre:
                        got[h, 0] = rows(qs[h][:M2], pre_sc[t, g * HG + h].astype(F32), qs[h][M2:])
                    res[h] = bf(got[h, 0], got[h, 1], got[h, 2])
                return res

            held = {}

            def hook(it):
                if INV_AT <= it < INV_AT + NT:
                    conv_inv(t + 2, it - INV_AT)
                if it == NU:
                    held["x"] = x_sc[seg(t), LN]
                    held["y"] = y_seg(t)
            out = attend(proj, R, mask12, hook)
            op_sc[...] = out[RH:]
            return finish(t, held["x"], held["y"], out[0:M2], out[M2:RH])

        def steps(i, carry):
            x2 = None
            for j in range(UNROLL):
                x2 = step(1 + i * UNROLL + j, x2)
            return carry

        def phase(p, carry):
            @pl.when(p == 1)
            def _():
                for cp in in_copies(2):
                    cp.wait()

            @pl.when(p >= 2)
            def _():
                out_copy((p - 2) * PH, PH).start()

            with jax.named_scope("steps"):
                jax.lax.fori_loop(p * PHI, (p + 1) * PHI, steps, 0)
            return carry

        for cp in in_copies(1):
            cp.wait()
        jax.lax.fori_loop(0, NPH, phase, 0)
        out_copy((NPH - 2) * PH, NSEG - 2 - (NPH - 2) * PH).start()

        with jax.named_scope("step_last"):
            x4 = side2(NSEG, op_sc[...])
            n2 = _ln(x2_sc[(NSEG - 1) & 3])
            left_q = value_lhs(n2)
            left = staged(lambda p: value_lhs(rows(h_sc[...], n2), None, p), [(PIN_X4, x4, NT)])
            carry1 = {}
            out = attend(lambda k: plain_qkv(left_q, left(k), k, carry1),
                         SEG, make_mask(RH, (1,), M2))
            side2(NSEG + 1, out)
        out_copy(NSEG - 2, 2).start()
        out_copy(0, NSEG).wait()
        return carry

    jax.lax.fori_loop(0, never_sm[0] + 1, main, 0)


def pallas_interleave_layers__memory_aug_recurrent_mem_tr__ssm_conv_h3__prompt_kernel(
    A_x, A_mem0, A_Wq, A_Wk, A_Wv, A_Wo, A_seg_len,
    B_q, B_k, B_v, B_shift_k, B_ssm_k, B_ssm_D,
):
    del B_q
    seg = int(A_seg_len) if isinstance(A_seg_len, (int, np.integer)) else CB // NQ
    return _run(A_x, A_mem0, A_Wq, A_Wk, A_Wv, A_Wo, B_k, B_v, B_shift_k, B_ssm_k, B_ssm_D, SEG=seg)


@functools.partial(jax.jit, static_argnames=("SEG",))
def _run(A_x, A_mem0, A_Wq, A_Wk, A_Wv, A_Wo, B_k, B_v, B_shift_k, B_ssm_k, B_ssm_D, *, SEG):
    B, S, DM = A_x.shape
    assert B == 1
    H, DH = A_Wq.shape[1], A_Wq.shape[2]
    M = A_mem0.shape[1]
    KS = B_shift_k.shape[1]
    R = 2 * (M + SEG)
    NSEG = S // SEG
    NRB = (NSEG - 1) // RB
    NB = S // CB
    QB = CB // NQ
    NCH = 3 * H // HG
    DP = -(-DM // 256) * 256
    fwd, inv = _dft_constants()

    kern = functools.partial(_kernel, S=S, DM=DM, H=H, DH=DH, M=M, SEG=SEG)
    any_spec = pl.BlockSpec(memory_space=pl.ANY)
    out = pl.pallas_call(
        kern,
        out_shape=jax.ShapeDtypeStruct((S, DM), A_x.dtype),
        in_specs=[any_spec] * 13,
        out_specs=any_spec,
        scratch_shapes=[
            pltpu.VMEM((NB + 2, NQ, QB // 8, DM // 128, 4, 8, 128), F32),
            pltpu.VMEM((NQ, 2 * QB, DM), F32),
            pltpu.VMEM((2, 2, NQ, QB, DM), BF16),
            pltpu.VMEM((4, SEG, DM), F32),
            pltpu.VMEM((2 * CB, DP), F32),
            pltpu.VMEM((S, DP), BF16),
            pltpu.VMEM((SEG, DM), F32),
            pltpu.VMEM((NSEG, NPA, SEG, DH), BF16),
            pltpu.VMEM((NSEG, SEG // 2, DM + 384), U32),
            pltpu.VMEM((NCH - NRB + 2, N_TILES, 64, DH), U32),
            pltpu.VMEM((NRB - 1, N_TILES, 64, DH), U32),
            pltpu.VMEM((H * DH, DM), BF16),
            pltpu.VMEM((H // HG, N_TILES, 64, DH), U32),
            pltpu.VMEM((S, DP), BF16),
            pltpu.VMEM((S, DP), BF16),
            pltpu.VMEM((NB, DM, CB), BF16),
            pltpu.VMEM((NCH, DM // 16, 8, 2 * HG, DH), BF16),
            pltpu.VMEM((S, DP), A_x.dtype),
            pltpu.VMEM(fwd.shape, BF16),
            pltpu.VMEM(inv.shape, BF16),
            pltpu.VMEM((S + KPAD, DP), BF16),
            pltpu.VMEM((RB * SEG // 2, DM + 384), U32),
            pltpu.VMEM((2 * M, DM), F32),
            pltpu.VMEM((KS + 1, 8, DM), F32),
            pltpu.VMEM((M, DM), BF16),
            pltpu.VMEM((KS, DM), BF16),
            pltpu.VMEM((DM,), BF16),
            pltpu.SMEM((1,), jnp.int32),
            pltpu.SemaphoreType.DMA(((NSEG - 1) // RB,)),
            pltpu.SemaphoreType.DMA((3,)),
            pltpu.SemaphoreType.DMA((NCH + 2,)),
            pltpu.SemaphoreType.DMA(()),
        ],
        compiler_params=pltpu.CompilerParams(vmem_limit_bytes=120 * 1024 * 1024),
    )(
        A_x.reshape(S, DM), A_mem0.reshape(M, DM),
        *[w.reshape(DM // 16, 2, 8, H, DH) for w in (A_Wq, A_Wk, A_Wv)],
        A_Wo.reshape(H * DH, DM), B_k.reshape(S, DM), B_v.reshape(S, DM),
        B_shift_k.T, B_ssm_k, B_ssm_D,
        jnp.asarray(fwd, BF16), jnp.asarray(inv, BF16),
    )
    return out.reshape(B, S, DM)
```

```python
import functools

import numpy as np
import jax
import jax.numpy as jnp
import jax.experimental.pallas as pl
import jax.experimental.pallas.tpu as pltpu

F32 = jnp.float32
BF16 = jnp.bfloat16
U32 = jnp.uint32

CB = 128
NQ = 4
KPAD = 16
HG = 8
NPA = 16
RB = 9
PRO_PW, PRO_X0, PRO_XN, PRO_XD = 24, 3, 3, 2
PRO_T, WO_T = (20, 2820), (20, 6200)
UNROLL = 3
PHI = 3
INV_AT, PIN_U, PIN_X4 = 7, 2, 6

LHS = ({(0, 0): 1}, {(0, 0): 1, (1, 0): 1}, {(0, 1): 1, (1, 1): 1}, {(1, 1): 1}, {(0, 0): 1, (1, 1): 1},
       {(0, 1): 1, (0, 0): -1}, {(1, 1): 1, (1, 0): -1}, {(0, 2): 1}, {(1, 2): 1},
       {(0, 0): 1, (1, 0): 1, (1, 2): -1}, {(0, 2): 1, (1, 2): 1, (0, 0): -1, (1, 0): -1},
       {(1, 2): 1, (1, 0): -1}, {(0, 1): 1, (1, 1): 1, (0, 2): -1},
       {(0, 2): 1, (1, 2): 1, (0, 1): -1, (1, 1): -1}, {(0, 1): 1, (0, 2): -1})
RHS = ({(0, 0): 1, (1, 0): 1, (0, 2): -1}, {(0, 0): 1, (2, 0): 1, (0, 1): -1},
       {(1, 1): 1, (2, 1): 1, (1, 0): -1}, {(1, 1): 1, (0, 1): 1, (1, 2): -1}, {(0, 1): 1, (1, 0): 1},
       {(1, 0): 1}, {(0, 1): 1}, {(2, 2): 1, (1, 2): 1, (2, 0): -1}, {(2, 2): 1, (0, 2): 1, (2, 1): -1},
       {(0, 2): 1, (2, 0): 1}, {(2, 0): 1}, {(0, 2): 1}, {(1, 2): 1, (2, 1): 1}, {(2, 1): 1}, {(1, 2): 1})
RIDE = {0: {0: 1}, 3: {1: 1}, 5: {1: 1, 0: -1}, 6: {1: 1, 0: -1}, 7: {2: 1}, 10: {2: 1}, 11: {0: 1},
        12: {2: 1}, 14: {1: 1, 2: -1}}
RIDE_TILE = ({0: 0, 3: 1, 5: 5, 6: 5}, {0: 2, 3: 3, 5: 6, 6: 6, 7: 4, 10: 4, 11: 2, 12: 4, 14: 7})
AHEAD = ((3, 0), (3, 5), (0, 0), (0, 5), (0, 14), (0, 7), (1, 0), (1, 5))
LAT_S, GAP_S, LAT_P, LAT_O = 300, 200, 620, 250
ORDER = (0, 4, 5, 2, 3, 1, 6, 9, 11, 10, 13, 12, 8, 14, 7)
TRIPLES = ((0, 1, 2), (4, 5, 3))
T_TRI, T_LAST, T_TAIL, N_TILES = (28, 43), 58, 65, 68


def _lin(terms, get):
    acc = None
    for key, sign in terms.items():
        v = get(key)
        acc = v if acc is None else (acc + v if sign > 0 else acc - v)
    return acc


def _combine(product, n, nr, paired, x2_last=False):
    m = functools.lru_cache(None)(product)

    def r(i):
        return m(i)[:nr]

    def x(i):
        return m(i)[nr:] if i in RIDE else m(i)
    if not paired:
        rid = [m(0) + m(5), m(3) - m(6)]
        if n == 3:
            v = m(10) + m(11)
            rid = [rid[0] + v, rid[1] + m(12) + m(14), m(7) + v + m(14)]
        return rid
    if not x2_last:
        x(0)
        p = x(4) - x(0)
        a = m(0) + m(5)
        w = x(4) + x(5) + x(2) - x(3)
        p = p + x(1)
        b = m(3) - m(6)
        rid, top, bot = [a[:nr], b[:nr]], [a[nr:], w], [p - x(6), b[nr:]]
        if n == 3:
            t = x(9) + x(11)
            t0 = t + x(10)
            v = r(10) + r(11)
            rid[0], top[0], bot[0] = rid[0] + v, top[0] + t0, bot[0] - t
            x(13), x(12)
            z = x(8) - x(11)
            u = x(12) - x(14)
            t1 = u + x(13)
            rid[1], top[1], bot[1] = rid[1] + r(12) + r(14), top[1] - u, bot[1] + t1
            c = m(7) + m(14)
            rid.append(c[:nr] + v)
            top.append(c[nr:] + t0)
            bot.append(z + t1)
        return [jnp.concatenate(p, axis=0) for p in zip(rid, top, bot)]
    a = m(0) + m(5)
    w = x(4) + x(5) - x(3)
    top = [a[nr:], w + x(2)]
    if n == 3:
        t = x(11) + x(9)
        t0 = t + x(10)
        v = r(10) + r(11)
        u = x(12) - x(14)
        top = [top[0] + t0, top[1] - u, x(7) + t0 + x(14)]
    b = m(3) - m(6)
    rid = [a[:nr], b[:nr]]
    bot = [x(4) - x(0) - x(6), b[nr:]]
    if n == 3:
        rid = [rid[0] + v, rid[1] + r(12) + r(14), r(7) + v + r(14)]
        t1 = u + x(13)
        bot = [bot[0] - t, bot[1] + t1, t1 - x(11) + x(8)]
    bot[0] = bot[0] + x(1)
    return [jnp.concatenate(p, axis=0) for p in zip(rid, top, bot)]


def _dft_constants():
    qb = CB // NQ
    hb = qb // 2
    n = np.arange(CB, dtype=np.float64)
    f = np.concatenate([q * qb + np.concatenate([np.arange(0, qb, 2), np.arange(1, qb, 2)])
                        for q in range(NQ)])
    w = np.pi * (2.0 * f + 1.0) / (2 * CB)
    ang = (w[:, None] * (n[None, :] - (CB - 1) / 4.0)).reshape(NQ, qb, CB)
    fwd = np.concatenate([np.cos(ang), -np.sin(ang)], axis=1)
    inv = np.zeros((NQ, 2, hb, CB))
    for p in range(NQ):
        m = (NQ - 1 - p) * hb + np.arange(hb)
        ang = (m[:, None] + 0.5) * w[None, :]
        inv[p, 0] = np.cos(ang) / CB
        inv[p, 1] = -np.sin(ang) / CB
    return fwd.astype(np.float32), inv.astype(np.float32)


def _flip_rows(x):
    i = jax.lax.broadcasted_iota(jnp.int32, (8, x.shape[1]), 0)
    out = []
    for r in range(x.shape[0] - 8, -8, -8):
        v = pltpu.roll(x[r:r + 8], 4, 0)
        for b in (2, 1):
            v = jnp.where((i & b) == 0, pltpu.roll(v, 8 - b, 0), pltpu.roll(v, b, 0))
        out.append(v)
    return jnp.concatenate(out, axis=0)


def _ln(x, eps=1e-5):
    d = x.shape[-1]
    m = jnp.sum(x, axis=-1, keepdims=True) * (1.0 / d)
    xc = x - m
    v = jnp.sum(xc * xc, axis=-1, keepdims=True) * (1.0 / d)
    return xc * jax.lax.rsqrt(v + eps)


def _dot(a, b):
    return jnp.dot(a, b, preferred_element_type=F32)


def _dot_nt(a, b):
    return jax.lax.dot_general(a, b, (((1,), (1,)), ((), ())), preferred_element_type=F32)


def _pack(x):
    return pltpu.bitcast(x.astype(BF16), U32)


def _unpack(x):
    return pltpu.bitcast(x, BF16)


def _tile(x, n):
    return x[:, n * 128:(n + 1) * 128]


def _ext(r):
    return _pack(jnp.concatenate(
        [r, _tile(r, 1) - _tile(r, 0), _tile(r, 3) - _tile(r, 2), _tile(r, 3) - _tile(r, 4)], axis=1))


def _in_order(actions):
    def body(i, c):
        for j, act in enumerate(actions):
            pl.when(i == j)(act)
        return c
    jax.lax.fori_loop(0, len(actions), body, 0)


def _kernel(x_hbm, mem0_hbm, wq_hbm, wk_hbm, wv_hbm, wo_hbm, k_hbm, v_hbm,
            sh_hbm, sk_hbm, sd_hbm, fwd_hbm, inv_hbm, o_hbm,
            sp_sc, kr_sc, wf_sc, x2_sc, y_sc, u_sc, op_sc, pre_sc, xn_sc, wa_sc, wb_sc, wo_sc, wc_sc,
            x_sc, v_sc, sk_sc, st_sc, out_sc, fwd_ref, inv_ref,
            k_sc, hp_sc, h_sc, co_sc, mem0_ref, sh_ref, sd_ref,
            never_sm, sem_x, sem_in, sem_w, sem_out,
            *, S, DM, H, DH, M, SEG):
    NSEG = S // SEG
    M2 = 2 * M
    S2 = SEG // 2
    R = M2 + 2 * SEG
    RH = M2 + SEG
    NB = S // CB
    QB = CB // NQ
    HB = QB // 2
    NT = DM // 128
    PH = PHI * UNROLL
    NRB = (NSEG - 1) // RB
    NPH = (NSEG - 1) // PH
    NG = H // HG
    NCH = 3 * NG
    NPASS = NPA // HG
    NU = 3 * NG
    KS = sh_ref.shape[0]
    UL = 2 * NQ + 1
    LN = pl.ds(0, DM)
    assert NT == 5 and HG == 8 and DH == 128 and 2 <= KS <= 8 and QB == SEG and NRB * RB == NSEG - 1 and NPH * PH == NSEG - 1 and NPASS == 2 and 2 * NRB >= NCH + 1

    mem0_copy = pltpu.make_async_copy(mem0_hbm, mem0_ref, sem_x.at[0])
    small = [pltpu.make_async_copy(s, d, sem_in.at[0]) for s, d in [
        (sh_hbm, sh_ref), (sd_hbm, sd_ref), (fwd_hbm, fwd_ref), (inv_hbm, inv_ref)]]

    def x_copy(b):
        if isinstance(b, int) and b == 0:
            rows = pl.ds(0, (RB + 1) * SEG)
        else:
            rows = pl.ds(pl.multiple_of((b * RB + 1) * SEG, SEG), RB * SEG)
        return pltpu.make_async_copy(x_hbm.at[rows], x_sc.at[rows, LN], sem_x.at[b])

    kb = (0, (UL + 1) * SEG, (UL + PH + 1) * SEG, S)
    sb = (0, 2, (PH + 2) // NQ + 2, NB)

    def in_copies(part):
        def rng(b):
            return pl.ds(b[part], b[part + 1] - b[part])
        sem = sem_in.at[part]
        return [
            pltpu.make_async_copy(k_hbm.at[rng(kb)],
                                  k_sc.at[pl.ds(KPAD + kb[part], kb[part + 1] - kb[part]), LN], sem),
            pltpu.make_async_copy(v_hbm.at[rng(kb)], v_sc.at[rng(kb), LN], sem),
        ] + [pltpu.make_async_copy(sk_hbm.at[:, pl.ds(c * CB, CB)], sk_sc.at[c], sem)
             for c in range(sb[part], sb[part + 1])]

    def w_copies(ci, dst=None, part=None):
        src = (wq_hbm, wk_hbm, wv_hbm)[ci // NG]
        dst = ci if dst is None else dst
        spans = {None: [(0, DM // 16)], 0: [(0, 16)], 1: [(16, DM // 16)]}[part]
        sem = sem_w.at[NCH + 1 if part == 1 else dst]
        return [pltpu.make_async_copy(
            src.at[pl.ds(lo, hi - lo), hf, :, pl.ds((ci % NG) * HG, HG), :],
            st_sc.at[dst, pl.ds(lo, hi - lo), :, pl.ds(hf * HG, HG), :], sem)
            for lo, hi in spans for hf in range(2)]

    wo_copy = pltpu.make_async_copy(wo_hbm, wo_sc, sem_w.at[NCH])

    def out_copy(lo, n):
        rows = pl.ds(lo * SEG if isinstance(lo, int) else pl.multiple_of(lo * SEG, SEG), n * SEG)
        return pltpu.make_async_copy(out_sc.at[rows, LN], o_hbm.at[rows], sem_out)

    def start_all(cps):
        def act():
            for cp in cps:
                cp.start()
        return act

    order = [[mem0_copy, x_copy(0)], w_copies(0, part=0), w_copies(0, part=1), [x_copy(1)], [x_copy(2)]]
    for ci in range(1, NCH):
        order.append(w_copies(ci) + ([x_copy(ci + 2)] if ci + 2 < NRB else []))
        if ci == NRB - 2:
            order.append(small + in_copies(0))
    order += [[wo_copy], in_copies(1), in_copies(2)]
    for i in range(0, len(order), 5):
        _in_order([start_all(cps) for cps in order[i:i + 5]])

    never_sm[0] = 0
    k_sc[0:KPAD, LN] = jnp.zeros((KPAD, DM), BF16)
    sp_sc[NB + 1] = jnp.zeros(sp_sc.shape[1:], F32)
    op_sc[...] = jnp.zeros(op_sc.shape, F32)
    x2_sc[...] = jnp.zeros(x2_sc.shape, F32)
    y_sc[2 * CB - SEG:, LN] = jnp.zeros((SEG, DM), F32)
    mem0_copy.wait()
    x_copy(0).wait()
    for sg in range(RB + 1):
        xn_sc[sg] = _ext(_ln(x_sc[sg * SEG:(sg + 1) * SEG, LN].astype(F32)))

    def clip(i, hi):
        return min(max(i, 0), hi) if isinstance(i, int) else jnp.clip(i, 0, hi)

    def scaled(i, m):
        return i * m if isinstance(i, int) else pl.multiple_of(i * m, m)

    def seg(i):
        return pl.ds(scaled(clip(i, NSEG - 1), SEG), SEG)

    def conv_u(s, ln=LN):
        r0 = scaled(clip(s, NSEG - 1), SEG)
        kk = k_sc[pl.ds(r0, KPAD + SEG), ln].astype(F32)[KPAD - 8:]

        def coef(j, rows):
            return jnp.concatenate([co_sc[j, :, ln]] * (rows // 8), axis=0)
        sft = [kk] + [pltpu.roll(kk, j, 0) for j in range(2, KS, 2)]
        ev = functools.reduce(jnp.add, [sft[j // 2][8:] * coef(j, SEG) for j in range(0, KS, 2)])
        od = functools.reduce(jnp.add, [sft[j // 2] * coef(j, SEG + 8) for j in range(1, KS, 2)])
        ks = ev + pltpu.roll(od, 1, 0)[8:]
        u = ks * v_sc[pl.ds(r0, SEG), ln].astype(F32)
        u_sc[pl.ds(r0, SEG), ln] = u.astype(BF16)
        return u

    def conv_fwd(c, q):
        cc = clip(c, NB - 1)
        f = fwd_ref[q]
        uf = _dot(f, u_sc[pl.ds(scaled(cc, CB), CB), LN])
        kf = _dot_nt(f, sk_sc[cc])
        return uf, kf

    def put_spec(cs, q, which, val):
        for n in range(NT):
            v = val[:, n * 128:(n + 1) * 128].reshape(2, QB // 8, 8, 128)
            sp_sc[cs, q, :, n, which:which + 2] = jnp.stack([v[0], v[1]], axis=1)

    def conv_spec(c, q):
        uf, kf = conv_fwd(c, q)
        cs = clip(c, NB)
        put_spec(cs, q, 0, uf)
        pk = kr_sc[q]
        kr_sc[q] = kf
        kp = jnp.concatenate([
            kf[0:HB] - pk[QB:QB + HB],
            kf[HB:QB] + pk[QB + HB:],
            kf[QB:QB + HB] + pk[0:HB],
            kf[QB + HB:] - pk[HB:QB]], axis=0)
        put_spec(cs, q, 2, kp)

    MAC_PIECES = [(rb, n) for rb in range(QB // 16) for n in range(NT)]

    def conv_mac(c, q, piece, nterms, link=None):
        rb2, n = piece
        cs = clip(c, NB)
        rbs = slice(2 * rb2, 2 * rb2 + 2)
        us, ks = [], []
        for j in range(nterms):
            if isinstance(cs, int):
                uj, kj = j, cs - j
            else:
                uj = jnp.minimum(j, cs)
                kj = jnp.where(cs - j >= 0, cs - j, NB + 1)
            us.append(sp_sc[uj, q, rbs, n, 0:2])
            ks.append(sp_sc[kj, q, rbs, n, 2:4])
        acc = []
        for rb in range(2):
            z = jnp.zeros((8, 128), F32) if not link else jnp.where(never_sm[0] > 0, link[0], 0.0)
            ar = ai = z
            for u, k in zip(us, ks):
                ar = ar + u[rb, 0] * k[rb, 0]
                ai = ai + u[rb, 0] * k[rb, 1]
                ar = ar - u[rb, 1] * k[rb, 1]
                ai = ai + u[rb, 1] * k[rb, 0]
            acc.append((ar, ai))
            if link is not None:
                link[:] = [ar]
        ln = slice(n * 128, (n + 1) * 128)
        w = jnp.concatenate([acc[0][0], acc[1][0], acc[0][1], acc[1][1]], axis=0).astype(BF16)
        wf_sc[c & 1, 0, q, rb2 * 16:rb2 * 16 + 16, ln] = w[0:16]
        wf_sc[c & 1, 1, q, rb2 * 16:rb2 * 16 + 16, ln] = w[16:]

    def conv_inv(tt, n):
        cb = tt // NQ
        p = tt % NQ
        ln = slice(n * 128, (n + 1) * 128)
        ev = _dot(inv_ref[p, 0], wf_sc[cb & 1, 0, :, :, ln].reshape(CB, 128))
        od = _dot(inv_ref[p, 1], wf_sc[cb & 1, 1, :, :, ln].reshape(CB, 128))
        sd = jnp.concatenate([co_sc[KS, :, ln]] * (HB // 8), axis=0)
        for r, val in ((p, _flip_rows(ev - od)), (2 * NQ - 1 - p, ev + od)):
            ur = scaled(clip(cb, NB - 1) * (2 * NQ) + r, HB)
            yr = scaled((cb & 1) * (2 * NQ) + r, HB)
            y_sc[pl.ds(yr, HB), ln] = val + u_sc[pl.ds(ur, HB), ln].astype(F32) * sd

    def y_seg(s):
        return y_sc[pl.ds(scaled(s & (2 * NQ - 1), SEG), SEG), LN]

    scale = DH ** -0.5
    cexp = scale * float(np.log2(np.e))

    def make_mask(n, x_layers, q0=0):
        qi = jax.lax.broadcasted_iota(jnp.int32, (n - q0, n), 0) + q0
        ki = jax.lax.broadcasted_iota(jnp.int32, (n - q0, n), 1)

        def layer(i):
            xl = jnp.where(i < M2 + SEG, x_layers[0], x_layers[-1])
            return jnp.where(i < M, 0, jnp.where(i < M2, 1, xl))
        same = layer(qi) == layer(ki)
        ok = same & ((qi < M2) | (ki < M2) | (qi >= ki))
        fill = jnp.where(same, -1e9 / scale, -jnp.inf).astype(F32)
        return ok, fill

    def probs(q, k, mask):
        ok, fill = mask
        s = _dot_nt(q, k)
        s = jnp.where(ok, s, fill)
        m = jnp.max(s, axis=-1, keepdims=True)
        p = jnp.exp2((s - m) * cexp)
        l = jnp.sum(p, axis=-1, keepdims=True)
        r = pl.reciprocal(l, approx=True)
        r = r * (2.0 - l * r)
        return (p * r).astype(BF16)

    def w_slot(ci):
        return (wb_sc, ci) if 1 <= ci < NRB - 1 else (wa_sc, max(ci - (NRB - 2), 0))

    def rows(*parts):
        return jnp.concatenate(parts, axis=0)

    def cols(*parts):
        return jnp.concatenate(parts, axis=1)

    def bf(*xs):
        return tuple(x.astype(BF16) for x in xs)

    def xn(s):
        return xn_sc[clip(s, NSEG - 1)]

    clock = [0]
    queue = []
    recent = [None]

    def later(delay, act):
        queue.append((clock[0] + delay, act))

    def run_due(force=False):
        while queue:
            item = min(queue, key=lambda it: it[0])
            if item[0] > clock[0] and not force:
                break
            queue.remove(item)
            clock[0] = max(clock[0], item[0])
            item[1]()

    def mm(a, w):
        run_due()
        clock[0] += a.shape[0] * w.size // (4 * 128 * 128)
        recent[0] = _dot(a, w)
        return recent[0]

    def spread(work, ref, slot, count, t0, t1):
        def act():
            ref[slot, N_TILES - 1, 0:8, :] = pltpu.bitcast(recent[0][0:8, 0:DH], U32)
            next(work)
        for i in range(count):
            later(t0 + i * (t1 - t0) // count, act)

    def packed_lhs(rid):
        def lhs(parts, i):
            return _unpack(cols(*[_tile(rid, 4 if i is None else RIDE_TILE[p][i]) for p in parts]))
        return lhs, 2 * rid.shape[0], False

    def value_lhs(rid, pair=None, pins=None):
        @functools.lru_cache(None)
        def lhs(parts, i):
            def one(p):
                if i is None:
                    return rows(*[_tile(r, 4) for r in (rid,) + (pair or ())])
                ps = [_lin(RIDE[i], lambda k: _tile(rid, 2 * p + k))] if i in RIDE else []
                if pair:
                    ps.append(_lin(LHS[i], lambda rk: _tile(pair[rk[0]], 2 * p + rk[1])))
                for v in (pins or {}).get((p, i), ()):
                    ps[-1] = rows(*([ps[-1][:-SEG]] if ps[-1].shape[0] > SEG else []),
                                  jnp.where(never_sm[0] > 0, v, ps[-1][-SEG:]))
                return rows(*ps)
            return cols(*[one(p) for p in parts]).astype(BF16)
        return lhs, rid.shape[0], pair is not None

    def product(tile, u, lhs, i):
        base = T_TRI[u] if u < 2 else T_LAST
        if u == 3:
            a, w = lhs((0,), i), tile(4 * i + 1)
        elif i < 7:
            a, w = lhs((0, 1), i), rows(tile(4 * i + (0, 2, 3)[u]), tile(base + i))
        else:
            a, w = lhs((1,), i), tile(base + i)
        return mm(a, w)

    def unit(tile, u, left, carry, ahead=()):
        lhs, nr, paired = left

        def comb(uu, n):
            return _combine(lambda i: ahead[uu, i] if (uu, i) in ahead else product(tile, uu, lhs, i),
                            n, nr, paired)
        if u == 2:
            c = comb(2, 2)
            return {6 + j: mm(lhs((1,), None), tile(T_TAIL + j)) + c[j] for j in range(2)}
        if u == 0:
            carry[2], carry[3] = comb(3, 2)
        c = comb(u, 3)
        hs = TRIPLES[u]
        return {hs[0]: c[0], hs[1]: c[1], hs[2]: c[2] + carry.pop(hs[2])}

    def w_tiles(g, mats):
        slots = [w_slot(mi * NG + g) for mi in mats]
        return lambda i: _unpack(cols(*[ref[k, i] for ref, k in slots]))

    def attend(proj, n, mask, hook=None, raw=False):
        full = n == R
        nr = M2 if full else n
        parts = {}
        os_ = {}

        def add_forms(g, hs, ids):
            for i in range(7 if len(hs) == 2 else 15):
                ps = []
                if i in RIDE:
                    ps.append(_lin(RIDE[i], lambda k: os_[hs[k]][:nr]))
                if full:
                    ps.append(_lin(LHS[i], lambda rk: os_[hs[rk[1]]][M2 + rk[0] * SEG:RH + rk[0] * SEG]))
                if ps:
                    a = rows(*ps).astype(BF16)
                    for part, tid in ids(i):
                        parts.setdefault((part, i), []).append((g, a, tid))

        def prod(key, g0, g1):
            if raw:
                a = cols(*[parts[h] for h in range(g0 * HG, g1 * HG)])
                return mm(a, wo_sc[g0 * HG * DH:g1 * HG * DH, key * 128:(key + 1) * 128])
            sel = [p for p in parts[key] if g0 <= p[0] < g1]
            return mm(cols(*[p[1] for p in sel]), _unpack(rows(*[wc_sc[p[0], p[2]] for p in sel])))

        def forms(g, u, hs):
            if raw:
                parts.update({g * HG + h: os_[h].astype(BF16) for h in hs})
            elif u < 2:
                add_forms(g, TRIPLES[u], lambda i: [(1, T_TRI[u] + i)] + ([(0, 4 * i + 2 * u)] if i < 7 else []))
                if u == 1:
                    add_forms(g, (2, 3), lambda i: [(0, 4 * i + 1)])
            else:
                add_forms(g, (6, 7), lambda i: [(0, 4 * i + 3), (1, T_LAST + i)])
                for j in range(2):
                    parts[1, 7].append((g, os_[6 + j][:min(n, RH)].astype(BF16), T_TAIL + j))
                    if full:
                        parts[1, 8].append((g, os_[6 + j][RH:].astype(BF16), T_TAIL + j))

        def head(g, u, h, qkv, done):
            def values(p):
                os_[h] = _dot(p, qkv[h][2])
                clock[0] += n // 4
                done.append(h)
                if len(done) == len(qkv):
                    forms(g, u, done)

            def scores():
                p = probs(qkv[h][0], qkv[h][1], mask)
                clock[0] += n // 4
                later(LAT_P, lambda: values(p))
            return scores

        for it in range(NU):
            qkv = proj(it)
            done = []
            for i, h in enumerate(qkv):
                later(LAT_S + i * GAP_S * n // R, head(*divmod(it, 3), h, qkv, done))
            if hook is not None:
                hook(it)
        last = [(0, 1), (1, 1), (1, 8), (1, 13)]
        keys = range(NT) if raw else sorted(parts, key=lambda k: (k[1] == 6, k[0], ORDER.index(k[1])))
        m = {}
        end = None
        for key in keys:
            if end is None and not queue:
                end = clock[0] + LAT_O
            if key not in last and (end is None or clock[0] < end):
                m[key] = prod(key, 0, NG - 1)
        run_due(True)
        if hook is not None:
            hook(NU)
        early = list(m)
        for key in keys:
            if key not in early and key not in last and (raw or key[1] != 6):
                m[key] = prod(key, 0, NG)
        for key in early:
            m[key] = prod(key, NG - 1, NG) + m[key]
        if raw:
            return cols(*[m[i] for i in range(NT)])
        for key in ((0, 6), (1, 6)):
            if key not in early:
                m[key] = prod(key, 0, NG)
        res = []
        for part in range(2):
            res += _combine(lambda i: m[part, i] if (part, i) in m else prod((part, i), 0, NG),
                            2 + part, nr, full, True)
        return cols(*res)

    def side2(t, a2):
        x3 = x2_sc[(t - 2) & 3] + a2
        x4 = x3 + _ln(x3) * y_seg(t - 2)
        out_sc[seg(t - 2), LN] = x4.astype(out_sc.dtype)
        return x4

    def finish(t, xr, yt, mem, a1):
        x1 = xr.astype(F32) + a1
        x2 = x1 + _ln(x1) * yt
        h_sc[...] = mem
        x2_sc[t & 3] = x2
        return x2

    def staged(make, pins):
        keys = ((0, 0), (1, 0), (0, 3), (1, 3), (0, 5))
        events = sorted({0} | {g0 + n // per for g0, _, per in pins for n in range(NT)})
        made = {}
        for e in events:
            act = {}
            for g0, v, per in pins:
                for n in range(NT):
                    if g0 + n // per <= e:
                        act.setdefault(keys[n], []).append(_tile(v, n))
            made[e] = make(act)
        return lambda k: made[max(e for e in events if e <= k)]

    def wait_chunk(ci):
        for cp in w_copies(0, ci):
            cp.wait()

    def w_block(ci, b):
        x = pltpu.bitcast(st_sc[ci, b], U32)
        sub = jax.lax.broadcasted_iota(jnp.int32, (8, DH), 0)
        res = []
        for par in range(2):
            v = [x[2 * i + par] for i in range(4)]
            for bit in (2, 1):
                keep = (sub & bit) == 0
                for i in range(4):
                    if not i & bit:
                        a, c = v[i], v[i + bit]
                        v[i] = jnp.where(keep, a, pltpu.roll(c, bit, 0))
                        v[i + bit] = jnp.where(keep, pltpu.roll(a, 8 - bit, 0), c)
            res.append(v)
        return res

    def rhs_tiles(part, plain, value, pack, swap):
        def one(i, base, hs):
            terms = {kj: sg for kj, sg in RHS[i].items() if max(kj) < len(hs)}

            def at(kj):
                k, j = kj[::-1] if swap else kj
                return base + k, hs[j]
            if len(terms) == 1:
                return plain(*at(next(iter(terms))))
            return pack(_lin(terms, lambda kj: value(*at(kj))))
        if part == 0:
            for p in range(4):
                for i in range(7):
                    yield 4 * i + p, one(i, 0, (2 * p, 2 * p + 1))
        else:
            for u in range(2):
                for i in range(15):
                    yield T_TRI[u] + i, one(i, 2, TRIPLES[u])
            for i in range(7):
                yield T_LAST + i, one(i, 2, (6, 7))
            for j in range(2):
                yield T_TAIL + j, plain(4, 6 + j)

    GROUPS = ((0, 12, T_TRI[0]), (T_TRI[0], T_TRI[1], T_LAST, T_TAIL + 2))
    NGRP = 8 * (len(GROUPS[0]) + len(GROUPS[1]) - 2)

    def put_tiles(dst, slot, r0, part, tiles):
        out = dict(tiles)
        for lo, hi in zip(GROUPS[part], GROUPS[part][1:]):
            dst[slot, lo:hi, pl.ds(r0, 8), :] = jnp.stack([out[i] for i in range(lo, hi)])
            yield

    def chunk_work(item):
        for b in range(8):
            for part in range(2):
                yield from item(part, b)

    def relayout(ci, dst, slot, part, b):
        hi_m = U32(0xFFFF0000)
        t = {k: w_block(ci, 8 * k + b) for k in ((0, 1), (2, 3, 4))[part]}

        def plain(k, h):
            a, c = t[k][0][h // 2], t[k][1][h // 2]
            return (a >> 16) | (c & hi_m) if h % 2 else (a & U32(0xFFFF)) | (c << 16)

        @functools.lru_cache(None)
        def value(k, h):
            w = cols(t[k][0][h // 2], t[k][1][h // 2])
            return pltpu.bitcast(w & hi_m if h % 2 else w << 16, F32)

        def pack(v):
            r = pltpu.bitcast(v.astype(BF16).astype(F32), U32)
            return (r[:, :DH] >> 16) | r[:, DH:]
        yield from put_tiles(dst, slot, scaled(b, 8), part, rhs_tiles(part, plain, value, pack, False))

    def main(_, carry):
        for part in range(2):
            def relayout0(b, c, part=part):
                list(relayout(0, wa_sc, 0, part, b))
                return c
            with jax.named_scope("wait_w"):
                for cp in w_copies(0, part=part):
                    cp.wait()
            with jax.named_scope("relayout"):
                jax.lax.fori_loop(0, 8, relayout0, 0)

        def pro_stage(ps_, b):
            n = ps_ * NRB + b
            with jax.named_scope("wait_w"):
                if ps_ == 0:
                    @pl.when(b + 1 < NRB)
                    def _():
                        x_copy(b + 1).wait()

                @pl.when((n >= 2) & (n <= NCH))
                def _():
                    wait_chunk(n - 1)
            cr = jnp.clip(n - 1, 0, NCH - 1)
            dst, slot = (wb_sc, cr) if ps_ == 0 else (wa_sc, cr - (NRB - 2))
            bl = jnp.minimum(b + 1, NRB - 1)
            PW = PRO_PW
            npc = RB * S2 // PW
            assert npc * PW == RB * S2 and 2 * NRB > UL

            def body(i, c):
                s0 = b * RB + 1
                for sg in range(RB):
                    hp_sc[sg * S2:(sg + 1) * S2, :] = xn_sc[s0 + sg]
                spread(chunk_work(functools.partial(relayout, cr, dst, slot)), dst, jnp.minimum(never_sm[0], 0), NGRP, *PRO_T)
                for pi in range(npc):
                    carry = {}
                    for u in range(3):
                        pos = 3 * pi + u
                        hx = hp_sc[pi * PW:(pi + 1) * PW, :]
                        for k in range(max(RB, 2 * NT)):
                            if PRO_X0 + k * PRO_XN // PRO_XD != pos:
                                continue
                            if ps_ == 0 and k < RB:
                                sn = bl * RB + 1 + k
                                xv = _ext(_ln(x_sc[seg(sn), LN].astype(F32)))
                                xn_sc[sn] = xv
                                hx = rows(hx[:-S2], jnp.where(never_sm[0] > 0, xv, hx[-S2:]))
                            if ps_ == 1 and k < 2 * NT:
                                conv_u(jnp.minimum(2 * b + k // NT, UL),
                                       slice((k % NT) * 128, (k % NT + 1) * 128))
                        for h, r in unit(w_tiles(ps_, (0,)), u, packed_lhs(hx), carry).items():
                            for a in range(0, 2 * PW, 16):
                                sg, off = divmod(2 * pi * PW + a, SEG)
                                pre_sc[s0 + sg, ps_ * HG + h, off:off + 16, :] = r[a:a + 16].astype(BF16)
                assert not queue
                return c
            assert PRO_X0 + (max(RB, 2 * NT) - 1) * PRO_XN // PRO_XD < 3 * npc
            with jax.named_scope("fused"):
                jax.lax.fori_loop(0, never_sm[0] + 1, body, 0)

        for ps_ in range(NPASS):
            if ps_ == 1:
                with jax.named_scope("wait_in0"):
                    for cp in small + in_copies(0):
                        cp.wait()
                sh = sh_ref[...].astype(F32)
                for j in range(KS):
                    co_sc[j] = jnp.broadcast_to(sh[j:j + 1], (8, DM))
                co_sc[KS] = jnp.broadcast_to(sd_ref[...].astype(F32).reshape(1, DM), (8, DM))

            def blk(b, c, ps_=ps_):
                pro_stage(ps_, b)
                return c
            jax.lax.fori_loop(0, NRB, blk, 0)

        def warm_block0(q):
            uf, kf = conv_fwd(0, q)
            put_spec(0, q, 0, uf)
            put_spec(0, q, 2, kf)
            kr_sc[q] = kf
            ur, um, kr, km = uf[:QB], uf[QB:], kf[:QB], kf[QB:]
            wf_sc[0, 0, q] = (ur * kr - um * km).astype(BF16)
            wf_sc[0, 1, q] = (ur * km + um * kr).astype(BF16)

        def wo_operands(g, part, b):
            def src(k, h):
                r = (g * HG + h) * DH + 16 * b
                return wo_sc[r:r + 16, k * 128:(k + 1) * 128]
            tiles = rhs_tiles(part, lambda k, h: _pack(src(k, h)),
                              functools.lru_cache(None)(lambda k, h: src(k, h).astype(F32)), _pack, True)
            yield from put_tiles(wc_sc, g, 8 * b, part, tiles)

        def wo_work():
            for g in range(NG):
                yield from chunk_work(functools.partial(wo_operands, g))

        def plain_qkv(eq, ekv, k, carry):
            g, u = divmod(k, 3)
            res = []
            for mats, e in (((1,), ekv), ((2,), ekv), ((0,), eq)):
                res.append(unit(w_tiles(g, mats), u, e, carry.setdefault(mats, {})))
            return {h: bf(res[2][h], res[0][h], res[1][h]) for h in res[0]}

        with jax.named_scope("wait_wo"):
            wo_copy.wait()
        with jax.named_scope("step0"):
            mem0 = mem0_ref[...].astype(F32)
            e0 = packed_lhs(rows(_ext(rows(mem0, mem0)), xn(0)))

            carry0 = {}
            spread(wo_work(), wc_sc, jnp.minimum(never_sm[0], 0), NG * NGRP, *WO_T)

            def hook0(it):
                if it < NQ:
                    warm_block0(it)
                if 5 <= it < 5 + NT:
                    for p in range(2):
                        conv_inv(p, it - 5)
            out = attend(lambda k: plain_qkv(e0, e0, k, carry0), RH, make_mask(RH, (0,)), hook0, True)
            y0 = y_seg(0)
            for q in range(2):
                conv_spec(1, q)
            for n in range(NT):
                conv_inv(2, n)
            finish(0, x_sc[0:SEG, LN], y0, rows(out[0:M], mem0), out[M2:])
            for q in range(2):
                for piece in MAC_PIECES:
                    conv_mac(1, q, piece, 2)

        mask12 = make_mask(R, (0, 1))

        def step(t, x2):
            c, q = (t + 1) // NQ + 1, (t + 1) % NQ
            mem = h_sc[...]
            n1 = _unpack(xn(t)[:, 0:DM]).astype(F32)
            lead = value_lhs(mem, (n1, None))[0]
            ahead = {ui: product(w_tiles(0, (1, 2)), ui[0], lead, ui[1]) for ui in AHEAD}
            if x2 is None:
                x2 = x2_sc[(t - 1) & 3]
            conv_spec(c, q)
            link = []
            for piece in MAC_PIECES:
                conv_mac(c, q, piece, NB, link)
            n2 = _ln(x2)
            x4 = side2(t, op_sc[...])
            un = conv_u(t + UL)
            left = staged(lambda p: value_lhs(mem, (n1, n2), p), [(PIN_U, un, 2), (PIN_X4, x4, NT)])
            left_q = value_lhs(rows(mem, n2))
            carry = {}

            def proj(k):
                g, u = divmod(k, 3)
                pre = g * HG < NPA
                if pre:
                    qs = unit(w_tiles(g, (0,)), u, left_q, carry.setdefault("q", {}))
                rs = unit(w_tiles(g, (1, 2) if pre else (1, 2, 0)), u, left(k), carry.setdefault("kv", {}),
                          ahead if g == 0 else ())
                res = {}
                for h, r in rs.items():
                    if pre:
                        qq = rows(qs[h][:M2], pre_sc[t, g * HG + h].astype(F32), qs[h][M2:])
                    else:
                        qq = r[:, 2 * DH:]
                    res[h] = bf(qq, r[:, :DH], r[:, DH:2 * DH])
                return res

            held = {}

            def hook(it):
                if INV_AT <= it < INV_AT + NT:
                    conv_inv(t + 2, it - INV_AT)
                if it == NU:
                    held["x"] = x_sc[seg(t), LN]
                    held["y"] = y_seg(t)
            out = attend(proj, R, mask12, hook)
            op_sc[...] = out[RH:]
            return finish(t, held["x"], held["y"], out[0:M2], out[M2:RH])

        def steps(i, carry):
            x2 = None
            for j in range(UNROLL):
                x2 = step(1 + i * UNROLL + j, x2)
            return carry

        def phase(p, carry):
            @pl.when(p == 1)
            def _():
                for cp in in_copies(2):
                    cp.wait()

            @pl.when(p >= 2)
            def _():
                out_copy((p - 2) * PH, PH).start()

            with jax.named_scope("steps"):
                jax.lax.fori_loop(p * PHI, (p + 1) * PHI, steps, 0)
            return carry

        for cp in in_copies(1):
            cp.wait()
        jax.lax.fori_loop(0, NPH, phase, 0)
        out_copy((NPH - 2) * PH, NSEG - 2 - (NPH - 2) * PH).start()

        with jax.named_scope("step_last"):
            x4 = side2(NSEG, op_sc[...])
            n2 = _ln(x2_sc[(NSEG - 1) & 3])
            left_q = value_lhs(n2)
            left = staged(lambda p: value_lhs(rows(h_sc[...], n2), None, p), [(PIN_X4, x4, NT)])
            carry1 = {}
            out = attend(lambda k: plain_qkv(left_q, left(k), k, carry1),
                         SEG, make_mask(RH, (1,), M2))
            side2(NSEG + 1, out)
        out_copy(NSEG - 2, 2).start()
        out_copy(0, NSEG).wait()
        return carry

    jax.lax.fori_loop(0, never_sm[0] + 1, main, 0)


def pallas_interleave_layers__memory_aug_recurrent_mem_tr__ssm_conv_h3__prompt_kernel(
    A_x, A_mem0, A_Wq, A_Wk, A_Wv, A_Wo, A_seg_len,
    B_q, B_k, B_v, B_shift_k, B_ssm_k, B_ssm_D,
):
    del B_q
    seg = int(A_seg_len) if isinstance(A_seg_len, (int, np.integer)) else CB // NQ
    return _run(A_x, A_mem0, A_Wq, A_Wk, A_Wv, A_Wo, B_k, B_v, B_shift_k, B_ssm_k, B_ssm_D, SEG=seg)


@functools.partial(jax.jit, static_argnames=("SEG",))
def _run(A_x, A_mem0, A_Wq, A_Wk, A_Wv, A_Wo, B_k, B_v, B_shift_k, B_ssm_k, B_ssm_D, *, SEG):
    B, S, DM = A_x.shape
    assert B == 1
    H, DH = A_Wq.shape[1], A_Wq.shape[2]
    M = A_mem0.shape[1]
    KS = B_shift_k.shape[1]
    R = 2 * (M + SEG)
    NSEG = S // SEG
    NRB = (NSEG - 1) // RB
    NB = S // CB
    QB = CB // NQ
    NCH = 3 * H // HG
    DP = -(-DM // 256) * 256
    fwd, inv = _dft_constants()

    kern = functools.partial(_kernel, S=S, DM=DM, H=H, DH=DH, M=M, SEG=SEG)
    any_spec = pl.BlockSpec(memory_space=pl.ANY)
    out = pl.pallas_call(
        kern,
        out_shape=jax.ShapeDtypeStruct((S, DM), A_x.dtype),
        in_specs=[any_spec] * 13,
        out_specs=any_spec,
        scratch_shapes=[
            pltpu.VMEM((NB + 2, NQ, QB // 8, DM // 128, 4, 8, 128), F32),
            pltpu.VMEM((NQ, 2 * QB, DM), F32),
            pltpu.VMEM((2, 2, NQ, QB, DM), BF16),
            pltpu.VMEM((4, SEG, DM), F32),
            pltpu.VMEM((2 * CB, DP), F32),
            pltpu.VMEM((S, DP), BF16),
            pltpu.VMEM((SEG, DM), F32),
            pltpu.VMEM((NSEG, NPA, SEG, DH), BF16),
            pltpu.VMEM((NSEG, SEG // 2, DM + 384), U32),
            pltpu.VMEM((NCH - NRB + 2, N_TILES, 64, DH), U32),
            pltpu.VMEM((NRB - 1, N_TILES, 64, DH), U32),
            pltpu.VMEM((H * DH, DM), BF16),
            pltpu.VMEM((H // HG, N_TILES, 64, DH), U32),
            pltpu.VMEM((S, DP), BF16),
            pltpu.VMEM((S, DP), BF16),
            pltpu.VMEM((NB, DM, CB), BF16),
            pltpu.VMEM((NCH, DM // 16, 8, 2 * HG, DH), BF16),
            pltpu.VMEM((S, DP), A_x.dtype),
            pltpu.VMEM(fwd.shape, BF16),
            pltpu.VMEM(inv.shape, BF16),
            pltpu.VMEM((S + KPAD, DP), BF16),
            pltpu.VMEM((RB * SEG // 2, DM + 384), U32),
            pltpu.VMEM((2 * M, DM), F32),
            pltpu.VMEM((KS + 1, 8, DM), F32),
            pltpu.VMEM((M, DM), BF16),
            pltpu.VMEM((KS, DM), BF16),
            pltpu.VMEM((DM,), BF16),
            pltpu.SMEM((1,), jnp.int32),
            pltpu.SemaphoreType.DMA(((NSEG - 1) // RB,)),
            pltpu.SemaphoreType.DMA((3,)),
            pltpu.SemaphoreType.DMA((NCH + 2,)),
            pltpu.SemaphoreType.DMA(()),
        ],
        compiler_params=pltpu.CompilerParams(vmem_limit_bytes=120 * 1024 * 1024),
    )(
        A_x.reshape(S, DM), A_mem0.reshape(M, DM),
        *[w.reshape(DM // 16, 2, 8, H, DH) for w in (A_Wq, A_Wk, A_Wv)],
        A_Wo.reshape(H * DH, DM), B_k.reshape(S, DM), B_v.reshape(S, DM),
        B_shift_k.T, B_ssm_k, B_ssm_D,
        jnp.asarray(fwd, BF16), jnp.asarray(inv, BF16),
    )
    return out.reshape(B, S, DM)
```

```python
import functools

import numpy as np
import jax
import jax.numpy as jnp
import jax.experimental.pallas as pl
import jax.experimental.pallas.tpu as pltpu

F32 = jnp.float32
BF16 = jnp.bfloat16
U32 = jnp.uint32

CB = 128
NQ = 4
KPAD = 16
HG = 8
NPA = 16
RB = 9
PRO_PW, PRO_X0, PRO_XN, PRO_XD = 24, 3, 3, 2
PRO_T, WO_T = (20, 2820), (20, 6200)
UNROLL = 3
PHI = 3
INV_AT, PIN_U, PIN_X4 = 7, 2, 6

LHS = ({(0, 0): 1}, {(0, 0): 1, (1, 0): 1}, {(0, 1): 1, (1, 1): 1}, {(1, 1): 1}, {(0, 0): 1, (1, 1): 1},
       {(0, 1): 1, (0, 0): -1}, {(1, 1): 1, (1, 0): -1}, {(0, 2): 1}, {(1, 2): 1},
       {(0, 0): 1, (1, 0): 1, (1, 2): -1}, {(0, 2): 1, (1, 2): 1, (0, 0): -1, (1, 0): -1},
       {(1, 2): 1, (1, 0): -1}, {(0, 1): 1, (1, 1): 1, (0, 2): -1},
       {(0, 2): 1, (1, 2): 1, (0, 1): -1, (1, 1): -1}, {(0, 1): 1, (0, 2): -1})
RHS = ({(0, 0): 1, (1, 0): 1, (0, 2): -1}, {(0, 0): 1, (2, 0): 1, (0, 1): -1},
       {(1, 1): 1, (2, 1): 1, (1, 0): -1}, {(1, 1): 1, (0, 1): 1, (1, 2): -1}, {(0, 1): 1, (1, 0): 1},
       {(1, 0): 1}, {(0, 1): 1}, {(2, 2): 1, (1, 2): 1, (2, 0): -1}, {(2, 2): 1, (0, 2): 1, (2, 1): -1},
       {(0, 2): 1, (2, 0): 1}, {(2, 0): 1}, {(0, 2): 1}, {(1, 2): 1, (2, 1): 1}, {(2, 1): 1}, {(1, 2): 1})
RIDE = {0: {0: 1}, 3: {1: 1}, 5: {1: 1, 0: -1}, 6: {1: 1, 0: -1}, 7: {2: 1}, 10: {2: 1}, 11: {0: 1},
        12: {2: 1}, 14: {1: 1, 2: -1}}
RIDE_TILE = ({0: 0, 3: 1, 5: 5, 6: 5}, {0: 2, 3: 3, 5: 6, 6: 6, 7: 4, 10: 4, 11: 2, 12: 4, 14: 7})
AHEAD = ((3, 0), (3, 5), (0, 0), (0, 5), (0, 14), (0, 7), (1, 0), (1, 5))
LAT = (300, 200, 620, 250)
LAT_FIRST, LAT_LAST = (300, 120, 620, 250), (250, 120, 520, 200)
ORDER = (0, 4, 5, 2, 3, 1, 6, 9, 11, 10, 13, 12, 8, 14, 7)
TRIPLES = ((0, 1, 2), (4, 5, 3))
T_TRI, T_LAST, T_TAIL, N_TILES = (28, 43), 58, 65, 68


def _lin(terms, get):
    acc = None
    for key, sign in terms.items():
        v = get(key)
        acc = v if acc is None else (acc + v if sign > 0 else acc - v)
    return acc


def _combine(product, n, nr, paired, x2_last=False):
    m = functools.lru_cache(None)(product)

    def r(i):
        return m(i)[:nr]

    def x(i):
        return m(i)[nr:] if i in RIDE else m(i)
    if not paired:
        rid = [m(0) + m(5), m(3) - m(6)]
        if n == 3:
            v = m(10) + m(11)
            rid = [rid[0] + v, rid[1] + m(12) + m(14), m(7) + v + m(14)]
        return rid
    if not x2_last:
        x(0)
        p = x(4) - x(0)
        a = m(0) + m(5)
        w = x(4) + x(5) + x(2) - x(3)
        p = p + x(1)
        b = m(3) - m(6)
        rid, top, bot = [a[:nr], b[:nr]], [a[nr:], w], [p - x(6), b[nr:]]
        if n == 3:
            t = x(9) + x(11)
            t0 = t + x(10)
            v = r(10) + r(11)
            rid[0], top[0], bot[0] = rid[0] + v, top[0] + t0, bot[0] - t
            x(13), x(12)
            z = x(8) - x(11)
            u = x(12) - x(14)
            t1 = u + x(13)
            rid[1], top[1], bot[1] = rid[1] + r(12) + r(14), top[1] - u, bot[1] + t1
            c = m(7) + m(14)
            rid.append(c[:nr] + v)
            top.append(c[nr:] + t0)
            bot.append(z + t1)
        return [jnp.concatenate(p, axis=0) for p in zip(rid, top, bot)]
    a = m(0) + m(5)
    w = x(4) + x(5) - x(3)
    top = [a[nr:], w + x(2)]
    if n == 3:
        t = x(11) + x(9)
        t0 = t + x(10)
        v = r(10) + r(11)
        u = x(12) - x(14)
        top = [top[0] + t0, top[1] - u, x(7) + t0 + x(14)]
    b = m(3) - m(6)
    rid = [a[:nr], b[:nr]]
    bot = [x(4) - x(0) - x(6), b[nr:]]
    if n == 3:
        rid = [rid[0] + v, rid[1] + r(12) + r(14), r(7) + v + r(14)]
        t1 = u + x(13)
        bot = [bot[0] - t, bot[1] + t1, t1 - x(11) + x(8)]
    bot[0] = bot[0] + x(1)
    return [jnp.concatenate(p, axis=0) for p in zip(rid, top, bot)]


def _dft_constants():
    qb = CB // NQ
    hb = qb // 2
    n = np.arange(CB, dtype=np.float64)
    f = np.concatenate([q * qb + np.concatenate([np.arange(0, qb, 2), np.arange(1, qb, 2)])
                        for q in range(NQ)])
    w = np.pi * (2.0 * f + 1.0) / (2 * CB)
    ang = (w[:, None] * (n[None, :] - (CB - 1) / 4.0)).reshape(NQ, qb, CB)
    fwd = np.concatenate([np.cos(ang), -np.sin(ang)], axis=1)
    inv = np.zeros((NQ, 2, hb, CB))
    for p in range(NQ):
        m = (NQ - 1 - p) * hb + np.arange(hb)
        ang = (m[:, None] + 0.5) * w[None, :]
        inv[p, 0] = np.cos(ang) / CB
        inv[p, 1] = -np.sin(ang) / CB
    return fwd.astype(np.float32), inv.astype(np.float32)


def _flip_rows(x):
    i = jax.lax.broadcasted_iota(jnp.int32, (8, x.shape[1]), 0)
    out = []
    for r in range(x.shape[0] - 8, -8, -8):
        v = pltpu.roll(x[r:r + 8], 4, 0)
        for b in (2, 1):
            v = jnp.where((i & b) == 0, pltpu.roll(v, 8 - b, 0), pltpu.roll(v, b, 0))
        out.append(v)
    return jnp.concatenate(out, axis=0)


def _ln(x, eps=1e-5):
    d = x.shape[-1]
    m = jnp.sum(x, axis=-1, keepdims=True) * (1.0 / d)
    xc = x - m
    v = jnp.sum(xc * xc, axis=-1, keepdims=True) * (1.0 / d)
    return xc * jax.lax.rsqrt(v + eps)


def _dot(a, b):
    return jnp.dot(a, b, preferred_element_type=F32)


def _dot_nt(a, b):
    return jax.lax.dot_general(a, b, (((1,), (1,)), ((), ())), preferred_element_type=F32)


def _pack(x):
    return pltpu.bitcast(x.astype(BF16), U32)


def _unpack(x):
    return pltpu.bitcast(x, BF16)


def _tile(x, n):
    return x[:, n * 128:(n + 1) * 128]


def _ext(r):
    return _pack(jnp.concatenate(
        [r, _tile(r, 1) - _tile(r, 0), _tile(r, 3) - _tile(r, 2), _tile(r, 3) - _tile(r, 4)], axis=1))


def _in_order(actions):
    def body(i, c):
        for j, act in enumerate(actions):
            pl.when(i == j)(act)
        return c
    jax.lax.fori_loop(0, len(actions), body, 0)


def _kernel(x_hbm, mem0_hbm, wq_hbm, wk_hbm, wv_hbm, wo_hbm, k_hbm, v_hbm,
            sh_hbm, sk_hbm, sd_hbm, fwd_hbm, inv_hbm, o_hbm,
            sp_sc, kr_sc, wf_sc, x2_sc, y_sc, u_sc, op_sc, pre_sc, xn_sc, wa_sc, wb_sc, wo_sc, wc_sc,
            x_sc, v_sc, sk_sc, st_sc, out_sc, fwd_ref, inv_ref,
            k_sc, hp_sc, h_sc, co_sc, mem0_ref, sh_ref, sd_ref,
            never_sm, sem_x, sem_in, sem_w, sem_out,
            *, S, DM, H, DH, M, SEG):
    NSEG = S // SEG
    M2 = 2 * M
    S2 = SEG // 2
    R = M2 + 2 * SEG
    RH = M2 + SEG
    NB = S // CB
    QB = CB // NQ
    HB = QB // 2
    NT = DM // 128
    PH = PHI * UNROLL
    NRB = (NSEG - 1) // RB
    NPH = (NSEG - 1) // PH
    NG = H // HG
    NCH = 3 * NG
    NPASS = NPA // HG
    NU = 3 * NG
    KS = sh_ref.shape[0]
    UL = 2 * NQ + 1
    LN = pl.ds(0, DM)
    assert NT == 5 and HG == 8 and DH == 128 and 2 <= KS <= 8 and QB == SEG and NRB * RB == NSEG - 1 and NPH * PH == NSEG - 1 and NPASS == 2 and 2 * NRB >= NCH + 1

    mem0_copy = pltpu.make_async_copy(mem0_hbm, mem0_ref, sem_x.at[0])
    small = [pltpu.make_async_copy(s, d, sem_in.at[0]) for s, d in [
        (sh_hbm, sh_ref), (sd_hbm, sd_ref), (fwd_hbm, fwd_ref), (inv_hbm, inv_ref)]]

    def x_copy(b):
        if isinstance(b, int) and b == 0:
            rows = pl.ds(0, (RB + 1) * SEG)
        else:
            rows = pl.ds(pl.multiple_of((b * RB + 1) * SEG, SEG), RB * SEG)
        return pltpu.make_async_copy(x_hbm.at[rows], x_sc.at[rows, LN], sem_x.at[b])

    kb = (0, (UL + 1) * SEG, (UL + PH + 1) * SEG, S)
    sb = (0, 2, (PH + 2) // NQ + 2, NB)

    def in_copies(part):
        def rng(b):
            return pl.ds(b[part], b[part + 1] - b[part])
        sem = sem_in.at[part]
        return [
            pltpu.make_async_copy(k_hbm.at[rng(kb)],
                                  k_sc.at[pl.ds(KPAD + kb[part], kb[part + 1] - kb[part]), LN], sem),
            pltpu.make_async_copy(v_hbm.at[rng(kb)], v_sc.at[rng(kb), LN], sem),
        ] + [pltpu.make_async_copy(sk_hbm.at[:, pl.ds(c * CB, CB)], sk_sc.at[c], sem)
             for c in range(sb[part], sb[part + 1])]

    def w_copies(ci, dst=None, part=None):
        src = (wq_hbm, wk_hbm, wv_hbm)[ci // NG]
        dst = ci if dst is None else dst
        spans = {None: [(0, DM // 16)], 0: [(0, 16)], 1: [(16, DM // 16)]}[part]
        sem = sem_w.at[NCH + 1 if part == 1 else dst]
        return [pltpu.make_async_copy(
            src.at[pl.ds(lo, hi - lo), hf, :, pl.ds((ci % NG) * HG, HG), :],
            st_sc.at[dst, pl.ds(lo, hi - lo), :, pl.ds(hf * HG, HG), :], sem)
            for lo, hi in spans for hf in range(2)]

    wo_copy = pltpu.make_async_copy(wo_hbm, wo_sc, sem_w.at[NCH])

    def out_copy(lo, n):
        rows = pl.ds(lo * SEG if isinstance(lo, int) else pl.multiple_of(lo * SEG, SEG), n * SEG)
        return pltpu.make_async_copy(out_sc.at[rows, LN], o_hbm.at[rows], sem_out)

    def start_all(cps):
        def act():
            for cp in cps:
                cp.start()
        return act

    order = [[mem0_copy, x_copy(0)], w_copies(0, part=1), w_copies(0, part=0), [x_copy(1)], [x_copy(2)]]
    for ci in range(1, NCH):
        order.append(w_copies(ci) + ([x_copy(ci + 2)] if ci + 2 < NRB else []))
        if ci == NRB - 2:
            order.append(small + in_copies(0))
    order += [[wo_copy], in_copies(1), in_copies(2)]
    for i in range(0, len(order), 5):
        _in_order([start_all(cps) for cps in order[i:i + 5]])

    never_sm[0] = 0
    k_sc[0:KPAD, LN] = jnp.zeros((KPAD, DM), BF16)
    sp_sc[NB + 1] = jnp.zeros(sp_sc.shape[1:], F32)
    op_sc[...] = jnp.zeros(op_sc.shape, F32)
    x2_sc[...] = jnp.zeros(x2_sc.shape, F32)
    y_sc[2 * CB - SEG:, LN] = jnp.zeros((SEG, DM), F32)
    mem0_copy.wait()
    x_copy(0).wait()
    for sg in range(RB + 1):
        xn_sc[sg] = _ext(_ln(x_sc[sg * SEG:(sg + 1) * SEG, LN].astype(F32)))

    def clip(i, hi):
        return min(max(i, 0), hi) if isinstance(i, int) else jnp.clip(i, 0, hi)

    def scaled(i, m):
        return i * m if isinstance(i, int) else pl.multiple_of(i * m, m)

    def seg(i):
        return pl.ds(scaled(clip(i, NSEG - 1), SEG), SEG)

    def conv_u(s, ln=LN):
        r0 = scaled(clip(s, NSEG - 1), SEG)
        kk = k_sc[pl.ds(r0, KPAD + SEG), ln].astype(F32)[KPAD - 8:]

        def coef(j, rows):
            return jnp.concatenate([co_sc[j, :, ln]] * (rows // 8), axis=0)
        sft = [kk] + [pltpu.roll(kk, j, 0) for j in range(2, KS, 2)]
        ev = functools.reduce(jnp.add, [sft[j // 2][8:] * coef(j, SEG) for j in range(0, KS, 2)])
        od = functools.reduce(jnp.add, [sft[j // 2] * coef(j, SEG + 8) for j in range(1, KS, 2)])
        ks = ev + pltpu.roll(od, 1, 0)[8:]
        u = ks * v_sc[pl.ds(r0, SEG), ln].astype(F32)
        u_sc[pl.ds(r0, SEG), ln] = u.astype(BF16)
        return u

    def conv_fwd(c, q):
        cc = clip(c, NB - 1)
        f = fwd_ref[q]
        uf = _dot(f, u_sc[pl.ds(scaled(cc, CB), CB), LN])
        kf = _dot_nt(f, sk_sc[cc])
        return uf, kf

    def put_spec(cs, q, which, val):
        for n in range(NT):
            v = val[:, n * 128:(n + 1) * 128].reshape(2, QB // 8, 8, 128)
            sp_sc[cs, q, :, n, which:which + 2] = jnp.stack([v[0], v[1]], axis=1)

    def conv_spec(c, q):
        uf, kf = conv_fwd(c, q)
        cs = clip(c, NB)
        put_spec(cs, q, 0, uf)
        pk = kr_sc[q]
        kr_sc[q] = kf
        kp = jnp.concatenate([
            kf[0:HB] - pk[QB:QB + HB],
            kf[HB:QB] + pk[QB + HB:],
            kf[QB:QB + HB] + pk[0:HB],
            kf[QB + HB:] - pk[HB:QB]], axis=0)
        put_spec(cs, q, 2, kp)

    MAC_PIECES = [(rb, n) for rb in range(QB // 16) for n in range(NT)]

    def conv_mac(c, q, piece, nterms, link=None):
        rb2, n = piece
        cs = clip(c, NB)
        rbs = slice(2 * rb2, 2 * rb2 + 2)
        us, ks = [], []
        for j in range(nterms):
            if isinstance(cs, int):
                uj, kj = j, cs - j
            else:
                uj = jnp.minimum(j, cs)
                kj = jnp.where(cs - j >= 0, cs - j, NB + 1)
            us.append(sp_sc[uj, q, rbs, n, 0:2])
            ks.append(sp_sc[kj, q, rbs, n, 2:4])
        acc = []
        for rb in range(2):
            z = jnp.zeros((8, 128), F32) if not link else jnp.where(never_sm[0] > 0, link[0], 0.0)
            ar = ai = z
            for u, k in zip(us, ks):
                ar = ar + u[rb, 0] * k[rb, 0]
                ai = ai + u[rb, 0] * k[rb, 1]
                ar = ar - u[rb, 1] * k[rb, 1]
                ai = ai + u[rb, 1] * k[rb, 0]
            acc.append((ar, ai))
            if link is not None:
                link[:] = [ar]
        ln = slice(n * 128, (n + 1) * 128)
        w = jnp.concatenate([acc[0][0], acc[1][0], acc[0][1], acc[1][1]], axis=0).astype(BF16)
        wf_sc[c & 1, 0, q, rb2 * 16:rb2 * 16 + 16, ln] = w[0:16]
        wf_sc[c & 1, 1, q, rb2 * 16:rb2 * 16 + 16, ln] = w[16:]

    def conv_inv(tt, n):
        cb = tt // NQ
        p = tt % NQ
        ln = slice(n * 128, (n + 1) * 128)
        ev = _dot(inv_ref[p, 0], wf_sc[cb & 1, 0, :, :, ln].reshape(CB, 128))
        od = _dot(inv_ref[p, 1], wf_sc[cb & 1, 1, :, :, ln].reshape(CB, 128))
        sd = jnp.concatenate([co_sc[KS, :, ln]] * (HB // 8), axis=0)
        for r, val in ((p, _flip_rows(ev - od)), (2 * NQ - 1 - p, ev + od)):
            ur = scaled(clip(cb, NB - 1) * (2 * NQ) + r, HB)
            yr = scaled((cb & 1) * (2 * NQ) + r, HB)
            y_sc[pl.ds(yr, HB), ln] = val + u_sc[pl.ds(ur, HB), ln].astype(F32) * sd

    def y_seg(s):
        return y_sc[pl.ds(scaled(s & (2 * NQ - 1), SEG), SEG), LN]

    scale = DH ** -0.5
    cexp = scale * float(np.log2(np.e))

    def make_mask(n, x_layers, q0=0):
        qi = jax.lax.broadcasted_iota(jnp.int32, (n - q0, n), 0) + q0
        ki = jax.lax.broadcasted_iota(jnp.int32, (n - q0, n), 1)

        def layer(i):
            xl = jnp.where(i < M2 + SEG, x_layers[0], x_layers[-1])
            return jnp.where(i < M, 0, jnp.where(i < M2, 1, xl))
        same = layer(qi) == layer(ki)
        ok = same & ((qi < M2) | (ki < M2) | (qi >= ki))
        fill = jnp.where(same, -1e9 / scale, -jnp.inf).astype(F32)
        return ok, fill

    def probs(q, k, mask):
        ok, fill = mask
        s = _dot_nt(q, k)
        s = jnp.where(ok, s, fill)
        m = jnp.max(s, axis=-1, keepdims=True)
        p = jnp.exp2((s - m) * cexp)
        l = jnp.sum(p, axis=-1, keepdims=True)
        r = pl.reciprocal(l, approx=True)
        r = r * (2.0 - l * r)
        return (p * r).astype(BF16)

    def w_slot(ci):
        return (wb_sc, ci) if 1 <= ci < NRB - 1 else (wa_sc, max(ci - (NRB - 2), 0))

    def rows(*parts):
        return jnp.concatenate(parts, axis=0)

    def cols(*parts):
        return jnp.concatenate(parts, axis=1)

    def bf(*xs):
        return tuple(x.astype(BF16) for x in xs)

    def xn(s):
        return xn_sc[clip(s, NSEG - 1)]

    clock = [0]
    queue = []
    recent = [None]

    def later(delay, act):
        queue.append((clock[0] + delay, act))

    def run_due(force=False):
        while queue:
            item = min(queue, key=lambda it: it[0])
            if item[0] > clock[0] and not force:
                break
            queue.remove(item)
            clock[0] = max(clock[0], item[0])
            item[1]()

    def mm(a, w):
        run_due()
        clock[0] += a.shape[0] * w.size // (4 * 128 * 128)
        recent[0] = _dot(a, w)
        return recent[0]

    def spread(work, ref, slot, count, t0, t1):
        def act():
            ref[slot, N_TILES - 1, 0:8, :] = pltpu.bitcast(recent[0][0:8, 0:DH], U32)
            next(work)
        for i in range(count):
            later(t0 + i * (t1 - t0) // count, act)

    def packed_lhs(rid):
        def lhs(parts, i):
            return _unpack(cols(*[_tile(rid, 4 if i is None else RIDE_TILE[p][i]) for p in parts]))
        return lhs, 2 * rid.shape[0], False

    def value_lhs(rid, pair=None, pins=None):
        @functools.lru_cache(None)
        def lhs(parts, i):
            def one(p):
                if i is None:
                    return rows(*[_tile(r, 4) for r in (rid,) + (pair or ())])
                ps = [_lin(RIDE[i], lambda k: _tile(rid, 2 * p + k))] if i in RIDE else []
                if pair:
                    ps.append(_lin(LHS[i], lambda rk: _tile(pair[rk[0]], 2 * p + rk[1])))
                for v in (pins or {}).get((p, i), ()):
                    ps[-1] = rows(*([ps[-1][:-SEG]] if ps[-1].shape[0] > SEG else []),
                                  jnp.where(never_sm[0] > 0, v, ps[-1][-SEG:]))
                return rows(*ps)
            return cols(*[one(p) for p in parts]).astype(BF16)
        return lhs, rid.shape[0], pair is not None

    def product(tile, u, lhs, i):
        base = T_TRI[u] if u < 2 else T_LAST
        if u == 3:
            a, w = lhs((0,), i), tile(4 * i + 1)
        elif i < 7:
            a, w = lhs((0, 1), i), rows(tile(4 * i + (0, 2, 3)[u]), tile(base + i))
        else:
            a, w = lhs((1,), i), tile(base + i)
        return mm(a, w)

    def unit(tile, u, left, carry, ahead=()):
        lhs, nr, paired = left

        def comb(uu, n):
            return _combine(lambda i: ahead[uu, i] if (uu, i) in ahead else product(tile, uu, lhs, i),
                            n, nr, paired)
        if u == 2:
            c = comb(2, 2)
            return {6 + j: mm(lhs((1,), None), tile(T_TAIL + j)) + c[j] for j in range(2)}
        if u == 0:
            carry[2], carry[3] = comb(3, 2)
        c = comb(u, 3)
        hs = TRIPLES[u]
        return {hs[0]: c[0], hs[1]: c[1], hs[2]: c[2] + carry.pop(hs[2])}

    def w_tiles(g, mats):
        slots = [w_slot(mi * NG + g) for mi in mats]
        return lambda i: _unpack(cols(*[ref[k, i] for ref, k in slots]))

    def attend(proj, n, mask, hook=None, raw=False):
        full = n == R
        LAT_S, GAP_S, LAT_P, LAT_O = LAT if full else LAT_FIRST if raw else LAT_LAST
        nr = M2 if full else n
        parts = {}
        os_ = {}

        def add_forms(g, hs, ids):
            for i in range(7 if len(hs) == 2 else 15):
                ps = []
                if i in RIDE:
                    ps.append(_lin(RIDE[i], lambda k: os_[hs[k]][:nr]))
                if full:
                    ps.append(_lin(LHS[i], lambda rk: os_[hs[rk[1]]][M2 + rk[0] * SEG:RH + rk[0] * SEG]))
                if ps:
                    a = rows(*ps).astype(BF16)
                    for part, tid in ids(i):
                        parts.setdefault((part, i), []).append((g, a, tid))

        def prod(key, g0, g1):
            if raw:
                a = cols(*[parts[h] for h in range(g0 * HG, g1 * HG)])
                return mm(a, wo_sc[g0 * HG * DH:g1 * HG * DH, key * 128:(key + 1) * 128])
            sel = [p for p in parts[key] if g0 <= p[0] < g1]
            return mm(cols(*[p[1] for p in sel]), _unpack(rows(*[wc_sc[p[0], p[2]] for p in sel])))

        def forms(g, u, hs):
            if raw:
                parts.update({g * HG + h: os_[h].astype(BF16) for h in hs})
            elif u < 2:
                add_forms(g, TRIPLES[u], lambda i: [(1, T_TRI[u] + i)] + ([(0, 4 * i + 2 * u)] if i < 7 else []))
                if u == 1:
                    add_forms(g, (2, 3), lambda i: [(0, 4 * i + 1)])
            else:
                add_forms(g, (6, 7), lambda i: [(0, 4 * i + 3), (1, T_LAST + i)])
                for j in range(2):
                    parts[1, 7].append((g, os_[6 + j][:min(n, RH)].astype(BF16), T_TAIL + j))
                    if full:
                        parts[1, 8].append((g, os_[6 + j][RH:].astype(BF16), T_TAIL + j))

        def head(g, u, h, qkv, done):
            def values(p):
                os_[h] = _dot(p, qkv[h][2])
                clock[0] += n // 4
                done.append(h)
                if len(done) == len(qkv):
                    forms(g, u, done)

            def scores():
                p = probs(qkv[h][0], qkv[h][1], mask)
                clock[0] += n // 4
                later(LAT_P, lambda: values(p))
            return scores

        for it in range(NU):
            qkv = proj(it)
            done = []
            for i, h in enumerate(qkv):
                later(LAT_S + i * GAP_S, head(*divmod(it, 3), h, qkv, done))
            if hook is not None:
                hook(it)
        last = [(0, 1), (1, 1), (1, 8), (1, 13)]
        keys = range(NT) if raw else sorted(parts, key=lambda k: (k[1] == 6, k[0], ORDER.index(k[1])))
        m = {}
        end = None
        for key in keys:
            if end is None and not queue:
                end = clock[0] + LAT_O
            if key not in last and (end is None or clock[0] < end):
                m[key] = prod(key, 0, NG - 1)
        run_due(True)
        if hook is not None:
            hook(NU)
        early = list(m)
        for key in keys:
            if key not in early and key not in last and (raw or key[1] != 6):
                m[key] = prod(key, 0, NG)
        for key in early:
            m[key] = prod(key, NG - 1, NG) + m[key]
        if raw:
            return cols(*[m[i] for i in range(NT)])
        for key in ((0, 6), (1, 6)):
            if key not in early:
                m[key] = prod(key, 0, NG)
        res = []
        for part in range(2):
            res += _combine(lambda i: m[part, i] if (part, i) in m else prod((part, i), 0, NG),
                            2 + part, nr, full, True)
        return cols(*res)

    def side2(t, a2):
        x3 = x2_sc[(t - 2) & 3] + a2
        x4 = x3 + _ln(x3) * y_seg(t - 2)
        out_sc[seg(t - 2), LN] = x4.astype(out_sc.dtype)
        return x4

    def finish(t, xr, yt, mem, a1):
        x1 = xr.astype(F32) + a1
        x2 = x1 + _ln(x1) * yt
        h_sc[...] = mem
        x2_sc[t & 3] = x2
        return x2

    def staged(make, pins):
        keys = ((0, 0), (1, 0), (0, 3), (1, 3), (0, 5))
        events = sorted({0} | {g0 + n // per for g0, _, per in pins for n in range(NT)})
        made = {}
        for e in events:
            act = {}
            for g0, v, per in pins:
                for n in range(NT):
                    if g0 + n // per <= e:
                        act.setdefault(keys[n], []).append(_tile(v, n))
            made[e] = make(act)
        return lambda k: made[max(e for e in events if e <= k)]

    def wait_chunk(ci):
        for cp in w_copies(0, ci):
            cp.wait()

    def w_block(ci, b):
        x = pltpu.bitcast(st_sc[ci, b], U32)
        sub = jax.lax.broadcasted_iota(jnp.int32, (8, DH), 0)
        res = []
        for par in range(2):
            v = [x[2 * i + par] for i in range(4)]
            for bit in (2, 1):
                keep = (sub & bit) == 0
                for i in range(4):
                    if not i & bit:
                        a, c = v[i], v[i + bit]
                        v[i] = jnp.where(keep, a, pltpu.roll(c, bit, 0))
                        v[i + bit] = jnp.where(keep, pltpu.roll(a, 8 - bit, 0), c)
            res.append(v)
        return res

    def rhs_tiles(part, plain, value, pack, swap):
        def one(i, base, hs):
            terms = {kj: sg for kj, sg in RHS[i].items() if max(kj) < len(hs)}

            def at(kj):
                k, j = kj[::-1] if swap else kj
                return base + k, hs[j]
            if len(terms) == 1:
                return plain(*at(next(iter(terms))))
            return pack(_lin(terms, lambda kj: value(*at(kj))))
        if part == 0:
            for p in range(4):
                for i in range(7):
                    yield 4 * i + p, one(i, 0, (2 * p, 2 * p + 1))
        else:
            for u in range(2):
                for i in range(15):
                    yield T_TRI[u] + i, one(i, 2, TRIPLES[u])
            for i in range(7):
                yield T_LAST + i, one(i, 2, (6, 7))
            for j in range(2):
                yield T_TAIL + j, plain(4, 6 + j)

    GROUPS = ((0, 12, T_TRI[0]), (T_TRI[0], T_TRI[1], T_LAST, T_TAIL + 2))
    NGRP = 8 * (len(GROUPS[0]) + len(GROUPS[1]) - 2)

    def put_tiles(dst, slot, r0, part, tiles):
        out = dict(tiles)
        for lo, hi in zip(GROUPS[part], GROUPS[part][1:]):
            dst[slot, lo:hi, pl.ds(r0, 8), :] = jnp.stack([out[i] for i in range(lo, hi)])
            yield

    def chunk_work(item):
        for b in range(8):
            for part in range(2):
                yield from item(part, b)

    def relayout(ci, dst, slot, part, b):
        hi_m = U32(0xFFFF0000)
        t = {k: w_block(ci, 8 * k + b) for k in ((0, 1), (2, 3, 4))[part]}

        def plain(k, h):
            a, c = t[k][0][h // 2], t[k][1][h // 2]
            return (a >> 16) | (c & hi_m) if h % 2 else (a & U32(0xFFFF)) | (c << 16)

        @functools.lru_cache(None)
        def value(k, h):
            w = cols(t[k][0][h // 2], t[k][1][h // 2])
            return pltpu.bitcast(w & hi_m if h % 2 else w << 16, F32)

        def pack(v):
            r = pltpu.bitcast(v.astype(BF16).astype(F32), U32)
            return (r[:, :DH] >> 16) | r[:, DH:]
        yield from put_tiles(dst, slot, scaled(b, 8), part, rhs_tiles(part, plain, value, pack, False))

    def main(_, carry):
        for part in (1, 0):
            def relayout0(b, c, part=part):
                list(relayout(0, wa_sc, 0, part, b))
                return c
            with jax.named_scope("wait_w"):
                for cp in w_copies(0, part=part):
                    cp.wait()
            with jax.named_scope("relayout"):
                jax.lax.fori_loop(0, 8, relayout0, 0, unroll=2 - part)

        def pro_stage(ps_, b):
            n = ps_ * NRB + b
            with jax.named_scope("wait_w"):
                if ps_ == 0:
                    @pl.when(b + 1 < NRB)
                    def _():
                        x_copy(b + 1).wait()

                @pl.when((n >= 2) & (n <= NCH))
                def _():
                    wait_chunk(n - 1)
            cr = jnp.clip(n - 1, 0, NCH - 1)
            dst, slot = (wb_sc, cr) if ps_ == 0 else (wa_sc, cr - (NRB - 2))
            bl = jnp.minimum(b + 1, NRB - 1)
            PW = PRO_PW
            npc = RB * S2 // PW
            assert npc * PW == RB * S2 and 2 * NRB > UL

            def body(i, c):
                s0 = b * RB + 1
                for sg in range(RB):
                    hp_sc[sg * S2:(sg + 1) * S2, :] = xn_sc[s0 + sg]
                spread(chunk_work(functools.partial(relayout, cr, dst, slot)), dst, jnp.minimum(never_sm[0], 0), NGRP, *PRO_T)
                for pi in range(npc):
                    carry = {}
                    for u in range(3):
                        pos = 3 * pi + u
                        hx = hp_sc[pi * PW:(pi + 1) * PW, :]
                        for k in range(max(RB, 2 * NT)):
                            if PRO_X0 + k * PRO_XN // PRO_XD != pos:
                                continue
                            if ps_ == 0 and k < RB:
                                sn = bl * RB + 1 + k
                                xv = _ext(_ln(x_sc[seg(sn), LN].astype(F32)))
                                xn_sc[sn] = xv
                                hx = rows(hx[:-S2], jnp.where(never_sm[0] > 0, xv, hx[-S2:]))
                            if ps_ == 1 and k < 2 * NT:
                                conv_u(jnp.minimum(2 * b + k // NT, UL),
                                       slice((k % NT) * 128, (k % NT + 1) * 128))
                        for h, r in unit(w_tiles(ps_, (0,)), u, packed_lhs(hx), carry).items():
                            for a in range(0, 2 * PW, 16):
                                sg, off = divmod(2 * pi * PW + a, SEG)
                                pre_sc[s0 + sg, ps_ * HG + h, off:off + 16, :] = r[a:a + 16].astype(BF16)
                assert not queue
                return c
            assert PRO_X0 + (max(RB, 2 * NT) - 1) * PRO_XN // PRO_XD < 3 * npc
            with jax.named_scope("fused"):
                jax.lax.fori_loop(0, never_sm[0] + 1, body, 0)

        for ps_ in range(NPASS):
            if ps_ == 1:
                with jax.named_scope("wait_in0"):
                    for cp in small + in_copies(0):
                        cp.wait()
                sh = sh_ref[...].astype(F32)
                for j in range(KS):
                    co_sc[j] = jnp.broadcast_to(sh[j:j + 1], (8, DM))
                co_sc[KS] = jnp.broadcast_to(sd_ref[...].astype(F32).reshape(1, DM), (8, DM))

            def blk(b, c, ps_=ps_):
                pro_stage(ps_, b)
                return c
            jax.lax.fori_loop(0, NRB, blk, 0)

        def warm_block0(q):
            uf, kf = conv_fwd(0, q)
            put_spec(0, q, 0, uf)
            put_spec(0, q, 2, kf)
            kr_sc[q] = kf
            ur, um, kr, km = uf[:QB], uf[QB:], kf[:QB], kf[QB:]
            wf_sc[0, 0, q] = (ur * kr - um * km).astype(BF16)
            wf_sc[0, 1, q] = (ur * km + um * kr).astype(BF16)

        def wo_operands(g, part, b):
            def src(k, h):
                r = (g * HG + h) * DH + 16 * b
                return wo_sc[r:r + 16, k * 128:(k + 1) * 128]
            tiles = rhs_tiles(part, lambda k, h: _pack(src(k, h)),
                              functools.lru_cache(None)(lambda k, h: src(k, h).astype(F32)), _pack, True)
            yield from put_tiles(wc_sc, g, 8 * b, part, tiles)

        def wo_work():
            for g in range(NG):
                yield from chunk_work(functools.partial(wo_operands, g))

        def plain_qkv(eq, ekv, k, carry):
            g, u = divmod(k, 3)
            res = []
            for mats, e in (((1,), ekv), ((2,), ekv), ((0,), eq)):
                res.append(unit(w_tiles(g, mats), u, e, carry.setdefault(mats, {})))
            return {h: bf(res[2][h], res[0][h], res[1][h]) for h in res[0]}

        with jax.named_scope("wait_wo"):
            wo_copy.wait()
        with jax.named_scope("step0"):
            mem0 = mem0_ref[...].astype(F32)
            e0 = packed_lhs(rows(_ext(rows(mem0, mem0)), xn(0)))

            carry0 = {}
            spread(wo_work(), wc_sc, jnp.minimum(never_sm[0], 0), NG * NGRP, *WO_T)

            def hook0(it):
                if it < NQ:
                    warm_block0(it)
                if 5 <= it < 5 + NT:
                    for p in range(2):
                        conv_inv(p, it - 5)
            out = attend(lambda k: plain_qkv(e0, e0, k, carry0), RH, make_mask(RH, (0,)), hook0, True)
            y0 = y_seg(0)
            for q in range(2):
                conv_spec(1, q)
            for n in range(NT):
                conv_inv(2, n)
            finish(0, x_sc[0:SEG, LN], y0, rows(out[0:M], mem0), out[M2:])
            for q in range(2):
                for piece in MAC_PIECES:
                    conv_mac(1, q, piece, 2)

        mask12 = make_mask(R, (0, 1))

        def step(t, x2):
            c, q = (t + 1) // NQ + 1, (t + 1) % NQ
            mem = h_sc[...]
            n1 = _unpack(xn(t)[:, 0:DM]).astype(F32)
            lead = value_lhs(mem, (n1, None))[0]
            ahead = {ui: product(w_tiles(0, (1, 2)), ui[0], lead, ui[1]) for ui in AHEAD}
            if x2 is None:
                x2 = x2_sc[(t - 1) & 3]
            conv_spec(c, q)
            link = []
            for piece in MAC_PIECES:
                conv_mac(c, q, piece, NB, link)
            n2 = _ln(x2)
            x4 = side2(t, op_sc[...])
            un = conv_u(t + UL)
            left = staged(lambda p: value_lhs(mem, (n1, n2), p), [(PIN_U, un, 2), (PIN_X4, x4, NT)])
            left_q = value_lhs(rows(mem, n2))
            carry = {}

            def proj(k):
                g, u = divmod(k, 3)
                pre = g * HG < NPA
                if pre:
                    qs = unit(w_tiles(g, (0,)), u, left_q, carry.setdefault("q", {}))
                rs = unit(w_tiles(g, (1, 2) if pre else (1, 2, 0)), u, left(k), carry.setdefault("kv", {}),
                          ahead if g == 0 else ())
                res = {}
                for h, r in rs.items():
                    if pre:
                        qq = rows(qs[h][:M2], pre_sc[t, g * HG + h].astype(F32), qs[h][M2:])
                    else:
                        qq = r[:, 2 * DH:]
                    res[h] = bf(qq, r[:, :DH], r[:, DH:2 * DH])
                return res

            held = {}

            def hook(it):
                if INV_AT <= it < INV_AT + NT:
                    conv_inv(t + 2, it - INV_AT)
                if it == NU:
                    held["x"] = x_sc[seg(t), LN]
                    held["y"] = y_seg(t)
            out = attend(proj, R, mask12, hook)
            op_sc[...] = out[RH:]
            return finish(t, held["x"], held["y"], out[0:M2], out[M2:RH])

        def steps(i, carry):
            x2 = None
            for j in range(UNROLL):
                x2 = step(1 + i * UNROLL + j, x2)
            return carry

        def phase(p, carry):
            @pl.when(p == 1)
            def _():
                for cp in in_copies(2):
                    cp.wait()

            @pl.when(p >= 2)
            def _():
                out_copy((p - 2) * PH, PH).start()

            with jax.named_scope("steps"):
                jax.lax.fori_loop(p * PHI, (p + 1) * PHI, steps, 0)
            return carry

        for cp in in_copies(1):
            cp.wait()
        jax.lax.fori_loop(0, NPH, phase, 0)
        out_copy((NPH - 2) * PH, NSEG - 2 - (NPH - 2) * PH).start()

        with jax.named_scope("step_last"):
            x4 = side2(NSEG, op_sc[...])
            n2 = _ln(x2_sc[(NSEG - 1) & 3])
            left_q = value_lhs(n2)
            left = staged(lambda p: value_lhs(rows(h_sc[...], n2), None, p), [(PIN_X4, x4, NT)])
            carry1 = {}
            out = attend(lambda k: plain_qkv(left_q, left(k), k, carry1),
                         SEG, make_mask(RH, (1,), M2))
            side2(NSEG + 1, out)
        out_copy(NSEG - 2, 2).start()
        out_copy(0, NSEG).wait()
        return carry

    jax.lax.fori_loop(0, never_sm[0] + 1, main, 0)


def pallas_interleave_layers__memory_aug_recurrent_mem_tr__ssm_conv_h3__prompt_kernel(
    A_x, A_mem0, A_Wq, A_Wk, A_Wv, A_Wo, A_seg_len,
    B_q, B_k, B_v, B_shift_k, B_ssm_k, B_ssm_D,
):
    del B_q
    seg = int(A_seg_len) if isinstance(A_seg_len, (int, np.integer)) else CB // NQ
    return _run(A_x, A_mem0, A_Wq, A_Wk, A_Wv, A_Wo, B_k, B_v, B_shift_k, B_ssm_k, B_ssm_D, SEG=seg)


@functools.partial(jax.jit, static_argnames=("SEG",))
def _run(A_x, A_mem0, A_Wq, A_Wk, A_Wv, A_Wo, B_k, B_v, B_shift_k, B_ssm_k, B_ssm_D, *, SEG):
    B, S, DM = A_x.shape
    assert B == 1
    H, DH = A_Wq.shape[1], A_Wq.shape[2]
    M = A_mem0.shape[1]
    KS = B_shift_k.shape[1]
    R = 2 * (M + SEG)
    NSEG = S // SEG
    NRB = (NSEG - 1) // RB
    NB = S // CB
    QB = CB // NQ
    NCH = 3 * H // HG
    DP = -(-DM // 256) * 256
    fwd, inv = _dft_constants()

    kern = functools.partial(_kernel, S=S, DM=DM, H=H, DH=DH, M=M, SEG=SEG)
    any_spec = pl.BlockSpec(memory_space=pl.ANY)
    out = pl.pallas_call(
        kern,
        out_shape=jax.ShapeDtypeStruct((S, DM), A_x.dtype),
        in_specs=[any_spec] * 13,
        out_specs=any_spec,
        scratch_shapes=[
            pltpu.VMEM((NB + 2, NQ, QB // 8, DM // 128, 4, 8, 128), F32),
            pltpu.VMEM((NQ, 2 * QB, DM), F32),
            pltpu.VMEM((2, 2, NQ, QB, DM), BF16),
            pltpu.VMEM((4, SEG, DM), F32),
            pltpu.VMEM((2 * CB, DP), F32),
            pltpu.VMEM((S, DP), BF16),
            pltpu.VMEM((SEG, DM), F32),
            pltpu.VMEM((NSEG, NPA, SEG, DH), BF16),
            pltpu.VMEM((NSEG, SEG // 2, DM + 384), U32),
            pltpu.VMEM((NCH - NRB + 2, N_TILES, 64, DH), U32),
            pltpu.VMEM((NRB - 1, N_TILES, 64, DH), U32),
            pltpu.VMEM((H * DH, DM), BF16),
            pltpu.VMEM((H // HG, N_TILES, 64, DH), U32),
            pltpu.VMEM((S, DP), BF16),
            pltpu.VMEM((S, DP), BF16),
            pltpu.VMEM((NB, DM, CB), BF16),
            pltpu.VMEM((NCH, DM // 16, 8, 2 * HG, DH), BF16),
            pltpu.VMEM((S, DP), A_x.dtype),
            pltpu.VMEM(fwd.shape, BF16),
            pltpu.VMEM(inv.shape, BF16),
            pltpu.VMEM((S + KPAD, DP), BF16),
            pltpu.VMEM((RB * SEG // 2, DM + 384), U32),
            pltpu.VMEM((2 * M, DM), F32),
            pltpu.VMEM((KS + 1, 8, DM), F32),
            pltpu.VMEM((M, DM), BF16),
            pltpu.VMEM((KS, DM), BF16),
            pltpu.VMEM((DM,), BF16),
            pltpu.SMEM((1,), jnp.int32),
            pltpu.SemaphoreType.DMA(((NSEG - 1) // RB,)),
            pltpu.SemaphoreType.DMA((3,)),
            pltpu.SemaphoreType.DMA((NCH + 2,)),
            pltpu.SemaphoreType.DMA(()),
        ],
        compiler_params=pltpu.CompilerParams(vmem_limit_bytes=120 * 1024 * 1024),
    )(
        A_x.reshape(S, DM), A_mem0.reshape(M, DM),
        *[w.reshape(DM // 16, 2, 8, H, DH) for w in (A_Wq, A_Wk, A_Wv)],
        A_Wo.reshape(H * DH, DM), B_k.reshape(S, DM), B_v.reshape(S, DM),
        B_shift_k.T, B_ssm_k, B_ssm_D,
        jnp.asarray(fwd, BF16), jnp.asarray(inv, BF16),
    )
    return out.reshape(B, S, DM)
```

```python
import functools

import numpy as np
import jax
import jax.numpy as jnp
import jax.experimental.pallas as pl
import jax.experimental.pallas.tpu as pltpu

F32 = jnp.float32
BF16 = jnp.bfloat16
U32 = jnp.uint32

CB = 128
NQ = 4
KPAD = 16
HG = 8
NPA = 16
RB = 9
PRO_PW, PRO_X0, PRO_XN, PRO_XD = 24, 3, 3, 2
PRO_T, WO_T = (20, 2820), (20, 6200)
UNROLL = 3
PHI = 3
INV_AT, PIN_U, PIN_X4 = 7, 2, 6

LHS = ({(0, 0): 1}, {(0, 0): 1, (1, 0): 1}, {(0, 1): 1, (1, 1): 1}, {(1, 1): 1}, {(0, 0): 1, (1, 1): 1},
       {(0, 1): 1, (0, 0): -1}, {(1, 1): 1, (1, 0): -1}, {(0, 2): 1}, {(1, 2): 1},
       {(0, 0): 1, (1, 0): 1, (1, 2): -1}, {(0, 2): 1, (1, 2): 1, (0, 0): -1, (1, 0): -1},
       {(1, 2): 1, (1, 0): -1}, {(0, 1): 1, (1, 1): 1, (0, 2): -1},
       {(0, 2): 1, (1, 2): 1, (0, 1): -1, (1, 1): -1}, {(0, 1): 1, (0, 2): -1})
RHS = ({(0, 0): 1, (1, 0): 1, (0, 2): -1}, {(0, 0): 1, (2, 0): 1, (0, 1): -1},
       {(1, 1): 1, (2, 1): 1, (1, 0): -1}, {(1, 1): 1, (0, 1): 1, (1, 2): -1}, {(0, 1): 1, (1, 0): 1},
       {(1, 0): 1}, {(0, 1): 1}, {(2, 2): 1, (1, 2): 1, (2, 0): -1}, {(2, 2): 1, (0, 2): 1, (2, 1): -1},
       {(0, 2): 1, (2, 0): 1}, {(2, 0): 1}, {(0, 2): 1}, {(1, 2): 1, (2, 1): 1}, {(2, 1): 1}, {(1, 2): 1})
RIDE = {0: {0: 1}, 3: {1: 1}, 5: {1: 1, 0: -1}, 6: {1: 1, 0: -1}, 7: {2: 1}, 10: {2: 1}, 11: {0: 1},
        12: {2: 1}, 14: {1: 1, 2: -1}}
RIDE_TILE = ({0: 0, 3: 1, 5: 5, 6: 5}, {0: 2, 3: 3, 5: 6, 6: 6, 7: 4, 10: 4, 11: 2, 12: 4, 14: 7})
AHEAD = ((3, 0), (3, 5), (0, 0), (0, 5), (0, 14), (0, 7), (1, 0), (1, 5))
LAT = (300, 200, 620, 250)
LAT_FIRST, LAT_LAST = (300, 120, 620, 250), (250, 120, 520, 200)
ORDER = (0, 4, 5, 2, 3, 1, 6, 9, 11, 10, 13, 12, 8, 14, 7)
TRIPLES = ((0, 1, 2), (4, 5, 3))
T_TRI, T_LAST, T_TAIL, N_TILES = (28, 43), 58, 65, 68


def _lin(terms, get):
    acc = None
    for key, sign in terms.items():
        v = get(key)
        acc = v if acc is None else (acc + v if sign > 0 else acc - v)
    return acc


def _combine(product, n, nr, paired, x2_last=False):
    m = functools.lru_cache(None)(product)

    def r(i):
        return m(i)[:nr]

    def x(i):
        return m(i)[nr:] if i in RIDE else m(i)
    if not paired:
        rid = [m(0) + m(5), m(3) - m(6)]
        if n == 3:
            v = m(10) + m(11)
            rid = [rid[0] + v, rid[1] + m(12) + m(14), m(7) + v + m(14)]
        return rid
    if not x2_last:
        x(0)
        p = x(4) - x(0)
        a = m(0) + m(5)
        w = x(4) + x(5) + x(2) - x(3)
        p = p + x(1)
        b = m(3) - m(6)
        rid, top, bot = [a[:nr], b[:nr]], [a[nr:], w], [p - x(6), b[nr:]]
        if n == 3:
            t = x(9) + x(11)
            t0 = t + x(10)
            v = r(10) + r(11)
            rid[0], top[0], bot[0] = rid[0] + v, top[0] + t0, bot[0] - t
            x(13), x(12)
            z = x(8) - x(11)
            u = x(12) - x(14)
            t1 = u + x(13)
            rid[1], top[1], bot[1] = rid[1] + r(12) + r(14), top[1] - u, bot[1] + t1
            c = m(7) + m(14)
            rid.append(c[:nr] + v)
            top.append(c[nr:] + t0)
            bot.append(z + t1)
        return [jnp.concatenate(p, axis=0) for p in zip(rid, top, bot)]
    a = m(0) + m(5)
    w = x(4) + x(5) - x(3)
    top = [a[nr:], w + x(2)]
    if n == 3:
        t = x(11) + x(9)
        t0 = t + x(10)
        v = r(10) + r(11)
        u = x(12) - x(14)
        top = [top[0] + t0, top[1] - u, x(7) + t0 + x(14)]

    def rest():
        b = m(3) - m(6)
        rid = [a[:nr], b[:nr]]
        bot = [x(4) - x(0) - x(6), b[nr:]]
        if n == 3:
            rid = [rid[0] + v, rid[1] + r(12) + r(14), r(7) + v + r(14)]
        yield
        if n == 3:
            t1 = u + x(13)
            bot = [bot[0] - t, bot[1] + t1, t1 - x(11) + x(8)]
        bot[0] = bot[0] + x(1)
        yield [jnp.concatenate(p, axis=0) for p in zip(rid, top, bot)]
    return rest()


def _dft_constants():
    qb = CB // NQ
    hb = qb // 2
    n = np.arange(CB, dtype=np.float64)
    f = np.concatenate([q * qb + np.concatenate([np.arange(0, qb, 2), np.arange(1, qb, 2)])
                        for q in range(NQ)])
    w = np.pi * (2.0 * f + 1.0) / (2 * CB)
    ang = (w[:, None] * (n[None, :] - (CB - 1) / 4.0)).reshape(NQ, qb, CB)
    fwd = np.concatenate([np.cos(ang), -np.sin(ang)], axis=1)
    inv = np.zeros((NQ, 2, hb, CB))
    for p in range(NQ):
        m = (NQ - 1 - p) * hb + np.arange(hb)
        ang = (m[:, None] + 0.5) * w[None, :]
        inv[p, 0] = np.cos(ang) / CB
        inv[p, 1] = -np.sin(ang) / CB
    return fwd.astype(np.float32), inv.astype(np.float32)


def _flip_rows(x):
    i = jax.lax.broadcasted_iota(jnp.int32, (8, x.shape[1]), 0)
    out = []
    for r in range(x.shape[0] - 8, -8, -8):
        v = pltpu.roll(x[r:r + 8], 4, 0)
        for b in (2, 1):
            v = jnp.where((i & b) == 0, pltpu.roll(v, 8 - b, 0), pltpu.roll(v, b, 0))
        out.append(v)
    return jnp.concatenate(out, axis=0)


def _ln(x, eps=1e-5):
    d = x.shape[-1]
    m = jnp.sum(x, axis=-1, keepdims=True) * (1.0 / d)
    xc = x - m
    v = jnp.sum(xc * xc, axis=-1, keepdims=True) * (1.0 / d)
    return xc * jax.lax.rsqrt(v + eps)


def _dot(a, b):
    return jnp.dot(a, b, preferred_element_type=F32)


def _dot_nt(a, b):
    return jax.lax.dot_general(a, b, (((1,), (1,)), ((), ())), preferred_element_type=F32)


def _pack(x):
    return pltpu.bitcast(x.astype(BF16), U32)


def _unpack(x):
    return pltpu.bitcast(x, BF16)


def _tile(x, n):
    return x[:, n * 128:(n + 1) * 128]


def _ext(r):
    return _pack(jnp.concatenate(
        [r, _tile(r, 1) - _tile(r, 0), _tile(r, 3) - _tile(r, 2), _tile(r, 3) - _tile(r, 4)], axis=1))


def _in_order(actions):
    def body(i, c):
        for j, act in enumerate(actions):
            pl.when(i == j)(act)
        return c
    jax.lax.fori_loop(0, len(actions), body, 0)


def _kernel(x_hbm, mem0_hbm, wq_hbm, wk_hbm, wv_hbm, wo_hbm, k_hbm, v_hbm,
            sh_hbm, sk_hbm, sd_hbm, fwd_hbm, inv_hbm, o_hbm,
            sp_sc, kr_sc, wf_sc, x2_sc, y_sc, u_sc, op_sc, pre_sc, xn_sc, wa_sc, wb_sc, wo_sc, wc_sc,
            x_sc, v_sc, sk_sc, st_sc, out_sc, fwd_ref, inv_ref,
            k_sc, hp_sc, h_sc, co_sc, mem0_ref, sh_ref, sd_ref,
            never_sm, sem_x, sem_in, sem_w, sem_out,
            *, S, DM, H, DH, M, SEG):
    NSEG = S // SEG
    M2 = 2 * M
    S2 = SEG // 2
    R = M2 + 2 * SEG
    RH = M2 + SEG
    NB = S // CB
    QB = CB // NQ
    HB = QB // 2
    NT = DM // 128
    PH = PHI * UNROLL
    NRB = (NSEG - 1) // RB
    NPH = (NSEG - 1) // PH
    NG = H // HG
    NCH = 3 * NG
    NPASS = NPA // HG
    NU = 3 * NG
    KS = sh_ref.shape[0]
    UL = 2 * NQ + 1
    LN = pl.ds(0, DM)
    assert NT == 5 and HG == 8 and DH == 128 and 2 <= KS <= 8 and QB == SEG and NRB * RB == NSEG - 1 and NPH * PH == NSEG - 1 and NPASS == 2 and 2 * NRB >= NCH + 1

    mem0_copy = pltpu.make_async_copy(mem0_hbm, mem0_ref, sem_x.at[0])
    small = [pltpu.make_async_copy(s, d, sem_in.at[0]) for s, d in [
        (sh_hbm, sh_ref), (sd_hbm, sd_ref), (fwd_hbm, fwd_ref), (inv_hbm, inv_ref)]]

    def x_copy(b):
        if isinstance(b, int) and b == 0:
            rows = pl.ds(0, (RB + 1) * SEG)
        else:
            rows = pl.ds(pl.multiple_of((b * RB + 1) * SEG, SEG), RB * SEG)
        return pltpu.make_async_copy(x_hbm.at[rows], x_sc.at[rows, LN], sem_x.at[b])

    kb = (0, (UL + 1) * SEG, (UL + PH + 1) * SEG, S)
    sb = (0, 2, (PH + 2) // NQ + 2, NB)

    def in_copies(part):
        def rng(b):
            return pl.ds(b[part], b[part + 1] - b[part])
        sem = sem_in.at[part]
        return [
            pltpu.make_async_copy(k_hbm.at[rng(kb)],
                                  k_sc.at[pl.ds(KPAD + kb[part], kb[part + 1] - kb[part]), LN], sem),
            pltpu.make_async_copy(v_hbm.at[rng(kb)], v_sc.at[rng(kb), LN], sem),
        ] + [pltpu.make_async_copy(sk_hbm.at[:, pl.ds(c * CB, CB)], sk_sc.at[c], sem)
             for c in range(sb[part], sb[part + 1])]

    def w_copies(ci, dst=None, part=None):
        src = (wq_hbm, wk_hbm, wv_hbm)[ci // NG]
        dst = ci if dst is None else dst
        spans = {None: [(0, DM // 16)], 0: [(0, 16)], 1: [(16, DM // 16)]}[part]
        sem = sem_w.at[NCH + 1 if part == 1 else dst]
        return [pltpu.make_async_copy(
            src.at[pl.ds(lo, hi - lo), hf, :, pl.ds((ci % NG) * HG, HG), :],
            st_sc.at[dst, pl.ds(lo, hi - lo), :, pl.ds(hf * HG, HG), :], sem)
            for lo, hi in spans for hf in range(2)]

    wo_copy = pltpu.make_async_copy(wo_hbm, wo_sc, sem_w.at[NCH])

    def out_copy(lo, n):
        rows = pl.ds(lo * SEG if isinstance(lo, int) else pl.multiple_of(lo * SEG, SEG), n * SEG)
        return pltpu.make_async_copy(out_sc.at[rows, LN], o_hbm.at[rows], sem_out)

    def start_all(cps):
        def act():
            for cp in cps:
                cp.start()
        return act

    order = [[mem0_copy, x_copy(0)], w_copies(0, part=1), w_copies(0, part=0), [x_copy(1)], [x_copy(2)]]
    for ci in range(1, NCH):
        order.append(w_copies(ci) + ([x_copy(ci + 2)] if ci + 2 < NRB else []))
        if ci == NRB - 2:
            order.append(small + in_copies(0))
    order += [[wo_copy], in_copies(1), in_copies(2)]
    for i in range(0, len(order), 5):
        _in_order([start_all(cps) for cps in order[i:i + 5]])

    never_sm[0] = 0
    k_sc[0:KPAD, LN] = jnp.zeros((KPAD, DM), BF16)
    sp_sc[NB + 1] = jnp.zeros(sp_sc.shape[1:], F32)
    op_sc[...] = jnp.zeros(op_sc.shape, F32)
    x2_sc[...] = jnp.zeros(x2_sc.shape, F32)
    y_sc[2 * CB - SEG:, LN] = jnp.zeros((SEG, DM), F32)
    mem0_copy.wait()
    x_copy(0).wait()
    for sg in range(RB + 1):
        xn_sc[sg] = _ext(_ln(x_sc[sg * SEG:(sg + 1) * SEG, LN].astype(F32)))

    def clip(i, hi):
        return min(max(i, 0), hi) if isinstance(i, int) else jnp.clip(i, 0, hi)

    def scaled(i, m):
        return i * m if isinstance(i, int) else pl.multiple_of(i * m, m)

    def seg(i):
        return pl.ds(scaled(clip(i, NSEG - 1), SEG), SEG)

    def conv_u(s, ln=LN):
        r0 = scaled(clip(s, NSEG - 1), SEG)
        kk = k_sc[pl.ds(r0, KPAD + SEG), ln].astype(F32)[KPAD - 8:]

        def coef(j, rows):
            return jnp.concatenate([co_sc[j, :, ln]] * (rows // 8), axis=0)
        sft = [kk] + [pltpu.roll(kk, j, 0) for j in range(2, KS, 2)]
        ev = functools.reduce(jnp.add, [sft[j // 2][8:] * coef(j, SEG) for j in range(0, KS, 2)])
        od = functools.reduce(jnp.add, [sft[j // 2] * coef(j, SEG + 8) for j in range(1, KS, 2)])
        ks = ev + pltpu.roll(od, 1, 0)[8:]
        u = ks * v_sc[pl.ds(r0, SEG), ln].astype(F32)
        u_sc[pl.ds(r0, SEG), ln] = u.astype(BF16)
        return u

    def conv_fwd(c, q):
        cc = clip(c, NB - 1)
        f = fwd_ref[q]
        uf = _dot(f, u_sc[pl.ds(scaled(cc, CB), CB), LN])
        kf = _dot_nt(f, sk_sc[cc])
        return uf, kf

    def put_spec(cs, q, which, val):
        for n in range(NT):
            v = val[:, n * 128:(n + 1) * 128].reshape(2, QB // 8, 8, 128)
            sp_sc[cs, q, :, n, which:which + 2] = jnp.stack([v[0], v[1]], axis=1)

    def conv_spec(c, q):
        uf, kf = conv_fwd(c, q)
        cs = clip(c, NB)
        put_spec(cs, q, 0, uf)
        pk = kr_sc[q]
        kr_sc[q] = kf
        kp = jnp.concatenate([
            kf[0:HB] - pk[QB:QB + HB],
            kf[HB:QB] + pk[QB + HB:],
            kf[QB:QB + HB] + pk[0:HB],
            kf[QB + HB:] - pk[HB:QB]], axis=0)
        put_spec(cs, q, 2, kp)

    MAC_PIECES = [(rb, n) for rb in range(QB // 16) for n in range(NT)]

    def conv_mac(c, q, piece, nterms, link=None):
        rb2, n = piece
        cs = clip(c, NB)
        rbs = slice(2 * rb2, 2 * rb2 + 2)
        us, ks = [], []
        for j in range(nterms):
            if isinstance(cs, int):
                uj, kj = j, cs - j
            else:
                uj = jnp.minimum(j, cs)
                kj = jnp.where(cs - j >= 0, cs - j, NB + 1)
            us.append(sp_sc[uj, q, rbs, n, 0:2])
            ks.append(sp_sc[kj, q, rbs, n, 2:4])
        acc = []
        for rb in range(2):
            z = jnp.zeros((8, 128), F32) if not link else jnp.where(never_sm[0] > 0, link[0], 0.0)
            ar = ai = z
            for u, k in zip(us, ks):
                ar = ar + u[rb, 0] * k[rb, 0]
                ai = ai + u[rb, 0] * k[rb, 1]
                ar = ar - u[rb, 1] * k[rb, 1]
                ai = ai + u[rb, 1] * k[rb, 0]
            acc.append((ar, ai))
            if link is not None:
                link[:] = [ar]
        ln = slice(n * 128, (n + 1) * 128)
        w = jnp.concatenate([acc[0][0], acc[1][0], acc[0][1], acc[1][1]], axis=0).astype(BF16)
        wf_sc[c & 1, 0, q, rb2 * 16:rb2 * 16 + 16, ln] = w[0:16]
        wf_sc[c & 1, 1, q, rb2 * 16:rb2 * 16 + 16, ln] = w[16:]

    def conv_inv(tt, n):
        cb = tt // NQ
        p = tt % NQ
        ln = slice(n * 128, (n + 1) * 128)
        ev = _dot(inv_ref[p, 0], wf_sc[cb & 1, 0, :, :, ln].reshape(CB, 128))
        od = _dot(inv_ref[p, 1], wf_sc[cb & 1, 1, :, :, ln].reshape(CB, 128))
        sd = jnp.concatenate([co_sc[KS, :, ln]] * (HB // 8), axis=0)
        for r, val in ((p, _flip_rows(ev - od)), (2 * NQ - 1 - p, ev + od)):
            ur = scaled(clip(cb, NB - 1) * (2 * NQ) + r, HB)
            yr = scaled((cb & 1) * (2 * NQ) + r, HB)
            y_sc[pl.ds(yr, HB), ln] = val + u_sc[pl.ds(ur, HB), ln].astype(F32) * sd

    def y_seg(s):
        return y_sc[pl.ds(scaled(s & (2 * NQ - 1), SEG), SEG), LN]

    scale = DH ** -0.5
    cexp = scale * float(np.log2(np.e))

    def make_mask(n, x_layers, q0=0):
        qi = jax.lax.broadcasted_iota(jnp.int32, (n - q0, n), 0) + q0
        ki = jax.lax.broadcasted_iota(jnp.int32, (n - q0, n), 1)

        def layer(i):
            xl = jnp.where(i < M2 + SEG, x_layers[0], x_layers[-1])
            return jnp.where(i < M, 0, jnp.where(i < M2, 1, xl))
        same = layer(qi) == layer(ki)
        ok = same & ((qi < M2) | (ki < M2) | (qi >= ki))
        fill = jnp.where(same, -1e9 / scale, -jnp.inf).astype(F32)
        return ok, fill

    def probs(q, k, mask):
        ok, fill = mask
        s = _dot_nt(q, k)
        s = jnp.where(ok, s, fill)
        m = jnp.max(s, axis=-1, keepdims=True)
        p = jnp.exp2((s - m) * cexp)
        l = jnp.sum(p, axis=-1, keepdims=True)
        r = pl.reciprocal(l, approx=True)
        r = r * (2.0 - l * r)
        return (p * r).astype(BF16)

    def w_slot(ci):
        return (wb_sc, ci) if 1 <= ci < NRB - 1 else (wa_sc, max(ci - (NRB - 2), 0))

    def rows(*parts):
        return jnp.concatenate(parts, axis=0)

    def cols(*parts):
        return jnp.concatenate(parts, axis=1)

    def bf(*xs):
        return tuple(x.astype(BF16) for x in xs)

    def xn(s):
        return xn_sc[clip(s, NSEG - 1)]

    clock = [0]
    queue = []
    recent = [None]

    def later(delay, act):
        queue.append((clock[0] + delay, act))

    def run_due(force=False):
        while queue:
            item = min(queue, key=lambda it: it[0])
            if item[0] > clock[0] and not force:
                break
            queue.remove(item)
            clock[0] = max(clock[0], item[0])
            item[1]()

    def mm(a, w):
        run_due()
        clock[0] += a.shape[0] * w.size // (4 * 128 * 128)
        recent[0] = _dot(a, w)
        return recent[0]

    def spread(work, ref, slot, count, t0, t1):
        def act():
            ref[slot, N_TILES - 1, 0:8, :] = pltpu.bitcast(recent[0][0:8, 0:DH], U32)
            next(work)
        for i in range(count):
            later(t0 + i * (t1 - t0) // count, act)

    def packed_lhs(rid):
        def lhs(parts, i):
            return _unpack(cols(*[_tile(rid, 4 if i is None else RIDE_TILE[p][i]) for p in parts]))
        return lhs, 2 * rid.shape[0], False

    def value_lhs(rid, pair=None, pins=None):
        @functools.lru_cache(None)
        def lhs(parts, i):
            def one(p):
                if i is None:
                    return rows(*[_tile(r, 4) for r in (rid,) + (pair or ())])
                ps = [_lin(RIDE[i], lambda k: _tile(rid, 2 * p + k))] if i in RIDE else []
                if pair:
                    ps.append(_lin(LHS[i], lambda rk: _tile(pair[rk[0]], 2 * p + rk[1])))
                for v in (pins or {}).get((p, i), ()):
                    ps[-1] = rows(*([ps[-1][:-SEG]] if ps[-1].shape[0] > SEG else []),
                                  jnp.where(never_sm[0] > 0, v, ps[-1][-SEG:]))
                return rows(*ps)
            return cols(*[one(p) for p in parts]).astype(BF16)
        return lhs, rid.shape[0], pair is not None

    def product(tile, u, lhs, i):
        base = T_TRI[u] if u < 2 else T_LAST
        if u == 3:
            a, w = lhs((0,), i), tile(4 * i + 1)
        elif i < 7:
            a, w = lhs((0, 1), i), rows(tile(4 * i + (0, 2, 3)[u]), tile(base + i))
        else:
            a, w = lhs((1,), i), tile(base + i)
        return mm(a, w)

    def unit(tile, u, left, carry, ahead=()):
        lhs, nr, paired = left

        def comb(uu, n):
            return _combine(lambda i: ahead[uu, i] if (uu, i) in ahead else product(tile, uu, lhs, i),
                            n, nr, paired)
        if u == 2:
            c = comb(2, 2)
            return {6 + j: mm(lhs((1,), None), tile(T_TAIL + j)) + c[j] for j in range(2)}
        if u == 0:
            carry[2], carry[3] = comb(3, 2)
        c = comb(u, 3)
        hs = TRIPLES[u]
        return {hs[0]: c[0], hs[1]: c[1], hs[2]: c[2] + carry.pop(hs[2])}

    def w_tiles(g, mats):
        slots = [w_slot(mi * NG + g) for mi in mats]
        return lambda i: _unpack(cols(*[ref[k, i] for ref, k in slots]))

    def attend(proj, n, mask, hook=None, raw=False):
        full = n == R
        LAT_S, GAP_S, LAT_P, LAT_O = LAT if full else LAT_FIRST if raw else LAT_LAST
        nr = M2 if full else n
        parts = {}
        os_ = {}

        def add_forms(g, hs, ids):
            for i in range(7 if len(hs) == 2 else 15):
                ps = []
                if i in RIDE:
                    ps.append(_lin(RIDE[i], lambda k: os_[hs[k]][:nr]))
                if full:
                    ps.append(_lin(LHS[i], lambda rk: os_[hs[rk[1]]][M2 + rk[0] * SEG:RH + rk[0] * SEG]))
                if ps:
                    a = rows(*ps).astype(BF16)
                    for part, tid in ids(i):
                        parts.setdefault((part, i), []).append((g, a, tid))

        def prod(key, g0, g1):
            assert len(ready) >= 3 * g1
            if raw:
                a = cols(*[parts[h] for h in range(g0 * HG, g1 * HG)])
                return mm(a, wo_sc[g0 * HG * DH:g1 * HG * DH, key * 128:(key + 1) * 128])
            sel = [p for p in parts[key] if g0 <= p[0] < g1]
            return mm(cols(*[p[1] for p in sel]), _unpack(rows(*[wc_sc[p[0], p[2]] for p in sel])))

        ready = []

        def forms(g, u, hs):
            assert len(ready) == 3 * g + u
            ready.append(u)
            if raw:
                parts.update({g * HG + h: os_[h].astype(BF16) for h in hs})
            elif u < 2:
                add_forms(g, TRIPLES[u], lambda i: [(1, T_TRI[u] + i)] + ([(0, 4 * i + 2 * u)] if i < 7 else []))
                if u == 1:
                    add_forms(g, (2, 3), lambda i: [(0, 4 * i + 1)])
            else:
                add_forms(g, (6, 7), lambda i: [(0, 4 * i + 3), (1, T_LAST + i)])
                for j in range(2):
                    parts[1, 7].append((g, os_[6 + j][:min(n, RH)].astype(BF16), T_TAIL + j))
                    if full:
                        parts[1, 8].append((g, os_[6 + j][RH:].astype(BF16), T_TAIL + j))

        def head(g, u, h, qkv, done):
            def values(p):
                assert len(ready) >= 3 * g + u - 1
                os_[h] = _dot(p, qkv[h][2])
                clock[0] += n // 4
                done.append(h)
                if len(done) == len(qkv):
                    forms(g, u, done)

            def scores():
                p = probs(qkv[h][0], qkv[h][1], mask)
                clock[0] += n // 4
                later(LAT_P, lambda: values(p))
            return scores

        for it in range(NU):
            qkv = proj(it)
            done = []
            for i, h in enumerate(qkv):
                later(LAT_S + i * GAP_S, head(*divmod(it, 3), h, qkv, done))
            if hook is not None:
                hook(it)
        last = [(0, 1), (1, 1), (1, 8), (1, 13)]
        keys = range(NT) if raw else sorted(parts, key=lambda k: (k[1] == 6, k[0], ORDER.index(k[1])))
        m = {}
        end = None
        for key in keys:
            if end is None and not queue:
                end = clock[0] + LAT_O
            if key not in last and (end is None or clock[0] < end):
                m[key] = prod(key, 0, NG - 1)
        run_due(True)
        if hook is not None:
            hook(NU)
        early = list(m)
        for key in keys:
            if key not in early and key not in last and (raw or key[1] != 6):
                m[key] = prod(key, 0, NG)
        for key in early:
            m[key] = prod(key, NG - 1, NG) + m[key]
        if raw:
            return cols(*[m[i] for i in range(NT)])
        res = [_combine(lambda i, p=p: m[p, i] if (p, i) in m else prod((p, i), 0, NG), 2 + p, nr, full, True)
               for p in range(2)]
        if full:
            [next(g) for g in res]
            res = [next(g) for g in res]
        return cols(*(res[0] + res[1]))

    def side2(t, a2):
        x3 = x2_sc[(t - 2) & 3] + a2
        x4 = x3 + _ln(x3) * y_seg(t - 2)
        out_sc[seg(t - 2), LN] = x4.astype(out_sc.dtype)
        return x4

    def finish(t, xr, yt, mem, a1):
        x1 = xr.astype(F32) + a1
        x2 = x1 + _ln(x1) * yt
        h_sc[...] = mem
        x2_sc[t & 3] = x2
        return x2

    def staged(make, pins):
        keys = ((0, 0), (1, 0), (0, 3), (1, 3), (0, 5))
        events = sorted({0} | {g0 + n // per for g0, _, per in pins for n in range(NT)})
        made = {}
        for e in events:
            act = {}
            for g0, v, per in pins:
                for n in range(NT):
                    if g0 + n // per <= e:
                        act.setdefault(keys[n], []).append(_tile(v, n))
            made[e] = make(act)
        return lambda k: made[max(e for e in events if e <= k)]

    def wait_chunk(ci):
        for cp in w_copies(0, ci):
            cp.wait()

    def w_block(ci, b):
        x = pltpu.bitcast(st_sc[ci, b], U32)
        sub = jax.lax.broadcasted_iota(jnp.int32, (8, DH), 0)
        res = []
        for par in range(2):
            v = [x[2 * i + par] for i in range(4)]
            for bit in (2, 1):
                keep = (sub & bit) == 0
                for i in range(4):
                    if not i & bit:
                        a, c = v[i], v[i + bit]
                        v[i] = jnp.where(keep, a, pltpu.roll(c, bit, 0))
                        v[i + bit] = jnp.where(keep, pltpu.roll(a, 8 - bit, 0), c)
            res.append(v)
        return res

    def rhs_tiles(part, plain, value, pack, swap):
        def one(i, base, hs):
            terms = {kj: sg for kj, sg in RHS[i].items() if max(kj) < len(hs)}

            def at(kj):
                k, j = kj[::-1] if swap else kj
                return base + k, hs[j]
            if len(terms) == 1:
                return plain(*at(next(iter(terms))))
            return pack(_lin(terms, lambda kj: value(*at(kj))))
        if part == 0:
            for p in range(4):
                for i in range(7):
                    yield 4 * i + p, one(i, 0, (2 * p, 2 * p + 1))
        else:
            for u in range(2):
                for i in range(15):
                    yield T_TRI[u] + i, one(i, 2, TRIPLES[u])
            for i in range(7):
                yield T_LAST + i, one(i, 2, (6, 7))
            for j in range(2):
                yield T_TAIL + j, plain(4, 6 + j)

    GROUPS = ((0, 12, T_TRI[0]), (T_TRI[0], T_TRI[1], T_LAST, T_TAIL + 2))
    NGRP = 8 * (len(GROUPS[0]) + len(GROUPS[1]) - 2)

    def put_tiles(dst, slot, r0, part, tiles):
        out = dict(tiles)
        for lo, hi in zip(GROUPS[part], GROUPS[part][1:]):
            dst[slot, lo:hi, pl.ds(r0, 8), :] = jnp.stack([out[i] for i in range(lo, hi)])
            yield

    def chunk_work(item):
        for b in range(8):
            for part in range(2):
                yield from item(part, b)

    def relayout(ci, dst, slot, part, b):
        hi_m = U32(0xFFFF0000)
        t = {k: w_block(ci, 8 * k + b) for k in ((0, 1), (2, 3, 4))[part]}

        def plain(k, h):
            a, c = t[k][0][h // 2], t[k][1][h // 2]
            return (a >> 16) | (c & hi_m) if h % 2 else (a & U32(0xFFFF)) | (c << 16)

        @functools.lru_cache(None)
        def value(k, h):
            w = cols(t[k][0][h // 2], t[k][1][h // 2])
            return pltpu.bitcast(w & hi_m if h % 2 else w << 16, F32)

        def pack(v):
            r = pltpu.bitcast(v.astype(BF16).astype(F32), U32)
            return (r[:, :DH] >> 16) | r[:, DH:]
        yield from put_tiles(dst, slot, scaled(b, 8), part, rhs_tiles(part, plain, value, pack, False))

    def main(_, carry):
        for part in (1, 0):
            def relayout0(b, c, part=part):
                list(relayout(0, wa_sc, 0, part, b))
                return c
            with jax.named_scope("wait_w"):
                for cp in w_copies(0, part=part):
                    cp.wait()
            with jax.named_scope("relayout"):
                jax.lax.fori_loop(0, 8, relayout0, 0, unroll=2 - part)

        def pro_stage(ps_, b):
            n = ps_ * NRB + b
            with jax.named_scope("wait_w"):
                if ps_ == 0:
                    @pl.when(b + 1 < NRB)
                    def _():
                        x_copy(b + 1).wait()

                @pl.when((n >= 2) & (n <= NCH))
                def _():
                    wait_chunk(n - 1)
            cr = jnp.clip(n - 1, 0, NCH - 1)
            dst, slot = (wb_sc, cr) if ps_ == 0 else (wa_sc, cr - (NRB - 2))
            bl = jnp.minimum(b + 1, NRB - 1)
            PW = PRO_PW
            npc = RB * S2 // PW
            assert npc * PW == RB * S2 and 2 * NRB > UL

            def body(i, c):
                s0 = b * RB + 1
                for sg in range(RB):
                    hp_sc[sg * S2:(sg + 1) * S2, :] = xn_sc[s0 + sg]
                spread(chunk_work(functools.partial(relayout, cr, dst, slot)), dst, jnp.minimum(never_sm[0], 0), NGRP, *PRO_T)
                for pi in range(npc):
                    carry = {}
                    for u in range(3):
                        pos = 3 * pi + u
                        hx = hp_sc[pi * PW:(pi + 1) * PW, :]
                        for k in range(max(RB, 2 * NT)):
                            if PRO_X0 + k * PRO_XN // PRO_XD != pos:
                                continue
                            if ps_ == 0 and k < RB:
                                sn = bl * RB + 1 + k
                                xv = _ext(_ln(x_sc[seg(sn), LN].astype(F32)))
                                xn_sc[sn] = xv
                                hx = rows(hx[:-S2], jnp.where(never_sm[0] > 0, xv, hx[-S2:]))
                            if ps_ == 1 and k < 2 * NT:
                                conv_u(jnp.minimum(2 * b + k // NT, UL),
                                       slice((k % NT) * 128, (k % NT + 1) * 128))
                        for h, r in unit(w_tiles(ps_, (0,)), u, packed_lhs(hx), carry).items():
                            for a in range(0, 2 * PW, 16):
                                sg, off = divmod(2 * pi * PW + a, SEG)
                                pre_sc[s0 + sg, ps_ * HG + h, off:off + 16, :] = r[a:a + 16].astype(BF16)
                assert not queue
                return c
            assert PRO_X0 + (max(RB, 2 * NT) - 1) * PRO_XN // PRO_XD < 3 * npc
            with jax.named_scope("fused"):
                jax.lax.fori_loop(0, never_sm[0] + 1, body, 0)

        for ps_ in range(NPASS):
            if ps_ == 1:
                with jax.named_scope("wait_in0"):
                    for cp in small + in_copies(0):
                        cp.wait()
                sh = sh_ref[...].astype(F32)
                for j in range(KS):
                    co_sc[j] = jnp.broadcast_to(sh[j:j + 1], (8, DM))
                co_sc[KS] = jnp.broadcast_to(sd_ref[...].astype(F32).reshape(1, DM), (8, DM))

            def blk(b, c, ps_=ps_):
                pro_stage(ps_, b)
                return c
            jax.lax.fori_loop(0, NRB, blk, 0)

        def warm_block0(q):
            uf, kf = conv_fwd(0, q)
            put_spec(0, q, 0, uf)
            put_spec(0, q, 2, kf)
            kr_sc[q] = kf
            ur, um, kr, km = uf[:QB], uf[QB:], kf[:QB], kf[QB:]
            wf_sc[0, 0, q] = (ur * kr - um * km).astype(BF16)
            wf_sc[0, 1, q] = (ur * km + um * kr).astype(BF16)

        def wo_operands(g, part, b):
            def src(k, h):
                r = (g * HG + h) * DH + 16 * b
                return wo_sc[r:r + 16, k * 128:(k + 1) * 128]
            tiles = rhs_tiles(part, lambda k, h: _pack(src(k, h)),
                              functools.lru_cache(None)(lambda k, h: src(k, h).astype(F32)), _pack, True)
            yield from put_tiles(wc_sc, g, 8 * b, part, tiles)

        def wo_work():
            for g in range(NG):
                yield from chunk_work(functools.partial(wo_operands, g))

        def plain_qkv(eq, ekv, k, carry):
            g, u = divmod(k, 3)
            res = []
            for mats, e in (((1,), ekv), ((2,), ekv), ((0,), eq)):
                res.append(unit(w_tiles(g, mats), u, e, carry.setdefault(mats, {})))
            return {h: bf(res[2][h], res[0][h], res[1][h]) for h in res[0]}

        with jax.named_scope("wait_wo"):
            wo_copy.wait()
        with jax.named_scope("step0"):
            mem0 = mem0_ref[...].astype(F32)
            e0 = packed_lhs(rows(_ext(rows(mem0, mem0)), xn(0)))

            carry0 = {}
            spread(wo_work(), wc_sc, jnp.minimum(never_sm[0], 0), NG * NGRP, *WO_T)

            def hook0(it):
                if it < NQ:
                    warm_block0(it)
                if 5 <= it < 5 + NT:
                    for p in range(2):
                        conv_inv(p, it - 5)
            out = attend(lambda k: plain_qkv(e0, e0, k, carry0), RH, make_mask(RH, (0,)), hook0, True)
            y0 = y_seg(0)
            for q in range(2):
                conv_spec(1, q)
            for n in range(NT):
                conv_inv(2, n)
            finish(0, x_sc[0:SEG, LN], y0, rows(out[0:M], mem0), out[M2:])
            for q in range(2):
                for piece in MAC_PIECES:
                    conv_mac(1, q, piece, 2)

        mask12 = make_mask(R, (0, 1))

        def step(t, x2):
            c, q = (t + 1) // NQ + 1, (t + 1) % NQ
            mem = h_sc[...]
            n1 = _unpack(xn(t)[:, 0:DM]).astype(F32)
            lead = value_lhs(mem, (n1, None))[0]
            ahead = {ui: product(w_tiles(0, (1, 2)), ui[0], lead, ui[1]) for ui in AHEAD}
            if x2 is None:
                x2 = x2_sc[(t - 1) & 3]
            conv_spec(c, q)
            link = []
            for piece in MAC_PIECES:
                conv_mac(c, q, piece, NB, link)
            n2 = _ln(x2)
            x4 = side2(t, op_sc[...])
            un = conv_u(t + UL)
            left = staged(lambda p: value_lhs(mem, (n1, n2), p), [(PIN_U, un, 2), (PIN_X4, x4, NT)])
            left_q = value_lhs(rows(mem, n2))
            carry = {}

            def proj(k):
                g, u = divmod(k, 3)
                pre = g * HG < NPA
                if pre:
                    qs = unit(w_tiles(g, (0,)), u, left_q, carry.setdefault("q", {}))
                rs = unit(w_tiles(g, (1, 2) if pre else (1, 2, 0)), u, left(k), carry.setdefault("kv", {}),
                          ahead if g == 0 else ())
                res = {}
                for h, r in rs.items():
                    if pre:
                        qq = rows(qs[h][:M2], pre_sc[t, g * HG + h].astype(F32), qs[h][M2:])
                    else:
                        qq = r[:, 2 * DH:]
                    res[h] = bf(qq, r[:, :DH], r[:, DH:2 * DH])
                return res

            held = {}

            def hook(it):
                if INV_AT <= it < INV_AT + NT:
                    conv_inv(t + 2, it - INV_AT)
                if it == NU:
                    held["x"] = x_sc[seg(t), LN]
                    held["y"] = y_seg(t)
            out = attend(proj, R, mask12, hook)
            op_sc[...] = out[RH:]
            return finish(t, held["x"], held["y"], out[0:M2], out[M2:RH])

        def steps(i, carry):
            x2 = None
            for j in range(UNROLL):
                x2 = step(1 + i * UNROLL + j, x2)
            return carry

        def phase(p, carry):
            @pl.when(p == 1)
            def _():
                for cp in in_copies(2):
                    cp.wait()

            @pl.when(p >= 2)
            def _():
                out_copy((p - 2) * PH, PH).start()

            with jax.named_scope("steps"):
                jax.lax.fori_loop(p * PHI, (p + 1) * PHI, steps, 0)
            return carry

        for cp in in_copies(1):
            cp.wait()
        jax.lax.fori_loop(0, NPH, phase, 0)
        out_copy((NPH - 2) * PH, NSEG - 2 - (NPH - 2) * PH).start()

        with jax.named_scope("step_last"):
            x4 = side2(NSEG, op_sc[...])
            n2 = _ln(x2_sc[(NSEG - 1) & 3])
            left_q = value_lhs(n2)
            left = staged(lambda p: value_lhs(rows(h_sc[...], n2), None, p), [(PIN_X4, x4, NT)])
            carry1 = {}
            out = attend(lambda k: plain_qkv(left_q, left(k), k, carry1),
                         SEG, make_mask(RH, (1,), M2))
            side2(NSEG + 1, out)
        out_copy(NSEG - 2, 2).start()
        out_copy(0, NSEG).wait()
        return carry

    jax.lax.fori_loop(0, never_sm[0] + 1, main, 0)


def pallas_interleave_layers__memory_aug_recurrent_mem_tr__ssm_conv_h3__prompt_kernel(
    A_x, A_mem0, A_Wq, A_Wk, A_Wv, A_Wo, A_seg_len,
    B_q, B_k, B_v, B_shift_k, B_ssm_k, B_ssm_D,
):
    del B_q
    seg = int(A_seg_len) if isinstance(A_seg_len, (int, np.integer)) else CB // NQ
    return _run(A_x, A_mem0, A_Wq, A_Wk, A_Wv, A_Wo, B_k, B_v, B_shift_k, B_ssm_k, B_ssm_D, SEG=seg)


@functools.partial(jax.jit, static_argnames=("SEG",))
def _run(A_x, A_mem0, A_Wq, A_Wk, A_Wv, A_Wo, B_k, B_v, B_shift_k, B_ssm_k, B_ssm_D, *, SEG):
    B, S, DM = A_x.shape
    assert B == 1
    H, DH = A_Wq.shape[1], A_Wq.shape[2]
    M = A_mem0.shape[1]
    KS = B_shift_k.shape[1]
    R = 2 * (M + SEG)
    NSEG = S // SEG
    NRB = (NSEG - 1) // RB
    NB = S // CB
    QB = CB // NQ
    NCH = 3 * H // HG
    DP = -(-DM // 256) * 256
    fwd, inv = _dft_constants()

    kern = functools.partial(_kernel, S=S, DM=DM, H=H, DH=DH, M=M, SEG=SEG)
    any_spec = pl.BlockSpec(memory_space=pl.ANY)
    out = pl.pallas_call(
        kern,
        out_shape=jax.ShapeDtypeStruct((S, DM), A_x.dtype),
        in_specs=[any_spec] * 13,
        out_specs=any_spec,
        scratch_shapes=[
            pltpu.VMEM((NB + 2, NQ, QB // 8, DM // 128, 4, 8, 128), F32),
            pltpu.VMEM((NQ, 2 * QB, DM), F32),
            pltpu.VMEM((2, 2, NQ, QB, DM), BF16),
            pltpu.VMEM((4, SEG, DM), F32),
            pltpu.VMEM((2 * CB, DP), F32),
            pltpu.VMEM((S, DP), BF16),
            pltpu.VMEM((SEG, DM), F32),
            pltpu.VMEM((NSEG, NPA, SEG, DH), BF16),
            pltpu.VMEM((NSEG, SEG // 2, DM + 384), U32),
            pltpu.VMEM((NCH - NRB + 2, N_TILES, 64, DH), U32),
            pltpu.VMEM((NRB - 1, N_TILES, 64, DH), U32),
            pltpu.VMEM((H * DH, DM), BF16),
            pltpu.VMEM((H // HG, N_TILES, 64, DH), U32),
            pltpu.VMEM((S, DP), BF16),
            pltpu.VMEM((S, DP), BF16),
            pltpu.VMEM((NB, DM, CB), BF16),
            pltpu.VMEM((NCH, DM // 16, 8, 2 * HG, DH), BF16),
            pltpu.VMEM((S, DP), A_x.dtype),
            pltpu.VMEM(fwd.shape, BF16),
            pltpu.VMEM(inv.shape, BF16),
            pltpu.VMEM((S + KPAD, DP), BF16),
            pltpu.VMEM((RB * SEG // 2, DM + 384), U32),
            pltpu.VMEM((2 * M, DM), F32),
            pltpu.VMEM((KS + 1, 8, DM), F32),
            pltpu.VMEM((M, DM), BF16),
            pltpu.VMEM((KS, DM), BF16),
            pltpu.VMEM((DM,), BF16),
            pltpu.SMEM((1,), jnp.int32),
            pltpu.SemaphoreType.DMA(((NSEG - 1) // RB,)),
            pltpu.SemaphoreType.DMA((3,)),
            pltpu.SemaphoreType.DMA((NCH + 2,)),
            pltpu.SemaphoreType.DMA(()),
        ],
        compiler_params=pltpu.CompilerParams(vmem_limit_bytes=120 * 1024 * 1024),
    )(
        A_x.reshape(S, DM), A_mem0.reshape(M, DM),
        *[w.reshape(DM // 16, 2, 8, H, DH) for w in (A_Wq, A_Wk, A_Wv)],
        A_Wo.reshape(H * DH, DM), B_k.reshape(S, DM), B_v.reshape(S, DM),
        B_shift_k.T, B_ssm_k, B_ssm_D,
        jnp.asarray(fwd, BF16), jnp.asarray(inv, BF16),
    )
    return out.reshape(B, S, DM)
```
